```python
import jax
import jax.numpy as jnp

def _softmax(x, axis=-1):
    return jax.nn.softmax(x, axis=axis)

def _gelu(x):
    return jax.nn.gelu(x, approximate=True)

def _silu(x):
    return jax.nn.silu(x)

def _sigmoid(x):
    return jax.nn.sigmoid(x)

def _layernorm(x, axis=-1, eps=1e-05):
    m = jnp.mean(x, axis=axis, keepdims=True)
    v = jnp.var(x, axis=axis, keepdims=True)
    return (x - m) / jnp.sqrt(v + eps)

def _scatter_add(tgt, idx, src, axis=0):
    return tgt.at[idx].add(src)

def _segment_sum(src, seg, n):
    return jax.ops.segment_sum(src, seg, n)

class _Rng:

    def __init__(self, key):
        self._k = key

    def _next(self):
        self._k, sub = jax.random.split(self._k)
        return sub

    def normal(self, shape):
        return jax.random.normal(self._next(), shape, dtype=jnp.bfloat16)

    def randint(self, lo, hi, shape):
        return jax.random.randint(self._next(), shape, lo, hi, dtype=jnp.int32)

    def uniform(self, shape, lo=0.0, hi=1.0):
        return jax.random.uniform(self._next(), shape, jnp.bfloat16, lo, hi)

    def permutation(self, n):
        return jax.random.permutation(self._next(), n)
kernel_name = 'parallel_sum__memory_aug_infini_attn__moe_arch_mod__prompt'

def setup_inputs():
    _rng = _Rng(jax.random.key(int.from_bytes(__import__("os").urandom(4), "little")))
    _w = lambda a: (lambda t: t.astype(jnp.bfloat16) if jnp.issubdtype(t.dtype, jnp.floating) else t)(jnp.asarray(a))

    def _A_setup():
        B, S, D, H = (1, 2048, 576, 32)
        N = 4
        L = max(1, S // N)
        sc = D ** (-0.5)
        return {'x': _w((lambda *s: _rng.normal(s) * 0.05)(B, N * L, D)), 'wq': _w((lambda *s: _rng.normal(s) * 0.05)(D, D) * sc), 'wk': _w((lambda *s: _rng.normal(s) * 0.05)(D, D) * sc), 'wv': _w((lambda *s: _rng.normal(s) * 0.05)(D, D) * sc), 'wo': _w((lambda *s: _rng.normal(s) * 0.05)(D, D) * sc), 'beta': _w((lambda *s: _rng.normal(s) * 0.05)(H))}
    _A_in = _A_setup()

    def _B_setup():
        B, S, D, F, C = (1, 2048, 576, 4608, 2)
        return {'x': _w((lambda *s: _rng.normal(s) * 0.05)(B, S, D)), 'w_r': _w((lambda *s: _rng.normal(s) * 0.05)(D)), 'w_gate': _w((lambda *s: _rng.normal(s) * 0.05)(D, F)), 'w_up': _w((lambda *s: _rng.normal(s) * 0.05)(D, F)), 'w_down': _w((lambda *s: _rng.normal(s) * 0.05)(F, D))}
    _B_in = _B_setup()
    return {'A_x': _A_in['x'], 'A_wq': _A_in['wq'], 'A_wk': _A_in['wk'], 'A_wv': _A_in['wv'], 'A_wo': _A_in['wo'], 'A_beta': _A_in['beta'], 'B_x': _B_in['x'], 'B_w_r': _B_in['w_r'], 'B_w_gate': _B_in['w_gate'], 'B_w_up': _B_in['w_up'], 'B_w_down': _B_in['w_down']}

def reference(A_x, A_wq, A_wk, A_wv, A_wo, A_beta, B_x, B_w_r, B_w_gate, B_w_up, B_w_down):

    def _A_ref(x, wq, wk, wv, wo, beta):
        B, S, D = x.shape
        H = 32
        Dh = D // H
        N = 4
        L = S // N
        q = (lambda x, *d: x.transpose(*d))((x @ wq).reshape(B, S, H, Dh), 0, 2, 1, 3).reshape(B, H, N, L, Dh)
        k = (lambda x, *d: x.transpose(*d))((x @ wk).reshape(B, S, H, Dh), 0, 2, 1, 3).reshape(B, H, N, L, Dh)
        v = (lambda x, *d: x.transpose(*d))((x @ wv).reshape(B, S, H, Dh), 0, 2, 1, 3).reshape(B, H, N, L, Dh)
        phi = lambda t: jnp.where(t > 0, t + 1.0, jnp.exp(t))
        scale = Dh ** (-0.5)
        ar = jnp.arange(L)
        mask = (lambda x, dt: x.astype(dt))(ar[:, None] < ar[None, :], x.dtype) * -1000000000.0
        g = _sigmoid(beta).reshape(1, H, 1, 1)
        M = jnp.einsum('bhd,bhe->bhde', q[:, :, 0, 0, :] * 0.0, q[:, :, 0, 0, :] * 0.0)
        z = q[:, :, 0, 0, :] * 0.0
        outs = []
        for s in range(N):
            qs, ks, vs = (q[:, :, s].copy(), k[:, :, s].copy(), v[:, :, s].copy())
            logits = jnp.einsum('bhqd,bhkd->bhqk', qs, ks) * scale + mask
            p = _softmax(logits, axis=-1)
            a_dot = jnp.einsum('bhqk,bhkd->bhqd', p, vs)
            pq = phi(qs)
            num = jnp.einsum('bhld,bhde->bhle', pq, M)
            den = jnp.einsum('bhld,bhd->bhl', pq, z)[..., None] + 1e-06
            a_mem = num / den
            o = g * a_mem + (1.0 - g) * a_dot
            outs.append(o)
            pk = phi(ks)
            M = M + jnp.einsum('bhld,bhle->bhde', pk, vs)
            z = z + jnp.einsum('bhld->bhd', pk)
        o = (lambda x, *d: x.transpose(*d))(jnp.stack(outs, 2).reshape(B, H, S, Dh), 0, 2, 1, 3).reshape(B, S, D)
        return o @ wo

    def _B_ref(x, w_r, w_gate, w_up, w_down):
        B, S, D = x.shape
        C = 2
        r = x @ w_r
        idx = jnp.argsort(-r, axis=-1)[:, :C]
        idx_e = jnp.repeat(idx.reshape(B, C, 1), D, axis=2)
        x_sel = jnp.take_along_axis(x, idx_e, axis=1)
        g = _silu(x_sel @ w_gate)
        u = x_sel @ w_up
        y = g * u @ w_down
        r_sel = _sigmoid(jnp.take_along_axis(r, idx, axis=1))
        y = y * r_sel.reshape(B, C, 1)
        b_off = (jnp.arange(B) * S).reshape(B, 1)
        flat_idx = (idx + b_off).reshape(B * C)
        zero = (x * 0.0).reshape(B * S, D)
        upd = _scatter_add(zero, flat_idx, y.reshape(B * C, D), axis=0)
        return x + upd.reshape(B, S, D)
    x = A_x
    xn = _layernorm(x, axis=-1)
    return x + _A_ref(xn, A_wq, A_wk, A_wv, A_wo, A_beta) + _B_ref(xn, B_w_r, B_w_gate, B_w_up, B_w_down)
```

```python
import functools

import jax
import jax.numpy as jnp
from jax import lax
from jax.experimental import pallas as pl
from jax.experimental.pallas import tpu as pltpu

bf16 = jnp.bfloat16
f32 = jnp.float32
u32 = jnp.uint32
i32 = jnp.int32

SEQ = 2048
D = 576
DP = 640
H = 32
DH = 18
NSEG = 4
L = 512
T = 128
HPG = 7
NG = 5
GW = HPG * DH
F = 4608
NH = 8
NUNIT = NSEG * H // NH
UPS = H // NH

LOG2E = 1.4426950408889634
QSCALE = (DH ** -0.5) * LOG2E
MASKVAL = -1000000000.0 * LOG2E
EPS_BF16 = 1.0013580322265625e-05
ONES_PAIR = 0x3F803F80

NT_DIMS = (((1,), (1,)), ((), ()))

SEM_X = 0
SEM_W = 4
SEM_MOE = 8
SEM_OUT = 11
NSEM = 15


def _bf(x):
    return pltpu.bitcast(x, bf16)


def _pack(x):
    return pltpu.bitcast(x.astype(bf16), u32)


def _round_bf16(x):
    return x.astype(bf16).astype(f32)


def _phi(t):
    return jnp.where(t > 0, t + 1.0, jnp.exp(t))


def _sigmoid(t):
    return 1.0 / (1.0 + jnp.exp(-t))


def _group_columns(w_u, g):
    rows = w_u.shape[0]
    lane = lax.broadcasted_iota(i32, (rows, T), 1)
    if g == 0:
        cols = w_u[:, 0:T]
    else:
        hi = w_u[:, g * T:(g + 1) * T] if g < NG - 1 else jnp.concatenate(
            [w_u[:, g * T:D], jnp.zeros((rows, (g + 1) * T - D), u32)], axis=1)
        lo = w_u[:, (g - 1) * T:g * T]
        cols = jnp.where(lane < 2 * g, pltpu.roll(lo, 2 * g, 1), pltpu.roll(hi, 2 * g, 1))
    return jnp.where(lane < GW, cols, u32(0))


def _kernel(x_hbm, wq_hbm, wk_hbm, wv_hbm, wo_hbm, beta_ref, wr_ref, wg_hbm, wu_hbm, wd_hbm,
            out_hbm,
            x_buf, w_buf, wg_buf, wu_buf, wd_buf, out_buf,
            wqk_u, wvt_u, wo_u, xn_u, qs_u, k_u, pq_u, pk_u, vt_u,
            r_buf, mt_acc, lm_u, am, g16, omg, mb,
            s0, m0, s1, m1, ot, y_buf, idx_smem, sems):

    def x_copy(s):
        return pltpu.make_async_copy(x_hbm.at[pl.ds(s * L, L)], x_buf.at[pl.ds(s * L, L)], sems.at[SEM_X + s])

    def w_copy(i):
        src = (wq_hbm, wk_hbm, wv_hbm, wo_hbm)[i]
        return pltpu.make_async_copy(src, w_buf.at[i], sems.at[SEM_W + i])

    def moe_copy(i):
        src = (wg_hbm, wu_hbm, wd_hbm)[i]
        dst = (wg_buf, wu_buf, wd_buf)[i]
        return pltpu.make_async_copy(src, dst, sems.at[SEM_MOE + i])

    def out_copy(s):
        return pltpu.make_async_copy(out_buf.at[pl.ds(s * L, L)], out_hbm.at[pl.ds(s * L, L)], sems.at[SEM_OUT + s])

    x_copy(0).start()
    for i in range(3):
        w_copy(i).start()
    for s in range(1, NSEG):
        x_copy(s).start()
    w_copy(3).start()
    for i in range(3):
        moe_copy(i).start()

    ki = lax.broadcasted_iota(i32, (T, T), 0)
    qi = lax.broadcasted_iota(i32, (T, T), 1)
    mb[...] = jnp.where(qi < ki, MASKVAL, 0.0).astype(f32)
    xn_u[:, D:DP] = jnp.zeros((SEQ // 2, DP - D), u32)
    ot[...] = jnp.zeros(ot.shape, f32)
    am[0] = jnp.zeros(am.shape[1:], f32)
    mt_acc[...] = jnp.zeros(mt_acc.shape, f32)
    g16[...] = jnp.zeros(g16.shape, f32)

    gate = _round_bf16(_sigmoid(beta_ref[...].astype(f32)))
    for h in range(H):
        gh = jnp.broadcast_to(gate[:, h:h + 1], (1, T))
        omg[h] = jnp.broadcast_to(_round_bf16(1.0 - gh), (8, T))
        g16[h // HPG, (h % HPG):(h % HPG) + 1, :] = gh

    def prep_cols(i):
        return pltpu.bitcast(w_buf[i], u32)

    zrows = jnp.zeros(((DP - D) // 2, T), u32)
    for i in range(2):
        w_copy(i).wait()
        w_u = prep_cols(i)
        for g in range(NG):
            c0 = (i * NG + g) * T
            wqk_u[0:D // 2, c0:c0 + T] = _group_columns(w_u, g)
            wqk_u[D // 2:DP // 2, c0:c0 + T] = zrows

    w_copy(2).wait()
    w_u = prep_cols(2)
    wr_row = wr_ref[...].astype(f32)
    wr_pad = jnp.concatenate([wr_row, jnp.zeros((1, DP - D), f32)], axis=1)
    for g in range(NG):
        cols = _bf(_group_columns(w_u, g))
        cols = jnp.concatenate([cols, jnp.zeros((DP - D, T), bf16)], axis=0)
        rows = cols.T.astype(f32)
        if g == 0:
            rid = lax.broadcasted_iota(i32, (T, DP), 0)
            rows = jnp.where(rid == GW, wr_pad, rows)
        wvt_u[g * (T // 2):(g + 1) * (T // 2), :] = _pack(rows)

    w_copy(3).wait()
    w_u = prep_cols(3)
    for g in range(NG):
        nrow = (GW if g < NG - 1 else D - (NG - 1) * GW) // 2
        blk = w_u[g * (GW // 2):g * (GW // 2) + nrow, :]
        wo_u[g * (T // 2):g * (T // 2) + nrow, :] = blk
        wo_u[g * (T // 2) + nrow:(g + 1) * (T // 2), :] = jnp.zeros((T // 2 - nrow, D), u32)

    def layernorm(s):
        RB = 64
        for b in range(L // RB):
            r0 = pl.multiple_of(s * L + b * RB, RB)
            x = x_buf[pl.ds(r0, RB), :].astype(f32)
            mean = jnp.sum(x, axis=-1, keepdims=True) / D
            xc32 = x - mean
            var = jnp.sum(xc32 * xc32, axis=-1, keepdims=True) / D
            den = _round_bf16(jnp.sqrt(_round_bf16(_round_bf16(var) + EPS_BF16)))
            xc = _round_bf16(x - _round_bf16(mean))
            xn = xc * (1.0 / den)
            xn_u[pl.ds(pl.multiple_of(r0 // 2, RB // 2), RB // 2), 0:D] = _pack(xn)

    def project(s):
        xs = _bf(xn_u[pl.ds(pl.multiple_of(s * (L // 2), L // 2), L // 2), :])
        for g in range(NG):
            q = jnp.dot(xs, _bf(wqk_u[:, g * T:(g + 1) * T]), preferred_element_type=f32)
            qs_u[s * NG + g] = _pack(q * QSCALE)
            pq_u[s * NG + g] = _pack(_phi(_round_bf16(q)))
            k = jnp.dot(xs, _bf(wqk_u[:, (NG + g) * T:(NG + g + 1) * T]), preferred_element_type=f32)
            k_u[s * NG + g] = _pack(k)
            pk_u[s * NG + g] = _pack(_phi(_round_bf16(k)))
        rid = lax.broadcasted_iota(i32, (T, L), 0)
        for g in range(NG):
            vt = lax.dot_general(_bf(wvt_u[g * (T // 2):(g + 1) * (T // 2), :]), xs, NT_DIMS,
                                 preferred_element_type=f32)
            if g == 0:
                r_buf[s] = jnp.broadcast_to(vt[GW:GW + 1, :], (8, L))
            vt = jnp.where(rid == T - 1, 1.0, vt)
            vt_u[s, g * (T // 2):(g + 1) * (T // 2), :] = _pack(vt)

    def seg_body(s, c):
        for ss in range(NSEG):
            @pl.when(s == ss)
            def _():
                x_copy(ss).wait()
        layernorm(s)
        project(s)
        return c

    lax.fori_loop(0, NSEG, seg_body, 0)

    e_id = lax.broadcasted_iota(i32, (T, T), 0)
    d_id = lax.broadcasted_iota(i32, (T, T), 1)
    same_head = ((e_id // DH) == (d_id // DH)) & (e_id < GW) & (d_id < GW)
    j16 = lax.broadcasted_iota(i32, (16, T), 0)
    d16 = lax.broadcasted_iota(i32, (16, T), 1)
    z_mask = ((d16 // DH) == j16) & (d16 < GW)

    def mem_body(s, c):
        for g in range(NG):
            upd = jnp.dot(_bf(vt_u[s, g * (T // 2):(g + 1) * (T // 2), :]), _bf(pk_u[s * NG + g]),
                          preferred_element_type=f32)
            mt = mt_acc[g] + upd
            mt_acc[g] = mt
            lhs = jnp.concatenate(
                [jnp.where(same_head, mt, 0.0),
                 jnp.where(z_mask, jnp.broadcast_to(mt[T - 1:T, :], (16, T)), 0.0)], axis=0)
            nd = lax.dot_general(lhs.astype(bf16), _bf(pq_u[(s + 1) * NG + g]), NT_DIMS,
                                 preferred_element_type=f32)
            scale = jnp.broadcast_to(g16[g][:, 0:1], (16, L)) / (nd[T:T + 16, :] + 1e-6)
            r8 = lax.broadcasted_iota(i32, (8, L), 0)
            for b in range(T // 8):
                j1 = min((8 * b) // DH, HPG - 1)
                j2 = min((8 * b + 7) // DH, HPG - 1)
                sc = jnp.broadcast_to(scale[j1:j1 + 1, :], (8, L))
                if j2 != j1:
                    sc = jnp.where(r8 < DH * j2 - 8 * b, sc, jnp.broadcast_to(scale[j2:j2 + 1, :], (8, L)))
                am[s + 1, g * T + 8 * b:g * T + 8 * b + 8, :] = nd[8 * b:8 * b + 8, :] * sc
        return c

    lax.fori_loop(0, NSEG - 1, mem_body, 0)

    rr = jnp.concatenate([r_buf[s][0:1, :] for s in range(NSEG)], axis=0)
    rr = _round_bf16(rr)
    tok = lax.broadcasted_iota(i32, (NSEG, L), 0) * L + lax.broadcasted_iota(i32, (NSEG, L), 1)
    m1v = jnp.max(rr)
    i1 = jnp.min(jnp.where(rr == m1v, tok, SEQ))
    rr2 = jnp.where(tok == i1, -jnp.inf, rr)
    m2v = jnp.max(rr2)
    i2 = jnp.min(jnp.where(rr2 == m2v, tok, SEQ))
    i1 = jnp.clip(i1, 0, SEQ - 1)
    i2 = jnp.clip(i2, 0, SEQ - 1)
    idx_smem[0] = i1
    idx_smem[1] = i2

    def token_row(i):
        blk = xn_u[pl.ds(pl.multiple_of((i // 16) * 8, 8), 8), :]
        sub = lax.broadcasted_iota(i32, (8, DP), 0)
        word = jnp.sum(jnp.where(sub == (i % 16) // 2, pltpu.bitcast(blk, i32), 0), axis=0, keepdims=True)
        bits = jnp.where(i % 2 == 1, word & jnp.int32(-65536), word << 16)
        return pltpu.bitcast(bits, f32)

    row16 = lax.broadcasted_iota(i32, (16, DP), 0)
    xsel = jnp.where(row16 == 0, token_row(i1), jnp.where(row16 == 1, token_row(i2), 0.0))
    xsel = xsel[:, 0:D].astype(bf16)

    moe_copy(0).wait()
    moe_copy(1).wait()
    gt = _round_bf16(jnp.dot(xsel, wg_buf[...], preferred_element_type=f32))
    up = _round_bf16(jnp.dot(xsel, wu_buf[...], preferred_element_type=f32))
    act = _round_bf16(gt * _sigmoid(gt))
    hid = (act * up).astype(bf16)
    moe_copy(2).wait()
    y = _round_bf16(jnp.dot(hid, wd_buf[...], preferred_element_type=f32))
    rsel = jnp.where(lax.broadcasted_iota(i32, (16, 1), 0) == 0, m1v, m2v)
    y_buf[...] = _round_bf16(y * _round_bf16(_sigmoid(rsel)))

    lane64 = lax.broadcasted_iota(i32, (T // 2, T), 1)
    row32 = lax.broadcasted_iota(i32, (32, T), 0)

    def stage_a(unit, u, qt, s_ref, m_ref):
        s = unit // UPS
        h = (unit % UPS) * NH + u
        g = h // HPG
        j = h - HPG * g
        sg = s * NG + g
        msk = (lane64 >= DH * j) & (lane64 < DH * j + DH)
        w = _bf(jnp.where(msk, qs_u[sg, qt * (T // 2):(qt + 1) * (T // 2), :], u32(0)))
        ms = []
        for c in range(qt + 1):
            kc = _bf(k_u[sg, c * (T // 2):(c + 1) * (T // 2), :])
            sc = lax.dot_general(kc, w, NT_DIMS, preferred_element_type=f32)
            if c == qt:
                sc = sc + mb[...]
            s_ref[u, qt, c * T:(c + 1) * T, :] = sc
            ms.append(jnp.max(sc, axis=0, keepdims=True))
        m = ms[0]
        for mm in ms[1:]:
            m = jnp.maximum(m, mm)
        m_ref[u, qt] = jnp.broadcast_to(m, (8, T))

    def stage_b(unit, u, qt, s_ref, m_ref):
        s = unit // UPS
        h = (unit % UPS) * NH + u
        g = h // HPG
        j = h - HPG * g
        n = T * (qt + 1)
        p = jnp.exp2(s_ref[u, qt, 0:n, :] - m_ref[u, qt][0:1]).astype(bf16)
        vw = vt_u[s, pl.ds(pl.multiple_of(g * (T // 2) + 8 * j, 8), 16), 0:n]
        sub = lax.broadcasted_iota(i32, (16, n), 0)
        vw = jnp.where(sub == 15, u32(ONES_PAIR), vw)
        o = jnp.dot(_bf(vw), p, preferred_element_type=f32)
        r1 = pl.multiple_of(g * T + 16 * j, 16)
        cs = omg[h][0:1] / o[31:32]
        res = am[s, pl.ds(r1, 32), qt * T:(qt + 1) * T] + o * cs
        msk = (row32 >= 2 * j) & (row32 < 2 * j + DH)
        pltpu.store(ot.at[pl.ds(r1, 32), qt * T:(qt + 1) * T], res, mask=msk)

    def out_proj(s):
        o_nat = ot[...].astype(bf16).T
        attn = jnp.dot(o_nat, _bf(wo_u[...]), preferred_element_type=f32)
        r0 = pl.multiple_of(s * L, L)
        xn = _bf(xn_u[pl.ds(pl.multiple_of(s * (L // 2), L // 2), L // 2), 0:D]).astype(f32)
        x = x_buf[pl.ds(r0, L), :].astype(f32)
        out_buf[pl.ds(r0, L), :] = (x + attn + xn).astype(bf16)
        for t in range(2):
            it = idx_smem[t]

            @pl.when(it // L == s)
            def _():
                b0 = pl.multiple_of((it // 16) * 16, 16)
                blk = out_buf[pl.ds(b0, 16), :].astype(f32)
                rid = lax.broadcasted_iota(i32, (16, D), 0)
                add = jnp.where(rid == it % 16, y_buf[t:t + 1, :], 0.0)
                out_buf[pl.ds(b0, 16), :] = (blk + add).astype(bf16)
        for ss in range(NSEG):
            @pl.when(s == ss)
            def _():
                out_copy(ss).start()

    def pair(ua, sa, ma, ub, sb, mbuf):
        for u in range(NH):
            for qt in range(4):
                if ua is not None:
                    stage_a(ua, u, qt, sa, ma)
                if ub is not None:
                    stage_b(ub, u, qt, sb, mbuf)

    pair(0, s0, m0, None, None, None)

    def att_body(i, c):
        u0 = 2 * i
        pair(u0 + 1, s1, m1, u0, s0, m0)
        pair(u0 + 2, s0, m0, u0 + 1, s1, m1)

        @pl.when((u0 + 2) % UPS == 0)
        def _():
            out_proj(u0 // UPS)
        return c

    lax.fori_loop(0, NUNIT // 2 - 1, att_body, 0)
    pair(NUNIT - 1, s1, m1, NUNIT - 2, s0, m0)
    pair(None, None, None, NUNIT - 1, s1, m1)
    out_proj(NSEG - 1)

    for s in range(NSEG):
        out_copy(s).wait()


@jax.jit
def pallas_parallel_sum__memory_aug_infini_attn__moe_arch_mod__prompt_kernel(
    A_x: jax.Array,
    A_wq: jax.Array,
    A_wk: jax.Array,
    A_wv: jax.Array,
    A_wo: jax.Array,
    A_beta: jax.Array,
    B_x: jax.Array,
    B_w_r: jax.Array,
    B_w_gate: jax.Array,
    B_w_up: jax.Array,
    B_w_down: jax.Array,
):
    del B_x
    any_spec = pl.BlockSpec(memory_space=pl.ANY)
    vmem_spec = pl.BlockSpec(memory_space=pltpu.VMEM)
    scratch = [
        pltpu.VMEM((SEQ, D), bf16),
        pltpu.VMEM((4, D, D), bf16),
        pltpu.VMEM((D, F), bf16),
        pltpu.VMEM((D, F), bf16),
        pltpu.VMEM((F, D), bf16),
        pltpu.VMEM((SEQ, D), bf16),
        pltpu.VMEM((DP // 2, 2 * DP), u32),
        pltpu.VMEM((DP // 2, DP), u32),
        pltpu.VMEM((DP // 2, D), u32),
        pltpu.VMEM((SEQ // 2, DP), u32),
        pltpu.VMEM((NSEG * NG, L // 2, T), u32),
        pltpu.VMEM((NSEG * NG, L // 2, T), u32),
        pltpu.VMEM((NSEG * NG, L // 2, T), u32),
        pltpu.VMEM((NSEG * NG, L // 2, T), u32),
        pltpu.VMEM((NSEG, DP // 2, L), u32),
        pltpu.VMEM((NSEG, 8, L), f32),
        pltpu.VMEM((NG, T, T), f32),
        pltpu.VMEM((8, T), u32),
        pltpu.VMEM((NSEG, DP, L), f32),
        pltpu.VMEM((NG, 16, T), f32),
        pltpu.VMEM((H, 8, T), f32),
        pltpu.VMEM((T, T), f32),
        pltpu.VMEM((NH, 4, L, T), f32),
        pltpu.VMEM((NH, 4, 8, T), f32),
        pltpu.VMEM((NH, 4, L, T), f32),
        pltpu.VMEM((NH, 4, 8, T), f32),
        pltpu.VMEM((DP, L), f32),
        pltpu.VMEM((16, D), f32),
        pltpu.SMEM((2,), i32),
        pltpu.SemaphoreType.DMA((NSEM,)),
    ]
    out = pl.pallas_call(
        _kernel,
        out_shape=jax.ShapeDtypeStruct((SEQ, D), bf16),
        in_specs=[any_spec, any_spec, any_spec, any_spec, any_spec, vmem_spec, vmem_spec,
                  any_spec, any_spec, any_spec],
        out_specs=any_spec,
        scratch_shapes=scratch,
        compiler_params=pltpu.CompilerParams(vmem_limit_bytes=110 * 1024 * 1024),
    )(A_x.reshape(SEQ, D), A_wq, A_wk, A_wv, A_wo, A_beta.reshape(1, H), B_w_r.reshape(1, D),
      B_w_gate, B_w_up, B_w_down)
    return out.reshape(1, SEQ, D)
```

```python
import jax
import jax.numpy as jnp
from jax import lax
from jax.experimental import pallas as pl
from jax.experimental.pallas import tpu as pltpu

bf16 = jnp.bfloat16
f32 = jnp.float32
u32 = jnp.uint32
i32 = jnp.int32

SEQ = 2048
D = 576
DP = 640
H = 32
DH = 18
NSEG = 4
L = 512
T = 128
TW = T // 2
HPG = 7
NG = 5
GW = HPG * DH
F = 4608
NH = 8
NUNIT = NSEG * H // NH
UPS = H // NH
NT = SEQ // T

LOG2E = 1.4426950408889634
QSCALE = (DH ** -0.5) * LOG2E
MASKVAL = -1000000000.0 * LOG2E
EPS_BF16 = 1.0013580322265625e-05
ONES_PAIR = 0x3F803F80

NT_DIMS = (((1,), (1,)), ((), ()))

SEM_X = 0
SEM_W = 4
SEM_MOE = 8
SEM_OUT = 11
NSEM = 15


def _bf(x):
    return pltpu.bitcast(x, bf16)


def _pack(x):
    return pltpu.bitcast(x.astype(bf16), u32)


def _round_bf16(x):
    return x.astype(bf16).astype(f32)


def _phi(t):
    return jnp.where(t > 0, t + 1.0, jnp.exp(t))


def _sigmoid(t):
    return 1.0 / (1.0 + jnp.exp(-t))


def _group_columns(w_u, g):
    rows = w_u.shape[0]
    lane = lax.broadcasted_iota(i32, (rows, T), 1)
    if g == 0:
        cols = w_u[:, 0:T]
    else:
        hi = w_u[:, g * T:(g + 1) * T] if g < NG - 1 else jnp.concatenate(
            [w_u[:, g * T:D], jnp.zeros((rows, (g + 1) * T - D), u32)], axis=1)
        lo = w_u[:, (g - 1) * T:g * T]
        cols = jnp.where(lane < 2 * g, pltpu.roll(lo, 2 * g, 1), pltpu.roll(hi, 2 * g, 1))
    return jnp.where(lane < GW, cols, u32(0))


def _kernel(x_hbm, wq_hbm, wk_hbm, wv_hbm, wo_hbm, beta_ref, wr_ref, wg_hbm, wu_hbm, wd_hbm,
            out_hbm,
            x_buf, w_buf, wg_buf, wu_buf, wd_buf, out_buf,
            wt_u, wot_u, xn_u, qs_u, k_u, pq_u, pk_u, vt_u,
            r_buf, mt_acc, am, g16, omg, mb,
            s0, m0, s1, m1, ot, ycol, sel_buf, sems):

    def x_copy(s):
        return pltpu.make_async_copy(x_hbm.at[:, pl.ds(s * L, L)], x_buf.at[:, pl.ds(s * L, L)],
                                     sems.at[SEM_X + s])

    def w_copy(i):
        src = (wq_hbm, wk_hbm, wv_hbm, wo_hbm)[i]
        return pltpu.make_async_copy(src, w_buf.at[i], sems.at[SEM_W + i])

    def moe_copy(i):
        src = (wg_hbm, wu_hbm, wd_hbm)[i]
        dst = (wg_buf, wu_buf, wd_buf)[i]
        return pltpu.make_async_copy(src, dst, sems.at[SEM_MOE + i])

    def out_copy(s):
        return pltpu.make_async_copy(out_buf.at[:, pl.ds(s * L, L)], out_hbm.at[:, pl.ds(s * L, L)],
                                     sems.at[SEM_OUT + s])

    for i in range(3):
        w_copy(i).start()
    for s in range(NSEG):
        x_copy(s).start()
    w_copy(3).start()
    for i in range(3):
        moe_copy(i).start()

    ki = lax.broadcasted_iota(i32, (T, T), 0)
    qi = lax.broadcasted_iota(i32, (T, T), 1)
    mb[...] = jnp.where(qi < ki, MASKVAL, 0.0).astype(f32)
    xn_u[:, D // 2:DP // 2, :] = jnp.zeros((NT, (DP - D) // 2, T), u32)
    ot[...] = jnp.zeros(ot.shape, f32)
    am[0] = jnp.zeros(am.shape[1:], f32)
    mt_acc[...] = jnp.zeros(mt_acc.shape, f32)
    g16[...] = jnp.zeros(g16.shape, f32)

    gate = _round_bf16(_sigmoid(beta_ref[...].astype(f32)))
    for h in range(H):
        gh = jnp.broadcast_to(gate[:, h:h + 1], (1, T))
        omg[h] = jnp.broadcast_to(_round_bf16(1.0 - gh), (8, T))
        g16[h // HPG, (h % HPG):(h % HPG) + 1, :] = gh

    wr_row = wr_ref[...].astype(f32)
    wr_pad = jnp.concatenate([wr_row, jnp.zeros((1, DP - D), f32)], axis=1)
    for i in range(3):
        w_copy(i).wait()
        w_u = pltpu.bitcast(w_buf[i], u32)
        for g in range(NG):
            cols = _bf(_group_columns(w_u, g))
            cols = jnp.concatenate([cols, jnp.zeros((DP - D, T), bf16)], axis=0)
            rows = cols.T
            if i == 2 and g == 0:
                rid = lax.broadcasted_iota(i32, (T, DP), 0)
                rows = jnp.where(rid == GW, wr_pad, rows.astype(f32)).astype(bf16)
            wt_u[(i * NG + g) * TW:(i * NG + g + 1) * TW, :] = pltpu.bitcast(rows, u32)

    def layernorm(s):
        for tt in range(L // T):
            c0 = pl.multiple_of(s * L + tt * T, T)
            x = x_buf[:, pl.ds(c0, T)].astype(f32)
            mean = jnp.sum(x, axis=0, keepdims=True) / D
            xc32 = x - mean
            var = jnp.sum(xc32 * xc32, axis=0, keepdims=True) / D
            den = _round_bf16(jnp.sqrt(_round_bf16(_round_bf16(var) + EPS_BF16)))
            xc = _round_bf16(x - _round_bf16(mean))
            xn_u[s * (L // T) + tt, 0:D // 2, :] = _pack(xc * (1.0 / den))

    def project(s):
        xs = jnp.concatenate([_bf(xn_u[s * (L // T) + tt]) for tt in range(L // T)], axis=1)
        rid = lax.broadcasted_iota(i32, (T, L), 0)
        for g in range(NG):
            def wrows(i):
                return _bf(wt_u[(i * NG + g) * TW:(i * NG + g + 1) * TW, :])
            q = jnp.dot(wrows(0), xs, preferred_element_type=f32)
            qs_u[s * NG + g] = _pack(q * QSCALE)
            pq_u[s * NG + g] = _pack(_phi(_round_bf16(q)))
            k = jnp.dot(wrows(1), xs, preferred_element_type=f32).astype(bf16)
            k_u[s * NG + g] = pltpu.bitcast(k.T, u32)
            pk_u[s * NG + g] = _pack(_phi(k.astype(f32)))
            vt = jnp.dot(wrows(2), xs, preferred_element_type=f32)
            if g == 0:
                r_buf[s] = jnp.broadcast_to(vt[GW:GW + 1, :], (8, L))
            vt = jnp.where(rid == T - 1, 1.0, vt)
            vt_u[s, g * TW:(g + 1) * TW, :] = _pack(vt)

    def seg_body(s, c):
        for ss in range(NSEG):
            @pl.when(s == ss)
            def _():
                x_copy(ss).wait()
        layernorm(s)
        project(s)
        return c

    lax.fori_loop(0, NSEG, seg_body, 0)

    w_copy(3).wait()
    wo = jnp.concatenate([w_buf[3], jnp.zeros((DP - D, D), bf16)], axis=0)
    wo = jnp.concatenate([wo, jnp.zeros((DP, DP - D), bf16)], axis=1)
    wo_t = pltpu.bitcast(wo.T, u32)[0:D // 2, 0:D]
    for g in range(NG):
        wot_u[:, g * T:(g + 1) * T] = _group_columns(wo_t, g)

    e_id = lax.broadcasted_iota(i32, (T, T), 0)
    d_id = lax.broadcasted_iota(i32, (T, T), 1)
    same_head = ((e_id // DH) == (d_id // DH)) & (e_id < GW) & (d_id < GW)
    j16 = lax.broadcasted_iota(i32, (16, T), 0)
    d16 = lax.broadcasted_iota(i32, (16, T), 1)
    z_mask = ((d16 // DH) == j16) & (d16 < GW)

    def mem_body(s, c):
        for g in range(NG):
            upd = lax.dot_general(_bf(vt_u[s, g * TW:(g + 1) * TW, :]), _bf(pk_u[s * NG + g]), NT_DIMS,
                                  preferred_element_type=f32)
            mt = mt_acc[g] + upd
            mt_acc[g] = mt
            lhs = jnp.concatenate(
                [jnp.where(same_head, mt, 0.0),
                 jnp.where(z_mask, jnp.broadcast_to(mt[T - 1:T, :], (16, T)), 0.0)], axis=0)
            nd = jnp.dot(lhs.astype(bf16), _bf(pq_u[(s + 1) * NG + g]),
                         preferred_element_type=f32)
            scale = jnp.broadcast_to(g16[g][:, 0:1], (16, L)) / (nd[T:T + 16, :] + 1e-6)
            r8 = lax.broadcasted_iota(i32, (8, L), 0)
            for b in range(T // 8):
                j1 = min((8 * b) // DH, HPG - 1)
                j2 = min((8 * b + 7) // DH, HPG - 1)
                sc = jnp.broadcast_to(scale[j1:j1 + 1, :], (8, L))
                if j2 != j1:
                    sc = jnp.where(r8 < DH * j2 - 8 * b, sc, jnp.broadcast_to(scale[j2:j2 + 1, :], (8, L)))
                am[s + 1, g * T + 8 * b:g * T + 8 * b + 8, :] = nd[8 * b:8 * b + 8, :] * sc
        return c

    lax.fori_loop(0, NSEG - 1, mem_body, 0)

    rr = jnp.concatenate([r_buf[s][0:1, :] for s in range(NSEG)], axis=0)
    rr = _round_bf16(rr)
    tok = lax.broadcasted_iota(i32, (NSEG, L), 0) * L + lax.broadcasted_iota(i32, (NSEG, L), 1)
    m1v = jnp.max(rr)
    i1 = jnp.min(jnp.where(rr == m1v, tok, SEQ))
    rr2 = jnp.where(tok == i1, -jnp.inf, rr)
    m2v = jnp.max(rr2)
    i2 = jnp.min(jnp.where(rr2 == m2v, tok, SEQ))
    i1 = jnp.clip(i1, 0, SEQ - 1)
    i2 = jnp.clip(i2, 0, SEQ - 1)

    row16 = lax.broadcasted_iota(i32, (16, T), 0)
    lane16 = lax.broadcasted_iota(i32, (16, T), 1)

    def token_rows(i, slot):
        onehot = jnp.where((row16 == slot) & (lane16 == i % T), 1.0, 0.0).astype(bf16)
        return lax.dot_general(onehot, _bf(xn_u[i // T]), NT_DIMS, preferred_element_type=f32)

    xsel = (token_rows(i1, 0) + token_rows(i2, 1))[:, 0:D].astype(bf16)

    moe_copy(0).wait()
    moe_copy(1).wait()
    gt = _round_bf16(jnp.dot(xsel, wg_buf[...], preferred_element_type=f32))
    up = _round_bf16(jnp.dot(xsel, wu_buf[...], preferred_element_type=f32))
    act = _round_bf16(gt * _sigmoid(gt))
    hid = (act * up).astype(bf16)
    moe_copy(2).wait()
    y = _round_bf16(lax.dot_general(hid, wd_buf[...], NT_DIMS, preferred_element_type=f32))
    rsel = jnp.where(lax.broadcasted_iota(i32, (16, 1), 0) == 0, m1v, m2v)
    y = _round_bf16(y * _round_bf16(_sigmoid(rsel)))
    y = jnp.concatenate([y, jnp.zeros((16, DP - D), f32)], axis=1)
    y = jnp.concatenate([y, jnp.zeros((T - 16, DP), f32)], axis=0)
    y_t = y.T
    for t in range(2):
        ycol[t] = jnp.broadcast_to(y_t[0:D, t:t + 1], (D, T))
    tok_l = lax.broadcasted_iota(i32, (8, SEQ), 1)
    sel_buf[0] = jnp.where(tok_l == i1, 1.0, 0.0)
    sel_buf[1] = jnp.where(tok_l == i2, 1.0, 0.0)

    row64 = lax.broadcasted_iota(i32, (TW, T), 0)
    row32 = lax.broadcasted_iota(i32, (32, T), 0)

    def stage_a(unit, u, qt, s_ref, m_ref):
        s = unit // UPS
        h = (unit % UPS) * NH + u
        g = h // HPG
        j = h - HPG * g
        sg = s * NG + g
        msk = (row64 >= (DH // 2) * j) & (row64 < (DH // 2) * (j + 1))
        w = _bf(jnp.where(msk, qs_u[sg, :, qt * T:(qt + 1) * T], u32(0)))
        ms = []
        for c in range(qt + 1):
            kc = _bf(k_u[sg, c * TW:(c + 1) * TW, :])
            sc = jnp.dot(kc, w, preferred_element_type=f32)
            if c == qt:
                sc = sc + mb[...]
            s_ref[u, qt, c * T:(c + 1) * T, :] = sc
            ms.append(jnp.max(sc, axis=0, keepdims=True))
        m = ms[0]
        for mm in ms[1:]:
            m = jnp.maximum(m, mm)
        m_ref[u, qt] = jnp.broadcast_to(m, (8, T))

    def stage_b(unit, u, qt, s_ref, m_ref):
        s = unit // UPS
        h = (unit % UPS) * NH + u
        g = h // HPG
        j = h - HPG * g
        n = T * (qt + 1)
        p = jnp.exp2(s_ref[u, qt, 0:n, :] - m_ref[u, qt][0:1]).astype(bf16)
        vw = vt_u[s, pl.ds(pl.multiple_of(g * TW + 8 * j, 8), 16), 0:n]
        sub = lax.broadcasted_iota(i32, (16, n), 0)
        vw = jnp.where(sub == 15, u32(ONES_PAIR), vw)
        o = jnp.dot(_bf(vw), p, preferred_element_type=f32)
        r1 = pl.multiple_of(g * T + 16 * j, 16)
        cs = omg[h][0:1] / o[31:32]
        res = am[s, pl.ds(r1, 32), qt * T:(qt + 1) * T] + o * cs
        msk = (row32 >= 2 * j) & (row32 < 2 * j + DH)
        pltpu.store(ot.at[pl.ds(r1, 32), qt * T:(qt + 1) * T], res, mask=msk)

    def out_proj(s):
        attn = jnp.dot(_bf(wot_u[...]), ot[...].astype(bf16), preferred_element_type=f32)
        for tt in range(L // T):
            c0 = pl.multiple_of(s * L + tt * T, T)
            xn = _bf(xn_u[s * (L // T) + tt, 0:D // 2, :]).astype(f32)
            x = x_buf[:, pl.ds(c0, T)].astype(f32)
            res = x + attn[:, tt * T:(tt + 1) * T] + xn
            for t in range(2):
                hit = sel_buf[t, 0:1, pl.ds(c0, T)] > 0.5
                res = res + jnp.where(hit, ycol[t], 0.0)
            out_buf[:, pl.ds(c0, T)] = res.astype(bf16)
        for ss in range(NSEG):
            @pl.when(s == ss)
            def _():
                out_copy(ss).start()

    def pair(ua, sa, ma, ub, sb, mbuf):
        for u in range(NH):
            for qt in range(4):
                if ua is not None:
                    stage_a(ua, u, qt, sa, ma)
                if ub is not None:
                    stage_b(ub, u, qt, sb, mbuf)

    pair(0, s0, m0, None, None, None)

    def att_body(i, c):
        u0 = 2 * i
        pair(u0 + 1, s1, m1, u0, s0, m0)
        pair(u0 + 2, s0, m0, u0 + 1, s1, m1)

        @pl.when((u0 + 2) % UPS == 0)
        def _():
            out_proj(u0 // UPS)
        return c

    lax.fori_loop(0, NUNIT // 2 - 1, att_body, 0)
    pair(NUNIT - 1, s1, m1, NUNIT - 2, s0, m0)
    pair(None, None, None, NUNIT - 1, s1, m1)
    out_proj(NSEG - 1)

    for s in range(NSEG):
        out_copy(s).wait()


@jax.jit
def pallas_parallel_sum__memory_aug_infini_attn__moe_arch_mod__prompt_kernel(
    A_x: jax.Array,
    A_wq: jax.Array,
    A_wk: jax.Array,
    A_wv: jax.Array,
    A_wo: jax.Array,
    A_beta: jax.Array,
    B_x: jax.Array,
    B_w_r: jax.Array,
    B_w_gate: jax.Array,
    B_w_up: jax.Array,
    B_w_down: jax.Array,
):
    del B_x
    any_spec = pl.BlockSpec(memory_space=pl.ANY)
    vmem_spec = pl.BlockSpec(memory_space=pltpu.VMEM)
    scratch = [
        pltpu.VMEM((D, SEQ), bf16),
        pltpu.VMEM((4, D, D), bf16),
        pltpu.VMEM((D, F), bf16),
        pltpu.VMEM((D, F), bf16),
        pltpu.VMEM((D, F), bf16),
        pltpu.VMEM((D, SEQ), bf16),
        pltpu.VMEM((3 * NG * TW, DP), u32),
        pltpu.VMEM((D // 2, DP), u32),
        pltpu.VMEM((NT, DP // 2, T), u32),
        pltpu.VMEM((NSEG * NG, TW, L), u32),
        pltpu.VMEM((NSEG * NG, L // 2, T), u32),
        pltpu.VMEM((NSEG * NG, TW, L), u32),
        pltpu.VMEM((NSEG * NG, TW, L), u32),
        pltpu.VMEM((NSEG, DP // 2, L), u32),
        pltpu.VMEM((NSEG, 8, L), f32),
        pltpu.VMEM((NG, T, T), f32),
        pltpu.VMEM((NSEG, DP, L), f32),
        pltpu.VMEM((NG, 16, T), f32),
        pltpu.VMEM((H, 8, T), f32),
        pltpu.VMEM((T, T), f32),
        pltpu.VMEM((NH, 4, L, T), f32),
        pltpu.VMEM((NH, 4, 8, T), f32),
        pltpu.VMEM((NH, 4, L, T), f32),
        pltpu.VMEM((NH, 4, 8, T), f32),
        pltpu.VMEM((DP, L), f32),
        pltpu.VMEM((2, D, T), f32),
        pltpu.VMEM((2, 8, SEQ), f32),
        pltpu.SemaphoreType.DMA((NSEM,)),
    ]
    x_t = jnp.transpose(A_x, (0, 2, 1)).reshape(D, SEQ)
    out_t = pl.pallas_call(
        _kernel,
        out_shape=jax.ShapeDtypeStruct((D, SEQ), bf16),
        in_specs=[any_spec, any_spec, any_spec, any_spec, any_spec, vmem_spec, vmem_spec,
                  any_spec, any_spec, any_spec],
        out_specs=any_spec,
        scratch_shapes=scratch,
        compiler_params=pltpu.CompilerParams(vmem_limit_bytes=110 * 1024 * 1024),
    )(x_t, A_wq, A_wk, A_wv, A_wo, A_beta.reshape(1, H), B_w_r.reshape(1, D),
      B_w_gate, B_w_up, B_w_down.T)
    return jnp.transpose(out_t.reshape(1, D, SEQ), (0, 2, 1))
```

```python
import contextlib

import jax
import jax.numpy as jnp
from jax import lax
from jax.experimental import pallas as pl
from jax.experimental.pallas import tpu as pltpu

bf16 = jnp.bfloat16
f32 = jnp.float32
u32 = jnp.uint32
i32 = jnp.int32

SEQ = 2048
D = 576
DP = 640
H = 32
DH = 18
NSEG = 4
L = 512
T = 128
TW = T // 2
HT = T // 2
TPS = L // T
HPG = 6
NG = 6
F = 4608
FC = 512
NP = 4
UPS = H // (2 * NP)
NUNIT = NSEG * UPS
NT = SEQ // T
LNW = 256
VB = 8 * DH

LOG2E = 1.4426950408889634
QSCALE = (DH ** -0.5) * LOG2E
MASKVAL = -1000000000.0 * LOG2E
EPS_BF16 = 1.0013580322265625e-05
ONES_PAIR = 0x3F803F80

NT_DIMS = (((1,), (1,)), ((), ()))

WT_Q = 0
WT_K = NG * TW
WT_V = 2 * NG * TW
WT_ROWS = WT_V + D // 2

SEM_X = 0
SEM_W = 4
SEM_MOE = 8
SEM_OUT = 11
NSEM = 18


PROFILE_SCOPES = False


def _scope(name):
    return jax.named_scope(name) if PROFILE_SCOPES else contextlib.nullcontext()


def _valid(g):
    return min(HPG * DH, D - g * HPG * DH)


def _rows(g):
    return -(-_valid(g) // 16) * 16


def _ewin(g):
    start = (g * HPG * DH // 16) * 16
    return start, g * HPG * DH - start, min(T, D - start)


def _bf(x):
    return pltpu.bitcast(x, bf16)


def _pack(x):
    return pltpu.bitcast(x.astype(bf16), u32)


def _round_bf16(x):
    return x.astype(bf16).astype(f32)


def _phi(t):
    return jnp.where(t > 0, t + 1.0, jnp.exp(t))


def _sigmoid(t):
    return 1.0 / (1.0 + jnp.exp(-t))


def _interleave(*lists):
    items = []
    for li, tasks in enumerate(lists):
        for k, t in enumerate(tasks):
            items.append(((k + 0.5) / len(tasks), li, k, t))
    items.sort(key=lambda it: it[:3])
    return [it[3] for it in items]


def _kernel(x_hbm, wq_hbm, wk_hbm, wv_hbm, wo_hbm, beta_ref, wr_ref, wg_hbm, wu_hbm, wd_hbm,
            out_hbm,
            x_buf, w_buf, wg_buf, wu_buf, wd_buf, out_buf,
            wt_u, wtd_u, wot_u, xn_u, xs_cur, xs_nxt, qs_u, k_u, pq_u, pk_u, vt_u, vwin,
            r_buf, mt_acc, am, g16, omg, mb, rowmask, smask,
            s0, m0, s1, m1, ot, y_acc, xsel_buf, ycol, sel_buf, sems):

    def x_copy(s):
        return pltpu.make_async_copy(x_hbm.at[:, pl.ds(s * L, L)], x_buf.at[:, pl.ds(s * L, L)],
                                     sems.at[SEM_X + s])

    def w_copy(i):
        src = (wq_hbm, wk_hbm, wv_hbm, wo_hbm)[i]
        return pltpu.make_async_copy(src, w_buf.at[i], sems.at[SEM_W + i])

    def moe_copy(i):
        src = (wg_hbm, wu_hbm, wd_hbm)[i]
        dst = (wg_buf, wu_buf, wd_buf)[i]
        return pltpu.make_async_copy(src, dst, sems.at[SEM_MOE + i])

    def out_copy(c0, width, sem):
        return pltpu.make_async_copy(out_buf.at[:, pl.ds(c0, width)], out_hbm.at[:, pl.ds(c0, width)],
                                     sems.at[SEM_OUT + sem])

    x_copy(0).start()
    w_copy(0).start()

    init_scope = _scope("init")
    init_scope.__enter__()
    kr = lax.broadcasted_iota(i32, (HT, T), 0)
    ql = lax.broadcasted_iota(i32, (HT, T), 1)
    mb[0] = jnp.where(ql < kr, MASKVAL, 0.0).astype(f32)
    mb[1] = jnp.where((ql >= HT) & (ql - HT < kr), MASKVAL, 0.0).astype(f32)
    mb[2] = jnp.where(ql % HT < kr, MASKVAL, 0.0).astype(f32)
    for j in range(HPG):
        rowmask[j] = jnp.where((kr >= (DH // 2) * j) & (kr < (DH // 2) * (j + 1)), u32(0xFFFFFFFF), u32(0))
    r32 = lax.broadcasted_iota(i32, (32, T), 0)
    for i in range(8):
        smask[i] = jnp.where((r32 >= 2 * i) & (r32 < 2 * i + DH), 1, 0)
    zpad = jnp.zeros(((DP - D) // 2, T), u32)
    for tt in range(TPS):
        xs_cur[tt, D // 2:DP // 2, :] = zpad
        xs_nxt[tt, D // 2:DP // 2, :] = zpad
    for tt in range(NT):
        xn_u[tt, D // 2:DP // 2, :] = zpad
    ot[D:DP, :] = jnp.zeros((DP - D, L), f32)
    am[0] = jnp.zeros(am.shape[1:], f32)
    mt_acc[...] = jnp.zeros(mt_acc.shape, f32)
    g16[...] = jnp.zeros(g16.shape, f32)
    for sg in range(NSEG * NG):
        r2 = _rows(sg % NG) // 2
        qs_u[sg, r2:TW, :] = jnp.zeros((TW - r2, L), u32)
        pq_u[sg, r2:TW, :] = jnp.zeros((TW - r2, L), u32)
        pk_u[sg, r2:TW, :] = jnp.zeros((TW - r2, L), u32)

    gate = _round_bf16(_sigmoid(beta_ref[...].reshape(1, H).astype(f32)))
    for h in range(H):
        gh = jnp.broadcast_to(gate[:, h:h + 1], (1, T))
        omg[h] = jnp.broadcast_to(_round_bf16(1.0 - gh), (8, T))
        g16[h // HPG, (h % HPG):(h % HPG) + 1, :] = gh

    init_scope.__exit__(None, None, None)

    def transpose_block(i, cb):
        c1 = min((cb + 1) * T, D)
        blk = w_buf[i, :, cb * T:c1]
        if c1 - cb * T < T:
            blk = jnp.concatenate([blk, jnp.zeros((D, T - (c1 - cb * T)), bf16)], axis=1)
        blk = jnp.concatenate([blk, jnp.zeros((DP - D, T), bf16)], axis=0)
        return pltpu.bitcast(blk.T, u32)

    def prep_dense(i, dst, base):
        def task(cb):
            nrow = min(TW, D // 2 - cb * TW)
            dst[base + cb * TW:base + cb * TW + nrow, :] = transpose_block(i, cb)[0:nrow]
        return [lambda cb=cb: task(cb) for cb in range(DP // T)]

    def prep_grouped(i, base):
        def regroup(g):
            nv, nr = _valid(g) // 2, _rows(g) // 2
            src = g * HPG * DH // 2
            wt_u[base + g * TW:base + g * TW + nv, :] = wtd_u[src:src + nv, :]
            pad = jnp.zeros((nr - nv, DP), u32)
            if i == 1 and g == 0:
                wr = wr_ref[...].reshape(1, D).astype(f32)
                wr = jnp.concatenate([wr, jnp.zeros((1, DP - D), f32)], axis=1)
                bits = lax.shift_right_logical(pltpu.bitcast(wr, u32), u32(16))
                rid = lax.broadcasted_iota(i32, (nr - nv, DP), 0)
                pad = jnp.where(rid == 0, bits, pad)
            wt_u[base + g * TW + nv:base + g * TW + nr, :] = pad
        return prep_dense(i, wtd_u, 0) + [lambda g=g: regroup(g) for g in range(NG)]

    def ln_block(c0):
        x = x_buf[:, pl.ds(c0, LNW)].astype(f32)
        mean = jnp.sum(x, axis=0, keepdims=True) / D
        xc32 = x - mean
        var = jnp.sum(xc32 * xc32, axis=0, keepdims=True) / D
        den = _round_bf16(jnp.sqrt(_round_bf16(_round_bf16(var) + EPS_BF16)))
        xc = _round_bf16(x - _round_bf16(mean))
        return _pack(xc * (1.0 / den))

    def ln_tasks(s, dst):
        def task(b):
            c0 = s * L + b * LNW
            if not isinstance(s, int):
                c0 = pl.multiple_of(c0, LNW)
            xn = ln_block(c0)
            for t in range(LNW // T):
                tt = b * (LNW // T) + t
                dst[tt, 0:D // 2, :] = xn[:, t * T:(t + 1) * T]
                xn_u[s * TPS + tt, 0:D // 2, :] = xn[:, t * T:(t + 1) * T]
        return [lambda b=b: task(b) for b in range(L // LNW)]

    def load_xs():
        return jnp.concatenate([_bf(xs_cur[tt]) for tt in range(TPS)], axis=1)

    def q_task(s, g):
        nr = _rows(g) // 2
        w = _bf(wt_u[WT_Q + g * TW:WT_Q + g * TW + nr, :])
        q = jnp.dot(w, load_xs(), preferred_element_type=f32)
        qp = _pack(q * QSCALE)
        qrot = jnp.concatenate([pltpu.roll(qp[:, t * T:(t + 1) * T], HT, 1) for t in range(TPS)], axis=1)
        rid = lax.broadcasted_iota(i32, (nr, L), 0)
        even = ((rid // (DH // 2)) % 2) == 0
        qs_u[s * NG + g, 0:nr, :] = jnp.where(even, qrot, qp)
        pq_u[s * NG + g, 0:nr, :] = _pack(_phi(_round_bf16(q)))

    def k_task(s, g):
        nr = _rows(g)
        w = _bf(wt_u[WT_K + g * TW:WT_K + g * TW + nr // 2, :])
        k = jnp.dot(w, load_xs(), preferred_element_type=f32)
        if g == 0:
            r_buf[s] = jnp.broadcast_to(k[_valid(0):_valid(0) + 1, :], (8, L))
        kp = _pack(k)
        pk_u[s * NG + g, 0:nr // 2, :] = _pack(_phi(_round_bf16(k)))
        kfull = _bf(jnp.concatenate([kp, jnp.zeros(((T - nr) // 2, L), u32)], axis=0))
        k_u[s * NG + g] = pltpu.bitcast(kfull.T, u32)

    def v_task(s, b):
        w = _bf(wt_u[WT_V + b * (VB // 2):WT_V + (b + 1) * (VB // 2), :])
        v = _pack(jnp.dot(w, load_xs(), preferred_element_type=f32))
        vt_u[s, b * (VB // 2):(b + 1) * (VB // 2), :] = v
        sub = lax.broadcasted_iota(i32, (16, L), 0)
        for hh in range(8):
            w8 = (9 * hh) // 8
            ones_row = 0 if 2 * hh == 14 else 15
            vwin[s * H + 8 * b + hh] = jnp.where(sub == ones_row, u32(ONES_PAIR), v[8 * w8:8 * w8 + 16, :])

    def q_tasks(s):
        return [lambda g=g: q_task(s, g) for g in range(NG)]

    def k_tasks(s):
        return [lambda g=g: k_task(s, g) for g in range(NG)]

    def v_tasks(s):
        return [lambda b=b: v_task(s, b) for b in range(D // VB)]

    def advance_xs():
        for tt in range(TPS):
            xs_cur[tt, 0:D // 2, :] = xs_nxt[tt, 0:D // 2, :]

    def run(tasks):
        for t in tasks:
            t()

    with _scope("p1_wait_x0"):
        x_copy(0).wait()
    w_copy(1).start()
    w_copy(2).start()
    with _scope("p1_wait_wq"):
        w_copy(0).wait()
    for s in range(1, NSEG):
        x_copy(s).start()
    w_copy(3).start()
    for i in range(3):
        moe_copy(i).start()
    with _scope("p1_ln0_prep_q"):
        run(_interleave(ln_tasks(0, xs_cur), prep_grouped(0, WT_Q)))
        w_copy(1).wait()
    with _scope("p1_q0"):
        run(_interleave(q_tasks(0), prep_grouped(1, WT_K)))
        w_copy(2).wait()
    with _scope("p1_k0"):
        run(_interleave(k_tasks(0), prep_dense(2, wt_u, WT_V)))
        x_copy(1).wait()
    with _scope("p1_v0"):
        run(_interleave(v_tasks(0), ln_tasks(1, xs_nxt)))
        advance_xs()
        w_copy(3).wait()
    with _scope("p1_prep_o"):
        run(prep_dense(3, wot_u, 0))

    def seg_body(s, c):
        for ss in range(2, NSEG):
            @pl.when(s + 1 == ss)
            def _():
                x_copy(ss).wait()
        nxt = jnp.minimum(s + 1, NSEG - 1)
        with _scope("p1_seg"):
            run(_interleave(q_tasks(s) + k_tasks(s) + v_tasks(s), ln_tasks(nxt, xs_nxt)))
            advance_xs()
        return c

    lax.fori_loop(1, NSEG, seg_body, 0)

    row64 = lax.broadcasted_iota(i32, (TW, T), 0)
    lane64 = lax.broadcasted_iota(i32, (TW, T), 1)
    row32 = lax.broadcasted_iota(i32, (32, T), 0)
    lane32 = lax.broadcasted_iota(i32, (32, T), 1)
    lane1 = lax.broadcasted_iota(i32, (1, T), 1)
    lane8 = lax.broadcasted_iota(i32, (8, T), 1)

    def stage_a(unit, u, qt, s_ref, m_ref):
        s = unit // UPS
        pi = (unit % UPS) * NP + u
        g = pi // (HPG // 2)
        j = 2 * (pi - (HPG // 2) * g)
        sg = s * NG + g
        n = T * (qt + 1)
        qw = qs_u[sg, :, qt * T:(qt + 1) * T]
        w_a = qw & rowmask[j]
        w_b = qw & rowmask[j + 1]
        w_ab = _bf(jnp.where(lane64 < HT, w_a, w_b))

        def colmax8(v):
            return jnp.max(v.reshape(v.shape[0] // 8, 8, T), axis=0)

        maxes = []
        for hd, w in enumerate((_bf(w_a), _bf(w_b))):
            m8 = None
            for c in range(qt):
                kc = _bf(k_u[sg, c * TW:(c + 1) * TW, :])
                sc = jnp.dot(kc, w, preferred_element_type=f32)
                s_ref[u, qt, hd * L + c * T:hd * L + (c + 1) * T, :] = sc
                m8 = colmax8(sc) if m8 is None else jnp.maximum(m8, colmax8(sc))
            kc = _bf(k_u[sg, qt * TW:qt * TW + TW // 2, :])
            sc = jnp.dot(kc, w, preferred_element_type=f32) + mb[1 - hd]
            s_ref[u, qt, hd * L + qt * T:hd * L + qt * T + HT, :] = sc
            m8 = colmax8(sc) if m8 is None else jnp.maximum(m8, colmax8(sc))
            maxes.append(m8)
        kc = _bf(k_u[sg, qt * TW + TW // 2:(qt + 1) * TW, :])
        sc = jnp.dot(kc, w_ab, preferred_element_type=f32) + mb[2]
        s_ref[u, qt, n - HT:n, :] = sc
        mab = colmax8(sc)
        m_a = jnp.where(lane8 < HT, jnp.maximum(maxes[0], mab), maxes[0])
        m_b = jnp.where(lane8 >= HT, jnp.maximum(maxes[1], mab), maxes[1])
        m_ref[u, qt, 0] = jnp.broadcast_to(jnp.max(m_a, axis=0, keepdims=True), (8, T))
        m_ref[u, qt, 1] = jnp.broadcast_to(jnp.max(m_b, axis=0, keepdims=True), (8, T))

    def stage_b(unit, u, qt, s_ref, m_ref):
        s = unit // UPS
        pi = (unit % UPS) * NP + u
        n = T * (qt + 1)
        m_a = m_ref[u, qt, 0][0:1]
        m_b = m_ref[u, qt, 1][0:1]
        p_ab = jnp.exp2(s_ref[u, qt, n - HT:n, :] - jnp.where(lane1 < HT, m_a, m_b))
        for hd, m in enumerate((m_a, m_b)):
            h = 2 * pi + hd
            p = jnp.exp2(s_ref[u, qt, hd * L:hd * L + n - HT, :] - m)
            keep = (lane64 < HT) if hd == 0 else (lane64 >= HT)
            p = jnp.concatenate([p, jnp.where(keep, p_ab, 0.0)], axis=0).astype(bf16)
            w8 = (9 * h) // 8
            off = DH * h - 16 * w8
            o = jnp.dot(_bf(vwin[s * H + h, :, 0:n]), p, preferred_element_type=f32)
            den = jnp.where(off == 14, o[0:1], o[31:32])
            o = o * (omg[h][0:1] / den)
            if hd == 0:
                o = pltpu.roll(o, HT, 1)
            r1 = pl.multiple_of(16 * w8, 16)
            res = am[s, pl.ds(r1, 32), qt * T:(qt + 1) * T] + o
            pltpu.store(ot.at[pl.ds(r1, 32), qt * T:(qt + 1) * T], res, mask=smask[off // 2] != 0)

    def a_tasks(unit, s_ref, m_ref):
        return [lambda u=u, qt=qt: stage_a(unit, u, qt, s_ref, m_ref) for u in range(NP) for qt in range(4)]

    def b_tasks(unit, s_ref, m_ref):
        return [lambda u=u, qt=qt: stage_b(unit, u, qt, s_ref, m_ref) for u in range(NP) for qt in range(4)]

    ones16 = jnp.where(lax.broadcasted_iota(i32, (8, L), 0) == 0, u32(0x3F80), u32(0))

    def mem_task(s, g):
        es, eoff, ne = _ewin(g)
        nv = _valid(g)
        lhs = _bf(jnp.concatenate([vt_u[s, es // 2:(es + ne) // 2, :], ones16], axis=0))
        upd = lax.dot_general(lhs, _bf(pk_u[s * NG + g]), NT_DIMS, preferred_element_type=f32)
        mt = mt_acc[g, 0:ne + 16, :] + upd
        mt_acc[g, 0:ne + 16, :] = mt
        e_loc = lax.broadcasted_iota(i32, (ne, T), 0) - eoff
        d_id = lax.broadcasted_iota(i32, (ne, T), 1)
        same_head = (e_loc >= 0) & (e_loc < nv) & (d_id < nv) & ((e_loc // DH) == (d_id // DH))
        j16 = lax.broadcasted_iota(i32, (16, T), 0)
        d16 = lax.broadcasted_iota(i32, (16, T), 1)
        z_mask = ((d16 // DH) == j16) & (d16 < nv)
        lm = jnp.concatenate(
            [jnp.where(same_head, mt[0:ne], 0.0),
             jnp.where(z_mask, jnp.broadcast_to(mt[ne:ne + 1, :], (16, T)), 0.0)], axis=0)
        nd = jnp.dot(lm.astype(bf16), _bf(pq_u[(s + 1) * NG + g]), preferred_element_type=f32)
        scale = jnp.broadcast_to(g16[g][:, 0:1], (16, L)) / (nd[ne:ne + 16, :] + 1e-6)
        r8 = lax.broadcasted_iota(i32, (8, L), 0)
        for b in range(ne // 8):
            lo, hi = 8 * b - eoff, 8 * b + 7 - eoff
            if hi < 0 or lo >= nv:
                continue
            j1, j2 = max(lo, 0) // DH, min(hi, nv - 1) // DH
            sc = jnp.broadcast_to(scale[j1:j1 + 1, :], (8, L))
            if j2 != j1:
                sc = jnp.where(r8 < DH * j2 - lo, sc, jnp.broadcast_to(scale[j2:j2 + 1, :], (8, L)))
            val = nd[8 * b:8 * b + 8, :] * sc
            dst = am.at[s + 1, es + 8 * b:es + 8 * b + 8, :]
            if lo >= 0 and hi < nv:
                dst[...] = val
            else:
                pltpu.store(dst, val, mask=(r8 + lo >= 0) & (r8 + lo < nv))

    mem_tasks = [lambda s=s, g=g: mem_task(s, g) for s in range(NSEG - 1) for g in range(NG)]

    for i in range(3):
        moe_copy(i).wait()
    rr = jnp.concatenate([r_buf[s][0:1, :] for s in range(NSEG)], axis=0)
    rr = _round_bf16(rr)
    tok = lax.broadcasted_iota(i32, (NSEG, L), 0) * L + lax.broadcasted_iota(i32, (NSEG, L), 1)
    m1v = jnp.max(rr)
    i1 = jnp.min(jnp.where(rr == m1v, tok, SEQ))
    rr2 = jnp.where(tok == i1, -jnp.inf, rr)
    m2v = jnp.max(rr2)
    i2 = jnp.min(jnp.where(rr2 == m2v, tok, SEQ))
    i1 = jnp.clip(i1, 0, SEQ - 1)
    i2 = jnp.clip(i2, 0, SEQ - 1)

    row16 = lax.broadcasted_iota(i32, (16, T), 0)
    lane16 = lax.broadcasted_iota(i32, (16, T), 1)

    def token_rows(i, slot):
        onehot = jnp.where((row16 == slot) & (lane16 == i % T), 1.0, 0.0).astype(bf16)
        return lax.dot_general(onehot, _bf(xn_u[i // T]), NT_DIMS, preferred_element_type=f32)

    def select_task():
        xsel_buf[...] = token_rows(i1, 0) + token_rows(i2, 1)
        y_acc[...] = jnp.zeros(y_acc.shape, f32)

    def moe_task(c):
        xsel = xsel_buf[:, 0:D].astype(bf16)
        cols = slice(c * FC, (c + 1) * FC)
        gt = _round_bf16(jnp.dot(xsel, wg_buf[:, cols], preferred_element_type=f32))
        up = _round_bf16(jnp.dot(xsel, wu_buf[:, cols], preferred_element_type=f32))
        hid = (_round_bf16(gt * _sigmoid(gt)) * up).astype(bf16)
        y_acc[...] += lax.dot_general(hid, wd_buf[:, cols], NT_DIMS, preferred_element_type=f32)

    def moe_finish():
        y = _round_bf16(y_acc[...])
        rsel = jnp.where(lax.broadcasted_iota(i32, (16, 1), 0) == 0, m1v, m2v)
        y = _round_bf16(y * _round_bf16(_sigmoid(rsel)))
        y = jnp.concatenate([y, jnp.zeros((16, DP - D), f32)], axis=1)
        y = jnp.concatenate([y, jnp.zeros((T - 16, DP), f32)], axis=0)
        y_t = y.T
        for t in range(2):
            ycol[t] = jnp.broadcast_to(y_t[0:D, t:t + 1], (D, T))
        tok_l = lax.broadcasted_iota(i32, (8, SEQ), 1)
        sel_buf[0] = jnp.where(tok_l == i1, 1.0, 0.0)
        sel_buf[1] = jnp.where(tok_l == i2, 1.0, 0.0)

    dense = _interleave(mem_tasks, a_tasks(0, s0, m0))
    moe_tasks = [lambda c=c: moe_task(c) for c in range(F // FC)]
    with _scope("p15_mix"):
        run(dense[0:2] + [select_task] + _interleave(dense[2:], moe_tasks))
        moe_finish()

    def out_proj(s, last):
        o_bf = ot[...].astype(bf16)
        w = _bf(wot_u[...])
        for tt in range(TPS):
            c0 = s * L + tt * T
            if not isinstance(s, int):
                c0 = pl.multiple_of(c0, T)
            attn = jnp.dot(w, o_bf[:, tt * T:(tt + 1) * T], preferred_element_type=f32)
            xn = _bf(xn_u[s * TPS + tt, 0:D // 2, :]).astype(f32)
            x = x_buf[:, pl.ds(c0, T)].astype(f32)
            res = x + attn + xn
            for t in range(2):
                hit = sel_buf[t, 0:1, pl.ds(c0, T)] > 0.5
                res = res + jnp.where(hit, ycol[t], 0.0)
            out_buf[:, pl.ds(c0, T)] = res.astype(bf16)
            if last:
                out_copy(c0, T, NSEG - 1 + tt).start()
        if not last:
            for ss in range(NSEG - 1):
                @pl.when(s == ss)
                def _():
                    out_copy(ss * L, L, ss).start()

    def pair(ua, sa, ma, ub, sb, mbuf):
        ta = a_tasks(ua, sa, ma)
        tb = b_tasks(ub, sb, mbuf)
        for x, y in zip(ta, tb):
            x()
            y()

    def att_body(i, c):
        u0 = 2 * i
        with _scope("att_body"):
            pair(u0 + 1, s1, m1, u0, s0, m0)
            pair(u0 + 2, s0, m0, u0 + 1, s1, m1)

        @pl.when((u0 + 2) % UPS == 0)
        def _():
            with _scope("outproj"):
                out_proj(u0 // UPS, False)
        return c

    lax.fori_loop(0, NUNIT // 2 - 1, att_body, 0)
    with _scope("att_tail"):
        pair(NUNIT - 1, s1, m1, NUNIT - 2, s0, m0)
    with _scope("att_lastb"):
        run(b_tasks(NUNIT - 1, s1, m1))
    with _scope("outproj_last"):
        out_proj(NSEG - 1, True)

    with _scope("out_wait"):
        for s in range(NSEG - 1):
            out_copy(s * L, L, s).wait()
        for tt in range(TPS):
            out_copy((NSEG - 1) * L + tt * T, T, NSEG - 1 + tt).wait()


@jax.jit
def pallas_parallel_sum__memory_aug_infini_attn__moe_arch_mod__prompt_kernel(
    A_x: jax.Array,
    A_wq: jax.Array,
    A_wk: jax.Array,
    A_wv: jax.Array,
    A_wo: jax.Array,
    A_beta: jax.Array,
    B_x: jax.Array,
    B_w_r: jax.Array,
    B_w_gate: jax.Array,
    B_w_up: jax.Array,
    B_w_down: jax.Array,
):
    del B_x
    any_spec = pl.BlockSpec(memory_space=pl.ANY)
    vmem_spec = pl.BlockSpec(memory_space=pltpu.VMEM)
    scratch = [
        pltpu.VMEM((D, SEQ), bf16),
        pltpu.VMEM((4, D, D), bf16),
        pltpu.VMEM((D, F), bf16),
        pltpu.VMEM((D, F), bf16),
        pltpu.VMEM((D, F), bf16),
        pltpu.VMEM((D, SEQ), bf16),
        pltpu.VMEM((WT_ROWS, DP), u32),
        pltpu.VMEM((D // 2, DP), u32),
        pltpu.VMEM((D // 2, DP), u32),
        pltpu.VMEM((NT, DP // 2, T), u32),
        pltpu.VMEM((TPS, DP // 2, T), u32),
        pltpu.VMEM((TPS, DP // 2, T), u32),
        pltpu.VMEM((NSEG * NG, TW, L), u32),
        pltpu.VMEM((NSEG * NG, L // 2, T), u32),
        pltpu.VMEM((NSEG * NG, TW, L), u32),
        pltpu.VMEM((NSEG * NG, TW, L), u32),
        pltpu.VMEM((NSEG, D // 2, L), u32),
        pltpu.VMEM((NSEG * H, 16, L), u32),
        pltpu.VMEM((NSEG, 8, L), f32),
        pltpu.VMEM((NG, T + 16, T), f32),
        pltpu.VMEM((NSEG, D, L), f32),
        pltpu.VMEM((NG, 16, T), f32),
        pltpu.VMEM((H, 8, T), f32),
        pltpu.VMEM((3, HT, T), f32),
        pltpu.VMEM((HPG, TW, T), u32),
        pltpu.VMEM((8, 32, T), i32),
        pltpu.VMEM((NP, 4, 2 * L, T), f32),
        pltpu.VMEM((NP, 4, 2, 8, T), f32),
        pltpu.VMEM((NP, 4, 2 * L, T), f32),
        pltpu.VMEM((NP, 4, 2, 8, T), f32),
        pltpu.VMEM((DP, L), f32),
        pltpu.VMEM((16, D), f32),
        pltpu.VMEM((16, DP), f32),
        pltpu.VMEM((2, D, T), f32),
        pltpu.VMEM((2, 8, SEQ), f32),
        pltpu.SemaphoreType.DMA((NSEM,)),
    ]
    x_t = jnp.transpose(A_x, (0, 2, 1)).reshape(D, SEQ)
    out_t = pl.pallas_call(
        _kernel,
        out_shape=jax.ShapeDtypeStruct((D, SEQ), bf16),
        in_specs=[any_spec, any_spec, any_spec, any_spec, any_spec, vmem_spec, vmem_spec,
                  any_spec, any_spec, any_spec],
        out_specs=any_spec,
        scratch_shapes=scratch,
        compiler_params=pltpu.CompilerParams(vmem_limit_bytes=110 * 1024 * 1024),
    )(x_t, A_wq, A_wk, A_wv, A_wo, A_beta, B_w_r, B_w_gate, B_w_up, B_w_down.T)
    return jnp.transpose(out_t.reshape(1, D, SEQ), (0, 2, 1))
```

```python
import contextlib

import jax
import jax.numpy as jnp
from jax import lax
from jax.experimental import pallas as pl
from jax.experimental.pallas import tpu as pltpu

bf16 = jnp.bfloat16
f32 = jnp.float32
u32 = jnp.uint32
i32 = jnp.int32

SEQ = 2048
D = 576
DP = 640
H = 32
DH = 18
NSEG = 4
L = 512
T = 128
TW = T // 2
HT = T // 2
TPS = L // T
HPG = 6
NG = 6
F = 4608
FPI = 5
NFT = F // T
NP = 4
UPS = H // (2 * NP)
NUNIT = NSEG * UPS
NT = SEQ // T
LNW = 256
VB = 8 * DH

LOG2E = 1.4426950408889634
QSCALE = (DH ** -0.5) * LOG2E
MASKVAL = -1000000000.0 * LOG2E
EPS_BF16 = 1.0013580322265625e-05
ONES_PAIR = 0x3F803F80

NT_DIMS = (((1,), (1,)), ((), ()))

WT_Q = 0
WT_K = NG * TW
WT_V = 2 * NG * TW
WT_ROWS = WT_V + D // 2

SEM_X = 0
SEM_W = 4
SEM_MOE = 8
SEM_OUT = 11
SEM_PATCH = SEM_OUT + 7
NSEM = 20


PROFILE_SCOPES = False


def _scope(name):
    return jax.named_scope(name) if PROFILE_SCOPES else contextlib.nullcontext()


def _valid(g):
    return min(HPG * DH, D - g * HPG * DH)


def _rows(g):
    return -(-_valid(g) // 16) * 16


def _ewin(g):
    start = (g * HPG * DH // 16) * 16
    return start, g * HPG * DH - start, min(T, D - start)


def _bf(x):
    return pltpu.bitcast(x, bf16)


def _pack(x):
    return pltpu.bitcast(x.astype(bf16), u32)


def _round_bf16(x):
    return x.astype(bf16).astype(f32)


def _phi(t):
    return jnp.where(t > 0, t + 1.0, jnp.exp(t))


def _sigmoid(t):
    return 1.0 / (1.0 + jnp.exp(-t))


def _interleave(*lists):
    items = []
    for li, tasks in enumerate(lists):
        for k, t in enumerate(tasks):
            items.append(((k + 0.5) / len(tasks), li, k, t))
    items.sort(key=lambda it: it[:3])
    return [it[3] for it in items]


def _kernel(x_hbm, wq_hbm, wk_hbm, wv_hbm, wo_hbm, beta_ref, wr_ref, wg_hbm, wu_hbm, wd_hbm,
            out_hbm,
            x_buf, w_buf, wg_buf, wu_buf, wd_buf, out_buf,
            wt_u, wtd_u, wot_u, xn_u, xs_cur, xs_nxt, qs_u, k_u, pq_u, pk_u, vt_u, vwin,
            r_buf, mt_acc, am, g16, omg, mb, rowmask, smask,
            s0, m0, s1, m1, ot, xf, ln_stat, y_acc, xsel_buf, hid_buf, ycol, sel_buf, sems):

    def x_copy(s):
        return pltpu.make_async_copy(x_hbm.at[:, pl.ds(s * L, L)], x_buf.at[:, pl.ds(s * L, L)],
                                     sems.at[SEM_X + s])

    def w_copy(i):
        src = (wq_hbm, wk_hbm, wv_hbm, wo_hbm)[i]
        return pltpu.make_async_copy(src, w_buf.at[i], sems.at[SEM_W + i])

    def moe_copy(i):
        src = (wg_hbm, wu_hbm, wd_hbm)[i]
        dst = (wg_buf, wu_buf, wd_buf)[i]
        return pltpu.make_async_copy(src, dst, sems.at[SEM_MOE + i])

    def out_copy(c0, width, sem):
        return pltpu.make_async_copy(out_buf.at[:, pl.ds(c0, width)], out_hbm.at[:, pl.ds(c0, width)],
                                     sems.at[SEM_OUT + sem])

    x_copy(0).start()
    w_copy(0).start()

    init_scope = _scope("init")
    init_scope.__enter__()
    kr = lax.broadcasted_iota(i32, (HT, T), 0)
    ql = lax.broadcasted_iota(i32, (HT, T), 1)
    mb[0] = jnp.where(ql < kr, MASKVAL, 0.0).astype(f32)
    mb[1] = jnp.where((ql >= HT) & (ql - HT < kr), MASKVAL, 0.0).astype(f32)
    mb[2] = jnp.where(ql % HT < kr, MASKVAL, 0.0).astype(f32)
    for j in range(HPG):
        rowmask[j] = jnp.where((kr >= (DH // 2) * j) & (kr < (DH // 2) * (j + 1)), u32(0xFFFFFFFF), u32(0))
    r32 = lax.broadcasted_iota(i32, (32, T), 0)
    for i in range(8):
        smask[i] = jnp.where((r32 >= 2 * i) & (r32 < 2 * i + DH), 1, 0)
    zpad = jnp.zeros(((DP - D) // 2, T), u32)
    for tt in range(TPS):
        xs_cur[tt, D // 2:DP // 2, :] = zpad
        xs_nxt[tt, D // 2:DP // 2, :] = zpad
    for tt in range(NT):
        xn_u[tt, D // 2:DP // 2, :] = zpad
    ot[D:DP, :] = jnp.zeros((DP - D, L), f32)
    am[0] = jnp.zeros(am.shape[1:], f32)
    mt_acc[...] = jnp.zeros(mt_acc.shape, f32)
    g16[...] = jnp.zeros(g16.shape, f32)
    for sg in range(NSEG * NG):
        r2 = _rows(sg % NG) // 2
        qs_u[sg, r2:TW, :] = jnp.zeros((TW - r2, L), u32)
        pq_u[sg, r2:TW, :] = jnp.zeros((TW - r2, L), u32)
        pk_u[sg, r2:TW, :] = jnp.zeros((TW - r2, L), u32)

    gate = _round_bf16(_sigmoid(beta_ref[...].reshape(1, H).astype(f32)))
    for h in range(H):
        gh = jnp.broadcast_to(gate[:, h:h + 1], (1, T))
        omg[h] = jnp.broadcast_to(_round_bf16(1.0 - gh), (8, T))
        g16[h // HPG, (h % HPG):(h % HPG) + 1, :] = gh

    init_scope.__exit__(None, None, None)

    def transpose_block(i, cb):
        c1 = min((cb + 1) * T, D)
        blk = w_buf[i, :, cb * T:c1]
        if c1 - cb * T < T:
            blk = jnp.concatenate([blk, jnp.zeros((D, T - (c1 - cb * T)), bf16)], axis=1)
        blk = jnp.concatenate([blk, jnp.zeros((DP - D, T), bf16)], axis=0)
        return pltpu.bitcast(blk.T, u32)

    def prep_dense(i, dst, base):
        def task(cb):
            nrow = min(TW, D // 2 - cb * TW)
            dst[base + cb * TW:base + cb * TW + nrow, :] = transpose_block(i, cb)[0:nrow]
        return [lambda cb=cb: task(cb) for cb in range(DP // T)]

    def prep_grouped(i, base):
        def regroup(g):
            nv, nr = _valid(g) // 2, _rows(g) // 2
            src = g * HPG * DH // 2
            wt_u[base + g * TW:base + g * TW + nv, :] = wtd_u[src:src + nv, :]
            pad = jnp.zeros((nr - nv, DP), u32)
            if i == 1 and g == 0:
                wr = wr_ref[...].reshape(1, D).astype(f32)
                wr = jnp.concatenate([wr, jnp.zeros((1, DP - D), f32)], axis=1)
                bits = lax.shift_right_logical(pltpu.bitcast(wr, u32), u32(16))
                rid = lax.broadcasted_iota(i32, (nr - nv, DP), 0)
                pad = jnp.where(rid == 0, bits, pad)
            wt_u[base + g * TW + nv:base + g * TW + nr, :] = pad
        return prep_dense(i, wtd_u, 0) + [lambda g=g: regroup(g) for g in range(NG)]

    def ln_tasks(s, dst):
        def col0(b):
            c0 = s * L + b * LNW
            return c0 if isinstance(s, int) else pl.multiple_of(c0, LNW)

        def mean_pass(b):
            acc = None
            for r in range(0, D, 64):
                x = x_buf[r:r + 64, pl.ds(col0(b), LNW)].astype(f32)
                xf[b, r:r + 64, :] = x
                part = jnp.sum(x.reshape(8, 8, LNW), axis=0)
                acc = part if acc is None else acc + part
            mean = jnp.sum(acc, axis=0, keepdims=True) / D
            ln_stat[b, 0] = jnp.broadcast_to(mean, (8, LNW))

        def var_pass(b):
            mean = ln_stat[b, 0][0:1]
            acc = None
            for r in range(0, D, 96):
                xc = xf[b, r:r + 96, :] - mean
                part = jnp.sum((xc * xc).reshape(12, 8, LNW), axis=0)
                acc = part if acc is None else acc + part
            var = jnp.sum(acc, axis=0, keepdims=True) / D
            den = _round_bf16(jnp.sqrt(_round_bf16(_round_bf16(var) + EPS_BF16)))
            ln_stat[b, 1] = jnp.broadcast_to(1.0 / den, (8, LNW))
            ln_stat[b, 0] = jnp.broadcast_to(_round_bf16(mean), (8, LNW))

        def norm_pass(b, half):
            mean_b = ln_stat[b, 0][0:1]
            inv = ln_stat[b, 1][0:1]
            for r in range(half * (D // 2), (half + 1) * (D // 2), 48):
                xn = _pack(_round_bf16(xf[b, r:r + 48, :] - mean_b) * inv)
                for t in range(LNW // T):
                    tt = b * (LNW // T) + t
                    dst[tt, r // 2:r // 2 + 24, :] = xn[:, t * T:(t + 1) * T]
                    xn_u[s * TPS + tt, r // 2:r // 2 + 24, :] = xn[:, t * T:(t + 1) * T]

        tasks = []
        for b in range(L // LNW):
            tasks += [lambda b=b: mean_pass(b), lambda b=b: var_pass(b),
                      lambda b=b: norm_pass(b, 0), lambda b=b: norm_pass(b, 1)]
        return tasks

    def load_xs():
        return jnp.concatenate([_bf(xs_cur[tt]) for tt in range(TPS)], axis=1)

    def q_task(s, g):
        nr = _rows(g) // 2
        w = _bf(wt_u[WT_Q + g * TW:WT_Q + g * TW + nr, :])
        q = jnp.dot(w, load_xs(), preferred_element_type=f32)
        qp = _pack(q * QSCALE)
        qrot = jnp.concatenate([pltpu.roll(qp[:, t * T:(t + 1) * T], HT, 1) for t in range(TPS)], axis=1)
        rid = lax.broadcasted_iota(i32, (nr, L), 0)
        even = ((rid // (DH // 2)) % 2) == 0
        qs_u[s * NG + g, 0:nr, :] = jnp.where(even, qrot, qp)
        pq_u[s * NG + g, 0:nr, :] = _pack(_phi(_round_bf16(q)))

    def k_task(s, g):
        nr = _rows(g)
        w = _bf(wt_u[WT_K + g * TW:WT_K + g * TW + nr // 2, :])
        k = jnp.dot(w, load_xs(), preferred_element_type=f32)
        if g == 0:
            r_buf[s] = jnp.broadcast_to(k[_valid(0):_valid(0) + 1, :], (8, L))
        kp = _pack(k)
        pk_u[s * NG + g, 0:nr // 2, :] = _pack(_phi(_round_bf16(k)))
        kfull = _bf(jnp.concatenate([kp, jnp.zeros(((T - nr) // 2, L), u32)], axis=0))
        k_u[s * NG + g] = pltpu.bitcast(kfull.T, u32)

    def v_task(s, b):
        w = _bf(wt_u[WT_V + b * (VB // 2):WT_V + (b + 1) * (VB // 2), :])
        v = _pack(jnp.dot(w, load_xs(), preferred_element_type=f32))
        vt_u[s, b * (VB // 2):(b + 1) * (VB // 2), :] = v
        sub = lax.broadcasted_iota(i32, (16, L), 0)
        for hh in range(8):
            w8 = (9 * hh) // 8
            ones_row = 0 if 2 * hh == 14 else 15
            vwin[s * H + 8 * b + hh] = jnp.where(sub == ones_row, u32(ONES_PAIR), v[8 * w8:8 * w8 + 16, :])

    def q_tasks(s):
        return [lambda g=g: q_task(s, g) for g in range(NG)]

    def k_tasks(s):
        return [lambda g=g: k_task(s, g) for g in range(NG)]

    def v_tasks(s):
        return [lambda b=b: v_task(s, b) for b in range(D // VB)]

    def advance_xs():
        for tt in range(TPS):
            xs_cur[tt, 0:D // 2, :] = xs_nxt[tt, 0:D // 2, :]

    def run(tasks):
        for t in tasks:
            t()

    with _scope("p1_wait_x0"):
        x_copy(0).wait()
    w_copy(1).start()
    w_copy(2).start()
    with _scope("p1_wait_wq"):
        w_copy(0).wait()
    for s in range(1, NSEG):
        x_copy(s).start()
    w_copy(3).start()
    for i in range(3):
        moe_copy(i).start()
    with _scope("p1_ln0_prep_q"):
        run(_interleave(ln_tasks(0, xs_cur), prep_grouped(0, WT_Q)))
        w_copy(1).wait()
    with _scope("p1_q0"):
        run(_interleave(q_tasks(0), prep_grouped(1, WT_K)))
        w_copy(2).wait()
    with _scope("p1_k0"):
        run(_interleave(k_tasks(0), prep_dense(2, wt_u, WT_V)))
        x_copy(1).wait()
    with _scope("p1_v0"):
        run(_interleave(v_tasks(0), ln_tasks(1, xs_nxt)))
        advance_xs()

    def seg_body(s, c):
        for ss in range(2, NSEG):
            @pl.when(s + 1 == ss)
            def _():
                x_copy(ss).wait()
        nxt = jnp.minimum(s + 1, NSEG - 1)
        with _scope("p1_seg"):
            run(_interleave(q_tasks(s) + k_tasks(s) + v_tasks(s), ln_tasks(nxt, xs_nxt)))
            advance_xs()
        return c

    lax.fori_loop(1, NSEG, seg_body, 0)

    row64 = lax.broadcasted_iota(i32, (TW, T), 0)
    lane64 = lax.broadcasted_iota(i32, (TW, T), 1)
    row32 = lax.broadcasted_iota(i32, (32, T), 0)
    lane32 = lax.broadcasted_iota(i32, (32, T), 1)
    lane1 = lax.broadcasted_iota(i32, (1, T), 1)
    lane8 = lax.broadcasted_iota(i32, (8, T), 1)

    def stage_a(unit, u, qt, s_ref, m_ref):
        s = unit // UPS
        pi = (unit % UPS) * NP + u
        g = pi // (HPG // 2)
        j = 2 * (pi - (HPG // 2) * g)
        sg = s * NG + g
        n = T * (qt + 1)
        qw = qs_u[sg, :, qt * T:(qt + 1) * T]
        w_a = qw & rowmask[j]
        w_b = qw & rowmask[j + 1]
        w_ab = _bf(jnp.where(lane64 < HT, w_a, w_b))

        def colmax8(v):
            return jnp.max(v.reshape(v.shape[0] // 8, 8, T), axis=0)

        maxes = []
        for hd, w in enumerate((_bf(w_a), _bf(w_b))):
            m8 = None
            for c in range(qt):
                kc = _bf(k_u[sg, c * TW:(c + 1) * TW, :])
                sc = jnp.dot(kc, w, preferred_element_type=f32)
                s_ref[u, qt, hd * L + c * T:hd * L + (c + 1) * T, :] = sc
                m8 = colmax8(sc) if m8 is None else jnp.maximum(m8, colmax8(sc))
            kc = _bf(k_u[sg, qt * TW:qt * TW + TW // 2, :])
            sc = jnp.dot(kc, w, preferred_element_type=f32) + mb[1 - hd]
            s_ref[u, qt, hd * L + qt * T:hd * L + qt * T + HT, :] = sc
            m8 = colmax8(sc) if m8 is None else jnp.maximum(m8, colmax8(sc))
            maxes.append(m8)
        kc = _bf(k_u[sg, qt * TW + TW // 2:(qt + 1) * TW, :])
        sc = jnp.dot(kc, w_ab, preferred_element_type=f32) + mb[2]
        s_ref[u, qt, n - HT:n, :] = sc
        mab = colmax8(sc)
        m_a = jnp.where(lane8 < HT, jnp.maximum(maxes[0], mab), maxes[0])
        m_b = jnp.where(lane8 >= HT, jnp.maximum(maxes[1], mab), maxes[1])
        m_ref[u, qt, 0] = jnp.broadcast_to(jnp.max(m_a, axis=0, keepdims=True), (8, T))
        m_ref[u, qt, 1] = jnp.broadcast_to(jnp.max(m_b, axis=0, keepdims=True), (8, T))

    def stage_b(unit, u, qt, s_ref, m_ref):
        s = unit // UPS
        pi = (unit % UPS) * NP + u
        n = T * (qt + 1)
        m_a = m_ref[u, qt, 0][0:1]
        m_b = m_ref[u, qt, 1][0:1]
        p_ab = jnp.exp2(s_ref[u, qt, n - HT:n, :] - jnp.where(lane1 < HT, m_a, m_b))
        for hd, m in enumerate((m_a, m_b)):
            h = 2 * pi + hd
            p = jnp.exp2(s_ref[u, qt, hd * L:hd * L + n - HT, :] - m)
            keep = (lane64 < HT) if hd == 0 else (lane64 >= HT)
            p = jnp.concatenate([p, jnp.where(keep, p_ab, 0.0)], axis=0).astype(bf16)
            w8 = (9 * h) // 8
            off = DH * h - 16 * w8
            o = jnp.dot(_bf(vwin[s * H + h, :, 0:n]), p, preferred_element_type=f32)
            den = jnp.where(off == 14, o[0:1], o[31:32])
            o = o * (omg[h][0:1] / den)
            if hd == 0:
                o = pltpu.roll(o, HT, 1)
            r1 = pl.multiple_of(16 * w8, 16)
            res = am[s, pl.ds(r1, 32), qt * T:(qt + 1) * T] + o
            pltpu.store(ot.at[pl.ds(r1, 32), qt * T:(qt + 1) * T], res, mask=smask[off // 2] != 0)

    def a_tasks(unit, s_ref, m_ref):
        return [lambda u=u, qt=qt: stage_a(unit, u, qt, s_ref, m_ref) for u in range(NP) for qt in range(4)]

    def b_tasks(unit, s_ref, m_ref):
        return [lambda u=u, qt=qt: stage_b(unit, u, qt, s_ref, m_ref) for u in range(NP) for qt in range(4)]

    ones16 = jnp.where(lax.broadcasted_iota(i32, (8, L), 0) == 0, u32(0x3F80), u32(0))

    def mem_task(s, g):
        es, eoff, ne = _ewin(g)
        nv = _valid(g)
        lhs = _bf(jnp.concatenate([vt_u[s, es // 2:(es + ne) // 2, :], ones16], axis=0))
        upd = lax.dot_general(lhs, _bf(pk_u[s * NG + g]), NT_DIMS, preferred_element_type=f32)
        mt = mt_acc[g, 0:ne + 16, :] + upd
        mt_acc[g, 0:ne + 16, :] = mt
        e_loc = lax.broadcasted_iota(i32, (ne, T), 0) - eoff
        d_id = lax.broadcasted_iota(i32, (ne, T), 1)
        same_head = (e_loc >= 0) & (e_loc < nv) & (d_id < nv) & ((e_loc // DH) == (d_id // DH))
        j16 = lax.broadcasted_iota(i32, (16, T), 0)
        d16 = lax.broadcasted_iota(i32, (16, T), 1)
        z_mask = ((d16 // DH) == j16) & (d16 < nv)
        lm = jnp.concatenate(
            [jnp.where(same_head, mt[0:ne], 0.0),
             jnp.where(z_mask, jnp.broadcast_to(mt[ne:ne + 1, :], (16, T)), 0.0)], axis=0)
        nd = jnp.dot(lm.astype(bf16), _bf(pq_u[(s + 1) * NG + g]), preferred_element_type=f32)
        scale = jnp.broadcast_to(g16[g][:, 0:1], (16, L)) / (nd[ne:ne + 16, :] + 1e-6)
        r8 = lax.broadcasted_iota(i32, (8, L), 0)
        for b in range(ne // 8):
            lo, hi = 8 * b - eoff, 8 * b + 7 - eoff
            if hi < 0 or lo >= nv:
                continue
            j1, j2 = max(lo, 0) // DH, min(hi, nv - 1) // DH
            sc = jnp.broadcast_to(scale[j1:j1 + 1, :], (8, L))
            if j2 != j1:
                sc = jnp.where(r8 < DH * j2 - lo, sc, jnp.broadcast_to(scale[j2:j2 + 1, :], (8, L)))
            val = nd[8 * b:8 * b + 8, :] * sc
            dst = am.at[s + 1, es + 8 * b:es + 8 * b + 8, :]
            if lo >= 0 and hi < nv:
                dst[...] = val
            else:
                pltpu.store(dst, val, mask=(r8 + lo >= 0) & (r8 + lo < nv))

    mem_tasks = [lambda s=s, g=g: mem_task(s, g) for s in range(NSEG - 1) for g in range(NG)]

    w_copy(3).wait()
    for i in range(3):
        moe_copy(i).wait()
    rr = jnp.concatenate([r_buf[s][0:1, :] for s in range(NSEG)], axis=0)
    rr = _round_bf16(rr)
    tok = lax.broadcasted_iota(i32, (NSEG, L), 0) * L + lax.broadcasted_iota(i32, (NSEG, L), 1)
    m1v = jnp.max(rr)
    i1 = jnp.min(jnp.where(rr == m1v, tok, SEQ))
    rr2 = jnp.where(tok == i1, -jnp.inf, rr)
    m2v = jnp.max(rr2)
    i2 = jnp.min(jnp.where(rr2 == m2v, tok, SEQ))
    i1 = jnp.clip(i1, 0, SEQ - 1)
    i2 = jnp.clip(i2, 0, SEQ - 1)

    row16 = lax.broadcasted_iota(i32, (16, T), 0)
    lane16 = lax.broadcasted_iota(i32, (16, T), 1)

    def token_rows(i, slot):
        onehot = jnp.where((row16 == slot) & (lane16 == i % T), 1.0, 0.0).astype(bf16)
        return lax.dot_general(onehot, _bf(xn_u[i // T]), NT_DIMS, preferred_element_type=f32)

    def select_task():
        xsel_buf[...] = _pack(token_rows(i1, 0) + token_rows(i2, 1))
        y_acc[...] = jnp.zeros(y_acc.shape, f32)

    def fcols(ft):
        return pl.ds(ft * T if isinstance(ft, int) else pl.multiple_of(ft * T, T), T)

    def moe_up_task(ft, k, which):
        xsel = _bf(xsel_buf[:, 0:D])
        w_ref = (wg_buf, wu_buf)[which]
        hid_buf[k, which] = jnp.dot(xsel, w_ref[:, fcols(ft)], preferred_element_type=f32)

    def moe_down_task(ft, k):
        gt = _round_bf16(hid_buf[k, 0])
        up = _round_bf16(hid_buf[k, 1])
        hid = (_round_bf16(gt * _sigmoid(gt)) * up).astype(bf16)
        y_acc[...] += lax.dot_general(hid, wd_buf[:, fcols(ft)], NT_DIMS, preferred_element_type=f32)

    def moe_tasks(ft0, count):
        ups = [lambda k=k, w=w: moe_up_task(ft0 + k, k, w) for k in range(count) for w in range(2)]
        downs = [lambda k=k: moe_down_task(ft0 + k, k) for k in range(count)]
        return ups + downs

    def moe_finish():
        y = _round_bf16(y_acc[...])
        rsel = jnp.where(lax.broadcasted_iota(i32, (16, 1), 0) == 0, m1v, m2v)
        y = _round_bf16(y * _round_bf16(_sigmoid(rsel)))
        y = jnp.concatenate([y, jnp.zeros((16, DP - D), f32)], axis=1)
        y = jnp.concatenate([y, jnp.zeros((T - 16, DP), f32)], axis=0)
        y_t = y.T
        for t in range(2):
            ycol[t] = jnp.broadcast_to(y_t[0:D, t:t + 1], (D, T))
        tok_l = lax.broadcasted_iota(i32, (8, L), 1) + (NSEG - 1) * L
        sel_buf[0] = jnp.where(tok_l == i1, 1.0, 0.0)
        sel_buf[1] = jnp.where(tok_l == i2, 1.0, 0.0)

    dense = _interleave(mem_tasks, a_tasks(0, s0, m0), prep_dense(3, wot_u, 0))
    with _scope("p15_mix"):
        run(dense[0:2] + [select_task] + dense[2:])

    def out_tile(s, tt, last):
        c0 = s * L + tt * T
        if not isinstance(s, int):
            c0 = pl.multiple_of(c0, T)
        o_bf = ot[:, (tt // 2) * 2 * T:(tt // 2 + 1) * 2 * T].astype(bf16)[:, (tt % 2) * T:(tt % 2 + 1) * T]
        attn = jnp.dot(_bf(wot_u[...]), o_bf, preferred_element_type=f32)
        xn = _bf(xn_u[s * TPS + tt, 0:D // 2, :]).astype(f32)
        x = x_buf[:, pl.ds(c0, T)].astype(f32)
        res = x + attn + xn
        if last:
            for t in range(2):
                hit = sel_buf[t, 0:1, tt * T:(tt + 1) * T] > 0.5
                res = res + jnp.where(hit, ycol[t], 0.0)
        out_buf[:, pl.ds(c0, T)] = res.astype(bf16)
        if last:
            out_copy(c0, T, NSEG - 1 + tt).start()

    def pair(ua, sa, ma, ub, sb, mbuf, extra):
        ab = []
        for x, y in zip(a_tasks(ua, sa, ma), b_tasks(ub, sb, mbuf)):
            ab.append(lambda x=x, y=y: (x(), y()))
        run(_interleave(ab, extra) if extra else ab)

    def att_body(i, c):
        u0 = 2 * i
        extra = moe_tasks(i * FPI, FPI)
        half = len(extra) // 2
        with _scope("att_body"):
            pair(u0 + 1, s1, m1, u0, s0, m0, extra[:half])
            pair(u0 + 2, s0, m0, u0 + 1, s1, m1, extra[half:])

        @pl.when((u0 + 2) % UPS == 0)
        def _():
            with _scope("outproj"):
                for tt in range(TPS):
                    out_tile(u0 // UPS, tt, False)
                for ss in range(NSEG - 1):
                    @pl.when(u0 // UPS == ss)
                    def _():
                        out_copy(ss * L, L, ss).start()
        return c

    nloop = NUNIT // 2 - 1
    lax.fori_loop(0, nloop, att_body, 0)
    with _scope("att_tail"):
        pair(NUNIT - 1, s1, m1, NUNIT - 2, s0, m0, moe_tasks(nloop * FPI, NFT - nloop * FPI))
        moe_finish()

    def patch(t, idx):
        inside = idx < (NSEG - 1) * L
        c0 = pl.multiple_of(jnp.where(inside, idx // T, 0) * T, T)
        lane = lax.broadcasted_iota(i32, (1, T), 1)
        hit = (lane == idx % T) & inside
        cur = out_buf[:, pl.ds(c0, T)].astype(f32)
        out_buf[:, pl.ds(c0, T)] = (cur + jnp.where(hit, ycol[t], 0.0)).astype(bf16)
        return out_copy(c0, T, 7 + t)

    with _scope("att_lastb"):
        for s in range(NSEG - 1):
            out_copy(s * L, L, s).wait()
        copy0 = patch(0, i1)
        copy0.start()
        last_b = [[lambda u=u, qt=qt: stage_b(NUNIT - 1, u, qt, s1, m1) for u in range(NP)] for qt in range(4)]
        run(last_b[0])
        run(last_b[1][0:2] + [lambda: out_tile(NSEG - 1, 0, True)] + last_b[1][2:])
        copy0.wait()
        copy1 = patch(1, i2)
        copy1.start()
        run(last_b[2][0:2] + [lambda: out_tile(NSEG - 1, 1, True)] + last_b[2][2:])
        run(last_b[3][0:2] + [lambda: out_tile(NSEG - 1, 2, True)] + last_b[3][2:])
        out_tile(NSEG - 1, 3, True)

    with _scope("out_wait"):
        copy1.wait()
        for tt in range(TPS):
            out_copy((NSEG - 1) * L + tt * T, T, NSEG - 1 + tt).wait()


@jax.jit
def pallas_parallel_sum__memory_aug_infini_attn__moe_arch_mod__prompt_kernel(
    A_x: jax.Array,
    A_wq: jax.Array,
    A_wk: jax.Array,
    A_wv: jax.Array,
    A_wo: jax.Array,
    A_beta: jax.Array,
    B_x: jax.Array,
    B_w_r: jax.Array,
    B_w_gate: jax.Array,
    B_w_up: jax.Array,
    B_w_down: jax.Array,
):
    del B_x
    any_spec = pl.BlockSpec(memory_space=pl.ANY)
    vmem_spec = pl.BlockSpec(memory_space=pltpu.VMEM)
    scratch = [
        pltpu.VMEM((D, SEQ), bf16),
        pltpu.VMEM((4, D, D), bf16),
        pltpu.VMEM((D, F), bf16),
        pltpu.VMEM((D, F), bf16),
        pltpu.VMEM((D, F), bf16),
        pltpu.VMEM((D, SEQ), bf16),
        pltpu.VMEM((WT_ROWS, DP), u32),
        pltpu.VMEM((D // 2, DP), u32),
        pltpu.VMEM((D // 2, DP), u32),
        pltpu.VMEM((NT, DP // 2, T), u32),
        pltpu.VMEM((TPS, DP // 2, T), u32),
        pltpu.VMEM((TPS, DP // 2, T), u32),
        pltpu.VMEM((NSEG * NG, TW, L), u32),
        pltpu.VMEM((NSEG * NG, L // 2, T), u32),
        pltpu.VMEM((NSEG * NG, TW, L), u32),
        pltpu.VMEM((NSEG * NG, TW, L), u32),
        pltpu.VMEM((NSEG, D // 2, L), u32),
        pltpu.VMEM((NSEG * H, 16, L), u32),
        pltpu.VMEM((NSEG, 8, L), f32),
        pltpu.VMEM((NG, T + 16, T), f32),
        pltpu.VMEM((NSEG, D, L), f32),
        pltpu.VMEM((NG, 16, T), f32),
        pltpu.VMEM((H, 8, T), f32),
        pltpu.VMEM((3, HT, T), f32),
        pltpu.VMEM((HPG, TW, T), u32),
        pltpu.VMEM((8, 32, T), i32),
        pltpu.VMEM((NP, 4, 2 * L, T), f32),
        pltpu.VMEM((NP, 4, 2, 8, T), f32),
        pltpu.VMEM((NP, 4, 2 * L, T), f32),
        pltpu.VMEM((NP, 4, 2, 8, T), f32),
        pltpu.VMEM((DP, L), f32),
        pltpu.VMEM((2, D, LNW), f32),
        pltpu.VMEM((2, 2, 8, LNW), f32),
        pltpu.VMEM((16, D), f32),
        pltpu.VMEM((8, DP), u32),
        pltpu.VMEM((FPI, 2, 16, T), f32),
        pltpu.VMEM((2, D, T), f32),
        pltpu.VMEM((2, 8, L), f32),
        pltpu.SemaphoreType.DMA((NSEM,)),
    ]
    x_t = jnp.transpose(A_x, (0, 2, 1)).reshape(D, SEQ)
    out_t = pl.pallas_call(
        _kernel,
        out_shape=jax.ShapeDtypeStruct((D, SEQ), bf16),
        in_specs=[any_spec, any_spec, any_spec, any_spec, any_spec, vmem_spec, vmem_spec,
                  any_spec, any_spec, any_spec],
        out_specs=any_spec,
        scratch_shapes=scratch,
        compiler_params=pltpu.CompilerParams(vmem_limit_bytes=110 * 1024 * 1024),
    )(x_t, A_wq, A_wk, A_wv, A_wo, A_beta, B_w_r, B_w_gate, B_w_up, B_w_down.T)
    return jnp.transpose(out_t.reshape(1, D, SEQ), (0, 2, 1))
```

```python
import contextlib

import jax
import jax.numpy as jnp
from jax import lax
from jax.experimental import pallas as pl
from jax.experimental.pallas import tpu as pltpu

bf16 = jnp.bfloat16
f32 = jnp.float32
u32 = jnp.uint32
i32 = jnp.int32

SEQ = 2048
D = 576
DP = 640
H = 32
DH = 18
NSEG = 4
L = 512
T = 128
TW = T // 2
HT = T // 2
TPS = L // T
HPG = 6
NG = 6
F = 4608
FPI = 5
NFT = F // T
NP = 4
UPS = H // (2 * NP)
NUNIT = NSEG * UPS
NT = SEQ // T
LNW = 256
VB = 8 * DH

LOG2E = 1.4426950408889634
QSCALE = (DH ** -0.5) * LOG2E
MASKVAL = -1000000000.0 * LOG2E
EPS_BF16 = 1.0013580322265625e-05
ONES_PAIR = 0x3F803F80

NT_DIMS = (((1,), (1,)), ((), ()))

WT_Q = 0
WT_K = NG * TW
WT_V = 2 * NG * TW
WT_ROWS = WT_V + D // 2

X_PIECES = ((0, LNW), (LNW, LNW), (L, L), (2 * L, L), (3 * L, L))
SEM_X = 0
SEM_W = 5
SEM_MOE = 9
SEM_OUT = 12
NSEM = 21


PROFILE_SCOPES = False
PACE = False
QT_ORDER = (3, 2, 1, 0)


def _scope(name):
    return jax.named_scope(name) if PROFILE_SCOPES else contextlib.nullcontext()


def _valid(g):
    return min(HPG * DH, D - g * HPG * DH)


def _rows(g):
    return -(-_valid(g) // 16) * 16


def _ewin(g):
    start = (g * HPG * DH // 16) * 16
    return start, g * HPG * DH - start, min(T, D - start)


def _bf(x):
    return pltpu.bitcast(x, bf16)


def _pack(x):
    return pltpu.bitcast(x.astype(bf16), u32)


def _round_bf16(x):
    return x.astype(bf16).astype(f32)


def _phi(t):
    return jnp.where(t > 0, t + 1.0, jnp.exp(t))


def _sigmoid(t):
    return 1.0 / (1.0 + jnp.exp(-t))


def _zero_after(v):
    bits = pltpu.bitcast(v[0:8, 0:LNW], u32)
    sixteen = jnp.uint32(16)
    bits = lax.shift_right_logical(lax.shift_right_logical(bits, sixteen), sixteen)
    return pltpu.bitcast(bits, f32) if PACE else None


def _interleave(*lists):
    items = []
    for li, tasks in enumerate(lists):
        for k, t in enumerate(tasks):
            items.append(((k + 0.5) / len(tasks), li, k, t))
    items.sort(key=lambda it: it[:3])
    return [it[3] for it in items]


def _kernel(x_hbm, wq_hbm, wk_hbm, wv_hbm, wo_hbm, beta_ref, wr_ref, wg_hbm, wu_hbm, wd_hbm,
            out_hbm,
            x_buf, w_buf, wg_buf, wu_buf, wd_buf, out_buf,
            wt_u, wtd_u, wot_u, xn_u, qs_u, k_u, pq_u, pk_u, vt_u, vwin,
            r_buf, mt_acc, am, g16, omg, mb, rowmask, smask,
            s0, m0, s1, m1, ot, xf, ln_stat, y_acc, xsel_buf, hid_buf, ycol, sel_buf, sems):

    def x_copy(i):
        c0, width = X_PIECES[i]
        return pltpu.make_async_copy(x_hbm.at[:, pl.ds(c0, width)], x_buf.at[:, pl.ds(c0, width)],
                                     sems.at[SEM_X + i])

    def w_copy(i):
        src = (wq_hbm, wk_hbm, wv_hbm, wo_hbm)[i]
        return pltpu.make_async_copy(src, w_buf.at[i], sems.at[SEM_W + i])

    def moe_copy(i):
        src = (wg_hbm, wu_hbm, wd_hbm)[i]
        dst = (wg_buf, wu_buf, wd_buf)[i]
        return pltpu.make_async_copy(src, dst, sems.at[SEM_MOE + i])

    def out_copy(c0, width, sem):
        return pltpu.make_async_copy(out_buf.at[:, pl.ds(c0, width)], out_hbm.at[:, pl.ds(c0, width)],
                                     sems.at[SEM_OUT + sem])

    w_copy(0).start()
    x_copy(0).start()
    x_copy(1).start()
    w_copy(1).start()
    w_copy(2).start()

    init_scope = _scope("init")
    init_scope.__enter__()
    kr = lax.broadcasted_iota(i32, (HT, T), 0)
    ql = lax.broadcasted_iota(i32, (HT, T), 1)
    mb[0] = jnp.where(ql < kr, MASKVAL, 0.0).astype(f32)
    mb[1] = jnp.where((ql >= HT) & (ql - HT < kr), MASKVAL, 0.0).astype(f32)
    mb[2] = jnp.where(ql % HT < kr, MASKVAL, 0.0).astype(f32)
    for j in range(HPG):
        rowmask[j] = jnp.where((kr >= (DH // 2) * j) & (kr < (DH // 2) * (j + 1)), u32(0xFFFFFFFF), u32(0))
    r32 = lax.broadcasted_iota(i32, (32, T), 0)
    for i in range(8):
        smask[i] = jnp.where((r32 >= 2 * i) & (r32 < 2 * i + DH), 1, 0)
    zpad = jnp.zeros(((DP - D) // 2, T), u32)
    for tt in range(NT):
        xn_u[tt, D // 2:DP // 2, :] = zpad
    ot[D:DP, :] = jnp.zeros((DP - D, L), f32)
    am[0] = jnp.zeros(am.shape[1:], f32)
    mt_acc[...] = jnp.zeros(mt_acc.shape, f32)
    g16[...] = jnp.zeros(g16.shape, f32)
    for sg in range(NSEG * NG):
        r2 = _rows(sg % NG) // 2
        qs_u[sg, r2:TW, :] = jnp.zeros((TW - r2, L), u32)
        pq_u[sg, r2:TW, :] = jnp.zeros((TW - r2, L), u32)
        pk_u[sg, r2:TW, :] = jnp.zeros((TW - r2, L), u32)

    gate = _round_bf16(_sigmoid(beta_ref[...].reshape(1, H).astype(f32)))
    for h in range(H):
        gh = jnp.broadcast_to(gate[:, h:h + 1], (1, T))
        omg[h] = jnp.broadcast_to(_round_bf16(1.0 - gh), (8, T))
        g16[h // HPG, (h % HPG):(h % HPG) + 1, :] = gh

    init_scope.__exit__(None, None, None)

    pace = [None]

    def transpose_block(i, cb):
        c1 = min((cb + 1) * T, D)
        blk = w_buf[i, :, cb * T:c1]
        if c1 - cb * T < T:
            blk = jnp.concatenate([blk, jnp.zeros((D, T - (c1 - cb * T)), bf16)], axis=1)
        blk = jnp.concatenate([blk, jnp.zeros((DP - D, T), bf16)], axis=0)
        return pltpu.bitcast(blk.T, u32)

    def prep_dense(i, dst, base):
        def task(cb):
            nrow = min(TW, D // 2 - cb * TW)
            dst[base + cb * TW:base + cb * TW + nrow, :] = transpose_block(i, cb)[0:nrow]
        return [lambda cb=cb: task(cb) for cb in range(DP // T)]

    def prep_grouped(i, base):
        def regroup(g):
            nv, nr = _valid(g) // 2, _rows(g) // 2
            src = g * HPG * DH // 2
            wt_u[base + g * TW:base + g * TW + nv, :] = wtd_u[src:src + nv, :]
            pad = jnp.zeros((nr - nv, DP), u32)
            if i == 1 and g == 0:
                wr = wr_ref[...].reshape(1, D).astype(f32)
                wr = jnp.concatenate([wr, jnp.zeros((1, DP - D), f32)], axis=1)
                bits = lax.shift_right_logical(pltpu.bitcast(wr, u32), u32(16))
                rid = lax.broadcasted_iota(i32, (nr - nv, DP), 0)
                pad = jnp.where(rid == 0, bits, pad)
            wt_u[base + g * TW + nv:base + g * TW + nr, :] = pad
        return prep_dense(i, wtd_u, 0) + [lambda g=g: regroup(g) for g in range(NG)]

    def ln_tasks(s):
        def mean_pass(b):
            c0 = s * L + b * LNW
            if not isinstance(s, int):
                c0 = pl.multiple_of(c0, LNW)
            acc = pace[0]
            for r in range(0, D, 64):
                x = x_buf[r:r + 64, pl.ds(c0, LNW)].astype(f32)
                xf[b, r:r + 64, :] = x
                part = jnp.sum(x.reshape(8, 8, LNW), axis=0)
                acc = part if acc is None else acc + part
            mean = jnp.sum(acc, axis=0, keepdims=True) / D
            ln_stat[b, 0] = jnp.broadcast_to(mean, (8, LNW))

        def var_pass(b):
            bd = b
            mean = ln_stat[b, 0][0:1]
            if pace[0] is not None:
                mean = mean + pace[0][0:1]
            acc = None
            for r in range(0, D, 96):
                xc = xf[bd, r:r + 96, :] - mean
                part = jnp.sum((xc * xc).reshape(12, 8, LNW), axis=0)
                acc = part if acc is None else acc + part
            var = jnp.sum(acc, axis=0, keepdims=True) / D
            den = _round_bf16(jnp.sqrt(_round_bf16(_round_bf16(var) + EPS_BF16)))
            ln_stat[b, 1] = jnp.broadcast_to(1.0 / den, (8, LNW))
            ln_stat[b, 0] = jnp.broadcast_to(_round_bf16(mean), (8, LNW))

        def norm_pass(b, half):
            bd = b
            mean_b = ln_stat[b, 0][0:1]
            if pace[0] is not None:
                mean_b = mean_b + pace[0][0:1]
            inv = ln_stat[b, 1][0:1]
            for r in range(half * (D // 2), (half + 1) * (D // 2), 48):
                xn = _pack(_round_bf16(xf[bd, r:r + 48, :] - mean_b) * inv)
                for t in range(LNW // T):
                    tt = b * (LNW // T) + t
                    xn_u[s * TPS + tt, r // 2:r // 2 + 24, :] = xn[:, t * T:(t + 1) * T]

        tasks = []
        for b in range(L // LNW):
            tasks += [lambda b=b: mean_pass(b), lambda b=b: var_pass(b),
                      lambda b=b: norm_pass(b, 0), lambda b=b: norm_pass(b, 1)]
        return tasks

    def load_xs(s, t0, t1):
        return jnp.concatenate([_bf(xn_u[s * TPS + tt]) for tt in range(t0, t1)], axis=1)

    def q_task(s, g, t0=0, t1=TPS):
        nr = _rows(g) // 2
        w = _bf(wt_u[WT_Q + g * TW:WT_Q + g * TW + nr, :])
        q = jnp.dot(w, load_xs(s, t0, t1), preferred_element_type=f32)
        pace[0] = _zero_after(q)
        qp = _pack(q * QSCALE)
        qrot = jnp.concatenate([pltpu.roll(qp[:, t * T:(t + 1) * T], HT, 1) for t in range(t1 - t0)], axis=1)
        rid = lax.broadcasted_iota(i32, qp.shape, 0)
        even = ((rid // (DH // 2)) % 2) == 0
        qs_u[s * NG + g, 0:nr, t0 * T:t1 * T] = jnp.where(even, qrot, qp)
        pq_u[s * NG + g, 0:nr, t0 * T:t1 * T] = _pack(_phi(_round_bf16(q)))

    def k_task(s, g):
        nr = _rows(g)
        w = _bf(wt_u[WT_K + g * TW:WT_K + g * TW + nr // 2, :])
        k = jnp.dot(w, load_xs(s, 0, TPS), preferred_element_type=f32)
        pace[0] = _zero_after(k)
        if g == 0:
            r_buf[s] = jnp.broadcast_to(k[_valid(0):_valid(0) + 1, :], (8, L))
        kp = _pack(k)
        pk_u[s * NG + g, 0:nr // 2, :] = _pack(_phi(_round_bf16(k)))
        kfull = _bf(jnp.concatenate([kp, jnp.zeros(((T - nr) // 2, L), u32)], axis=0))
        k_u[s * NG + g] = pltpu.bitcast(kfull.T, u32)

    def v_task(s, b):
        w = _bf(wt_u[WT_V + b * (VB // 2):WT_V + (b + 1) * (VB // 2), :])
        v = jnp.dot(w, load_xs(s, 0, TPS), preferred_element_type=f32)
        pace[0] = _zero_after(v)
        v = _pack(v)
        vt_u[s, b * (VB // 2):(b + 1) * (VB // 2), :] = v
        sub = lax.broadcasted_iota(i32, (16, L), 0)
        for hh in range(8):
            w8 = (9 * hh) // 8
            ones_row = 0 if 2 * hh == 14 else 15
            vwin[s * H + 8 * b + hh] = jnp.where(sub == ones_row, u32(ONES_PAIR), v[8 * w8:8 * w8 + 16, :])

    def q_tasks(s, t0=0, t1=TPS):
        return [lambda g=g: q_task(s, g, t0, t1) for g in range(NG)]

    def k_tasks(s):
        return [lambda g=g: k_task(s, g) for g in range(NG)]

    def v_tasks(s):
        return [lambda b=b: v_task(s, b) for b in range(D // VB)]

    def run(tasks):
        for t in tasks:
            t()

    ln0 = ln_tasks(0)
    prep_q = prep_grouped(0, WT_Q)
    with _scope("p1_wait_wq"):
        w_copy(0).wait()
    with _scope("p1_prep_q"):
        run(prep_q[0:3])
        x_copy(0).wait()
    for i in range(2, len(X_PIECES)):
        x_copy(i).start()
    w_copy(3).start()
    for i in range(3):
        moe_copy(i).start()
    with _scope("p1_ln0a"):
        run(_interleave(prep_q[3:], ln0[0:4]))
        x_copy(1).wait()
    with _scope("p1_q0a"):
        run(_interleave(q_tasks(0, 0, 2), ln0[4:8]))
        w_copy(1).wait()
    with _scope("p1_q0b"):
        run(_interleave(q_tasks(0, 2, 4), prep_grouped(1, WT_K)))
        w_copy(2).wait()
    with _scope("p1_k0"):
        run(_interleave(k_tasks(0), prep_dense(2, wt_u, WT_V)))
        x_copy(2).wait()
    with _scope("p1_v0"):
        run(_interleave(v_tasks(0), ln_tasks(1)))

    def seg_body(s, c):
        for ss in range(2, NSEG):
            @pl.when(s + 1 == ss)
            def _():
                x_copy(ss + 1).wait()
        nxt = jnp.minimum(s + 1, NSEG - 1)
        pace[0] = None
        with _scope("p1_seg"):
            run(_interleave(q_tasks(s) + k_tasks(s) + v_tasks(s), ln_tasks(nxt)))
        return c

    lax.fori_loop(1, NSEG, seg_body, 0)

    row64 = lax.broadcasted_iota(i32, (TW, T), 0)
    lane64 = lax.broadcasted_iota(i32, (TW, T), 1)
    row32 = lax.broadcasted_iota(i32, (32, T), 0)
    lane32 = lax.broadcasted_iota(i32, (32, T), 1)
    lane1 = lax.broadcasted_iota(i32, (1, T), 1)
    lane8 = lax.broadcasted_iota(i32, (8, T), 1)

    def stage_a(unit, u, qt, s_ref, m_ref):
        s = unit // UPS
        pi = (unit % UPS) * NP + u
        g = pi // (HPG // 2)
        j = 2 * (pi - (HPG // 2) * g)
        sg = s * NG + g
        n = T * (qt + 1)
        qw = qs_u[sg, :, qt * T:(qt + 1) * T]
        w_a = qw & rowmask[j]
        w_b = qw & rowmask[j + 1]
        w_ab = _bf(jnp.where(lane64 < HT, w_a, w_b))

        def colmax8(v):
            return jnp.max(v.reshape(v.shape[0] // 8, 8, T), axis=0)

        maxes = []
        for hd, w in enumerate((_bf(w_a), _bf(w_b))):
            m8 = None
            for c in range(qt):
                kc = _bf(k_u[sg, c * TW:(c + 1) * TW, :])
                sc = jnp.dot(kc, w, preferred_element_type=f32)
                s_ref[u, qt, hd * L + c * T:hd * L + (c + 1) * T, :] = sc
                m8 = colmax8(sc) if m8 is None else jnp.maximum(m8, colmax8(sc))
            kc = _bf(k_u[sg, qt * TW:qt * TW + TW // 2, :])
            sc = jnp.dot(kc, w, preferred_element_type=f32) + mb[1 - hd]
            s_ref[u, qt, hd * L + qt * T:hd * L + qt * T + HT, :] = sc
            m8 = colmax8(sc) if m8 is None else jnp.maximum(m8, colmax8(sc))
            maxes.append(m8)
        kc = _bf(k_u[sg, qt * TW + TW // 2:(qt + 1) * TW, :])
        sc = jnp.dot(kc, w_ab, preferred_element_type=f32) + mb[2]
        s_ref[u, qt, n - HT:n, :] = sc
        mab = colmax8(sc)
        m_a = jnp.where(lane8 < HT, jnp.maximum(maxes[0], mab), maxes[0])
        m_b = jnp.where(lane8 >= HT, jnp.maximum(maxes[1], mab), maxes[1])
        m_ref[u, qt, 0] = jnp.broadcast_to(jnp.max(m_a, axis=0, keepdims=True), (8, T))
        m_ref[u, qt, 1] = jnp.broadcast_to(jnp.max(m_b, axis=0, keepdims=True), (8, T))

    def stage_b(unit, u, qt, s_ref, m_ref):
        s = unit // UPS
        pi = (unit % UPS) * NP + u
        n = T * (qt + 1)
        m_a = m_ref[u, qt, 0][0:1]
        m_b = m_ref[u, qt, 1][0:1]
        p_ab = jnp.exp2(s_ref[u, qt, n - HT:n, :] - jnp.where(lane1 < HT, m_a, m_b))
        for hd, m in enumerate((m_a, m_b)):
            h = 2 * pi + hd
            p = jnp.exp2(s_ref[u, qt, hd * L:hd * L + n - HT, :] - m)
            keep = (lane64 < HT) if hd == 0 else (lane64 >= HT)
            p = jnp.concatenate([p, jnp.where(keep, p_ab, 0.0)], axis=0).astype(bf16)
            w8 = (9 * h) // 8
            off = DH * h - 16 * w8
            o = jnp.dot(_bf(vwin[s * H + h, :, 0:n]), p, preferred_element_type=f32)
            den = jnp.where(off == 14, o[0:1], o[31:32])
            o = o * (omg[h][0:1] / den)
            if hd == 0:
                o = pltpu.roll(o, HT, 1)
            r1 = pl.multiple_of(16 * w8, 16)
            res = am[s, pl.ds(r1, 32), qt * T:(qt + 1) * T] + o
            pltpu.store(ot.at[pl.ds(r1, 32), qt * T:(qt + 1) * T], res, mask=smask[off // 2] != 0)

    def a_tasks(unit, s_ref, m_ref):
        return [lambda u=u, qt=qt: stage_a(unit, u, qt, s_ref, m_ref) for u in range(NP) for qt in QT_ORDER]

    def b_tasks(unit, s_ref, m_ref):
        return [lambda u=u, qt=qt: stage_b(unit, u, qt, s_ref, m_ref) for u in range(NP) for qt in QT_ORDER]

    ones16 = jnp.where(lax.broadcasted_iota(i32, (8, L), 0) == 0, u32(0x3F80), u32(0))

    def mem_task(s, g):
        es, eoff, ne = _ewin(g)
        nv = _valid(g)
        lhs = _bf(jnp.concatenate([vt_u[s, es // 2:(es + ne) // 2, :], ones16], axis=0))
        upd = lax.dot_general(lhs, _bf(pk_u[s * NG + g]), NT_DIMS, preferred_element_type=f32)
        mt = mt_acc[g, 0:ne + 16, :] + upd
        mt_acc[g, 0:ne + 16, :] = mt
        e_loc = lax.broadcasted_iota(i32, (ne, T), 0) - eoff
        d_id = lax.broadcasted_iota(i32, (ne, T), 1)
        same_head = (e_loc >= 0) & (e_loc < nv) & (d_id < nv) & ((e_loc // DH) == (d_id // DH))
        j16 = lax.broadcasted_iota(i32, (16, T), 0)
        d16 = lax.broadcasted_iota(i32, (16, T), 1)
        z_mask = ((d16 // DH) == j16) & (d16 < nv)
        lm = jnp.concatenate(
            [jnp.where(same_head, mt[0:ne], 0.0),
             jnp.where(z_mask, jnp.broadcast_to(mt[ne:ne + 1, :], (16, T)), 0.0)], axis=0)
        nd = jnp.dot(lm.astype(bf16), _bf(pq_u[(s + 1) * NG + g]), preferred_element_type=f32)
        scale = jnp.broadcast_to(g16[g][:, 0:1], (16, L)) / (nd[ne:ne + 16, :] + 1e-6)
        r8 = lax.broadcasted_iota(i32, (8, L), 0)
        for b in range(ne // 8):
            lo, hi = 8 * b - eoff, 8 * b + 7 - eoff
            if hi < 0 or lo >= nv:
                continue
            j1, j2 = max(lo, 0) // DH, min(hi, nv - 1) // DH
            sc = jnp.broadcast_to(scale[j1:j1 + 1, :], (8, L))
            if j2 != j1:
                sc = jnp.where(r8 < DH * j2 - lo, sc, jnp.broadcast_to(scale[j2:j2 + 1, :], (8, L)))
            val = nd[8 * b:8 * b + 8, :] * sc
            dst = am.at[s + 1, es + 8 * b:es + 8 * b + 8, :]
            if lo >= 0 and hi < nv:
                dst[...] = val
            else:
                pltpu.store(dst, val, mask=(r8 + lo >= 0) & (r8 + lo < nv))

    mem_tasks = [lambda s=s, g=g: mem_task(s, g) for s in range(NSEG - 1) for g in range(NG)]

    w_copy(3).wait()
    for i in range(3):
        moe_copy(i).wait()
    rr = jnp.concatenate([r_buf[s][0:1, :] for s in range(NSEG)], axis=0)
    rr = _round_bf16(rr)
    tok = lax.broadcasted_iota(i32, (NSEG, L), 0) * L + lax.broadcasted_iota(i32, (NSEG, L), 1)
    m1v = jnp.max(rr)
    i1 = jnp.min(jnp.where(rr == m1v, tok, SEQ))
    rr2 = jnp.where(tok == i1, -jnp.inf, rr)
    m2v = jnp.max(rr2)
    i2 = jnp.min(jnp.where(rr2 == m2v, tok, SEQ))
    i1 = jnp.clip(i1, 0, SEQ - 1)
    i2 = jnp.clip(i2, 0, SEQ - 1)

    row16 = lax.broadcasted_iota(i32, (16, T), 0)
    lane16 = lax.broadcasted_iota(i32, (16, T), 1)

    def token_rows(i, slot):
        onehot = jnp.where((row16 == slot) & (lane16 == i % T), 1.0, 0.0).astype(bf16)
        return lax.dot_general(onehot, _bf(xn_u[i // T]), NT_DIMS, preferred_element_type=f32)

    def select_task():
        xsel_buf[...] = _pack(token_rows(i1, 0) + token_rows(i2, 1))
        y_acc[...] = jnp.zeros(y_acc.shape, f32)

    def fcols(ft):
        return pl.ds(ft * T if isinstance(ft, int) else pl.multiple_of(ft * T, T), T)

    def moe_up_task(ft, k, which):
        xsel = _bf(xsel_buf[:, 0:D])
        w_ref = (wg_buf, wu_buf)[which]
        hid_buf[k, which] = jnp.dot(xsel, w_ref[:, fcols(ft)], preferred_element_type=f32)

    def moe_down_task(ft, k):
        gt = _round_bf16(hid_buf[k, 0])
        up = _round_bf16(hid_buf[k, 1])
        hid = (_round_bf16(gt * _sigmoid(gt)) * up).astype(bf16)
        y_acc[...] += lax.dot_general(hid, wd_buf[:, fcols(ft)], NT_DIMS, preferred_element_type=f32)

    def moe_tasks(ft0, count):
        ups = [lambda k=k, w=w: moe_up_task(ft0 + k, k, w) for k in range(count) for w in range(2)]
        downs = [lambda k=k: moe_down_task(ft0 + k, k) for k in range(count)]
        return ups + downs

    def moe_finish():
        y = _round_bf16(y_acc[...])
        rsel = jnp.where(lax.broadcasted_iota(i32, (16, 1), 0) == 0, m1v, m2v)
        y = _round_bf16(y * _round_bf16(_sigmoid(rsel)))
        y = jnp.concatenate([y, jnp.zeros((16, DP - D), f32)], axis=1)
        y = jnp.concatenate([y, jnp.zeros((T - 16, DP), f32)], axis=0)
        y_t = y.T
        for t in range(2):
            ycol[t] = jnp.broadcast_to(y_t[0:D, t:t + 1], (D, T))
        tok_l = lax.broadcasted_iota(i32, (8, L), 1) + (NSEG - 1) * L
        sel_buf[0] = jnp.where(tok_l == i1, 1.0, 0.0)
        sel_buf[1] = jnp.where(tok_l == i2, 1.0, 0.0)

    nloop = NUNIT // 2 - 1
    dense = _interleave(mem_tasks, a_tasks(0, s0, m0), prep_dense(3, wot_u, 0))
    with _scope("p15_mix"):
        run(dense[0:2] + [select_task] + _interleave(dense[2:], moe_tasks(nloop * FPI, NFT - nloop * FPI)))

    def out_tile(s, tt, last):
        c0 = s * L + tt * T
        if not isinstance(s, int):
            c0 = pl.multiple_of(c0, T)
        o_bf = ot[:, (tt // 2) * 2 * T:(tt // 2 + 1) * 2 * T].astype(bf16)[:, (tt % 2) * T:(tt % 2 + 1) * T]
        nchunk = 4 if last else 1
        rows = D // nchunk
        for rc in range(nchunk):
            r0 = rc * rows
            attn = jnp.dot(_bf(wot_u[r0 // 2:(r0 + rows) // 2, :]), o_bf, preferred_element_type=f32)
            xn = _bf(xn_u[s * TPS + tt, r0 // 2:(r0 + rows) // 2, :]).astype(f32)
            x = x_buf[r0:r0 + rows, pl.ds(c0, T)].astype(f32)
            res = x + attn + xn
            if last:
                for t in range(2):
                    hit = sel_buf[t, 0:1, tt * T:(tt + 1) * T] > 0.5
                    res = res + jnp.where(hit, ycol[t, r0:r0 + rows, :], 0.0)
            out_buf[r0:r0 + rows, pl.ds(c0, T)] = res.astype(bf16)
        if last:
            out_copy(c0, T, NSEG - 1 + tt).start()

    def pair(ua, sa, ma, ub, sb, mbuf, extra):
        ab = []
        for x, y in zip(a_tasks(ua, sa, ma), b_tasks(ub, sb, mbuf)):
            ab.append(lambda x=x, y=y: (y(), x()))
        run(_interleave(ab, extra) if extra else ab)

    def att_body(i, c):
        u0 = 2 * i
        extra = moe_tasks(i * FPI, FPI)
        half = len(extra) // 2
        with _scope("att_body"):
            pair(u0 + 1, s1, m1, u0, s0, m0, extra[:half])
            pair(u0 + 2, s0, m0, u0 + 1, s1, m1, extra[half:])

        @pl.when((u0 + 2) % UPS == 0)
        def _():
            with _scope("outproj"):
                for tt in range(TPS):
                    out_tile(u0 // UPS, tt, False)
                for ss in range(NSEG - 1):
                    @pl.when(u0 // UPS == ss)
                    def _():
                        out_copy(ss * L, L, ss).start()
        return c

    lax.fori_loop(0, nloop, att_body, 0)

    def patch(t, idx):
        inside = idx < (NSEG - 1) * L
        c0 = pl.multiple_of(jnp.where(inside, idx // T, 0) * T, T)
        lane = lax.broadcasted_iota(i32, (1, T), 1)
        hit = (lane == idx % T) & inside
        cur = out_buf[:, pl.ds(c0, T)].astype(f32)
        out_buf[:, pl.ds(c0, T)] = (cur + jnp.where(hit, ycol[t], 0.0)).astype(bf16)
        return out_copy(c0, T, 7 + t)

    with _scope("att_tail"):
        for s in range(NSEG - 1):
            out_copy(s * L, L, s).wait()
        moe_finish()
        copy0 = patch(0, i1)
        copy0.start()
        pair(NUNIT - 1, s1, m1, NUNIT - 2, s0, m0, None)

    with _scope("att_lastb"):
        copy0.wait()
        copy1 = patch(1, i2)
        copy1.start()
        last_b = [[lambda u=u, qt=qt: stage_b(NUNIT - 1, u, qt, s1, m1) for u in range(NP)] for qt in range(4)]
        run(last_b[3])
        for qt in (2, 1, 0):
            run(last_b[qt][0:2] + [lambda qt=qt: out_tile(NSEG - 1, qt + 1, True)] + last_b[qt][2:])
        out_tile(NSEG - 1, 0, True)

    with _scope("out_wait"):
        copy1.wait()
        for tt in range(TPS):
            out_copy((NSEG - 1) * L + tt * T, T, NSEG - 1 + tt).wait()


@jax.jit
def pallas_parallel_sum__memory_aug_infini_attn__moe_arch_mod__prompt_kernel(
    A_x: jax.Array,
    A_wq: jax.Array,
    A_wk: jax.Array,
    A_wv: jax.Array,
    A_wo: jax.Array,
    A_beta: jax.Array,
    B_x: jax.Array,
    B_w_r: jax.Array,
    B_w_gate: jax.Array,
    B_w_up: jax.Array,
    B_w_down: jax.Array,
):
    del B_x
    any_spec = pl.BlockSpec(memory_space=pl.ANY)
    vmem_spec = pl.BlockSpec(memory_space=pltpu.VMEM)
    scratch = [
        pltpu.VMEM((D, SEQ), bf16),
        pltpu.VMEM((4, D, D), bf16),
        pltpu.VMEM((D, F), bf16),
        pltpu.VMEM((D, F), bf16),
        pltpu.VMEM((D, F), bf16),
        pltpu.VMEM((D, SEQ), bf16),
        pltpu.VMEM((WT_ROWS, DP), u32),
        pltpu.VMEM((D // 2, DP), u32),
        pltpu.VMEM((D // 2, DP), u32),
        pltpu.VMEM((NT, DP // 2, T), u32),
        pltpu.VMEM((NSEG * NG, TW, L), u32),
        pltpu.VMEM((NSEG * NG, L // 2, T), u32),
        pltpu.VMEM((NSEG * NG, TW, L), u32),
        pltpu.VMEM((NSEG * NG, TW, L), u32),
        pltpu.VMEM((NSEG, D // 2, L), u32),
        pltpu.VMEM((NSEG * H, 16, L), u32),
        pltpu.VMEM((NSEG, 8, L), f32),
        pltpu.VMEM((NG, T + 16, T), f32),
        pltpu.VMEM((NSEG, D, L), f32),
        pltpu.VMEM((NG, 16, T), f32),
        pltpu.VMEM((H, 8, T), f32),
        pltpu.VMEM((3, HT, T), f32),
        pltpu.VMEM((HPG, TW, T), u32),
        pltpu.VMEM((8, 32, T), i32),
        pltpu.VMEM((NP, 4, 2 * L, T), f32),
        pltpu.VMEM((NP, 4, 2, 8, T), f32),
        pltpu.VMEM((NP, 4, 2 * L, T), f32),
        pltpu.VMEM((NP, 4, 2, 8, T), f32),
        pltpu.VMEM((DP, L), f32),
        pltpu.VMEM((2, D, LNW), f32),
        pltpu.VMEM((2, 2, 8, LNW), f32),
        pltpu.VMEM((16, D), f32),
        pltpu.VMEM((8, DP), u32),
        pltpu.VMEM((FPI, 2, 16, T), f32),
        pltpu.VMEM((2, D, T), f32),
        pltpu.VMEM((2, 8, L), f32),
        pltpu.SemaphoreType.DMA((NSEM,)),
    ]
    x_t = jnp.transpose(A_x, (0, 2, 1)).reshape(D, SEQ)
    out_t = pl.pallas_call(
        _kernel,
        out_shape=jax.ShapeDtypeStruct((D, SEQ), bf16),
        in_specs=[any_spec, any_spec, any_spec, any_spec, any_spec, vmem_spec, vmem_spec,
                  any_spec, any_spec, any_spec],
        out_specs=any_spec,
        scratch_shapes=scratch,
        compiler_params=pltpu.CompilerParams(vmem_limit_bytes=110 * 1024 * 1024),
    )(x_t, A_wq, A_wk, A_wv, A_wo, A_beta, B_w_r, B_w_gate, B_w_up, B_w_down.T)
    return jnp.transpose(out_t.reshape(1, D, SEQ), (0, 2, 1))
```

```python
import contextlib

import jax
import jax.numpy as jnp
from jax import lax
from jax.experimental import pallas as pl
from jax.experimental.pallas import tpu as pltpu

bf16 = jnp.bfloat16
f32 = jnp.float32
u32 = jnp.uint32
i32 = jnp.int32

SEQ = 2048
D = 576
DP = 640
H = 32
DH = 18
NSEG = 4
L = 512
T = 128
TW = T // 2
HT = T // 2
TPS = L // T
HPG = 6
NG = 6
F = 4608
FPI = 5
NFT = F // T
NP = 4
UPS = H // (2 * NP)
NUNIT = NSEG * UPS
NT = SEQ // T
LNW = 256
VB = 8 * DH

LOG2E = 1.4426950408889634
QSCALE = (DH ** -0.5) * LOG2E
MASKVAL = -1000000000.0 * LOG2E
EPS_BF16 = 1.0013580322265625e-05
ONES_PAIR = 0x3F803F80

NT_DIMS = (((1,), (1,)), ((), ()))

WT_Q = 0
WT_K = NG * TW
WT_V = 2 * NG * TW
WT_ROWS = WT_V + D // 2

X_PIECES = ((0, LNW), (LNW, LNW), (L, L), (2 * L, L), (3 * L, L))
SEM_X = 0
SEM_W = 5
SEM_MOE = 9
SEM_OUT = 12
NSEM = 21


PROFILE_SCOPES = False
PACE = False
TAIL_BARRIERS = False
QT_ORDER = (3, 2, 1, 0)


def _scope(name):
    return jax.named_scope(name) if PROFILE_SCOPES else contextlib.nullcontext()


def _valid(g):
    return min(HPG * DH, D - g * HPG * DH)


def _rows(g):
    return -(-_valid(g) // 16) * 16


def _ewin(g):
    start = (g * HPG * DH // 16) * 16
    return start, g * HPG * DH - start, min(T, D - start)


def _bf(x):
    return pltpu.bitcast(x, bf16)


def _pack(x):
    return pltpu.bitcast(x.astype(bf16), u32)


def _round_bf16(x):
    return x.astype(bf16).astype(f32)


def _phi(t):
    return jnp.where(t > 0, t + 1.0, jnp.exp(t))


def _sigmoid(t):
    return 1.0 / (1.0 + jnp.exp(-t))


def _zero_after(v):
    bits = pltpu.bitcast(v[0:8, 0:LNW], u32)
    sixteen = jnp.uint32(16)
    bits = lax.shift_right_logical(lax.shift_right_logical(bits, sixteen), sixteen)
    return pltpu.bitcast(bits, f32) if PACE else None


def _interleave(*lists):
    items = []
    for li, tasks in enumerate(lists):
        for k, t in enumerate(tasks):
            items.append(((k + 0.5) / len(tasks), li, k, t))
    items.sort(key=lambda it: it[:3])
    return [it[3] for it in items]


def _kernel(x_hbm, wq_hbm, wk_hbm, wv_hbm, wo_hbm, beta_ref, wr_ref, wg_hbm, wu_hbm, wd_hbm,
            out_hbm,
            x_buf, w_buf, wg_buf, wu_buf, wd_buf, out_buf,
            wt_u, wtd_u, wot_u, xn_u, qs_u, k_u, pq_u, pk_u, vt_u, vwin,
            r_buf, mt_acc, am, g16, omg, mb, rowmask, smask,
            s0, m0, s1, m1, ot, xf, ln_stat, y_acc, xsel_buf, hid_buf, sems):

    def x_copy(i):
        c0, width = X_PIECES[i]
        return pltpu.make_async_copy(x_hbm.at[:, pl.ds(c0, width)], x_buf.at[:, pl.ds(c0, width)],
                                     sems.at[SEM_X + i])

    def w_copy(i):
        src = (wq_hbm, wk_hbm, wv_hbm, wo_hbm)[i]
        return pltpu.make_async_copy(src, w_buf.at[i], sems.at[SEM_W + i])

    def moe_copy(i):
        src = (wg_hbm, wu_hbm, wd_hbm)[i]
        dst = (wg_buf, wu_buf, wd_buf)[i]
        return pltpu.make_async_copy(src, dst, sems.at[SEM_MOE + i])

    def out_copy(c0, width, sem):
        return pltpu.make_async_copy(out_buf.at[:, pl.ds(c0, width)], out_hbm.at[:, pl.ds(c0, width)],
                                     sems.at[SEM_OUT + sem])

    w_copy(0).start()
    x_copy(0).start()
    x_copy(1).start()
    w_copy(1).start()
    w_copy(2).start()

    init_scope = _scope("init")
    init_scope.__enter__()
    kr = lax.broadcasted_iota(i32, (HT, T), 0)
    ql = lax.broadcasted_iota(i32, (HT, T), 1)
    mb[0] = jnp.where(ql < kr, MASKVAL, 0.0).astype(f32)
    mb[1] = jnp.where((ql >= HT) & (ql - HT < kr), MASKVAL, 0.0).astype(f32)
    mb[2] = jnp.where(ql % HT < kr, MASKVAL, 0.0).astype(f32)
    for j in range(HPG):
        rowmask[j] = jnp.where((kr >= (DH // 2) * j) & (kr < (DH // 2) * (j + 1)), u32(0xFFFFFFFF), u32(0))
    r32 = lax.broadcasted_iota(i32, (32, T), 0)
    for i in range(8):
        smask[i] = jnp.where((r32 >= 2 * i) & (r32 < 2 * i + DH), 1, 0)
    zpad = jnp.zeros(((DP - D) // 2, T), u32)
    for tt in range(NT):
        xn_u[tt, D // 2:DP // 2, :] = zpad
    ot[D:DP, :] = jnp.zeros((DP - D, L), f32)
    am[0] = jnp.zeros(am.shape[1:], f32)
    mt_acc[...] = jnp.zeros(mt_acc.shape, f32)
    g16[...] = jnp.zeros(g16.shape, f32)
    for sg in range(NSEG * NG):
        r2 = _rows(sg % NG) // 2
        qs_u[sg, r2:TW, :] = jnp.zeros((TW - r2, L), u32)
        pq_u[sg, r2:TW, :] = jnp.zeros((TW - r2, L), u32)
        pk_u[sg, r2:TW, :] = jnp.zeros((TW - r2, L), u32)

    gate = _round_bf16(_sigmoid(beta_ref[...].reshape(1, H).astype(f32)))
    for h in range(H):
        gh = jnp.broadcast_to(gate[:, h:h + 1], (1, T))
        omg[h] = jnp.broadcast_to(_round_bf16(1.0 - gh), (8, T))
        g16[h // HPG, (h % HPG):(h % HPG) + 1, :] = gh

    init_scope.__exit__(None, None, None)

    pace = [None]

    def transpose_block(i, cb):
        c1 = min((cb + 1) * T, D)
        blk = w_buf[i, :, cb * T:c1]
        if c1 - cb * T < T:
            blk = jnp.concatenate([blk, jnp.zeros((D, T - (c1 - cb * T)), bf16)], axis=1)
        blk = jnp.concatenate([blk, jnp.zeros((DP - D, T), bf16)], axis=0)
        return pltpu.bitcast(blk.T, u32)

    def prep_dense(i, dst, base):
        def task(cb):
            nrow = min(TW, D // 2 - cb * TW)
            dst[base + cb * TW:base + cb * TW + nrow, :] = transpose_block(i, cb)[0:nrow]
        return [lambda cb=cb: task(cb) for cb in range(DP // T)]

    def prep_grouped(i, base):
        def regroup(g):
            nv, nr = _valid(g) // 2, _rows(g) // 2
            src = g * HPG * DH // 2
            wt_u[base + g * TW:base + g * TW + nv, :] = wtd_u[src:src + nv, :]
            pad = jnp.zeros((nr - nv, DP), u32)
            if i == 1 and g == 0:
                wr = wr_ref[...].reshape(1, D).astype(f32)
                wr = jnp.concatenate([wr, jnp.zeros((1, DP - D), f32)], axis=1)
                bits = lax.shift_right_logical(pltpu.bitcast(wr, u32), u32(16))
                rid = lax.broadcasted_iota(i32, (nr - nv, DP), 0)
                pad = jnp.where(rid == 0, bits, pad)
            wt_u[base + g * TW + nv:base + g * TW + nr, :] = pad
        return prep_dense(i, wtd_u, 0) + [lambda g=g: regroup(g) for g in range(NG)]

    def ln_tasks(s):
        def mean_pass(b):
            c0 = s * L + b * LNW
            if not isinstance(s, int):
                c0 = pl.multiple_of(c0, LNW)
            acc = pace[0]
            for r in range(0, D, 64):
                x = x_buf[r:r + 64, pl.ds(c0, LNW)].astype(f32)
                xf[b, r:r + 64, :] = x
                part = jnp.sum(x.reshape(8, 8, LNW), axis=0)
                acc = part if acc is None else acc + part
            mean = jnp.sum(acc, axis=0, keepdims=True) / D
            ln_stat[b, 0] = jnp.broadcast_to(mean, (8, LNW))

        def var_pass(b):
            bd = b
            mean = ln_stat[b, 0][0:1]
            if pace[0] is not None:
                mean = mean + pace[0][0:1]
            acc = None
            for r in range(0, D, 96):
                xc = xf[bd, r:r + 96, :] - mean
                part = jnp.sum((xc * xc).reshape(12, 8, LNW), axis=0)
                acc = part if acc is None else acc + part
            var = jnp.sum(acc, axis=0, keepdims=True) / D
            den = _round_bf16(jnp.sqrt(_round_bf16(_round_bf16(var) + EPS_BF16)))
            ln_stat[b, 1] = jnp.broadcast_to(1.0 / den, (8, LNW))
            ln_stat[b, 0] = jnp.broadcast_to(_round_bf16(mean), (8, LNW))

        def norm_pass(b, half):
            bd = b
            mean_b = ln_stat[b, 0][0:1]
            if pace[0] is not None:
                mean_b = mean_b + pace[0][0:1]
            inv = ln_stat[b, 1][0:1]
            for r in range(half * (D // 2), (half + 1) * (D // 2), 48):
                xn = _pack(_round_bf16(xf[bd, r:r + 48, :] - mean_b) * inv)
                for t in range(LNW // T):
                    tt = b * (LNW // T) + t
                    xn_u[s * TPS + tt, r // 2:r // 2 + 24, :] = xn[:, t * T:(t + 1) * T]

        tasks = []
        for b in range(L // LNW):
            tasks += [lambda b=b: mean_pass(b), lambda b=b: var_pass(b),
                      lambda b=b: norm_pass(b, 0), lambda b=b: norm_pass(b, 1)]
        return tasks

    def load_xs(s, t0, t1):
        return jnp.concatenate([_bf(xn_u[s * TPS + tt]) for tt in range(t0, t1)], axis=1)

    def q_task(s, g, t0=0, t1=TPS):
        nr = _rows(g) // 2
        w = _bf(wt_u[WT_Q + g * TW:WT_Q + g * TW + nr, :])
        q = jnp.dot(w, load_xs(s, t0, t1), preferred_element_type=f32)
        pace[0] = _zero_after(q)
        qp = _pack(q * QSCALE)
        qrot = jnp.concatenate([pltpu.roll(qp[:, t * T:(t + 1) * T], HT, 1) for t in range(t1 - t0)], axis=1)
        rid = lax.broadcasted_iota(i32, qp.shape, 0)
        even = ((rid // (DH // 2)) % 2) == 0
        qs_u[s * NG + g, 0:nr, t0 * T:t1 * T] = jnp.where(even, qrot, qp)
        pq_u[s * NG + g, 0:nr, t0 * T:t1 * T] = _pack(_phi(_round_bf16(q)))

    def k_task(s, g):
        nr = _rows(g)
        w = _bf(wt_u[WT_K + g * TW:WT_K + g * TW + nr // 2, :])
        k = jnp.dot(w, load_xs(s, 0, TPS), preferred_element_type=f32)
        pace[0] = _zero_after(k)
        if g == 0:
            r_buf[s] = jnp.broadcast_to(k[_valid(0):_valid(0) + 1, :], (8, L))
        kp = _pack(k)
        pk_u[s * NG + g, 0:nr // 2, :] = _pack(_phi(_round_bf16(k)))
        kfull = _bf(jnp.concatenate([kp, jnp.zeros(((T - nr) // 2, L), u32)], axis=0))
        k_u[s * NG + g] = pltpu.bitcast(kfull.T, u32)

    def v_task(s, b):
        w = _bf(wt_u[WT_V + b * (VB // 2):WT_V + (b + 1) * (VB // 2), :])
        v = jnp.dot(w, load_xs(s, 0, TPS), preferred_element_type=f32)
        pace[0] = _zero_after(v)
        v = _pack(v)
        vt_u[s, b * (VB // 2):(b + 1) * (VB // 2), :] = v
        sub = lax.broadcasted_iota(i32, (16, L), 0)
        for hh in range(8):
            w8 = (9 * hh) // 8
            ones_row = 0 if 2 * hh == 14 else 15
            vwin[s * H + 8 * b + hh] = jnp.where(sub == ones_row, u32(ONES_PAIR), v[8 * w8:8 * w8 + 16, :])

    def q_tasks(s, t0=0, t1=TPS):
        return [lambda g=g: q_task(s, g, t0, t1) for g in range(NG)]

    def k_tasks(s):
        return [lambda g=g: k_task(s, g) for g in range(NG)]

    def v_tasks(s):
        return [lambda b=b: v_task(s, b) for b in range(D // VB)]

    def run(tasks):
        for t in tasks:
            t()

    ln0 = ln_tasks(0)
    prep_q = prep_grouped(0, WT_Q)
    with _scope("p1_wait_wq"):
        w_copy(0).wait()
    with _scope("p1_prep_q"):
        run(prep_q[0:3])
        x_copy(0).wait()
    for i in range(2, len(X_PIECES)):
        x_copy(i).start()
    w_copy(3).start()
    for i in range(3):
        moe_copy(i).start()
    with _scope("p1_ln0a"):
        run(_interleave(prep_q[3:], ln0[0:4]))
        x_copy(1).wait()
    with _scope("p1_q0a"):
        run(_interleave(q_tasks(0, 0, 2), ln0[4:8]))
        w_copy(1).wait()
    with _scope("p1_q0b"):
        run(_interleave(q_tasks(0, 2, 4), prep_grouped(1, WT_K)))
        w_copy(2).wait()
    with _scope("p1_k0"):
        run(_interleave(k_tasks(0), prep_dense(2, wt_u, WT_V)))
        x_copy(2).wait()
    with _scope("p1_v0"):
        run(_interleave(v_tasks(0), ln_tasks(1)))

    def seg_body(s, c):
        for ss in range(2, NSEG):
            @pl.when(s + 1 == ss)
            def _():
                x_copy(ss + 1).wait()
        nxt = jnp.minimum(s + 1, NSEG - 1)
        pace[0] = None
        with _scope("p1_seg"):
            run(_interleave(q_tasks(s) + k_tasks(s) + v_tasks(s), ln_tasks(nxt)))
        return c

    lax.fori_loop(1, NSEG, seg_body, 0)

    row64 = lax.broadcasted_iota(i32, (TW, T), 0)
    lane64 = lax.broadcasted_iota(i32, (TW, T), 1)
    row32 = lax.broadcasted_iota(i32, (32, T), 0)
    lane32 = lax.broadcasted_iota(i32, (32, T), 1)
    lane1 = lax.broadcasted_iota(i32, (1, T), 1)
    lane8 = lax.broadcasted_iota(i32, (8, T), 1)

    def stage_a(unit, u, qt, s_ref, m_ref):
        s = unit // UPS
        pi = (unit % UPS) * NP + u
        g = pi // (HPG // 2)
        j = 2 * (pi - (HPG // 2) * g)
        sg = s * NG + g
        n = T * (qt + 1)
        qw = qs_u[sg, :, qt * T:(qt + 1) * T]
        w_a = qw & rowmask[j]
        w_b = qw & rowmask[j + 1]
        w_ab = _bf(jnp.where(lane64 < HT, w_a, w_b))

        def colmax8(v):
            return jnp.max(v.reshape(v.shape[0] // 8, 8, T), axis=0)

        maxes = []
        for hd, w in enumerate((_bf(w_a), _bf(w_b))):
            m8 = None
            for c in range(qt):
                kc = _bf(k_u[sg, c * TW:(c + 1) * TW, :])
                sc = jnp.dot(kc, w, preferred_element_type=f32)
                s_ref[u, qt, hd * L + c * T:hd * L + (c + 1) * T, :] = sc
                m8 = colmax8(sc) if m8 is None else jnp.maximum(m8, colmax8(sc))
            kc = _bf(k_u[sg, qt * TW:qt * TW + TW // 2, :])
            sc = jnp.dot(kc, w, preferred_element_type=f32) + mb[1 - hd]
            s_ref[u, qt, hd * L + qt * T:hd * L + qt * T + HT, :] = sc
            m8 = colmax8(sc) if m8 is None else jnp.maximum(m8, colmax8(sc))
            maxes.append(m8)
        kc = _bf(k_u[sg, qt * TW + TW // 2:(qt + 1) * TW, :])
        sc = jnp.dot(kc, w_ab, preferred_element_type=f32) + mb[2]
        s_ref[u, qt, n - HT:n, :] = sc
        mab = colmax8(sc)
        m_a = jnp.where(lane8 < HT, jnp.maximum(maxes[0], mab), maxes[0])
        m_b = jnp.where(lane8 >= HT, jnp.maximum(maxes[1], mab), maxes[1])
        m_ref[u, qt, 0] = jnp.broadcast_to(jnp.max(m_a, axis=0, keepdims=True), (8, T))
        m_ref[u, qt, 1] = jnp.broadcast_to(jnp.max(m_b, axis=0, keepdims=True), (8, T))

    def stage_b(unit, u, qt, s_ref, m_ref):
        s = unit // UPS
        pi = (unit % UPS) * NP + u
        n = T * (qt + 1)
        m_a = m_ref[u, qt, 0][0:1]
        m_b = m_ref[u, qt, 1][0:1]
        p_ab = jnp.exp2(s_ref[u, qt, n - HT:n, :] - jnp.where(lane1 < HT, m_a, m_b))
        for hd, m in enumerate((m_a, m_b)):
            h = 2 * pi + hd
            p = jnp.exp2(s_ref[u, qt, hd * L:hd * L + n - HT, :] - m)
            keep = (lane64 < HT) if hd == 0 else (lane64 >= HT)
            p = jnp.concatenate([p, jnp.where(keep, p_ab, 0.0)], axis=0).astype(bf16)
            w8 = (9 * h) // 8
            off = DH * h - 16 * w8
            o = jnp.dot(_bf(vwin[s * H + h, :, 0:n]), p, preferred_element_type=f32)
            den = jnp.where(off == 14, o[0:1], o[31:32])
            o = o * (omg[h][0:1] / den)
            if hd == 0:
                o = pltpu.roll(o, HT, 1)
            r1 = pl.multiple_of(16 * w8, 16)
            res = am[s, pl.ds(r1, 32), qt * T:(qt + 1) * T] + o
            pltpu.store(ot.at[pl.ds(r1, 32), qt * T:(qt + 1) * T], res, mask=smask[off // 2] != 0)

    def a_tasks(unit, s_ref, m_ref):
        return [lambda u=u, qt=qt: stage_a(unit, u, qt, s_ref, m_ref) for u in range(NP) for qt in QT_ORDER]

    def b_tasks(unit, s_ref, m_ref):
        return [lambda u=u, qt=qt: stage_b(unit, u, qt, s_ref, m_ref) for u in range(NP) for qt in QT_ORDER]

    ones16 = jnp.where(lax.broadcasted_iota(i32, (8, L), 0) == 0, u32(0x3F80), u32(0))

    def mem_task(s, g):
        es, eoff, ne = _ewin(g)
        nv = _valid(g)
        lhs = _bf(jnp.concatenate([vt_u[s, es // 2:(es + ne) // 2, :], ones16], axis=0))
        upd = lax.dot_general(lhs, _bf(pk_u[s * NG + g]), NT_DIMS, preferred_element_type=f32)
        mt = mt_acc[g, 0:ne + 16, :] + upd
        mt_acc[g, 0:ne + 16, :] = mt
        e_loc = lax.broadcasted_iota(i32, (ne, T), 0) - eoff
        d_id = lax.broadcasted_iota(i32, (ne, T), 1)
        same_head = (e_loc >= 0) & (e_loc < nv) & (d_id < nv) & ((e_loc // DH) == (d_id // DH))
        j16 = lax.broadcasted_iota(i32, (16, T), 0)
        d16 = lax.broadcasted_iota(i32, (16, T), 1)
        z_mask = ((d16 // DH) == j16) & (d16 < nv)
        lm = jnp.concatenate(
            [jnp.where(same_head, mt[0:ne], 0.0),
             jnp.where(z_mask, jnp.broadcast_to(mt[ne:ne + 1, :], (16, T)), 0.0)], axis=0)
        nd = jnp.dot(lm.astype(bf16), _bf(pq_u[(s + 1) * NG + g]), preferred_element_type=f32)
        scale = jnp.broadcast_to(g16[g][:, 0:1], (16, L)) / (nd[ne:ne + 16, :] + 1e-6)
        r8 = lax.broadcasted_iota(i32, (8, L), 0)
        for b in range(ne // 8):
            lo, hi = 8 * b - eoff, 8 * b + 7 - eoff
            if hi < 0 or lo >= nv:
                continue
            j1, j2 = max(lo, 0) // DH, min(hi, nv - 1) // DH
            sc = jnp.broadcast_to(scale[j1:j1 + 1, :], (8, L))
            if j2 != j1:
                sc = jnp.where(r8 < DH * j2 - lo, sc, jnp.broadcast_to(scale[j2:j2 + 1, :], (8, L)))
            val = nd[8 * b:8 * b + 8, :] * sc
            dst = am.at[s + 1, es + 8 * b:es + 8 * b + 8, :]
            if lo >= 0 and hi < nv:
                dst[...] = val
            else:
                pltpu.store(dst, val, mask=(r8 + lo >= 0) & (r8 + lo < nv))

    mem_tasks = [lambda s=s, g=g: mem_task(s, g) for s in range(NSEG - 1) for g in range(NG)]

    w_copy(3).wait()
    for i in range(3):
        moe_copy(i).wait()
    rr = jnp.concatenate([r_buf[s][0:1, :] for s in range(NSEG)], axis=0)
    rr = _round_bf16(rr)
    tok = lax.broadcasted_iota(i32, (NSEG, L), 0) * L + lax.broadcasted_iota(i32, (NSEG, L), 1)
    m1v = jnp.max(rr)
    i1 = jnp.min(jnp.where(rr == m1v, tok, SEQ))
    rr2 = jnp.where(tok == i1, -jnp.inf, rr)
    m2v = jnp.max(rr2)
    i2 = jnp.min(jnp.where(rr2 == m2v, tok, SEQ))
    i1 = jnp.clip(i1, 0, SEQ - 1)
    i2 = jnp.clip(i2, 0, SEQ - 1)

    row16 = lax.broadcasted_iota(i32, (16, T), 0)
    lane16 = lax.broadcasted_iota(i32, (16, T), 1)

    def token_rows(i, slot):
        onehot = jnp.where((row16 == slot) & (lane16 == i % T), 1.0, 0.0).astype(bf16)
        return lax.dot_general(onehot, _bf(xn_u[i // T]), NT_DIMS, preferred_element_type=f32)

    def select_task():
        xsel_buf[...] = _pack(token_rows(i1, 0) + token_rows(i2, 1))
        y_acc[...] = jnp.zeros(y_acc.shape, f32)

    def fcols(ft):
        return pl.ds(ft * T if isinstance(ft, int) else pl.multiple_of(ft * T, T), T)

    def moe_up_task(ft, k, which):
        xsel = _bf(xsel_buf[:, 0:D])
        w_ref = (wg_buf, wu_buf)[which]
        hid_buf[k, which] = jnp.dot(xsel, w_ref[:, fcols(ft)], preferred_element_type=f32)

    def moe_down_task(ft, k):
        gt = _round_bf16(hid_buf[k, 0])
        up = _round_bf16(hid_buf[k, 1])
        hid = (_round_bf16(gt * _sigmoid(gt)) * up).astype(bf16)
        y_acc[...] += lax.dot_general(hid, wd_buf[:, fcols(ft)], NT_DIMS, preferred_element_type=f32)

    def moe_tasks(ft0, count):
        ups = [lambda k=k, w=w: moe_up_task(ft0 + k, k, w) for k in range(count) for w in range(2)]
        downs = [lambda k=k: moe_down_task(ft0 + k, k) for k in range(count)]
        return ups + downs

    def moe_finish():
        y = _round_bf16(y_acc[...])
        rsel = jnp.where(lax.broadcasted_iota(i32, (16, 1), 0) == 0, m1v, m2v)
        y = _round_bf16(y * _round_bf16(_sigmoid(rsel)))
        y = jnp.concatenate([y, jnp.zeros((16, DP - D), f32)], axis=1)
        y = jnp.concatenate([jnp.zeros((HT, DP), f32), y, jnp.zeros((T - HT - 16, DP), f32)], axis=0)
        y_t = jnp.concatenate([y.T[0:D], jnp.zeros((D, T), f32)], axis=1)
        y_u = _pack(y_t)[:, 0:T]
        lane = lax.broadcasted_iota(i32, (D // 2, T), 1)
        wot_u[:, DP - T:DP] = jnp.where(lane < HT, wot_u[:, DP - T:DP], y_u)
        tok_l = lax.broadcasted_iota(i32, (8, L), 1) + (NSEG - 1) * L
        rid = lax.broadcasted_iota(i32, (8, L), 0)
        ot[D:D + 8, :] = jnp.where(((rid == 0) & (tok_l == i1)) | ((rid == 1) & (tok_l == i2)), 1.0, 0.0)

    nloop = NUNIT // 2 - 1
    dense = _interleave(mem_tasks, a_tasks(0, s0, m0), prep_dense(3, wot_u, 0))
    with _scope("p15_mix"):
        run(dense[0:2] + [select_task] + _interleave(dense[2:], moe_tasks(nloop * FPI, NFT - nloop * FPI)))

    def out_tile(s, tt, last):
        c0 = s * L + tt * T
        if not isinstance(s, int):
            c0 = pl.multiple_of(c0, T)
        o_bf = ot[:, (tt // 2) * 2 * T:(tt // 2 + 1) * 2 * T].astype(bf16)[:, (tt % 2) * T:(tt % 2 + 1) * T]
        nchunk = 4 if last else 1
        rows = D // nchunk
        for rc in range(nchunk):
            r0 = rc * rows
            attn = jnp.dot(_bf(wot_u[r0 // 2:(r0 + rows) // 2, :]), o_bf, preferred_element_type=f32)
            xn = _bf(xn_u[s * TPS + tt, r0 // 2:(r0 + rows) // 2, :]).astype(f32)
            x = x_buf[r0:r0 + rows, pl.ds(c0, T)].astype(f32)
            res = x + attn + xn
            out_buf[r0:r0 + rows, pl.ds(c0, T)] = res.astype(bf16)

    def pair(ua, sa, ma, ub, sb, mbuf, extra):
        ab = []
        for x, y in zip(a_tasks(ua, sa, ma), b_tasks(ub, sb, mbuf)):
            ab.append(lambda x=x, y=y: (y(), x()))
        run(_interleave(ab, extra) if extra else ab)

    def att_body(i, c):
        u0 = 2 * i
        extra = moe_tasks(i * FPI, FPI)
        half = len(extra) // 2
        with _scope("att_body"):
            pair(u0 + 1, s1, m1, u0, s0, m0, extra[:half])
            pair(u0 + 2, s0, m0, u0 + 1, s1, m1, extra[half:])

        @pl.when((u0 + 2) % UPS == 0)
        def _():
            with _scope("outproj"):
                for tt in range(TPS):
                    out_tile(u0 // UPS, tt, False)
                for ss in range(NSEG - 1):
                    @pl.when(u0 // UPS == ss)
                    def _():
                        out_copy(ss * L, L, ss).start()
        return c

    lax.fori_loop(0, nloop, att_body, 0)

    npatch = (NSEG - 1) * TPS

    def patch_tile(idx):
        return jnp.where(idx < npatch * T, idx // T, 0)

    tile0 = patch_tile(i1)
    tile1 = patch_tile(i2)
    tile1 = jnp.where(tile1 == tile0, (tile0 + 1) % npatch, tile1)

    def patch(tile):
        c0 = pl.multiple_of(tile * T, T)
        rid = lax.broadcasted_iota(i32, (T, T), 0)
        tok_l = lax.broadcasted_iota(i32, (T, T), 1) + c0
        hit = ((rid == HT) & (tok_l == i1)) | ((rid == HT + 1) & (tok_l == i2))
        onehot = jnp.where(hit, 1.0, 0.0).astype(bf16)
        for rc in range(4):
            r0, r1 = rc * (D // 4), (rc + 1) * (D // 4)
            upd = jnp.dot(_bf(wot_u[r0 // 2:r1 // 2, DP - T:DP]), onehot, preferred_element_type=f32)
            cur = out_buf[r0:r1, pl.ds(c0, T)].astype(f32)
            out_buf[r0:r1, pl.ds(c0, T)] = (cur + upd).astype(bf16)

    patch_copies = [out_copy(pl.multiple_of(tile0 * T, T), T, 7), out_copy(pl.multiple_of(tile1 * T, T), T, 8)]
    last_copies = [out_copy((NSEG - 1) * L + tt * T, T, NSEG - 1 + tt) for tt in range(TPS)]

    def a_last(qt):
        return [lambda u=u: stage_a(NUNIT - 1, u, qt, s1, m1) for u in range(NP)]

    def b_prev(qt):
        return [lambda u=u: stage_b(NUNIT - 2, u, qt, s0, m0) for u in range(NP)]

    def b_last(qt):
        return [lambda u=u: stage_b(NUNIT - 1, u, qt, s1, m1) for u in range(NP)]

    def o_last(tt):
        return [lambda: out_tile(NSEG - 1, tt, True)]

    def region(name, fn):
        if TAIL_BARRIERS:
            @pl.when(i1 >= 0)
            def _():
                with _scope(name):
                    fn()
        else:
            with _scope(name):
                fn()

    def tail_1():
        run(_interleave(b_prev(3), a_last(3)))
        moe_finish()
        run(_interleave(b_prev(2), a_last(2), b_last(3)))
        patch(tile0)
        patch(tile1)
        run(_interleave(b_prev(1), a_last(1), b_last(2), o_last(3)))
        for cp in patch_copies + [last_copies[3]]:
            cp.start()

    def tail_2():
        run(_interleave(b_prev(0), a_last(0), b_last(1), o_last(2)))
        run(_interleave(b_last(0), o_last(1)))
        last_copies[2].start()
        last_copies[1].start()

    def tail_3():
        out_tile(NSEG - 1, 0, True)
        last_copies[0].start()

    for s in range(NSEG - 1):
        out_copy(s * L, L, s).wait()
    region("tail_1", tail_1)
    region("tail_2", tail_2)
    region("tail_3", tail_3)

    with _scope("out_wait"):
        for cp in patch_copies + last_copies:
            cp.wait()


@jax.jit
def pallas_parallel_sum__memory_aug_infini_attn__moe_arch_mod__prompt_kernel(
    A_x: jax.Array,
    A_wq: jax.Array,
    A_wk: jax.Array,
    A_wv: jax.Array,
    A_wo: jax.Array,
    A_beta: jax.Array,
    B_x: jax.Array,
    B_w_r: jax.Array,
    B_w_gate: jax.Array,
    B_w_up: jax.Array,
    B_w_down: jax.Array,
):
    del B_x
    any_spec = pl.BlockSpec(memory_space=pl.ANY)
    vmem_spec = pl.BlockSpec(memory_space=pltpu.VMEM)
    scratch = [
        pltpu.VMEM((D, SEQ), bf16),
        pltpu.VMEM((4, D, D), bf16),
        pltpu.VMEM((D, F), bf16),
        pltpu.VMEM((D, F), bf16),
        pltpu.VMEM((D, F), bf16),
        pltpu.VMEM((D, SEQ), bf16),
        pltpu.VMEM((WT_ROWS, DP), u32),
        pltpu.VMEM((D // 2, DP), u32),
        pltpu.VMEM((D // 2, DP), u32),
        pltpu.VMEM((NT, DP // 2, T), u32),
        pltpu.VMEM((NSEG * NG, TW, L), u32),
        pltpu.VMEM((NSEG * NG, L // 2, T), u32),
        pltpu.VMEM((NSEG * NG, TW, L), u32),
        pltpu.VMEM((NSEG * NG, TW, L), u32),
        pltpu.VMEM((NSEG, D // 2, L), u32),
        pltpu.VMEM((NSEG * H, 16, L), u32),
        pltpu.VMEM((NSEG, 8, L), f32),
        pltpu.VMEM((NG, T + 16, T), f32),
        pltpu.VMEM((NSEG, D, L), f32),
        pltpu.VMEM((NG, 16, T), f32),
        pltpu.VMEM((H, 8, T), f32),
        pltpu.VMEM((3, HT, T), f32),
        pltpu.VMEM((HPG, TW, T), u32),
        pltpu.VMEM((8, 32, T), i32),
        pltpu.VMEM((NP, 4, 2 * L, T), f32),
        pltpu.VMEM((NP, 4, 2, 8, T), f32),
        pltpu.VMEM((NP, 4, 2 * L, T), f32),
        pltpu.VMEM((NP, 4, 2, 8, T), f32),
        pltpu.VMEM((DP, L), f32),
        pltpu.VMEM((2, D, LNW), f32),
        pltpu.VMEM((2, 2, 8, LNW), f32),
        pltpu.VMEM((16, D), f32),
        pltpu.VMEM((8, DP), u32),
        pltpu.VMEM((FPI, 2, 16, T), f32),
        pltpu.SemaphoreType.DMA((NSEM,)),
    ]
    x_t = jnp.transpose(A_x, (0, 2, 1)).reshape(D, SEQ)
    out_t = pl.pallas_call(
        _kernel,
        out_shape=jax.ShapeDtypeStruct((D, SEQ), bf16),
        in_specs=[any_spec, any_spec, any_spec, any_spec, any_spec, vmem_spec, vmem_spec,
                  any_spec, any_spec, any_spec],
        out_specs=any_spec,
        scratch_shapes=scratch,
        compiler_params=pltpu.CompilerParams(vmem_limit_bytes=110 * 1024 * 1024),
    )(x_t, A_wq, A_wk, A_wv, A_wo, A_beta, B_w_r, B_w_gate, B_w_up, B_w_down.T)
    return jnp.transpose(out_t.reshape(1, D, SEQ), (0, 2, 1))
```

```python
import contextlib

import jax
import jax.numpy as jnp
from jax import lax
from jax.experimental import pallas as pl
from jax.experimental.pallas import tpu as pltpu

bf16 = jnp.bfloat16
f32 = jnp.float32
u32 = jnp.uint32
i32 = jnp.int32

SEQ = 2048
D = 576
DP = 640
H = 32
DH = 18
NSEG = 4
L = 512
T = 128
TW = T // 2
HT = T // 2
TPS = L // T
HPG = 6
NG = 6
F = 4608
FPI = 12
FPB = 3
NFT = F // T
NP = 4
UPS = H // (2 * NP)
NUNIT = NSEG * UPS
NT = SEQ // T
LNW = 256
VB = 8 * DH

LOG2E = 1.4426950408889634
QSCALE = (DH ** -0.5) * LOG2E
MASKVAL = -1000000000.0 * LOG2E
EPS_BF16 = 1.0013580322265625e-05
ONES_PAIR = 0x3F803F80

NT_DIMS = (((1,), (1,)), ((), ()))

WT_Q = 0
WT_K = NG * TW
WT_V = 2 * NG * TW
WT_ROWS = WT_V + D // 2

X_PIECES = ((0, LNW), (LNW, LNW), (L, L), (2 * L, L), (3 * L, L))
SEM_X = 0
SEM_W = 5
SEM_MOE = 9
SEM_OUT = 12
NSEM = 21


PROFILE_SCOPES = False
PACE = False
TAIL_BARRIERS = False
QT_ORDER = (3, 2, 1, 0)


def _scope(name):
    return jax.named_scope(name) if PROFILE_SCOPES else contextlib.nullcontext()


def _valid(g):
    return min(HPG * DH, D - g * HPG * DH)


def _rows(g):
    return -(-_valid(g) // 16) * 16


def _ewin(g):
    start = (g * HPG * DH // 16) * 16
    return start, g * HPG * DH - start, min(T, D - start)


def _bf(x):
    return pltpu.bitcast(x, bf16)


def _pack(x):
    return pltpu.bitcast(x.astype(bf16), u32)


def _round_bf16(x):
    return x.astype(bf16).astype(f32)


def _phi(t):
    return jnp.where(t > 0, t + 1.0, jnp.exp(t))


def _sigmoid(t):
    return 1.0 / (1.0 + jnp.exp(-t))


def _zero_after(v):
    bits = pltpu.bitcast(v[0:8, 0:LNW], u32)
    sixteen = jnp.uint32(16)
    bits = lax.shift_right_logical(lax.shift_right_logical(bits, sixteen), sixteen)
    return pltpu.bitcast(bits, f32) if PACE else None


def _interleave(*lists):
    items = []
    for li, tasks in enumerate(lists):
        for k, t in enumerate(tasks):
            items.append(((k + 0.5) / len(tasks), li, k, t))
    items.sort(key=lambda it: it[:3])
    return [it[3] for it in items]


def _kernel(x_hbm, wq_hbm, wk_hbm, wv_hbm, wo_hbm, beta_ref, wr_ref, wg_hbm, wu_hbm, wd_hbm,
            out_hbm,
            x_buf, w_buf, wg_buf, wu_buf, wd_buf, out_buf,
            wt_u, wtd_u, wot_u, xn_u, qs_u, k_u, pq_u, pk_u, vt_u, vwin,
            r_buf, mt_acc, am, g16, omg, mb, rowmask, smask,
            s0, m0, s1, m1, ot, xf, ln_stat, y_acc, xsel_buf, hid_buf, sems):

    def x_copy(i):
        c0, width = X_PIECES[i]
        return pltpu.make_async_copy(x_hbm.at[:, pl.ds(c0, width)], x_buf.at[:, pl.ds(c0, width)],
                                     sems.at[SEM_X + i])

    def w_copy(i):
        src = (wq_hbm, wk_hbm, wv_hbm, wo_hbm)[i]
        return pltpu.make_async_copy(src, w_buf.at[i], sems.at[SEM_W + i])

    def moe_copy(i):
        src = (wg_hbm, wu_hbm, wd_hbm)[i]
        dst = (wg_buf, wu_buf, wd_buf)[i]
        return pltpu.make_async_copy(src, dst, sems.at[SEM_MOE + i])

    def out_copy(c0, width, sem):
        return pltpu.make_async_copy(out_buf.at[:, pl.ds(c0, width)], out_hbm.at[:, pl.ds(c0, width)],
                                     sems.at[SEM_OUT + sem])

    w_copy(0).start()
    x_copy(0).start()
    x_copy(1).start()
    w_copy(1).start()
    w_copy(2).start()

    init_scope = _scope("init")
    init_scope.__enter__()
    kr = lax.broadcasted_iota(i32, (HT, T), 0)
    ql = lax.broadcasted_iota(i32, (HT, T), 1)
    mb[0] = jnp.where(ql < kr, MASKVAL, 0.0).astype(f32)
    mb[1] = jnp.where((ql >= HT) & (ql - HT < kr), MASKVAL, 0.0).astype(f32)
    mb[2] = jnp.where(ql % HT < kr, MASKVAL, 0.0).astype(f32)
    for j in range(HPG):
        rowmask[j] = jnp.where((kr >= (DH // 2) * j) & (kr < (DH // 2) * (j + 1)), u32(0xFFFFFFFF), u32(0))
    r32 = lax.broadcasted_iota(i32, (32, T), 0)
    for i in range(8):
        smask[i] = jnp.where((r32 >= 2 * i) & (r32 < 2 * i + DH), 1, 0)
    zpad = jnp.zeros(((DP - D) // 2, T), u32)
    for tt in range(NT):
        xn_u[tt, D // 2:DP // 2, :] = zpad
    ot[D:DP, :] = jnp.zeros((DP - D, L), f32)
    am[0] = jnp.zeros(am.shape[1:], f32)
    mt_acc[...] = jnp.zeros(mt_acc.shape, f32)
    g16[...] = jnp.zeros(g16.shape, f32)
    for sg in range(NSEG * NG):
        r2 = _rows(sg % NG) // 2
        qs_u[sg, r2:TW, :] = jnp.zeros((TW - r2, L), u32)
        pq_u[sg, r2:TW, :] = jnp.zeros((TW - r2, L), u32)
        pk_u[sg, r2:TW, :] = jnp.zeros((TW - r2, L), u32)

    gate = _round_bf16(_sigmoid(beta_ref[...].reshape(1, H).astype(f32)))
    for h in range(H):
        gh = jnp.broadcast_to(gate[:, h:h + 1], (1, T))
        omg[h] = jnp.broadcast_to(_round_bf16(1.0 - gh), (8, T))
        g16[h // HPG, (h % HPG):(h % HPG) + 1, :] = gh

    init_scope.__exit__(None, None, None)

    pace = [None]

    def transpose_block(i, cb):
        c1 = min((cb + 1) * T, D)
        blk = w_buf[i, :, cb * T:c1]
        if c1 - cb * T < T:
            blk = jnp.concatenate([blk, jnp.zeros((D, T - (c1 - cb * T)), bf16)], axis=1)
        blk = jnp.concatenate([blk, jnp.zeros((DP - D, T), bf16)], axis=0)
        return pltpu.bitcast(blk.T, u32)

    def prep_dense(i, dst, base):
        def task(cb):
            nrow = min(TW, D // 2 - cb * TW)
            dst[base + cb * TW:base + cb * TW + nrow, :] = transpose_block(i, cb)[0:nrow]
        return [lambda cb=cb: task(cb) for cb in range(DP // T)]

    def prep_grouped(i, base):
        def regroup(g):
            nv, nr = _valid(g) // 2, _rows(g) // 2
            src = g * HPG * DH // 2
            wt_u[base + g * TW:base + g * TW + nv, :] = wtd_u[src:src + nv, :]
            pad = jnp.zeros((nr - nv, DP), u32)
            if i == 1 and g == 0:
                wr = wr_ref[...].reshape(1, D).astype(f32)
                wr = jnp.concatenate([wr, jnp.zeros((1, DP - D), f32)], axis=1)
                bits = lax.shift_right_logical(pltpu.bitcast(wr, u32), u32(16))
                rid = lax.broadcasted_iota(i32, (nr - nv, DP), 0)
                pad = jnp.where(rid == 0, bits, pad)
            wt_u[base + g * TW + nv:base + g * TW + nr, :] = pad
        return prep_dense(i, wtd_u, 0) + [lambda g=g: regroup(g) for g in range(NG)]

    def ln_tasks(s):
        def mean_pass(b):
            c0 = s * L + b * LNW
            if not isinstance(s, int):
                c0 = pl.multiple_of(c0, LNW)
            acc = pace[0]
            for r in range(0, D, 64):
                x = x_buf[r:r + 64, pl.ds(c0, LNW)].astype(f32)
                xf[b, r:r + 64, :] = x
                part = jnp.sum(x.reshape(8, 8, LNW), axis=0)
                acc = part if acc is None else acc + part
            mean = jnp.sum(acc, axis=0, keepdims=True) / D
            ln_stat[b, 0] = jnp.broadcast_to(mean, (8, LNW))

        def var_pass(b):
            bd = b
            mean = ln_stat[b, 0][0:1]
            if pace[0] is not None:
                mean = mean + pace[0][0:1]
            acc = None
            for r in range(0, D, 96):
                xc = xf[bd, r:r + 96, :] - mean
                part = jnp.sum((xc * xc).reshape(12, 8, LNW), axis=0)
                acc = part if acc is None else acc + part
            var = jnp.sum(acc, axis=0, keepdims=True) / D
            den = _round_bf16(jnp.sqrt(_round_bf16(_round_bf16(var) + EPS_BF16)))
            ln_stat[b, 1] = jnp.broadcast_to(1.0 / den, (8, LNW))
            ln_stat[b, 0] = jnp.broadcast_to(_round_bf16(mean), (8, LNW))

        def norm_pass(b, half):
            bd = b
            mean_b = ln_stat[b, 0][0:1]
            if pace[0] is not None:
                mean_b = mean_b + pace[0][0:1]
            inv = ln_stat[b, 1][0:1]
            for r in range(half * (D // 2), (half + 1) * (D // 2), 48):
                xn = _pack(_round_bf16(xf[bd, r:r + 48, :] - mean_b) * inv)
                for t in range(LNW // T):
                    tt = b * (LNW // T) + t
                    xn_u[s * TPS + tt, r // 2:r // 2 + 24, :] = xn[:, t * T:(t + 1) * T]

        tasks = []
        for b in range(L // LNW):
            tasks += [lambda b=b: mean_pass(b), lambda b=b: var_pass(b),
                      lambda b=b: norm_pass(b, 0), lambda b=b: norm_pass(b, 1)]
        return tasks

    def load_xs(s, t0, t1):
        return jnp.concatenate([_bf(xn_u[s * TPS + tt]) for tt in range(t0, t1)], axis=1)

    def q_task(s, g, t0=0, t1=TPS):
        nr = _rows(g) // 2
        w = _bf(wt_u[WT_Q + g * TW:WT_Q + g * TW + nr, :])
        q = jnp.dot(w, load_xs(s, t0, t1), preferred_element_type=f32)
        pace[0] = _zero_after(q)
        qp = _pack(q * QSCALE)
        qrot = jnp.concatenate([pltpu.roll(qp[:, t * T:(t + 1) * T], HT, 1) for t in range(t1 - t0)], axis=1)
        rid = lax.broadcasted_iota(i32, qp.shape, 0)
        even = ((rid // (DH // 2)) % 2) == 0
        qs_u[s * NG + g, 0:nr, t0 * T:t1 * T] = jnp.where(even, qrot, qp)
        pq_u[s * NG + g, 0:nr, t0 * T:t1 * T] = _pack(_phi(_round_bf16(q)))

    def k_task(s, g):
        nr = _rows(g)
        w = _bf(wt_u[WT_K + g * TW:WT_K + g * TW + nr // 2, :])
        k = jnp.dot(w, load_xs(s, 0, TPS), preferred_element_type=f32)
        pace[0] = _zero_after(k)
        if g == 0:
            r_buf[s] = jnp.broadcast_to(k[_valid(0):_valid(0) + 1, :], (8, L))
        kp = _pack(k)
        pk_u[s * NG + g, 0:nr // 2, :] = _pack(_phi(_round_bf16(k)))
        kfull = _bf(jnp.concatenate([kp, jnp.zeros(((T - nr) // 2, L), u32)], axis=0))
        k_u[s * NG + g] = pltpu.bitcast(kfull.T, u32)

    def v_task(s, b):
        w = _bf(wt_u[WT_V + b * (VB // 2):WT_V + (b + 1) * (VB // 2), :])
        v = jnp.dot(w, load_xs(s, 0, TPS), preferred_element_type=f32)
        pace[0] = _zero_after(v)
        v = _pack(v)
        vt_u[s, b * (VB // 2):(b + 1) * (VB // 2), :] = v
        sub = lax.broadcasted_iota(i32, (16, L), 0)
        for hh in range(8):
            w8 = (9 * hh) // 8
            ones_row = 0 if 2 * hh == 14 else 15
            vwin[s * H + 8 * b + hh] = jnp.where(sub == ones_row, u32(ONES_PAIR), v[8 * w8:8 * w8 + 16, :])

    def q_tasks(s, t0=0, t1=TPS):
        return [lambda g=g: q_task(s, g, t0, t1) for g in range(NG)]

    def k_tasks(s):
        return [lambda g=g: k_task(s, g) for g in range(NG)]

    def v_tasks(s):
        return [lambda b=b: v_task(s, b) for b in range(D // VB)]

    def run(tasks):
        for t in tasks:
            t()

    ln0 = ln_tasks(0)
    prep_q = prep_grouped(0, WT_Q)
    with _scope("p1_wait_wq"):
        w_copy(0).wait()
    with _scope("p1_prep_q"):
        run(prep_q[0:3])
        x_copy(0).wait()
    for i in range(2, len(X_PIECES)):
        x_copy(i).start()
    w_copy(3).start()
    for i in range(3):
        moe_copy(i).start()
    with _scope("p1_ln0a"):
        run(_interleave(prep_q[3:], ln0[0:4]))
        x_copy(1).wait()
    with _scope("p1_q0a"):
        run(_interleave(q_tasks(0, 0, 2), ln0[4:8]))
        w_copy(1).wait()
    with _scope("p1_q0b"):
        run(_interleave(q_tasks(0, 2, 4), prep_grouped(1, WT_K)))
        w_copy(2).wait()
    with _scope("p1_k0"):
        run(_interleave(k_tasks(0), prep_dense(2, wt_u, WT_V)))
        x_copy(2).wait()
    with _scope("p1_v0"):
        run(_interleave(v_tasks(0), ln_tasks(1)))

    def seg_body(s, c):
        for ss in range(2, NSEG):
            @pl.when(s + 1 == ss)
            def _():
                x_copy(ss + 1).wait()
        nxt = jnp.minimum(s + 1, NSEG - 1)
        pace[0] = None
        with _scope("p1_seg"):
            run(_interleave(q_tasks(s) + k_tasks(s) + v_tasks(s), ln_tasks(nxt)))
        return c

    lax.fori_loop(1, NSEG, seg_body, 0)

    row64 = lax.broadcasted_iota(i32, (TW, T), 0)
    lane64 = lax.broadcasted_iota(i32, (TW, T), 1)
    row32 = lax.broadcasted_iota(i32, (32, T), 0)
    lane32 = lax.broadcasted_iota(i32, (32, T), 1)
    lane1 = lax.broadcasted_iota(i32, (1, T), 1)
    lane8 = lax.broadcasted_iota(i32, (8, T), 1)

    def stage_a(unit, u, qt, s_ref, m_ref):
        s = unit // UPS
        pi = (unit % UPS) * NP + u
        g = pi // (HPG // 2)
        j = 2 * (pi - (HPG // 2) * g)
        sg = s * NG + g
        n = T * (qt + 1)
        qw = qs_u[sg, :, qt * T:(qt + 1) * T]
        w_a = qw & rowmask[j]
        w_b = qw & rowmask[j + 1]
        w_ab = _bf(jnp.where(lane64 < HT, w_a, w_b))

        def colmax8(v):
            return jnp.max(v.reshape(v.shape[0] // 8, 8, T), axis=0)

        maxes = []
        for hd, w in enumerate((_bf(w_a), _bf(w_b))):
            m8 = None
            for c in range(qt):
                kc = _bf(k_u[sg, c * TW:(c + 1) * TW, :])
                sc = jnp.dot(kc, w, preferred_element_type=f32)
                s_ref[u, qt, hd * L + c * T:hd * L + (c + 1) * T, :] = sc
                m8 = colmax8(sc) if m8 is None else jnp.maximum(m8, colmax8(sc))
            kc = _bf(k_u[sg, qt * TW:qt * TW + TW // 2, :])
            sc = jnp.dot(kc, w, preferred_element_type=f32) + mb[1 - hd]
            s_ref[u, qt, hd * L + qt * T:hd * L + qt * T + HT, :] = sc
            m8 = colmax8(sc) if m8 is None else jnp.maximum(m8, colmax8(sc))
            maxes.append(m8)
        kc = _bf(k_u[sg, qt * TW + TW // 2:(qt + 1) * TW, :])
        sc = jnp.dot(kc, w_ab, preferred_element_type=f32) + mb[2]
        s_ref[u, qt, n - HT:n, :] = sc
        mab = colmax8(sc)
        m_a = jnp.where(lane8 < HT, jnp.maximum(maxes[0], mab), maxes[0])
        m_b = jnp.where(lane8 >= HT, jnp.maximum(maxes[1], mab), maxes[1])
        m_ref[u, qt, 0] = jnp.broadcast_to(jnp.max(m_a, axis=0, keepdims=True), (8, T))
        m_ref[u, qt, 1] = jnp.broadcast_to(jnp.max(m_b, axis=0, keepdims=True), (8, T))

    def stage_b(unit, u, qt, s_ref, m_ref):
        s = unit // UPS
        pi = (unit % UPS) * NP + u
        n = T * (qt + 1)
        m_a = m_ref[u, qt, 0][0:1]
        m_b = m_ref[u, qt, 1][0:1]
        p_ab = jnp.exp2(s_ref[u, qt, n - HT:n, :] - jnp.where(lane1 < HT, m_a, m_b))
        for hd, m in enumerate((m_a, m_b)):
            h = 2 * pi + hd
            p = jnp.exp2(s_ref[u, qt, hd * L:hd * L + n - HT, :] - m)
            keep = (lane64 < HT) if hd == 0 else (lane64 >= HT)
            p = jnp.concatenate([p, jnp.where(keep, p_ab, 0.0)], axis=0).astype(bf16)
            w8 = (9 * h) // 8
            off = DH * h - 16 * w8
            o = jnp.dot(_bf(vwin[s * H + h, :, 0:n]), p, preferred_element_type=f32)
            den = jnp.where(off == 14, o[0:1], o[31:32])
            o = o * (omg[h][0:1] / den)
            if hd == 0:
                o = pltpu.roll(o, HT, 1)
            r1 = pl.multiple_of(16 * w8, 16)
            res = am[s, pl.ds(r1, 32), qt * T:(qt + 1) * T] + o
            pltpu.store(ot.at[pl.ds(r1, 32), qt * T:(qt + 1) * T], res, mask=smask[off // 2] != 0)

    def a_tasks(unit, s_ref, m_ref):
        return [lambda u=u, qt=qt: stage_a(unit, u, qt, s_ref, m_ref) for u in range(NP) for qt in QT_ORDER]

    def b_tasks(unit, s_ref, m_ref):
        return [lambda u=u, qt=qt: stage_b(unit, u, qt, s_ref, m_ref) for u in range(NP) for qt in QT_ORDER]

    ones16 = jnp.where(lax.broadcasted_iota(i32, (8, L), 0) == 0, u32(0x3F80), u32(0))

    def mem_task(s, g):
        es, eoff, ne = _ewin(g)
        nv = _valid(g)
        lhs = _bf(jnp.concatenate([vt_u[s, es // 2:(es + ne) // 2, :], ones16], axis=0))
        upd = lax.dot_general(lhs, _bf(pk_u[s * NG + g]), NT_DIMS, preferred_element_type=f32)
        mt = mt_acc[g, 0:ne + 16, :] + upd
        mt_acc[g, 0:ne + 16, :] = mt
        e_loc = lax.broadcasted_iota(i32, (ne, T), 0) - eoff
        d_id = lax.broadcasted_iota(i32, (ne, T), 1)
        same_head = (e_loc >= 0) & (e_loc < nv) & (d_id < nv) & ((e_loc // DH) == (d_id // DH))
        j16 = lax.broadcasted_iota(i32, (16, T), 0)
        d16 = lax.broadcasted_iota(i32, (16, T), 1)
        z_mask = ((d16 // DH) == j16) & (d16 < nv)
        lm = jnp.concatenate(
            [jnp.where(same_head, mt[0:ne], 0.0),
             jnp.where(z_mask, jnp.broadcast_to(mt[ne:ne + 1, :], (16, T)), 0.0)], axis=0)
        nd = jnp.dot(lm.astype(bf16), _bf(pq_u[(s + 1) * NG + g]), preferred_element_type=f32)
        scale = jnp.broadcast_to(g16[g][:, 0:1], (16, L)) / (nd[ne:ne + 16, :] + 1e-6)
        r8 = lax.broadcasted_iota(i32, (8, L), 0)
        for b in range(ne // 8):
            lo, hi = 8 * b - eoff, 8 * b + 7 - eoff
            if hi < 0 or lo >= nv:
                continue
            j1, j2 = max(lo, 0) // DH, min(hi, nv - 1) // DH
            sc = jnp.broadcast_to(scale[j1:j1 + 1, :], (8, L))
            if j2 != j1:
                sc = jnp.where(r8 < DH * j2 - lo, sc, jnp.broadcast_to(scale[j2:j2 + 1, :], (8, L)))
            val = nd[8 * b:8 * b + 8, :] * sc
            dst = am.at[s + 1, es + 8 * b:es + 8 * b + 8, :]
            if lo >= 0 and hi < nv:
                dst[...] = val
            else:
                pltpu.store(dst, val, mask=(r8 + lo >= 0) & (r8 + lo < nv))

    mem_tasks = [lambda s=s, g=g: mem_task(s, g) for s in range(NSEG - 1) for g in range(NG)]

    w_copy(3).wait()
    for i in range(3):
        moe_copy(i).wait()
    rr = jnp.concatenate([r_buf[s][0:1, :] for s in range(NSEG)], axis=0)
    rr = _round_bf16(rr)
    tok = lax.broadcasted_iota(i32, (NSEG, L), 0) * L + lax.broadcasted_iota(i32, (NSEG, L), 1)
    m1v = jnp.max(rr)
    i1 = jnp.min(jnp.where(rr == m1v, tok, SEQ))
    rr2 = jnp.where(tok == i1, -jnp.inf, rr)
    m2v = jnp.max(rr2)
    i2 = jnp.min(jnp.where(rr2 == m2v, tok, SEQ))
    i1 = jnp.clip(i1, 0, SEQ - 1)
    i2 = jnp.clip(i2, 0, SEQ - 1)

    row16 = lax.broadcasted_iota(i32, (16, T), 0)
    lane16 = lax.broadcasted_iota(i32, (16, T), 1)

    def token_rows(i, slot):
        onehot = jnp.where((row16 == slot) & (lane16 == i % T), 1.0, 0.0).astype(bf16)
        return lax.dot_general(onehot, _bf(xn_u[i // T]), NT_DIMS, preferred_element_type=f32)

    def select_task():
        xsel_buf[...] = _pack(token_rows(i1, 0) + token_rows(i2, 1))
        y_acc[...] = jnp.zeros(y_acc.shape, f32)

    def fcols(ft):
        return pl.ds(ft * T if isinstance(ft, int) else pl.multiple_of(ft * T, T), T)

    def moe_up_task(ft, k, which):
        xsel = _bf(xsel_buf[:, 0:D])
        w_ref = (wg_buf, wu_buf)[which]
        hid_buf[k, which] = jnp.dot(xsel, w_ref[:, fcols(ft)], preferred_element_type=f32)

    def moe_down_task(ft, k):
        gt = _round_bf16(hid_buf[k, 0])
        up = _round_bf16(hid_buf[k, 1])
        hid = (_round_bf16(gt * _sigmoid(gt)) * up).astype(bf16)
        y_acc[...] += lax.dot_general(hid, wd_buf[:, fcols(ft)], NT_DIMS, preferred_element_type=f32)

    def moe_tasks(ft0, count):
        tasks = []
        for k0 in range(0, count, FPB):
            ks = range(k0, min(k0 + FPB, count))
            tasks += [lambda k=k, w=w: moe_up_task(ft0 + k, k, w) for k in ks for w in range(2)]
            tasks += [lambda k=k: moe_down_task(ft0 + k, k) for k in ks]
        return tasks

    def moe_finish():
        y = _round_bf16(y_acc[...])
        rsel = jnp.where(lax.broadcasted_iota(i32, (16, 1), 0) == 0, m1v, m2v)
        y = _round_bf16(y * _round_bf16(_sigmoid(rsel)))
        y = jnp.concatenate([y, jnp.zeros((16, DP - D), f32)], axis=1)
        y = jnp.concatenate([jnp.zeros((HT, DP), f32), y, jnp.zeros((T - HT - 16, DP), f32)], axis=0)
        y_t = jnp.concatenate([y.T[0:D], jnp.zeros((D, T), f32)], axis=1)
        y_u = _pack(y_t)[:, 0:T]
        lane = lax.broadcasted_iota(i32, (D // 2, T), 1)
        wot_u[:, DP - T:DP] = jnp.where(lane < HT, wot_u[:, DP - T:DP], y_u)
        tok_l = lax.broadcasted_iota(i32, (8, L), 1) + (NSEG - 1) * L
        rid = lax.broadcasted_iota(i32, (8, L), 0)
        ot[D:D + 8, :] = jnp.where(((rid == 0) & (tok_l == i1)) | ((rid == 1) & (tok_l == i2)), 1.0, 0.0)

    dense = _interleave(mem_tasks, a_tasks(0, s0, m0), prep_dense(3, wot_u, 0))
    with _scope("p15_mix"):
        run(dense[0:2] + [select_task] + dense[2:])

    def out_tile(s, tt, last):
        c0 = s * L + tt * T
        if not isinstance(s, int):
            c0 = pl.multiple_of(c0, T)
        o_bf = ot[:, tt * T:(tt + 1) * T].astype(bf16)
        nchunk = 4
        rows = D // nchunk
        for rc in range(nchunk):
            r0 = rc * rows
            attn = jnp.dot(_bf(wot_u[r0 // 2:(r0 + rows) // 2, :]), o_bf, preferred_element_type=f32)
            xn = _bf(xn_u[s * TPS + tt, r0 // 2:(r0 + rows) // 2, :]).astype(f32)
            x = x_buf[r0:r0 + rows, pl.ds(c0, T)].astype(f32)
            res = x + attn + xn
            out_buf[r0:r0 + rows, pl.ds(c0, T)] = res.astype(bf16)

    bufs = ((s0, m0), (s1, m1))

    def pair_tasks(ua, ub):
        tasks = []
        for x, y in zip(a_tasks(ua[0], *bufs[ua[1]]), b_tasks(ub[0], *bufs[ub[1]])):
            tasks += [y, x]
        return tasks

    def seg_end(s, last, extra_first):
        u2, u3 = UPS * s + 2, UPS * s + 3

        def by_qt(fn, unit, par, qt):
            return [lambda u=u: fn(unit, u, qt, *bufs[par]) for u in range(NP)]

        steps = []
        for step in range(7):
            lists = []
            if step < 4:
                lists.append(by_qt(stage_b, u2, 0, 3 - step))
                lists.append(by_qt(stage_a, u3, 1, 3 - step))
            if 1 <= step < 5:
                lists.append(by_qt(stage_b, u3, 1, 4 - step))
            if not last and 2 <= step < 6:
                lists.append(by_qt(stage_a, u3 + 1, 0, 5 - step))
            if step >= 3:
                lists.append([lambda tt=6 - step: out_tile(s, tt, last)])
            steps.append(_interleave(*lists))
        return steps

    def seg_att(s, c):
        u0 = UPS * s
        tasks = pair_tasks((u0 + 1, 1), (u0, 0)) + pair_tasks((u0 + 2, 0), (u0 + 1, 1))
        for step in seg_end(s, False, None)[0:5]:
            tasks += step
        with _scope("att_seg"):
            run(_interleave(tasks, moe_tasks(s * FPI, FPI)))
            for step in seg_end(s, False, None)[5:]:
                run(step)
        out_copy(pl.multiple_of(s * L, L), L, s).start()
        return c

    lax.fori_loop(0, NSEG - 1, seg_att, 0)

    npatch = (NSEG - 1) * TPS

    def patch_tile(idx):
        return jnp.where(idx < npatch * T, idx // T, 0)

    tile0 = patch_tile(i1)
    tile1 = patch_tile(i2)
    tile1 = jnp.where(tile1 == tile0, (tile0 + 1) % npatch, tile1)

    def patch(tile):
        c0 = pl.multiple_of(tile * T, T)
        rid = lax.broadcasted_iota(i32, (T, T), 0)
        tok_l = lax.broadcasted_iota(i32, (T, T), 1) + c0
        hit = ((rid == HT) & (tok_l == i1)) | ((rid == HT + 1) & (tok_l == i2))
        onehot = jnp.where(hit, 1.0, 0.0).astype(bf16)
        for rc in range(4):
            r0, r1 = rc * (D // 4), (rc + 1) * (D // 4)
            upd = jnp.dot(_bf(wot_u[r0 // 2:r1 // 2, DP - T:DP]), onehot, preferred_element_type=f32)
            cur = out_buf[r0:r1, pl.ds(c0, T)].astype(f32)
            out_buf[r0:r1, pl.ds(c0, T)] = (cur + upd).astype(bf16)

    patch_copies = [out_copy(pl.multiple_of(tile0 * T, T), T, 7), out_copy(pl.multiple_of(tile1 * T, T), T, 8)]
    last_copies = [out_copy((NSEG - 1) * L + tt * T, T, NSEG - 1 + tt) for tt in range(TPS)]

    sl = NSEG - 1
    ul = UPS * sl
    with _scope("tail_1"):
        moe_finish()
        run(pair_tasks((ul + 1, 1), (ul, 0)))
        for s in range(NSEG - 1):
            out_copy(s * L, L, s).wait()
    with _scope("tail_2"):
        patch(tile0)
        patch(tile1)
        run(pair_tasks((ul + 2, 0), (ul + 1, 1)))
        for cp in patch_copies:
            cp.start()
        steps = seg_end(sl, True, None)
        for step in steps[0:5]:
            run(step)
        last_copies[3].start()
        last_copies[2].start()
    with _scope("tail_3"):
        run(steps[5])
        run(steps[6])
        last_copies[1].start()
        last_copies[0].start()

    with _scope("out_wait"):
        for cp in patch_copies + last_copies:
            cp.wait()


@jax.jit
def pallas_parallel_sum__memory_aug_infini_attn__moe_arch_mod__prompt_kernel(
    A_x: jax.Array,
    A_wq: jax.Array,
    A_wk: jax.Array,
    A_wv: jax.Array,
    A_wo: jax.Array,
    A_beta: jax.Array,
    B_x: jax.Array,
    B_w_r: jax.Array,
    B_w_gate: jax.Array,
    B_w_up: jax.Array,
    B_w_down: jax.Array,
):
    del B_x
    any_spec = pl.BlockSpec(memory_space=pl.ANY)
    vmem_spec = pl.BlockSpec(memory_space=pltpu.VMEM)
    scratch = [
        pltpu.VMEM((D, SEQ), bf16),
        pltpu.VMEM((4, D, D), bf16),
        pltpu.VMEM((D, F), bf16),
        pltpu.VMEM((D, F), bf16),
        pltpu.VMEM((D, F), bf16),
        pltpu.VMEM((D, SEQ), bf16),
        pltpu.VMEM((WT_ROWS, DP), u32),
        pltpu.VMEM((D // 2, DP), u32),
        pltpu.VMEM((D // 2, DP), u32),
        pltpu.VMEM((NT, DP // 2, T), u32),
        pltpu.VMEM((NSEG * NG, TW, L), u32),
        pltpu.VMEM((NSEG * NG, L // 2, T), u32),
        pltpu.VMEM((NSEG * NG, TW, L), u32),
        pltpu.VMEM((NSEG * NG, TW, L), u32),
        pltpu.VMEM((NSEG, D // 2, L), u32),
        pltpu.VMEM((NSEG * H, 16, L), u32),
        pltpu.VMEM((NSEG, 8, L), f32),
        pltpu.VMEM((NG, T + 16, T), f32),
        pltpu.VMEM((NSEG, D, L), f32),
        pltpu.VMEM((NG, 16, T), f32),
        pltpu.VMEM((H, 8, T), f32),
        pltpu.VMEM((3, HT, T), f32),
        pltpu.VMEM((HPG, TW, T), u32),
        pltpu.VMEM((8, 32, T), i32),
        pltpu.VMEM((NP, 4, 2 * L, T), f32),
        pltpu.VMEM((NP, 4, 2, 8, T), f32),
        pltpu.VMEM((NP, 4, 2 * L, T), f32),
        pltpu.VMEM((NP, 4, 2, 8, T), f32),
        pltpu.VMEM((DP, L), f32),
        pltpu.VMEM((2, D, LNW), f32),
        pltpu.VMEM((2, 2, 8, LNW), f32),
        pltpu.VMEM((16, D), f32),
        pltpu.VMEM((8, DP), u32),
        pltpu.VMEM((FPI, 2, 16, T), f32),
        pltpu.SemaphoreType.DMA((NSEM,)),
    ]
    x_t = jnp.transpose(A_x, (0, 2, 1)).reshape(D, SEQ)
    out_t = pl.pallas_call(
        _kernel,
        out_shape=jax.ShapeDtypeStruct((D, SEQ), bf16),
        in_specs=[any_spec, any_spec, any_spec, any_spec, any_spec, vmem_spec, vmem_spec,
                  any_spec, any_spec, any_spec],
        out_specs=any_spec,
        scratch_shapes=scratch,
        compiler_params=pltpu.CompilerParams(vmem_limit_bytes=110 * 1024 * 1024),
    )(x_t, A_wq, A_wk, A_wv, A_wo, A_beta, B_w_r, B_w_gate, B_w_up, B_w_down.T)
    return jnp.transpose(out_t.reshape(1, D, SEQ), (0, 2, 1))
```

```python
import contextlib

import jax
import jax.numpy as jnp
from jax import lax
from jax.experimental import pallas as pl
from jax.experimental.pallas import tpu as pltpu

bf16 = jnp.bfloat16
f32 = jnp.float32
u32 = jnp.uint32
i32 = jnp.int32

SEQ = 2048
D = 576
DP = 640
H = 32
DH = 18
NSEG = 4
L = 512
T = 128
TW = T // 2
HT = T // 2
TPS = L // T
HPG = 6
NG = 6
F = 4608
FPI = 12
FPB = 3
NFT = F // T
NP = 4
UPS = H // (2 * NP)
NUNIT = NSEG * UPS
NT = SEQ // T
LNW = 256
VB = 8 * DH

LOG2E = 1.4426950408889634
QSCALE = (DH ** -0.5) * LOG2E
MASKVAL = -1000000000.0 * LOG2E
EPS_BF16 = 1.0013580322265625e-05
ONES_PAIR = 0x3F803F80

NT_DIMS = (((1,), (1,)), ((), ()))

WT_Q = 0
WT_K = NG * TW
WT_V = 2 * NG * TW
WT_ROWS = WT_V + D // 2

X_PIECES = ((0, LNW), (LNW, LNW), (L, L), (2 * L, L), (3 * L, L))
SEM_X = 0
SEM_W = 5
SEM_MOE = 9
SEM_OUT = 12
SEM_SMALL = 21
NSEM = 23


PROFILE_SCOPES = False
PACE = False
TAIL_BARRIERS = False
QT_ORDER = (3, 2, 1, 0)


def _scope(name):
    return jax.named_scope(name) if PROFILE_SCOPES else contextlib.nullcontext()


def _valid(g):
    return min(HPG * DH, D - g * HPG * DH)


def _rows(g):
    return -(-_valid(g) // 16) * 16


def _ewin(g):
    start = (g * HPG * DH // 16) * 16
    return start, g * HPG * DH - start, min(T, D - start)


def _bf(x):
    return pltpu.bitcast(x, bf16)


def _pack(x):
    return pltpu.bitcast(x.astype(bf16), u32)


def _round_bf16(x):
    return x.astype(bf16).astype(f32)


def _phi(t):
    return jnp.where(t > 0, t + 1.0, jnp.exp(t))


def _sigmoid(t):
    return 1.0 / (1.0 + jnp.exp(-t))


def _zero_after(v):
    bits = pltpu.bitcast(v[0:8, 0:LNW], u32)
    sixteen = jnp.uint32(16)
    bits = lax.shift_right_logical(lax.shift_right_logical(bits, sixteen), sixteen)
    return pltpu.bitcast(bits, f32) if PACE else None


def _interleave(*lists):
    items = []
    for li, tasks in enumerate(lists):
        for k, t in enumerate(tasks):
            items.append(((k + 0.5) / len(tasks), li, k, t))
    items.sort(key=lambda it: it[:3])
    return [it[3] for it in items]


def _kernel(x_hbm, wq_hbm, wk_hbm, wv_hbm, wo_hbm, beta_hbm, wr_hbm, wg_hbm, wu_hbm, wd_hbm,
            out_hbm,
            beta_ref, wr_ref, x_buf, w_buf, wg_buf, wu_buf, wd_buf, out_buf,
            wt_u, wtd_u, wot_u, xn_u, qs_u, k_u, pq_u, pk_u, vt_u, vwin,
            r_buf, mt_acc, am, g16, omg, mb, rowmask, smask,
            s0, m0, s1, m1, ot, xf, ln_stat, y_acc, xsel_buf, hid_buf, sems):

    def x_copy(i):
        c0, width = X_PIECES[i]
        return pltpu.make_async_copy(x_hbm.at[:, pl.ds(c0, width)], x_buf.at[:, pl.ds(c0, width)],
                                     sems.at[SEM_X + i])

    def w_copy(i):
        src = (wq_hbm, wk_hbm, wv_hbm, wo_hbm)[i]
        return pltpu.make_async_copy(src, w_buf.at[i], sems.at[SEM_W + i])

    def moe_copy(i):
        src = (wg_hbm, wu_hbm, wd_hbm)[i]
        dst = (wg_buf, wu_buf, wd_buf)[i]
        return pltpu.make_async_copy(src, dst, sems.at[SEM_MOE + i])

    def out_copy(c0, width, sem):
        return pltpu.make_async_copy(out_buf.at[:, pl.ds(c0, width)], out_hbm.at[:, pl.ds(c0, width)],
                                     sems.at[SEM_OUT + sem])

    small_copies = [pltpu.make_async_copy(beta_hbm, beta_ref, sems.at[SEM_SMALL]),
                    pltpu.make_async_copy(wr_hbm, wr_ref, sems.at[SEM_SMALL + 1])]
    w_copy(0).start()
    x_copy(0).start()
    x_copy(1).start()
    for cp in small_copies:
        cp.start()
    w_copy(1).start()
    w_copy(2).start()

    init_scope = _scope("init")
    init_scope.__enter__()
    kr = lax.broadcasted_iota(i32, (HT, T), 0)
    ql = lax.broadcasted_iota(i32, (HT, T), 1)
    mb[0] = jnp.where(ql < kr, MASKVAL, 0.0).astype(f32)
    mb[1] = jnp.where((ql >= HT) & (ql - HT < kr), MASKVAL, 0.0).astype(f32)
    mb[2] = jnp.where(ql % HT < kr, MASKVAL, 0.0).astype(f32)
    for j in range(HPG):
        rowmask[j] = jnp.where((kr >= (DH // 2) * j) & (kr < (DH // 2) * (j + 1)), u32(0xFFFFFFFF), u32(0))
    r32 = lax.broadcasted_iota(i32, (32, T), 0)
    for i in range(8):
        smask[i] = jnp.where((r32 >= 2 * i) & (r32 < 2 * i + DH), 1, 0)
    zpad = jnp.zeros(((DP - D) // 2, T), u32)
    for tt in range(NT):
        xn_u[tt, D // 2:DP // 2, :] = zpad
    ot[D:DP, :] = jnp.zeros((DP - D, L), f32)
    am[0] = jnp.zeros(am.shape[1:], f32)
    mt_acc[...] = jnp.zeros(mt_acc.shape, f32)
    g16[...] = jnp.zeros(g16.shape, f32)
    for sg in range(NSEG * NG):
        r2 = _rows(sg % NG) // 2
        qs_u[sg, r2:TW, :] = jnp.zeros((TW - r2, L), u32)
        pq_u[sg, r2:TW, :] = jnp.zeros((TW - r2, L), u32)
        pk_u[sg, r2:TW, :] = jnp.zeros((TW - r2, L), u32)

    init_scope.__exit__(None, None, None)

    pace = [None]

    def gate_tables():
        gate = _round_bf16(_sigmoid(beta_ref[...].reshape(1, H).astype(f32)))
        for h in range(H):
            gh = jnp.broadcast_to(gate[:, h:h + 1], (1, T))
            omg[h] = jnp.broadcast_to(_round_bf16(1.0 - gh), (8, T))
            g16[h // HPG, (h % HPG):(h % HPG) + 1, :] = gh

    def transpose_block(i, cb):
        c1 = min((cb + 1) * T, D)
        blk = w_buf[i, :, cb * T:c1]
        if c1 - cb * T < T:
            blk = jnp.concatenate([blk, jnp.zeros((D, T - (c1 - cb * T)), bf16)], axis=1)
        blk = jnp.concatenate([blk, jnp.zeros((DP - D, T), bf16)], axis=0)
        return pltpu.bitcast(blk.T, u32)

    def prep_dense(i, dst, base):
        def task(cb):
            nrow = min(TW, D // 2 - cb * TW)
            dst[base + cb * TW:base + cb * TW + nrow, :] = transpose_block(i, cb)[0:nrow]
        return [lambda cb=cb: task(cb) for cb in range(DP // T)]

    def prep_grouped(i, base):
        def regroup(g):
            nv, nr = _valid(g) // 2, _rows(g) // 2
            src = g * HPG * DH // 2
            wt_u[base + g * TW:base + g * TW + nv, :] = wtd_u[src:src + nv, :]
            pad = jnp.zeros((nr - nv, DP), u32)
            if i == 1 and g == 0:
                wr = wr_ref[...].reshape(1, D).astype(f32)
                wr = jnp.concatenate([wr, jnp.zeros((1, DP - D), f32)], axis=1)
                bits = lax.shift_right_logical(pltpu.bitcast(wr, u32), u32(16))
                rid = lax.broadcasted_iota(i32, (nr - nv, DP), 0)
                pad = jnp.where(rid == 0, bits, pad)
            wt_u[base + g * TW + nv:base + g * TW + nr, :] = pad
        return prep_dense(i, wtd_u, 0) + [lambda g=g: regroup(g) for g in range(NG)]

    def ln_tasks(s):
        def mean_pass(b):
            c0 = s * L + b * LNW
            if not isinstance(s, int):
                c0 = pl.multiple_of(c0, LNW)
            acc = pace[0]
            for r in range(0, D, 64):
                x = x_buf[r:r + 64, pl.ds(c0, LNW)].astype(f32)
                xf[b, r:r + 64, :] = x
                part = jnp.sum(x.reshape(8, 8, LNW), axis=0)
                acc = part if acc is None else acc + part
            mean = jnp.sum(acc, axis=0, keepdims=True) / D
            ln_stat[b, 0] = jnp.broadcast_to(mean, (8, LNW))

        def var_pass(b):
            bd = b
            mean = ln_stat[b, 0][0:1]
            if pace[0] is not None:
                mean = mean + pace[0][0:1]
            acc = None
            for r in range(0, D, 96):
                xc = xf[bd, r:r + 96, :] - mean
                part = jnp.sum((xc * xc).reshape(12, 8, LNW), axis=0)
                acc = part if acc is None else acc + part
            var = jnp.sum(acc, axis=0, keepdims=True) / D
            den = _round_bf16(jnp.sqrt(_round_bf16(_round_bf16(var) + EPS_BF16)))
            ln_stat[b, 1] = jnp.broadcast_to(1.0 / den, (8, LNW))
            ln_stat[b, 0] = jnp.broadcast_to(_round_bf16(mean), (8, LNW))

        def norm_pass(b, half):
            bd = b
            mean_b = ln_stat[b, 0][0:1]
            if pace[0] is not None:
                mean_b = mean_b + pace[0][0:1]
            inv = ln_stat[b, 1][0:1]
            for r in range(half * (D // 2), (half + 1) * (D // 2), 48):
                xn = _pack(_round_bf16(xf[bd, r:r + 48, :] - mean_b) * inv)
                for t in range(LNW // T):
                    tt = b * (LNW // T) + t
                    xn_u[s * TPS + tt, r // 2:r // 2 + 24, :] = xn[:, t * T:(t + 1) * T]

        tasks = []
        for b in range(L // LNW):
            tasks += [lambda b=b: mean_pass(b), lambda b=b: var_pass(b),
                      lambda b=b: norm_pass(b, 0), lambda b=b: norm_pass(b, 1)]
        return tasks

    def load_xs(s, t0, t1):
        return jnp.concatenate([_bf(xn_u[s * TPS + tt]) for tt in range(t0, t1)], axis=1)

    def q_task(s, g, t0=0, t1=TPS):
        nr = _rows(g) // 2
        w = _bf(wt_u[WT_Q + g * TW:WT_Q + g * TW + nr, :])
        q = jnp.dot(w, load_xs(s, t0, t1), preferred_element_type=f32)
        pace[0] = _zero_after(q)
        qp = _pack(q * QSCALE)
        qrot = jnp.concatenate([pltpu.roll(qp[:, t * T:(t + 1) * T], HT, 1) for t in range(t1 - t0)], axis=1)
        rid = lax.broadcasted_iota(i32, qp.shape, 0)
        even = ((rid // (DH // 2)) % 2) == 0
        qs_u[s * NG + g, 0:nr, t0 * T:t1 * T] = jnp.where(even, qrot, qp)
        pq_u[s * NG + g, 0:nr, t0 * T:t1 * T] = _pack(_phi(_round_bf16(q)))

    def k_task(s, g):
        nr = _rows(g)
        w = _bf(wt_u[WT_K + g * TW:WT_K + g * TW + nr // 2, :])
        k = jnp.dot(w, load_xs(s, 0, TPS), preferred_element_type=f32)
        pace[0] = _zero_after(k)
        if g == 0:
            r_buf[s] = jnp.broadcast_to(k[_valid(0):_valid(0) + 1, :], (8, L))
        kp = _pack(k)
        pk_u[s * NG + g, 0:nr // 2, :] = _pack(_phi(_round_bf16(k)))
        kfull = _bf(jnp.concatenate([kp, jnp.zeros(((T - nr) // 2, L), u32)], axis=0))
        k_u[s * NG + g] = pltpu.bitcast(kfull.T, u32)

    def v_task(s, b):
        w = _bf(wt_u[WT_V + b * (VB // 2):WT_V + (b + 1) * (VB // 2), :])
        v = jnp.dot(w, load_xs(s, 0, TPS), preferred_element_type=f32)
        pace[0] = _zero_after(v)
        v = _pack(v)
        vt_u[s, b * (VB // 2):(b + 1) * (VB // 2), :] = v
        sub = lax.broadcasted_iota(i32, (16, L), 0)
        for hh in range(8):
            w8 = (9 * hh) // 8
            ones_row = 0 if 2 * hh == 14 else 15
            vwin[s * H + 8 * b + hh] = jnp.where(sub == ones_row, u32(ONES_PAIR), v[8 * w8:8 * w8 + 16, :])

    def q_tasks(s, t0=0, t1=TPS):
        return [lambda g=g: q_task(s, g, t0, t1) for g in range(NG)]

    def k_tasks(s):
        return [lambda g=g: k_task(s, g) for g in range(NG)]

    def v_tasks(s):
        return [lambda b=b: v_task(s, b) for b in range(D // VB)]

    def run(tasks):
        for t in tasks:
            t()

    ln0 = ln_tasks(0)
    prep_q = prep_grouped(0, WT_Q)
    with _scope("p1_wait_wq"):
        w_copy(0).wait()
    with _scope("p1_prep_q"):
        run(prep_q[0:3])
        x_copy(0).wait()
    for i in range(2, len(X_PIECES)):
        x_copy(i).start()
    w_copy(3).start()
    for i in range(3):
        moe_copy(i).start()
    with _scope("p1_ln0a"):
        run(_interleave(prep_q[3:], ln0[0:4]))
        x_copy(1).wait()
    with _scope("p1_q0a"):
        run(_interleave(q_tasks(0, 0, 2), ln0[4:8]))
        w_copy(1).wait()
        for cp in small_copies:
            cp.wait()
    with _scope("p1_q0b"):
        run(_interleave(q_tasks(0, 2, 4), prep_grouped(1, WT_K), [gate_tables]))
        w_copy(2).wait()
    with _scope("p1_k0"):
        run(_interleave(k_tasks(0), prep_dense(2, wt_u, WT_V)))
        x_copy(2).wait()
    with _scope("p1_v0"):
        run(_interleave(v_tasks(0), ln_tasks(1)))

    def seg_body(s, c):
        for ss in range(2, NSEG):
            @pl.when(s + 1 == ss)
            def _():
                x_copy(ss + 1).wait()
        nxt = jnp.minimum(s + 1, NSEG - 1)
        pace[0] = None
        with _scope("p1_seg"):
            run(_interleave(q_tasks(s) + k_tasks(s) + v_tasks(s), ln_tasks(nxt)))
        return c

    lax.fori_loop(1, NSEG, seg_body, 0)

    row64 = lax.broadcasted_iota(i32, (TW, T), 0)
    lane64 = lax.broadcasted_iota(i32, (TW, T), 1)
    row32 = lax.broadcasted_iota(i32, (32, T), 0)
    lane32 = lax.broadcasted_iota(i32, (32, T), 1)
    lane1 = lax.broadcasted_iota(i32, (1, T), 1)
    lane8 = lax.broadcasted_iota(i32, (8, T), 1)

    def stage_a(unit, u, qt, s_ref, m_ref):
        s = unit // UPS
        pi = (unit % UPS) * NP + u
        g = pi // (HPG // 2)
        j = 2 * (pi - (HPG // 2) * g)
        sg = s * NG + g
        n = T * (qt + 1)
        qw = qs_u[sg, :, qt * T:(qt + 1) * T]
        w_a = qw & rowmask[j]
        w_b = qw & rowmask[j + 1]
        w_ab = _bf(jnp.where(lane64 < HT, w_a, w_b))

        def colmax8(v):
            return jnp.max(v.reshape(v.shape[0] // 8, 8, T), axis=0)

        maxes = []
        for hd, w in enumerate((_bf(w_a), _bf(w_b))):
            m8 = None
            for c in range(qt):
                kc = _bf(k_u[sg, c * TW:(c + 1) * TW, :])
                sc = jnp.dot(kc, w, preferred_element_type=f32)
                s_ref[u, qt, hd * L + c * T:hd * L + (c + 1) * T, :] = sc
                m8 = colmax8(sc) if m8 is None else jnp.maximum(m8, colmax8(sc))
            kc = _bf(k_u[sg, qt * TW:qt * TW + TW // 2, :])
            sc = jnp.dot(kc, w, preferred_element_type=f32) + mb[1 - hd]
            s_ref[u, qt, hd * L + qt * T:hd * L + qt * T + HT, :] = sc
            m8 = colmax8(sc) if m8 is None else jnp.maximum(m8, colmax8(sc))
            maxes.append(m8)
        kc = _bf(k_u[sg, qt * TW + TW // 2:(qt + 1) * TW, :])
        sc = jnp.dot(kc, w_ab, preferred_element_type=f32) + mb[2]
        s_ref[u, qt, n - HT:n, :] = sc
        mab = colmax8(sc)
        m_a = jnp.where(lane8 < HT, jnp.maximum(maxes[0], mab), maxes[0])
        m_b = jnp.where(lane8 >= HT, jnp.maximum(maxes[1], mab), maxes[1])
        m_ref[u, qt, 0] = jnp.broadcast_to(jnp.max(m_a, axis=0, keepdims=True), (8, T))
        m_ref[u, qt, 1] = jnp.broadcast_to(jnp.max(m_b, axis=0, keepdims=True), (8, T))

    def stage_b(unit, u, qt, s_ref, m_ref):
        s = unit // UPS
        pi = (unit % UPS) * NP + u
        n = T * (qt + 1)
        m_a = m_ref[u, qt, 0][0:1]
        m_b = m_ref[u, qt, 1][0:1]
        p_ab = jnp.exp2(s_ref[u, qt, n - HT:n, :] - jnp.where(lane1 < HT, m_a, m_b))
        for hd, m in enumerate((m_a, m_b)):
            h = 2 * pi + hd
            p = jnp.exp2(s_ref[u, qt, hd * L:hd * L + n - HT, :] - m)
            keep = (lane64 < HT) if hd == 0 else (lane64 >= HT)
            p = jnp.concatenate([p, jnp.where(keep, p_ab, 0.0)], axis=0).astype(bf16)
            w8 = (9 * h) // 8
            off = DH * h - 16 * w8
            o = jnp.dot(_bf(vwin[s * H + h, :, 0:n]), p, preferred_element_type=f32)
            den = jnp.where(off == 14, o[0:1], o[31:32])
            o = o * (omg[h][0:1] / den)
            if hd == 0:
                o = pltpu.roll(o, HT, 1)
            r1 = pl.multiple_of(16 * w8, 16)
            res = am[s, pl.ds(r1, 32), qt * T:(qt + 1) * T] + o
            pltpu.store(ot.at[pl.ds(r1, 32), qt * T:(qt + 1) * T], res, mask=smask[off // 2] != 0)

    def a_tasks(unit, s_ref, m_ref):
        return [lambda u=u, qt=qt: stage_a(unit, u, qt, s_ref, m_ref) for u in range(NP) for qt in QT_ORDER]

    def b_tasks(unit, s_ref, m_ref):
        return [lambda u=u, qt=qt: stage_b(unit, u, qt, s_ref, m_ref) for u in range(NP) for qt in QT_ORDER]

    ones16 = jnp.where(lax.broadcasted_iota(i32, (8, L), 0) == 0, u32(0x3F80), u32(0))

    def mem_task(s, g):
        es, eoff, ne = _ewin(g)
        nv = _valid(g)
        lhs = _bf(jnp.concatenate([vt_u[s, es // 2:(es + ne) // 2, :], ones16], axis=0))
        upd = lax.dot_general(lhs, _bf(pk_u[s * NG + g]), NT_DIMS, preferred_element_type=f32)
        mt = mt_acc[g, 0:ne + 16, :] + upd
        mt_acc[g, 0:ne + 16, :] = mt
        e_loc = lax.broadcasted_iota(i32, (ne, T), 0) - eoff
        d_id = lax.broadcasted_iota(i32, (ne, T), 1)
        same_head = (e_loc >= 0) & (e_loc < nv) & (d_id < nv) & ((e_loc // DH) == (d_id // DH))
        j16 = lax.broadcasted_iota(i32, (16, T), 0)
        d16 = lax.broadcasted_iota(i32, (16, T), 1)
        z_mask = ((d16 // DH) == j16) & (d16 < nv)
        lm = jnp.concatenate(
            [jnp.where(same_head, mt[0:ne], 0.0),
             jnp.where(z_mask, jnp.broadcast_to(mt[ne:ne + 1, :], (16, T)), 0.0)], axis=0)
        nd = jnp.dot(lm.astype(bf16), _bf(pq_u[(s + 1) * NG + g]), preferred_element_type=f32)
        scale = jnp.broadcast_to(g16[g][:, 0:1], (16, L)) / (nd[ne:ne + 16, :] + 1e-6)
        r8 = lax.broadcasted_iota(i32, (8, L), 0)
        for b in range(ne // 8):
            lo, hi = 8 * b - eoff, 8 * b + 7 - eoff
            if hi < 0 or lo >= nv:
                continue
            j1, j2 = max(lo, 0) // DH, min(hi, nv - 1) // DH
            sc = jnp.broadcast_to(scale[j1:j1 + 1, :], (8, L))
            if j2 != j1:
                sc = jnp.where(r8 < DH * j2 - lo, sc, jnp.broadcast_to(scale[j2:j2 + 1, :], (8, L)))
            val = nd[8 * b:8 * b + 8, :] * sc
            dst = am.at[s + 1, es + 8 * b:es + 8 * b + 8, :]
            if lo >= 0 and hi < nv:
                dst[...] = val
            else:
                pltpu.store(dst, val, mask=(r8 + lo >= 0) & (r8 + lo < nv))

    mem_tasks = [lambda s=s, g=g: mem_task(s, g) for s in range(NSEG - 1) for g in range(NG)]

    w_copy(3).wait()
    for i in range(3):
        moe_copy(i).wait()
    rr = jnp.concatenate([r_buf[s][0:1, :] for s in range(NSEG)], axis=0)
    rr = _round_bf16(rr)
    tok = lax.broadcasted_iota(i32, (NSEG, L), 0) * L + lax.broadcasted_iota(i32, (NSEG, L), 1)
    m1v = jnp.max(rr)
    i1 = jnp.min(jnp.where(rr == m1v, tok, SEQ))
    rr2 = jnp.where(tok == i1, -jnp.inf, rr)
    m2v = jnp.max(rr2)
    i2 = jnp.min(jnp.where(rr2 == m2v, tok, SEQ))
    i1 = jnp.clip(i1, 0, SEQ - 1)
    i2 = jnp.clip(i2, 0, SEQ - 1)

    row16 = lax.broadcasted_iota(i32, (16, T), 0)
    lane16 = lax.broadcasted_iota(i32, (16, T), 1)

    def token_rows(i, slot):
        onehot = jnp.where((row16 == slot) & (lane16 == i % T), 1.0, 0.0).astype(bf16)
        return lax.dot_general(onehot, _bf(xn_u[i // T]), NT_DIMS, preferred_element_type=f32)

    def select_task():
        xsel_buf[...] = _pack(token_rows(i1, 0) + token_rows(i2, 1))
        y_acc[...] = jnp.zeros(y_acc.shape, f32)

    def fcols(ft):
        return pl.ds(ft * T if isinstance(ft, int) else pl.multiple_of(ft * T, T), T)

    def moe_up_task(ft, k, which):
        xsel = _bf(xsel_buf[:, 0:D])
        w_ref = (wg_buf, wu_buf)[which]
        hid_buf[k, which] = jnp.dot(xsel, w_ref[:, fcols(ft)], preferred_element_type=f32)

    def moe_down_task(ft, k):
        gt = _round_bf16(hid_buf[k, 0])
        up = _round_bf16(hid_buf[k, 1])
        hid = (_round_bf16(gt * _sigmoid(gt)) * up).astype(bf16)
        y_acc[...] += lax.dot_general(hid, wd_buf[:, fcols(ft)], NT_DIMS, preferred_element_type=f32)

    def moe_tasks(ft0, count):
        tasks = []
        for k0 in range(0, count, FPB):
            ks = range(k0, min(k0 + FPB, count))
            tasks += [lambda k=k, w=w: moe_up_task(ft0 + k, k, w) for k in ks for w in range(2)]
            tasks += [lambda k=k: moe_down_task(ft0 + k, k) for k in ks]
        return tasks

    def moe_finish():
        y = _round_bf16(y_acc[...])
        rsel = jnp.where(lax.broadcasted_iota(i32, (16, 1), 0) == 0, m1v, m2v)
        y = _round_bf16(y * _round_bf16(_sigmoid(rsel)))
        y = jnp.concatenate([y, jnp.zeros((16, DP - D), f32)], axis=1)
        y = jnp.concatenate([jnp.zeros((HT, DP), f32), y, jnp.zeros((T - HT - 16, DP), f32)], axis=0)
        y_t = jnp.concatenate([y.T[0:D], jnp.zeros((D, T), f32)], axis=1)
        y_u = _pack(y_t)[:, 0:T]
        lane = lax.broadcasted_iota(i32, (D // 2, T), 1)
        wot_u[:, DP - T:DP] = jnp.where(lane < HT, wot_u[:, DP - T:DP], y_u)
        tok_l = lax.broadcasted_iota(i32, (8, L), 1) + (NSEG - 1) * L
        rid = lax.broadcasted_iota(i32, (8, L), 0)
        ot[D:D + 8, :] = jnp.where(((rid == 0) & (tok_l == i1)) | ((rid == 1) & (tok_l == i2)), 1.0, 0.0)

    dense = _interleave(mem_tasks, a_tasks(0, s0, m0), prep_dense(3, wot_u, 0))
    with _scope("p15_mix"):
        run(dense[0:2] + [select_task] + dense[2:])

    def out_tile(s, tt, last):
        c0 = s * L + tt * T
        if not isinstance(s, int):
            c0 = pl.multiple_of(c0, T)
        o_bf = ot[:, tt * T:(tt + 1) * T].astype(bf16)
        nchunk = 4
        rows = D // nchunk
        for rc in range(nchunk):
            r0 = rc * rows
            attn = jnp.dot(_bf(wot_u[r0 // 2:(r0 + rows) // 2, :]), o_bf, preferred_element_type=f32)
            xn = _bf(xn_u[s * TPS + tt, r0 // 2:(r0 + rows) // 2, :]).astype(f32)
            x = x_buf[r0:r0 + rows, pl.ds(c0, T)].astype(f32)
            res = x + attn + xn
            out_buf[r0:r0 + rows, pl.ds(c0, T)] = res.astype(bf16)

    bufs = ((s0, m0), (s1, m1))

    def pair_tasks(ua, ub):
        tasks = []
        for x, y in zip(a_tasks(ua[0], *bufs[ua[1]]), b_tasks(ub[0], *bufs[ub[1]])):
            tasks += [y, x]
        return tasks

    def seg_end(s, last, extra_first):
        u2, u3 = UPS * s + 2, UPS * s + 3

        def by_qt(fn, unit, par, qt):
            return [lambda u=u: fn(unit, u, qt, *bufs[par]) for u in range(NP)]

        steps = []
        for step in range(7):
            lists = []
            if step < 4:
                lists.append(by_qt(stage_b, u2, 0, 3 - step))
                lists.append(by_qt(stage_a, u3, 1, 3 - step))
            if 1 <= step < 5:
                lists.append(by_qt(stage_b, u3, 1, 4 - step))
            if not last and 2 <= step < 6:
                lists.append(by_qt(stage_a, u3 + 1, 0, 5 - step))
            if step >= 3:
                lists.append([lambda tt=6 - step: out_tile(s, tt, last)])
            steps.append(_interleave(*lists))
        return steps

    def seg_att(s, c):
        u0 = UPS * s
        tasks = pair_tasks((u0 + 1, 1), (u0, 0)) + pair_tasks((u0 + 2, 0), (u0 + 1, 1))
        for step in seg_end(s, False, None)[0:5]:
            tasks += step
        with _scope("att_seg"):
            run(_interleave(tasks, moe_tasks(s * FPI, FPI)))
            for step in seg_end(s, False, None)[5:]:
                run(step)
        out_copy(pl.multiple_of(s * L, L), L, s).start()
        return c

    lax.fori_loop(0, NSEG - 1, seg_att, 0)

    npatch = (NSEG - 1) * TPS

    def patch_tile(idx):
        return jnp.where(idx < npatch * T, idx // T, 0)

    tile0 = patch_tile(i1)
    tile1 = patch_tile(i2)
    tile1 = jnp.where(tile1 == tile0, (tile0 + 1) % npatch, tile1)

    def patch(tile):
        c0 = pl.multiple_of(tile * T, T)
        rid = lax.broadcasted_iota(i32, (T, T), 0)
        tok_l = lax.broadcasted_iota(i32, (T, T), 1) + c0
        hit = ((rid == HT) & (tok_l == i1)) | ((rid == HT + 1) & (tok_l == i2))
        onehot = jnp.where(hit, 1.0, 0.0).astype(bf16)
        for rc in range(4):
            r0, r1 = rc * (D // 4), (rc + 1) * (D // 4)
            upd = jnp.dot(_bf(wot_u[r0 // 2:r1 // 2, DP - T:DP]), onehot, preferred_element_type=f32)
            cur = out_buf[r0:r1, pl.ds(c0, T)].astype(f32)
            out_buf[r0:r1, pl.ds(c0, T)] = (cur + upd).astype(bf16)

    patch_copies = [out_copy(pl.multiple_of(tile0 * T, T), T, 7), out_copy(pl.multiple_of(tile1 * T, T), T, 8)]
    last_copies = [out_copy((NSEG - 1) * L + tt * T, T, NSEG - 1 + tt) for tt in range(TPS)]

    sl = NSEG - 1
    ul = UPS * sl
    with _scope("tail_1"):
        moe_finish()
        run(pair_tasks((ul + 1, 1), (ul, 0)))
        for s in range(NSEG - 1):
            out_copy(s * L, L, s).wait()
    with _scope("tail_2"):
        patch(tile0)
        patch(tile1)
        run(pair_tasks((ul + 2, 0), (ul + 1, 1)))
        for cp in patch_copies:
            cp.start()
        steps = seg_end(sl, True, None)
        for step in steps[0:5]:
            run(step)
        last_copies[3].start()
        last_copies[2].start()
    with _scope("tail_3"):
        run(steps[5])
        run(steps[6])
        last_copies[1].start()
        last_copies[0].start()

    with _scope("out_wait"):
        for cp in patch_copies + last_copies:
            cp.wait()


@jax.jit
def pallas_parallel_sum__memory_aug_infini_attn__moe_arch_mod__prompt_kernel(
    A_x: jax.Array,
    A_wq: jax.Array,
    A_wk: jax.Array,
    A_wv: jax.Array,
    A_wo: jax.Array,
    A_beta: jax.Array,
    B_x: jax.Array,
    B_w_r: jax.Array,
    B_w_gate: jax.Array,
    B_w_up: jax.Array,
    B_w_down: jax.Array,
):
    del B_x
    any_spec = pl.BlockSpec(memory_space=pl.ANY)
    scratch = [
        pltpu.VMEM((H,), bf16),
        pltpu.VMEM((D,), bf16),
        pltpu.VMEM((D, SEQ), bf16),
        pltpu.VMEM((4, D, D), bf16),
        pltpu.VMEM((D, F), bf16),
        pltpu.VMEM((D, F), bf16),
        pltpu.VMEM((D, F), bf16),
        pltpu.VMEM((D, SEQ), bf16),
        pltpu.VMEM((WT_ROWS, DP), u32),
        pltpu.VMEM((D // 2, DP), u32),
        pltpu.VMEM((D // 2, DP), u32),
        pltpu.VMEM((NT, DP // 2, T), u32),
        pltpu.VMEM((NSEG * NG, TW, L), u32),
        pltpu.VMEM((NSEG * NG, L // 2, T), u32),
        pltpu.VMEM((NSEG * NG, TW, L), u32),
        pltpu.VMEM((NSEG * NG, TW, L), u32),
        pltpu.VMEM((NSEG, D // 2, L), u32),
        pltpu.VMEM((NSEG * H, 16, L), u32),
        pltpu.VMEM((NSEG, 8, L), f32),
        pltpu.VMEM((NG, T + 16, T), f32),
        pltpu.VMEM((NSEG, D, L), f32),
        pltpu.VMEM((NG, 16, T), f32),
        pltpu.VMEM((H, 8, T), f32),
        pltpu.VMEM((3, HT, T), f32),
        pltpu.VMEM((HPG, TW, T), u32),
        pltpu.VMEM((8, 32, T), i32),
        pltpu.VMEM((NP, 4, 2 * L, T), f32),
        pltpu.VMEM((NP, 4, 2, 8, T), f32),
        pltpu.VMEM((NP, 4, 2 * L, T), f32),
        pltpu.VMEM((NP, 4, 2, 8, T), f32),
        pltpu.VMEM((DP, L), f32),
        pltpu.VMEM((2, D, LNW), f32),
        pltpu.VMEM((2, 2, 8, LNW), f32),
        pltpu.VMEM((16, D), f32),
        pltpu.VMEM((8, DP), u32),
        pltpu.VMEM((FPI, 2, 16, T), f32),
        pltpu.SemaphoreType.DMA((NSEM,)),
    ]
    x_t = jnp.transpose(A_x, (0, 2, 1)).reshape(D, SEQ)
    out_t = pl.pallas_call(
        _kernel,
        out_shape=jax.ShapeDtypeStruct((D, SEQ), bf16),
        in_specs=[any_spec] * 10,
        out_specs=any_spec,
        scratch_shapes=scratch,
        compiler_params=pltpu.CompilerParams(vmem_limit_bytes=110 * 1024 * 1024),
    )(x_t, A_wq, A_wk, A_wv, A_wo, A_beta, B_w_r, B_w_gate, B_w_up, B_w_down.T)
    return jnp.transpose(out_t.reshape(1, D, SEQ), (0, 2, 1))
```

```python
import contextlib

import jax
import jax.numpy as jnp
from jax import lax
from jax.experimental import pallas as pl
from jax.experimental.pallas import tpu as pltpu

bf16 = jnp.bfloat16
f32 = jnp.float32
u32 = jnp.uint32
i32 = jnp.int32

SEQ = 2048
D = 576
DP = 640
H = 32
DH = 18
NSEG = 4
L = 512
T = 128
TW = T // 2
HT = T // 2
TPS = L // T
HPG = 6
NG = 6
F = 4608
FPI = 12
FPB = 3
NFT = F // T
NP = 4
UPS = H // (2 * NP)
NUNIT = NSEG * UPS
NT = SEQ // T
LNW = 256
VB = 8 * DH

LOG2E = 1.4426950408889634
QSCALE = (DH ** -0.5) * LOG2E
MASKVAL = -1000000000.0 * LOG2E
EPS_BF16 = 1.0013580322265625e-05
ONES_PAIR = 0x3F803F80

NT_DIMS = (((1,), (1,)), ((), ()))

WT_Q = 0
WT_K = NG * TW
WT_V = 2 * NG * TW
WT_ROWS = WT_V + D // 2

X_PIECES = ((0, LNW), (LNW, LNW), (L, L), (2 * L, L), (3 * L, L))
SEM_X = 0
SEM_W = 5
SEM_MOE = 9
SEM_OUT = 12
SEM_SMALL = 21
NSEM = 23


PROFILE_SCOPES = False
PACE = False
TAIL_BARRIERS = False
QT_ORDER = (3, 2, 1, 0)


def _scope(name):
    return jax.named_scope(name) if PROFILE_SCOPES else contextlib.nullcontext()


def _valid(g):
    return min(HPG * DH, D - g * HPG * DH)


def _rows(g):
    return -(-_valid(g) // 16) * 16


def _ewin(g):
    start = (g * HPG * DH // 16) * 16
    return start, g * HPG * DH - start, min(T, D - start)


def _bf(x):
    return pltpu.bitcast(x, bf16)


def _pack(x):
    return pltpu.bitcast(x.astype(bf16), u32)


def _round_bf16(x):
    return x.astype(bf16).astype(f32)


def _phi(t):
    return jnp.where(t > 0, t + 1.0, jnp.exp(t))


def _sigmoid(t):
    return 1.0 / (1.0 + jnp.exp(-t))


def _zero_after(v):
    bits = pltpu.bitcast(v[0:8, 0:LNW], u32)
    sixteen = jnp.uint32(16)
    bits = lax.shift_right_logical(lax.shift_right_logical(bits, sixteen), sixteen)
    return pltpu.bitcast(bits, f32) if PACE else None


def _interleave(*lists):
    items = []
    for li, tasks in enumerate(lists):
        for k, t in enumerate(tasks):
            items.append(((k + 0.5) / len(tasks), li, k, t))
    items.sort(key=lambda it: it[:3])
    return [it[3] for it in items]


def _kernel(x_hbm, wq_hbm, wk_hbm, wv_hbm, wo_hbm, beta_hbm, wr_hbm, wg_hbm, wu_hbm, wd_hbm,
            out_hbm,
            beta_ref, wr_ref, x_buf, w_buf, wg_buf, wu_buf, wd_buf, out_buf,
            wt_u, wtd_u, wot_u, xn_u, qs_u, k_u, pq_u, pk_u, vt_u, vwin,
            r_buf, mt_acc, am, g16, omg, mb, rowmask, smask,
            s0, m0, s1, m1, ot0, ot1, ot2, ot3, xf, ln_stat, y_acc, xsel_buf, hid_buf, sems):

    def x_copy(i):
        c0, width = X_PIECES[i]
        return pltpu.make_async_copy(x_hbm.at[:, pl.ds(c0, width)], x_buf.at[:, pl.ds(c0, width)],
                                     sems.at[SEM_X + i])

    def w_copy(i):
        src = (wq_hbm, wk_hbm, wv_hbm, wo_hbm)[i]
        return pltpu.make_async_copy(src, w_buf.at[i], sems.at[SEM_W + i])

    def moe_copy(i):
        src = (wg_hbm, wu_hbm, wd_hbm)[i]
        dst = (wg_buf, wu_buf, wd_buf)[i]
        return pltpu.make_async_copy(src, dst, sems.at[SEM_MOE + i])

    def out_copy(c0, width, sem):
        return pltpu.make_async_copy(out_buf.at[:, pl.ds(c0, width)], out_hbm.at[:, pl.ds(c0, width)],
                                     sems.at[SEM_OUT + sem])

    small_copies = [pltpu.make_async_copy(beta_hbm, beta_ref, sems.at[SEM_SMALL]),
                    pltpu.make_async_copy(wr_hbm, wr_ref, sems.at[SEM_SMALL + 1])]
    w_copy(0).start()
    x_copy(0).start()
    x_copy(1).start()
    for cp in small_copies:
        cp.start()
    w_copy(1).start()
    w_copy(2).start()

    init_scope = _scope("init")
    init_scope.__enter__()
    kr = lax.broadcasted_iota(i32, (HT, T), 0)
    ql = lax.broadcasted_iota(i32, (HT, T), 1)
    mb[0] = jnp.where(ql < kr, MASKVAL, 0.0).astype(f32)
    mb[1] = jnp.where((ql >= HT) & (ql - HT < kr), MASKVAL, 0.0).astype(f32)
    mb[2] = jnp.where(ql % HT < kr, MASKVAL, 0.0).astype(f32)
    for j in range(HPG):
        rowmask[j] = jnp.where((kr >= (DH // 2) * j) & (kr < (DH // 2) * (j + 1)), u32(0xFFFFFFFF), u32(0))
    r32 = lax.broadcasted_iota(i32, (32, T), 0)
    for i in range(8):
        smask[i] = jnp.where((r32 >= 2 * i) & (r32 < 2 * i + DH), 1, 0)
    zpad = jnp.zeros(((DP - D) // 2, T), u32)
    for tt in range(NT):
        xn_u[tt, D // 2:DP // 2, :] = zpad
    ots = (ot0, ot1, ot2, ot3)
    for o_ref in ots:
        o_ref[D:DP, :] = jnp.zeros((DP - D, T), f32)
    am[0] = jnp.zeros(am.shape[1:], f32)
    mt_acc[...] = jnp.zeros(mt_acc.shape, f32)
    g16[...] = jnp.zeros(g16.shape, f32)
    for sg in range(NSEG * NG):
        r2 = _rows(sg % NG) // 2
        qs_u[sg, r2:TW, :] = jnp.zeros((TW - r2, L), u32)
        pq_u[sg, r2:TW, :] = jnp.zeros((TW - r2, L), u32)
        pk_u[sg, r2:TW, :] = jnp.zeros((TW - r2, L), u32)

    init_scope.__exit__(None, None, None)

    pace = [None]

    def gate_tables():
        gate = _round_bf16(_sigmoid(beta_ref[...].reshape(1, H).astype(f32)))
        for h in range(H):
            gh = jnp.broadcast_to(gate[:, h:h + 1], (1, T))
            omg[h] = jnp.broadcast_to(_round_bf16(1.0 - gh), (8, T))
            g16[h // HPG, (h % HPG):(h % HPG) + 1, :] = gh

    def transpose_block(i, cb):
        c1 = min((cb + 1) * T, D)
        blk = w_buf[i, :, cb * T:c1]
        if c1 - cb * T < T:
            blk = jnp.concatenate([blk, jnp.zeros((D, T - (c1 - cb * T)), bf16)], axis=1)
        blk = jnp.concatenate([blk, jnp.zeros((DP - D, T), bf16)], axis=0)
        return pltpu.bitcast(blk.T, u32)

    def prep_dense(i, dst, base):
        def task(cb):
            nrow = min(TW, D // 2 - cb * TW)
            dst[base + cb * TW:base + cb * TW + nrow, :] = transpose_block(i, cb)[0:nrow]
        return [lambda cb=cb: task(cb) for cb in range(DP // T)]

    def prep_grouped(i, base):
        def regroup(g):
            nv, nr = _valid(g) // 2, _rows(g) // 2
            src = g * HPG * DH // 2
            wt_u[base + g * TW:base + g * TW + nv, :] = wtd_u[src:src + nv, :]
            pad = jnp.zeros((nr - nv, DP), u32)
            if i == 1 and g == 0:
                wr = wr_ref[...].reshape(1, D).astype(f32)
                wr = jnp.concatenate([wr, jnp.zeros((1, DP - D), f32)], axis=1)
                bits = lax.shift_right_logical(pltpu.bitcast(wr, u32), u32(16))
                rid = lax.broadcasted_iota(i32, (nr - nv, DP), 0)
                pad = jnp.where(rid == 0, bits, pad)
            wt_u[base + g * TW + nv:base + g * TW + nr, :] = pad
        return prep_dense(i, wtd_u, 0) + [lambda g=g: regroup(g) for g in range(NG)]

    def ln_tasks(s):
        def mean_pass(b):
            c0 = s * L + b * LNW
            if not isinstance(s, int):
                c0 = pl.multiple_of(c0, LNW)
            acc = pace[0]
            for r in range(0, D, 64):
                x = x_buf[r:r + 64, pl.ds(c0, LNW)].astype(f32)
                xf[b, r:r + 64, :] = x
                part = jnp.sum(x.reshape(8, 8, LNW), axis=0)
                acc = part if acc is None else acc + part
            mean = jnp.sum(acc, axis=0, keepdims=True) / D
            ln_stat[b, 0] = jnp.broadcast_to(mean, (8, LNW))

        def var_pass(b):
            bd = b
            mean = ln_stat[b, 0][0:1]
            if pace[0] is not None:
                mean = mean + pace[0][0:1]
            acc = None
            for r in range(0, D, 96):
                xc = xf[bd, r:r + 96, :] - mean
                part = jnp.sum((xc * xc).reshape(12, 8, LNW), axis=0)
                acc = part if acc is None else acc + part
            var = jnp.sum(acc, axis=0, keepdims=True) / D
            den = _round_bf16(jnp.sqrt(_round_bf16(_round_bf16(var) + EPS_BF16)))
            ln_stat[b, 1] = jnp.broadcast_to(1.0 / den, (8, LNW))
            ln_stat[b, 0] = jnp.broadcast_to(_round_bf16(mean), (8, LNW))

        def norm_pass(b, half):
            bd = b
            mean_b = ln_stat[b, 0][0:1]
            if pace[0] is not None:
                mean_b = mean_b + pace[0][0:1]
            inv = ln_stat[b, 1][0:1]
            for r in range(half * (D // 2), (half + 1) * (D // 2), 48):
                xn = _pack(_round_bf16(xf[bd, r:r + 48, :] - mean_b) * inv)
                for t in range(LNW // T):
                    tt = b * (LNW // T) + t
                    xn_u[s * TPS + tt, r // 2:r // 2 + 24, :] = xn[:, t * T:(t + 1) * T]

        tasks = []
        for b in range(L // LNW):
            tasks += [lambda b=b: mean_pass(b), lambda b=b: var_pass(b),
                      lambda b=b: norm_pass(b, 0), lambda b=b: norm_pass(b, 1)]
        return tasks

    def load_xs(s, t0, t1):
        return jnp.concatenate([_bf(xn_u[s * TPS + tt]) for tt in range(t0, t1)], axis=1)

    def q_task(s, g, t0=0, t1=TPS):
        nr = _rows(g) // 2
        w = _bf(wt_u[WT_Q + g * TW:WT_Q + g * TW + nr, :])
        q = jnp.dot(w, load_xs(s, t0, t1), preferred_element_type=f32)
        pace[0] = _zero_after(q)
        qp = _pack(q * QSCALE)
        qrot = jnp.concatenate([pltpu.roll(qp[:, t * T:(t + 1) * T], HT, 1) for t in range(t1 - t0)], axis=1)
        rid = lax.broadcasted_iota(i32, qp.shape, 0)
        even = ((rid // (DH // 2)) % 2) == 0
        qs_u[s * NG + g, 0:nr, t0 * T:t1 * T] = jnp.where(even, qrot, qp)
        pq_u[s * NG + g, 0:nr, t0 * T:t1 * T] = _pack(_phi(_round_bf16(q)))

    def k_task(s, g):
        nr = _rows(g)
        w = _bf(wt_u[WT_K + g * TW:WT_K + g * TW + nr // 2, :])
        k = jnp.dot(w, load_xs(s, 0, TPS), preferred_element_type=f32)
        pace[0] = _zero_after(k)
        if g == 0:
            r_buf[s] = jnp.broadcast_to(k[_valid(0):_valid(0) + 1, :], (8, L))
        kp = _pack(k)
        pk_u[s * NG + g, 0:nr // 2, :] = _pack(_phi(_round_bf16(k)))
        kfull = _bf(jnp.concatenate([kp, jnp.zeros(((T - nr) // 2, L), u32)], axis=0))
        k_u[s * NG + g] = pltpu.bitcast(kfull.T, u32)

    def v_task(s, b):
        w = _bf(wt_u[WT_V + b * (VB // 2):WT_V + (b + 1) * (VB // 2), :])
        v = jnp.dot(w, load_xs(s, 0, TPS), preferred_element_type=f32)
        pace[0] = _zero_after(v)
        v = _pack(v)
        vt_u[s, b * (VB // 2):(b + 1) * (VB // 2), :] = v
        sub = lax.broadcasted_iota(i32, (16, L), 0)
        for hh in range(8):
            w8 = (9 * hh) // 8
            ones_row = 0 if 2 * hh == 14 else 15
            vwin[s * H + 8 * b + hh] = jnp.where(sub == ones_row, u32(ONES_PAIR), v[8 * w8:8 * w8 + 16, :])

    def q_tasks(s, t0=0, t1=TPS):
        return [lambda g=g: q_task(s, g, t0, t1) for g in range(NG)]

    def k_tasks(s):
        return [lambda g=g: k_task(s, g) for g in range(NG)]

    def v_tasks(s):
        return [lambda b=b: v_task(s, b) for b in range(D // VB)]

    def run(tasks):
        for t in tasks:
            t()

    ln0 = ln_tasks(0)
    prep_q = prep_grouped(0, WT_Q)
    with _scope("p1_wait_wq"):
        w_copy(0).wait()
    with _scope("p1_prep_q"):
        run(prep_q[0:3])
        x_copy(0).wait()
    for i in range(2, len(X_PIECES)):
        x_copy(i).start()
    w_copy(3).start()
    for i in range(3):
        moe_copy(i).start()
    with _scope("p1_ln0a"):
        run(_interleave(prep_q[3:], ln0[0:4]))
        x_copy(1).wait()
    with _scope("p1_q0a"):
        run(_interleave(q_tasks(0, 0, 2), ln0[4:8]))
        w_copy(1).wait()
        for cp in small_copies:
            cp.wait()
    with _scope("p1_q0b"):
        run(_interleave(q_tasks(0, 2, 4), prep_grouped(1, WT_K), [gate_tables]))
        w_copy(2).wait()
    with _scope("p1_k0"):
        run(_interleave(k_tasks(0), prep_dense(2, wt_u, WT_V)))
        x_copy(2).wait()
    with _scope("p1_v0"):
        run(_interleave(v_tasks(0), ln_tasks(1)))

    def seg_body(s, c):
        for ss in range(2, NSEG):
            @pl.when(s + 1 == ss)
            def _():
                x_copy(ss + 1).wait()
        nxt = jnp.minimum(s + 1, NSEG - 1)
        pace[0] = None
        with _scope("p1_seg"):
            run(_interleave(q_tasks(s) + k_tasks(s) + v_tasks(s), ln_tasks(nxt)))
        return c

    lax.fori_loop(1, NSEG, seg_body, 0)

    row64 = lax.broadcasted_iota(i32, (TW, T), 0)
    lane64 = lax.broadcasted_iota(i32, (TW, T), 1)
    row32 = lax.broadcasted_iota(i32, (32, T), 0)
    lane32 = lax.broadcasted_iota(i32, (32, T), 1)
    lane1 = lax.broadcasted_iota(i32, (1, T), 1)
    lane8 = lax.broadcasted_iota(i32, (8, T), 1)

    def stage_a(unit, u, qt, s_ref, m_ref):
        s = unit // UPS
        pi = (unit % UPS) * NP + u
        g = pi // (HPG // 2)
        j = 2 * (pi - (HPG // 2) * g)
        sg = s * NG + g
        n = T * (qt + 1)
        qw = qs_u[sg, :, qt * T:(qt + 1) * T]
        w_a = qw & rowmask[j]
        w_b = qw & rowmask[j + 1]
        w_ab = _bf(jnp.where(lane64 < HT, w_a, w_b))

        def colmax8(v):
            return jnp.max(v.reshape(v.shape[0] // 8, 8, T), axis=0)

        maxes = []
        for hd, w in enumerate((_bf(w_a), _bf(w_b))):
            m8 = None
            for c in range(qt):
                kc = _bf(k_u[sg, c * TW:(c + 1) * TW, :])
                sc = jnp.dot(kc, w, preferred_element_type=f32)
                s_ref[u, qt, hd * L + c * T:hd * L + (c + 1) * T, :] = sc
                m8 = colmax8(sc) if m8 is None else jnp.maximum(m8, colmax8(sc))
            kc = _bf(k_u[sg, qt * TW:qt * TW + TW // 2, :])
            sc = jnp.dot(kc, w, preferred_element_type=f32) + mb[1 - hd]
            s_ref[u, qt, hd * L + qt * T:hd * L + qt * T + HT, :] = sc
            m8 = colmax8(sc) if m8 is None else jnp.maximum(m8, colmax8(sc))
            maxes.append(m8)
        kc = _bf(k_u[sg, qt * TW + TW // 2:(qt + 1) * TW, :])
        sc = jnp.dot(kc, w_ab, preferred_element_type=f32) + mb[2]
        s_ref[u, qt, n - HT:n, :] = sc
        mab = colmax8(sc)
        m_a = jnp.where(lane8 < HT, jnp.maximum(maxes[0], mab), maxes[0])
        m_b = jnp.where(lane8 >= HT, jnp.maximum(maxes[1], mab), maxes[1])
        m_ref[u, qt, 0] = jnp.broadcast_to(jnp.max(m_a, axis=0, keepdims=True), (8, T))
        m_ref[u, qt, 1] = jnp.broadcast_to(jnp.max(m_b, axis=0, keepdims=True), (8, T))

    def stage_b(unit, u, qt, s_ref, m_ref):
        s = unit // UPS
        pi = (unit % UPS) * NP + u
        n = T * (qt + 1)
        m_a = m_ref[u, qt, 0][0:1]
        m_b = m_ref[u, qt, 1][0:1]
        p_ab = jnp.exp2(s_ref[u, qt, n - HT:n, :] - jnp.where(lane1 < HT, m_a, m_b))
        for hd, m in enumerate((m_a, m_b)):
            h = 2 * pi + hd
            p = jnp.exp2(s_ref[u, qt, hd * L:hd * L + n - HT, :] - m)
            keep = (lane64 < HT) if hd == 0 else (lane64 >= HT)
            p = jnp.concatenate([p, jnp.where(keep, p_ab, 0.0)], axis=0).astype(bf16)
            w8 = (9 * h) // 8
            off = DH * h - 16 * w8
            o = jnp.dot(_bf(vwin[s * H + h, :, 0:n]), p, preferred_element_type=f32)
            den = jnp.where(off == 14, o[0:1], o[31:32])
            o = o * (omg[h][0:1] / den)
            if hd == 0:
                o = pltpu.roll(o, HT, 1)
            r1 = pl.multiple_of(16 * w8, 16)
            res = am[s, pl.ds(r1, 32), qt * T:(qt + 1) * T] + o
            pltpu.store(ots[qt].at[pl.ds(r1, 32), :], res, mask=smask[off // 2] != 0)

    def a_tasks(unit, s_ref, m_ref):
        return [lambda u=u, qt=qt: stage_a(unit, u, qt, s_ref, m_ref) for u in range(NP) for qt in QT_ORDER]

    def b_tasks(unit, s_ref, m_ref):
        return [lambda u=u, qt=qt: stage_b(unit, u, qt, s_ref, m_ref) for u in range(NP) for qt in QT_ORDER]

    ones16 = jnp.where(lax.broadcasted_iota(i32, (8, L), 0) == 0, u32(0x3F80), u32(0))

    def mem_task(s, g):
        es, eoff, ne = _ewin(g)
        nv = _valid(g)
        lhs = _bf(jnp.concatenate([vt_u[s, es // 2:(es + ne) // 2, :], ones16], axis=0))
        upd = lax.dot_general(lhs, _bf(pk_u[s * NG + g]), NT_DIMS, preferred_element_type=f32)
        mt = mt_acc[g, 0:ne + 16, :] + upd
        mt_acc[g, 0:ne + 16, :] = mt
        e_loc = lax.broadcasted_iota(i32, (ne, T), 0) - eoff
        d_id = lax.broadcasted_iota(i32, (ne, T), 1)
        same_head = (e_loc >= 0) & (e_loc < nv) & (d_id < nv) & ((e_loc // DH) == (d_id // DH))
        j16 = lax.broadcasted_iota(i32, (16, T), 0)
        d16 = lax.broadcasted_iota(i32, (16, T), 1)
        z_mask = ((d16 // DH) == j16) & (d16 < nv)
        lm = jnp.concatenate(
            [jnp.where(same_head, mt[0:ne], 0.0),
             jnp.where(z_mask, jnp.broadcast_to(mt[ne:ne + 1, :], (16, T)), 0.0)], axis=0)
        nd = jnp.dot(lm.astype(bf16), _bf(pq_u[(s + 1) * NG + g]), preferred_element_type=f32)
        scale = jnp.broadcast_to(g16[g][:, 0:1], (16, L)) / (nd[ne:ne + 16, :] + 1e-6)
        r8 = lax.broadcasted_iota(i32, (8, L), 0)
        for b in range(ne // 8):
            lo, hi = 8 * b - eoff, 8 * b + 7 - eoff
            if hi < 0 or lo >= nv:
                continue
            j1, j2 = max(lo, 0) // DH, min(hi, nv - 1) // DH
            sc = jnp.broadcast_to(scale[j1:j1 + 1, :], (8, L))
            if j2 != j1:
                sc = jnp.where(r8 < DH * j2 - lo, sc, jnp.broadcast_to(scale[j2:j2 + 1, :], (8, L)))
            val = nd[8 * b:8 * b + 8, :] * sc
            dst = am.at[s + 1, es + 8 * b:es + 8 * b + 8, :]
            if lo >= 0 and hi < nv:
                dst[...] = val
            else:
                pltpu.store(dst, val, mask=(r8 + lo >= 0) & (r8 + lo < nv))

    mem_tasks = [lambda s=s, g=g: mem_task(s, g) for s in range(NSEG - 1) for g in range(NG)]

    w_copy(3).wait()
    for i in range(3):
        moe_copy(i).wait()
    rr = jnp.concatenate([r_buf[s][0:1, :] for s in range(NSEG)], axis=0)
    rr = _round_bf16(rr)
    tok = lax.broadcasted_iota(i32, (NSEG, L), 0) * L + lax.broadcasted_iota(i32, (NSEG, L), 1)
    m1v = jnp.max(rr)
    i1 = jnp.min(jnp.where(rr == m1v, tok, SEQ))
    rr2 = jnp.where(tok == i1, -jnp.inf, rr)
    m2v = jnp.max(rr2)
    i2 = jnp.min(jnp.where(rr2 == m2v, tok, SEQ))
    i1 = jnp.clip(i1, 0, SEQ - 1)
    i2 = jnp.clip(i2, 0, SEQ - 1)

    row16 = lax.broadcasted_iota(i32, (16, T), 0)
    lane16 = lax.broadcasted_iota(i32, (16, T), 1)

    def token_rows(i, slot):
        onehot = jnp.where((row16 == slot) & (lane16 == i % T), 1.0, 0.0).astype(bf16)
        return lax.dot_general(onehot, _bf(xn_u[i // T]), NT_DIMS, preferred_element_type=f32)

    def select_task():
        xsel_buf[...] = _pack(token_rows(i1, 0) + token_rows(i2, 1))
        y_acc[...] = jnp.zeros(y_acc.shape, f32)

    def fcols(ft):
        return pl.ds(ft * T if isinstance(ft, int) else pl.multiple_of(ft * T, T), T)

    def moe_up_task(ft, k, which):
        xsel = _bf(xsel_buf[:, 0:D])
        w_ref = (wg_buf, wu_buf)[which]
        hid_buf[k, which] = jnp.dot(xsel, w_ref[:, fcols(ft)], preferred_element_type=f32)

    def moe_down_task(ft, k):
        gt = _round_bf16(hid_buf[k, 0])
        up = _round_bf16(hid_buf[k, 1])
        hid = (_round_bf16(gt * _sigmoid(gt)) * up).astype(bf16)
        y_acc[...] += lax.dot_general(hid, wd_buf[:, fcols(ft)], NT_DIMS, preferred_element_type=f32)

    def moe_tasks(ft0, count):
        tasks = []
        for k0 in range(0, count, FPB):
            ks = range(k0, min(k0 + FPB, count))
            tasks += [lambda k=k, w=w: moe_up_task(ft0 + k, k, w) for k in ks for w in range(2)]
            tasks += [lambda k=k: moe_down_task(ft0 + k, k) for k in ks]
        return tasks

    def moe_finish():
        y = _round_bf16(y_acc[...])
        rsel = jnp.where(lax.broadcasted_iota(i32, (16, 1), 0) == 0, m1v, m2v)
        y = _round_bf16(y * _round_bf16(_sigmoid(rsel)))
        y = jnp.concatenate([y, jnp.zeros((16, DP - D), f32)], axis=1)
        y = jnp.concatenate([jnp.zeros((HT, DP), f32), y, jnp.zeros((T - HT - 16, DP), f32)], axis=0)
        y_t = jnp.concatenate([y.T[0:D], jnp.zeros((D, T), f32)], axis=1)
        y_u = _pack(y_t)[:, 0:T]
        lane = lax.broadcasted_iota(i32, (D // 2, T), 1)
        wot_u[:, DP - T:DP] = jnp.where(lane < HT, wot_u[:, DP - T:DP], y_u)
        rid = lax.broadcasted_iota(i32, (8, T), 0)
        for tt in range(TPS):
            tok_l = lax.broadcasted_iota(i32, (8, T), 1) + (NSEG - 1) * L + tt * T
            ots[tt][D:D + 8, :] = jnp.where(((rid == 0) & (tok_l == i1)) | ((rid == 1) & (tok_l == i2)), 1.0, 0.0)

    dense = _interleave(mem_tasks, a_tasks(0, s0, m0), prep_dense(3, wot_u, 0))
    with _scope("p15_mix"):
        run(dense[0:2] + [select_task] + dense[2:])

    def out_tile(s, tt, last):
        c0 = s * L + tt * T
        if not isinstance(s, int):
            c0 = pl.multiple_of(c0, T)
        o_bf = ots[tt][...].astype(bf16)
        nchunk = 4
        rows = D // nchunk
        for rc in range(nchunk):
            r0 = rc * rows
            attn = jnp.dot(_bf(wot_u[r0 // 2:(r0 + rows) // 2, :]), o_bf, preferred_element_type=f32)
            xn = _bf(xn_u[s * TPS + tt, r0 // 2:(r0 + rows) // 2, :]).astype(f32)
            x = x_buf[r0:r0 + rows, pl.ds(c0, T)].astype(f32)
            res = x + attn + xn
            out_buf[r0:r0 + rows, pl.ds(c0, T)] = res.astype(bf16)

    bufs = ((s0, m0), (s1, m1))

    def pair_tasks(ua, ub):
        tasks = []
        for x, y in zip(a_tasks(ua[0], *bufs[ua[1]]), b_tasks(ub[0], *bufs[ub[1]])):
            tasks += [y, x]
        return tasks

    def seg_end(s, last, extra_first):
        u2, u3 = UPS * s + 2, UPS * s + 3

        def by_qt(fn, unit, par, qt):
            return [lambda u=u: fn(unit, u, qt, *bufs[par]) for u in range(NP)]

        steps = []
        for step in range(7):
            lists = []
            if step < 4:
                lists.append(by_qt(stage_b, u2, 0, 3 - step))
                lists.append(by_qt(stage_a, u3, 1, 3 - step))
            if 1 <= step < 5:
                lists.append(by_qt(stage_b, u3, 1, 4 - step))
            if not last and 2 <= step < 6:
                lists.append(by_qt(stage_a, u3 + 1, 0, 5 - step))
            if step >= 3:
                lists.append([lambda tt=6 - step: out_tile(s, tt, last)])
            steps.append(_interleave(*lists))
        return steps

    def seg_att(s, c):
        u0 = UPS * s
        tasks = pair_tasks((u0 + 1, 1), (u0, 0)) + pair_tasks((u0 + 2, 0), (u0 + 1, 1))
        for step in seg_end(s, False, None)[0:5]:
            tasks += step
        with _scope("att_seg"):
            run(_interleave(tasks, moe_tasks(s * FPI, FPI)))
            for step in seg_end(s, False, None)[5:]:
                run(step)
        out_copy(pl.multiple_of(s * L, L), L, s).start()
        return c

    lax.fori_loop(0, NSEG - 1, seg_att, 0)

    npatch = (NSEG - 1) * TPS

    def patch_tile(idx):
        return jnp.where(idx < npatch * T, idx // T, 0)

    tile0 = patch_tile(i1)
    tile1 = patch_tile(i2)
    tile1 = jnp.where(tile1 == tile0, (tile0 + 1) % npatch, tile1)

    def patch(tile):
        c0 = pl.multiple_of(tile * T, T)
        rid = lax.broadcasted_iota(i32, (T, T), 0)
        tok_l = lax.broadcasted_iota(i32, (T, T), 1) + c0
        hit = ((rid == HT) & (tok_l == i1)) | ((rid == HT + 1) & (tok_l == i2))
        onehot = jnp.where(hit, 1.0, 0.0).astype(bf16)
        for rc in range(4):
            r0, r1 = rc * (D // 4), (rc + 1) * (D // 4)
            upd = jnp.dot(_bf(wot_u[r0 // 2:r1 // 2, DP - T:DP]), onehot, preferred_element_type=f32)
            cur = out_buf[r0:r1, pl.ds(c0, T)].astype(f32)
            out_buf[r0:r1, pl.ds(c0, T)] = (cur + upd).astype(bf16)

    patch_copies = [out_copy(pl.multiple_of(tile0 * T, T), T, 7), out_copy(pl.multiple_of(tile1 * T, T), T, 8)]
    last_copies = [out_copy((NSEG - 1) * L + tt * T, T, NSEG - 1 + tt) for tt in range(TPS)]

    sl = NSEG - 1
    ul = UPS * sl
    with _scope("tail_1"):
        moe_finish()
        run(pair_tasks((ul + 1, 1), (ul, 0)))
        for s in range(NSEG - 1):
            out_copy(s * L, L, s).wait()
    with _scope("tail_2"):
        patch(tile0)
        patch(tile1)
        run(pair_tasks((ul + 2, 0), (ul + 1, 1)))
        for cp in patch_copies:
            cp.start()
        steps = seg_end(sl, True, None)
        for step in steps[0:5]:
            run(step)
        last_copies[3].start()
        last_copies[2].start()
    with _scope("tail_3"):
        run(steps[5])
        run(steps[6])
        last_copies[1].start()
        last_copies[0].start()

    with _scope("out_wait"):
        for cp in patch_copies + last_copies:
            cp.wait()


@jax.jit
def pallas_parallel_sum__memory_aug_infini_attn__moe_arch_mod__prompt_kernel(
    A_x: jax.Array,
    A_wq: jax.Array,
    A_wk: jax.Array,
    A_wv: jax.Array,
    A_wo: jax.Array,
    A_beta: jax.Array,
    B_x: jax.Array,
    B_w_r: jax.Array,
    B_w_gate: jax.Array,
    B_w_up: jax.Array,
    B_w_down: jax.Array,
):
    del B_x
    any_spec = pl.BlockSpec(memory_space=pl.ANY)
    scratch = [
        pltpu.VMEM((H,), bf16),
        pltpu.VMEM((D,), bf16),
        pltpu.VMEM((D, SEQ), bf16),
        pltpu.VMEM((4, D, D), bf16),
        pltpu.VMEM((D, F), bf16),
        pltpu.VMEM((D, F), bf16),
        pltpu.VMEM((D, F), bf16),
        pltpu.VMEM((D, SEQ), bf16),
        pltpu.VMEM((WT_ROWS, DP), u32),
        pltpu.VMEM((D // 2, DP), u32),
        pltpu.VMEM((D // 2, DP), u32),
        pltpu.VMEM((NT, DP // 2, T), u32),
        pltpu.VMEM((NSEG * NG, TW, L), u32),
        pltpu.VMEM((NSEG * NG, L // 2, T), u32),
        pltpu.VMEM((NSEG * NG, TW, L), u32),
        pltpu.VMEM((NSEG * NG, TW, L), u32),
        pltpu.VMEM((NSEG, D // 2, L), u32),
        pltpu.VMEM((NSEG * H, 16, L), u32),
        pltpu.VMEM((NSEG, 8, L), f32),
        pltpu.VMEM((NG, T + 16, T), f32),
        pltpu.VMEM((NSEG, D, L), f32),
        pltpu.VMEM((NG, 16, T), f32),
        pltpu.VMEM((H, 8, T), f32),
        pltpu.VMEM((3, HT, T), f32),
        pltpu.VMEM((HPG, TW, T), u32),
        pltpu.VMEM((8, 32, T), i32),
        pltpu.VMEM((NP, 4, 2 * L, T), f32),
        pltpu.VMEM((NP, 4, 2, 8, T), f32),
        pltpu.VMEM((NP, 4, 2 * L, T), f32),
        pltpu.VMEM((NP, 4, 2, 8, T), f32),
        pltpu.VMEM((DP, T), f32),
        pltpu.VMEM((DP, T), f32),
        pltpu.VMEM((DP, T), f32),
        pltpu.VMEM((DP, T), f32),
        pltpu.VMEM((2, D, LNW), f32),
        pltpu.VMEM((2, 2, 8, LNW), f32),
        pltpu.VMEM((16, D), f32),
        pltpu.VMEM((8, DP), u32),
        pltpu.VMEM((FPI, 2, 16, T), f32),
        pltpu.SemaphoreType.DMA((NSEM,)),
    ]
    x_t = jnp.transpose(A_x, (0, 2, 1)).reshape(D, SEQ)
    out_t = pl.pallas_call(
        _kernel,
        out_shape=jax.ShapeDtypeStruct((D, SEQ), bf16),
        in_specs=[any_spec] * 10,
        out_specs=any_spec,
        scratch_shapes=scratch,
        compiler_params=pltpu.CompilerParams(vmem_limit_bytes=110 * 1024 * 1024),
    )(x_t, A_wq, A_wk, A_wv, A_wo, A_beta, B_w_r, B_w_gate, B_w_up, B_w_down.T)
    return jnp.transpose(out_t.reshape(1, D, SEQ), (0, 2, 1))
```

```python
import contextlib

import jax
import jax.numpy as jnp
from jax import lax
from jax.experimental import pallas as pl
from jax.experimental.pallas import tpu as pltpu

bf16 = jnp.bfloat16
f32 = jnp.float32
u32 = jnp.uint32
i32 = jnp.int32

SEQ = 2048
D = 576
DP = 640
H = 32
DH = 18
NSEG = 4
L = 512
T = 128
TW = T // 2
HT = T // 2
TPS = L // T
HPG = 6
NG = 6
F = 4608
FPI = 12
FPB = 3
NFT = F // T
NP = 4
UPS = H // (2 * NP)
NUNIT = NSEG * UPS
NT = SEQ // T
LNW = 256
BT = LNW // T
NORM_PARTS = 6
VB = 8 * DH

LOG2E = 1.4426950408889634
QSCALE = (DH ** -0.5) * LOG2E
MASKVAL = -1000000000.0 * LOG2E
EPS_BF16 = 1.0013580322265625e-05
ONES_PAIR = 0x3F803F80

NT_DIMS = (((1,), (1,)), ((), ()))

WT_Q = 0
WT_K = NG * TW
WT_V = 2 * NG * TW
WT_ROWS = WT_V + D // 2

X_PIECES = ((0, LNW), (LNW, LNW), (L, L), (2 * L, L), (3 * L, L))
SEM_X = 0
SEM_W = 5
SEM_MOE = 9
SEM_OUT = 12
SEM_SMALL = 21
NSEM = 23


PROFILE_SCOPES = False
PACE = True
TAIL_BARRIERS = False
QT_ORDER = (3, 2, 1, 0)


def _scope(name):
    return jax.named_scope(name) if PROFILE_SCOPES else contextlib.nullcontext()


def _valid(g):
    return min(HPG * DH, D - g * HPG * DH)


def _rows(g):
    return -(-_valid(g) // 16) * 16


def _ewin(g):
    start = (g * HPG * DH // 16) * 16
    return start, g * HPG * DH - start, min(T, D - start)


def _bf(x):
    return pltpu.bitcast(x, bf16)


def _pack(x):
    return pltpu.bitcast(x.astype(bf16), u32)


def _round_bf16(x):
    return x.astype(bf16).astype(f32)


def _phi(t):
    return jnp.where(t > 0, t + 1.0, jnp.exp(t))


def _sigmoid(t):
    return 1.0 / (1.0 + jnp.exp(-t))


def _zero_after(v):
    bits = pltpu.bitcast(v[0:8, 0:LNW], u32)
    sixteen = jnp.uint32(16)
    bits = lax.shift_right_logical(lax.shift_right_logical(bits, sixteen), sixteen)
    return pltpu.bitcast(bits, f32) if PACE else None


def _interleave(*lists):
    items = []
    for li, tasks in enumerate(lists):
        for k, t in enumerate(tasks):
            items.append(((k + 0.5) / len(tasks), li, k, t))
    items.sort(key=lambda it: it[:3])
    return [it[3] for it in items]


def _kernel(x_hbm, wq_hbm, wk_hbm, wv_hbm, wo_hbm, beta_hbm, wr_hbm, wg_hbm, wu_hbm, wd_hbm,
            out_hbm,
            beta_ref, wr_ref, x_buf, w_buf, wg_buf, wu_buf, wd_buf, out_buf,
            wt_u, wtd_u, wot_u, xn_u, xs_a, xs_b, qs_u, k_u, pq_u, pk_u, vt_u, vwin,
            r_buf, mt_acc, am, g16, omg, mb, rowmask, smask,
            s0, m0, s1, m1, ot0, ot1, ot2, ot3, xf, ln_stat, y_acc, xsel_buf, hid_buf, sems):

    def x_copy(i):
        c0, width = X_PIECES[i]
        return pltpu.make_async_copy(x_hbm.at[:, pl.ds(c0, width)], x_buf.at[:, pl.ds(c0, width)],
                                     sems.at[SEM_X + i])

    def w_copy(i):
        src = (wq_hbm, wk_hbm, wv_hbm, wo_hbm)[i]
        return pltpu.make_async_copy(src, w_buf.at[i], sems.at[SEM_W + i])

    def moe_copy(i):
        src = (wg_hbm, wu_hbm, wd_hbm)[i]
        dst = (wg_buf, wu_buf, wd_buf)[i]
        return pltpu.make_async_copy(src, dst, sems.at[SEM_MOE + i])

    def out_copy(c0, width, sem):
        return pltpu.make_async_copy(out_buf.at[:, pl.ds(c0, width)], out_hbm.at[:, pl.ds(c0, width)],
                                     sems.at[SEM_OUT + sem])

    small_copies = [pltpu.make_async_copy(beta_hbm, beta_ref, sems.at[SEM_SMALL]),
                    pltpu.make_async_copy(wr_hbm, wr_ref, sems.at[SEM_SMALL + 1])]
    w_copy(0).start()
    x_copy(0).start()
    x_copy(1).start()
    for cp in small_copies:
        cp.start()
    w_copy(1).start()
    w_copy(2).start()

    init_scope = _scope("init")
    init_scope.__enter__()
    kr = lax.broadcasted_iota(i32, (HT, T), 0)
    ql = lax.broadcasted_iota(i32, (HT, T), 1)
    mb[0] = jnp.where(ql < kr, MASKVAL, 0.0).astype(f32)
    mb[1] = jnp.where((ql >= HT) & (ql - HT < kr), MASKVAL, 0.0).astype(f32)
    mb[2] = jnp.where(ql % HT < kr, MASKVAL, 0.0).astype(f32)
    for j in range(HPG):
        rowmask[j] = jnp.where((kr >= (DH // 2) * j) & (kr < (DH // 2) * (j + 1)), u32(0xFFFFFFFF), u32(0))
    r32 = lax.broadcasted_iota(i32, (32, T), 0)
    for i in range(8):
        smask[i] = jnp.where((r32 >= 2 * i) & (r32 < 2 * i + DH), 1, 0)
    zpad = jnp.zeros(((DP - D) // 2, T), u32)
    for tt in range(NT):
        xn_u[tt, D // 2:DP // 2, :] = zpad
    for tt in range(BT):
        xs_a[tt, D // 2:DP // 2, :] = zpad
        xs_b[tt, D // 2:DP // 2, :] = zpad
    ots = (ot0, ot1, ot2, ot3)
    for o_ref in ots:
        o_ref[D:DP, :] = jnp.zeros((DP - D, T), f32)
    am[0] = jnp.zeros(am.shape[1:], f32)
    mt_acc[...] = jnp.zeros(mt_acc.shape, f32)
    g16[...] = jnp.zeros(g16.shape, f32)
    for sg in range(NSEG * NG):
        r2 = _rows(sg % NG) // 2
        qs_u[sg, r2:TW, :] = jnp.zeros((TW - r2, L), u32)
        pq_u[sg, r2:TW, :] = jnp.zeros((TW - r2, L), u32)
        pk_u[sg, r2:TW, :] = jnp.zeros((TW - r2, L), u32)

    init_scope.__exit__(None, None, None)

    pace = [None]

    def gate_tables():
        gate = _round_bf16(_sigmoid(beta_ref[...].reshape(1, H).astype(f32)))
        for h in range(H):
            gh = jnp.broadcast_to(gate[:, h:h + 1], (1, T))
            omg[h] = jnp.broadcast_to(_round_bf16(1.0 - gh), (8, T))
            g16[h // HPG, (h % HPG):(h % HPG) + 1, :] = gh

    def transpose_block(i, cb):
        c1 = min((cb + 1) * T, D)
        blk = w_buf[i, :, cb * T:c1]
        if c1 - cb * T < T:
            blk = jnp.concatenate([blk, jnp.zeros((D, T - (c1 - cb * T)), bf16)], axis=1)
        blk = jnp.concatenate([blk, jnp.zeros((DP - D, T), bf16)], axis=0)
        return pltpu.bitcast(blk.T, u32)

    def prep_dense(i, dst, base):
        def task(cb):
            nrow = min(TW, D // 2 - cb * TW)
            dst[base + cb * TW:base + cb * TW + nrow, :] = transpose_block(i, cb)[0:nrow]
        return [lambda cb=cb: task(cb) for cb in range(DP // T)]

    def prep_grouped(i, base):
        def regroup(g):
            nv, nr = _valid(g) // 2, _rows(g) // 2
            src = g * HPG * DH // 2
            wt_u[base + g * TW:base + g * TW + nv, :] = wtd_u[src:src + nv, :]
            pad = jnp.zeros((nr - nv, DP), u32)
            if i == 1 and g == 0:
                wr = wr_ref[...].reshape(1, D).astype(f32)
                wr = jnp.concatenate([wr, jnp.zeros((1, DP - D), f32)], axis=1)
                bits = lax.shift_right_logical(pltpu.bitcast(wr, u32), u32(16))
                rid = lax.broadcasted_iota(i32, (nr - nv, DP), 0)
                pad = jnp.where(rid == 0, bits, pad)
            wt_u[base + g * TW + nv:base + g * TW + nr, :] = pad
        return prep_dense(i, wtd_u, 0) + [lambda g=g: regroup(g) for g in range(NG)]

    def ln_tasks(s, p, stage):
        c0 = s * L + p * LNW
        if not isinstance(s, int):
            c0 = pl.multiple_of(c0, LNW)

        def mean_pass():
            acc = pace[0]
            for r in range(0, D, 64):
                x = x_buf[r:r + 64, pl.ds(c0, LNW)].astype(f32)
                xf[p, r:r + 64, :] = x
                part = jnp.sum(x.reshape(8, 8, LNW), axis=0)
                acc = part if acc is None else acc + part
            mean = jnp.sum(acc, axis=0, keepdims=True) / D
            ln_stat[p, 0] = jnp.broadcast_to(mean, (8, LNW))

        def var_pass():
            mean = ln_stat[p, 0][0:1]
            if pace[0] is not None:
                mean = mean + pace[0][0:1]
            acc = None
            for r in range(0, D, 96):
                xc = xf[p, r:r + 96, :] - mean
                part = jnp.sum((xc * xc).reshape(12, 8, LNW), axis=0)
                acc = part if acc is None else acc + part
            var = jnp.sum(acc, axis=0, keepdims=True) / D
            den = _round_bf16(jnp.sqrt(_round_bf16(_round_bf16(var) + EPS_BF16)))
            ln_stat[p, 1] = jnp.broadcast_to(1.0 / den, (8, LNW))
            ln_stat[p, 0] = jnp.broadcast_to(_round_bf16(mean), (8, LNW))

        def norm_pass(part):
            mean_b = ln_stat[p, 0][0:1]
            if pace[0] is not None:
                mean_b = mean_b + pace[0][0:1]
            inv = ln_stat[p, 1][0:1]
            step = D // NORM_PARTS
            for r in range(part * step, (part + 1) * step, 48):
                xn = _pack(_round_bf16(xf[p, r:r + 48, :] - mean_b) * inv)
                for t in range(BT):
                    xn_u[s * TPS + p * BT + t, r // 2:r // 2 + 24, :] = xn[:, t * T:(t + 1) * T]
                    if stage is not None:
                        stage[t, r // 2:r // 2 + 24, :] = xn[:, t * T:(t + 1) * T]

        return [mean_pass, var_pass] + [lambda part=part: norm_pass(part) for part in range(NORM_PARTS)]

    def load_xs(s, p, stage):
        if stage is None:
            tiles = [xn_u[s * TPS + p * BT + t] for t in range(BT)]
        else:
            tiles = [stage[t] for t in range(BT)]
        return jnp.concatenate([_bf(t) for t in tiles], axis=1)

    def q_task(s, p, stage, g):
        nr = _rows(g) // 2
        cols = slice(p * LNW, (p + 1) * LNW)
        w = _bf(wt_u[WT_Q + g * TW:WT_Q + g * TW + nr, :])
        q = jnp.dot(w, load_xs(s, p, stage), preferred_element_type=f32)
        pace[0] = _zero_after(q)
        qp = _pack(q * QSCALE)
        qrot = jnp.concatenate([pltpu.roll(qp[:, t * T:(t + 1) * T], HT, 1) for t in range(BT)], axis=1)
        rid = lax.broadcasted_iota(i32, qp.shape, 0)
        even = ((rid // (DH // 2)) % 2) == 0
        qs_u[s * NG + g, 0:nr, cols] = jnp.where(even, qrot, qp)
        pq_u[s * NG + g, 0:nr, cols] = _pack(_phi(_round_bf16(q)))

    def k_task(s, p, stage, g):
        nr = _rows(g)
        cols = slice(p * LNW, (p + 1) * LNW)
        w = _bf(wt_u[WT_K + g * TW:WT_K + g * TW + nr // 2, :])
        k = jnp.dot(w, load_xs(s, p, stage), preferred_element_type=f32)
        pace[0] = _zero_after(k)
        if g == 0:
            r_buf[s, :, cols] = jnp.broadcast_to(k[_valid(0):_valid(0) + 1, :], (8, LNW))
        kp = _pack(k)
        pk_u[s * NG + g, 0:nr // 2, cols] = _pack(_phi(_round_bf16(k)))
        kfull = _bf(jnp.concatenate([kp, jnp.zeros(((T - nr) // 2, LNW), u32)], axis=0))
        k_u[s * NG + g, p * (LNW // 2):(p + 1) * (LNW // 2), :] = pltpu.bitcast(kfull.T, u32)

    def v_task(s, p, stage, b):
        cols = slice(p * LNW, (p + 1) * LNW)
        w = _bf(wt_u[WT_V + b * (VB // 2):WT_V + (b + 1) * (VB // 2), :])
        v = jnp.dot(w, load_xs(s, p, stage), preferred_element_type=f32)
        pace[0] = _zero_after(v)
        v = _pack(v)
        vt_u[s, b * (VB // 2):(b + 1) * (VB // 2), cols] = v
        sub = lax.broadcasted_iota(i32, (16, LNW), 0)
        for hh in range(8):
            w8 = (9 * hh) // 8
            ones_row = 0 if 2 * hh == 14 else 15
            vwin[s * H + 8 * b + hh, :, cols] = jnp.where(sub == ones_row, u32(ONES_PAIR), v[8 * w8:8 * w8 + 16, :])

    def q_tasks(s, p, stage=None):
        return [lambda g=g: q_task(s, p, stage, g) for g in range(NG)]

    def k_tasks(s, p, stage=None):
        return [lambda g=g: k_task(s, p, stage, g) for g in range(NG)]

    def v_tasks(s, p, stage=None):
        return [lambda b=b: v_task(s, p, stage, b) for b in range(D // VB)]

    def run(tasks):
        for t in tasks:
            t()

    prep_q = prep_grouped(0, WT_Q)
    with _scope("p1_wait_wq"):
        w_copy(0).wait()
    with _scope("p1_prep_q"):
        run(prep_q[0:3])
        x_copy(0).wait()
    for i in range(2, len(X_PIECES)):
        x_copy(i).start()
    w_copy(3).start()
    for i in range(3):
        moe_copy(i).start()
    with _scope("p1_ln0a"):
        run(_interleave(prep_q[3:], ln_tasks(0, 0, None)))
        x_copy(1).wait()
    with _scope("p1_q0a"):
        run(_interleave(q_tasks(0, 0), ln_tasks(0, 1, None)))
        w_copy(1).wait()
        for cp in small_copies:
            cp.wait()
    with _scope("p1_q0b"):
        run(_interleave(q_tasks(0, 1), prep_grouped(1, WT_K), [gate_tables]))
        w_copy(2).wait()
    with _scope("p1_k0"):
        run(_interleave(k_tasks(0, 0) + k_tasks(0, 1), prep_dense(2, wt_u, WT_V)))
        x_copy(2).wait()
    with _scope("p1_v0"):
        run(_interleave(v_tasks(0, 0) + v_tasks(0, 1), ln_tasks(1, 0, xs_a)))

    def seg_body(s, c):
        for ss in range(2, NSEG):
            @pl.when(s + 1 == ss)
            def _():
                x_copy(ss + 1).wait()
        nxt = jnp.minimum(s + 1, NSEG - 1)
        pace[0] = None
        with _scope("p1_seg"):
            first = q_tasks(s, 0, xs_a) + k_tasks(s, 0, xs_a) + v_tasks(s, 0, xs_a)
            run(_interleave(first, ln_tasks(s, 1, xs_b)))
            second = q_tasks(s, 1, xs_b) + k_tasks(s, 1, xs_b) + v_tasks(s, 1, xs_b)
            run(_interleave(second, ln_tasks(nxt, 0, xs_a)))
        return c

    lax.fori_loop(1, NSEG, seg_body, 0)

    row64 = lax.broadcasted_iota(i32, (TW, T), 0)
    lane64 = lax.broadcasted_iota(i32, (TW, T), 1)
    row32 = lax.broadcasted_iota(i32, (32, T), 0)
    lane32 = lax.broadcasted_iota(i32, (32, T), 1)
    lane1 = lax.broadcasted_iota(i32, (1, T), 1)
    lane8 = lax.broadcasted_iota(i32, (8, T), 1)

    def stage_a(unit, u, qt, s_ref, m_ref):
        s = unit // UPS
        pi = (unit % UPS) * NP + u
        g = pi // (HPG // 2)
        j = 2 * (pi - (HPG // 2) * g)
        sg = s * NG + g
        n = T * (qt + 1)
        qw = qs_u[sg, :, qt * T:(qt + 1) * T]
        w_a = qw & rowmask[j]
        w_b = qw & rowmask[j + 1]
        w_ab = _bf(jnp.where(lane64 < HT, w_a, w_b))

        def colmax8(v):
            return jnp.max(v.reshape(v.shape[0] // 8, 8, T), axis=0)

        maxes = []
        for hd, w in enumerate((_bf(w_a), _bf(w_b))):
            m8 = None
            for c in range(qt):
                kc = _bf(k_u[sg, c * TW:(c + 1) * TW, :])
                sc = jnp.dot(kc, w, preferred_element_type=f32)
                s_ref[u, qt, hd * L + c * T:hd * L + (c + 1) * T, :] = sc
                m8 = colmax8(sc) if m8 is None else jnp.maximum(m8, colmax8(sc))
            kc = _bf(k_u[sg, qt * TW:qt * TW + TW // 2, :])
            sc = jnp.dot(kc, w, preferred_element_type=f32) + mb[1 - hd]
            s_ref[u, qt, hd * L + qt * T:hd * L + qt * T + HT, :] = sc
            m8 = colmax8(sc) if m8 is None else jnp.maximum(m8, colmax8(sc))
            maxes.append(m8)
        kc = _bf(k_u[sg, qt * TW + TW // 2:(qt + 1) * TW, :])
        sc = jnp.dot(kc, w_ab, preferred_element_type=f32) + mb[2]
        s_ref[u, qt, n - HT:n, :] = sc
        mab = colmax8(sc)
        m_a = jnp.where(lane8 < HT, jnp.maximum(maxes[0], mab), maxes[0])
        m_b = jnp.where(lane8 >= HT, jnp.maximum(maxes[1], mab), maxes[1])
        m_ref[u, qt, 0] = jnp.broadcast_to(jnp.max(m_a, axis=0, keepdims=True), (8, T))
        m_ref[u, qt, 1] = jnp.broadcast_to(jnp.max(m_b, axis=0, keepdims=True), (8, T))

    def stage_b(unit, u, qt, s_ref, m_ref):
        s = unit // UPS
        pi = (unit % UPS) * NP + u
        n = T * (qt + 1)
        m_a = m_ref[u, qt, 0][0:1]
        m_b = m_ref[u, qt, 1][0:1]
        p_ab = jnp.exp2(s_ref[u, qt, n - HT:n, :] - jnp.where(lane1 < HT, m_a, m_b))
        for hd, m in enumerate((m_a, m_b)):
            h = 2 * pi + hd
            p = jnp.exp2(s_ref[u, qt, hd * L:hd * L + n - HT, :] - m)
            keep = (lane64 < HT) if hd == 0 else (lane64 >= HT)
            p = jnp.concatenate([p, jnp.where(keep, p_ab, 0.0)], axis=0).astype(bf16)
            w8 = (9 * h) // 8
            off = DH * h - 16 * w8
            o = jnp.dot(_bf(vwin[s * H + h, :, 0:n]), p, preferred_element_type=f32)
            den = jnp.where(off == 14, o[0:1], o[31:32])
            o = o * (omg[h][0:1] / den)
            if hd == 0:
                o = pltpu.roll(o, HT, 1)
            r1 = pl.multiple_of(16 * w8, 16)
            res = am[s, pl.ds(r1, 32), qt * T:(qt + 1) * T] + o
            pltpu.store(ots[qt].at[pl.ds(r1, 32), :], res, mask=smask[off // 2] != 0)

    def a_tasks(unit, s_ref, m_ref):
        return [lambda u=u, qt=qt: stage_a(unit, u, qt, s_ref, m_ref) for u in range(NP) for qt in QT_ORDER]

    def b_tasks(unit, s_ref, m_ref):
        return [lambda u=u, qt=qt: stage_b(unit, u, qt, s_ref, m_ref) for u in range(NP) for qt in QT_ORDER]

    ones16 = jnp.where(lax.broadcasted_iota(i32, (8, L), 0) == 0, u32(0x3F80), u32(0))

    def mem_task(s, g):
        es, eoff, ne = _ewin(g)
        nv = _valid(g)
        lhs = _bf(jnp.concatenate([vt_u[s, es // 2:(es + ne) // 2, :], ones16], axis=0))
        upd = lax.dot_general(lhs, _bf(pk_u[s * NG + g]), NT_DIMS, preferred_element_type=f32)
        mt = mt_acc[g, 0:ne + 16, :] + upd
        mt_acc[g, 0:ne + 16, :] = mt
        e_loc = lax.broadcasted_iota(i32, (ne, T), 0) - eoff
        d_id = lax.broadcasted_iota(i32, (ne, T), 1)
        same_head = (e_loc >= 0) & (e_loc < nv) & (d_id < nv) & ((e_loc // DH) == (d_id // DH))
        j16 = lax.broadcasted_iota(i32, (16, T), 0)
        d16 = lax.broadcasted_iota(i32, (16, T), 1)
        z_mask = ((d16 // DH) == j16) & (d16 < nv)
        lm = jnp.concatenate(
            [jnp.where(same_head, mt[0:ne], 0.0),
             jnp.where(z_mask, jnp.broadcast_to(mt[ne:ne + 1, :], (16, T)), 0.0)], axis=0)
        nd = jnp.dot(lm.astype(bf16), _bf(pq_u[(s + 1) * NG + g]), preferred_element_type=f32)
        scale = jnp.broadcast_to(g16[g][:, 0:1], (16, L)) / (nd[ne:ne + 16, :] + 1e-6)
        r8 = lax.broadcasted_iota(i32, (8, L), 0)
        for b in range(ne // 8):
            lo, hi = 8 * b - eoff, 8 * b + 7 - eoff
            if hi < 0 or lo >= nv:
                continue
            j1, j2 = max(lo, 0) // DH, min(hi, nv - 1) // DH
            sc = jnp.broadcast_to(scale[j1:j1 + 1, :], (8, L))
            if j2 != j1:
                sc = jnp.where(r8 < DH * j2 - lo, sc, jnp.broadcast_to(scale[j2:j2 + 1, :], (8, L)))
            val = nd[8 * b:8 * b + 8, :] * sc
            dst = am.at[s + 1, es + 8 * b:es + 8 * b + 8, :]
            if lo >= 0 and hi < nv:
                dst[...] = val
            else:
                pltpu.store(dst, val, mask=(r8 + lo >= 0) & (r8 + lo < nv))

    mem_tasks = [lambda s=s, g=g: mem_task(s, g) for s in range(NSEG - 1) for g in range(NG)]

    w_copy(3).wait()
    for i in range(3):
        moe_copy(i).wait()
    rr = jnp.concatenate([r_buf[s][0:1, :] for s in range(NSEG)], axis=0)
    rr = _round_bf16(rr)
    tok = lax.broadcasted_iota(i32, (NSEG, L), 0) * L + lax.broadcasted_iota(i32, (NSEG, L), 1)
    m1v = jnp.max(rr)
    i1 = jnp.min(jnp.where(rr == m1v, tok, SEQ))
    rr2 = jnp.where(tok == i1, -jnp.inf, rr)
    m2v = jnp.max(rr2)
    i2 = jnp.min(jnp.where(rr2 == m2v, tok, SEQ))
    i1 = jnp.clip(i1, 0, SEQ - 1)
    i2 = jnp.clip(i2, 0, SEQ - 1)

    row16 = lax.broadcasted_iota(i32, (16, T), 0)
    lane16 = lax.broadcasted_iota(i32, (16, T), 1)

    def token_rows(i, slot):
        onehot = jnp.where((row16 == slot) & (lane16 == i % T), 1.0, 0.0).astype(bf16)
        return lax.dot_general(onehot, _bf(xn_u[i // T]), NT_DIMS, preferred_element_type=f32)

    def select_task():
        xsel_buf[...] = _pack(token_rows(i1, 0) + token_rows(i2, 1))
        y_acc[...] = jnp.zeros(y_acc.shape, f32)

    def fcols(ft):
        return pl.ds(ft * T if isinstance(ft, int) else pl.multiple_of(ft * T, T), T)

    def moe_up_task(ft, k, which):
        xsel = _bf(xsel_buf[:, 0:D])
        w_ref = (wg_buf, wu_buf)[which]
        hid_buf[k, which] = jnp.dot(xsel, w_ref[:, fcols(ft)], preferred_element_type=f32)

    def moe_down_task(ft, k):
        gt = _round_bf16(hid_buf[k, 0])
        up = _round_bf16(hid_buf[k, 1])
        hid = (_round_bf16(gt * _sigmoid(gt)) * up).astype(bf16)
        y_acc[...] += lax.dot_general(hid, wd_buf[:, fcols(ft)], NT_DIMS, preferred_element_type=f32)

    def moe_tasks(ft0, count):
        tasks = []
        for k0 in range(0, count, FPB):
            ks = range(k0, min(k0 + FPB, count))
            tasks += [lambda k=k, w=w: moe_up_task(ft0 + k, k, w) for k in ks for w in range(2)]
            tasks += [lambda k=k: moe_down_task(ft0 + k, k) for k in ks]
        return tasks

    def moe_finish():
        y = _round_bf16(y_acc[...])
        rsel = jnp.where(lax.broadcasted_iota(i32, (16, 1), 0) == 0, m1v, m2v)
        y = _round_bf16(y * _round_bf16(_sigmoid(rsel)))
        y = jnp.concatenate([y, jnp.zeros((16, DP - D), f32)], axis=1)
        y = jnp.concatenate([jnp.zeros((HT, DP), f32), y, jnp.zeros((T - HT - 16, DP), f32)], axis=0)
        y_t = jnp.concatenate([y.T[0:D], jnp.zeros((D, T), f32)], axis=1)
        y_u = _pack(y_t)[:, 0:T]
        lane = lax.broadcasted_iota(i32, (D // 2, T), 1)
        wot_u[:, DP - T:DP] = jnp.where(lane < HT, wot_u[:, DP - T:DP], y_u)
        rid = lax.broadcasted_iota(i32, (8, T), 0)
        for tt in range(TPS):
            tok_l = lax.broadcasted_iota(i32, (8, T), 1) + (NSEG - 1) * L + tt * T
            ots[tt][D:D + 8, :] = jnp.where(((rid == 0) & (tok_l == i1)) | ((rid == 1) & (tok_l == i2)), 1.0, 0.0)

    dense = _interleave(mem_tasks, a_tasks(0, s0, m0), prep_dense(3, wot_u, 0))
    with _scope("p15_mix"):
        run(dense[0:2] + [select_task] + dense[2:])

    def out_tile(s, tt, last):
        c0 = s * L + tt * T
        if not isinstance(s, int):
            c0 = pl.multiple_of(c0, T)
        o_bf = ots[tt][...].astype(bf16)
        nchunk = 4
        rows = D // nchunk
        for rc in range(nchunk):
            r0 = rc * rows
            attn = jnp.dot(_bf(wot_u[r0 // 2:(r0 + rows) // 2, :]), o_bf, preferred_element_type=f32)
            xn = _bf(xn_u[s * TPS + tt, r0 // 2:(r0 + rows) // 2, :]).astype(f32)
            x = x_buf[r0:r0 + rows, pl.ds(c0, T)].astype(f32)
            res = x + attn + xn
            out_buf[r0:r0 + rows, pl.ds(c0, T)] = res.astype(bf16)

    bufs = ((s0, m0), (s1, m1))

    def pair_tasks(ua, ub):
        tasks = []
        for x, y in zip(a_tasks(ua[0], *bufs[ua[1]]), b_tasks(ub[0], *bufs[ub[1]])):
            tasks += [y, x]
        return tasks

    def seg_end(s, last, extra_first):
        u2, u3 = UPS * s + 2, UPS * s + 3

        def by_qt(fn, unit, par, qt):
            return [lambda u=u: fn(unit, u, qt, *bufs[par]) for u in range(NP)]

        steps = []
        for step in range(7):
            lists = []
            if step < 4:
                lists.append(by_qt(stage_b, u2, 0, 3 - step))
                lists.append(by_qt(stage_a, u3, 1, 3 - step))
            if 1 <= step < 5:
                lists.append(by_qt(stage_b, u3, 1, 4 - step))
            if not last and 2 <= step < 6:
                lists.append(by_qt(stage_a, u3 + 1, 0, 5 - step))
            if step >= 3:
                lists.append([lambda tt=6 - step: out_tile(s, tt, last)])
            steps.append(_interleave(*lists))
        return steps

    def seg_att(s, c):
        u0 = UPS * s
        tasks = pair_tasks((u0 + 1, 1), (u0, 0)) + pair_tasks((u0 + 2, 0), (u0 + 1, 1))
        for step in seg_end(s, False, None)[0:5]:
            tasks += step
        with _scope("att_seg"):
            run(_interleave(tasks, moe_tasks(s * FPI, FPI)))
            for step in seg_end(s, False, None)[5:]:
                run(step)
        out_copy(pl.multiple_of(s * L, L), L, s).start()
        return c

    lax.fori_loop(0, NSEG - 1, seg_att, 0)

    npatch = (NSEG - 1) * TPS

    def patch_tile(idx):
        return jnp.where(idx < npatch * T, idx // T, 0)

    tile0 = patch_tile(i1)
    tile1 = patch_tile(i2)
    tile1 = jnp.where(tile1 == tile0, (tile0 + 1) % npatch, tile1)

    def patch(tile):
        c0 = pl.multiple_of(tile * T, T)
        rid = lax.broadcasted_iota(i32, (T, T), 0)
        tok_l = lax.broadcasted_iota(i32, (T, T), 1) + c0
        hit = ((rid == HT) & (tok_l == i1)) | ((rid == HT + 1) & (tok_l == i2))
        onehot = jnp.where(hit, 1.0, 0.0).astype(bf16)
        for rc in range(4):
            r0, r1 = rc * (D // 4), (rc + 1) * (D // 4)
            upd = jnp.dot(_bf(wot_u[r0 // 2:r1 // 2, DP - T:DP]), onehot, preferred_element_type=f32)
            cur = out_buf[r0:r1, pl.ds(c0, T)].astype(f32)
            out_buf[r0:r1, pl.ds(c0, T)] = (cur + upd).astype(bf16)

    patch_copies = [out_copy(pl.multiple_of(tile0 * T, T), T, 7), out_copy(pl.multiple_of(tile1 * T, T), T, 8)]
    last_copies = [out_copy((NSEG - 1) * L + tt * T, T, NSEG - 1 + tt) for tt in range(TPS)]

    sl = NSEG - 1
    ul = UPS * sl
    with _scope("tail_1"):
        moe_finish()
        run(pair_tasks((ul + 1, 1), (ul, 0)))
        for s in range(NSEG - 1):
            out_copy(s * L, L, s).wait()
    with _scope("tail_2"):
        patch(tile0)
        patch(tile1)
        run(pair_tasks((ul + 2, 0), (ul + 1, 1)))
        for cp in patch_copies:
            cp.start()
        steps = seg_end(sl, True, None)
        for step in steps[0:5]:
            run(step)
        last_copies[3].start()
        last_copies[2].start()
    with _scope("tail_3"):
        run(steps[5])
        run(steps[6])
        last_copies[1].start()
        last_copies[0].start()

    with _scope("out_wait"):
        for cp in patch_copies + last_copies:
            cp.wait()


@jax.jit
def pallas_parallel_sum__memory_aug_infini_attn__moe_arch_mod__prompt_kernel(
    A_x: jax.Array,
    A_wq: jax.Array,
    A_wk: jax.Array,
    A_wv: jax.Array,
    A_wo: jax.Array,
    A_beta: jax.Array,
    B_x: jax.Array,
    B_w_r: jax.Array,
    B_w_gate: jax.Array,
    B_w_up: jax.Array,
    B_w_down: jax.Array,
):
    del B_x
    any_spec = pl.BlockSpec(memory_space=pl.ANY)
    scratch = [
        pltpu.VMEM((H,), bf16),
        pltpu.VMEM((D,), bf16),
        pltpu.VMEM((D, SEQ), bf16),
        pltpu.VMEM((4, D, D), bf16),
        pltpu.VMEM((D, F), bf16),
        pltpu.VMEM((D, F), bf16),
        pltpu.VMEM((D, F), bf16),
        pltpu.VMEM((D, SEQ), bf16),
        pltpu.VMEM((WT_ROWS, DP), u32),
        pltpu.VMEM((D // 2, DP), u32),
        pltpu.VMEM((D // 2, DP), u32),
        pltpu.VMEM((NT, DP // 2, T), u32),
        pltpu.VMEM((BT, DP // 2, T), u32),
        pltpu.VMEM((BT, DP // 2, T), u32),
        pltpu.VMEM((NSEG * NG, TW, L), u32),
        pltpu.VMEM((NSEG * NG, L // 2, T), u32),
        pltpu.VMEM((NSEG * NG, TW, L), u32),
        pltpu.VMEM((NSEG * NG, TW, L), u32),
        pltpu.VMEM((NSEG, D // 2, L), u32),
        pltpu.VMEM((NSEG * H, 16, L), u32),
        pltpu.VMEM((NSEG, 8, L), f32),
        pltpu.VMEM((NG, T + 16, T), f32),
        pltpu.VMEM((NSEG, D, L), f32),
        pltpu.VMEM((NG, 16, T), f32),
        pltpu.VMEM((H, 8, T), f32),
        pltpu.VMEM((3, HT, T), f32),
        pltpu.VMEM((HPG, TW, T), u32),
        pltpu.VMEM((8, 32, T), i32),
        pltpu.VMEM((NP, 4, 2 * L, T), f32),
        pltpu.VMEM((NP, 4, 2, 8, T), f32),
        pltpu.VMEM((NP, 4, 2 * L, T), f32),
        pltpu.VMEM((NP, 4, 2, 8, T), f32),
        pltpu.VMEM((DP, T), f32),
        pltpu.VMEM((DP, T), f32),
        pltpu.VMEM((DP, T), f32),
        pltpu.VMEM((DP, T), f32),
        pltpu.VMEM((2, D, LNW), f32),
        pltpu.VMEM((2, 2, 8, LNW), f32),
        pltpu.VMEM((16, D), f32),
        pltpu.VMEM((8, DP), u32),
        pltpu.VMEM((FPI, 2, 16, T), f32),
        pltpu.SemaphoreType.DMA((NSEM,)),
    ]
    x_t = jnp.transpose(A_x, (0, 2, 1)).reshape(D, SEQ)
    out_t = pl.pallas_call(
        _kernel,
        out_shape=jax.ShapeDtypeStruct((D, SEQ), bf16),
        in_specs=[any_spec] * 10,
        out_specs=any_spec,
        scratch_shapes=scratch,
        compiler_params=pltpu.CompilerParams(vmem_limit_bytes=110 * 1024 * 1024),
    )(x_t, A_wq, A_wk, A_wv, A_wo, A_beta, B_w_r, B_w_gate, B_w_up, B_w_down.T)
    return jnp.transpose(out_t.reshape(1, D, SEQ), (0, 2, 1))
```

```python
import contextlib

import jax
import jax.numpy as jnp
from jax import lax
from jax.experimental import pallas as pl
from jax.experimental.pallas import tpu as pltpu

bf16 = jnp.bfloat16
f32 = jnp.float32
u32 = jnp.uint32
i32 = jnp.int32

SEQ = 2048
D = 576
DP = 640
H = 32
DH = 18
NSEG = 4
L = 512
T = 128
TW = T // 2
HT = T // 2
TPS = L // T
HPG = 6
NG = 6
F = 4608
FPI = 12
FPB = 3
NFT = F // T
NP = 4
UPS = H // (2 * NP)
NUNIT = NSEG * UPS
NT = SEQ // T
LNW = 256
BT = LNW // T
NORM_PARTS = 6
VB = 8 * DH

LOG2E = 1.4426950408889634
QSCALE = (DH ** -0.5) * LOG2E
MASKVAL = -1000000000.0 * LOG2E
EPS_BF16 = 1.0013580322265625e-05
ONES_PAIR = 0x3F803F80

NT_DIMS = (((1,), (1,)), ((), ()))

WT_Q = 0
WT_K = NG * TW
WT_V = 2 * NG * TW
WT_ROWS = WT_V + D // 2

X_PIECES = ((0, LNW), (LNW, LNW), (L, L), (2 * L, L), (3 * L, L))
SEM_X = 0
SEM_W = 5
SEM_MOE = 9
SEM_OUT = 12
SEM_SMALL = 21
NSEM = 23


PROFILE_SCOPES = False
PACE = True
TAIL_BARRIERS = False
QT_ORDER = (3, 2, 1, 0)


def _scope(name):
    return jax.named_scope(name) if PROFILE_SCOPES else contextlib.nullcontext()


def _valid(g):
    return min(HPG * DH, D - g * HPG * DH)


def _rows(g):
    return -(-_valid(g) // 16) * 16


def _ewin(g):
    start = (g * HPG * DH // 16) * 16
    return start, g * HPG * DH - start, min(T, D - start)


def _bf(x):
    return pltpu.bitcast(x, bf16)


def _pack(x):
    return pltpu.bitcast(x.astype(bf16), u32)


def _round_bf16(x):
    return x.astype(bf16).astype(f32)


def _phi(t):
    return jnp.where(t > 0, t + 1.0, jnp.exp(t))


def _sigmoid(t):
    return 1.0 / (1.0 + jnp.exp(-t))


def _zero_after(v):
    bits = pltpu.bitcast(v[0:8, 0:LNW], u32)
    sixteen = jnp.uint32(16)
    bits = lax.shift_right_logical(lax.shift_right_logical(bits, sixteen), sixteen)
    return pltpu.bitcast(bits, f32) if PACE else None


def _interleave(*lists):
    items = []
    for li, tasks in enumerate(lists):
        for k, t in enumerate(tasks):
            items.append(((k + 0.5) / len(tasks), li, k, t))
    items.sort(key=lambda it: it[:3])
    return [it[3] for it in items]


def _kernel(x_hbm, wq_hbm, wk_hbm, wv_hbm, wo_hbm, beta_hbm, wr_hbm, wg_hbm, wu_hbm, wd_hbm,
            out_hbm,
            beta_ref, wr_ref, x_buf, w_buf, wg_buf, wu_buf, wd_buf, out_buf,
            wt_u, wtd_u, wot_u, xn_u, xs_a, xs_b, qs_u, k_u, pq_u, pk_u, vt_u, vwin,
            r_buf, mt_acc, am, g16, omg, mb, rowmask, smask,
            s0, m0, s1, m1, ot0, ot1, ot2, ot3, xf, ln_stat, y_acc, xsel_buf, hid_buf, sems):

    def x_copy(i):
        c0, width = X_PIECES[i]
        return pltpu.make_async_copy(x_hbm.at[:, pl.ds(c0, width)], x_buf.at[:, pl.ds(c0, width)],
                                     sems.at[SEM_X + i])

    def w_copy(i):
        src = (wq_hbm, wk_hbm, wv_hbm, wo_hbm)[i]
        return pltpu.make_async_copy(src, w_buf.at[i], sems.at[SEM_W + i])

    def moe_copy(i):
        src = (wg_hbm, wu_hbm, wd_hbm)[i]
        dst = (wg_buf, wu_buf, wd_buf)[i]
        return pltpu.make_async_copy(src, dst, sems.at[SEM_MOE + i])

    def out_copy(c0, width, sem):
        return pltpu.make_async_copy(out_buf.at[:, pl.ds(c0, width)], out_hbm.at[:, pl.ds(c0, width)],
                                     sems.at[SEM_OUT + sem])

    small_copies = [pltpu.make_async_copy(beta_hbm, beta_ref, sems.at[SEM_SMALL]),
                    pltpu.make_async_copy(wr_hbm, wr_ref, sems.at[SEM_SMALL + 1])]
    w_copy(0).start()
    x_copy(0).start()
    x_copy(1).start()
    for cp in small_copies:
        cp.start()
    w_copy(1).start()
    w_copy(2).start()

    init_scope = _scope("init")
    init_scope.__enter__()
    kr = lax.broadcasted_iota(i32, (HT, T), 0)
    ql = lax.broadcasted_iota(i32, (HT, T), 1)
    mb[0] = jnp.where(ql < kr, MASKVAL, 0.0).astype(f32)
    mb[1] = jnp.where((ql >= HT) & (ql - HT < kr), MASKVAL, 0.0).astype(f32)
    mb[2] = jnp.where(ql % HT < kr, MASKVAL, 0.0).astype(f32)
    for j in range(HPG):
        rowmask[j] = jnp.where((kr >= (DH // 2) * j) & (kr < (DH // 2) * (j + 1)), u32(0xFFFFFFFF), u32(0))
    r32 = lax.broadcasted_iota(i32, (32, T), 0)
    for i in range(8):
        smask[i] = jnp.where((r32 >= 2 * i) & (r32 < 2 * i + DH), 1, 0)
    zpad = jnp.zeros(((DP - D) // 2, T), u32)
    for tt in range(NT):
        xn_u[tt, D // 2:DP // 2, :] = zpad
    for tt in range(BT):
        xs_a[tt, D // 2:DP // 2, :] = zpad
        xs_b[tt, D // 2:DP // 2, :] = zpad
    ots = (ot0, ot1, ot2, ot3)
    for o_ref in ots:
        o_ref[D:DP, :] = jnp.zeros((DP - D, T), f32)
    am[0] = jnp.zeros(am.shape[1:], f32)
    mt_acc[...] = jnp.zeros(mt_acc.shape, f32)
    g16[...] = jnp.zeros(g16.shape, f32)
    for sg in range(NSEG * NG):
        r2 = _rows(sg % NG) // 2
        qs_u[sg, r2:TW, :] = jnp.zeros((TW - r2, L), u32)
        pq_u[sg, r2:TW, :] = jnp.zeros((TW - r2, L), u32)
        pk_u[sg, r2:TW, :] = jnp.zeros((TW - r2, L), u32)

    init_scope.__exit__(None, None, None)

    pace = [None]

    def gate_tables():
        gate = _round_bf16(_sigmoid(beta_ref[...].reshape(1, H).astype(f32)))
        for h in range(H):
            gh = jnp.broadcast_to(gate[:, h:h + 1], (1, T))
            omg[h] = jnp.broadcast_to(_round_bf16(1.0 - gh), (8, T))
            g16[h // HPG, (h % HPG):(h % HPG) + 1, :] = gh

    def transpose_block(i, cb):
        c1 = min((cb + 1) * T, D)
        blk = w_buf[i, :, cb * T:c1]
        if c1 - cb * T < T:
            blk = jnp.concatenate([blk, jnp.zeros((D, T - (c1 - cb * T)), bf16)], axis=1)
        blk = jnp.concatenate([blk, jnp.zeros((DP - D, T), bf16)], axis=0)
        return pltpu.bitcast(blk.T, u32)

    def prep_dense(i, dst, base):
        def task(cb):
            nrow = min(TW, D // 2 - cb * TW)
            dst[base + cb * TW:base + cb * TW + nrow, :] = transpose_block(i, cb)[0:nrow]
        return [lambda cb=cb: task(cb) for cb in range(DP // T)]

    def prep_grouped(i, base):
        def regroup(g):
            nv, nr = _valid(g) // 2, _rows(g) // 2
            src = g * HPG * DH // 2
            wt_u[base + g * TW:base + g * TW + nv, :] = wtd_u[src:src + nv, :]
            pad = jnp.zeros((nr - nv, DP), u32)
            if i == 1 and g == 0:
                wr = wr_ref[...].reshape(1, D).astype(f32)
                wr = jnp.concatenate([wr, jnp.zeros((1, DP - D), f32)], axis=1)
                bits = lax.shift_right_logical(pltpu.bitcast(wr, u32), u32(16))
                rid = lax.broadcasted_iota(i32, (nr - nv, DP), 0)
                pad = jnp.where(rid == 0, bits, pad)
            wt_u[base + g * TW + nv:base + g * TW + nr, :] = pad
        return prep_dense(i, wtd_u, 0) + [lambda g=g: regroup(g) for g in range(NG)]

    def ln_tasks(s, p, stage):
        c0 = s * L + p * LNW
        if not isinstance(s, int):
            c0 = pl.multiple_of(c0, LNW)

        def mean_pass():
            acc = pace[0]
            for r in range(0, D, 64):
                x = x_buf[r:r + 64, pl.ds(c0, LNW)].astype(f32)
                xf[p, r:r + 64, :] = x
                part = jnp.sum(x.reshape(8, 8, LNW), axis=0)
                acc = part if acc is None else acc + part
            mean = jnp.sum(acc, axis=0, keepdims=True) / D
            ln_stat[p, 0] = jnp.broadcast_to(mean, (8, LNW))

        def var_pass():
            mean = ln_stat[p, 0][0:1]
            if pace[0] is not None:
                mean = mean + pace[0][0:1]
            acc = None
            for r in range(0, D, 96):
                xc = xf[p, r:r + 96, :] - mean
                part = jnp.sum((xc * xc).reshape(12, 8, LNW), axis=0)
                acc = part if acc is None else acc + part
            var = jnp.sum(acc, axis=0, keepdims=True) / D
            den = _round_bf16(jnp.sqrt(_round_bf16(_round_bf16(var) + EPS_BF16)))
            ln_stat[p, 1] = jnp.broadcast_to(1.0 / den, (8, LNW))
            ln_stat[p, 0] = jnp.broadcast_to(_round_bf16(mean), (8, LNW))

        def norm_pass(part):
            mean_b = ln_stat[p, 0][0:1]
            if pace[0] is not None:
                mean_b = mean_b + pace[0][0:1]
            inv = ln_stat[p, 1][0:1]
            step = D // NORM_PARTS
            for r in range(part * step, (part + 1) * step, 48):
                xn = _pack(_round_bf16(xf[p, r:r + 48, :] - mean_b) * inv)
                for t in range(BT):
                    xn_u[s * TPS + p * BT + t, r // 2:r // 2 + 24, :] = xn[:, t * T:(t + 1) * T]
                    if stage is not None:
                        stage[t, r // 2:r // 2 + 24, :] = xn[:, t * T:(t + 1) * T]

        return [mean_pass, var_pass] + [lambda part=part: norm_pass(part) for part in range(NORM_PARTS)]

    def load_xs(s, p, stage):
        if stage is None:
            tiles = [xn_u[s * TPS + p * BT + t] for t in range(BT)]
        else:
            tiles = [stage[t] for t in range(BT)]
        return jnp.concatenate([_bf(t) for t in tiles], axis=1)

    def q_task(s, p, stage, g):
        nr = _rows(g) // 2
        cols = slice(p * LNW, (p + 1) * LNW)
        w = _bf(wt_u[WT_Q + g * TW:WT_Q + g * TW + nr, :])
        q = jnp.dot(w, load_xs(s, p, stage), preferred_element_type=f32)
        pace[0] = _zero_after(q)
        qp = _pack(q * QSCALE)
        qrot = jnp.concatenate([pltpu.roll(qp[:, t * T:(t + 1) * T], HT, 1) for t in range(BT)], axis=1)
        rid = lax.broadcasted_iota(i32, qp.shape, 0)
        even = ((rid // (DH // 2)) % 2) == 0
        qs_u[s * NG + g, 0:nr, cols] = jnp.where(even, qrot, qp)
        pq_u[s * NG + g, 0:nr, cols] = _pack(_phi(_round_bf16(q)))

    def k_task(s, p, stage, g):
        nr = _rows(g)
        cols = slice(p * LNW, (p + 1) * LNW)
        w = _bf(wt_u[WT_K + g * TW:WT_K + g * TW + nr // 2, :])
        k = jnp.dot(w, load_xs(s, p, stage), preferred_element_type=f32)
        pace[0] = _zero_after(k)
        if g == 0:
            r_buf[s, :, cols] = jnp.broadcast_to(k[_valid(0):_valid(0) + 1, :], (8, LNW))
        kp = _pack(k)
        pk_u[s * NG + g, 0:nr // 2, cols] = _pack(_phi(_round_bf16(k)))
        kfull = _bf(jnp.concatenate([kp, jnp.zeros(((T - nr) // 2, LNW), u32)], axis=0))
        k_u[s * NG + g, p * (LNW // 2):(p + 1) * (LNW // 2), :] = pltpu.bitcast(kfull.T, u32)

    def v_task(s, p, stage, b):
        cols = slice(p * LNW, (p + 1) * LNW)
        w = _bf(wt_u[WT_V + b * (VB // 2):WT_V + (b + 1) * (VB // 2), :])
        v = jnp.dot(w, load_xs(s, p, stage), preferred_element_type=f32)
        pace[0] = _zero_after(v)
        v = _pack(v)
        vt_u[s, b * (VB // 2):(b + 1) * (VB // 2), cols] = v
        sub = lax.broadcasted_iota(i32, (16, LNW), 0)
        for hh in range(8):
            w8 = (9 * hh) // 8
            ones_row = 0 if 2 * hh == 14 else 15
            vwin[s * H + 8 * b + hh, :, cols] = jnp.where(sub == ones_row, u32(ONES_PAIR), v[8 * w8:8 * w8 + 16, :])

    def q_tasks(s, p, stage=None):
        return [lambda g=g: q_task(s, p, stage, g) for g in range(NG)]

    def k_tasks(s, p, stage=None):
        return [lambda g=g: k_task(s, p, stage, g) for g in range(NG)]

    def v_tasks(s, p, stage=None):
        return [lambda b=b: v_task(s, p, stage, b) for b in range(D // VB)]

    def run(tasks):
        for t in tasks:
            t()

    prep_q = prep_grouped(0, WT_Q)
    with _scope("p1_wait_wq"):
        w_copy(0).wait()
    with _scope("p1_prep_q"):
        run(prep_q[0:3])
        x_copy(0).wait()
    for i in range(2, len(X_PIECES)):
        x_copy(i).start()
    w_copy(3).start()
    for i in range(3):
        moe_copy(i).start()
    with _scope("p1_ln0a"):
        run(_interleave(prep_q[3:], ln_tasks(0, 0, None)))
        x_copy(1).wait()
    with _scope("p1_q0a"):
        run(_interleave(q_tasks(0, 0), ln_tasks(0, 1, None)))
        w_copy(1).wait()
        for cp in small_copies:
            cp.wait()
    k0 = k_tasks(0, 0) + k_tasks(0, 1)
    with _scope("p1_q0b"):
        run(_interleave(q_tasks(0, 1), prep_grouped(1, WT_K), [gate_tables]))
        run(k0[0:NG])
        w_copy(2).wait()
        x_copy(2).wait()
    with _scope("p1_k0v0"):
        run(_interleave(k0[NG:], prep_dense(2, wt_u, WT_V)))
        run(_interleave(v_tasks(0, 0) + v_tasks(0, 1), ln_tasks(1, 0, xs_a)))

    def seg_body(s, c):
        for ss in range(2, NSEG):
            @pl.when(s + 1 == ss)
            def _():
                x_copy(ss + 1).wait()
        nxt = jnp.minimum(s + 1, NSEG - 1)
        pace[0] = None
        with _scope("p1_seg"):
            first = q_tasks(s, 0, xs_a) + k_tasks(s, 0, xs_a) + v_tasks(s, 0, xs_a)
            run(_interleave(first, ln_tasks(s, 1, xs_b)))
            second = q_tasks(s, 1, xs_b) + k_tasks(s, 1, xs_b) + v_tasks(s, 1, xs_b)
            run(_interleave(second, ln_tasks(nxt, 0, xs_a)))
        return c

    lax.fori_loop(1, NSEG, seg_body, 0)

    row64 = lax.broadcasted_iota(i32, (TW, T), 0)
    lane64 = lax.broadcasted_iota(i32, (TW, T), 1)
    row32 = lax.broadcasted_iota(i32, (32, T), 0)
    lane32 = lax.broadcasted_iota(i32, (32, T), 1)
    lane1 = lax.broadcasted_iota(i32, (1, T), 1)
    lane8 = lax.broadcasted_iota(i32, (8, T), 1)

    def stage_a(unit, u, qt, s_ref, m_ref):
        s = unit // UPS
        pi = (unit % UPS) * NP + u
        g = pi // (HPG // 2)
        j = 2 * (pi - (HPG // 2) * g)
        sg = s * NG + g
        n = T * (qt + 1)
        qw = qs_u[sg, :, qt * T:(qt + 1) * T]
        w_a = qw & rowmask[j]
        w_b = qw & rowmask[j + 1]
        w_ab = _bf(jnp.where(lane64 < HT, w_a, w_b))

        def colmax8(v):
            return jnp.max(v.reshape(v.shape[0] // 8, 8, T), axis=0)

        maxes = []
        for hd, w in enumerate((_bf(w_a), _bf(w_b))):
            m8 = None
            for c in range(qt):
                kc = _bf(k_u[sg, c * TW:(c + 1) * TW, :])
                sc = jnp.dot(kc, w, preferred_element_type=f32)
                s_ref[u, qt, hd * L + c * T:hd * L + (c + 1) * T, :] = sc
                m8 = colmax8(sc) if m8 is None else jnp.maximum(m8, colmax8(sc))
            kc = _bf(k_u[sg, qt * TW:qt * TW + TW // 2, :])
            sc = jnp.dot(kc, w, preferred_element_type=f32) + mb[1 - hd]
            s_ref[u, qt, hd * L + qt * T:hd * L + qt * T + HT, :] = sc
            m8 = colmax8(sc) if m8 is None else jnp.maximum(m8, colmax8(sc))
            maxes.append(m8)
        kc = _bf(k_u[sg, qt * TW + TW // 2:(qt + 1) * TW, :])
        sc = jnp.dot(kc, w_ab, preferred_element_type=f32) + mb[2]
        s_ref[u, qt, n - HT:n, :] = sc
        mab = colmax8(sc)
        m_a = jnp.where(lane8 < HT, jnp.maximum(maxes[0], mab), maxes[0])
        m_b = jnp.where(lane8 >= HT, jnp.maximum(maxes[1], mab), maxes[1])
        m_ref[u, qt, 0] = jnp.broadcast_to(jnp.max(m_a, axis=0, keepdims=True), (8, T))
        m_ref[u, qt, 1] = jnp.broadcast_to(jnp.max(m_b, axis=0, keepdims=True), (8, T))

    def stage_b(unit, u, qt, s_ref, m_ref):
        s = unit // UPS
        pi = (unit % UPS) * NP + u
        n = T * (qt + 1)
        m_a = m_ref[u, qt, 0][0:1]
        m_b = m_ref[u, qt, 1][0:1]
        p_ab = jnp.exp2(s_ref[u, qt, n - HT:n, :] - jnp.where(lane1 < HT, m_a, m_b))
        for hd, m in enumerate((m_a, m_b)):
            h = 2 * pi + hd
            p = jnp.exp2(s_ref[u, qt, hd * L:hd * L + n - HT, :] - m)
            keep = (lane64 < HT) if hd == 0 else (lane64 >= HT)
            p = jnp.concatenate([p, jnp.where(keep, p_ab, 0.0)], axis=0).astype(bf16)
            w8 = (9 * h) // 8
            off = DH * h - 16 * w8
            o = jnp.dot(_bf(vwin[s * H + h, :, 0:n]), p, preferred_element_type=f32)
            den = jnp.where(off == 14, o[0:1], o[31:32])
            o = o * (omg[h][0:1] / den)
            if hd == 0:
                o = pltpu.roll(o, HT, 1)
            r1 = pl.multiple_of(16 * w8, 16)
            res = am[s, pl.ds(r1, 32), qt * T:(qt + 1) * T] + o
            pltpu.store(ots[qt].at[pl.ds(r1, 32), :], res, mask=smask[off // 2] != 0)

    def a_tasks(unit, s_ref, m_ref):
        return [lambda u=u, qt=qt: stage_a(unit, u, qt, s_ref, m_ref) for u in range(NP) for qt in QT_ORDER]

    def b_tasks(unit, s_ref, m_ref):
        return [lambda u=u, qt=qt: stage_b(unit, u, qt, s_ref, m_ref) for u in range(NP) for qt in QT_ORDER]

    ones16 = jnp.where(lax.broadcasted_iota(i32, (8, L), 0) == 0, u32(0x3F80), u32(0))

    def mem_task(s, g):
        es, eoff, ne = _ewin(g)
        nv = _valid(g)
        lhs = _bf(jnp.concatenate([vt_u[s, es // 2:(es + ne) // 2, :], ones16], axis=0))
        upd = lax.dot_general(lhs, _bf(pk_u[s * NG + g]), NT_DIMS, preferred_element_type=f32)
        mt = mt_acc[g, 0:ne + 16, :] + upd
        mt_acc[g, 0:ne + 16, :] = mt
        e_loc = lax.broadcasted_iota(i32, (ne, T), 0) - eoff
        d_id = lax.broadcasted_iota(i32, (ne, T), 1)
        same_head = (e_loc >= 0) & (e_loc < nv) & (d_id < nv) & ((e_loc // DH) == (d_id // DH))
        j16 = lax.broadcasted_iota(i32, (16, T), 0)
        d16 = lax.broadcasted_iota(i32, (16, T), 1)
        z_mask = ((d16 // DH) == j16) & (d16 < nv)
        lm = jnp.concatenate(
            [jnp.where(same_head, mt[0:ne], 0.0),
             jnp.where(z_mask, jnp.broadcast_to(mt[ne:ne + 1, :], (16, T)), 0.0)], axis=0)
        nd = jnp.dot(lm.astype(bf16), _bf(pq_u[(s + 1) * NG + g]), preferred_element_type=f32)
        scale = jnp.broadcast_to(g16[g][:, 0:1], (16, L)) / (nd[ne:ne + 16, :] + 1e-6)
        r8 = lax.broadcasted_iota(i32, (8, L), 0)
        for b in range(ne // 8):
            lo, hi = 8 * b - eoff, 8 * b + 7 - eoff
            if hi < 0 or lo >= nv:
                continue
            j1, j2 = max(lo, 0) // DH, min(hi, nv - 1) // DH
            sc = jnp.broadcast_to(scale[j1:j1 + 1, :], (8, L))
            if j2 != j1:
                sc = jnp.where(r8 < DH * j2 - lo, sc, jnp.broadcast_to(scale[j2:j2 + 1, :], (8, L)))
            val = nd[8 * b:8 * b + 8, :] * sc
            dst = am.at[s + 1, es + 8 * b:es + 8 * b + 8, :]
            if lo >= 0 and hi < nv:
                dst[...] = val
            else:
                pltpu.store(dst, val, mask=(r8 + lo >= 0) & (r8 + lo < nv))

    mem_tasks = [lambda s=s, g=g: mem_task(s, g) for s in range(NSEG - 1) for g in range(NG)]

    w_copy(3).wait()
    for i in range(3):
        moe_copy(i).wait()
    rr = jnp.concatenate([r_buf[s][0:1, :] for s in range(NSEG)], axis=0)
    rr = _round_bf16(rr)
    tok = lax.broadcasted_iota(i32, (NSEG, L), 0) * L + lax.broadcasted_iota(i32, (NSEG, L), 1)
    m1v = jnp.max(rr)
    i1 = jnp.min(jnp.where(rr == m1v, tok, SEQ))
    rr2 = jnp.where(tok == i1, -jnp.inf, rr)
    m2v = jnp.max(rr2)
    i2 = jnp.min(jnp.where(rr2 == m2v, tok, SEQ))
    i1 = jnp.clip(i1, 0, SEQ - 1)
    i2 = jnp.clip(i2, 0, SEQ - 1)

    row16 = lax.broadcasted_iota(i32, (16, T), 0)
    lane16 = lax.broadcasted_iota(i32, (16, T), 1)

    def token_rows(i, slot):
        onehot = jnp.where((row16 == slot) & (lane16 == i % T), 1.0, 0.0).astype(bf16)
        return lax.dot_general(onehot, _bf(xn_u[i // T]), NT_DIMS, preferred_element_type=f32)

    def select_task():
        xsel_buf[...] = _pack(token_rows(i1, 0) + token_rows(i2, 1))
        y_acc[...] = jnp.zeros(y_acc.shape, f32)

    def fcols(ft):
        return pl.ds(ft * T if isinstance(ft, int) else pl.multiple_of(ft * T, T), T)

    def moe_up_task(ft, k, which):
        xsel = _bf(xsel_buf[:, 0:D])
        w_ref = (wg_buf, wu_buf)[which]
        hid_buf[k, which] = jnp.dot(xsel, w_ref[:, fcols(ft)], preferred_element_type=f32)

    def moe_down_task(ft, k):
        gt = _round_bf16(hid_buf[k, 0])
        up = _round_bf16(hid_buf[k, 1])
        hid = (_round_bf16(gt * _sigmoid(gt)) * up).astype(bf16)
        y_acc[...] += lax.dot_general(hid, wd_buf[:, fcols(ft)], NT_DIMS, preferred_element_type=f32)

    def moe_tasks(ft0, count):
        tasks = []
        for k0 in range(0, count, FPB):
            ks = range(k0, min(k0 + FPB, count))
            tasks += [lambda k=k, w=w: moe_up_task(ft0 + k, k, w) for k in ks for w in range(2)]
            tasks += [lambda k=k: moe_down_task(ft0 + k, k) for k in ks]
        return tasks

    def moe_finish():
        y = _round_bf16(y_acc[...])
        rsel = jnp.where(lax.broadcasted_iota(i32, (16, 1), 0) == 0, m1v, m2v)
        y = _round_bf16(y * _round_bf16(_sigmoid(rsel)))
        y = jnp.concatenate([y, jnp.zeros((16, DP - D), f32)], axis=1)
        y = jnp.concatenate([jnp.zeros((HT, DP), f32), y, jnp.zeros((T - HT - 16, DP), f32)], axis=0)
        y_t = jnp.concatenate([y.T[0:D], jnp.zeros((D, T), f32)], axis=1)
        y_u = _pack(y_t)[:, 0:T]
        lane = lax.broadcasted_iota(i32, (D // 2, T), 1)
        wot_u[:, DP - T:DP] = jnp.where(lane < HT, wot_u[:, DP - T:DP], y_u)
        rid = lax.broadcasted_iota(i32, (8, T), 0)
        for tt in range(TPS):
            tok_l = lax.broadcasted_iota(i32, (8, T), 1) + (NSEG - 1) * L + tt * T
            ots[tt][D:D + 8, :] = jnp.where(((rid == 0) & (tok_l == i1)) | ((rid == 1) & (tok_l == i2)), 1.0, 0.0)

    dense = _interleave(mem_tasks, a_tasks(0, s0, m0), prep_dense(3, wot_u, 0))
    with _scope("p15_mix"):
        cut = (2 * len(dense)) // 3
        run(dense[:cut] + [select_task] + dense[cut:])

    def out_tile(s, tt, last):
        c0 = s * L + tt * T
        if not isinstance(s, int):
            c0 = pl.multiple_of(c0, T)
        o_bf = ots[tt][...].astype(bf16)
        nchunk = 4
        rows = D // nchunk
        for rc in range(nchunk):
            r0 = rc * rows
            attn = jnp.dot(_bf(wot_u[r0 // 2:(r0 + rows) // 2, :]), o_bf, preferred_element_type=f32)
            xn = _bf(xn_u[s * TPS + tt, r0 // 2:(r0 + rows) // 2, :]).astype(f32)
            x = x_buf[r0:r0 + rows, pl.ds(c0, T)].astype(f32)
            res = x + attn + xn
            out_buf[r0:r0 + rows, pl.ds(c0, T)] = res.astype(bf16)

    bufs = ((s0, m0), (s1, m1))

    def pair_tasks(ua, ub):
        tasks = []
        for x, y in zip(a_tasks(ua[0], *bufs[ua[1]]), b_tasks(ub[0], *bufs[ub[1]])):
            tasks += [y, x]
        return tasks

    def seg_end(s, last, extra_first):
        u2, u3 = UPS * s + 2, UPS * s + 3

        def by_qt(fn, unit, par, qt):
            return [lambda u=u: fn(unit, u, qt, *bufs[par]) for u in range(NP)]

        steps = []
        for step in range(7):
            lists = []
            if step < 4:
                lists.append(by_qt(stage_b, u2, 0, 3 - step))
                lists.append(by_qt(stage_a, u3, 1, 3 - step))
            if 1 <= step < 5:
                lists.append(by_qt(stage_b, u3, 1, 4 - step))
            if not last and 2 <= step < 6:
                lists.append(by_qt(stage_a, u3 + 1, 0, 5 - step))
            if step >= 3:
                lists.append([lambda tt=6 - step: out_tile(s, tt, last)])
            steps.append(_interleave(*lists))
        return steps

    def seg_att(s, c):
        u0 = UPS * s
        tasks = pair_tasks((u0 + 1, 1), (u0, 0)) + pair_tasks((u0 + 2, 0), (u0 + 1, 1))
        for step in seg_end(s, False, None)[0:5]:
            tasks += step
        with _scope("att_seg"):
            run(_interleave(tasks, moe_tasks(s * FPI, FPI)))
            for step in seg_end(s, False, None)[5:]:
                run(step)
        out_copy(pl.multiple_of(s * L, L), L, s).start()
        return c

    lax.fori_loop(0, NSEG - 1, seg_att, 0)

    npatch = (NSEG - 1) * TPS

    def patch_tile(idx):
        return jnp.where(idx < npatch * T, idx // T, 0)

    tile0 = patch_tile(i1)
    tile1 = patch_tile(i2)
    tile1 = jnp.where(tile1 == tile0, (tile0 + 1) % npatch, tile1)

    def patch(tile):
        c0 = pl.multiple_of(tile * T, T)
        rid = lax.broadcasted_iota(i32, (T, T), 0)
        tok_l = lax.broadcasted_iota(i32, (T, T), 1) + c0
        hit = ((rid == HT) & (tok_l == i1)) | ((rid == HT + 1) & (tok_l == i2))
        onehot = jnp.where(hit, 1.0, 0.0).astype(bf16)
        for rc in range(4):
            r0, r1 = rc * (D // 4), (rc + 1) * (D // 4)
            upd = jnp.dot(_bf(wot_u[r0 // 2:r1 // 2, DP - T:DP]), onehot, preferred_element_type=f32)
            cur = out_buf[r0:r1, pl.ds(c0, T)].astype(f32)
            out_buf[r0:r1, pl.ds(c0, T)] = (cur + upd).astype(bf16)

    patch_copies = [out_copy(pl.multiple_of(tile0 * T, T), T, 7), out_copy(pl.multiple_of(tile1 * T, T), T, 8)]
    last_copies = [out_copy((NSEG - 1) * L + tt * T, T, NSEG - 1 + tt) for tt in range(TPS)]

    sl = NSEG - 1
    ul = UPS * sl
    with _scope("tail_1"):
        moe_finish()
        run(pair_tasks((ul + 1, 1), (ul, 0)))
        for s in range(NSEG - 1):
            out_copy(s * L, L, s).wait()
    with _scope("tail_2"):
        patch(tile0)
        patch(tile1)
        run(pair_tasks((ul + 2, 0), (ul + 1, 1)))
        for cp in patch_copies:
            cp.start()
        steps = seg_end(sl, True, None)
        for step in steps[0:5]:
            run(step)
        last_copies[3].start()
        last_copies[2].start()
    with _scope("tail_3"):
        run(steps[5])
        run(steps[6])
        last_copies[1].start()
        last_copies[0].start()

    with _scope("out_wait"):
        for cp in patch_copies + last_copies:
            cp.wait()


@jax.jit
def pallas_parallel_sum__memory_aug_infini_attn__moe_arch_mod__prompt_kernel(
    A_x: jax.Array,
    A_wq: jax.Array,
    A_wk: jax.Array,
    A_wv: jax.Array,
    A_wo: jax.Array,
    A_beta: jax.Array,
    B_x: jax.Array,
    B_w_r: jax.Array,
    B_w_gate: jax.Array,
    B_w_up: jax.Array,
    B_w_down: jax.Array,
):
    del B_x
    any_spec = pl.BlockSpec(memory_space=pl.ANY)
    scratch = [
        pltpu.VMEM((H,), bf16),
        pltpu.VMEM((D,), bf16),
        pltpu.VMEM((D, SEQ), bf16),
        pltpu.VMEM((4, D, D), bf16),
        pltpu.VMEM((D, F), bf16),
        pltpu.VMEM((D, F), bf16),
        pltpu.VMEM((D, F), bf16),
        pltpu.VMEM((D, SEQ), bf16),
        pltpu.VMEM((WT_ROWS, DP), u32),
        pltpu.VMEM((D // 2, DP), u32),
        pltpu.VMEM((D // 2, DP), u32),
        pltpu.VMEM((NT, DP // 2, T), u32),
        pltpu.VMEM((BT, DP // 2, T), u32),
        pltpu.VMEM((BT, DP // 2, T), u32),
        pltpu.VMEM((NSEG * NG, TW, L), u32),
        pltpu.VMEM((NSEG * NG, L // 2, T), u32),
        pltpu.VMEM((NSEG * NG, TW, L), u32),
        pltpu.VMEM((NSEG * NG, TW, L), u32),
        pltpu.VMEM((NSEG, D // 2, L), u32),
        pltpu.VMEM((NSEG * H, 16, L), u32),
        pltpu.VMEM((NSEG, 8, L), f32),
        pltpu.VMEM((NG, T + 16, T), f32),
        pltpu.VMEM((NSEG, D, L), f32),
        pltpu.VMEM((NG, 16, T), f32),
        pltpu.VMEM((H, 8, T), f32),
        pltpu.VMEM((3, HT, T), f32),
        pltpu.VMEM((HPG, TW, T), u32),
        pltpu.VMEM((8, 32, T), i32),
        pltpu.VMEM((NP, 4, 2 * L, T), f32),
        pltpu.VMEM((NP, 4, 2, 8, T), f32),
        pltpu.VMEM((NP, 4, 2 * L, T), f32),
        pltpu.VMEM((NP, 4, 2, 8, T), f32),
        pltpu.VMEM((DP, T), f32),
        pltpu.VMEM((DP, T), f32),
        pltpu.VMEM((DP, T), f32),
        pltpu.VMEM((DP, T), f32),
        pltpu.VMEM((2, D, LNW), f32),
        pltpu.VMEM((2, 2, 8, LNW), f32),
        pltpu.VMEM((16, D), f32),
        pltpu.VMEM((8, DP), u32),
        pltpu.VMEM((FPI, 2, 16, T), f32),
        pltpu.SemaphoreType.DMA((NSEM,)),
    ]
    x_t = jnp.transpose(A_x, (0, 2, 1)).reshape(D, SEQ)
    out_t = pl.pallas_call(
        _kernel,
        out_shape=jax.ShapeDtypeStruct((D, SEQ), bf16),
        in_specs=[any_spec] * 10,
        out_specs=any_spec,
        scratch_shapes=scratch,
        compiler_params=pltpu.CompilerParams(vmem_limit_bytes=110 * 1024 * 1024),
    )(x_t, A_wq, A_wk, A_wv, A_wo, A_beta, B_w_r, B_w_gate, B_w_up, B_w_down.T)
    return jnp.transpose(out_t.reshape(1, D, SEQ), (0, 2, 1))
```

```python
import contextlib

import jax
import jax.numpy as jnp
from jax import lax
from jax.experimental import pallas as pl
from jax.experimental.pallas import tpu as pltpu

bf16 = jnp.bfloat16
f32 = jnp.float32
u32 = jnp.uint32
i32 = jnp.int32

SEQ = 2048
D = 576
DP = 640
H = 32
DH = 18
NSEG = 4
L = 512
T = 128
TW = T // 2
HT = T // 2
TPS = L // T
HPG = 6
NG = 6
F = 4608
FPI = 12
FPB = 3
NFT = F // T
NP = 4
UPS = H // (2 * NP)
NUNIT = NSEG * UPS
NT = SEQ // T
LNW = 256
BT = LNW // T
NORM_PARTS = 6
VB = 8 * DH

LOG2E = 1.4426950408889634
QSCALE = (DH ** -0.5) * LOG2E
MASKVAL = -1000000000.0 * LOG2E
EPS_BF16 = 1.0013580322265625e-05
ONES_PAIR = 0x3F803F80

NT_DIMS = (((1,), (1,)), ((), ()))

WT_Q = 0
WT_K = NG * TW
WT_V = 2 * NG * TW
WT_ROWS = WT_V + D // 2

X_PIECES = ((0, LNW), (LNW, LNW), (L, L), (2 * L, L), (3 * L, L))
SEM_X = 0
SEM_W = 5
SEM_MOE = 9
SEM_OUT = 12
SEM_SMALL = 21
NSEM = 23


PROFILE_SCOPES = False
PACE = True
TAIL_BARRIERS = False
QT_ORDER = (3, 2, 1, 0)


def _scope(name):
    return jax.named_scope(name) if PROFILE_SCOPES else contextlib.nullcontext()


def _valid(g):
    return min(HPG * DH, D - g * HPG * DH)


def _rows(g):
    return -(-_valid(g) // 16) * 16


def _ewin(g):
    start = (g * HPG * DH // 16) * 16
    return start, g * HPG * DH - start, min(T, D - start)


def _bf(x):
    return pltpu.bitcast(x, bf16)


def _pack(x):
    return pltpu.bitcast(x.astype(bf16), u32)


def _round_bf16(x):
    return x.astype(bf16).astype(f32)


def _phi(t):
    return jnp.where(t > 0, t + 1.0, jnp.exp(t))


def _sigmoid(t):
    return 1.0 / (1.0 + jnp.exp(-t))


def _zero_after(v):
    bits = pltpu.bitcast(v[0:8, 0:LNW], u32)
    sixteen = jnp.uint32(16)
    bits = lax.shift_right_logical(lax.shift_right_logical(bits, sixteen), sixteen)
    return pltpu.bitcast(bits, f32) if PACE else None


def _interleave(*lists):
    items = []
    for li, tasks in enumerate(lists):
        for k, t in enumerate(tasks):
            items.append(((k + 0.5) / len(tasks), li, k, t))
    items.sort(key=lambda it: it[:3])
    return [it[3] for it in items]


def _kernel(x_hbm, wq_hbm, wk_hbm, wv_hbm, wo_hbm, beta_hbm, wr_hbm, wg_hbm, wu_hbm, wd_hbm,
            out_hbm,
            beta_ref, wr_ref, x_buf, w_buf, wg_buf, wu_buf, wd_buf, out_buf,
            wt_u, wtd_u, wot_u, xn_u, xs_a, xs_b, qs_u, k_u, pq_u, pk_u, vt_u, vwin,
            r_buf, mt_acc, am, g16, omg, mb,
            s0, m0, s1, m1, ot0, ot1, ot2, ot3, xf, ln_stat, y_acc, xsel_buf, hid_buf, sems):

    def x_copy(i):
        c0, width = X_PIECES[i]
        return pltpu.make_async_copy(x_hbm.at[:, pl.ds(c0, width)], x_buf.at[:, pl.ds(c0, width)],
                                     sems.at[SEM_X + i])

    def w_copy(i):
        src = (wq_hbm, wk_hbm, wv_hbm, wo_hbm)[i]
        return pltpu.make_async_copy(src, w_buf.at[i], sems.at[SEM_W + i])

    def moe_copy(i):
        src = (wg_hbm, wu_hbm, wd_hbm)[i]
        dst = (wg_buf, wu_buf, wd_buf)[i]
        return pltpu.make_async_copy(src, dst, sems.at[SEM_MOE + i])

    def out_copy(c0, width, sem):
        return pltpu.make_async_copy(out_buf.at[:, pl.ds(c0, width)], out_hbm.at[:, pl.ds(c0, width)],
                                     sems.at[SEM_OUT + sem])

    small_copies = [pltpu.make_async_copy(beta_hbm, beta_ref, sems.at[SEM_SMALL]),
                    pltpu.make_async_copy(wr_hbm, wr_ref, sems.at[SEM_SMALL + 1])]
    w_copy(0).start()
    x_copy(0).start()
    x_copy(1).start()
    for cp in small_copies:
        cp.start()
    w_copy(1).start()
    w_copy(2).start()

    init_scope = _scope("init")
    init_scope.__enter__()
    kr = lax.broadcasted_iota(i32, (HT, T), 0)
    ql = lax.broadcasted_iota(i32, (HT, T), 1)
    mb[0] = jnp.where(ql < kr, MASKVAL, 0.0).astype(f32)
    mb[1] = jnp.where((ql >= HT) & (ql - HT < kr), MASKVAL, 0.0).astype(f32)
    mb[2] = jnp.where(ql % HT < kr, MASKVAL, 0.0).astype(f32)
    zpad = jnp.zeros(((DP - D) // 2, T), u32)
    for tt in range(NT):
        xn_u[tt, D // 2:DP // 2, :] = zpad
    for tt in range(BT):
        xs_a[tt, D // 2:DP // 2, :] = zpad
        xs_b[tt, D // 2:DP // 2, :] = zpad
    ots = (ot0, ot1, ot2, ot3)
    for o_ref in ots:
        o_ref[D:DP, :] = jnp.zeros((DP - D, T), f32)
    am[0] = jnp.zeros(am.shape[1:], f32)
    mt_acc[...] = jnp.zeros(mt_acc.shape, f32)
    g16[...] = jnp.zeros(g16.shape, f32)
    for sg in range(NSEG * NG):
        r2 = _rows(sg % NG) // 2
        qs_u[sg, r2:TW, :] = jnp.zeros((TW - r2, L), u32)
        pq_u[sg, r2:TW, :] = jnp.zeros((TW - r2, L), u32)
        pk_u[sg, r2:TW, :] = jnp.zeros((TW - r2, L), u32)

    init_scope.__exit__(None, None, None)

    pace = [None]

    def gate_tables():
        gate = _round_bf16(_sigmoid(beta_ref[...].reshape(1, H).astype(f32)))
        for h in range(H):
            gh = jnp.broadcast_to(gate[:, h:h + 1], (1, T))
            omg[h] = jnp.broadcast_to(_round_bf16(1.0 - gh), (8, T))
            g16[h // HPG, (h % HPG):(h % HPG) + 1, :] = gh

    def transpose_block(i, cb):
        c1 = min((cb + 1) * T, D)
        blk = w_buf[i, :, cb * T:c1]
        if c1 - cb * T < T:
            blk = jnp.concatenate([blk, jnp.zeros((D, T - (c1 - cb * T)), bf16)], axis=1)
        blk = jnp.concatenate([blk, jnp.zeros((DP - D, T), bf16)], axis=0)
        return pltpu.bitcast(blk.T, u32)

    def prep_dense(i, dst, base):
        def task(cb):
            nrow = min(TW, D // 2 - cb * TW)
            dst[base + cb * TW:base + cb * TW + nrow, :] = transpose_block(i, cb)[0:nrow]
        return [lambda cb=cb: task(cb) for cb in range(DP // T)]

    def prep_grouped(i, base):
        def regroup(g):
            nv, nr = _valid(g) // 2, _rows(g) // 2
            src = g * HPG * DH // 2
            wt_u[base + g * TW:base + g * TW + nv, :] = wtd_u[src:src + nv, :]
            pad = jnp.zeros((nr - nv, DP), u32)
            if i == 1 and g == 0:
                wr = wr_ref[...].reshape(1, D).astype(f32)
                wr = jnp.concatenate([wr, jnp.zeros((1, DP - D), f32)], axis=1)
                bits = lax.shift_right_logical(pltpu.bitcast(wr, u32), u32(16))
                rid = lax.broadcasted_iota(i32, (nr - nv, DP), 0)
                pad = jnp.where(rid == 0, bits, pad)
            wt_u[base + g * TW + nv:base + g * TW + nr, :] = pad
        return prep_dense(i, wtd_u, 0) + [lambda g=g: regroup(g) for g in range(NG)]

    def ln_tasks(s, p, stage):
        c0 = s * L + p * LNW
        if not isinstance(s, int):
            c0 = pl.multiple_of(c0, LNW)

        def mean_pass():
            acc = pace[0]
            for r in range(0, D, 64):
                x = x_buf[r:r + 64, pl.ds(c0, LNW)].astype(f32)
                xf[p, r:r + 64, :] = x
                part = jnp.sum(x.reshape(8, 8, LNW), axis=0)
                acc = part if acc is None else acc + part
            mean = jnp.sum(acc, axis=0, keepdims=True) / D
            ln_stat[p, 0] = jnp.broadcast_to(mean, (8, LNW))

        def var_pass():
            mean = ln_stat[p, 0][0:1]
            if pace[0] is not None:
                mean = mean + pace[0][0:1]
            acc = None
            for r in range(0, D, 96):
                xc = xf[p, r:r + 96, :] - mean
                part = jnp.sum((xc * xc).reshape(12, 8, LNW), axis=0)
                acc = part if acc is None else acc + part
            var = jnp.sum(acc, axis=0, keepdims=True) / D
            den = _round_bf16(jnp.sqrt(_round_bf16(_round_bf16(var) + EPS_BF16)))
            ln_stat[p, 1] = jnp.broadcast_to(1.0 / den, (8, LNW))
            ln_stat[p, 0] = jnp.broadcast_to(_round_bf16(mean), (8, LNW))

        def norm_pass(part):
            mean_b = ln_stat[p, 0][0:1]
            if pace[0] is not None:
                mean_b = mean_b + pace[0][0:1]
            inv = ln_stat[p, 1][0:1]
            step = D // NORM_PARTS
            for r in range(part * step, (part + 1) * step, 48):
                xn = _pack(_round_bf16(xf[p, r:r + 48, :] - mean_b) * inv)
                for t in range(BT):
                    xn_u[s * TPS + p * BT + t, r // 2:r // 2 + 24, :] = xn[:, t * T:(t + 1) * T]
                    if stage is not None:
                        stage[t, r // 2:r // 2 + 24, :] = xn[:, t * T:(t + 1) * T]

        return [mean_pass, var_pass] + [lambda part=part: norm_pass(part) for part in range(NORM_PARTS)]

    def load_xs(s, p, stage):
        if stage is None:
            tiles = [xn_u[s * TPS + p * BT + t] for t in range(BT)]
        else:
            tiles = [stage[t] for t in range(BT)]
        return jnp.concatenate([_bf(t) for t in tiles], axis=1)

    def q_task(s, p, stage, g):
        nr = _rows(g) // 2
        cols = slice(p * LNW, (p + 1) * LNW)
        w = _bf(wt_u[WT_Q + g * TW:WT_Q + g * TW + nr, :])
        q = jnp.dot(w, load_xs(s, p, stage), preferred_element_type=f32)
        pace[0] = _zero_after(q)
        qp = _pack(q * QSCALE)
        qrot = jnp.concatenate([pltpu.roll(qp[:, t * T:(t + 1) * T], HT, 1) for t in range(BT)], axis=1)
        rid = lax.broadcasted_iota(i32, qp.shape, 0)
        even = ((rid // (DH // 2)) % 2) == 0
        qs_u[s * NG + g, 0:nr, cols] = jnp.where(even, qrot, qp)
        pq_u[s * NG + g, 0:nr, cols] = _pack(_phi(_round_bf16(q)))

    def k_task(s, p, stage, g):
        nr = _rows(g)
        cols = slice(p * LNW, (p + 1) * LNW)
        w = _bf(wt_u[WT_K + g * TW:WT_K + g * TW + nr // 2, :])
        k = jnp.dot(w, load_xs(s, p, stage), preferred_element_type=f32)
        pace[0] = _zero_after(k)
        if g == 0:
            r_buf[s, :, cols] = jnp.broadcast_to(k[_valid(0):_valid(0) + 1, :], (8, LNW))
        kp = _pack(k)
        pk_u[s * NG + g, 0:nr // 2, cols] = _pack(_phi(_round_bf16(k)))
        kfull = _bf(jnp.concatenate([kp, jnp.zeros(((T - nr) // 2, LNW), u32)], axis=0))
        k_u[s * NG + g, p * (LNW // 2):(p + 1) * (LNW // 2), :] = pltpu.bitcast(kfull.T, u32)

    def v_task(s, p, stage, b):
        cols = slice(p * LNW, (p + 1) * LNW)
        w = _bf(wt_u[WT_V + b * (VB // 2):WT_V + (b + 1) * (VB // 2), :])
        v = jnp.dot(w, load_xs(s, p, stage), preferred_element_type=f32)
        pace[0] = _zero_after(v)
        v = _pack(v)
        vt_u[s, b * (VB // 2):(b + 1) * (VB // 2), cols] = v
        sub = lax.broadcasted_iota(i32, (16, LNW), 0)
        for hh in range(8):
            w8 = (9 * hh) // 8
            ones_row = 0 if 2 * hh == 14 else 15
            vwin[s * H + 8 * b + hh, :, cols] = jnp.where(sub == ones_row, u32(ONES_PAIR), v[8 * w8:8 * w8 + 16, :])

    def q_tasks(s, p, stage=None):
        return [lambda g=g: q_task(s, p, stage, g) for g in range(NG)]

    def k_tasks(s, p, stage=None):
        return [lambda g=g: k_task(s, p, stage, g) for g in range(NG)]

    def v_tasks(s, p, stage=None):
        return [lambda b=b: v_task(s, p, stage, b) for b in range(D // VB)]

    def run(tasks):
        for t in tasks:
            t()

    prep_q = prep_grouped(0, WT_Q)
    with _scope("p1_wait_wq"):
        w_copy(0).wait()
    with _scope("p1_prep_q"):
        run(prep_q[0:3])
        x_copy(0).wait()
    for i in range(2, len(X_PIECES)):
        x_copy(i).start()
    w_copy(3).start()
    for i in range(3):
        moe_copy(i).start()
    with _scope("p1_ln0a"):
        run(_interleave(prep_q[3:], ln_tasks(0, 0, None)))
        x_copy(1).wait()
    with _scope("p1_q0a"):
        run(_interleave(q_tasks(0, 0), ln_tasks(0, 1, None)))
        w_copy(1).wait()
        for cp in small_copies:
            cp.wait()
    k0 = k_tasks(0, 0) + k_tasks(0, 1)
    with _scope("p1_q0b"):
        run(_interleave(q_tasks(0, 1), prep_grouped(1, WT_K), [gate_tables]))
        run(k0[0:NG])
        w_copy(2).wait()
        x_copy(2).wait()
    with _scope("p1_k0v0"):
        run(_interleave(k0[NG:], prep_dense(2, wt_u, WT_V)))
        run(_interleave(v_tasks(0, 0) + v_tasks(0, 1), ln_tasks(1, 0, xs_a)))

    def seg_body(s, c):
        for ss in range(2, NSEG):
            @pl.when(s + 1 == ss)
            def _():
                x_copy(ss + 1).wait()
        nxt = jnp.minimum(s + 1, NSEG - 1)
        pace[0] = None
        with _scope("p1_seg"):
            first = q_tasks(s, 0, xs_a) + k_tasks(s, 0, xs_a) + v_tasks(s, 0, xs_a)
            run(_interleave(first, ln_tasks(s, 1, xs_b)))
            second = q_tasks(s, 1, xs_b) + k_tasks(s, 1, xs_b) + v_tasks(s, 1, xs_b)
            run(_interleave(second, ln_tasks(nxt, 0, xs_a)))
        return c

    lax.fori_loop(1, NSEG, seg_body, 0)

    bufs = ((s0, m0), (s1, m1))
    lane64 = lax.broadcasted_iota(i32, (TW, T), 1)
    lane1 = lax.broadcasted_iota(i32, (1, T), 1)
    lane8 = lax.broadcasted_iota(i32, (8, T), 1)

    def head_rows(qw, j):
        lo, hi = (DH // 2) * j, (DH // 2) * (j + 1)
        r0, r1 = (lo // 8) * 8, -(-hi // 8) * 8
        rid = lax.broadcasted_iota(i32, (r1 - r0, T), 0) + r0
        part = jnp.where((rid >= lo) & (rid < hi), qw[r0:r1], u32(0))
        pieces = [jnp.zeros((r0, T), u32)] * (r0 > 0) + [part] + [jnp.zeros((TW - r1, T), u32)] * (r1 < TW)
        return jnp.concatenate(pieces, axis=0)

    def stage_a(unit, u, qt):
        s, k = unit
        s_ref, m_ref = bufs[k % 2]
        pi = k * NP + u
        g = pi // (HPG // 2)
        j = 2 * (pi - (HPG // 2) * g)
        sg = s * NG + g
        n = T * (qt + 1)
        qw = qs_u[sg, :, qt * T:(qt + 1) * T]
        w_a = head_rows(qw, j)
        w_b = head_rows(qw, j + 1)
        w_ab = _bf(jnp.where(lane64 < HT, w_a, w_b))

        def colmax8(v):
            return jnp.max(v.reshape(v.shape[0] // 8, 8, T), axis=0)

        maxes = []
        for hd, w in enumerate((_bf(w_a), _bf(w_b))):
            m8 = None
            for c in range(qt):
                kc = _bf(k_u[sg, c * TW:(c + 1) * TW, :])
                sc = jnp.dot(kc, w, preferred_element_type=f32)
                s_ref[u, qt, hd * L + c * T:hd * L + (c + 1) * T, :] = sc
                m8 = colmax8(sc) if m8 is None else jnp.maximum(m8, colmax8(sc))
            kc = _bf(k_u[sg, qt * TW:qt * TW + TW // 2, :])
            sc = jnp.dot(kc, w, preferred_element_type=f32) + mb[1 - hd]
            s_ref[u, qt, hd * L + qt * T:hd * L + qt * T + HT, :] = sc
            m8 = colmax8(sc) if m8 is None else jnp.maximum(m8, colmax8(sc))
            maxes.append(m8)
        kc = _bf(k_u[sg, qt * TW + TW // 2:(qt + 1) * TW, :])
        sc = jnp.dot(kc, w_ab, preferred_element_type=f32) + mb[2]
        s_ref[u, qt, n - HT:n, :] = sc
        mab = colmax8(sc)
        m_a = jnp.where(lane8 < HT, jnp.maximum(maxes[0], mab), maxes[0])
        m_b = jnp.where(lane8 >= HT, jnp.maximum(maxes[1], mab), maxes[1])
        m_ref[u, qt, 0] = jnp.broadcast_to(jnp.max(m_a, axis=0, keepdims=True), (8, T))
        m_ref[u, qt, 1] = jnp.broadcast_to(jnp.max(m_b, axis=0, keepdims=True), (8, T))

    def stage_b(unit, u, qt):
        s, k = unit
        s_ref, m_ref = bufs[k % 2]
        pi = k * NP + u
        n = T * (qt + 1)
        m_a = m_ref[u, qt, 0][0:1]
        m_b = m_ref[u, qt, 1][0:1]
        p_ab = jnp.exp2(s_ref[u, qt, n - HT:n, :] - jnp.where(lane1 < HT, m_a, m_b))
        for hd, m in enumerate((m_a, m_b)):
            h = 2 * pi + hd
            p = jnp.exp2(s_ref[u, qt, hd * L:hd * L + n - HT, :] - m)
            keep = (lane64 < HT) if hd == 0 else (lane64 >= HT)
            p = jnp.concatenate([p, jnp.where(keep, p_ab, 0.0)], axis=0).astype(bf16)
            w0 = ((DH * h) // 16) * 16
            off = DH * h - w0
            o = jnp.dot(_bf(vwin[s * H + h, :, 0:n]), p, preferred_element_type=f32)
            den = o[0:1] if off == 14 else o[31:32]
            r0, r1 = (off // 8) * 8, -(-(off + DH) // 8) * 8
            o = o[r0:r1] * (omg[h][0:1] / den)
            if hd == 0:
                o = pltpu.roll(o, HT, 1)
            res = am[s, w0 + r0:w0 + r1, qt * T:(qt + 1) * T] + o
            rid = lax.broadcasted_iota(i32, (r1 - r0, T), 0) + r0
            pltpu.store(ots[qt].at[w0 + r0:w0 + r1, :], res, mask=(rid >= off) & (rid < off + DH))

    def a_tasks(unit):
        return [lambda u=u, qt=qt: stage_a(unit, u, qt) for u in range(NP) for qt in QT_ORDER]

    def b_tasks(unit):
        return [lambda u=u, qt=qt: stage_b(unit, u, qt) for u in range(NP) for qt in QT_ORDER]

    ones16 = jnp.where(lax.broadcasted_iota(i32, (8, L), 0) == 0, u32(0x3F80), u32(0))

    def mem_task(s, g):
        es, eoff, ne = _ewin(g)
        nv = _valid(g)
        lhs = _bf(jnp.concatenate([vt_u[s, es // 2:(es + ne) // 2, :], ones16], axis=0))
        upd = lax.dot_general(lhs, _bf(pk_u[s * NG + g]), NT_DIMS, preferred_element_type=f32)
        mt = mt_acc[g, 0:ne + 16, :] + upd
        mt_acc[g, 0:ne + 16, :] = mt
        e_loc = lax.broadcasted_iota(i32, (ne, T), 0) - eoff
        d_id = lax.broadcasted_iota(i32, (ne, T), 1)
        same_head = (e_loc >= 0) & (e_loc < nv) & (d_id < nv) & ((e_loc // DH) == (d_id // DH))
        j16 = lax.broadcasted_iota(i32, (16, T), 0)
        d16 = lax.broadcasted_iota(i32, (16, T), 1)
        z_mask = ((d16 // DH) == j16) & (d16 < nv)
        lm = jnp.concatenate(
            [jnp.where(same_head, mt[0:ne], 0.0),
             jnp.where(z_mask, jnp.broadcast_to(mt[ne:ne + 1, :], (16, T)), 0.0)], axis=0)
        nd = jnp.dot(lm.astype(bf16), _bf(pq_u[(s + 1) * NG + g]), preferred_element_type=f32)
        scale = jnp.broadcast_to(g16[g][:, 0:1], (16, L)) / (nd[ne:ne + 16, :] + 1e-6)
        r8 = lax.broadcasted_iota(i32, (8, L), 0)
        for b in range(ne // 8):
            lo, hi = 8 * b - eoff, 8 * b + 7 - eoff
            if hi < 0 or lo >= nv:
                continue
            j1, j2 = max(lo, 0) // DH, min(hi, nv - 1) // DH
            sc = jnp.broadcast_to(scale[j1:j1 + 1, :], (8, L))
            if j2 != j1:
                sc = jnp.where(r8 < DH * j2 - lo, sc, jnp.broadcast_to(scale[j2:j2 + 1, :], (8, L)))
            val = nd[8 * b:8 * b + 8, :] * sc
            dst = am.at[s + 1, es + 8 * b:es + 8 * b + 8, :]
            if lo >= 0 and hi < nv:
                dst[...] = val
            else:
                pltpu.store(dst, val, mask=(r8 + lo >= 0) & (r8 + lo < nv))

    mem_tasks = [lambda s=s, g=g: mem_task(s, g) for s in range(NSEG - 1) for g in range(NG)]

    w_copy(3).wait()
    for i in range(3):
        moe_copy(i).wait()
    rr = jnp.concatenate([r_buf[s][0:1, :] for s in range(NSEG)], axis=0)
    rr = _round_bf16(rr)
    tok = lax.broadcasted_iota(i32, (NSEG, L), 0) * L + lax.broadcasted_iota(i32, (NSEG, L), 1)
    m1v = jnp.max(rr)
    i1 = jnp.min(jnp.where(rr == m1v, tok, SEQ))
    rr2 = jnp.where(tok == i1, -jnp.inf, rr)
    m2v = jnp.max(rr2)
    i2 = jnp.min(jnp.where(rr2 == m2v, tok, SEQ))
    i1 = jnp.clip(i1, 0, SEQ - 1)
    i2 = jnp.clip(i2, 0, SEQ - 1)

    row16 = lax.broadcasted_iota(i32, (16, T), 0)
    lane16 = lax.broadcasted_iota(i32, (16, T), 1)

    def token_rows(i, slot):
        onehot = jnp.where((row16 == slot) & (lane16 == i % T), 1.0, 0.0).astype(bf16)
        return lax.dot_general(onehot, _bf(xn_u[i // T]), NT_DIMS, preferred_element_type=f32)

    def select_task():
        xsel_buf[...] = _pack(token_rows(i1, 0) + token_rows(i2, 1))
        y_acc[...] = jnp.zeros(y_acc.shape, f32)

    def fcols(ft):
        return pl.ds(ft * T if isinstance(ft, int) else pl.multiple_of(ft * T, T), T)

    def moe_up_task(ft, k, which):
        xsel = _bf(xsel_buf[:, 0:D])
        w_ref = (wg_buf, wu_buf)[which]
        hid_buf[k, which] = jnp.dot(xsel, w_ref[:, fcols(ft)], preferred_element_type=f32)

    def moe_down_task(ft, k):
        gt = _round_bf16(hid_buf[k, 0])
        up = _round_bf16(hid_buf[k, 1])
        hid = (_round_bf16(gt * _sigmoid(gt)) * up).astype(bf16)
        y_acc[...] += lax.dot_general(hid, wd_buf[:, fcols(ft)], NT_DIMS, preferred_element_type=f32)

    def moe_tasks(ft0, count):
        tasks = []
        for k0 in range(0, count, FPB):
            ks = range(k0, min(k0 + FPB, count))
            tasks += [lambda k=k, w=w: moe_up_task(ft0 + k, k, w) for k in ks for w in range(2)]
            tasks += [lambda k=k: moe_down_task(ft0 + k, k) for k in ks]
        return tasks

    def moe_finish():
        y = _round_bf16(y_acc[...])
        rsel = jnp.where(lax.broadcasted_iota(i32, (16, 1), 0) == 0, m1v, m2v)
        y = _round_bf16(y * _round_bf16(_sigmoid(rsel)))
        y = jnp.concatenate([y, jnp.zeros((16, DP - D), f32)], axis=1)
        y = jnp.concatenate([jnp.zeros((HT, DP), f32), y, jnp.zeros((T - HT - 16, DP), f32)], axis=0)
        y_t = jnp.concatenate([y.T[0:D], jnp.zeros((D, T), f32)], axis=1)
        y_u = _pack(y_t)[:, 0:T]
        lane = lax.broadcasted_iota(i32, (D // 2, T), 1)
        wot_u[:, DP - T:DP] = jnp.where(lane < HT, wot_u[:, DP - T:DP], y_u)
        rid = lax.broadcasted_iota(i32, (8, T), 0)
        for tt in range(TPS):
            tok_l = lax.broadcasted_iota(i32, (8, T), 1) + (NSEG - 1) * L + tt * T
            ots[tt][D:D + 8, :] = jnp.where(((rid == 0) & (tok_l == i1)) | ((rid == 1) & (tok_l == i2)), 1.0, 0.0)

    dense = _interleave(mem_tasks, a_tasks((0, 0)), prep_dense(3, wot_u, 0))
    with _scope("p15_mix"):
        cut = (2 * len(dense)) // 3
        run(dense[:cut] + [select_task] + dense[cut:])

    def out_tile(s, tt, last):
        c0 = s * L + tt * T
        if not isinstance(s, int):
            c0 = pl.multiple_of(c0, T)
        o_bf = ots[tt][...].astype(bf16)
        nchunk = 4
        rows = D // nchunk
        for rc in range(nchunk):
            r0 = rc * rows
            attn = jnp.dot(_bf(wot_u[r0 // 2:(r0 + rows) // 2, :]), o_bf, preferred_element_type=f32)
            xn = _bf(xn_u[s * TPS + tt, r0 // 2:(r0 + rows) // 2, :]).astype(f32)
            x = x_buf[r0:r0 + rows, pl.ds(c0, T)].astype(f32)
            res = x + attn + xn
            out_buf[r0:r0 + rows, pl.ds(c0, T)] = res.astype(bf16)

    def pair_tasks(ua, ub):
        tasks = []
        for x, y in zip(a_tasks(ua), b_tasks(ub)):
            tasks += [y, x]
        return tasks

    def seg_end(s, last):
        def by_qt(fn, unit, qt):
            return [lambda u=u: fn(unit, u, qt) for u in range(NP)]

        steps = []
        for step in range(7):
            lists = []
            if step < 4:
                lists.append(by_qt(stage_b, (s, 2), 3 - step))
                lists.append(by_qt(stage_a, (s, 3), 3 - step))
            if 1 <= step < 5:
                lists.append(by_qt(stage_b, (s, 3), 4 - step))
            if not last and 2 <= step < 6:
                lists.append(by_qt(stage_a, (s + 1, 0), 5 - step))
            if step >= 3:
                lists.append([lambda tt=6 - step: out_tile(s, tt, last)])
            steps.append(_interleave(*lists))
        return steps

    def seg_att(s, c):
        tasks = pair_tasks((s, 1), (s, 0)) + pair_tasks((s, 2), (s, 1))
        steps = seg_end(s, False)
        for step in steps[0:5]:
            tasks += step
        with _scope("att_seg"):
            run(_interleave(tasks, moe_tasks(s * FPI, FPI)))
            for step in steps[5:]:
                run(step)
        out_copy(pl.multiple_of(s * L, L), L, s).start()
        return c

    lax.fori_loop(0, NSEG - 1, seg_att, 0)

    npatch = (NSEG - 1) * TPS

    def patch_tile(idx):
        return jnp.where(idx < npatch * T, idx // T, 0)

    tile0 = patch_tile(i1)
    tile1 = patch_tile(i2)
    tile1 = jnp.where(tile1 == tile0, (tile0 + 1) % npatch, tile1)

    def patch(tile):
        c0 = pl.multiple_of(tile * T, T)
        rid = lax.broadcasted_iota(i32, (T, T), 0)
        tok_l = lax.broadcasted_iota(i32, (T, T), 1) + c0
        hit = ((rid == HT) & (tok_l == i1)) | ((rid == HT + 1) & (tok_l == i2))
        onehot = jnp.where(hit, 1.0, 0.0).astype(bf16)
        for rc in range(4):
            r0, r1 = rc * (D // 4), (rc + 1) * (D // 4)
            upd = jnp.dot(_bf(wot_u[r0 // 2:r1 // 2, DP - T:DP]), onehot, preferred_element_type=f32)
            cur = out_buf[r0:r1, pl.ds(c0, T)].astype(f32)
            out_buf[r0:r1, pl.ds(c0, T)] = (cur + upd).astype(bf16)

    patch_copies = [out_copy(pl.multiple_of(tile0 * T, T), T, 7), out_copy(pl.multiple_of(tile1 * T, T), T, 8)]
    last_copies = [out_copy((NSEG - 1) * L + tt * T, T, NSEG - 1 + tt) for tt in range(TPS)]

    sl = NSEG - 1
    with _scope("tail_1"):
        moe_finish()
        run(pair_tasks((sl, 1), (sl, 0)))
        for s in range(NSEG - 1):
            out_copy(s * L, L, s).wait()
    with _scope("tail_2"):
        patch(tile0)
        patch(tile1)
        run(pair_tasks((sl, 2), (sl, 1)))
        for cp in patch_copies:
            cp.start()
        steps = seg_end(sl, True)
        for step in steps[0:5]:
            run(step)
        last_copies[3].start()
        last_copies[2].start()
    with _scope("tail_3"):
        run(steps[5])
        run(steps[6])
        last_copies[1].start()
        last_copies[0].start()

    with _scope("out_wait"):
        for cp in patch_copies + last_copies:
            cp.wait()


@jax.jit
def pallas_parallel_sum__memory_aug_infini_attn__moe_arch_mod__prompt_kernel(
    A_x: jax.Array,
    A_wq: jax.Array,
    A_wk: jax.Array,
    A_wv: jax.Array,
    A_wo: jax.Array,
    A_beta: jax.Array,
    B_x: jax.Array,
    B_w_r: jax.Array,
    B_w_gate: jax.Array,
    B_w_up: jax.Array,
    B_w_down: jax.Array,
):
    del B_x
    any_spec = pl.BlockSpec(memory_space=pl.ANY)
    scratch = [
        pltpu.VMEM((H,), bf16),
        pltpu.VMEM((D,), bf16),
        pltpu.VMEM((D, SEQ), bf16),
        pltpu.VMEM((4, D, D), bf16),
        pltpu.VMEM((D, F), bf16),
        pltpu.VMEM((D, F), bf16),
        pltpu.VMEM((D, F), bf16),
        pltpu.VMEM((D, SEQ), bf16),
        pltpu.VMEM((WT_ROWS, DP), u32),
        pltpu.VMEM((D // 2, DP), u32),
        pltpu.VMEM((D // 2, DP), u32),
        pltpu.VMEM((NT, DP // 2, T), u32),
        pltpu.VMEM((BT, DP // 2, T), u32),
        pltpu.VMEM((BT, DP // 2, T), u32),
        pltpu.VMEM((NSEG * NG, TW, L), u32),
        pltpu.VMEM((NSEG * NG, L // 2, T), u32),
        pltpu.VMEM((NSEG * NG, TW, L), u32),
        pltpu.VMEM((NSEG * NG, TW, L), u32),
        pltpu.VMEM((NSEG, D // 2, L), u32),
        pltpu.VMEM((NSEG * H, 16, L), u32),
        pltpu.VMEM((NSEG, 8, L), f32),
        pltpu.VMEM((NG, T + 16, T), f32),
        pltpu.VMEM((NSEG, D, L), f32),
        pltpu.VMEM((NG, 16, T), f32),
        pltpu.VMEM((H, 8, T), f32),
        pltpu.VMEM((3, HT, T), f32),
        pltpu.VMEM((NP, 4, 2 * L, T), f32),
        pltpu.VMEM((NP, 4, 2, 8, T), f32),
        pltpu.VMEM((NP, 4, 2 * L, T), f32),
        pltpu.VMEM((NP, 4, 2, 8, T), f32),
        pltpu.VMEM((DP, T), f32),
        pltpu.VMEM((DP, T), f32),
        pltpu.VMEM((DP, T), f32),
        pltpu.VMEM((DP, T), f32),
        pltpu.VMEM((2, D, LNW), f32),
        pltpu.VMEM((2, 2, 8, LNW), f32),
        pltpu.VMEM((16, D), f32),
        pltpu.VMEM((8, DP), u32),
        pltpu.VMEM((FPI, 2, 16, T), f32),
        pltpu.SemaphoreType.DMA((NSEM,)),
    ]
    x_t = jnp.transpose(A_x, (0, 2, 1)).reshape(D, SEQ)
    out_t = pl.pallas_call(
        _kernel,
        out_shape=jax.ShapeDtypeStruct((D, SEQ), bf16),
        in_specs=[any_spec] * 10,
        out_specs=any_spec,
        scratch_shapes=scratch,
        compiler_params=pltpu.CompilerParams(vmem_limit_bytes=110 * 1024 * 1024),
    )(x_t, A_wq, A_wk, A_wv, A_wo, A_beta, B_w_r, B_w_gate, B_w_up, B_w_down.T)
    return jnp.transpose(out_t.reshape(1, D, SEQ), (0, 2, 1))
```

```python
import contextlib

import jax
import jax.numpy as jnp
from jax import lax
from jax.experimental import pallas as pl
from jax.experimental.pallas import tpu as pltpu

bf16 = jnp.bfloat16
f32 = jnp.float32
u32 = jnp.uint32
i32 = jnp.int32

SEQ = 2048
D = 576
DP = 640
H = 32
DH = 18
NSEG = 4
L = 512
T = 128
TW = T // 2
HT = T // 2
TPS = L // T
HPG = 6
NG = 6
F = 4608
FPI = 12
FPB = 3
NFT = F // T
NP = 4
UPS = H // (2 * NP)
NUNIT = NSEG * UPS
NT = SEQ // T
LNW = 256
BT = LNW // T
NORM_PARTS = 6
VB = 8 * DH

LOG2E = 1.4426950408889634
QSCALE = (DH ** -0.5) * LOG2E
MASKVAL = -1000000000.0 * LOG2E
EPS_BF16 = 1.0013580322265625e-05
ONES_PAIR = 0x3F803F80

NT_DIMS = (((1,), (1,)), ((), ()))

WT_Q = 0
WT_K = NG * TW
WT_V = 2 * NG * TW
WT_ROWS = WT_V + D // 2

X_PIECES = ((0, LNW), (LNW, LNW), (L, L), (2 * L, L), (3 * L, L))
SEM_X = 0
SEM_W = 5
SEM_MOE = 9
SEM_OUT = 12
SEM_SMALL = 21
NSEM = 23


PROFILE_SCOPES = False
PACE = True
TAIL_BARRIERS = False
QT_ORDER = (3, 2, 1, 0)


def _scope(name):
    return jax.named_scope(name) if PROFILE_SCOPES else contextlib.nullcontext()


def _valid(g):
    return min(HPG * DH, D - g * HPG * DH)


def _rows(g):
    return -(-_valid(g) // 16) * 16


def _ewin(g):
    start = (g * HPG * DH // 16) * 16
    return start, g * HPG * DH - start, min(T, D - start)


def _bf(x):
    return pltpu.bitcast(x, bf16)


def _pack(x):
    return pltpu.bitcast(x.astype(bf16), u32)


def _round_bf16(x):
    return x.astype(bf16).astype(f32)


def _phi(t):
    return jnp.where(t > 0, t + 1.0, jnp.exp(t))


def _sigmoid(t):
    return 1.0 / (1.0 + jnp.exp(-t))


def _zero_after(v):
    bits = pltpu.bitcast(v[0:8, 0:LNW], u32)
    sixteen = jnp.uint32(16)
    bits = lax.shift_right_logical(lax.shift_right_logical(bits, sixteen), sixteen)
    return pltpu.bitcast(bits, f32) if PACE else None


def _interleave(*lists):
    items = []
    for li, tasks in enumerate(lists):
        for k, t in enumerate(tasks):
            items.append(((k + 0.5) / len(tasks), li, k, t))
    items.sort(key=lambda it: it[:3])
    return [it[3] for it in items]


def _kernel(x_hbm, wq_hbm, wk_hbm, wv_hbm, wo_hbm, beta_hbm, wr_hbm, wg_hbm, wu_hbm, wd_hbm,
            out_hbm,
            beta_ref, wr_ref, x_buf, w_buf, wg_buf, wu_buf, wd_buf, out_buf,
            wt_u, wtd_u, wot_u, xn_u, xs_a, xs_b, qs_u, k_u, pq_u, pk_u, vt_u, vwin,
            r_buf, mt_acc, lm_f, am, g16, omg, mb,
            s0, m0, s1, m1, ot0, ot1, ot2, ot3, xf, ln_stat, y_acc, xsel_buf, hid_buf, sems):

    def x_copy(i):
        c0, width = X_PIECES[i]
        return pltpu.make_async_copy(x_hbm.at[:, pl.ds(c0, width)], x_buf.at[:, pl.ds(c0, width)],
                                     sems.at[SEM_X + i])

    def w_copy(i):
        src = (wq_hbm, wk_hbm, wv_hbm, wo_hbm)[i]
        return pltpu.make_async_copy(src, w_buf.at[i], sems.at[SEM_W + i])

    def moe_copy(i):
        src = (wg_hbm, wu_hbm, wd_hbm)[i]
        dst = (wg_buf, wu_buf, wd_buf)[i]
        return pltpu.make_async_copy(src, dst, sems.at[SEM_MOE + i])

    def out_copy(c0, width, sem):
        return pltpu.make_async_copy(out_buf.at[:, pl.ds(c0, width)], out_hbm.at[:, pl.ds(c0, width)],
                                     sems.at[SEM_OUT + sem])

    small_copies = [pltpu.make_async_copy(beta_hbm, beta_ref, sems.at[SEM_SMALL]),
                    pltpu.make_async_copy(wr_hbm, wr_ref, sems.at[SEM_SMALL + 1])]
    w_copy(0).start()
    x_copy(0).start()
    x_copy(1).start()
    for cp in small_copies:
        cp.start()
    w_copy(1).start()
    w_copy(2).start()

    init_scope = _scope("init")
    init_scope.__enter__()
    kr = lax.broadcasted_iota(i32, (HT, T), 0)
    ql = lax.broadcasted_iota(i32, (HT, T), 1)
    mb[0] = jnp.where(ql < kr, MASKVAL, 0.0).astype(f32)
    mb[1] = jnp.where((ql >= HT) & (ql - HT < kr), MASKVAL, 0.0).astype(f32)
    mb[2] = jnp.where(ql % HT < kr, MASKVAL, 0.0).astype(f32)
    zpad = jnp.zeros(((DP - D) // 2, T), u32)
    for tt in range(NT):
        xn_u[tt, D // 2:DP // 2, :] = zpad
    for tt in range(BT):
        xs_a[tt, D // 2:DP // 2, :] = zpad
        xs_b[tt, D // 2:DP // 2, :] = zpad
    ots = (ot0, ot1, ot2, ot3)
    for o_ref in ots:
        o_ref[D:DP, :] = jnp.zeros((DP - D, T), f32)
    am[0] = jnp.zeros(am.shape[1:], f32)
    mt_acc[...] = jnp.zeros(mt_acc.shape, f32)
    g16[...] = jnp.zeros(g16.shape, f32)
    for sg in range(NSEG * NG):
        r2 = _rows(sg % NG) // 2
        qs_u[sg, r2:TW, :] = jnp.zeros((TW - r2, L), u32)
        pq_u[sg, r2:TW, :] = jnp.zeros((TW - r2, L), u32)
        pk_u[sg, r2:TW, :] = jnp.zeros((TW - r2, L), u32)

    init_scope.__exit__(None, None, None)

    pace = [None]

    def gate_tables():
        gate = _round_bf16(_sigmoid(beta_ref[...].reshape(1, H).astype(f32)))
        for h in range(H):
            gh = jnp.broadcast_to(gate[:, h:h + 1], (1, T))
            omg[h] = jnp.broadcast_to(_round_bf16(1.0 - gh), (8, T))
            g16[h // HPG, (h % HPG):(h % HPG) + 1, :] = gh

    def transpose_block(i, cb):
        c1 = min((cb + 1) * T, D)
        blk = w_buf[i, :, cb * T:c1]
        if c1 - cb * T < T:
            blk = jnp.concatenate([blk, jnp.zeros((D, T - (c1 - cb * T)), bf16)], axis=1)
        blk = jnp.concatenate([blk, jnp.zeros((DP - D, T), bf16)], axis=0)
        return pltpu.bitcast(blk.T, u32)

    def prep_dense(i, dst, base):
        def task(cb):
            nrow = min(TW, D // 2 - cb * TW)
            dst[base + cb * TW:base + cb * TW + nrow, :] = transpose_block(i, cb)[0:nrow]
        return [lambda cb=cb: task(cb) for cb in range(DP // T)]

    def prep_grouped(i, base):
        def regroup(g):
            nv, nr = _valid(g) // 2, _rows(g) // 2
            src = g * HPG * DH // 2
            wt_u[base + g * TW:base + g * TW + nv, :] = wtd_u[src:src + nv, :]
            pad = jnp.zeros((nr - nv, DP), u32)
            if i == 1 and g == 0:
                wr = wr_ref[...].reshape(1, D).astype(f32)
                wr = jnp.concatenate([wr, jnp.zeros((1, DP - D), f32)], axis=1)
                bits = lax.shift_right_logical(pltpu.bitcast(wr, u32), u32(16))
                rid = lax.broadcasted_iota(i32, (nr - nv, DP), 0)
                pad = jnp.where(rid == 0, bits, pad)
            wt_u[base + g * TW + nv:base + g * TW + nr, :] = pad
        return prep_dense(i, wtd_u, 0) + [lambda g=g: regroup(g) for g in range(NG)]

    def ln_tasks(s, p, stage):
        c0 = s * L + p * LNW
        if not isinstance(s, int):
            c0 = pl.multiple_of(c0, LNW)

        def mean_pass():
            acc = pace[0]
            for r in range(0, D, 64):
                x = x_buf[r:r + 64, pl.ds(c0, LNW)].astype(f32)
                xf[p, r:r + 64, :] = x
                part = jnp.sum(x.reshape(8, 8, LNW), axis=0)
                acc = part if acc is None else acc + part
            mean = jnp.sum(acc, axis=0, keepdims=True) / D
            ln_stat[p, 0] = jnp.broadcast_to(mean, (8, LNW))

        def var_pass():
            mean = ln_stat[p, 0][0:1]
            if pace[0] is not None:
                mean = mean + pace[0][0:1]
            acc = None
            for r in range(0, D, 96):
                xc = xf[p, r:r + 96, :] - mean
                part = jnp.sum((xc * xc).reshape(12, 8, LNW), axis=0)
                acc = part if acc is None else acc + part
            var = jnp.sum(acc, axis=0, keepdims=True) / D
            den = _round_bf16(jnp.sqrt(_round_bf16(_round_bf16(var) + EPS_BF16)))
            ln_stat[p, 1] = jnp.broadcast_to(1.0 / den, (8, LNW))
            ln_stat[p, 0] = jnp.broadcast_to(_round_bf16(mean), (8, LNW))

        def norm_pass(part):
            mean_b = ln_stat[p, 0][0:1]
            if pace[0] is not None:
                mean_b = mean_b + pace[0][0:1]
            inv = ln_stat[p, 1][0:1]
            step = D // NORM_PARTS
            for r in range(part * step, (part + 1) * step, 48):
                xn = _pack(_round_bf16(xf[p, r:r + 48, :] - mean_b) * inv)
                for t in range(BT):
                    xn_u[s * TPS + p * BT + t, r // 2:r // 2 + 24, :] = xn[:, t * T:(t + 1) * T]
                    if stage is not None:
                        stage[t, r // 2:r // 2 + 24, :] = xn[:, t * T:(t + 1) * T]

        return [mean_pass, var_pass] + [lambda part=part: norm_pass(part) for part in range(NORM_PARTS)]

    def load_xs(s, p, stage):
        if stage is None:
            tiles = [xn_u[s * TPS + p * BT + t] for t in range(BT)]
        else:
            tiles = [stage[t] for t in range(BT)]
        return jnp.concatenate([_bf(t) for t in tiles], axis=1)

    def q_task(s, p, stage, g):
        nr = _rows(g) // 2
        cols = slice(p * LNW, (p + 1) * LNW)
        w = _bf(wt_u[WT_Q + g * TW:WT_Q + g * TW + nr, :])
        q = jnp.dot(w, load_xs(s, p, stage), preferred_element_type=f32)
        pace[0] = _zero_after(q)
        qp = _pack(q * QSCALE)
        qrot = jnp.concatenate([pltpu.roll(qp[:, t * T:(t + 1) * T], HT, 1) for t in range(BT)], axis=1)
        rid = lax.broadcasted_iota(i32, qp.shape, 0)
        even = ((rid // (DH // 2)) % 2) == 0
        qs_u[s * NG + g, 0:nr, cols] = jnp.where(even, qrot, qp)
        pq_u[s * NG + g, 0:nr, cols] = _pack(_phi(_round_bf16(q)))

    def k_task(s, p, stage, g):
        nr = _rows(g)
        cols = slice(p * LNW, (p + 1) * LNW)
        w = _bf(wt_u[WT_K + g * TW:WT_K + g * TW + nr // 2, :])
        k = jnp.dot(w, load_xs(s, p, stage), preferred_element_type=f32)
        pace[0] = _zero_after(k)
        if g == 0:
            r_buf[s, :, cols] = jnp.broadcast_to(k[_valid(0):_valid(0) + 1, :], (8, LNW))
        kp = _pack(k)
        pk_u[s * NG + g, 0:nr // 2, cols] = _pack(_phi(_round_bf16(k)))
        kfull = _bf(jnp.concatenate([kp, jnp.zeros(((T - nr) // 2, LNW), u32)], axis=0))
        k_u[s * NG + g, p * (LNW // 2):(p + 1) * (LNW // 2), :] = pltpu.bitcast(kfull.T, u32)

    def v_task(s, p, stage, b):
        cols = slice(p * LNW, (p + 1) * LNW)
        w = _bf(wt_u[WT_V + b * (VB // 2):WT_V + (b + 1) * (VB // 2), :])
        v = jnp.dot(w, load_xs(s, p, stage), preferred_element_type=f32)
        pace[0] = _zero_after(v)
        v = _pack(v)
        vt_u[s, b * (VB // 2):(b + 1) * (VB // 2), cols] = v
        sub = lax.broadcasted_iota(i32, (16, LNW), 0)
        for hh in range(8):
            w8 = (9 * hh) // 8
            ones_row = 0 if 2 * hh == 14 else 15
            vwin[s * H + 8 * b + hh, :, cols] = jnp.where(sub == ones_row, u32(ONES_PAIR), v[8 * w8:8 * w8 + 16, :])

    def q_tasks(s, p, stage=None):
        return [lambda g=g: q_task(s, p, stage, g) for g in range(NG)]

    def k_tasks(s, p, stage=None):
        return [lambda g=g: k_task(s, p, stage, g) for g in range(NG)]

    def v_tasks(s, p, stage=None):
        return [lambda b=b: v_task(s, p, stage, b) for b in range(D // VB)]

    def mem_layout(g):
        es, eoff, _ = _ewin(g)
        nv = _valid(g)
        ne = -(-(eoff + nv) // 16) * 16
        ones_row = 0 if eoff >= 2 else eoff + nv
        nh = nv // DH
        den_row = 0 if eoff >= nh else ne
        return es, eoff, nv, ne, ones_row, den_row, max(ne, den_row + 16 * (den_row > 0))

    def mem_update(sp, g):
        es, eoff, nv, ne, ones_row, den_row, nr = mem_layout(g)
        win = vt_u[sp, es // 2:(es + ne) // 2, :]
        wid = lax.broadcasted_iota(i32, win.shape, 0)
        lhs = _bf(jnp.where(wid == ones_row // 2, u32(ONES_PAIR), win))
        upd = lax.dot_general(lhs, _bf(pk_u[sp * NG + g]), NT_DIMS, preferred_element_type=f32)
        mt = mt_acc[g, 0:ne, :] + upd
        mt_acc[g, 0:ne, :] = mt
        z = jnp.broadcast_to(mt[ones_row:ones_row + 1, :], (nr, T))
        if nr > ne:
            mt = jnp.concatenate([mt, jnp.zeros((nr - ne, T), f32)], axis=0)
        row = lax.broadcasted_iota(i32, (nr, T), 0)
        d_id = lax.broadcasted_iota(i32, (nr, T), 1)
        e_loc = row - eoff
        same_head = (e_loc >= 0) & (e_loc < nv) & (d_id < nv) & ((e_loc // DH) == (d_id // DH))
        den_hit = (row >= den_row) & (d_id < nv) & ((d_id // DH) == row - den_row)
        lm_f[g, 0:nr, :] = jnp.where(same_head, mt, jnp.where(den_hit, z, 0.0))

    def mem_retrieve(s, g):
        es, eoff, nv, ne, ones_row, den_row, nr = mem_layout(g)
        nd = jnp.dot(lm_f[g, 0:nr, :].astype(bf16), _bf(pq_u[s * NG + g]), preferred_element_type=f32)
        scale = jnp.broadcast_to(g16[g][:, 0:1], (8, L)) / (nd[den_row:den_row + 8, :] + 1e-6)
        r8 = lax.broadcasted_iota(i32, (8, L), 0)
        for b in range(ne // 8):
            lo, hi = 8 * b - eoff, 8 * b + 7 - eoff
            if hi < 0 or lo >= nv:
                continue
            j1, j2 = max(lo, 0) // DH, min(hi, nv - 1) // DH
            sc = jnp.broadcast_to(scale[j1:j1 + 1, :], (8, L))
            if j2 != j1:
                sc = jnp.where(r8 < DH * j2 - lo, sc, jnp.broadcast_to(scale[j2:j2 + 1, :], (8, L)))
            val = nd[8 * b:8 * b + 8, :] * sc
            dst = am.at[s, es + 8 * b:es + 8 * b + 8, :]
            if lo >= 0 and hi < nv:
                dst[...] = val
            else:
                pltpu.store(dst, val, mask=(r8 + lo >= 0) & (r8 + lo < nv))

    def run(tasks):
        for t in tasks:
            t()

    prep_q = prep_grouped(0, WT_Q)
    with _scope("p1_wait_wq"):
        w_copy(0).wait()
    with _scope("p1_prep_q"):
        run(prep_q[0:3])
        x_copy(0).wait()
    for i in range(2, len(X_PIECES)):
        x_copy(i).start()
    w_copy(3).start()
    for i in range(3):
        moe_copy(i).start()
    with _scope("p1_ln0a"):
        run(_interleave(prep_q[3:], ln_tasks(0, 0, None)))
        x_copy(1).wait()
    with _scope("p1_q0a"):
        run(_interleave(q_tasks(0, 0), ln_tasks(0, 1, None)))
        w_copy(1).wait()
        for cp in small_copies:
            cp.wait()
    k0 = k_tasks(0, 0) + k_tasks(0, 1)
    with _scope("p1_q0b"):
        run(_interleave(q_tasks(0, 1), prep_grouped(1, WT_K), [gate_tables]))
        run(k0[0:NG])
        w_copy(2).wait()
        x_copy(2).wait()
    with _scope("p1_k0v0"):
        run(_interleave(k0[NG:], prep_dense(2, wt_u, WT_V)))
        run(_interleave(v_tasks(0, 0) + v_tasks(0, 1), ln_tasks(1, 0, xs_a)))

    def seg_body(s, c):
        for ss in range(2, NSEG):
            @pl.when(s + 1 == ss)
            def _():
                x_copy(ss + 1).wait()
        nxt = jnp.minimum(s + 1, NSEG - 1)
        pace[0] = None
        with _scope("p1_seg"):
            updates = [lambda g=g: mem_update(s - 1, g) for g in range(NG)]
            retrieves = [lambda g=g: mem_retrieve(s, g) for g in range(NG)]
            first = _interleave(q_tasks(s, 0, xs_a), updates) + k_tasks(s, 0, xs_a) + v_tasks(s, 0, xs_a)
            run(_interleave(first, ln_tasks(s, 1, xs_b)))
            second = q_tasks(s, 1, xs_b) + _interleave(k_tasks(s, 1, xs_b) + v_tasks(s, 1, xs_b), retrieves)
            run(_interleave(second, ln_tasks(nxt, 0, xs_a)))
        return c

    lax.fori_loop(1, NSEG, seg_body, 0)

    bufs = ((s0, m0), (s1, m1))
    lane64 = lax.broadcasted_iota(i32, (TW, T), 1)
    lane1 = lax.broadcasted_iota(i32, (1, T), 1)
    lane8 = lax.broadcasted_iota(i32, (8, T), 1)

    def head_rows(qw, j):
        lo, hi = (DH // 2) * j, (DH // 2) * (j + 1)
        r0, r1 = (lo // 8) * 8, -(-hi // 8) * 8
        rid = lax.broadcasted_iota(i32, (r1 - r0, T), 0) + r0
        part = jnp.where((rid >= lo) & (rid < hi), qw[r0:r1], u32(0))
        pieces = [jnp.zeros((r0, T), u32)] * (r0 > 0) + [part] + [jnp.zeros((TW - r1, T), u32)] * (r1 < TW)
        return jnp.concatenate(pieces, axis=0)

    def stage_a(unit, u, qt):
        s, k = unit
        s_ref, m_ref = bufs[k % 2]
        pi = k * NP + u
        g = pi // (HPG // 2)
        j = 2 * (pi - (HPG // 2) * g)
        sg = s * NG + g
        n = T * (qt + 1)
        qw = qs_u[sg, :, qt * T:(qt + 1) * T]
        w_a = head_rows(qw, j)
        w_b = head_rows(qw, j + 1)
        w_ab = _bf(jnp.where(lane64 < HT, w_a, w_b))

        def colmax8(v):
            return jnp.max(v.reshape(v.shape[0] // 8, 8, T), axis=0)

        maxes = []
        for hd, w in enumerate((_bf(w_a), _bf(w_b))):
            m8 = None
            for c in range(qt):
                kc = _bf(k_u[sg, c * TW:(c + 1) * TW, :])
                sc = jnp.dot(kc, w, preferred_element_type=f32)
                s_ref[u, qt, hd * L + c * T:hd * L + (c + 1) * T, :] = sc
                m8 = colmax8(sc) if m8 is None else jnp.maximum(m8, colmax8(sc))
            kc = _bf(k_u[sg, qt * TW:qt * TW + TW // 2, :])
            sc = jnp.dot(kc, w, preferred_element_type=f32) + mb[1 - hd]
            s_ref[u, qt, hd * L + qt * T:hd * L + qt * T + HT, :] = sc
            m8 = colmax8(sc) if m8 is None else jnp.maximum(m8, colmax8(sc))
            maxes.append(m8)
        kc = _bf(k_u[sg, qt * TW + TW // 2:(qt + 1) * TW, :])
        sc = jnp.dot(kc, w_ab, preferred_element_type=f32) + mb[2]
        s_ref[u, qt, n - HT:n, :] = sc
        mab = colmax8(sc)
        m_a = jnp.where(lane8 < HT, jnp.maximum(maxes[0], mab), maxes[0])
        m_b = jnp.where(lane8 >= HT, jnp.maximum(maxes[1], mab), maxes[1])
        m_ref[u, qt, 0] = jnp.broadcast_to(jnp.max(m_a, axis=0, keepdims=True), (8, T))
        m_ref[u, qt, 1] = jnp.broadcast_to(jnp.max(m_b, axis=0, keepdims=True), (8, T))

    def stage_b(unit, u, qt):
        s, k = unit
        s_ref, m_ref = bufs[k % 2]
        pi = k * NP + u
        n = T * (qt + 1)
        m_a = m_ref[u, qt, 0][0:1]
        m_b = m_ref[u, qt, 1][0:1]
        p_ab = jnp.exp2(s_ref[u, qt, n - HT:n, :] - jnp.where(lane1 < HT, m_a, m_b))
        for hd, m in enumerate((m_a, m_b)):
            h = 2 * pi + hd
            p = jnp.exp2(s_ref[u, qt, hd * L:hd * L + n - HT, :] - m)
            keep = (lane64 < HT) if hd == 0 else (lane64 >= HT)
            p = jnp.concatenate([p, jnp.where(keep, p_ab, 0.0)], axis=0).astype(bf16)
            w0 = ((DH * h) // 16) * 16
            off = DH * h - w0
            o = jnp.dot(_bf(vwin[s * H + h, :, 0:n]), p, preferred_element_type=f32)
            den = o[0:1] if off == 14 else o[31:32]
            r0, r1 = (off // 8) * 8, -(-(off + DH) // 8) * 8
            o = o[r0:r1] * (omg[h][0:1] / den)
            if hd == 0:
                o = pltpu.roll(o, HT, 1)
            res = am[s, w0 + r0:w0 + r1, qt * T:(qt + 1) * T] + o
            rid = lax.broadcasted_iota(i32, (r1 - r0, T), 0) + r0
            pltpu.store(ots[qt].at[w0 + r0:w0 + r1, :], res, mask=(rid >= off) & (rid < off + DH))

    def a_tasks(unit):
        return [lambda u=u, qt=qt: stage_a(unit, u, qt) for u in range(NP) for qt in QT_ORDER]

    def b_tasks(unit):
        return [lambda u=u, qt=qt: stage_b(unit, u, qt) for u in range(NP) for qt in QT_ORDER]

    w_copy(3).wait()
    for i in range(3):
        moe_copy(i).wait()
    rr = jnp.concatenate([r_buf[s][0:1, :] for s in range(NSEG)], axis=0)
    rr = _round_bf16(rr)
    tok = lax.broadcasted_iota(i32, (NSEG, L), 0) * L + lax.broadcasted_iota(i32, (NSEG, L), 1)
    m1v = jnp.max(rr)
    i1 = jnp.min(jnp.where(rr == m1v, tok, SEQ))
    rr2 = jnp.where(tok == i1, -jnp.inf, rr)
    m2v = jnp.max(rr2)
    i2 = jnp.min(jnp.where(rr2 == m2v, tok, SEQ))
    i1 = jnp.clip(i1, 0, SEQ - 1)
    i2 = jnp.clip(i2, 0, SEQ - 1)

    row16 = lax.broadcasted_iota(i32, (16, T), 0)
    lane16 = lax.broadcasted_iota(i32, (16, T), 1)

    def token_rows(i, slot):
        onehot = jnp.where((row16 == slot) & (lane16 == i % T), 1.0, 0.0).astype(bf16)
        return lax.dot_general(onehot, _bf(xn_u[i // T]), NT_DIMS, preferred_element_type=f32)

    def select_task():
        xsel_buf[...] = _pack(token_rows(i1, 0) + token_rows(i2, 1))
        y_acc[...] = jnp.zeros(y_acc.shape, f32)

    def fcols(ft):
        return pl.ds(ft * T if isinstance(ft, int) else pl.multiple_of(ft * T, T), T)

    def moe_up_task(ft, k, which):
        xsel = _bf(xsel_buf[:, 0:D])
        w_ref = (wg_buf, wu_buf)[which]
        hid_buf[k, which] = jnp.dot(xsel, w_ref[:, fcols(ft)], preferred_element_type=f32)

    def moe_down_task(ft, k):
        gt = _round_bf16(hid_buf[k, 0])
        up = _round_bf16(hid_buf[k, 1])
        hid = (_round_bf16(gt * _sigmoid(gt)) * up).astype(bf16)
        y_acc[...] += lax.dot_general(hid, wd_buf[:, fcols(ft)], NT_DIMS, preferred_element_type=f32)

    def moe_tasks(ft0, count):
        tasks = []
        for k0 in range(0, count, FPB):
            ks = range(k0, min(k0 + FPB, count))
            tasks += [lambda k=k, w=w: moe_up_task(ft0 + k, k, w) for k in ks for w in range(2)]
            tasks += [lambda k=k: moe_down_task(ft0 + k, k) for k in ks]
        return tasks

    def moe_finish():
        y = _round_bf16(y_acc[...])
        rsel = jnp.where(lax.broadcasted_iota(i32, (16, 1), 0) == 0, m1v, m2v)
        y = _round_bf16(y * _round_bf16(_sigmoid(rsel)))
        y = jnp.concatenate([y, jnp.zeros((16, DP - D), f32)], axis=1)
        y = jnp.concatenate([jnp.zeros((HT, DP), f32), y, jnp.zeros((T - HT - 16, DP), f32)], axis=0)
        y_t = jnp.concatenate([y.T[0:D], jnp.zeros((D, T), f32)], axis=1)
        y_u = _pack(y_t)[:, 0:T]
        lane = lax.broadcasted_iota(i32, (D // 2, T), 1)
        wot_u[:, DP - T:DP] = jnp.where(lane < HT, wot_u[:, DP - T:DP], y_u)
        rid = lax.broadcasted_iota(i32, (8, T), 0)
        for tt in range(TPS):
            tok_l = lax.broadcasted_iota(i32, (8, T), 1) + (NSEG - 1) * L + tt * T
            ots[tt][D:D + 8, :] = jnp.where(((rid == 0) & (tok_l == i1)) | ((rid == 1) & (tok_l == i2)), 1.0, 0.0)

    dense = _interleave(a_tasks((0, 0)), prep_dense(3, wot_u, 0))
    with _scope("p15_mix"):
        cut = (2 * len(dense)) // 3
        run(dense[:cut] + [select_task] + dense[cut:])

    def out_tile(s, tt, last):
        c0 = s * L + tt * T
        if not isinstance(s, int):
            c0 = pl.multiple_of(c0, T)
        o_bf = ots[tt][...].astype(bf16)
        nchunk = 4
        rows = D // nchunk
        for rc in range(nchunk):
            r0 = rc * rows
            attn = jnp.dot(_bf(wot_u[r0 // 2:(r0 + rows) // 2, :]), o_bf, preferred_element_type=f32)
            xn = _bf(xn_u[s * TPS + tt, r0 // 2:(r0 + rows) // 2, :]).astype(f32)
            x = x_buf[r0:r0 + rows, pl.ds(c0, T)].astype(f32)
            res = x + attn + xn
            out_buf[r0:r0 + rows, pl.ds(c0, T)] = res.astype(bf16)

    def pair_tasks(ua, ub):
        tasks = []
        for x, y in zip(a_tasks(ua), b_tasks(ub)):
            tasks += [y, x]
        return tasks

    def seg_end(s, last):
        def by_qt(fn, unit, qt):
            return [lambda u=u: fn(unit, u, qt) for u in range(NP)]

        steps = []
        for step in range(7):
            lists = []
            if step < 4:
                lists.append(by_qt(stage_b, (s, 2), 3 - step))
                lists.append(by_qt(stage_a, (s, 3), 3 - step))
            if 1 <= step < 5:
                lists.append(by_qt(stage_b, (s, 3), 4 - step))
            if not last and 2 <= step < 6:
                lists.append(by_qt(stage_a, (s + 1, 0), 5 - step))
            if step >= 3:
                lists.append([lambda tt=6 - step: out_tile(s, tt, last)])
            steps.append(_interleave(*lists))
        return steps

    def seg_att(s, c):
        tasks = pair_tasks((s, 1), (s, 0)) + pair_tasks((s, 2), (s, 1))
        steps = seg_end(s, False)
        for step in steps[0:5]:
            tasks += step
        with _scope("att_seg"):
            run(_interleave(tasks, moe_tasks(s * FPI, FPI)))
            for step in steps[5:]:
                run(step)
        out_copy(pl.multiple_of(s * L, L), L, s).start()
        return c

    lax.fori_loop(0, NSEG - 1, seg_att, 0)

    npatch = (NSEG - 1) * TPS

    def patch_tile(idx):
        return jnp.where(idx < npatch * T, idx // T, 0)

    tile0 = patch_tile(i1)
    tile1 = patch_tile(i2)
    tile1 = jnp.where(tile1 == tile0, (tile0 + 1) % npatch, tile1)

    def patch(tile):
        c0 = pl.multiple_of(tile * T, T)
        rid = lax.broadcasted_iota(i32, (T, T), 0)
        tok_l = lax.broadcasted_iota(i32, (T, T), 1) + c0
        hit = ((rid == HT) & (tok_l == i1)) | ((rid == HT + 1) & (tok_l == i2))
        onehot = jnp.where(hit, 1.0, 0.0).astype(bf16)
        for rc in range(4):
            r0, r1 = rc * (D // 4), (rc + 1) * (D // 4)
            upd = jnp.dot(_bf(wot_u[r0 // 2:r1 // 2, DP - T:DP]), onehot, preferred_element_type=f32)
            cur = out_buf[r0:r1, pl.ds(c0, T)].astype(f32)
            out_buf[r0:r1, pl.ds(c0, T)] = (cur + upd).astype(bf16)

    patch_copies = [out_copy(pl.multiple_of(tile0 * T, T), T, 7), out_copy(pl.multiple_of(tile1 * T, T), T, 8)]
    last_copies = [out_copy((NSEG - 1) * L + tt * T, T, NSEG - 1 + tt) for tt in range(TPS)]

    sl = NSEG - 1
    with _scope("tail_1"):
        moe_finish()
        run(pair_tasks((sl, 1), (sl, 0)))
        for s in range(NSEG - 1):
            out_copy(s * L, L, s).wait()
    with _scope("tail_2"):
        patch(tile0)
        patch(tile1)
        run(pair_tasks((sl, 2), (sl, 1)))
        for cp in patch_copies:
            cp.start()
        steps = seg_end(sl, True)
        for step in steps[0:5]:
            run(step)
        last_copies[3].start()
        last_copies[2].start()
    with _scope("tail_3"):
        run(steps[5])
        run(steps[6])
        last_copies[1].start()
        last_copies[0].start()

    with _scope("out_wait"):
        for cp in patch_copies + last_copies:
            cp.wait()


@jax.jit
def pallas_parallel_sum__memory_aug_infini_attn__moe_arch_mod__prompt_kernel(
    A_x: jax.Array,
    A_wq: jax.Array,
    A_wk: jax.Array,
    A_wv: jax.Array,
    A_wo: jax.Array,
    A_beta: jax.Array,
    B_x: jax.Array,
    B_w_r: jax.Array,
    B_w_gate: jax.Array,
    B_w_up: jax.Array,
    B_w_down: jax.Array,
):
    del B_x
    any_spec = pl.BlockSpec(memory_space=pl.ANY)
    scratch = [
        pltpu.VMEM((H,), bf16),
        pltpu.VMEM((D,), bf16),
        pltpu.VMEM((D, SEQ), bf16),
        pltpu.VMEM((4, D, D), bf16),
        pltpu.VMEM((D, F), bf16),
        pltpu.VMEM((D, F), bf16),
        pltpu.VMEM((D, F), bf16),
        pltpu.VMEM((D, SEQ), bf16),
        pltpu.VMEM((WT_ROWS, DP), u32),
        pltpu.VMEM((D // 2, DP), u32),
        pltpu.VMEM((D // 2, DP), u32),
        pltpu.VMEM((NT, DP // 2, T), u32),
        pltpu.VMEM((BT, DP // 2, T), u32),
        pltpu.VMEM((BT, DP // 2, T), u32),
        pltpu.VMEM((NSEG * NG, TW, L), u32),
        pltpu.VMEM((NSEG * NG, L // 2, T), u32),
        pltpu.VMEM((NSEG * NG, TW, L), u32),
        pltpu.VMEM((NSEG * NG, TW, L), u32),
        pltpu.VMEM((NSEG, D // 2, L), u32),
        pltpu.VMEM((NSEG * H, 16, L), u32),
        pltpu.VMEM((NSEG, 8, L), f32),
        pltpu.VMEM((NG, T, T), f32),
        pltpu.VMEM((NG, T, T), f32),
        pltpu.VMEM((NSEG, D, L), f32),
        pltpu.VMEM((NG, 8, T), f32),
        pltpu.VMEM((H, 8, T), f32),
        pltpu.VMEM((3, HT, T), f32),
        pltpu.VMEM((NP, 4, 2 * L, T), f32),
        pltpu.VMEM((NP, 4, 2, 8, T), f32),
        pltpu.VMEM((NP, 4, 2 * L, T), f32),
        pltpu.VMEM((NP, 4, 2, 8, T), f32),
        pltpu.VMEM((DP, T), f32),
        pltpu.VMEM((DP, T), f32),
        pltpu.VMEM((DP, T), f32),
        pltpu.VMEM((DP, T), f32),
        pltpu.VMEM((2, D, LNW), f32),
        pltpu.VMEM((2, 2, 8, LNW), f32),
        pltpu.VMEM((16, D), f32),
        pltpu.VMEM((8, DP), u32),
        pltpu.VMEM((FPI, 2, 16, T), f32),
        pltpu.SemaphoreType.DMA((NSEM,)),
    ]
    x_t = jnp.transpose(A_x, (0, 2, 1)).reshape(D, SEQ)
    out_t = pl.pallas_call(
        _kernel,
        out_shape=jax.ShapeDtypeStruct((D, SEQ), bf16),
        in_specs=[any_spec] * 10,
        out_specs=any_spec,
        scratch_shapes=scratch,
        compiler_params=pltpu.CompilerParams(vmem_limit_bytes=110 * 1024 * 1024),
    )(x_t, A_wq, A_wk, A_wv, A_wo, A_beta, B_w_r, B_w_gate, B_w_up, B_w_down.T)
    return jnp.transpose(out_t.reshape(1, D, SEQ), (0, 2, 1))
```

```python
import contextlib

import jax
import jax.numpy as jnp
from jax import lax
from jax.experimental import pallas as pl
from jax.experimental.pallas import tpu as pltpu

bf16 = jnp.bfloat16
f32 = jnp.float32
u32 = jnp.uint32
i32 = jnp.int32

SEQ = 2048
D = 576
DP = 640
H = 32
DH = 18
NSEG = 4
L = 512
T = 128
TW = T // 2
HT = T // 2
TPS = L // T
HPG = 6
NG = 6
F = 4608
FPI = 12
FPB = 3
NFT = F // T
NP = 4
UPS = H // (2 * NP)
NUNIT = NSEG * UPS
NT = SEQ // T
LNW = 256
BT = LNW // T
NORM_PARTS = 6
VB = 8 * DH

LOG2E = 1.4426950408889634
QSCALE = (DH ** -0.5) * LOG2E
MASKVAL = -1000000000.0 * LOG2E
EPS_BF16 = 1.0013580322265625e-05
ONES_PAIR = 0x3F803F80

NT_DIMS = (((1,), (1,)), ((), ()))

WT_Q = 0
WT_K = NG * TW
WT_V = 2 * NG * TW
WT_ROWS = WT_V + D // 2

X_PIECES = ((0, LNW), (LNW, LNW), (L, L), (2 * L, L), (3 * L, L))
SEM_X = 0
SEM_W = 5
SEM_MOE = 9
SEM_OUT = 12
SEM_SMALL = 21
SEM_WQB = 23
SEM_FINAL = 24
NSEM = 28
WQ_SPLIT = 2 * T


PROFILE_SCOPES = False
PACE = True
TAIL_BARRIERS = False
QT_ORDER = (3, 2, 1, 0)


def _scope(name):
    return jax.named_scope(name) if PROFILE_SCOPES else contextlib.nullcontext()


def _valid(g):
    return min(HPG * DH, D - g * HPG * DH)


def _rows(g):
    return -(-_valid(g) // 16) * 16


def _ewin(g):
    start = (g * HPG * DH // 16) * 16
    return start, g * HPG * DH - start, min(T, D - start)


def _bf(x):
    return pltpu.bitcast(x, bf16)


def _pack(x):
    return pltpu.bitcast(x.astype(bf16), u32)


def _round_bf16(x):
    return x.astype(bf16).astype(f32)


def _phi(t):
    return jnp.where(t > 0, t + 1.0, jnp.exp(t))


def _sigmoid(t):
    return 1.0 / (1.0 + jnp.exp(-t))


def _zero_after(v):
    bits = pltpu.bitcast(v[0:8, 0:LNW], u32)
    sixteen = jnp.uint32(16)
    bits = lax.shift_right_logical(lax.shift_right_logical(bits, sixteen), sixteen)
    return pltpu.bitcast(bits, f32) if PACE else None


def _interleave(*lists):
    items = []
    for li, tasks in enumerate(lists):
        for k, t in enumerate(tasks):
            items.append(((k + 0.5) / len(tasks), li, k, t))
    items.sort(key=lambda it: it[:3])
    return [it[3] for it in items]


def _kernel(x_hbm, wq_hbm, wk_hbm, wv_hbm, wo_hbm, beta_hbm, wr_hbm, wg_hbm, wu_hbm, wd_hbm,
            out_hbm,
            beta_ref, wr_ref, x_buf, w_buf, wg_buf, wu_buf, wd_buf, out_buf,
            wt_u, wtd_u, wot_u, xn_u, xs_a, xs_b, qs_u, k_u, pq_u, pk_u, vt_u, vwin,
            r_buf, mt_acc, lm_f, am, g16, omg, mb,
            s0, m0, s1, m1, ot0, ot1, ot2, ot3, xf, ln_stat, y_acc, xsel_buf, hid_buf, sems):

    def x_copy(i):
        c0, width = X_PIECES[i]
        return pltpu.make_async_copy(x_hbm.at[:, pl.ds(c0, width)], x_buf.at[:, pl.ds(c0, width)],
                                     sems.at[SEM_X + i])

    def w_copy(i):
        src = (wq_hbm, wk_hbm, wv_hbm, wo_hbm)[i]
        return pltpu.make_async_copy(src, w_buf.at[i], sems.at[SEM_W + i])

    wq_first = pltpu.make_async_copy(wq_hbm.at[:, 0:WQ_SPLIT], w_buf.at[0, :, 0:WQ_SPLIT], sems.at[SEM_W])
    wq_rest = pltpu.make_async_copy(wq_hbm.at[:, WQ_SPLIT:D], w_buf.at[0, :, WQ_SPLIT:D], sems.at[SEM_WQB])

    def moe_copy(i):
        src = (wg_hbm, wu_hbm, wd_hbm)[i]
        dst = (wg_buf, wu_buf, wd_buf)[i]
        return pltpu.make_async_copy(src, dst, sems.at[SEM_MOE + i])

    def out_copy(c0, width, sem):
        return pltpu.make_async_copy(out_buf.at[:, pl.ds(c0, width)], out_hbm.at[:, pl.ds(c0, width)],
                                     sems.at[SEM_OUT + sem])

    small_copies = [pltpu.make_async_copy(beta_hbm, beta_ref, sems.at[SEM_SMALL]),
                    pltpu.make_async_copy(wr_hbm, wr_ref, sems.at[SEM_SMALL + 1])]
    x_copy(0).start()
    wq_first.start()
    wq_rest.start()
    x_copy(1).start()
    for cp in small_copies:
        cp.start()
    w_copy(1).start()
    w_copy(2).start()

    init_scope = _scope("init")
    init_scope.__enter__()
    kr = lax.broadcasted_iota(i32, (HT, T), 0)
    ql = lax.broadcasted_iota(i32, (HT, T), 1)
    mb[0] = jnp.where(ql < kr, MASKVAL, 0.0).astype(f32)
    mb[1] = jnp.where((ql >= HT) & (ql - HT < kr), MASKVAL, 0.0).astype(f32)
    mb[2] = jnp.where(ql % HT < kr, MASKVAL, 0.0).astype(f32)
    zpad = jnp.zeros(((DP - D) // 2, T), u32)
    for tt in range(NT):
        xn_u[tt, D // 2:DP // 2, :] = zpad
    for tt in range(BT):
        xs_a[tt, D // 2:DP // 2, :] = zpad
        xs_b[tt, D // 2:DP // 2, :] = zpad
    ots = (ot0, ot1, ot2, ot3)
    for o_ref in ots:
        o_ref[D:DP, :] = jnp.zeros((DP - D, T), f32)
    am[0] = jnp.zeros(am.shape[1:], f32)
    mt_acc[...] = jnp.zeros(mt_acc.shape, f32)
    g16[...] = jnp.zeros(g16.shape, f32)
    for sg in range(NSEG * NG):
        r2 = _rows(sg % NG) // 2
        qs_u[sg, r2:TW, :] = jnp.zeros((TW - r2, L), u32)
        pq_u[sg, r2:TW, :] = jnp.zeros((TW - r2, L), u32)
        pk_u[sg, r2:TW, :] = jnp.zeros((TW - r2, L), u32)

    init_scope.__exit__(None, None, None)

    pace = [None]

    def gate_tables():
        gate = _round_bf16(_sigmoid(beta_ref[...].reshape(1, H).astype(f32)))
        for h in range(H):
            gh = jnp.broadcast_to(gate[:, h:h + 1], (1, T))
            omg[h] = jnp.broadcast_to(_round_bf16(1.0 - gh), (8, T))
            g16[h // HPG, (h % HPG):(h % HPG) + 1, :] = gh

    def transpose_block(i, cb):
        c1 = min((cb + 1) * T, D)
        blk = w_buf[i, :, cb * T:c1]
        if c1 - cb * T < T:
            blk = jnp.concatenate([blk, jnp.zeros((D, T - (c1 - cb * T)), bf16)], axis=1)
        blk = jnp.concatenate([blk, jnp.zeros((DP - D, T), bf16)], axis=0)
        return pltpu.bitcast(blk.T, u32)

    def prep_dense(i, dst, base):
        def task(cb):
            nrow = min(TW, D // 2 - cb * TW)
            dst[base + cb * TW:base + cb * TW + nrow, :] = transpose_block(i, cb)[0:nrow]
        return [lambda cb=cb: task(cb) for cb in range(DP // T)]

    def prep_grouped(i, base):
        def regroup(g):
            nv, nr = _valid(g) // 2, _rows(g) // 2
            src = g * HPG * DH // 2
            wt_u[base + g * TW:base + g * TW + nv, :] = wtd_u[src:src + nv, :]
            pad = jnp.zeros((nr - nv, DP), u32)
            if i == 1 and g == 0:
                wr = wr_ref[...].reshape(1, D).astype(f32)
                wr = jnp.concatenate([wr, jnp.zeros((1, DP - D), f32)], axis=1)
                bits = lax.shift_right_logical(pltpu.bitcast(wr, u32), u32(16))
                rid = lax.broadcasted_iota(i32, (nr - nv, DP), 0)
                pad = jnp.where(rid == 0, bits, pad)
            wt_u[base + g * TW + nv:base + g * TW + nr, :] = pad
        return prep_dense(i, wtd_u, 0) + [lambda g=g: regroup(g) for g in range(NG)]

    def ln_tasks(s, p, stage):
        c0 = s * L + p * LNW
        if not isinstance(s, int):
            c0 = pl.multiple_of(c0, LNW)

        def mean_pass():
            acc = pace[0]
            for r in range(0, D, 64):
                x = x_buf[r:r + 64, pl.ds(c0, LNW)].astype(f32)
                xf[p, r:r + 64, :] = x
                part = jnp.sum(x.reshape(8, 8, LNW), axis=0)
                acc = part if acc is None else acc + part
            mean = jnp.sum(acc, axis=0, keepdims=True) / D
            ln_stat[p, 0] = jnp.broadcast_to(mean, (8, LNW))

        def var_pass():
            mean = ln_stat[p, 0][0:1]
            if pace[0] is not None:
                mean = mean + pace[0][0:1]
            acc = None
            for r in range(0, D, 96):
                xc = xf[p, r:r + 96, :] - mean
                part = jnp.sum((xc * xc).reshape(12, 8, LNW), axis=0)
                acc = part if acc is None else acc + part
            var = jnp.sum(acc, axis=0, keepdims=True) / D
            den = _round_bf16(jnp.sqrt(_round_bf16(_round_bf16(var) + EPS_BF16)))
            ln_stat[p, 1] = jnp.broadcast_to(1.0 / den, (8, LNW))
            ln_stat[p, 0] = jnp.broadcast_to(_round_bf16(mean), (8, LNW))

        def norm_pass(part):
            mean_b = ln_stat[p, 0][0:1]
            if pace[0] is not None:
                mean_b = mean_b + pace[0][0:1]
            inv = ln_stat[p, 1][0:1]
            step = D // NORM_PARTS
            for r in range(part * step, (part + 1) * step, 48):
                xn = _pack(_round_bf16(xf[p, r:r + 48, :] - mean_b) * inv)
                for t in range(BT):
                    xn_u[s * TPS + p * BT + t, r // 2:r // 2 + 24, :] = xn[:, t * T:(t + 1) * T]
                    if stage is not None:
                        stage[t, r // 2:r // 2 + 24, :] = xn[:, t * T:(t + 1) * T]

        return [mean_pass, var_pass] + [lambda part=part: norm_pass(part) for part in range(NORM_PARTS)]

    def load_xs(s, p, stage):
        if stage is None:
            tiles = [xn_u[s * TPS + p * BT + t] for t in range(BT)]
        else:
            tiles = [stage[t] for t in range(BT)]
        return jnp.concatenate([_bf(t) for t in tiles], axis=1)

    def q_task(s, p, stage, g):
        nr = _rows(g) // 2
        cols = slice(p * LNW, (p + 1) * LNW)
        w = _bf(wt_u[WT_Q + g * TW:WT_Q + g * TW + nr, :])
        q = jnp.dot(w, load_xs(s, p, stage), preferred_element_type=f32)
        pace[0] = _zero_after(q)
        qp = _pack(q * QSCALE)
        qrot = jnp.concatenate([pltpu.roll(qp[:, t * T:(t + 1) * T], HT, 1) for t in range(BT)], axis=1)
        rid = lax.broadcasted_iota(i32, qp.shape, 0)
        even = ((rid // (DH // 2)) % 2) == 0
        qs_u[s * NG + g, 0:nr, cols] = jnp.where(even, qrot, qp)
        pq_u[s * NG + g, 0:nr, cols] = _pack(_phi(_round_bf16(q)))

    def k_task(s, p, stage, g):
        nr = _rows(g)
        cols = slice(p * LNW, (p + 1) * LNW)
        w = _bf(wt_u[WT_K + g * TW:WT_K + g * TW + nr // 2, :])
        k = jnp.dot(w, load_xs(s, p, stage), preferred_element_type=f32)
        pace[0] = _zero_after(k)
        if g == 0:
            r_buf[s, :, cols] = jnp.broadcast_to(k[_valid(0):_valid(0) + 1, :], (8, LNW))
        kp = _pack(k)
        pk_u[s * NG + g, 0:nr // 2, cols] = _pack(_phi(_round_bf16(k)))
        kfull = _bf(jnp.concatenate([kp, jnp.zeros(((T - nr) // 2, LNW), u32)], axis=0))
        k_u[s * NG + g, p * (LNW // 2):(p + 1) * (LNW // 2), :] = pltpu.bitcast(kfull.T, u32)

    def v_task(s, p, stage, b):
        cols = slice(p * LNW, (p + 1) * LNW)
        w = _bf(wt_u[WT_V + b * (VB // 2):WT_V + (b + 1) * (VB // 2), :])
        v = jnp.dot(w, load_xs(s, p, stage), preferred_element_type=f32)
        pace[0] = _zero_after(v)
        v = _pack(v)
        vt_u[s, b * (VB // 2):(b + 1) * (VB // 2), cols] = v
        sub = lax.broadcasted_iota(i32, (16, LNW), 0)
        for hh in range(8):
            w8 = (9 * hh) // 8
            ones_row = 0 if 2 * hh == 14 else 15
            vwin[s * H + 8 * b + hh, :, cols] = jnp.where(sub == ones_row, u32(ONES_PAIR), v[8 * w8:8 * w8 + 16, :])

    def q_tasks(s, p, stage=None):
        return [lambda g=g: q_task(s, p, stage, g) for g in range(NG)]

    def k_tasks(s, p, stage=None):
        return [lambda g=g: k_task(s, p, stage, g) for g in range(NG)]

    def v_tasks(s, p, stage=None):
        return [lambda b=b: v_task(s, p, stage, b) for b in range(D // VB)]

    def mem_layout(g):
        es, eoff, _ = _ewin(g)
        nv = _valid(g)
        ne = -(-(eoff + nv) // 16) * 16
        ones_row = 0 if eoff >= 2 else eoff + nv
        nh = nv // DH
        den_row = 0 if eoff >= nh else ne
        return es, eoff, nv, ne, ones_row, den_row, max(ne, den_row + 16 * (den_row > 0))

    def mem_update(sp, g):
        es, eoff, nv, ne, ones_row, den_row, nr = mem_layout(g)
        win = vt_u[sp, es // 2:(es + ne) // 2, :]
        wid = lax.broadcasted_iota(i32, win.shape, 0)
        lhs = _bf(jnp.where(wid == ones_row // 2, u32(ONES_PAIR), win))
        upd = lax.dot_general(lhs, _bf(pk_u[sp * NG + g]), NT_DIMS, preferred_element_type=f32)
        mt = mt_acc[g, 0:ne, :] + upd
        mt_acc[g, 0:ne, :] = mt
        z = jnp.broadcast_to(mt[ones_row:ones_row + 1, :], (nr, T))
        if nr > ne:
            mt = jnp.concatenate([mt, jnp.zeros((nr - ne, T), f32)], axis=0)
        row = lax.broadcasted_iota(i32, (nr, T), 0)
        d_id = lax.broadcasted_iota(i32, (nr, T), 1)
        e_loc = row - eoff
        same_head = (e_loc >= 0) & (e_loc < nv) & (d_id < nv) & ((e_loc // DH) == (d_id // DH))
        den_hit = (row >= den_row) & (d_id < nv) & ((d_id // DH) == row - den_row)
        lm_f[g, 0:nr, :] = jnp.where(same_head, mt, jnp.where(den_hit, z, 0.0))

    def mem_retrieve(s, g):
        es, eoff, nv, ne, ones_row, den_row, nr = mem_layout(g)
        nd = jnp.dot(lm_f[g, 0:nr, :].astype(bf16), _bf(pq_u[s * NG + g]), preferred_element_type=f32)
        scale = jnp.broadcast_to(g16[g][:, 0:1], (8, L)) / (nd[den_row:den_row + 8, :] + 1e-6)
        r8 = lax.broadcasted_iota(i32, (8, L), 0)
        for b in range(ne // 8):
            lo, hi = 8 * b - eoff, 8 * b + 7 - eoff
            if hi < 0 or lo >= nv:
                continue
            j1, j2 = max(lo, 0) // DH, min(hi, nv - 1) // DH
            sc = jnp.broadcast_to(scale[j1:j1 + 1, :], (8, L))
            if j2 != j1:
                sc = jnp.where(r8 < DH * j2 - lo, sc, jnp.broadcast_to(scale[j2:j2 + 1, :], (8, L)))
            val = nd[8 * b:8 * b + 8, :] * sc
            dst = am.at[s, es + 8 * b:es + 8 * b + 8, :]
            if lo >= 0 and hi < nv:
                dst[...] = val
            else:
                pltpu.store(dst, val, mask=(r8 + lo >= 0) & (r8 + lo < nv))

    def run(tasks):
        for t in tasks:
            t()

    prep_q = prep_grouped(0, WT_Q)
    nblk = DP // T
    q0a = q_tasks(0, 0)
    with _scope("p1_wait_x0"):
        x_copy(0).wait()
    for i in range(2, len(X_PIECES)):
        x_copy(i).start()
    w_copy(3).start()
    for i in range(3):
        moe_copy(i).start()
    with _scope("p1_ln0a"):
        run(ln_tasks(0, 0, None))
        wq_first.wait()
    with _scope("p1_q0a_first"):
        run(prep_q[0:2] + prep_q[nblk:nblk + 2] + q0a[0:2])
        wq_rest.wait()
        x_copy(1).wait()
    with _scope("p1_q0a"):
        run(prep_q[2:nblk] + prep_q[nblk + 2:])
        run(_interleave(q0a[2:], ln_tasks(0, 1, None)))
        w_copy(1).wait()
        for cp in small_copies:
            cp.wait()
    k0 = k_tasks(0, 0) + k_tasks(0, 1)
    with _scope("p1_q0b"):
        run(_interleave(q_tasks(0, 1), prep_grouped(1, WT_K), [gate_tables]))
        run(k0[0:NG])
        w_copy(2).wait()
        x_copy(2).wait()
    with _scope("p1_k0v0"):
        run(_interleave(k0[NG:], prep_dense(2, wt_u, WT_V)))
        run(_interleave(v_tasks(0, 0) + v_tasks(0, 1), ln_tasks(1, 0, xs_a)))

    def seg_body(s, c):
        for ss in range(2, NSEG):
            @pl.when(s + 1 == ss)
            def _():
                x_copy(ss + 1).wait()
        nxt = jnp.minimum(s + 1, NSEG - 1)
        pace[0] = None
        with _scope("p1_seg"):
            updates = [lambda g=g: mem_update(s - 1, g) for g in range(NG)]
            retrieves = [lambda g=g: mem_retrieve(s, g) for g in range(NG)]
            first = _interleave(q_tasks(s, 0, xs_a), updates) + k_tasks(s, 0, xs_a) + v_tasks(s, 0, xs_a)
            run(_interleave(first, ln_tasks(s, 1, xs_b)))
            second = q_tasks(s, 1, xs_b) + _interleave(k_tasks(s, 1, xs_b) + v_tasks(s, 1, xs_b), retrieves)
            run(_interleave(second, ln_tasks(nxt, 0, xs_a)))
        return c

    lax.fori_loop(1, NSEG, seg_body, 0)

    bufs = ((s0, m0), (s1, m1))
    lane64 = lax.broadcasted_iota(i32, (TW, T), 1)
    lane1 = lax.broadcasted_iota(i32, (1, T), 1)
    lane8 = lax.broadcasted_iota(i32, (8, T), 1)

    def head_rows(qw, j):
        lo, hi = (DH // 2) * j, (DH // 2) * (j + 1)
        r0, r1 = (lo // 8) * 8, -(-hi // 8) * 8
        rid = lax.broadcasted_iota(i32, (r1 - r0, T), 0) + r0
        part = jnp.where((rid >= lo) & (rid < hi), qw[r0:r1], u32(0))
        pieces = [jnp.zeros((r0, T), u32)] * (r0 > 0) + [part] + [jnp.zeros((TW - r1, T), u32)] * (r1 < TW)
        return jnp.concatenate(pieces, axis=0)

    def stage_a(unit, u, qt):
        s, k = unit
        s_ref, m_ref = bufs[k % 2]
        pi = k * NP + u
        g = pi // (HPG // 2)
        j = 2 * (pi - (HPG // 2) * g)
        sg = s * NG + g
        n = T * (qt + 1)
        qw = qs_u[sg, :, qt * T:(qt + 1) * T]
        w_a = head_rows(qw, j)
        w_b = head_rows(qw, j + 1)
        w_ab = _bf(jnp.where(lane64 < HT, w_a, w_b))

        def colmax8(v):
            return jnp.max(v.reshape(v.shape[0] // 8, 8, T), axis=0)

        maxes = []
        for hd, w in enumerate((_bf(w_a), _bf(w_b))):
            m8 = None
            for c in range(qt):
                kc = _bf(k_u[sg, c * TW:(c + 1) * TW, :])
                sc = jnp.dot(kc, w, preferred_element_type=f32)
                s_ref[u, qt, hd * L + c * T:hd * L + (c + 1) * T, :] = sc
                m8 = colmax8(sc) if m8 is None else jnp.maximum(m8, colmax8(sc))
            kc = _bf(k_u[sg, qt * TW:qt * TW + TW // 2, :])
            sc = jnp.dot(kc, w, preferred_element_type=f32) + mb[1 - hd]
            s_ref[u, qt, hd * L + qt * T:hd * L + qt * T + HT, :] = sc
            m8 = colmax8(sc) if m8 is None else jnp.maximum(m8, colmax8(sc))
            maxes.append(m8)
        kc = _bf(k_u[sg, qt * TW + TW // 2:(qt + 1) * TW, :])
        sc = jnp.dot(kc, w_ab, preferred_element_type=f32) + mb[2]
        s_ref[u, qt, n - HT:n, :] = sc
        mab = colmax8(sc)
        m_a = jnp.where(lane8 < HT, jnp.maximum(maxes[0], mab), maxes[0])
        m_b = jnp.where(lane8 >= HT, jnp.maximum(maxes[1], mab), maxes[1])
        m_ref[u, qt, 0] = jnp.broadcast_to(jnp.max(m_a, axis=0, keepdims=True), (8, T))
        m_ref[u, qt, 1] = jnp.broadcast_to(jnp.max(m_b, axis=0, keepdims=True), (8, T))

    def stage_b(unit, u, qt):
        s, k = unit
        s_ref, m_ref = bufs[k % 2]
        pi = k * NP + u
        n = T * (qt + 1)
        m_a = m_ref[u, qt, 0][0:1]
        m_b = m_ref[u, qt, 1][0:1]
        p_ab = jnp.exp2(s_ref[u, qt, n - HT:n, :] - jnp.where(lane1 < HT, m_a, m_b))
        for hd, m in enumerate((m_a, m_b)):
            h = 2 * pi + hd
            p = jnp.exp2(s_ref[u, qt, hd * L:hd * L + n - HT, :] - m)
            keep = (lane64 < HT) if hd == 0 else (lane64 >= HT)
            p = jnp.concatenate([p, jnp.where(keep, p_ab, 0.0)], axis=0).astype(bf16)
            w0 = ((DH * h) // 16) * 16
            off = DH * h - w0
            o = jnp.dot(_bf(vwin[s * H + h, :, 0:n]), p, preferred_element_type=f32)
            den = o[0:1] if off == 14 else o[31:32]
            r0, r1 = (off // 8) * 8, -(-(off + DH) // 8) * 8
            o = o[r0:r1] * (omg[h][0:1] / den)
            if hd == 0:
                o = pltpu.roll(o, HT, 1)
            res = am[s, w0 + r0:w0 + r1, qt * T:(qt + 1) * T] + o
            rid = lax.broadcasted_iota(i32, (r1 - r0, T), 0) + r0
            pltpu.store(ots[qt].at[w0 + r0:w0 + r1, :], res, mask=(rid >= off) & (rid < off + DH))

    def a_tasks(unit):
        return [lambda u=u, qt=qt: stage_a(unit, u, qt) for u in range(NP) for qt in QT_ORDER]

    def b_tasks(unit):
        return [lambda u=u, qt=qt: stage_b(unit, u, qt) for u in range(NP) for qt in QT_ORDER]

    w_copy(3).wait()
    for i in range(3):
        moe_copy(i).wait()
    rr = jnp.concatenate([r_buf[s][0:1, :] for s in range(NSEG)], axis=0)
    rr = _round_bf16(rr)
    tok = lax.broadcasted_iota(i32, (NSEG, L), 0) * L + lax.broadcasted_iota(i32, (NSEG, L), 1)
    m1v = jnp.max(rr)
    i1 = jnp.min(jnp.where(rr == m1v, tok, SEQ))
    rr2 = jnp.where(tok == i1, -jnp.inf, rr)
    m2v = jnp.max(rr2)
    i2 = jnp.min(jnp.where(rr2 == m2v, tok, SEQ))
    i1 = jnp.clip(i1, 0, SEQ - 1)
    i2 = jnp.clip(i2, 0, SEQ - 1)

    row16 = lax.broadcasted_iota(i32, (16, T), 0)
    lane16 = lax.broadcasted_iota(i32, (16, T), 1)

    def token_rows(i, slot):
        onehot = jnp.where((row16 == slot) & (lane16 == i % T), 1.0, 0.0).astype(bf16)
        return lax.dot_general(onehot, _bf(xn_u[i // T]), NT_DIMS, preferred_element_type=f32)

    def select_task():
        xsel_buf[...] = _pack(token_rows(i1, 0) + token_rows(i2, 1))
        y_acc[...] = jnp.zeros(y_acc.shape, f32)

    def fcols(ft):
        return pl.ds(ft * T if isinstance(ft, int) else pl.multiple_of(ft * T, T), T)

    def moe_up_task(ft, k, which):
        xsel = _bf(xsel_buf[:, 0:D])
        w_ref = (wg_buf, wu_buf)[which]
        hid_buf[k, which] = jnp.dot(xsel, w_ref[:, fcols(ft)], preferred_element_type=f32)

    def moe_down_task(ft, k):
        gt = _round_bf16(hid_buf[k, 0])
        up = _round_bf16(hid_buf[k, 1])
        hid = (_round_bf16(gt * _sigmoid(gt)) * up).astype(bf16)
        y_acc[...] += lax.dot_general(hid, wd_buf[:, fcols(ft)], NT_DIMS, preferred_element_type=f32)

    def moe_tasks(ft0, count):
        tasks = []
        for k0 in range(0, count, FPB):
            ks = range(k0, min(k0 + FPB, count))
            tasks += [lambda k=k, w=w: moe_up_task(ft0 + k, k, w) for k in ks for w in range(2)]
            tasks += [lambda k=k: moe_down_task(ft0 + k, k) for k in ks]
        return tasks

    def moe_finish():
        y = _round_bf16(y_acc[...])
        rsel = jnp.where(lax.broadcasted_iota(i32, (16, 1), 0) == 0, m1v, m2v)
        y = _round_bf16(y * _round_bf16(_sigmoid(rsel)))
        y = jnp.concatenate([y, jnp.zeros((16, DP - D), f32)], axis=1)
        y = jnp.concatenate([jnp.zeros((HT, DP), f32), y, jnp.zeros((T - HT - 16, DP), f32)], axis=0)
        y_t = jnp.concatenate([y.T[0:D], jnp.zeros((D, T), f32)], axis=1)
        y_u = _pack(y_t)[:, 0:T]
        lane = lax.broadcasted_iota(i32, (D // 2, T), 1)
        wot_u[:, DP - T:DP] = jnp.where(lane < HT, wot_u[:, DP - T:DP], y_u)
        rid = lax.broadcasted_iota(i32, (8, T), 0)
        for tt in range(TPS):
            tok_l = lax.broadcasted_iota(i32, (8, T), 1) + (NSEG - 1) * L + tt * T
            ots[tt][D:D + 8, :] = jnp.where(((rid == 0) & (tok_l == i1)) | ((rid == 1) & (tok_l == i2)), 1.0, 0.0)

    dense = _interleave(a_tasks((0, 0)), prep_dense(3, wot_u, 0))
    with _scope("p15_mix"):
        cut = (2 * len(dense)) // 3
        run(dense[:cut] + [select_task] + dense[cut:])

    def out_tile(s, tt, last, chunk_copies=None):
        c0 = s * L + tt * T
        if not isinstance(s, int):
            c0 = pl.multiple_of(c0, T)
        o_bf = ots[tt][...].astype(bf16)
        nchunk = 4
        rows = D // nchunk
        for rc in range(nchunk):
            r0 = rc * rows
            attn = jnp.dot(_bf(wot_u[r0 // 2:(r0 + rows) // 2, :]), o_bf, preferred_element_type=f32)
            xn = _bf(xn_u[s * TPS + tt, r0 // 2:(r0 + rows) // 2, :]).astype(f32)
            x = x_buf[r0:r0 + rows, pl.ds(c0, T)].astype(f32)
            res = x + attn + xn
            out_buf[r0:r0 + rows, pl.ds(c0, T)] = res.astype(bf16)
            if chunk_copies is not None:
                chunk_copies[rc].start()

    def pair_tasks(ua, ub):
        tasks = []
        for x, y in zip(a_tasks(ua), b_tasks(ub)):
            tasks += [y, x]
        return tasks

    def seg_end(s, last):
        def by_qt(fn, unit, qt):
            return [lambda u=u: fn(unit, u, qt) for u in range(NP)]

        steps = []
        for step in range(7):
            lists = []
            if step < 4:
                lists.append(by_qt(stage_b, (s, 2), 3 - step))
                lists.append(by_qt(stage_a, (s, 3), 3 - step))
            if 1 <= step < 5:
                lists.append(by_qt(stage_b, (s, 3), 4 - step))
            if not last and 2 <= step < 6:
                lists.append(by_qt(stage_a, (s + 1, 0), 5 - step))
            if step >= 3:
                lists.append([lambda tt=6 - step: out_tile(s, tt, last)])
            steps.append(_interleave(*lists))
        return steps

    def seg_att(s, c):
        tasks = pair_tasks((s, 1), (s, 0)) + pair_tasks((s, 2), (s, 1))
        steps = seg_end(s, False)
        for step in steps[0:5]:
            tasks += step
        with _scope("att_seg"):
            run(_interleave(tasks, moe_tasks(s * FPI, FPI)))
            for step in steps[5:]:
                run(step)
        out_copy(pl.multiple_of(s * L, L), L, s).start()
        return c

    lax.fori_loop(0, NSEG - 1, seg_att, 0)

    npatch = (NSEG - 1) * TPS

    def patch_tile(idx):
        return jnp.where(idx < npatch * T, idx // T, 0)

    tile0 = patch_tile(i1)
    tile1 = patch_tile(i2)
    tile1 = jnp.where(tile1 == tile0, (tile0 + 1) % npatch, tile1)

    def patch(tile):
        c0 = pl.multiple_of(tile * T, T)
        rid = lax.broadcasted_iota(i32, (T, T), 0)
        tok_l = lax.broadcasted_iota(i32, (T, T), 1) + c0
        hit = ((rid == HT) & (tok_l == i1)) | ((rid == HT + 1) & (tok_l == i2))
        onehot = jnp.where(hit, 1.0, 0.0).astype(bf16)
        for rc in range(4):
            r0, r1 = rc * (D // 4), (rc + 1) * (D // 4)
            upd = jnp.dot(_bf(wot_u[r0 // 2:r1 // 2, DP - T:DP]), onehot, preferred_element_type=f32)
            cur = out_buf[r0:r1, pl.ds(c0, T)].astype(f32)
            out_buf[r0:r1, pl.ds(c0, T)] = (cur + upd).astype(bf16)

    patch_copies = [out_copy(pl.multiple_of(tile0 * T, T), T, 7), out_copy(pl.multiple_of(tile1 * T, T), T, 8)]
    last_copies = [out_copy((NSEG - 1) * L + tt * T, T, NSEG - 1 + tt) for tt in range(1, TPS)]
    c_fin = (NSEG - 1) * L
    final_copies = [
        pltpu.make_async_copy(out_buf.at[rc * (D // 4):(rc + 1) * (D // 4), c_fin:c_fin + T],
                              out_hbm.at[rc * (D // 4):(rc + 1) * (D // 4), c_fin:c_fin + T],
                              sems.at[SEM_FINAL + rc]) for rc in range(4)]

    sl = NSEG - 1
    with _scope("tail_1"):
        moe_finish()
        run(pair_tasks((sl, 1), (sl, 0)))
        for s in range(NSEG - 1):
            out_copy(s * L, L, s).wait()
    with _scope("tail_2"):
        patch(tile0)
        patch(tile1)
        run(pair_tasks((sl, 2), (sl, 1)))
        for cp in patch_copies:
            cp.start()
        steps = seg_end(sl, True)
        for step in steps[0:5]:
            run(step)
        last_copies[2].start()
        last_copies[1].start()
    with _scope("tail_3"):
        run(steps[5])
        last_copies[0].start()
        out_tile(sl, 0, True, final_copies)

    with _scope("out_wait"):
        for cp in patch_copies + last_copies + final_copies:
            cp.wait()


@jax.jit
def pallas_parallel_sum__memory_aug_infini_attn__moe_arch_mod__prompt_kernel(
    A_x: jax.Array,
    A_wq: jax.Array,
    A_wk: jax.Array,
    A_wv: jax.Array,
    A_wo: jax.Array,
    A_beta: jax.Array,
    B_x: jax.Array,
    B_w_r: jax.Array,
    B_w_gate: jax.Array,
    B_w_up: jax.Array,
    B_w_down: jax.Array,
):
    del B_x
    any_spec = pl.BlockSpec(memory_space=pl.ANY)
    scratch = [
        pltpu.VMEM((H,), bf16),
        pltpu.VMEM((D,), bf16),
        pltpu.VMEM((D, SEQ), bf16),
        pltpu.VMEM((4, D, D), bf16),
        pltpu.VMEM((D, F), bf16),
        pltpu.VMEM((D, F), bf16),
        pltpu.VMEM((D, F), bf16),
        pltpu.VMEM((D, SEQ), bf16),
        pltpu.VMEM((WT_ROWS, DP), u32),
        pltpu.VMEM((D // 2, DP), u32),
        pltpu.VMEM((D // 2, DP), u32),
        pltpu.VMEM((NT, DP // 2, T), u32),
        pltpu.VMEM((BT, DP // 2, T), u32),
        pltpu.VMEM((BT, DP // 2, T), u32),
        pltpu.VMEM((NSEG * NG, TW, L), u32),
        pltpu.VMEM((NSEG * NG, L // 2, T), u32),
        pltpu.VMEM((NSEG * NG, TW, L), u32),
        pltpu.VMEM((NSEG * NG, TW, L), u32),
        pltpu.VMEM((NSEG, D // 2, L), u32),
        pltpu.VMEM((NSEG * H, 16, L), u32),
        pltpu.VMEM((NSEG, 8, L), f32),
        pltpu.VMEM((NG, T, T), f32),
        pltpu.VMEM((NG, T, T), f32),
        pltpu.VMEM((NSEG, D, L), f32),
        pltpu.VMEM((NG, 8, T), f32),
        pltpu.VMEM((H, 8, T), f32),
        pltpu.VMEM((3, HT, T), f32),
        pltpu.VMEM((NP, 4, 2 * L, T), f32),
        pltpu.VMEM((NP, 4, 2, 8, T), f32),
        pltpu.VMEM((NP, 4, 2 * L, T), f32),
        pltpu.VMEM((NP, 4, 2, 8, T), f32),
        pltpu.VMEM((DP, T), f32),
        pltpu.VMEM((DP, T), f32),
        pltpu.VMEM((DP, T), f32),
        pltpu.VMEM((DP, T), f32),
        pltpu.VMEM((2, D, LNW), f32),
        pltpu.VMEM((2, 2, 8, LNW), f32),
        pltpu.VMEM((16, D), f32),
        pltpu.VMEM((8, DP), u32),
        pltpu.VMEM((FPI, 2, 16, T), f32),
        pltpu.SemaphoreType.DMA((NSEM,)),
    ]
    x_t = jnp.transpose(A_x, (0, 2, 1)).reshape(D, SEQ)
    out_t = pl.pallas_call(
        _kernel,
        out_shape=jax.ShapeDtypeStruct((D, SEQ), bf16),
        in_specs=[any_spec] * 10,
        out_specs=any_spec,
        scratch_shapes=scratch,
        compiler_params=pltpu.CompilerParams(vmem_limit_bytes=110 * 1024 * 1024),
    )(x_t, A_wq, A_wk, A_wv, A_wo, A_beta, B_w_r, B_w_gate, B_w_up, B_w_down.T)
    return jnp.transpose(out_t.reshape(1, D, SEQ), (0, 2, 1))
```

```python
import contextlib

import jax
import jax.numpy as jnp
from jax import lax
from jax.experimental import pallas as pl
from jax.experimental.pallas import tpu as pltpu

bf16 = jnp.bfloat16
f32 = jnp.float32
u32 = jnp.uint32
i32 = jnp.int32

SEQ = 2048
D = 576
DP = 640
H = 32
DH = 18
NSEG = 4
L = 512
T = 128
TW = T // 2
HT = T // 2
TPS = L // T
HPG = 6
NG = 6
F = 4608
FPI = 12
FPB = 3
NFT = F // T
NP = 4
UPS = H // (2 * NP)
NUNIT = NSEG * UPS
NT = SEQ // T
LNW = 256
BT = LNW // T
NORM_PARTS = 6
VB = 8 * DH

LOG2E = 1.4426950408889634
QSCALE = (DH ** -0.5) * LOG2E
MASKVAL = -1000000000.0 * LOG2E
EPS_BF16 = 1.0013580322265625e-05
ONES_PAIR = 0x3F803F80

NT_DIMS = (((1,), (1,)), ((), ()))

WT_Q = 0
WT_K = NG * TW
WT_V = 2 * NG * TW
WT_ROWS = WT_V + D // 2

X_PIECES = ((0, LNW), (LNW, LNW), (L, L), (2 * L, L), (3 * L, L))
SEM_X = 0
SEM_W = 5
SEM_MOE = 9
SEM_OUT = 12
SEM_SMALL = 21
SEM_WQB = 23
SEM_FINAL = 24
NSEM = 28
WQ_SPLIT = 2 * T


PROFILE_SCOPES = False
PACE = True
TAIL_BARRIERS = False
QT_ORDER = (3, 2, 1, 0)


def _scope(name):
    return jax.named_scope(name) if PROFILE_SCOPES else contextlib.nullcontext()


def _valid(g):
    return min(HPG * DH, D - g * HPG * DH)


def _rows(g):
    return -(-_valid(g) // 16) * 16


def _ewin(g):
    start = (g * HPG * DH // 16) * 16
    return start, g * HPG * DH - start, min(T, D - start)


def _bf(x):
    return pltpu.bitcast(x, bf16)


def _pack(x):
    return pltpu.bitcast(x.astype(bf16), u32)


def _round_bf16(x):
    return x.astype(bf16).astype(f32)


def _phi(t):
    return jnp.where(t > 0, t + 1.0, jnp.exp(t))


def _sigmoid(t):
    return 1.0 / (1.0 + jnp.exp(-t))


def _zero_after(v):
    bits = pltpu.bitcast(v[0:8, 0:LNW], u32)
    sixteen = jnp.uint32(16)
    bits = lax.shift_right_logical(lax.shift_right_logical(bits, sixteen), sixteen)
    return pltpu.bitcast(bits, f32) if PACE else None


def _interleave(*lists):
    items = []
    for li, tasks in enumerate(lists):
        for k, t in enumerate(tasks):
            items.append(((k + 0.5) / len(tasks), li, k, t))
    items.sort(key=lambda it: it[:3])
    return [it[3] for it in items]


def _kernel(x_hbm, wq_hbm, wk_hbm, wv_hbm, wo_hbm, beta_hbm, wr_hbm, wg_hbm, wu_hbm, wd_hbm,
            out_hbm,
            beta_ref, wr_ref, x_buf, w_buf, wg_buf, wu_buf, wd_buf, out_buf,
            wt_u, wtd_u, wot_u, xn_u, xs_a, xs_b, qs_u, k_u, pq_u, pk_u, vt_u, vwin,
            r_buf, mt_acc, lm_f, am, g16, omg, mb,
            s0, m0, s1, m1, ot0, ot1, ot2, ot3, xf, ln_stat, y_acc, xsel_buf, hid_buf, sems):

    def x_copy(i):
        c0, width = X_PIECES[i]
        return pltpu.make_async_copy(x_hbm.at[:, pl.ds(c0, width)], x_buf.at[:, pl.ds(c0, width)],
                                     sems.at[SEM_X + i])

    def w_copy(i):
        src = (wq_hbm, wk_hbm, wv_hbm, wo_hbm)[i]
        return pltpu.make_async_copy(src, w_buf.at[i], sems.at[SEM_W + i])

    wq_first = pltpu.make_async_copy(wq_hbm.at[:, 0:WQ_SPLIT], w_buf.at[0, :, 0:WQ_SPLIT], sems.at[SEM_W])
    wq_rest = pltpu.make_async_copy(wq_hbm.at[:, WQ_SPLIT:D], w_buf.at[0, :, WQ_SPLIT:D], sems.at[SEM_WQB])

    def moe_copy(i):
        src = (wg_hbm, wu_hbm, wd_hbm)[i]
        dst = (wg_buf, wu_buf, wd_buf)[i]
        return pltpu.make_async_copy(src, dst, sems.at[SEM_MOE + i])

    def out_copy(c0, width, sem):
        return pltpu.make_async_copy(out_buf.at[:, pl.ds(c0, width)], out_hbm.at[:, pl.ds(c0, width)],
                                     sems.at[SEM_OUT + sem])

    small_copies = [pltpu.make_async_copy(beta_hbm, beta_ref, sems.at[SEM_SMALL]),
                    pltpu.make_async_copy(wr_hbm, wr_ref, sems.at[SEM_SMALL + 1])]
    x_copy(0).start()
    wq_first.start()
    wq_rest.start()
    x_copy(1).start()
    for cp in small_copies:
        cp.start()
    w_copy(1).start()
    w_copy(2).start()

    init_scope = _scope("init")
    init_scope.__enter__()
    kr = lax.broadcasted_iota(i32, (HT, T), 0)
    ql = lax.broadcasted_iota(i32, (HT, T), 1)
    mb[0] = jnp.where(ql < kr, MASKVAL, 0.0).astype(f32)
    mb[1] = jnp.where((ql >= HT) & (ql - HT < kr), MASKVAL, 0.0).astype(f32)
    mb[2] = jnp.where(ql % HT < kr, MASKVAL, 0.0).astype(f32)
    zpad = jnp.zeros(((DP - D) // 2, T), u32)
    for tt in range(NT):
        xn_u[tt, D // 2:DP // 2, :] = zpad
    for tt in range(BT):
        xs_a[tt, D // 2:DP // 2, :] = zpad
        xs_b[tt, D // 2:DP // 2, :] = zpad
    ots = (ot0, ot1, ot2, ot3)
    for o_ref in ots:
        o_ref[D:DP, :] = jnp.zeros((DP - D, T), f32)
    am[0] = jnp.zeros(am.shape[1:], f32)
    mt_acc[...] = jnp.zeros(mt_acc.shape, f32)
    g16[...] = jnp.zeros(g16.shape, f32)
    for sg in range(NSEG * NG):
        r2 = _rows(sg % NG) // 2
        qs_u[sg, r2:TW, :] = jnp.zeros((TW - r2, L), u32)
        pq_u[sg, r2:TW, :] = jnp.zeros((TW - r2, L), u32)
        pk_u[sg, r2:TW, :] = jnp.zeros((TW - r2, L), u32)

    init_scope.__exit__(None, None, None)

    pace = [None]

    def gate_tables():
        gate = _round_bf16(_sigmoid(beta_ref[...].reshape(1, H).astype(f32)))
        for h in range(H):
            gh = jnp.broadcast_to(gate[:, h:h + 1], (1, T))
            omg[h] = jnp.broadcast_to(_round_bf16(1.0 - gh), (8, T))
            g16[h // HPG, (h % HPG):(h % HPG) + 1, :] = gh

    def transpose_block(i, cb):
        c1 = min((cb + 1) * T, D)
        blk = w_buf[i, :, cb * T:c1]
        if c1 - cb * T < T:
            blk = jnp.concatenate([blk, jnp.zeros((D, T - (c1 - cb * T)), bf16)], axis=1)
        blk = jnp.concatenate([blk, jnp.zeros((DP - D, T), bf16)], axis=0)
        return pltpu.bitcast(blk.T, u32)

    def prep_dense(i, dst, base):
        def task(cb):
            nrow = min(TW, D // 2 - cb * TW)
            dst[base + cb * TW:base + cb * TW + nrow, :] = transpose_block(i, cb)[0:nrow]
        return [lambda cb=cb: task(cb) for cb in range(DP // T)]

    def prep_grouped(i, base):
        def regroup(g):
            nv, nr = _valid(g) // 2, _rows(g) // 2
            src = g * HPG * DH // 2
            wt_u[base + g * TW:base + g * TW + nv, :] = wtd_u[src:src + nv, :]
            pad = jnp.zeros((nr - nv, DP), u32)
            if i == 1 and g == 0:
                wr = wr_ref[...].reshape(1, D).astype(f32)
                wr = jnp.concatenate([wr, jnp.zeros((1, DP - D), f32)], axis=1)
                bits = lax.shift_right_logical(pltpu.bitcast(wr, u32), u32(16))
                rid = lax.broadcasted_iota(i32, (nr - nv, DP), 0)
                pad = jnp.where(rid == 0, bits, pad)
            wt_u[base + g * TW + nv:base + g * TW + nr, :] = pad
        return prep_dense(i, wtd_u, 0) + [lambda g=g: regroup(g) for g in range(NG)]

    def ln_tasks(s, p, stage):
        c0 = s * L + p * LNW
        if not isinstance(s, int):
            c0 = pl.multiple_of(c0, LNW)

        def mean_pass():
            acc = pace[0]
            for r in range(0, D, 64):
                x = x_buf[r:r + 64, pl.ds(c0, LNW)].astype(f32)
                xf[p, r:r + 64, :] = x
                part = jnp.sum(x.reshape(8, 8, LNW), axis=0)
                acc = part if acc is None else acc + part
            mean = jnp.sum(acc, axis=0, keepdims=True) / D
            ln_stat[p, 0] = jnp.broadcast_to(mean, (8, LNW))

        def var_pass():
            mean = ln_stat[p, 0][0:1]
            if pace[0] is not None:
                mean = mean + pace[0][0:1]
            acc = None
            for r in range(0, D, 96):
                xc = xf[p, r:r + 96, :] - mean
                part = jnp.sum((xc * xc).reshape(12, 8, LNW), axis=0)
                acc = part if acc is None else acc + part
            var = jnp.sum(acc, axis=0, keepdims=True) / D
            den = _round_bf16(jnp.sqrt(_round_bf16(_round_bf16(var) + EPS_BF16)))
            ln_stat[p, 1] = jnp.broadcast_to(1.0 / den, (8, LNW))
            ln_stat[p, 0] = jnp.broadcast_to(_round_bf16(mean), (8, LNW))

        def norm_pass(part):
            mean_b = ln_stat[p, 0][0:1]
            if pace[0] is not None:
                mean_b = mean_b + pace[0][0:1]
            inv = ln_stat[p, 1][0:1]
            step = D // NORM_PARTS
            for r in range(part * step, (part + 1) * step, 48):
                xn = _pack(_round_bf16(xf[p, r:r + 48, :] - mean_b) * inv)
                for t in range(BT):
                    xn_u.at[s * TPS + p * BT + t][r // 2:r // 2 + 24, :] = xn[:, t * T:(t + 1) * T]
                    if stage is not None:
                        stage.at[t][r // 2:r // 2 + 24, :] = xn[:, t * T:(t + 1) * T]

        return [mean_pass, var_pass] + [lambda part=part: norm_pass(part) for part in range(NORM_PARTS)]

    def load_xs(s, p, stage):
        if stage is None:
            tiles = [xn_u[s * TPS + p * BT + t] for t in range(BT)]
        else:
            tiles = [stage[t] for t in range(BT)]
        return jnp.concatenate([_bf(t) for t in tiles], axis=1)

    def q_task(s, p, stage, g):
        nr = _rows(g) // 2
        cols = slice(p * LNW, (p + 1) * LNW)
        w = _bf(wt_u[WT_Q + g * TW:WT_Q + g * TW + nr, :])
        q = jnp.dot(w, load_xs(s, p, stage), preferred_element_type=f32)
        pace[0] = _zero_after(q)
        qp = _pack(q * QSCALE)
        qrot = jnp.concatenate([pltpu.roll(qp[:, t * T:(t + 1) * T], HT, 1) for t in range(BT)], axis=1)
        rid = lax.broadcasted_iota(i32, qp.shape, 0)
        even = ((rid // (DH // 2)) % 2) == 0
        qs_u.at[s * NG + g][0:nr, cols] = jnp.where(even, qrot, qp)
        pq_u.at[s * NG + g][0:nr, cols] = _pack(_phi(q))

    def k_task(s, p, stage, g):
        nr = _rows(g)
        cols = slice(p * LNW, (p + 1) * LNW)
        w = _bf(wt_u[WT_K + g * TW:WT_K + g * TW + nr // 2, :])
        k = jnp.dot(w, load_xs(s, p, stage), preferred_element_type=f32)
        pace[0] = _zero_after(k)
        if g == 0:
            r_buf[s, :, cols] = jnp.broadcast_to(k[_valid(0):_valid(0) + 1, :], (8, LNW))
        kp = _pack(k)
        pk_u.at[s * NG + g][0:nr // 2, cols] = _pack(_phi(k))
        kfull = _bf(jnp.concatenate([kp, jnp.zeros(((T - nr) // 2, LNW), u32)], axis=0))
        k_u.at[s * NG + g][p * (LNW // 2):(p + 1) * (LNW // 2), :] = pltpu.bitcast(kfull.T, u32)

    def v_task(s, p, stage, b):
        cols = slice(p * LNW, (p + 1) * LNW)
        w = _bf(wt_u[WT_V + b * (VB // 2):WT_V + (b + 1) * (VB // 2), :])
        v = jnp.dot(w, load_xs(s, p, stage), preferred_element_type=f32)
        pace[0] = _zero_after(v)
        v = _pack(v)
        vt_u.at[s][b * (VB // 2):(b + 1) * (VB // 2), cols] = v
        sub = lax.broadcasted_iota(i32, (16, LNW), 0)
        for hh in range(8):
            w8 = (9 * hh) // 8
            ones_row = 0 if 2 * hh == 14 else 15
            vwin.at[s * H + 8 * b + hh][:, cols] = jnp.where(sub == ones_row, u32(ONES_PAIR), v[8 * w8:8 * w8 + 16, :])

    def q_tasks(s, p, stage=None):
        return [lambda g=g: q_task(s, p, stage, g) for g in range(NG)]

    def k_tasks(s, p, stage=None):
        return [lambda g=g: k_task(s, p, stage, g) for g in range(NG)]

    def v_tasks(s, p, stage=None):
        return [lambda b=b: v_task(s, p, stage, b) for b in range(D // VB)]

    def mem_layout(g):
        es, eoff, _ = _ewin(g)
        nv = _valid(g)
        ne = -(-(eoff + nv) // 16) * 16
        ones_row = 0 if eoff >= 2 else eoff + nv
        nh = nv // DH
        den_row = 0 if eoff >= nh else ne
        return es, eoff, nv, ne, ones_row, den_row, max(ne, den_row + 16 * (den_row > 0))

    def mem_update(sp, g):
        es, eoff, nv, ne, ones_row, den_row, nr = mem_layout(g)
        win = vt_u[sp, es // 2:(es + ne) // 2, :]
        wid = lax.broadcasted_iota(i32, win.shape, 0)
        lhs = _bf(jnp.where(wid == ones_row // 2, u32(ONES_PAIR), win))
        upd = lax.dot_general(lhs, _bf(pk_u[sp * NG + g]), NT_DIMS, preferred_element_type=f32)
        mt = mt_acc[g, 0:ne, :] + upd
        mt_acc[g, 0:ne, :] = mt
        z = jnp.broadcast_to(mt[ones_row:ones_row + 1, :], (nr, T))
        if nr > ne:
            mt = jnp.concatenate([mt, jnp.zeros((nr - ne, T), f32)], axis=0)
        row = lax.broadcasted_iota(i32, (nr, T), 0)
        d_id = lax.broadcasted_iota(i32, (nr, T), 1)
        e_loc = row - eoff
        same_head = (e_loc >= 0) & (e_loc < nv) & (d_id < nv) & ((e_loc // DH) == (d_id // DH))
        den_hit = (row >= den_row) & (d_id < nv) & ((d_id // DH) == row - den_row)
        lm_f[g, 0:nr, :] = jnp.where(same_head, mt, jnp.where(den_hit, z, 0.0))

    def mem_retrieve(s, g):
        es, eoff, nv, ne, ones_row, den_row, nr = mem_layout(g)
        nd = jnp.dot(lm_f[g, 0:nr, :].astype(bf16), _bf(pq_u[s * NG + g]), preferred_element_type=f32)
        scale = jnp.broadcast_to(g16[g][:, 0:1], (8, L)) / (nd[den_row:den_row + 8, :] + 1e-6)
        r8 = lax.broadcasted_iota(i32, (8, L), 0)
        for b in range(ne // 8):
            lo, hi = 8 * b - eoff, 8 * b + 7 - eoff
            if hi < 0 or lo >= nv:
                continue
            j1, j2 = max(lo, 0) // DH, min(hi, nv - 1) // DH
            sc = jnp.broadcast_to(scale[j1:j1 + 1, :], (8, L))
            if j2 != j1:
                sc = jnp.where(r8 < DH * j2 - lo, sc, jnp.broadcast_to(scale[j2:j2 + 1, :], (8, L)))
            val = nd[8 * b:8 * b + 8, :] * sc
            dst = am.at[s, es + 8 * b:es + 8 * b + 8, :]
            if lo >= 0 and hi < nv:
                dst[...] = val
            else:
                pltpu.store(dst, val, mask=(r8 + lo >= 0) & (r8 + lo < nv))

    def run(tasks):
        for t in tasks:
            t()

    prep_q = prep_grouped(0, WT_Q)
    nblk = DP // T
    q0a = q_tasks(0, 0)
    with _scope("p1_wait_x0"):
        x_copy(0).wait()
    for i in range(2, len(X_PIECES)):
        x_copy(i).start()
    w_copy(3).start()
    for i in range(3):
        moe_copy(i).start()
    with _scope("p1_ln0a"):
        run(ln_tasks(0, 0, None))
        wq_first.wait()
    with _scope("p1_q0a_first"):
        run(prep_q[0:2] + prep_q[nblk:nblk + 2] + q0a[0:2])
        wq_rest.wait()
        x_copy(1).wait()
    with _scope("p1_q0a"):
        run(prep_q[2:nblk] + prep_q[nblk + 2:])
        run(_interleave(q0a[2:], ln_tasks(0, 1, None)))
        w_copy(1).wait()
        for cp in small_copies:
            cp.wait()
    k0 = k_tasks(0, 0) + k_tasks(0, 1)
    with _scope("p1_q0b"):
        run(_interleave(q_tasks(0, 1), prep_grouped(1, WT_K), [gate_tables]))
        run(k0[0:NG])
        w_copy(2).wait()
        x_copy(2).wait()
    with _scope("p1_k0v0"):
        run(_interleave(k0[NG:], prep_dense(2, wt_u, WT_V)))
        run(_interleave(v_tasks(0, 0) + v_tasks(0, 1), ln_tasks(1, 0, xs_a)))

    def seg_body(s, c):
        for ss in range(2, NSEG):
            @pl.when(s + 1 == ss)
            def _():
                x_copy(ss + 1).wait()
        nxt = jnp.minimum(s + 1, NSEG - 1)
        pace[0] = None
        with _scope("p1_seg"):
            updates = [lambda g=g: mem_update(s - 1, g) for g in range(NG)]
            retrieves = [lambda g=g: mem_retrieve(s, g) for g in range(NG)]
            first = _interleave(q_tasks(s, 0, xs_a), updates) + k_tasks(s, 0, xs_a) + v_tasks(s, 0, xs_a)
            run(_interleave(first, ln_tasks(s, 1, xs_b)))
            second = q_tasks(s, 1, xs_b) + _interleave(k_tasks(s, 1, xs_b) + v_tasks(s, 1, xs_b), retrieves)
            run(_interleave(second, ln_tasks(nxt, 0, xs_a)))
        return c

    lax.fori_loop(1, NSEG, seg_body, 0)

    bufs = ((s0, m0), (s1, m1))
    lane64 = lax.broadcasted_iota(i32, (TW, T), 1)
    lane1 = lax.broadcasted_iota(i32, (1, T), 1)
    lane8 = lax.broadcasted_iota(i32, (8, T), 1)

    def head_rows(qw, j):
        lo, hi = (DH // 2) * j, (DH // 2) * (j + 1)
        r0, r1 = (lo // 8) * 8, -(-hi // 8) * 8
        rid = lax.broadcasted_iota(i32, (r1 - r0, T), 0) + r0
        part = jnp.where((rid >= lo) & (rid < hi), qw[r0:r1], u32(0))
        pieces = [jnp.zeros((r0, T), u32)] * (r0 > 0) + [part] + [jnp.zeros((TW - r1, T), u32)] * (r1 < TW)
        return jnp.concatenate(pieces, axis=0)

    def stage_a(unit, u, qt):
        s, k = unit
        s_ref, m_ref = bufs[k % 2]
        pi = k * NP + u
        g = pi // (HPG // 2)
        j = 2 * (pi - (HPG // 2) * g)
        sg = s * NG + g
        n = T * (qt + 1)
        qw = qs_u[sg, :, qt * T:(qt + 1) * T]
        w_a = head_rows(qw, j)
        w_b = head_rows(qw, j + 1)
        w_ab = _bf(jnp.where(lane64 < HT, w_a, w_b))

        def colmax8(v):
            return jnp.max(v.reshape(v.shape[0] // 8, 8, T), axis=0)

        maxes = []
        for hd, w in enumerate((_bf(w_a), _bf(w_b))):
            m8 = None
            for c in range(qt):
                kc = _bf(k_u[sg, c * TW:(c + 1) * TW, :])
                sc = jnp.dot(kc, w, preferred_element_type=f32)
                s_ref[u, qt, hd * L + c * T:hd * L + (c + 1) * T, :] = sc
                m8 = colmax8(sc) if m8 is None else jnp.maximum(m8, colmax8(sc))
            kc = _bf(k_u[sg, qt * TW:qt * TW + TW // 2, :])
            sc = jnp.dot(kc, w, preferred_element_type=f32) + mb[1 - hd]
            s_ref[u, qt, hd * L + qt * T:hd * L + qt * T + HT, :] = sc
            m8 = colmax8(sc) if m8 is None else jnp.maximum(m8, colmax8(sc))
            maxes.append(m8)
        kc = _bf(k_u[sg, qt * TW + TW // 2:(qt + 1) * TW, :])
        sc = jnp.dot(kc, w_ab, preferred_element_type=f32) + mb[2]
        s_ref[u, qt, n - HT:n, :] = sc
        mab = colmax8(sc)
        m_a = jnp.where(lane8 < HT, jnp.maximum(maxes[0], mab), maxes[0])
        m_b = jnp.where(lane8 >= HT, jnp.maximum(maxes[1], mab), maxes[1])
        m_ref[u, qt, 0] = jnp.broadcast_to(jnp.max(m_a, axis=0, keepdims=True), (8, T))
        m_ref[u, qt, 1] = jnp.broadcast_to(jnp.max(m_b, axis=0, keepdims=True), (8, T))

    def stage_b(unit, u, qt):
        s, k = unit
        s_ref, m_ref = bufs[k % 2]
        pi = k * NP + u
        n = T * (qt + 1)
        m_a = m_ref[u, qt, 0][0:1]
        m_b = m_ref[u, qt, 1][0:1]
        p_ab = jnp.exp2(s_ref[u, qt, n - HT:n, :] - jnp.where(lane1 < HT, m_a, m_b))
        for hd, m in enumerate((m_a, m_b)):
            h = 2 * pi + hd
            p = jnp.exp2(s_ref[u, qt, hd * L:hd * L + n - HT, :] - m)
            keep = (lane64 < HT) if hd == 0 else (lane64 >= HT)
            p = jnp.concatenate([p, jnp.where(keep, p_ab, 0.0)], axis=0).astype(bf16)
            w0 = ((DH * h) // 16) * 16
            off = DH * h - w0
            o = jnp.dot(_bf(vwin[s * H + h, :, 0:n]), p, preferred_element_type=f32)
            den = o[0:1] if off == 14 else o[31:32]
            r0, r1 = (off // 8) * 8, -(-(off + DH) // 8) * 8
            o = o[r0:r1] * (omg[h][0:1] / den)
            if hd == 0:
                o = pltpu.roll(o, HT, 1)
            res = am[s, w0 + r0:w0 + r1, qt * T:(qt + 1) * T] + o
            rid = lax.broadcasted_iota(i32, (r1 - r0, T), 0) + r0
            pltpu.store(ots[qt].at[w0 + r0:w0 + r1, :], res, mask=(rid >= off) & (rid < off + DH))

    def a_tasks(unit):
        return [lambda u=u, qt=qt: stage_a(unit, u, qt) for u in range(NP) for qt in QT_ORDER]

    def b_tasks(unit):
        return [lambda u=u, qt=qt: stage_b(unit, u, qt) for u in range(NP) for qt in QT_ORDER]

    w_copy(3).wait()
    for i in range(3):
        moe_copy(i).wait()
    rr = jnp.concatenate([r_buf[s][0:1, :] for s in range(NSEG)], axis=0)
    rr = _round_bf16(rr)
    tok = lax.broadcasted_iota(i32, (NSEG, L), 0) * L + lax.broadcasted_iota(i32, (NSEG, L), 1)
    m1v = jnp.max(rr)
    i1 = jnp.min(jnp.where(rr == m1v, tok, SEQ))
    rr2 = jnp.where(tok == i1, -jnp.inf, rr)
    m2v = jnp.max(rr2)
    i2 = jnp.min(jnp.where(rr2 == m2v, tok, SEQ))
    i1 = jnp.clip(i1, 0, SEQ - 1)
    i2 = jnp.clip(i2, 0, SEQ - 1)

    row16 = lax.broadcasted_iota(i32, (16, T), 0)
    lane16 = lax.broadcasted_iota(i32, (16, T), 1)

    def token_rows(i, slot):
        onehot = jnp.where((row16 == slot) & (lane16 == i % T), 1.0, 0.0).astype(bf16)
        return lax.dot_general(onehot, _bf(xn_u[i // T]), NT_DIMS, preferred_element_type=f32)

    def select_task():
        xsel_buf[...] = _pack(token_rows(i1, 0) + token_rows(i2, 1))
        y_acc[...] = jnp.zeros(y_acc.shape, f32)

    def fcols(ft):
        return pl.ds(ft * T if isinstance(ft, int) else pl.multiple_of(ft * T, T), T)

    def moe_up_task(ft, k, which):
        xsel = _bf(xsel_buf[:, 0:D])
        w_ref = (wg_buf, wu_buf)[which]
        hid_buf[k, which] = jnp.dot(xsel, w_ref[:, fcols(ft)], preferred_element_type=f32)

    def moe_down_task(ft, k):
        gt = _round_bf16(hid_buf[k, 0])
        up = _round_bf16(hid_buf[k, 1])
        hid = (_round_bf16(gt * _sigmoid(gt)) * up).astype(bf16)
        y_acc[...] += lax.dot_general(hid, wd_buf[:, fcols(ft)], NT_DIMS, preferred_element_type=f32)

    def moe_tasks(ft0, count):
        tasks = []
        for k0 in range(0, count, FPB):
            ks = range(k0, min(k0 + FPB, count))
            tasks += [lambda k=k, w=w: moe_up_task(ft0 + k, k, w) for k in ks for w in range(2)]
            tasks += [lambda k=k: moe_down_task(ft0 + k, k) for k in ks]
        return tasks

    def moe_finish():
        y = _round_bf16(y_acc[...])
        rsel = jnp.where(lax.broadcasted_iota(i32, (16, 1), 0) == 0, m1v, m2v)
        y = _round_bf16(y * _round_bf16(_sigmoid(rsel)))
        y = jnp.concatenate([y, jnp.zeros((16, DP - D), f32)], axis=1)
        y = jnp.concatenate([jnp.zeros((HT, DP), f32), y, jnp.zeros((T - HT - 16, DP), f32)], axis=0)
        y_t = jnp.concatenate([y.T[0:D], jnp.zeros((D, T), f32)], axis=1)
        y_u = _pack(y_t)[:, 0:T]
        lane = lax.broadcasted_iota(i32, (D // 2, T), 1)
        wot_u[:, DP - T:DP] = jnp.where(lane < HT, wot_u[:, DP - T:DP], y_u)
        rid = lax.broadcasted_iota(i32, (8, T), 0)
        for tt in range(TPS):
            tok_l = lax.broadcasted_iota(i32, (8, T), 1) + (NSEG - 1) * L + tt * T
            ots[tt][D:D + 8, :] = jnp.where(((rid == 0) & (tok_l == i1)) | ((rid == 1) & (tok_l == i2)), 1.0, 0.0)

    dense = _interleave(a_tasks((0, 0)), prep_dense(3, wot_u, 0))
    with _scope("p15_mix"):
        cut = (2 * len(dense)) // 3
        run(dense[:cut] + [select_task] + dense[cut:])

    def out_tile(s, tt, last, chunk_copies=None):
        c0 = s * L + tt * T
        if not isinstance(s, int):
            c0 = pl.multiple_of(c0, T)
        o_bf = ots[tt][...].astype(bf16)
        nchunk = 4
        rows = D // nchunk
        for rc in range(nchunk):
            r0 = rc * rows
            attn = jnp.dot(_bf(wot_u[r0 // 2:(r0 + rows) // 2, :]), o_bf, preferred_element_type=f32)
            xn = _bf(xn_u[s * TPS + tt, r0 // 2:(r0 + rows) // 2, :]).astype(f32)
            x = x_buf[r0:r0 + rows, pl.ds(c0, T)].astype(f32)
            res = x + attn + xn
            out_buf[r0:r0 + rows, pl.ds(c0, T)] = res.astype(bf16)
            if chunk_copies is not None:
                chunk_copies[rc].start()

    def pair_tasks(ua, ub):
        tasks = []
        for x, y in zip(a_tasks(ua), b_tasks(ub)):
            tasks += [y, x]
        return tasks

    def seg_end(s, last):
        def by_qt(fn, unit, qt):
            return [lambda u=u: fn(unit, u, qt) for u in range(NP)]

        steps = []
        for step in range(7):
            lists = []
            if step < 4:
                lists.append(by_qt(stage_b, (s, 2), 3 - step))
                lists.append(by_qt(stage_a, (s, 3), 3 - step))
            if 1 <= step < 5:
                lists.append(by_qt(stage_b, (s, 3), 4 - step))
            if not last and 2 <= step < 6:
                lists.append(by_qt(stage_a, (s + 1, 0), 5 - step))
            if step >= 3:
                lists.append([lambda tt=6 - step: out_tile(s, tt, last)])
            steps.append(_interleave(*lists))
        return steps

    def seg_att(s, c):
        tasks = pair_tasks((s, 1), (s, 0)) + pair_tasks((s, 2), (s, 1))
        steps = seg_end(s, False)
        for step in steps[0:5]:
            tasks += step
        with _scope("att_seg"):
            run(_interleave(tasks, moe_tasks(s * FPI, FPI)))
            for step in steps[5:]:
                run(step)
        out_copy(pl.multiple_of(s * L, L), L, s).start()
        return c

    lax.fori_loop(0, NSEG - 1, seg_att, 0)

    npatch = (NSEG - 1) * TPS

    def patch_tile(idx):
        return jnp.where(idx < npatch * T, idx // T, 0)

    tile0 = patch_tile(i1)
    tile1 = patch_tile(i2)
    tile1 = jnp.where(tile1 == tile0, (tile0 + 1) % npatch, tile1)

    def patch(tile):
        c0 = pl.multiple_of(tile * T, T)
        rid = lax.broadcasted_iota(i32, (T, T), 0)
        tok_l = lax.broadcasted_iota(i32, (T, T), 1) + c0
        hit = ((rid == HT) & (tok_l == i1)) | ((rid == HT + 1) & (tok_l == i2))
        onehot = jnp.where(hit, 1.0, 0.0).astype(bf16)
        for rc in range(4):
            r0, r1 = rc * (D // 4), (rc + 1) * (D // 4)
            upd = jnp.dot(_bf(wot_u[r0 // 2:r1 // 2, DP - T:DP]), onehot, preferred_element_type=f32)
            cur = out_buf[r0:r1, pl.ds(c0, T)].astype(f32)
            out_buf[r0:r1, pl.ds(c0, T)] = (cur + upd).astype(bf16)

    patch_copies = [out_copy(pl.multiple_of(tile0 * T, T), T, 7), out_copy(pl.multiple_of(tile1 * T, T), T, 8)]
    last_copies = [out_copy((NSEG - 1) * L + tt * T, T, NSEG - 1 + tt) for tt in range(1, TPS)]
    c_fin = (NSEG - 1) * L
    final_copies = [
        pltpu.make_async_copy(out_buf.at[rc * (D // 4):(rc + 1) * (D // 4), c_fin:c_fin + T],
                              out_hbm.at[rc * (D // 4):(rc + 1) * (D // 4), c_fin:c_fin + T],
                              sems.at[SEM_FINAL + rc]) for rc in range(4)]

    sl = NSEG - 1
    with _scope("tail_1"):
        moe_finish()
        run(pair_tasks((sl, 1), (sl, 0)))
        for s in range(NSEG - 1):
            out_copy(s * L, L, s).wait()
    with _scope("tail_2"):
        patch(tile0)
        patch(tile1)
        run(pair_tasks((sl, 2), (sl, 1)))
        for cp in patch_copies:
            cp.start()
        steps = seg_end(sl, True)
        for step in steps[0:5]:
            run(step)
        last_copies[2].start()
        last_copies[1].start()
    with _scope("tail_3"):
        run(steps[5])
        last_copies[0].start()
        out_tile(sl, 0, True, final_copies)

    with _scope("out_wait"):
        for cp in patch_copies + last_copies + final_copies:
            cp.wait()


@jax.jit
def pallas_parallel_sum__memory_aug_infini_attn__moe_arch_mod__prompt_kernel(
    A_x: jax.Array,
    A_wq: jax.Array,
    A_wk: jax.Array,
    A_wv: jax.Array,
    A_wo: jax.Array,
    A_beta: jax.Array,
    B_x: jax.Array,
    B_w_r: jax.Array,
    B_w_gate: jax.Array,
    B_w_up: jax.Array,
    B_w_down: jax.Array,
):
    del B_x
    any_spec = pl.BlockSpec(memory_space=pl.ANY)
    scratch = [
        pltpu.VMEM((H,), bf16),
        pltpu.VMEM((D,), bf16),
        pltpu.VMEM((D, SEQ), bf16),
        pltpu.VMEM((4, D, D), bf16),
        pltpu.VMEM((D, F), bf16),
        pltpu.VMEM((D, F), bf16),
        pltpu.VMEM((D, F), bf16),
        pltpu.VMEM((D, SEQ), bf16),
        pltpu.VMEM((WT_ROWS, DP), u32),
        pltpu.VMEM((D // 2, DP), u32),
        pltpu.VMEM((D // 2, DP), u32),
        pltpu.VMEM((NT, DP // 2, T), u32),
        pltpu.VMEM((BT, DP // 2, T), u32),
        pltpu.VMEM((BT, DP // 2, T), u32),
        pltpu.VMEM((NSEG * NG, TW, L), u32),
        pltpu.VMEM((NSEG * NG, L // 2, T), u32),
        pltpu.VMEM((NSEG * NG, TW, L), u32),
        pltpu.VMEM((NSEG * NG, TW, L), u32),
        pltpu.VMEM((NSEG, D // 2, L), u32),
        pltpu.VMEM((NSEG * H, 16, L), u32),
        pltpu.VMEM((NSEG, 8, L), f32),
        pltpu.VMEM((NG, T, T), f32),
        pltpu.VMEM((NG, T, T), f32),
        pltpu.VMEM((NSEG, D, L), f32),
        pltpu.VMEM((NG, 8, T), f32),
        pltpu.VMEM((H, 8, T), f32),
        pltpu.VMEM((3, HT, T), f32),
        pltpu.VMEM((NP, 4, 2 * L, T), f32),
        pltpu.VMEM((NP, 4, 2, 8, T), f32),
        pltpu.VMEM((NP, 4, 2 * L, T), f32),
        pltpu.VMEM((NP, 4, 2, 8, T), f32),
        pltpu.VMEM((DP, T), f32),
        pltpu.VMEM((DP, T), f32),
        pltpu.VMEM((DP, T), f32),
        pltpu.VMEM((DP, T), f32),
        pltpu.VMEM((2, D, LNW), f32),
        pltpu.VMEM((2, 2, 8, LNW), f32),
        pltpu.VMEM((16, D), f32),
        pltpu.VMEM((8, DP), u32),
        pltpu.VMEM((FPI, 2, 16, T), f32),
        pltpu.SemaphoreType.DMA((NSEM,)),
    ]
    x_t = jnp.transpose(A_x, (0, 2, 1)).reshape(D, SEQ)
    out_t = pl.pallas_call(
        _kernel,
        out_shape=jax.ShapeDtypeStruct((D, SEQ), bf16),
        in_specs=[any_spec] * 10,
        out_specs=any_spec,
        scratch_shapes=scratch,
        compiler_params=pltpu.CompilerParams(vmem_limit_bytes=110 * 1024 * 1024),
    )(x_t, A_wq, A_wk, A_wv, A_wo, A_beta, B_w_r, B_w_gate, B_w_up, B_w_down.T)
    return jnp.transpose(out_t.reshape(1, D, SEQ), (0, 2, 1))
```

```python
import contextlib

import jax
import jax.numpy as jnp
from jax import lax
from jax.experimental import pallas as pl
from jax.experimental.pallas import tpu as pltpu

bf16 = jnp.bfloat16
f32 = jnp.float32
u32 = jnp.uint32
i32 = jnp.int32

SEQ = 2048
D = 576
DP = 640
H = 32
DH = 18
NSEG = 4
L = 512
T = 128
TW = T // 2
HT = T // 2
TPS = L // T
HPG = 6
NG = 6
F = 4608
FPI = 12
FPB = 3
NFT = F // T
NP = 4
UPS = H // (2 * NP)
NUNIT = NSEG * UPS
NT = SEQ // T
LNW = 256
BT = LNW // T
NORM_PARTS = 6
VB = 8 * DH

LOG2E = 1.4426950408889634
QSCALE = (DH ** -0.5) * LOG2E
MASKVAL = -1000000000.0 * LOG2E
EPS_BF16 = 1.0013580322265625e-05
ONES_PAIR = 0x3F803F80

NT_DIMS = (((1,), (1,)), ((), ()))

WT_Q = 0
WT_K = D // 2
WT_R = D
WT_V = D + 8
WT_ROWS = WT_V + D // 2
WT_ALLOC = 1056
NBLK = DP // T

X_PIECES = ((0, LNW), (LNW, LNW), (L, L), (2 * L, L), (3 * L, L))
SEM_X = 0
SEM_W = 5
SEM_MOE = 9
SEM_OUT = 12
SEM_SMALL = 21
SEM_WQB = 23
SEM_FINAL = 24
NSEM = 28
WQ_SPLIT = 2 * T


PROFILE_SCOPES = False
PACE = True
TAIL_BARRIERS = False
QT_ORDER = (3, 2, 1, 0)


def _scope(name):
    return jax.named_scope(name) if PROFILE_SCOPES else contextlib.nullcontext()


def _valid(g):
    return min(HPG * DH, D - g * HPG * DH)


def _ewin(g):
    start = (g * HPG * DH // 16) * 16
    return start, g * HPG * DH - start, min(T, D - start)


def _bf(x):
    return pltpu.bitcast(x, bf16)


def _pack(x):
    return pltpu.bitcast(x.astype(bf16), u32)


def _round_bf16(x):
    return x.astype(bf16).astype(f32)


def _phi(t):
    return jnp.where(t > 0, t + 1.0, jnp.exp(t))


def _sigmoid(t):
    return 1.0 / (1.0 + jnp.exp(-t))


def _zero_after(v):
    bits = pltpu.bitcast(v[0:8, 0:LNW], u32)
    sixteen = jnp.uint32(16)
    bits = lax.shift_right_logical(lax.shift_right_logical(bits, sixteen), sixteen)
    return pltpu.bitcast(bits, f32) if PACE else None


def _interleave(*lists):
    items = []
    for li, tasks in enumerate(lists):
        for k, t in enumerate(tasks):
            items.append(((k + 0.5) / len(tasks), li, k, t))
    items.sort(key=lambda it: it[:3])
    return [it[3] for it in items]


def _kernel(x_hbm, wq_hbm, wk_hbm, wv_hbm, wo_hbm, beta_hbm, wr_hbm, wg_hbm, wu_hbm, wd_hbm,
            out_hbm,
            beta_ref, wr_ref, x_buf, w_buf, wg_buf, wu_buf, wd_buf, out_buf,
            wt_u, kt_tmp, wot_u, xn_u, xs_a, xs_b, qs_u, k_u, pq_u, pk_u, vt_u, vwin,
            r_buf, mt_acc, lm_f, am, g16, omg, mb,
            s0, m0, s1, m1, ot0, ot1, ot2, ot3, xf, ln_stat, y_acc, xsel_buf, hid_buf, sems):

    def x_copy(i):
        c0, width = X_PIECES[i]
        return pltpu.make_async_copy(x_hbm.at[:, pl.ds(c0, width)], x_buf.at[:, pl.ds(c0, width)],
                                     sems.at[SEM_X + i])

    def w_copy(i):
        src = (wq_hbm, wk_hbm, wv_hbm, wo_hbm)[i]
        return pltpu.make_async_copy(src, w_buf.at[i], sems.at[SEM_W + i])

    wq_first = pltpu.make_async_copy(wq_hbm.at[:, 0:WQ_SPLIT], w_buf.at[0, :, 0:WQ_SPLIT], sems.at[SEM_W])
    wq_rest = pltpu.make_async_copy(wq_hbm.at[:, WQ_SPLIT:D], w_buf.at[0, :, WQ_SPLIT:D], sems.at[SEM_WQB])

    def moe_copy(i):
        src = (wg_hbm, wu_hbm, wd_hbm)[i]
        dst = (wg_buf, wu_buf, wd_buf)[i]
        return pltpu.make_async_copy(src, dst, sems.at[SEM_MOE + i])

    def out_copy(c0, width, sem):
        return pltpu.make_async_copy(out_buf.at[:, pl.ds(c0, width)], out_hbm.at[:, pl.ds(c0, width)],
                                     sems.at[SEM_OUT + sem])

    small_copies = [pltpu.make_async_copy(beta_hbm, beta_ref, sems.at[SEM_SMALL]),
                    pltpu.make_async_copy(wr_hbm, wr_ref, sems.at[SEM_SMALL + 1])]
    x_copy(0).start()
    wq_first.start()
    wq_rest.start()
    x_copy(1).start()
    for cp in small_copies:
        cp.start()
    w_copy(1).start()
    w_copy(2).start()

    init_scope = _scope("init")
    init_scope.__enter__()
    kr = lax.broadcasted_iota(i32, (HT, T), 0)
    ql = lax.broadcasted_iota(i32, (HT, T), 1)
    mb[0] = jnp.where(ql < kr, MASKVAL, 0.0).astype(f32)
    mb[1] = jnp.where((ql >= HT) & (ql - HT < kr), MASKVAL, 0.0).astype(f32)
    mb[2] = jnp.where(ql % HT < kr, MASKVAL, 0.0).astype(f32)
    zpad = jnp.zeros(((DP - D) // 2, T), u32)
    for tt in range(NT):
        xn_u[tt, D // 2:DP // 2, :] = zpad
    for tt in range(BT):
        xs_a[tt, D // 2:DP // 2, :] = zpad
        xs_b[tt, D // 2:DP // 2, :] = zpad
    ots = (ot0, ot1, ot2, ot3)
    for o_ref in ots:
        o_ref[D:DP, :] = jnp.zeros((DP - D, T), f32)
    am[0] = jnp.zeros(am.shape[1:], f32)
    mt_acc[...] = jnp.zeros(mt_acc.shape, f32)
    g16[...] = jnp.zeros(g16.shape, f32)

    init_scope.__exit__(None, None, None)

    pace = [None]

    def gate_tables():
        gate = _round_bf16(_sigmoid(beta_ref[...].reshape(1, H).astype(f32)))
        for h in range(H):
            gh = jnp.broadcast_to(gate[:, h:h + 1], (1, T))
            omg[h] = jnp.broadcast_to(_round_bf16(1.0 - gh), (8, T))
            g16[h // HPG, (h % HPG):(h % HPG) + 1, :] = gh

    def transpose_block(i, cb):
        c1 = min((cb + 1) * T, D)
        blk = w_buf[i, :, cb * T:c1]
        if c1 - cb * T < T:
            blk = jnp.concatenate([blk, jnp.zeros((D, T - (c1 - cb * T)), bf16)], axis=1)
        blk = jnp.concatenate([blk, jnp.zeros((DP - D, T), bf16)], axis=0)
        return pltpu.bitcast(blk.T, u32)

    def prep_dense(i, dst, base):
        def task(cb):
            nrow = min(TW, D // 2 - cb * TW)
            dst[base + cb * TW:base + cb * TW + nrow, :] = transpose_block(i, cb)[0:nrow]
        return [lambda cb=cb: task(cb) for cb in range(DP // T)]

    def router_row():
        wr = wr_ref[...].reshape(1, D).astype(f32)
        wr = jnp.concatenate([wr, jnp.zeros((1, DP - D), f32)], axis=1)
        bits = lax.shift_right_logical(pltpu.bitcast(wr, u32), u32(16))
        rid = lax.broadcasted_iota(i32, (8, DP), 0)
        wt_u[WT_R:WT_R + 8, :] = jnp.where(rid == 0, bits, u32(0))

    def ln_tasks(s, p, stage):
        c0 = s * L + p * LNW
        if not isinstance(s, int):
            c0 = pl.multiple_of(c0, LNW)

        def mean_pass():
            acc = pace[0]
            for r in range(0, D, 64):
                x = x_buf[r:r + 64, pl.ds(c0, LNW)].astype(f32)
                xf[p, r:r + 64, :] = x
                part = jnp.sum(x.reshape(8, 8, LNW), axis=0)
                acc = part if acc is None else acc + part
            mean = jnp.sum(acc, axis=0, keepdims=True) / D
            ln_stat[p, 0] = jnp.broadcast_to(mean, (8, LNW))

        def var_pass():
            mean = ln_stat[p, 0][0:1]
            if pace[0] is not None:
                mean = mean + pace[0][0:1]
            acc = None
            for r in range(0, D, 96):
                xc = xf[p, r:r + 96, :] - mean
                part = jnp.sum((xc * xc).reshape(12, 8, LNW), axis=0)
                acc = part if acc is None else acc + part
            var = jnp.sum(acc, axis=0, keepdims=True) / D
            den = _round_bf16(jnp.sqrt(_round_bf16(_round_bf16(var) + EPS_BF16)))
            ln_stat[p, 1] = jnp.broadcast_to(1.0 / den, (8, LNW))
            ln_stat[p, 0] = jnp.broadcast_to(_round_bf16(mean), (8, LNW))

        def norm_pass(part):
            mean_b = ln_stat[p, 0][0:1]
            if pace[0] is not None:
                mean_b = mean_b + pace[0][0:1]
            inv = ln_stat[p, 1][0:1]
            step = D // NORM_PARTS
            for r in range(part * step, (part + 1) * step, 48):
                xn = _pack(_round_bf16(xf[p, r:r + 48, :] - mean_b) * inv)
                for t in range(BT):
                    xn_u.at[s * TPS + p * BT + t][r // 2:r // 2 + 24, :] = xn[:, t * T:(t + 1) * T]
                    if stage is not None:
                        stage.at[t][r // 2:r // 2 + 24, :] = xn[:, t * T:(t + 1) * T]

        return [mean_pass, var_pass] + [lambda part=part: norm_pass(part) for part in range(NORM_PARTS)]

    def load_xs(s, p, stage):
        if stage is None:
            tiles = [xn_u[s * TPS + p * BT + t] for t in range(BT)]
        else:
            tiles = [stage[t] for t in range(BT)]
        return jnp.concatenate([_bf(t) for t in tiles], axis=1)

    def blk_rows(cb):
        return min(TW, D // 2 - cb * TW)

    def q_task(s, p, stage, cb):
        nr = blk_rows(cb)
        rows = slice(cb * TW, cb * TW + nr)
        cols = slice(p * LNW, (p + 1) * LNW)
        w = _bf(wt_u[WT_Q + cb * TW:WT_Q + cb * TW + nr, :])
        q = jnp.dot(w, load_xs(s, p, stage), preferred_element_type=f32)
        pace[0] = _zero_after(q)
        qp = _pack(q * QSCALE)
        qrot = jnp.concatenate([pltpu.roll(qp[:, t * T:(t + 1) * T], HT, 1) for t in range(BT)], axis=1)
        rid = lax.broadcasted_iota(i32, qp.shape, 0) + cb * TW
        even = ((rid // (DH // 2)) % 2) == 0
        qs_u.at[s][rows, cols] = jnp.where(even, qrot, qp)
        pq_u.at[s][rows, cols] = _pack(_phi(q))

    def k_task(s, p, stage, cb):
        nr = blk_rows(cb)
        rows = slice(cb * TW, cb * TW + nr)
        cols = slice(p * LNW, (p + 1) * LNW)
        extra = 8 if cb == NBLK - 1 else 0
        w = _bf(wt_u[WT_K + cb * TW:WT_K + cb * TW + nr + extra, :])
        k = jnp.dot(w, load_xs(s, p, stage), preferred_element_type=f32)
        pace[0] = _zero_after(k)
        if extra:
            r_buf[s, :, cols] = jnp.broadcast_to(k[2 * nr:2 * nr + 1, :], (8, LNW))
            k = k[0:2 * nr]
        kt_tmp.at[p][rows, :] = _pack(k)
        pk_u.at[s][rows, cols] = _pack(_phi(k))

    def kt_task(s, p, g):
        nv = _valid(g) // 2
        src = g * HPG * DH // 2
        kg = jnp.concatenate([kt_tmp[p, src:src + nv, :], jnp.zeros((TW - nv, LNW), u32)], axis=0)
        k_u.at[s * NG + g][p * (LNW // 2):(p + 1) * (LNW // 2), :] = pltpu.bitcast(_bf(kg).T, u32)

    def v_task(s, p, stage, b):
        cols = slice(p * LNW, (p + 1) * LNW)
        w = _bf(wt_u[WT_V + b * (VB // 2):WT_V + (b + 1) * (VB // 2), :])
        v = jnp.dot(w, load_xs(s, p, stage), preferred_element_type=f32)
        pace[0] = _zero_after(v)
        v = _pack(v)
        vt_u.at[s][b * (VB // 2):(b + 1) * (VB // 2), cols] = v
        sub = lax.broadcasted_iota(i32, (16, LNW), 0)
        for hh in range(8):
            w8 = (9 * hh) // 8
            ones_row = 0 if 2 * hh == 14 else 15
            vwin.at[s * H + 8 * b + hh][:, cols] = jnp.where(sub == ones_row, u32(ONES_PAIR), v[8 * w8:8 * w8 + 16, :])

    def q_tasks(s, p, stage=None):
        return [lambda cb=cb: q_task(s, p, stage, cb) for cb in range(NBLK)]

    def k_tasks(s, p, stage=None):
        tasks, done = [], 0
        for cb in range(NBLK):
            tasks.append(lambda cb=cb: k_task(s, p, stage, cb))
            while done < NG and done * HPG * DH + _valid(done) <= min((cb + 1) * T, D):
                tasks.append(lambda g=done: kt_task(s, p, g))
                done += 1
        return tasks

    def v_tasks(s, p, stage=None):
        return [lambda b=b: v_task(s, p, stage, b) for b in range(D // VB)]

    def mem_layout(g):
        es, eoff, _ = _ewin(g)
        nv = _valid(g)
        ne = -(-(eoff + nv) // 16) * 16
        ones_row = 0 if eoff >= 2 else eoff + nv
        nh = nv // DH
        den_row = 0 if eoff >= nh else ne
        return es, eoff, nv, ne, ones_row, den_row, max(ne, den_row + 16 * (den_row > 0))

    def mem_update(sp, g):
        es, eoff, nv, ne, ones_row, den_row, nr = mem_layout(g)
        nw = min(T, D - es)
        win = vt_u[sp, es // 2:(es + ne) // 2, :]
        wid = lax.broadcasted_iota(i32, win.shape, 0)
        lhs = _bf(jnp.where(wid == ones_row // 2, u32(ONES_PAIR), win))
        upd = lax.dot_general(lhs, _bf(pk_u[sp, es // 2:(es + nw) // 2, :]), NT_DIMS, preferred_element_type=f32)
        mt = mt_acc[g, 0:ne, 0:nw] + upd
        mt_acc[g, 0:ne, 0:nw] = mt
        z = jnp.broadcast_to(mt[ones_row:ones_row + 1, :], (nr, nw))
        if nr > ne:
            mt = jnp.concatenate([mt, jnp.zeros((nr - ne, nw), f32)], axis=0)
        row = lax.broadcasted_iota(i32, (nr, nw), 0)
        d_loc = lax.broadcasted_iota(i32, (nr, nw), 1) - eoff
        e_loc = row - eoff
        d_ok = (d_loc >= 0) & (d_loc < nv)
        same_head = (e_loc >= 0) & (e_loc < nv) & d_ok & ((e_loc // DH) == (d_loc // DH))
        den_hit = (row >= den_row) & d_ok & ((d_loc // DH) == row - den_row)
        lm_f[g, 0:nr, 0:nw] = jnp.where(same_head, mt, jnp.where(den_hit, z, 0.0))

    def mem_retrieve(s, g):
        es, eoff, nv, ne, ones_row, den_row, nr = mem_layout(g)
        nw = min(T, D - es)
        nd = jnp.dot(lm_f[g, 0:nr, 0:nw].astype(bf16), _bf(pq_u[s, es // 2:(es + nw) // 2, :]),
                     preferred_element_type=f32)
        scale = jnp.broadcast_to(g16[g][:, 0:1], (8, L)) / (nd[den_row:den_row + 8, :] + 1e-6)
        r8 = lax.broadcasted_iota(i32, (8, L), 0)
        for b in range(ne // 8):
            lo, hi = 8 * b - eoff, 8 * b + 7 - eoff
            if hi < 0 or lo >= nv:
                continue
            j1, j2 = max(lo, 0) // DH, min(hi, nv - 1) // DH
            sc = jnp.broadcast_to(scale[j1:j1 + 1, :], (8, L))
            if j2 != j1:
                sc = jnp.where(r8 < DH * j2 - lo, sc, jnp.broadcast_to(scale[j2:j2 + 1, :], (8, L)))
            val = nd[8 * b:8 * b + 8, :] * sc
            dst = am.at[s, es + 8 * b:es + 8 * b + 8, :]
            if lo >= 0 and hi < nv:
                dst[...] = val
            else:
                pltpu.store(dst, val, mask=(r8 + lo >= 0) & (r8 + lo < nv))

    def run(tasks):
        for t in tasks:
            t()

    prep_q = prep_dense(0, wt_u, WT_Q)
    q0a = q_tasks(0, 0)
    with _scope("p1_wait_x0"):
        x_copy(0).wait()
    for i in range(2, len(X_PIECES)):
        x_copy(i).start()
    w_copy(3).start()
    for i in range(3):
        moe_copy(i).start()
    with _scope("p1_ln0a"):
        run(ln_tasks(0, 0, None))
        wq_first.wait()
    with _scope("p1_q0a_first"):
        run(prep_q[0:2] + q0a[0:2])
        wq_rest.wait()
        x_copy(1).wait()
    with _scope("p1_q0a"):
        run(prep_q[2:])
        run(_interleave(q0a[2:], ln_tasks(0, 1, None)))
        w_copy(1).wait()
        for cp in small_copies:
            cp.wait()
    k0a, k0b = k_tasks(0, 0), k_tasks(0, 1)
    with _scope("p1_q0b"):
        run(_interleave(q_tasks(0, 1), prep_dense(1, wt_u, WT_K), [router_row, gate_tables]))
        run(k0a)
        w_copy(2).wait()
        x_copy(2).wait()
    with _scope("p1_k0v0"):
        run(_interleave(k0b, prep_dense(2, wt_u, WT_V)))
        run(_interleave(v_tasks(0, 0) + v_tasks(0, 1), ln_tasks(1, 0, xs_a)))

    def seg_body(s, c):
        for ss in range(2, NSEG):
            @pl.when(s + 1 == ss)
            def _():
                x_copy(ss + 1).wait()
        nxt = jnp.minimum(s + 1, NSEG - 1)
        pace[0] = None
        with _scope("p1_seg"):
            updates = [lambda g=g: mem_update(s - 1, g) for g in range(NG)]
            retrieves = [lambda g=g: mem_retrieve(s, g) for g in range(NG)]
            first = _interleave(q_tasks(s, 0, xs_a), updates) + k_tasks(s, 0, xs_a) + v_tasks(s, 0, xs_a)
            run(_interleave(first, ln_tasks(s, 1, xs_b)))
            second = q_tasks(s, 1, xs_b) + _interleave(k_tasks(s, 1, xs_b) + v_tasks(s, 1, xs_b), retrieves)
            run(_interleave(second, ln_tasks(nxt, 0, xs_a)))
        return c

    lax.fori_loop(1, NSEG, seg_body, 0)

    bufs = ((s0, m0), (s1, m1))
    lane64 = lax.broadcasted_iota(i32, (TW, T), 1)
    lane1 = lax.broadcasted_iota(i32, (1, T), 1)
    lane8 = lax.broadcasted_iota(i32, (8, T), 1)

    def pair_weights(s, pi, qt):
        hw = DH // 2
        j = 2 * (pi % (HPG // 2))
        src, dst = hw * 2 * pi, hw * j
        a0, t0 = (src // 8) * 8, (dst // 8) * 8
        nrow = min(32, D // 2 - a0)
        part = qs_u[s, a0:a0 + nrow, qt * T:(qt + 1) * T]
        if nrow < 32:
            part = jnp.concatenate([part, jnp.zeros((32 - nrow, T), u32)], axis=0)
        shift = (dst - t0) - (src - a0)
        if shift:
            part = pltpu.roll(part, shift % 32, 0)
        rid = lax.broadcasted_iota(i32, (32, T), 0) + t0
        out = []
        for lo in (dst, dst + hw):
            piece = jnp.where((rid >= lo) & (rid < lo + hw), part, u32(0))
            piece = piece[0:min(32, TW - t0)]
            pieces = [jnp.zeros((t0, T), u32)] * (t0 > 0) + [piece] + [jnp.zeros((TW - t0 - 32, T), u32)] * (t0 + 32 < TW)
            out.append(jnp.concatenate(pieces, axis=0))
        return out

    def stage_a(unit, u, qt):
        s, k = unit
        s_ref, m_ref = bufs[k % 2]
        pi = k * NP + u
        g = pi // (HPG // 2)
        sg = s * NG + g
        n = T * (qt + 1)
        w_a, w_b = pair_weights(s, pi, qt)
        w_ab = _bf(jnp.where(lane64 < HT, w_a, w_b))

        def colmax8(v):
            return jnp.max(v.reshape(v.shape[0] // 8, 8, T), axis=0)

        maxes = []
        for hd, w in enumerate((_bf(w_a), _bf(w_b))):
            m8 = None
            for c in range(qt):
                kc = _bf(k_u[sg, c * TW:(c + 1) * TW, :])
                sc = jnp.dot(kc, w, preferred_element_type=f32)
                s_ref[u, qt, hd * L + c * T:hd * L + (c + 1) * T, :] = sc
                m8 = colmax8(sc) if m8 is None else jnp.maximum(m8, colmax8(sc))
            kc = _bf(k_u[sg, qt * TW:qt * TW + TW // 2, :])
            sc = jnp.dot(kc, w, preferred_element_type=f32) + mb[1 - hd]
            s_ref[u, qt, hd * L + qt * T:hd * L + qt * T + HT, :] = sc
            m8 = colmax8(sc) if m8 is None else jnp.maximum(m8, colmax8(sc))
            maxes.append(m8)
        kc = _bf(k_u[sg, qt * TW + TW // 2:(qt + 1) * TW, :])
        sc = jnp.dot(kc, w_ab, preferred_element_type=f32) + mb[2]
        s_ref[u, qt, n - HT:n, :] = sc
        mab = colmax8(sc)
        m_a = jnp.where(lane8 < HT, jnp.maximum(maxes[0], mab), maxes[0])
        m_b = jnp.where(lane8 >= HT, jnp.maximum(maxes[1], mab), maxes[1])
        m_ref[u, qt, 0] = jnp.broadcast_to(jnp.max(m_a, axis=0, keepdims=True), (8, T))
        m_ref[u, qt, 1] = jnp.broadcast_to(jnp.max(m_b, axis=0, keepdims=True), (8, T))

    def stage_b(unit, u, qt):
        s, k = unit
        s_ref, m_ref = bufs[k % 2]
        pi = k * NP + u
        n = T * (qt + 1)
        m_a = m_ref[u, qt, 0][0:1]
        m_b = m_ref[u, qt, 1][0:1]
        p_ab = jnp.exp2(s_ref[u, qt, n - HT:n, :] - jnp.where(lane1 < HT, m_a, m_b))
        for hd, m in enumerate((m_a, m_b)):
            h = 2 * pi + hd
            p = jnp.exp2(s_ref[u, qt, hd * L:hd * L + n - HT, :] - m)
            keep = (lane64 < HT) if hd == 0 else (lane64 >= HT)
            p = jnp.concatenate([p, jnp.where(keep, p_ab, 0.0)], axis=0).astype(bf16)
            w0 = ((DH * h) // 16) * 16
            off = DH * h - w0
            o = jnp.dot(_bf(vwin[s * H + h, :, 0:n]), p, preferred_element_type=f32)
            den = o[0:1] if off == 14 else o[31:32]
            r0, r1 = (off // 8) * 8, -(-(off + DH) // 8) * 8
            o = o[r0:r1] * (omg[h][0:1] / den)
            if hd == 0:
                o = pltpu.roll(o, HT, 1)
            res = am[s, w0 + r0:w0 + r1, qt * T:(qt + 1) * T] + o
            rid = lax.broadcasted_iota(i32, (r1 - r0, T), 0) + r0
            pltpu.store(ots[qt].at[w0 + r0:w0 + r1, :], res, mask=(rid >= off) & (rid < off + DH))

    def a_tasks(unit):
        return [lambda u=u, qt=qt: stage_a(unit, u, qt) for u in range(NP) for qt in QT_ORDER]

    def b_tasks(unit):
        return [lambda u=u, qt=qt: stage_b(unit, u, qt) for u in range(NP) for qt in QT_ORDER]

    w_copy(3).wait()
    rr = jnp.concatenate([r_buf[s][0:1, :] for s in range(NSEG)], axis=0)
    rr = _round_bf16(rr)
    tok = lax.broadcasted_iota(i32, (NSEG, L), 0) * L + lax.broadcasted_iota(i32, (NSEG, L), 1)
    m1v = jnp.max(rr)
    i1 = jnp.min(jnp.where(rr == m1v, tok, SEQ))
    rr2 = jnp.where(tok == i1, -jnp.inf, rr)
    m2v = jnp.max(rr2)
    i2 = jnp.min(jnp.where(rr2 == m2v, tok, SEQ))
    i1 = jnp.clip(i1, 0, SEQ - 1)
    i2 = jnp.clip(i2, 0, SEQ - 1)

    row16 = lax.broadcasted_iota(i32, (16, T), 0)
    lane16 = lax.broadcasted_iota(i32, (16, T), 1)

    def token_rows(i, slot):
        onehot = jnp.where((row16 == slot) & (lane16 == i % T), 1.0, 0.0).astype(bf16)
        return lax.dot_general(onehot, _bf(xn_u[i // T]), NT_DIMS, preferred_element_type=f32)

    def select_task():
        xsel_buf[...] = _pack(token_rows(i1, 0) + token_rows(i2, 1))
        y_acc[...] = jnp.zeros(y_acc.shape, f32)

    def fcols(ft):
        return pl.ds(ft * T if isinstance(ft, int) else pl.multiple_of(ft * T, T), T)

    def moe_up_task(ft, k, which):
        xsel = _bf(xsel_buf[:, 0:D])
        w_ref = (wg_buf, wu_buf)[which]
        hid_buf[k, which] = jnp.dot(xsel, w_ref[:, fcols(ft)], preferred_element_type=f32)

    def moe_down_task(ft, k):
        gt = _round_bf16(hid_buf[k, 0])
        up = _round_bf16(hid_buf[k, 1])
        hid = (_round_bf16(gt * _sigmoid(gt)) * up).astype(bf16)
        y_acc[...] += lax.dot_general(hid, wd_buf[:, fcols(ft)], NT_DIMS, preferred_element_type=f32)

    def moe_tasks(ft0, count):
        tasks = []
        for k0 in range(0, count, FPB):
            ks = range(k0, min(k0 + FPB, count))
            tasks += [lambda k=k, w=w: moe_up_task(ft0 + k, k, w) for k in ks for w in range(2)]
            tasks += [lambda k=k: moe_down_task(ft0 + k, k) for k in ks]
        return tasks

    def moe_finish():
        y = _round_bf16(y_acc[...])
        rsel = jnp.where(lax.broadcasted_iota(i32, (16, 1), 0) == 0, m1v, m2v)
        y = _round_bf16(y * _round_bf16(_sigmoid(rsel)))
        y = jnp.concatenate([y, jnp.zeros((16, DP - D), f32)], axis=1)
        y = jnp.concatenate([jnp.zeros((HT, DP), f32), y, jnp.zeros((T - HT - 16, DP), f32)], axis=0)
        y_t = jnp.concatenate([y.T[0:D], jnp.zeros((D, T), f32)], axis=1)
        y_u = _pack(y_t)[:, 0:T]
        lane = lax.broadcasted_iota(i32, (D // 2, T), 1)
        wot_u[:, DP - T:DP] = jnp.where(lane < HT, wot_u[:, DP - T:DP], y_u)
        rid = lax.broadcasted_iota(i32, (8, T), 0)
        for tt in range(TPS):
            tok_l = lax.broadcasted_iota(i32, (8, T), 1) + (NSEG - 1) * L + tt * T
            ots[tt][D:D + 8, :] = jnp.where(((rid == 0) & (tok_l == i1)) | ((rid == 1) & (tok_l == i2)), 1.0, 0.0)

    dense = _interleave(a_tasks((0, 0)), prep_dense(3, wot_u, 0))
    with _scope("p15_mix"):
        cut = (2 * len(dense)) // 3
        run(dense[:cut] + [select_task] + dense[cut:])

    for i in range(3):
        moe_copy(i).wait()

    def out_tile(s, tt, last, chunk_copies=None):
        c0 = s * L + tt * T
        if not isinstance(s, int):
            c0 = pl.multiple_of(c0, T)
        o_bf = ots[tt][...].astype(bf16)
        nchunk = 4
        rows = D // nchunk
        for rc in range(nchunk):
            r0 = rc * rows
            attn = jnp.dot(_bf(wot_u[r0 // 2:(r0 + rows) // 2, :]), o_bf, preferred_element_type=f32)
            xn = _bf(xn_u[s * TPS + tt, r0 // 2:(r0 + rows) // 2, :]).astype(f32)
            x = x_buf[r0:r0 + rows, pl.ds(c0, T)].astype(f32)
            res = x + attn + xn
            out_buf[r0:r0 + rows, pl.ds(c0, T)] = res.astype(bf16)
            if chunk_copies is not None:
                chunk_copies[rc].start()

    def pair_tasks(ua, ub):
        tasks = []
        for x, y in zip(a_tasks(ua), b_tasks(ub)):
            tasks += [y, x]
        return tasks

    def seg_end(s, last):
        def by_qt(fn, unit, qt):
            return [lambda u=u: fn(unit, u, qt) for u in range(NP)]

        steps = []
        for step in range(7):
            lists = []
            if step < 4:
                lists.append(by_qt(stage_b, (s, 2), 3 - step))
                lists.append(by_qt(stage_a, (s, 3), 3 - step))
            if 1 <= step < 5:
                lists.append(by_qt(stage_b, (s, 3), 4 - step))
            if not last and 2 <= step < 6:
                lists.append(by_qt(stage_a, (s + 1, 0), 5 - step))
            if step >= 3:
                lists.append([lambda tt=6 - step: out_tile(s, tt, last)])
            steps.append(_interleave(*lists))
        return steps

    def seg_att(s, c):
        tasks = pair_tasks((s, 1), (s, 0)) + pair_tasks((s, 2), (s, 1))
        steps = seg_end(s, False)
        for step in steps[0:5]:
            tasks += step
        with _scope("att_seg"):
            run(_interleave(tasks, moe_tasks(s * FPI, FPI)))
            for step in steps[5:]:
                run(step)
        out_copy(pl.multiple_of(s * L, L), L, s).start()
        return c

    lax.fori_loop(0, NSEG - 1, seg_att, 0)

    npatch = (NSEG - 1) * TPS

    def patch_tile(idx):
        return jnp.where(idx < npatch * T, idx // T, 0)

    tile0 = patch_tile(i1)
    tile1 = patch_tile(i2)
    tile1 = jnp.where(tile1 == tile0, (tile0 + 1) % npatch, tile1)

    def patch(tile):
        c0 = pl.multiple_of(tile * T, T)
        rid = lax.broadcasted_iota(i32, (T, T), 0)
        tok_l = lax.broadcasted_iota(i32, (T, T), 1) + c0
        hit = ((rid == HT) & (tok_l == i1)) | ((rid == HT + 1) & (tok_l == i2))
        onehot = jnp.where(hit, 1.0, 0.0).astype(bf16)
        for rc in range(4):
            r0, r1 = rc * (D // 4), (rc + 1) * (D // 4)
            upd = jnp.dot(_bf(wot_u[r0 // 2:r1 // 2, DP - T:DP]), onehot, preferred_element_type=f32)
            cur = out_buf[r0:r1, pl.ds(c0, T)].astype(f32)
            out_buf[r0:r1, pl.ds(c0, T)] = (cur + upd).astype(bf16)

    patch_copies = [out_copy(pl.multiple_of(tile0 * T, T), T, 7), out_copy(pl.multiple_of(tile1 * T, T), T, 8)]
    last_copies = [out_copy((NSEG - 1) * L + tt * T, T, NSEG - 1 + tt) for tt in range(1, TPS)]
    c_fin = (NSEG - 1) * L
    final_copies = [
        pltpu.make_async_copy(out_buf.at[rc * (D // 4):(rc + 1) * (D // 4), c_fin:c_fin + T],
                              out_hbm.at[rc * (D // 4):(rc + 1) * (D // 4), c_fin:c_fin + T],
                              sems.at[SEM_FINAL + rc]) for rc in range(4)]

    sl = NSEG - 1
    with _scope("tail_1"):
        moe_finish()
        run(pair_tasks((sl, 1), (sl, 0)))
        for s in range(NSEG - 1):
            out_copy(s * L, L, s).wait()
    with _scope("tail_2"):
        patch(tile0)
        patch(tile1)
        run(pair_tasks((sl, 2), (sl, 1)))
        for cp in patch_copies:
            cp.start()
        steps = seg_end(sl, True)
        for step in steps[0:5]:
            run(step)
        last_copies[2].start()
        last_copies[1].start()
    with _scope("tail_3"):
        run(steps[5])
        last_copies[0].start()
        out_tile(sl, 0, True, final_copies)

    with _scope("out_wait"):
        for cp in patch_copies + last_copies + final_copies:
            cp.wait()


@jax.jit
def pallas_parallel_sum__memory_aug_infini_attn__moe_arch_mod__prompt_kernel(
    A_x: jax.Array,
    A_wq: jax.Array,
    A_wk: jax.Array,
    A_wv: jax.Array,
    A_wo: jax.Array,
    A_beta: jax.Array,
    B_x: jax.Array,
    B_w_r: jax.Array,
    B_w_gate: jax.Array,
    B_w_up: jax.Array,
    B_w_down: jax.Array,
):
    del B_x
    any_spec = pl.BlockSpec(memory_space=pl.ANY)
    scratch = [
        pltpu.VMEM((H,), bf16),
        pltpu.VMEM((D,), bf16),
        pltpu.VMEM((D, SEQ), bf16),
        pltpu.VMEM((4, D, D), bf16),
        pltpu.VMEM((D, F), bf16),
        pltpu.VMEM((D, F), bf16),
        pltpu.VMEM((D, F), bf16),
        pltpu.VMEM((D, SEQ), bf16),
        pltpu.VMEM((WT_ALLOC, DP), u32),
        pltpu.VMEM((2, D // 2, LNW), u32),
        pltpu.VMEM((D // 2, DP), u32),
        pltpu.VMEM((NT, DP // 2, T), u32),
        pltpu.VMEM((BT, DP // 2, T), u32),
        pltpu.VMEM((BT, DP // 2, T), u32),
        pltpu.VMEM((NSEG, D // 2, L), u32),
        pltpu.VMEM((NSEG * NG, L // 2, T), u32),
        pltpu.VMEM((NSEG, D // 2, L), u32),
        pltpu.VMEM((NSEG, D // 2, L), u32),
        pltpu.VMEM((NSEG, D // 2, L), u32),
        pltpu.VMEM((NSEG * H, 16, L), u32),
        pltpu.VMEM((NSEG, 8, L), f32),
        pltpu.VMEM((NG, T, T), f32),
        pltpu.VMEM((NG, T, T), f32),
        pltpu.VMEM((NSEG, D, L), f32),
        pltpu.VMEM((NG, 8, T), f32),
        pltpu.VMEM((H, 8, T), f32),
        pltpu.VMEM((3, HT, T), f32),
        pltpu.VMEM((NP, 4, 2 * L, T), f32),
        pltpu.VMEM((NP, 4, 2, 8, T), f32),
        pltpu.VMEM((NP, 4, 2 * L, T), f32),
        pltpu.VMEM((NP, 4, 2, 8, T), f32),
        pltpu.VMEM((DP, T), f32),
        pltpu.VMEM((DP, T), f32),
        pltpu.VMEM((DP, T), f32),
        pltpu.VMEM((DP, T), f32),
        pltpu.VMEM((2, D, LNW), f32),
        pltpu.VMEM((2, 2, 8, LNW), f32),
        pltpu.VMEM((16, D), f32),
        pltpu.VMEM((8, DP), u32),
        pltpu.VMEM((FPI, 2, 16, T), f32),
        pltpu.SemaphoreType.DMA((NSEM,)),
    ]
    x_t = jnp.transpose(A_x, (0, 2, 1)).reshape(D, SEQ)
    out_t = pl.pallas_call(
        _kernel,
        out_shape=jax.ShapeDtypeStruct((D, SEQ), bf16),
        in_specs=[any_spec] * 10,
        out_specs=any_spec,
        scratch_shapes=scratch,
        compiler_params=pltpu.CompilerParams(vmem_limit_bytes=110 * 1024 * 1024),
    )(x_t, A_wq, A_wk, A_wv, A_wo, A_beta, B_w_r, B_w_gate, B_w_up, B_w_down.T)
    return jnp.transpose(out_t.reshape(1, D, SEQ), (0, 2, 1))
```

```python
import contextlib

import jax
import jax.numpy as jnp
from jax import lax
from jax.experimental import pallas as pl
from jax.experimental.pallas import tpu as pltpu

bf16 = jnp.bfloat16
f32 = jnp.float32
u32 = jnp.uint32
i32 = jnp.int32

SEQ = 2048
D = 576
DP = 640
H = 32
DH = 18
NSEG = 4
L = 512
T = 128
TW = T // 2
HT = T // 2
TPS = L // T
HPG = 6
NG = 6
F = 4608
FPI = 12
FPB = 3
NFT = F // T
NP = 4
UPS = H // (2 * NP)
NUNIT = NSEG * UPS
NT = SEQ // T
LNW = 256
BT = LNW // T
NORM_PARTS = 6
VB = 8 * DH

LOG2E = 1.4426950408889634
QSCALE = (DH ** -0.5) * LOG2E
MASKVAL = -1000000000.0 * LOG2E
EPS_BF16 = 1.0013580322265625e-05
ONES_PAIR = 0x3F803F80

NT_DIMS = (((1,), (1,)), ((), ()))

WT_Q = 0
WT_K = D // 2
WT_R = D
WT_V = D + 8
WT_ROWS = WT_V + D // 2
WT_ALLOC = 1056
NBLK = DP // T

X_PIECES = ((0, LNW), (LNW, LNW), (L, L), (2 * L, L), (3 * L, L))
SEM_X = 0
SEM_W = 5
SEM_MOE = 9
SEM_OUT = 12
SEM_SMALL = 21
SEM_WQB = 23
SEM_FINAL = 24
NSEM = 28
WQ_SPLIT = 2 * T


PROFILE_SCOPES = False
PACE = True
TAIL_BARRIERS = False
QT_ORDER = (3, 2, 1, 0)


def _scope(name):
    return jax.named_scope(name) if PROFILE_SCOPES else contextlib.nullcontext()


def _valid(g):
    return min(HPG * DH, D - g * HPG * DH)


def _ewin(g):
    start = (g * HPG * DH // 16) * 16
    return start, g * HPG * DH - start, min(T, D - start)


def _bf(x):
    return pltpu.bitcast(x, bf16)


def _pack(x):
    return pltpu.bitcast(x.astype(bf16), u32)


def _round_bf16(x):
    return x.astype(bf16).astype(f32)


def _phi(t):
    return jnp.where(t > 0, t + 1.0, jnp.exp(t))


def _sigmoid(t):
    return 1.0 / (1.0 + jnp.exp(-t))


def _zero_after(v):
    bits = pltpu.bitcast(v[0:8, 0:LNW], u32)
    sixteen = jnp.uint32(16)
    bits = lax.shift_right_logical(lax.shift_right_logical(bits, sixteen), sixteen)
    return pltpu.bitcast(bits, f32) if PACE else None


def _interleave(*lists):
    items = []
    for li, tasks in enumerate(lists):
        for k, t in enumerate(tasks):
            items.append(((k + 0.5) / len(tasks), li, k, t))
    items.sort(key=lambda it: it[:3])
    return [it[3] for it in items]


def _kernel(x_hbm, wq_hbm, wk_hbm, wv_hbm, wo_hbm, beta_hbm, wr_hbm, wg_hbm, wu_hbm, wd_hbm,
            out_hbm,
            beta_ref, wr_ref, x_buf, w_buf, wg_buf, wu_buf, wd_buf, out_buf,
            wt_u, kt_tmp, wot_u, xn_u, xs_a, xs_b, qs_u, k_u, pq_u, pk_u, vt_u, vwin,
            r_buf, mt_acc, lm_f, am, g16, omg, mb,
            s0, m0, s1, m1, ot0, ot1, ot2, ot3, xf, ln_stat, y_acc, xsel_buf, hid_buf, sems):

    def x_copy(i):
        c0, width = X_PIECES[i]
        return pltpu.make_async_copy(x_hbm.at[:, pl.ds(c0, width)], x_buf.at[:, pl.ds(c0, width)],
                                     sems.at[SEM_X + i])

    def w_copy(i):
        src = (wq_hbm, wk_hbm, wv_hbm, wo_hbm)[i]
        return pltpu.make_async_copy(src, w_buf.at[i], sems.at[SEM_W + i])

    wq_first = pltpu.make_async_copy(wq_hbm.at[:, 0:WQ_SPLIT], w_buf.at[0, :, 0:WQ_SPLIT], sems.at[SEM_W])
    wq_rest = pltpu.make_async_copy(wq_hbm.at[:, WQ_SPLIT:D], w_buf.at[0, :, WQ_SPLIT:D], sems.at[SEM_WQB])

    def moe_copy(i):
        src = (wg_hbm, wu_hbm, wd_hbm)[i]
        dst = (wg_buf, wu_buf, wd_buf)[i]
        return pltpu.make_async_copy(src, dst, sems.at[SEM_MOE + i])

    def out_copy(c0, width, sem):
        return pltpu.make_async_copy(out_buf.at[:, pl.ds(c0, width)], out_hbm.at[:, pl.ds(c0, width)],
                                     sems.at[SEM_OUT + sem])

    small_copies = [pltpu.make_async_copy(beta_hbm, beta_ref, sems.at[SEM_SMALL]),
                    pltpu.make_async_copy(wr_hbm, wr_ref, sems.at[SEM_SMALL + 1])]
    x_copy(0).start()
    wq_first.start()
    wq_rest.start()
    x_copy(1).start()
    for cp in small_copies:
        cp.start()
    w_copy(1).start()
    w_copy(2).start()

    init_scope = _scope("init")
    init_scope.__enter__()
    kr = lax.broadcasted_iota(i32, (HT, T), 0)
    ql = lax.broadcasted_iota(i32, (HT, T), 1)
    mb[0] = jnp.where(ql < kr, MASKVAL, 0.0).astype(f32)
    mb[1] = jnp.where((ql >= HT) & (ql - HT < kr), MASKVAL, 0.0).astype(f32)
    mb[2] = jnp.where(ql % HT < kr, MASKVAL, 0.0).astype(f32)
    zpad = jnp.zeros(((DP - D) // 2, T), u32)
    for tt in range(NT):
        xn_u[tt, D // 2:DP // 2, :] = zpad
    for tt in range(BT):
        xs_a[tt, D // 2:DP // 2, :] = zpad
        xs_b[tt, D // 2:DP // 2, :] = zpad
    ots = (ot0, ot1, ot2, ot3)
    for o_ref in ots:
        o_ref[D:DP, :] = jnp.zeros((DP - D, T), f32)
    am[0] = jnp.zeros(am.shape[1:], f32)
    mt_acc[...] = jnp.zeros(mt_acc.shape, f32)
    g16[...] = jnp.zeros(g16.shape, f32)

    init_scope.__exit__(None, None, None)

    pace = [None]

    def gate_tables():
        gate = _round_bf16(_sigmoid(beta_ref[...].reshape(1, H).astype(f32)))
        for h in range(H):
            gh = jnp.broadcast_to(gate[:, h:h + 1], (1, T))
            omg[h] = jnp.broadcast_to(_round_bf16(1.0 - gh), (8, T))
            g16[h // HPG, (h % HPG):(h % HPG) + 1, :] = gh

    def transpose_block(i, cb):
        c1 = min((cb + 1) * T, D)
        blk = w_buf[i, :, cb * T:c1]
        if c1 - cb * T < T:
            blk = jnp.concatenate([blk, jnp.zeros((D, T - (c1 - cb * T)), bf16)], axis=1)
        blk = jnp.concatenate([blk, jnp.zeros((DP - D, T), bf16)], axis=0)
        return pltpu.bitcast(blk.T, u32)

    def prep_dense(i, dst, base):
        def task(cb):
            nrow = min(TW, D // 2 - cb * TW)
            dst[base + cb * TW:base + cb * TW + nrow, :] = transpose_block(i, cb)[0:nrow]
        return [lambda cb=cb: task(cb) for cb in range(DP // T)]

    def router_row():
        wr = wr_ref[...].reshape(1, D).astype(f32)
        wr = jnp.concatenate([wr, jnp.zeros((1, DP - D), f32)], axis=1)
        bits = lax.shift_right_logical(pltpu.bitcast(wr, u32), u32(16))
        rid = lax.broadcasted_iota(i32, (8, DP), 0)
        wt_u[WT_R:WT_R + 8, :] = jnp.where(rid == 0, bits, u32(0))

    def ln_tasks(s, p, stage):
        c0 = s * L + p * LNW
        if not isinstance(s, int):
            c0 = pl.multiple_of(c0, LNW)

        def mean_pass():
            acc = pace[0]
            for r in range(0, D, 64):
                x = x_buf[r:r + 64, pl.ds(c0, LNW)].astype(f32)
                xf[p, r:r + 64, :] = x
                part = jnp.sum(x.reshape(8, 8, LNW), axis=0)
                acc = part if acc is None else acc + part
            mean = jnp.sum(acc, axis=0, keepdims=True) / D
            ln_stat[p, 0] = jnp.broadcast_to(mean, (8, LNW))

        def var_pass():
            mean = ln_stat[p, 0][0:1]
            if pace[0] is not None:
                mean = mean + pace[0][0:1]
            acc = None
            for r in range(0, D, 96):
                xc = xf[p, r:r + 96, :] - mean
                part = jnp.sum((xc * xc).reshape(12, 8, LNW), axis=0)
                acc = part if acc is None else acc + part
            var = jnp.sum(acc, axis=0, keepdims=True) / D
            den = _round_bf16(jnp.sqrt(_round_bf16(_round_bf16(var) + EPS_BF16)))
            ln_stat[p, 1] = jnp.broadcast_to(1.0 / den, (8, LNW))
            ln_stat[p, 0] = jnp.broadcast_to(_round_bf16(mean), (8, LNW))

        def norm_pass(part):
            mean_b = ln_stat[p, 0][0:1]
            if pace[0] is not None:
                mean_b = mean_b + pace[0][0:1]
            inv = ln_stat[p, 1][0:1]
            step = D // NORM_PARTS
            for r in range(part * step, (part + 1) * step, 48):
                xn = _pack(_round_bf16(xf[p, r:r + 48, :] - mean_b) * inv)
                for t in range(BT):
                    xn_u.at[s * TPS + p * BT + t][r // 2:r // 2 + 24, :] = xn[:, t * T:(t + 1) * T]
                    if stage is not None:
                        stage.at[t][r // 2:r // 2 + 24, :] = xn[:, t * T:(t + 1) * T]

        return [mean_pass, var_pass] + [lambda part=part: norm_pass(part) for part in range(NORM_PARTS)]

    def load_xs(s, p, stage):
        if stage is None:
            tiles = [xn_u[s * TPS + p * BT + t] for t in range(BT)]
        else:
            tiles = [stage[t] for t in range(BT)]
        return jnp.concatenate([_bf(t) for t in tiles], axis=1)

    def blk_rows(cb):
        return min(TW, D // 2 - cb * TW)

    def q_task(s, p, stage, cb):
        nr = blk_rows(cb)
        rows = slice(cb * TW, cb * TW + nr)
        cols = slice(p * LNW, (p + 1) * LNW)
        w = _bf(wt_u[WT_Q + cb * TW:WT_Q + cb * TW + nr, :])
        q = jnp.dot(w, load_xs(s, p, stage), preferred_element_type=f32)
        pace[0] = _zero_after(q)
        qp = _pack(q * QSCALE)
        qrot = jnp.concatenate([pltpu.roll(qp[:, t * T:(t + 1) * T], HT, 1) for t in range(BT)], axis=1)
        rid = lax.broadcasted_iota(i32, qp.shape, 0) + cb * TW
        even = ((rid // (DH // 2)) % 2) == 0
        qs_u.at[s][rows, cols] = jnp.where(even, qrot, qp)
        pq_u.at[s][rows, cols] = _pack(_phi(q))

    def k_task(s, p, stage, cb):
        nr = blk_rows(cb)
        rows = slice(cb * TW, cb * TW + nr)
        cols = slice(p * LNW, (p + 1) * LNW)
        extra = 8 if cb == NBLK - 1 else 0
        w = _bf(wt_u[WT_K + cb * TW:WT_K + cb * TW + nr + extra, :])
        k = jnp.dot(w, load_xs(s, p, stage), preferred_element_type=f32)
        pace[0] = _zero_after(k)
        if extra:
            r_buf[s, :, cols] = jnp.broadcast_to(k[2 * nr:2 * nr + 1, :], (8, LNW))
            k = k[0:2 * nr]
        kt_tmp.at[p][rows, :] = _pack(k)
        pk_u.at[s][rows, cols] = _pack(_phi(k))

    def kt_task(s, p, g):
        nv = _valid(g) // 2
        src = g * HPG * DH // 2
        kg = jnp.concatenate([kt_tmp[p, src:src + nv, :], jnp.zeros((TW - nv, LNW), u32)], axis=0)
        k_u.at[s * NG + g][p * (LNW // 2):(p + 1) * (LNW // 2), :] = pltpu.bitcast(_bf(kg).T, u32)

    def v_task(s, p, stage, b):
        cols = slice(p * LNW, (p + 1) * LNW)
        w = _bf(wt_u[WT_V + b * (VB // 2):WT_V + (b + 1) * (VB // 2), :])
        v = jnp.dot(w, load_xs(s, p, stage), preferred_element_type=f32)
        pace[0] = _zero_after(v)
        v = _pack(v)
        vt_u.at[s][b * (VB // 2):(b + 1) * (VB // 2), cols] = v
        sub = lax.broadcasted_iota(i32, (16, LNW), 0)
        for hh in range(8):
            w8 = (9 * hh) // 8
            ones_row = 0 if 2 * hh == 14 else 15
            vwin.at[s * H + 8 * b + hh][:, cols] = jnp.where(sub == ones_row, u32(ONES_PAIR), v[8 * w8:8 * w8 + 16, :])

    def q_tasks(s, p, stage=None):
        return [lambda cb=cb: q_task(s, p, stage, cb) for cb in range(NBLK)]

    def k_tasks(s, p, stage=None):
        tasks, done = [], 0
        for cb in range(NBLK):
            tasks.append(lambda cb=cb: k_task(s, p, stage, cb))
            while done < NG and done * HPG * DH + _valid(done) <= min((cb + 1) * T, D):
                tasks.append(lambda g=done: kt_task(s, p, g))
                done += 1
        return tasks

    def v_tasks(s, p, stage=None):
        return [lambda b=b: v_task(s, p, stage, b) for b in range(D // VB)]

    def mem_layout(g):
        es, eoff, _ = _ewin(g)
        nv = _valid(g)
        ne = -(-(eoff + nv) // 16) * 16
        ones_row = 0 if eoff >= 2 else eoff + nv
        nh = nv // DH
        den_row = 0 if eoff >= nh else ne
        return es, eoff, nv, ne, ones_row, den_row, max(ne, den_row + 16 * (den_row > 0))

    def mem_update(sp, g):
        es, eoff, nv, ne, ones_row, den_row, nr = mem_layout(g)
        nw = min(T, D - es)
        win = vt_u[sp, es // 2:(es + ne) // 2, :]
        wid = lax.broadcasted_iota(i32, win.shape, 0)
        lhs = _bf(jnp.where(wid == ones_row // 2, u32(ONES_PAIR), win))
        upd = lax.dot_general(lhs, _bf(pk_u[sp, es // 2:(es + nw) // 2, :]), NT_DIMS, preferred_element_type=f32)
        mt = mt_acc[g, 0:ne, 0:nw] + upd
        mt_acc[g, 0:ne, 0:nw] = mt
        z = jnp.broadcast_to(mt[ones_row:ones_row + 1, :], (nr, nw))
        if nr > ne:
            mt = jnp.concatenate([mt, jnp.zeros((nr - ne, nw), f32)], axis=0)
        row = lax.broadcasted_iota(i32, (nr, nw), 0)
        d_loc = lax.broadcasted_iota(i32, (nr, nw), 1) - eoff
        e_loc = row - eoff
        d_ok = (d_loc >= 0) & (d_loc < nv)
        same_head = (e_loc >= 0) & (e_loc < nv) & d_ok & ((e_loc // DH) == (d_loc // DH))
        den_hit = (row >= den_row) & d_ok & ((d_loc // DH) == row - den_row)
        lm_f[g, 0:nr, 0:nw] = jnp.where(same_head, mt, jnp.where(den_hit, z, 0.0))

    def mem_retrieve(s, g):
        es, eoff, nv, ne, ones_row, den_row, nr = mem_layout(g)
        nw = min(T, D - es)
        nd = jnp.dot(lm_f[g, 0:nr, 0:nw].astype(bf16), _bf(pq_u[s, es // 2:(es + nw) // 2, :]),
                     preferred_element_type=f32)
        scale = jnp.broadcast_to(g16[g][:, 0:1], (8, L)) / (nd[den_row:den_row + 8, :] + 1e-6)
        r8 = lax.broadcasted_iota(i32, (8, L), 0)
        for b in range(ne // 8):
            lo, hi = 8 * b - eoff, 8 * b + 7 - eoff
            if hi < 0 or lo >= nv:
                continue
            j1, j2 = max(lo, 0) // DH, min(hi, nv - 1) // DH
            sc = jnp.broadcast_to(scale[j1:j1 + 1, :], (8, L))
            if j2 != j1:
                sc = jnp.where(r8 < DH * j2 - lo, sc, jnp.broadcast_to(scale[j2:j2 + 1, :], (8, L)))
            val = nd[8 * b:8 * b + 8, :] * sc
            dst = am.at[s, es + 8 * b:es + 8 * b + 8, :]
            if lo >= 0 and hi < nv:
                dst[...] = val
            else:
                pltpu.store(dst, val, mask=(r8 + lo >= 0) & (r8 + lo < nv))

    def run(tasks):
        for t in tasks:
            t()

    prep_q = prep_dense(0, wt_u, WT_Q)
    q0a = q_tasks(0, 0)
    with _scope("p1_wait_x0"):
        x_copy(0).wait()
    for i in range(2, len(X_PIECES)):
        x_copy(i).start()
    w_copy(3).start()
    for i in range(3):
        moe_copy(i).start()
    with _scope("p1_ln0a"):
        run(ln_tasks(0, 0, None))
        wq_first.wait()
    with _scope("p1_q0a_first"):
        run(prep_q[0:2] + q0a[0:2])
        wq_rest.wait()
        x_copy(1).wait()
    with _scope("p1_q0a"):
        run(prep_q[2:])
        run(_interleave(q0a[2:], ln_tasks(0, 1, None)))
        w_copy(1).wait()
        for cp in small_copies:
            cp.wait()
    k0a, k0b = k_tasks(0, 0), k_tasks(0, 1)
    with _scope("p1_q0b"):
        run(_interleave(q_tasks(0, 1), prep_dense(1, wt_u, WT_K), [router_row, gate_tables]))
        run(k0a)
        w_copy(2).wait()
        x_copy(2).wait()
    with _scope("p1_k0v0"):
        run(_interleave(k0b, prep_dense(2, wt_u, WT_V)))
        run(_interleave(v_tasks(0, 0) + v_tasks(0, 1), ln_tasks(1, 0, xs_a)))

    def seg_body(s, c):
        for ss in range(2, NSEG):
            @pl.when(s + 1 == ss)
            def _():
                x_copy(ss + 1).wait()
        nxt = jnp.minimum(s + 1, NSEG - 1)
        pace[0] = None
        with _scope("p1_seg"):
            updates = [lambda g=g: mem_update(s - 1, g) for g in range(NG)]
            retrieves = [lambda g=g: mem_retrieve(s, g) for g in range(NG)]
            first = _interleave(q_tasks(s, 0, xs_a), updates) + k_tasks(s, 0, xs_a) + v_tasks(s, 0, xs_a)
            run(_interleave(first, ln_tasks(s, 1, xs_b)))
            second = q_tasks(s, 1, xs_b) + _interleave(k_tasks(s, 1, xs_b) + v_tasks(s, 1, xs_b), retrieves)
            run(_interleave(second, ln_tasks(nxt, 0, xs_a)))
        return c

    lax.fori_loop(1, NSEG, seg_body, 0)

    bufs = ((s0, m0), (s1, m1))
    lane64 = lax.broadcasted_iota(i32, (TW, T), 1)
    lane1 = lax.broadcasted_iota(i32, (1, T), 1)
    lane8 = lax.broadcasted_iota(i32, (8, T), 1)

    def pair_weights(s, pi, qt):
        hw = DH // 2
        j = 2 * (pi % (HPG // 2))
        src, dst = hw * 2 * pi, hw * j
        a0, t0 = (src // 8) * 8, (dst // 8) * 8
        nrow = min(32, D // 2 - a0)
        part = qs_u[s, a0:a0 + nrow, qt * T:(qt + 1) * T]
        if nrow < 32:
            part = jnp.concatenate([part, jnp.zeros((32 - nrow, T), u32)], axis=0)
        shift = (dst - t0) - (src - a0)
        if shift:
            part = pltpu.roll(part, shift % 32, 0)
        rid = lax.broadcasted_iota(i32, (32, T), 0) + t0
        out = []
        for lo in (dst, dst + hw):
            piece = jnp.where((rid >= lo) & (rid < lo + hw), part, u32(0))
            piece = piece[0:min(32, TW - t0)]
            pieces = [jnp.zeros((t0, T), u32)] * (t0 > 0) + [piece] + [jnp.zeros((TW - t0 - 32, T), u32)] * (t0 + 32 < TW)
            out.append(jnp.concatenate(pieces, axis=0))
        return out

    def stage_a(unit, u, qt):
        s, k = unit
        s_ref, m_ref = bufs[k % 2]
        pi = k * NP + u
        g = pi // (HPG // 2)
        sg = s * NG + g
        n = T * (qt + 1)
        w_a, w_b = pair_weights(s, pi, qt)
        w_ab = _bf(jnp.where(lane64 < HT, w_a, w_b))

        def colmax8(v):
            return jnp.max(v.reshape(v.shape[0] // 8, 8, T), axis=0)

        maxes = []
        for hd, w in enumerate((_bf(w_a), _bf(w_b))):
            m8 = None
            for c in range(qt):
                kc = _bf(k_u[sg, c * TW:(c + 1) * TW, :])
                sc = jnp.dot(kc, w, preferred_element_type=f32)
                s_ref[u, qt, hd * L + c * T:hd * L + (c + 1) * T, :] = sc
                m8 = colmax8(sc) if m8 is None else jnp.maximum(m8, colmax8(sc))
            kc = _bf(k_u[sg, qt * TW:qt * TW + TW // 2, :])
            sc = jnp.dot(kc, w, preferred_element_type=f32) + mb[1 - hd]
            s_ref[u, qt, hd * L + qt * T:hd * L + qt * T + HT, :] = sc
            m8 = colmax8(sc) if m8 is None else jnp.maximum(m8, colmax8(sc))
            maxes.append(m8)
        kc = _bf(k_u[sg, qt * TW + TW // 2:(qt + 1) * TW, :])
        sc = jnp.dot(kc, w_ab, preferred_element_type=f32) + mb[2]
        s_ref[u, qt, n - HT:n, :] = sc
        mab = colmax8(sc)
        m_a = jnp.where(lane8 < HT, jnp.maximum(maxes[0], mab), maxes[0])
        m_b = jnp.where(lane8 >= HT, jnp.maximum(maxes[1], mab), maxes[1])
        m_ref[u, qt, 0] = jnp.broadcast_to(jnp.max(m_a, axis=0, keepdims=True), (8, T))
        m_ref[u, qt, 1] = jnp.broadcast_to(jnp.max(m_b, axis=0, keepdims=True), (8, T))

    def stage_b(unit, u, qt):
        s, k = unit
        s_ref, m_ref = bufs[k % 2]
        pi = k * NP + u
        n = T * (qt + 1)
        m_a = m_ref[u, qt, 0][0:1]
        m_b = m_ref[u, qt, 1][0:1]
        p_ab = jnp.exp2(s_ref[u, qt, n - HT:n, :] - jnp.where(lane1 < HT, m_a, m_b))
        for hd, m in enumerate((m_a, m_b)):
            h = 2 * pi + hd
            p = jnp.exp2(s_ref[u, qt, hd * L:hd * L + n - HT, :] - m)
            keep = (lane64 < HT) if hd == 0 else (lane64 >= HT)
            p = jnp.concatenate([p, jnp.where(keep, p_ab, 0.0)], axis=0).astype(bf16)
            w0 = ((DH * h) // 16) * 16
            off = DH * h - w0
            o = jnp.dot(_bf(vwin[s * H + h, :, 0:n]), p, preferred_element_type=f32)
            den = o[0:1] if off == 14 else o[31:32]
            r0, r1 = (off // 8) * 8, -(-(off + DH) // 8) * 8
            o = o[r0:r1] * (omg[h][0:1] / den)
            if hd == 0:
                o = pltpu.roll(o, HT, 1)
            res = am[s, w0 + r0:w0 + r1, qt * T:(qt + 1) * T] + o
            rid = lax.broadcasted_iota(i32, (r1 - r0, T), 0) + r0
            pltpu.store(ots[qt].at[w0 + r0:w0 + r1, :], res, mask=(rid >= off) & (rid < off + DH))

    def a_tasks(unit):
        return [lambda u=u, qt=qt: stage_a(unit, u, qt) for u in range(NP) for qt in QT_ORDER]

    def b_tasks(unit):
        return [lambda u=u, qt=qt: stage_b(unit, u, qt) for u in range(NP) for qt in QT_ORDER]

    w_copy(3).wait()
    rr = jnp.concatenate([r_buf[s][0:1, :] for s in range(NSEG)], axis=0)
    rr = _round_bf16(rr)
    tok = lax.broadcasted_iota(i32, (NSEG, L), 0) * L + lax.broadcasted_iota(i32, (NSEG, L), 1)
    m1v = jnp.max(rr)
    i1 = jnp.min(jnp.where(rr == m1v, tok, SEQ))
    rr2 = jnp.where(tok == i1, -jnp.inf, rr)
    m2v = jnp.max(rr2)
    i2 = jnp.min(jnp.where(rr2 == m2v, tok, SEQ))
    i1 = jnp.clip(i1, 0, SEQ - 1)
    i2 = jnp.clip(i2, 0, SEQ - 1)

    row16 = lax.broadcasted_iota(i32, (16, T), 0)
    lane16 = lax.broadcasted_iota(i32, (16, T), 1)

    def token_rows(i, slot):
        onehot = jnp.where((row16 == slot) & (lane16 == i % T), 1.0, 0.0).astype(bf16)
        return lax.dot_general(onehot, _bf(xn_u[i // T]), NT_DIMS, preferred_element_type=f32)

    def select_task():
        xsel_buf[...] = _pack(token_rows(i1, 0) + token_rows(i2, 1))
        y_acc[...] = jnp.zeros(y_acc.shape, f32)

    def fcols(ft):
        return pl.ds(ft * T if isinstance(ft, int) else pl.multiple_of(ft * T, T), T)

    def moe_up_task(ft, k, which):
        xsel = _bf(xsel_buf[:, 0:D])
        w_ref = (wg_buf, wu_buf)[which]
        hid_buf[k, which] = jnp.dot(xsel, w_ref[:, fcols(ft)], preferred_element_type=f32)

    def moe_down_task(ft, k):
        gt = _round_bf16(hid_buf[k, 0])
        up = _round_bf16(hid_buf[k, 1])
        hid = (_round_bf16(gt * _sigmoid(gt)) * up).astype(bf16)
        y_acc[...] += lax.dot_general(hid, wd_buf[:, fcols(ft)], NT_DIMS, preferred_element_type=f32)

    def moe_tasks(ft0, count):
        tasks = []
        for k0 in range(0, count, FPB):
            ks = range(k0, min(k0 + FPB, count))
            tasks += [lambda k=k, w=w: moe_up_task(ft0 + k, k, w) for k in ks for w in range(2)]
            tasks += [lambda k=k: moe_down_task(ft0 + k, k) for k in ks]
        return tasks

    def moe_finish():
        y = _round_bf16(y_acc[...])
        rsel = jnp.where(lax.broadcasted_iota(i32, (16, 1), 0) == 0, m1v, m2v)
        y = _round_bf16(y * _round_bf16(_sigmoid(rsel)))
        y = jnp.concatenate([y, jnp.zeros((16, DP - D), f32)], axis=1)
        y = jnp.concatenate([jnp.zeros((HT, DP), f32), y, jnp.zeros((T - HT - 16, DP), f32)], axis=0)
        y_t = jnp.concatenate([y.T[0:D], jnp.zeros((D, T), f32)], axis=1)
        y_u = _pack(y_t)[:, 0:T]
        lane = lax.broadcasted_iota(i32, (D // 2, T), 1)
        wot_u[:, DP - T:DP] = jnp.where(lane < HT, wot_u[:, DP - T:DP], y_u)
        rid = lax.broadcasted_iota(i32, (8, T), 0)
        for tt in range(TPS):
            tok_l = lax.broadcasted_iota(i32, (8, T), 1) + (NSEG - 1) * L + tt * T
            ots[tt][D:D + 8, :] = jnp.where(((rid == 0) & (tok_l == i1)) | ((rid == 1) & (tok_l == i2)), 1.0, 0.0)

    dense = _interleave(a_tasks((0, 0)), prep_dense(3, wot_u, 0))
    with _scope("p15_mix"):
        cut = (2 * len(dense)) // 3
        run(dense[:cut] + [select_task] + dense[cut:])

    for i in range(3):
        moe_copy(i).wait()

    def out_tile(s, tt, last, chunk_copies=None):
        c0 = s * L + tt * T
        if not isinstance(s, int):
            c0 = pl.multiple_of(c0, T)
        o_bf = ots[tt][...].astype(bf16)
        nchunk = 4
        rows = D // nchunk
        for rc in range(nchunk):
            r0 = rc * rows
            attn = jnp.dot(_bf(wot_u[r0 // 2:(r0 + rows) // 2, :]), o_bf, preferred_element_type=f32)
            xn = _bf(xn_u[s * TPS + tt, r0 // 2:(r0 + rows) // 2, :]).astype(f32)
            x = x_buf[r0:r0 + rows, pl.ds(c0, T)].astype(f32)
            res = x + attn + xn
            out_buf[r0:r0 + rows, pl.ds(c0, T)] = res.astype(bf16)
            if chunk_copies is not None:
                chunk_copies[rc].start()

    def pair_tasks(ua, ub):
        tasks = []
        for x, y in zip(a_tasks(ua), b_tasks(ub)):
            tasks += [y, x]
        return tasks

    def seg_end(s, last):
        def by_qt(fn, unit, qt):
            return [lambda u=u: fn(unit, u, qt) for u in range(NP)]

        steps = []
        for step in range(7):
            lists = []
            if step < 4:
                lists.append(by_qt(stage_b, (s, 2), 3 - step))
                lists.append(by_qt(stage_a, (s, 3), 3 - step))
            if 1 <= step < 5:
                lists.append(by_qt(stage_b, (s, 3), 4 - step))
            if not last and 2 <= step < 6:
                lists.append(by_qt(stage_a, (s + 1, 0), 5 - step))
            if step >= 3:
                lists.append([lambda tt=6 - step: out_tile(s, tt, last)])
            steps.append(_interleave(*lists))
        return steps

    def seg_att(s, c):
        tasks = pair_tasks((s, 1), (s, 0)) + pair_tasks((s, 2), (s, 1))
        steps = seg_end(s, False)
        for step in steps[0:5]:
            tasks += step
        with _scope("att_seg"):
            run(_interleave(tasks, moe_tasks(s * FPI, FPI)))
            for step in steps[5:]:
                run(step)

        @pl.when(s < NSEG - 2)
        def _():
            out_copy(pl.multiple_of(s * L, L), L, s).start()
        return c

    lax.fori_loop(0, NSEG - 1, seg_att, 0)

    npatch = (NSEG - 1) * TPS

    def patch_tile(idx):
        return jnp.where(idx < npatch * T, idx // T, 0)

    tile0 = patch_tile(i1)
    tile1 = patch_tile(i2)
    tile1 = jnp.where(tile1 == tile0, (tile0 + 1) % npatch, tile1)

    def patch(tile):
        c0 = pl.multiple_of(tile * T, T)
        rid = lax.broadcasted_iota(i32, (T, T), 0)
        tok_l = lax.broadcasted_iota(i32, (T, T), 1) + c0
        hit = ((rid == HT) & (tok_l == i1)) | ((rid == HT + 1) & (tok_l == i2))
        onehot = jnp.where(hit, 1.0, 0.0).astype(bf16)
        for rc in range(4):
            r0, r1 = rc * (D // 4), (rc + 1) * (D // 4)
            upd = jnp.dot(_bf(wot_u[r0 // 2:r1 // 2, DP - T:DP]), onehot, preferred_element_type=f32)
            cur = out_buf[r0:r1, pl.ds(c0, T)].astype(f32)
            out_buf[r0:r1, pl.ds(c0, T)] = (cur + upd).astype(bf16)

    sent = (NSEG - 2) * TPS
    resend0 = jnp.where(tile0 < sent, tile0, jnp.where(tile1 == 0, 1, 0))
    resend1 = jnp.where(tile1 < sent, tile1, jnp.where(resend0 == 0, 1, 0))
    patch_copies = [out_copy(pl.multiple_of(resend0 * T, T), T, 7), out_copy(pl.multiple_of(resend1 * T, T), T, 8),
                    out_copy((NSEG - 2) * L, L, NSEG - 2)]
    last_copies = [out_copy((NSEG - 1) * L + tt * T, T, NSEG - 1 + tt) for tt in range(1, TPS)]
    c_fin = (NSEG - 1) * L
    final_copies = [
        pltpu.make_async_copy(out_buf.at[rc * (D // 4):(rc + 1) * (D // 4), c_fin:c_fin + T],
                              out_hbm.at[rc * (D // 4):(rc + 1) * (D // 4), c_fin:c_fin + T],
                              sems.at[SEM_FINAL + rc]) for rc in range(4)]

    sl = NSEG - 1
    for s in range(NSEG - 2):
        out_copy(s * L, L, s).wait()
    with _scope("tail_2"):
        moe_finish()
        run(pair_tasks((sl, 1), (sl, 0)))
        patch(tile0)
        patch(tile1)
        run(pair_tasks((sl, 2), (sl, 1)))
        for cp in patch_copies:
            cp.start()
        steps = seg_end(sl, True)
        for step in steps[0:5]:
            run(step)
        last_copies[2].start()
        last_copies[1].start()
    with _scope("tail_3"):
        run(steps[5])
        last_copies[0].start()
        out_tile(sl, 0, True, final_copies)

    with _scope("out_wait"):
        for cp in patch_copies + last_copies + final_copies:
            cp.wait()


@jax.jit
def pallas_parallel_sum__memory_aug_infini_attn__moe_arch_mod__prompt_kernel(
    A_x: jax.Array,
    A_wq: jax.Array,
    A_wk: jax.Array,
    A_wv: jax.Array,
    A_wo: jax.Array,
    A_beta: jax.Array,
    B_x: jax.Array,
    B_w_r: jax.Array,
    B_w_gate: jax.Array,
    B_w_up: jax.Array,
    B_w_down: jax.Array,
):
    del B_x
    any_spec = pl.BlockSpec(memory_space=pl.ANY)
    scratch = [
        pltpu.VMEM((H,), bf16),
        pltpu.VMEM((D,), bf16),
        pltpu.VMEM((D, SEQ), bf16),
        pltpu.VMEM((4, D, D), bf16),
        pltpu.VMEM((D, F), bf16),
        pltpu.VMEM((D, F), bf16),
        pltpu.VMEM((D, F), bf16),
        pltpu.VMEM((D, SEQ), bf16),
        pltpu.VMEM((WT_ALLOC, DP), u32),
        pltpu.VMEM((2, D // 2, LNW), u32),
        pltpu.VMEM((D // 2, DP), u32),
        pltpu.VMEM((NT, DP // 2, T), u32),
        pltpu.VMEM((BT, DP // 2, T), u32),
        pltpu.VMEM((BT, DP // 2, T), u32),
        pltpu.VMEM((NSEG, D // 2, L), u32),
        pltpu.VMEM((NSEG * NG, L // 2, T), u32),
        pltpu.VMEM((NSEG, D // 2, L), u32),
        pltpu.VMEM((NSEG, D // 2, L), u32),
        pltpu.VMEM((NSEG, D // 2, L), u32),
        pltpu.VMEM((NSEG * H, 16, L), u32),
        pltpu.VMEM((NSEG, 8, L), f32),
        pltpu.VMEM((NG, T, T), f32),
        pltpu.VMEM((NG, T, T), f32),
        pltpu.VMEM((NSEG, D, L), f32),
        pltpu.VMEM((NG, 8, T), f32),
        pltpu.VMEM((H, 8, T), f32),
        pltpu.VMEM((3, HT, T), f32),
        pltpu.VMEM((NP, 4, 2 * L, T), f32),
        pltpu.VMEM((NP, 4, 2, 8, T), f32),
        pltpu.VMEM((NP, 4, 2 * L, T), f32),
        pltpu.VMEM((NP, 4, 2, 8, T), f32),
        pltpu.VMEM((DP, T), f32),
        pltpu.VMEM((DP, T), f32),
        pltpu.VMEM((DP, T), f32),
        pltpu.VMEM((DP, T), f32),
        pltpu.VMEM((2, D, LNW), f32),
        pltpu.VMEM((2, 2, 8, LNW), f32),
        pltpu.VMEM((16, D), f32),
        pltpu.VMEM((8, DP), u32),
        pltpu.VMEM((FPI, 2, 16, T), f32),
        pltpu.SemaphoreType.DMA((NSEM,)),
    ]
    x_t = jnp.transpose(A_x, (0, 2, 1)).reshape(D, SEQ)
    out_t = pl.pallas_call(
        _kernel,
        out_shape=jax.ShapeDtypeStruct((D, SEQ), bf16),
        in_specs=[any_spec] * 10,
        out_specs=any_spec,
        scratch_shapes=scratch,
        compiler_params=pltpu.CompilerParams(vmem_limit_bytes=110 * 1024 * 1024),
    )(x_t, A_wq, A_wk, A_wv, A_wo, A_beta, B_w_r, B_w_gate, B_w_up, B_w_down.T)
    return jnp.transpose(out_t.reshape(1, D, SEQ), (0, 2, 1))
```

```python
import contextlib

import jax
import jax.numpy as jnp
from jax import lax
from jax.experimental import pallas as pl
from jax.experimental.pallas import tpu as pltpu

bf16 = jnp.bfloat16
f32 = jnp.float32
u32 = jnp.uint32
i32 = jnp.int32

SEQ = 2048
D = 576
DP = 640
H = 32
DH = 18
NSEG = 4
L = 512
T = 128
TW = T // 2
HT = T // 2
TPS = L // T
HPG = 6
NG = 6
F = 4608
FPI = 12
FPB = 3
NFT = F // T
NP = 4
UPS = H // (2 * NP)
NUNIT = NSEG * UPS
NT = SEQ // T
LNW = 256
BT = LNW // T
NORM_PARTS = 6
VB = 8 * DH

LOG2E = 1.4426950408889634
QSCALE = (DH ** -0.5) * LOG2E
MASKVAL = -1000000000.0 * LOG2E
EPS_BF16 = 1.0013580322265625e-05
ONES_PAIR = 0x3F803F80

NT_DIMS = (((1,), (1,)), ((), ()))

WT_Q = 0
WT_K = D // 2
WT_R = D
WT_V = D + 8
WT_ROWS = WT_V + D // 2
WT_ALLOC = 1056
NBLK = DP // T

X_PIECES = ((0, LNW), (LNW, LNW), (L, L), (2 * L, L), (3 * L, L))
SEM_X = 0
SEM_W = 5
SEM_MOE = 9
SEM_OUT = 12
SEM_SMALL = 21
SEM_WQB = 23
SEM_FINAL = 24
NSEM = 28
WQ_SPLIT = 2 * T


PROFILE_SCOPES = False
PACE = True
TAIL_BARRIERS = False
QT_ORDER = (3, 2, 1, 0)


def _scope(name):
    return jax.named_scope(name) if PROFILE_SCOPES else contextlib.nullcontext()


def _valid(g):
    return min(HPG * DH, D - g * HPG * DH)


def _ewin(g):
    start = (g * HPG * DH // 16) * 16
    return start, g * HPG * DH - start, min(T, D - start)


def _bf(x):
    return pltpu.bitcast(x, bf16)


def _pack(x):
    return pltpu.bitcast(x.astype(bf16), u32)


def _round_bf16(x):
    return x.astype(bf16).astype(f32)


def _phi(t):
    return jnp.where(t > 0, t + 1.0, jnp.exp(t))


def _sigmoid(t):
    return 1.0 / (1.0 + jnp.exp(-t))


def _zero_after(v):
    bits = pltpu.bitcast(v[0:8, 0:LNW], u32)
    sixteen = jnp.uint32(16)
    bits = lax.shift_right_logical(lax.shift_right_logical(bits, sixteen), sixteen)
    return pltpu.bitcast(bits, f32) if PACE else None


def _interleave(*lists):
    items = []
    for li, tasks in enumerate(lists):
        for k, t in enumerate(tasks):
            items.append(((k + 0.5) / len(tasks), li, k, t))
    items.sort(key=lambda it: it[:3])
    return [it[3] for it in items]


def _kernel(x_hbm, wq_hbm, wk_hbm, wv_hbm, wo_hbm, beta_hbm, wr_hbm, wg_hbm, wu_hbm, wd_hbm,
            out_hbm,
            beta_ref, wr_ref, x_buf, w_buf, wg_buf, wu_buf, wd_buf, out_buf,
            wt_u, kt_tmp, wot_u, xn_u, xs_a, xs_b, qs_u, k_u, pq_u, pk_u, vt_u, vwin,
            r_buf, mt_acc, lm_f, am, g16, omg, mb,
            s0, m0, s1, m1, ot0, ot1, ot2, ot3, xf, ln_stat, y_acc, xsel_buf, hid_buf, sems):

    def x_copy(i):
        c0, width = X_PIECES[i]
        return pltpu.make_async_copy(x_hbm.at[:, pl.ds(c0, width)], x_buf.at[:, pl.ds(c0, width)],
                                     sems.at[SEM_X + i])

    def w_copy(i):
        src = (wq_hbm, wk_hbm, wv_hbm, wo_hbm)[i]
        return pltpu.make_async_copy(src, w_buf.at[i], sems.at[SEM_W + i])

    wq_first = pltpu.make_async_copy(wq_hbm.at[:, 0:WQ_SPLIT], w_buf.at[0, :, 0:WQ_SPLIT], sems.at[SEM_W])
    wq_rest = pltpu.make_async_copy(wq_hbm.at[:, WQ_SPLIT:D], w_buf.at[0, :, WQ_SPLIT:D], sems.at[SEM_WQB])

    moe_src = (wg_hbm, wu_hbm, wd_hbm)
    moe_dst = (wg_buf, wu_buf, wd_buf)

    def moe_start(i, ft):
        c0 = ft * T if isinstance(ft, int) else pl.multiple_of(ft * T, T)
        pltpu.make_async_copy(moe_src[i].at[:, pl.ds(c0, T)], moe_dst[i].at[ft], sems.at[SEM_MOE + i]).start()

    def moe_issue(first, last):
        for n in range(first, last):
            moe_start(n % 3, n // 3)

    def moe_wait(i):
        pltpu.make_async_copy(moe_dst[i], moe_dst[i], sems.at[SEM_MOE + i]).wait()

    def out_copy(c0, width, sem):
        return pltpu.make_async_copy(out_buf.at[:, pl.ds(c0, width)], out_hbm.at[:, pl.ds(c0, width)],
                                     sems.at[SEM_OUT + sem])

    small_copies = [pltpu.make_async_copy(beta_hbm, beta_ref, sems.at[SEM_SMALL]),
                    pltpu.make_async_copy(wr_hbm, wr_ref, sems.at[SEM_SMALL + 1])]
    x_copy(0).start()
    wq_first.start()
    wq_rest.start()
    x_copy(1).start()
    for cp in small_copies:
        cp.start()
    w_copy(1).start()
    w_copy(2).start()

    init_scope = _scope("init")
    init_scope.__enter__()
    kr = lax.broadcasted_iota(i32, (HT, T), 0)
    ql = lax.broadcasted_iota(i32, (HT, T), 1)
    mb[0] = jnp.where(ql < kr, MASKVAL, 0.0).astype(f32)
    mb[1] = jnp.where((ql >= HT) & (ql - HT < kr), MASKVAL, 0.0).astype(f32)
    mb[2] = jnp.where(ql % HT < kr, MASKVAL, 0.0).astype(f32)
    zpad = jnp.zeros(((DP - D) // 2, T), u32)
    for tt in range(NT):
        xn_u[tt, D // 2:DP // 2, :] = zpad
    for tt in range(BT):
        xs_a[tt, D // 2:DP // 2, :] = zpad
        xs_b[tt, D // 2:DP // 2, :] = zpad
    ots = (ot0, ot1, ot2, ot3)
    for o_ref in ots:
        o_ref[D:DP, :] = jnp.zeros((DP - D, T), f32)
    am[0] = jnp.zeros(am.shape[1:], f32)
    mt_acc[...] = jnp.zeros(mt_acc.shape, f32)
    g16[...] = jnp.zeros(g16.shape, f32)

    init_scope.__exit__(None, None, None)

    pace = [None]

    def gate_tables():
        gate = _round_bf16(_sigmoid(beta_ref[...].reshape(1, H).astype(f32)))
        for h in range(H):
            gh = jnp.broadcast_to(gate[:, h:h + 1], (1, T))
            omg[h] = jnp.broadcast_to(_round_bf16(1.0 - gh), (8, T))
            g16[h // HPG, (h % HPG):(h % HPG) + 1, :] = gh

    def transpose_block(i, cb):
        c1 = min((cb + 1) * T, D)
        blk = w_buf[i, :, cb * T:c1]
        if c1 - cb * T < T:
            blk = jnp.concatenate([blk, jnp.zeros((D, T - (c1 - cb * T)), bf16)], axis=1)
        blk = jnp.concatenate([blk, jnp.zeros((DP - D, T), bf16)], axis=0)
        return pltpu.bitcast(blk.T, u32)

    def prep_dense(i, dst, base):
        def task(cb):
            nrow = min(TW, D // 2 - cb * TW)
            dst[base + cb * TW:base + cb * TW + nrow, :] = transpose_block(i, cb)[0:nrow]
        return [lambda cb=cb: task(cb) for cb in range(DP // T)]

    def router_row():
        wr = wr_ref[...].reshape(1, D).astype(f32)
        wr = jnp.concatenate([wr, jnp.zeros((1, DP - D), f32)], axis=1)
        bits = lax.shift_right_logical(pltpu.bitcast(wr, u32), u32(16))
        rid = lax.broadcasted_iota(i32, (8, DP), 0)
        wt_u[WT_R:WT_R + 8, :] = jnp.where(rid == 0, bits, u32(0))

    def ln_tasks(s, p, stage):
        c0 = s * L + p * LNW
        if not isinstance(s, int):
            c0 = pl.multiple_of(c0, LNW)

        def mean_pass():
            acc = pace[0]
            for r in range(0, D, 64):
                x = x_buf[r:r + 64, pl.ds(c0, LNW)].astype(f32)
                xf[p, r:r + 64, :] = x
                part = jnp.sum(x.reshape(8, 8, LNW), axis=0)
                acc = part if acc is None else acc + part
            mean = jnp.sum(acc, axis=0, keepdims=True) / D
            ln_stat[p, 0] = jnp.broadcast_to(mean, (8, LNW))

        def var_pass():
            mean = ln_stat[p, 0][0:1]
            if pace[0] is not None:
                mean = mean + pace[0][0:1]
            acc = None
            for r in range(0, D, 96):
                xc = xf[p, r:r + 96, :] - mean
                part = jnp.sum((xc * xc).reshape(12, 8, LNW), axis=0)
                acc = part if acc is None else acc + part
            var = jnp.sum(acc, axis=0, keepdims=True) / D
            den = _round_bf16(jnp.sqrt(_round_bf16(_round_bf16(var) + EPS_BF16)))
            ln_stat[p, 1] = jnp.broadcast_to(1.0 / den, (8, LNW))
            ln_stat[p, 0] = jnp.broadcast_to(_round_bf16(mean), (8, LNW))

        def norm_pass(part):
            mean_b = ln_stat[p, 0][0:1]
            if pace[0] is not None:
                mean_b = mean_b + pace[0][0:1]
            inv = ln_stat[p, 1][0:1]
            step = D // NORM_PARTS
            for r in range(part * step, (part + 1) * step, 48):
                xn = _pack(_round_bf16(xf[p, r:r + 48, :] - mean_b) * inv)
                for t in range(BT):
                    xn_u.at[s * TPS + p * BT + t][r // 2:r // 2 + 24, :] = xn[:, t * T:(t + 1) * T]
                    if stage is not None:
                        stage.at[t][r // 2:r // 2 + 24, :] = xn[:, t * T:(t + 1) * T]

        return [mean_pass, var_pass] + [lambda part=part: norm_pass(part) for part in range(NORM_PARTS)]

    def load_xs(s, p, stage):
        if stage is None:
            tiles = [xn_u[s * TPS + p * BT + t] for t in range(BT)]
        else:
            tiles = [stage[t] for t in range(BT)]
        return jnp.concatenate([_bf(t) for t in tiles], axis=1)

    def blk_rows(cb):
        return min(TW, D // 2 - cb * TW)

    def q_task(s, p, stage, cb):
        nr = blk_rows(cb)
        rows = slice(cb * TW, cb * TW + nr)
        cols = slice(p * LNW, (p + 1) * LNW)
        w = _bf(wt_u[WT_Q + cb * TW:WT_Q + cb * TW + nr, :])
        q = jnp.dot(w, load_xs(s, p, stage), preferred_element_type=f32)
        pace[0] = _zero_after(q)
        qp = _pack(q * QSCALE)
        qrot = jnp.concatenate([pltpu.roll(qp[:, t * T:(t + 1) * T], HT, 1) for t in range(BT)], axis=1)
        rid = lax.broadcasted_iota(i32, qp.shape, 0) + cb * TW
        even = ((rid // (DH // 2)) % 2) == 0
        qs_u.at[s][rows, cols] = jnp.where(even, qrot, qp)
        pq_u.at[s][rows, cols] = _pack(_phi(q))

    def k_task(s, p, stage, cb):
        nr = blk_rows(cb)
        rows = slice(cb * TW, cb * TW + nr)
        cols = slice(p * LNW, (p + 1) * LNW)
        extra = 8 if cb == NBLK - 1 else 0
        w = _bf(wt_u[WT_K + cb * TW:WT_K + cb * TW + nr + extra, :])
        k = jnp.dot(w, load_xs(s, p, stage), preferred_element_type=f32)
        pace[0] = _zero_after(k)
        if extra:
            r_buf[s, :, cols] = jnp.broadcast_to(k[2 * nr:2 * nr + 1, :], (8, LNW))
            k = k[0:2 * nr]
        kt_tmp.at[p][rows, :] = _pack(k)
        pk_u.at[s][rows, cols] = _pack(_phi(k))

    def kt_task(s, p, g):
        nv = _valid(g) // 2
        src = g * HPG * DH // 2
        kg = jnp.concatenate([kt_tmp[p, src:src + nv, :], jnp.zeros((TW - nv, LNW), u32)], axis=0)
        k_u.at[s * NG + g][p * (LNW // 2):(p + 1) * (LNW // 2), :] = pltpu.bitcast(_bf(kg).T, u32)

    def v_task(s, p, stage, b):
        cols = slice(p * LNW, (p + 1) * LNW)
        w = _bf(wt_u[WT_V + b * (VB // 2):WT_V + (b + 1) * (VB // 2), :])
        v = jnp.dot(w, load_xs(s, p, stage), preferred_element_type=f32)
        pace[0] = _zero_after(v)
        v = _pack(v)
        vt_u.at[s][b * (VB // 2):(b + 1) * (VB // 2), cols] = v
        sub = lax.broadcasted_iota(i32, (16, LNW), 0)
        for hh in range(8):
            w8 = (9 * hh) // 8
            ones_row = 0 if 2 * hh == 14 else 15
            vwin.at[s * H + 8 * b + hh][:, cols] = jnp.where(sub == ones_row, u32(ONES_PAIR), v[8 * w8:8 * w8 + 16, :])

    def q_tasks(s, p, stage=None):
        return [lambda cb=cb: q_task(s, p, stage, cb) for cb in range(NBLK)]

    def k_tasks(s, p, stage=None):
        tasks, done = [], 0
        for cb in range(NBLK):
            tasks.append(lambda cb=cb: k_task(s, p, stage, cb))
            while done < NG and done * HPG * DH + _valid(done) <= min((cb + 1) * T, D):
                tasks.append(lambda g=done: kt_task(s, p, g))
                done += 1
        return tasks

    def v_tasks(s, p, stage=None):
        return [lambda b=b: v_task(s, p, stage, b) for b in range(D // VB)]

    def mem_layout(g):
        es, eoff, _ = _ewin(g)
        nv = _valid(g)
        ne = -(-(eoff + nv) // 16) * 16
        ones_row = 0 if eoff >= 2 else eoff + nv
        nh = nv // DH
        den_row = 0 if eoff >= nh else ne
        return es, eoff, nv, ne, ones_row, den_row, max(ne, den_row + 16 * (den_row > 0))

    def mem_update(sp, g):
        es, eoff, nv, ne, ones_row, den_row, nr = mem_layout(g)
        nw = min(T, D - es)
        win = vt_u[sp, es // 2:(es + ne) // 2, :]
        wid = lax.broadcasted_iota(i32, win.shape, 0)
        lhs = _bf(jnp.where(wid == ones_row // 2, u32(ONES_PAIR), win))
        upd = lax.dot_general(lhs, _bf(pk_u[sp, es // 2:(es + nw) // 2, :]), NT_DIMS, preferred_element_type=f32)
        mt = mt_acc[g, 0:ne, 0:nw] + upd
        mt_acc[g, 0:ne, 0:nw] = mt
        z = jnp.broadcast_to(mt[ones_row:ones_row + 1, :], (nr, nw))
        if nr > ne:
            mt = jnp.concatenate([mt, jnp.zeros((nr - ne, nw), f32)], axis=0)
        row = lax.broadcasted_iota(i32, (nr, nw), 0)
        d_loc = lax.broadcasted_iota(i32, (nr, nw), 1) - eoff
        e_loc = row - eoff
        d_ok = (d_loc >= 0) & (d_loc < nv)
        same_head = (e_loc >= 0) & (e_loc < nv) & d_ok & ((e_loc // DH) == (d_loc // DH))
        den_hit = (row >= den_row) & d_ok & ((d_loc // DH) == row - den_row)
        lm_f[g, 0:nr, 0:nw] = jnp.where(same_head, mt, jnp.where(den_hit, z, 0.0))

    def mem_retrieve(s, g):
        es, eoff, nv, ne, ones_row, den_row, nr = mem_layout(g)
        nw = min(T, D - es)
        nd = jnp.dot(lm_f[g, 0:nr, 0:nw].astype(bf16), _bf(pq_u[s, es // 2:(es + nw) // 2, :]),
                     preferred_element_type=f32)
        scale = jnp.broadcast_to(g16[g][:, 0:1], (8, L)) / (nd[den_row:den_row + 8, :] + 1e-6)
        r8 = lax.broadcasted_iota(i32, (8, L), 0)
        for b in range(ne // 8):
            lo, hi = 8 * b - eoff, 8 * b + 7 - eoff
            if hi < 0 or lo >= nv:
                continue
            j1, j2 = max(lo, 0) // DH, min(hi, nv - 1) // DH
            sc = jnp.broadcast_to(scale[j1:j1 + 1, :], (8, L))
            if j2 != j1:
                sc = jnp.where(r8 < DH * j2 - lo, sc, jnp.broadcast_to(scale[j2:j2 + 1, :], (8, L)))
            val = nd[8 * b:8 * b + 8, :] * sc
            dst = am.at[s, es + 8 * b:es + 8 * b + 8, :]
            if lo >= 0 and hi < nv:
                dst[...] = val
            else:
                pltpu.store(dst, val, mask=(r8 + lo >= 0) & (r8 + lo < nv))

    def run(tasks):
        for t in tasks:
            t()

    prep_q = prep_dense(0, wt_u, WT_Q)
    q0a = q_tasks(0, 0)
    with _scope("p1_wait_x0"):
        x_copy(0).wait()
    for i in range(2, len(X_PIECES)):
        x_copy(i).start()
    w_copy(3).start()
    moe_issue(0, 48)
    with _scope("p1_ln0a"):
        run(ln_tasks(0, 0, None))
        wq_first.wait()
    with _scope("p1_q0a_first"):
        run(prep_q[0:2] + q0a[0:2])
        wq_rest.wait()
        x_copy(1).wait()
    with _scope("p1_q0a"):
        run(prep_q[2:])
        run(_interleave(q0a[2:], ln_tasks(0, 1, None)))
        w_copy(1).wait()
        for cp in small_copies:
            cp.wait()
    k0a, k0b = k_tasks(0, 0), k_tasks(0, 1)
    with _scope("p1_q0b"):
        run(_interleave(q_tasks(0, 1), prep_dense(1, wt_u, WT_K), [router_row, gate_tables]))
        run(k0a)
        w_copy(2).wait()
        x_copy(2).wait()
    moe_issue(48, 60)
    with _scope("p1_k0v0"):
        run(_interleave(k0b, prep_dense(2, wt_u, WT_V)))
        run(_interleave(v_tasks(0, 0) + v_tasks(0, 1), ln_tasks(1, 0, xs_a)))

    moe_issue(60, 72)

    def seg_body(s, c):
        for ss in range(2, NSEG):
            @pl.when(s + 1 == ss)
            def _():
                x_copy(ss + 1).wait()
                if ss == NSEG - 1:
                    moe_issue(72, 3 * NFT)
        nxt = jnp.minimum(s + 1, NSEG - 1)
        pace[0] = None
        with _scope("p1_seg"):
            updates = [lambda g=g: mem_update(s - 1, g) for g in range(NG)]
            retrieves = [lambda g=g: mem_retrieve(s, g) for g in range(NG)]
            first = _interleave(q_tasks(s, 0, xs_a), updates) + k_tasks(s, 0, xs_a) + v_tasks(s, 0, xs_a)
            run(_interleave(first, ln_tasks(s, 1, xs_b)))
            second = q_tasks(s, 1, xs_b) + _interleave(k_tasks(s, 1, xs_b) + v_tasks(s, 1, xs_b), retrieves)
            run(_interleave(second, ln_tasks(nxt, 0, xs_a)))
        return c

    lax.fori_loop(1, NSEG, seg_body, 0)

    bufs = ((s0, m0), (s1, m1))
    lane64 = lax.broadcasted_iota(i32, (TW, T), 1)
    lane1 = lax.broadcasted_iota(i32, (1, T), 1)
    lane8 = lax.broadcasted_iota(i32, (8, T), 1)

    def pair_weights(s, pi, qt):
        hw = DH // 2
        j = 2 * (pi % (HPG // 2))
        src, dst = hw * 2 * pi, hw * j
        a0, t0 = (src // 8) * 8, (dst // 8) * 8
        nrow = min(32, D // 2 - a0)
        part = qs_u[s, a0:a0 + nrow, qt * T:(qt + 1) * T]
        if nrow < 32:
            part = jnp.concatenate([part, jnp.zeros((32 - nrow, T), u32)], axis=0)
        shift = (dst - t0) - (src - a0)
        if shift:
            part = pltpu.roll(part, shift % 32, 0)
        rid = lax.broadcasted_iota(i32, (32, T), 0) + t0
        out = []
        for lo in (dst, dst + hw):
            piece = jnp.where((rid >= lo) & (rid < lo + hw), part, u32(0))
            piece = piece[0:min(32, TW - t0)]
            pieces = [jnp.zeros((t0, T), u32)] * (t0 > 0) + [piece] + [jnp.zeros((TW - t0 - 32, T), u32)] * (t0 + 32 < TW)
            out.append(jnp.concatenate(pieces, axis=0))
        return out

    def stage_a(unit, u, qt):
        s, k = unit
        s_ref, m_ref = bufs[k % 2]
        pi = k * NP + u
        g = pi // (HPG // 2)
        sg = s * NG + g
        n = T * (qt + 1)
        w_a, w_b = pair_weights(s, pi, qt)
        w_ab = _bf(jnp.where(lane64 < HT, w_a, w_b))

        def colmax8(v):
            return jnp.max(v.reshape(v.shape[0] // 8, 8, T), axis=0)

        maxes = []
        for hd, w in enumerate((_bf(w_a), _bf(w_b))):
            m8 = None
            for c in range(qt):
                kc = _bf(k_u[sg, c * TW:(c + 1) * TW, :])
                sc = jnp.dot(kc, w, preferred_element_type=f32)
                s_ref[u, qt, hd * L + c * T:hd * L + (c + 1) * T, :] = sc
                m8 = colmax8(sc) if m8 is None else jnp.maximum(m8, colmax8(sc))
            kc = _bf(k_u[sg, qt * TW:qt * TW + TW // 2, :])
            sc = jnp.dot(kc, w, preferred_element_type=f32) + mb[1 - hd]
            s_ref[u, qt, hd * L + qt * T:hd * L + qt * T + HT, :] = sc
            m8 = colmax8(sc) if m8 is None else jnp.maximum(m8, colmax8(sc))
            maxes.append(m8)
        kc = _bf(k_u[sg, qt * TW + TW // 2:(qt + 1) * TW, :])
        sc = jnp.dot(kc, w_ab, preferred_element_type=f32) + mb[2]
        s_ref[u, qt, n - HT:n, :] = sc
        mab = colmax8(sc)
        m_a = jnp.where(lane8 < HT, jnp.maximum(maxes[0], mab), maxes[0])
        m_b = jnp.where(lane8 >= HT, jnp.maximum(maxes[1], mab), maxes[1])
        m_ref[u, qt, 0] = jnp.broadcast_to(jnp.max(m_a, axis=0, keepdims=True), (8, T))
        m_ref[u, qt, 1] = jnp.broadcast_to(jnp.max(m_b, axis=0, keepdims=True), (8, T))

    def stage_b(unit, u, qt):
        s, k = unit
        s_ref, m_ref = bufs[k % 2]
        pi = k * NP + u
        n = T * (qt + 1)
        m_a = m_ref[u, qt, 0][0:1]
        m_b = m_ref[u, qt, 1][0:1]
        p_ab = jnp.exp2(s_ref[u, qt, n - HT:n, :] - jnp.where(lane1 < HT, m_a, m_b))
        for hd, m in enumerate((m_a, m_b)):
            h = 2 * pi + hd
            p = jnp.exp2(s_ref[u, qt, hd * L:hd * L + n - HT, :] - m)
            keep = (lane64 < HT) if hd == 0 else (lane64 >= HT)
            p = jnp.concatenate([p, jnp.where(keep, p_ab, 0.0)], axis=0).astype(bf16)
            w0 = ((DH * h) // 16) * 16
            off = DH * h - w0
            o = jnp.dot(_bf(vwin[s * H + h, :, 0:n]), p, preferred_element_type=f32)
            den = o[0:1] if off == 14 else o[31:32]
            r0, r1 = (off // 8) * 8, -(-(off + DH) // 8) * 8
            o = o[r0:r1] * (omg[h][0:1] / den)
            if hd == 0:
                o = pltpu.roll(o, HT, 1)
            res = am[s, w0 + r0:w0 + r1, qt * T:(qt + 1) * T] + o
            rid = lax.broadcasted_iota(i32, (r1 - r0, T), 0) + r0
            pltpu.store(ots[qt].at[w0 + r0:w0 + r1, :], res, mask=(rid >= off) & (rid < off + DH))

    def a_tasks(unit):
        return [lambda u=u, qt=qt: stage_a(unit, u, qt) for u in range(NP) for qt in QT_ORDER]

    def b_tasks(unit):
        return [lambda u=u, qt=qt: stage_b(unit, u, qt) for u in range(NP) for qt in QT_ORDER]

    w_copy(3).wait()
    rr = jnp.concatenate([r_buf[s][0:1, :] for s in range(NSEG)], axis=0)
    rr = _round_bf16(rr)
    tok = lax.broadcasted_iota(i32, (NSEG, L), 0) * L + lax.broadcasted_iota(i32, (NSEG, L), 1)
    m1v = jnp.max(rr)
    i1 = jnp.min(jnp.where(rr == m1v, tok, SEQ))
    rr2 = jnp.where(tok == i1, -jnp.inf, rr)
    m2v = jnp.max(rr2)
    i2 = jnp.min(jnp.where(rr2 == m2v, tok, SEQ))
    i1 = jnp.clip(i1, 0, SEQ - 1)
    i2 = jnp.clip(i2, 0, SEQ - 1)

    row16 = lax.broadcasted_iota(i32, (16, T), 0)
    lane16 = lax.broadcasted_iota(i32, (16, T), 1)

    def token_rows(i, slot):
        onehot = jnp.where((row16 == slot) & (lane16 == i % T), 1.0, 0.0).astype(bf16)
        return lax.dot_general(onehot, _bf(xn_u[i // T]), NT_DIMS, preferred_element_type=f32)

    def select_task():
        xsel_buf[...] = _pack(token_rows(i1, 0) + token_rows(i2, 1))
        y_acc[...] = jnp.zeros(y_acc.shape, f32)

    def expert_tile(w_ref, ft):
        return _bf(w_ref.at[ft].bitcast(u32)[...])

    def moe_up_task(ft, k, which):
        xsel = _bf(xsel_buf[:, 0:D])
        w_ref = (wg_buf, wu_buf)[which]
        hid_buf[k, which] = jnp.dot(xsel, expert_tile(w_ref, ft), preferred_element_type=f32)

    def moe_down_task(ft, k):
        gt = _round_bf16(hid_buf[k, 0])
        up = _round_bf16(hid_buf[k, 1])
        hid = (_round_bf16(gt * _sigmoid(gt)) * up).astype(bf16)
        y_acc[...] += lax.dot_general(hid, expert_tile(wd_buf, ft), NT_DIMS, preferred_element_type=f32)

    def moe_tasks(ft0, count):
        tasks = []
        for k0 in range(0, count, FPB):
            ks = range(k0, min(k0 + FPB, count))
            tasks += [lambda k=k, w=w: moe_up_task(ft0 + k, k, w) for k in ks for w in range(2)]
            tasks += [lambda k=k: moe_down_task(ft0 + k, k) for k in ks]
        return tasks

    def moe_finish():
        y = _round_bf16(y_acc[...])
        rsel = jnp.where(lax.broadcasted_iota(i32, (16, 1), 0) == 0, m1v, m2v)
        y = _round_bf16(y * _round_bf16(_sigmoid(rsel)))
        y = jnp.concatenate([y, jnp.zeros((16, DP - D), f32)], axis=1)
        y = jnp.concatenate([jnp.zeros((HT, DP), f32), y, jnp.zeros((T - HT - 16, DP), f32)], axis=0)
        y_t = jnp.concatenate([y.T[0:D], jnp.zeros((D, T), f32)], axis=1)
        y_u = _pack(y_t)[:, 0:T]
        lane = lax.broadcasted_iota(i32, (D // 2, T), 1)
        wot_u[:, DP - T:DP] = jnp.where(lane < HT, wot_u[:, DP - T:DP], y_u)
        rid = lax.broadcasted_iota(i32, (8, T), 0)
        for tt in range(TPS):
            tok_l = lax.broadcasted_iota(i32, (8, T), 1) + (NSEG - 1) * L + tt * T
            ots[tt][D:D + 8, :] = jnp.where(((rid == 0) & (tok_l == i1)) | ((rid == 1) & (tok_l == i2)), 1.0, 0.0)

    dense = _interleave(a_tasks((0, 0)), prep_dense(3, wot_u, 0))
    with _scope("p15_mix"):
        cut = (2 * len(dense)) // 3
        run(dense[:cut] + [select_task] + dense[cut:])

    for i in range(3):
        moe_wait(i)

    def out_tile(s, tt, last, chunk_copies=None):
        c0 = s * L + tt * T
        if not isinstance(s, int):
            c0 = pl.multiple_of(c0, T)
        o_bf = ots[tt][...].astype(bf16)
        nchunk = 4
        rows = D // nchunk
        for rc in range(nchunk):
            r0 = rc * rows
            attn = jnp.dot(_bf(wot_u[r0 // 2:(r0 + rows) // 2, :]), o_bf, preferred_element_type=f32)
            xn = _bf(xn_u[s * TPS + tt, r0 // 2:(r0 + rows) // 2, :]).astype(f32)
            x = x_buf[r0:r0 + rows, pl.ds(c0, T)].astype(f32)
            res = x + attn + xn
            out_buf[r0:r0 + rows, pl.ds(c0, T)] = res.astype(bf16)
            if chunk_copies is not None:
                chunk_copies[rc].start()

    def pair_tasks(ua, ub):
        tasks = []
        for x, y in zip(a_tasks(ua), b_tasks(ub)):
            tasks += [y, x]
        return tasks

    def seg_end(s, last):
        def by_qt(fn, unit, qt):
            return [lambda u=u: fn(unit, u, qt) for u in range(NP)]

        steps = []
        for step in range(7):
            lists = []
            if step < 4:
                lists.append(by_qt(stage_b, (s, 2), 3 - step))
                lists.append(by_qt(stage_a, (s, 3), 3 - step))
            if 1 <= step < 5:
                lists.append(by_qt(stage_b, (s, 3), 4 - step))
            if not last and 2 <= step < 6:
                lists.append(by_qt(stage_a, (s + 1, 0), 5 - step))
            if step >= 3:
                lists.append([lambda tt=6 - step: out_tile(s, tt, last)])
            steps.append(_interleave(*lists))
        return steps

    def seg_att(s, c):
        tasks = pair_tasks((s, 1), (s, 0)) + pair_tasks((s, 2), (s, 1))
        steps = seg_end(s, False)
        for step in steps[0:5]:
            tasks += step
        with _scope("att_seg"):
            run(_interleave(tasks, moe_tasks(s * FPI, FPI)))
            for step in steps[5:]:
                run(step)

        @pl.when(s < NSEG - 2)
        def _():
            out_copy(pl.multiple_of(s * L, L), L, s).start()
        return c

    lax.fori_loop(0, NSEG - 1, seg_att, 0)

    npatch = (NSEG - 1) * TPS

    def patch_tile(idx):
        return jnp.where(idx < npatch * T, idx // T, 0)

    tile0 = patch_tile(i1)
    tile1 = patch_tile(i2)
    tile1 = jnp.where(tile1 == tile0, (tile0 + 1) % npatch, tile1)

    def patch(tile):
        c0 = pl.multiple_of(tile * T, T)
        rid = lax.broadcasted_iota(i32, (T, T), 0)
        tok_l = lax.broadcasted_iota(i32, (T, T), 1) + c0
        hit = ((rid == HT) & (tok_l == i1)) | ((rid == HT + 1) & (tok_l == i2))
        onehot = jnp.where(hit, 1.0, 0.0).astype(bf16)
        for rc in range(4):
            r0, r1 = rc * (D // 4), (rc + 1) * (D // 4)
            upd = jnp.dot(_bf(wot_u[r0 // 2:r1 // 2, DP - T:DP]), onehot, preferred_element_type=f32)
            cur = out_buf[r0:r1, pl.ds(c0, T)].astype(f32)
            out_buf[r0:r1, pl.ds(c0, T)] = (cur + upd).astype(bf16)

    sent = (NSEG - 2) * TPS
    resend0 = jnp.where(tile0 < sent, tile0, jnp.where(tile1 == 0, 1, 0))
    resend1 = jnp.where(tile1 < sent, tile1, jnp.where(resend0 == 0, 1, 0))
    patch_copies = [out_copy(pl.multiple_of(resend0 * T, T), T, 7), out_copy(pl.multiple_of(resend1 * T, T), T, 8),
                    out_copy((NSEG - 2) * L, L, NSEG - 2)]
    last_copies = [out_copy((NSEG - 1) * L + tt * T, T, NSEG - 1 + tt) for tt in range(1, TPS)]
    c_fin = (NSEG - 1) * L
    final_copies = [
        pltpu.make_async_copy(out_buf.at[rc * (D // 4):(rc + 1) * (D // 4), c_fin:c_fin + T],
                              out_hbm.at[rc * (D // 4):(rc + 1) * (D // 4), c_fin:c_fin + T],
                              sems.at[SEM_FINAL + rc]) for rc in range(4)]

    sl = NSEG - 1
    for s in range(NSEG - 2):
        out_copy(s * L, L, s).wait()
    with _scope("tail_2"):
        moe_finish()
        run(pair_tasks((sl, 1), (sl, 0)))
        patch(tile0)
        patch(tile1)
        run(pair_tasks((sl, 2), (sl, 1)))
        for cp in patch_copies:
            cp.start()
        steps = seg_end(sl, True)
        for step in steps[0:5]:
            run(step)
        last_copies[2].start()
        last_copies[1].start()
    with _scope("tail_3"):
        run(steps[5])
        last_copies[0].start()
        out_tile(sl, 0, True, final_copies)

    with _scope("out_wait"):
        for cp in patch_copies + last_copies + final_copies:
            cp.wait()


@jax.jit
def pallas_parallel_sum__memory_aug_infini_attn__moe_arch_mod__prompt_kernel(
    A_x: jax.Array,
    A_wq: jax.Array,
    A_wk: jax.Array,
    A_wv: jax.Array,
    A_wo: jax.Array,
    A_beta: jax.Array,
    B_x: jax.Array,
    B_w_r: jax.Array,
    B_w_gate: jax.Array,
    B_w_up: jax.Array,
    B_w_down: jax.Array,
):
    del B_x
    any_spec = pl.BlockSpec(memory_space=pl.ANY)
    scratch = [
        pltpu.VMEM((H,), bf16),
        pltpu.VMEM((D,), bf16),
        pltpu.VMEM((D, SEQ), bf16),
        pltpu.VMEM((4, D, D), bf16),
        pltpu.VMEM((NFT, D, T), bf16),
        pltpu.VMEM((NFT, D, T), bf16),
        pltpu.VMEM((NFT, D, T), bf16),
        pltpu.VMEM((D, SEQ), bf16),
        pltpu.VMEM((WT_ALLOC, DP), u32),
        pltpu.VMEM((2, D // 2, LNW), u32),
        pltpu.VMEM((D // 2, DP), u32),
        pltpu.VMEM((NT, DP // 2, T), u32),
        pltpu.VMEM((BT, DP // 2, T), u32),
        pltpu.VMEM((BT, DP // 2, T), u32),
        pltpu.VMEM((NSEG, D // 2, L), u32),
        pltpu.VMEM((NSEG * NG, L // 2, T), u32),
        pltpu.VMEM((NSEG, D // 2, L), u32),
        pltpu.VMEM((NSEG, D // 2, L), u32),
        pltpu.VMEM((NSEG, D // 2, L), u32),
        pltpu.VMEM((NSEG * H, 16, L), u32),
        pltpu.VMEM((NSEG, 8, L), f32),
        pltpu.VMEM((NG, T, T), f32),
        pltpu.VMEM((NG, T, T), f32),
        pltpu.VMEM((NSEG, D, L), f32),
        pltpu.VMEM((NG, 8, T), f32),
        pltpu.VMEM((H, 8, T), f32),
        pltpu.VMEM((3, HT, T), f32),
        pltpu.VMEM((NP, 4, 2 * L, T), f32),
        pltpu.VMEM((NP, 4, 2, 8, T), f32),
        pltpu.VMEM((NP, 4, 2 * L, T), f32),
        pltpu.VMEM((NP, 4, 2, 8, T), f32),
        pltpu.VMEM((DP, T), f32),
        pltpu.VMEM((DP, T), f32),
        pltpu.VMEM((DP, T), f32),
        pltpu.VMEM((DP, T), f32),
        pltpu.VMEM((2, D, LNW), f32),
        pltpu.VMEM((2, 2, 8, LNW), f32),
        pltpu.VMEM((16, D), f32),
        pltpu.VMEM((8, DP), u32),
        pltpu.VMEM((FPI, 2, 16, T), f32),
        pltpu.SemaphoreType.DMA((NSEM,)),
    ]
    x_t = jnp.transpose(A_x, (0, 2, 1)).reshape(D, SEQ)
    out_t = pl.pallas_call(
        _kernel,
        out_shape=jax.ShapeDtypeStruct((D, SEQ), bf16),
        in_specs=[any_spec] * 10,
        out_specs=any_spec,
        scratch_shapes=scratch,
        compiler_params=pltpu.CompilerParams(vmem_limit_bytes=110 * 1024 * 1024),
    )(x_t, A_wq, A_wk, A_wv, A_wo, A_beta, B_w_r, B_w_gate, B_w_up, B_w_down.T)
    return jnp.transpose(out_t.reshape(1, D, SEQ), (0, 2, 1))
```

```python
import contextlib

import jax
import jax.numpy as jnp
from jax import lax
from jax.experimental import pallas as pl
from jax.experimental.pallas import tpu as pltpu

bf16 = jnp.bfloat16
f32 = jnp.float32
u32 = jnp.uint32
i32 = jnp.int32

SEQ = 2048
D = 576
DP = 640
H = 32
DH = 18
NSEG = 4
L = 512
T = 128
TW = T // 2
HT = T // 2
TPS = L // T
HPG = 6
NG = 6
F = 4608
FPI = 12
FPB = 3
NFT = F // T
NP = 4
UPS = H // (2 * NP)
NUNIT = NSEG * UPS
NT = SEQ // T
LNW = 256
BT = LNW // T
NORM_PARTS = 6
VB = 8 * DH

LOG2E = 1.4426950408889634
QSCALE = (DH ** -0.5) * LOG2E
MASKVAL = -1000000000.0 * LOG2E
EPS_BF16 = 1.0013580322265625e-05
ONES_PAIR = 0x3F803F80

NT_DIMS = (((1,), (1,)), ((), ()))

WT_Q = 0
WT_K = D // 2
WT_R = D
WT_V = D + 8
WT_ROWS = WT_V + D // 2
WT_ALLOC = 1056
NBLK = DP // T

X_PIECES = ((0, LNW), (LNW, LNW), (L, L), (2 * L, L), (3 * L, L))
SEM_X = 0
SEM_W = 5
SEM_MOE = 9
SEM_OUT = 12
SEM_SMALL = 21
SEM_WQB = 23
SEM_FINAL = 24
NSEM = 28
WQ_SPLIT = 2 * T


PROFILE_SCOPES = False
PACE = True
TAIL_BARRIERS = False
QT_ORDER = (3, 2, 1, 0)


def _scope(name):
    return jax.named_scope(name) if PROFILE_SCOPES else contextlib.nullcontext()


def _valid(g):
    return min(HPG * DH, D - g * HPG * DH)


def _ewin(g):
    start = (g * HPG * DH // 16) * 16
    return start, g * HPG * DH - start, min(T, D - start)


def _bf(x):
    return pltpu.bitcast(x, bf16)


def _pack(x):
    return pltpu.bitcast(x.astype(bf16), u32)


def _round_bf16(x):
    return x.astype(bf16).astype(f32)


def _phi(t):
    return jnp.where(t > 0, t + 1.0, jnp.exp(t))


def _sigmoid(t):
    return 1.0 / (1.0 + jnp.exp(-t))


def _zero_after(v):
    bits = pltpu.bitcast(v[0:8, 0:LNW], u32)
    sixteen = jnp.uint32(16)
    bits = lax.shift_right_logical(lax.shift_right_logical(bits, sixteen), sixteen)
    return pltpu.bitcast(bits, f32) if PACE else None


def _interleave(*lists):
    items = []
    for li, tasks in enumerate(lists):
        for k, t in enumerate(tasks):
            items.append(((k + 0.5) / len(tasks), li, k, t))
    items.sort(key=lambda it: it[:3])
    return [it[3] for it in items]


def _kernel(x_hbm, wq_hbm, wk_hbm, wv_hbm, wo_hbm, beta_hbm, wr_hbm, wg_hbm, wu_hbm, wd_hbm,
            out_hbm,
            beta_ref, wr_ref, x_buf, w_buf, wg_buf, wu_buf, wd_buf, out_buf,
            wt_u, kt_tmp, wot_u, xn_u, xs_a, xs_b, qs_u, k_u, pq_u, pk_u, vt_u, vwin,
            r_buf, mt_acc, lm_f, mcode, am, g16, omg, mb,
            s0, m0, s1, m1, ot0, ot1, ot2, ot3, xf, ln_stat, y_acc, xsel_buf, hid_buf, sems):

    def x_copy(i):
        c0, width = X_PIECES[i]
        return pltpu.make_async_copy(x_hbm.at[:, pl.ds(c0, width)], x_buf.at[:, pl.ds(c0, width)],
                                     sems.at[SEM_X + i])

    def w_copy(i):
        src = (wq_hbm, wk_hbm, wv_hbm, wo_hbm)[i]
        return pltpu.make_async_copy(src, w_buf.at[i], sems.at[SEM_W + i])

    wq_first = pltpu.make_async_copy(wq_hbm.at[:, 0:WQ_SPLIT], w_buf.at[0, :, 0:WQ_SPLIT], sems.at[SEM_W])
    wq_rest = pltpu.make_async_copy(wq_hbm.at[:, WQ_SPLIT:D], w_buf.at[0, :, WQ_SPLIT:D], sems.at[SEM_WQB])

    moe_src = (wg_hbm, wu_hbm, wd_hbm)
    moe_dst = (wg_buf, wu_buf, wd_buf)

    def moe_start(i, ft):
        c0 = ft * T if isinstance(ft, int) else pl.multiple_of(ft * T, T)
        pltpu.make_async_copy(moe_src[i].at[:, pl.ds(c0, T)], moe_dst[i].at[ft], sems.at[SEM_MOE + i]).start()

    def moe_issue(first, last):
        for n in range(first, last):
            moe_start(n % 3, n // 3)

    def moe_wait(i):
        pltpu.make_async_copy(moe_dst[i], moe_dst[i], sems.at[SEM_MOE + i]).wait()

    def out_copy(c0, width, sem):
        return pltpu.make_async_copy(out_buf.at[:, pl.ds(c0, width)], out_hbm.at[:, pl.ds(c0, width)],
                                     sems.at[SEM_OUT + sem])

    small_copies = [pltpu.make_async_copy(beta_hbm, beta_ref, sems.at[SEM_SMALL]),
                    pltpu.make_async_copy(wr_hbm, wr_ref, sems.at[SEM_SMALL + 1])]
    x_copy(0).start()
    wq_first.start()
    wq_rest.start()
    x_copy(1).start()
    for cp in small_copies:
        cp.start()
    w_copy(1).start()
    w_copy(2).start()

    init_scope = _scope("init")
    init_scope.__enter__()
    kr = lax.broadcasted_iota(i32, (HT, T), 0)
    ql = lax.broadcasted_iota(i32, (HT, T), 1)
    mb[0] = jnp.where(ql < kr, MASKVAL, 0.0).astype(f32)
    mb[1] = jnp.where((ql >= HT) & (ql - HT < kr), MASKVAL, 0.0).astype(f32)
    mb[2] = jnp.where(ql % HT < kr, MASKVAL, 0.0).astype(f32)
    zpad = jnp.zeros(((DP - D) // 2, LNW), u32)
    for blk in range(SEQ // LNW):
        xn_u[blk, D // 2:DP // 2, :] = zpad
    xs_a[D // 2:DP // 2, :] = zpad
    xs_b[D // 2:DP // 2, :] = zpad
    ots = (ot0, ot1, ot2, ot3)
    for o_ref in ots:
        o_ref[D:DP, :] = jnp.zeros((DP - D, T), f32)
    am[0] = jnp.zeros(am.shape[1:], f32)
    mt_acc[...] = jnp.zeros(mt_acc.shape, f32)
    g16[...] = jnp.zeros(g16.shape, f32)

    init_scope.__exit__(None, None, None)

    pace = [None]

    def gate_tables():
        gate = _round_bf16(_sigmoid(beta_ref[...].reshape(1, H).astype(f32)))
        for h in range(H):
            gh = jnp.broadcast_to(gate[:, h:h + 1], (1, T))
            omg[h] = jnp.broadcast_to(_round_bf16(1.0 - gh), (8, T))
            g16[h // HPG, (h % HPG):(h % HPG) + 1, :] = gh

    def transpose_block(i, cb):
        c1 = min((cb + 1) * T, D)
        blk = w_buf[i, :, cb * T:c1]
        if c1 - cb * T < T:
            blk = jnp.concatenate([blk, jnp.zeros((D, T - (c1 - cb * T)), bf16)], axis=1)
        blk = jnp.concatenate([blk, jnp.zeros((DP - D, T), bf16)], axis=0)
        return pltpu.bitcast(blk.T, u32)

    def prep_dense(i, dst, base):
        def task(cb):
            nrow = min(TW, D // 2 - cb * TW)
            dst[base + cb * TW:base + cb * TW + nrow, :] = transpose_block(i, cb)[0:nrow]
        return [lambda cb=cb: task(cb) for cb in range(DP // T)]

    def router_row():
        wr = wr_ref[...].reshape(1, D).astype(f32)
        wr = jnp.concatenate([wr, jnp.zeros((1, DP - D), f32)], axis=1)
        bits = lax.shift_right_logical(pltpu.bitcast(wr, u32), u32(16))
        rid = lax.broadcasted_iota(i32, (8, DP), 0)
        wt_u[WT_R:WT_R + 8, :] = jnp.where(rid == 0, bits, u32(0))

    def ln_tasks(s, p, stage):
        c0 = s * L + p * LNW
        if not isinstance(s, int):
            c0 = pl.multiple_of(c0, LNW)

        def mean_pass():
            acc = pace[0]
            for r in range(0, D, 64):
                x = x_buf[r:r + 64, pl.ds(c0, LNW)].astype(f32)
                xf[p, r:r + 64, :] = x
                part = jnp.sum(x.reshape(8, 8, LNW), axis=0)
                acc = part if acc is None else acc + part
            mean = jnp.sum(acc, axis=0, keepdims=True) / D
            ln_stat[p, 0] = jnp.broadcast_to(mean, (8, LNW))

        def var_pass():
            mean = ln_stat[p, 0][0:1]
            if pace[0] is not None:
                mean = mean + pace[0][0:1]
            acc = None
            for r in range(0, D, 96):
                xc = xf[p, r:r + 96, :] - mean
                part = jnp.sum((xc * xc).reshape(12, 8, LNW), axis=0)
                acc = part if acc is None else acc + part
            var = jnp.sum(acc, axis=0, keepdims=True) / D
            den = _round_bf16(jnp.sqrt(_round_bf16(_round_bf16(var) + EPS_BF16)))
            ln_stat[p, 1] = jnp.broadcast_to(1.0 / den, (8, LNW))
            ln_stat[p, 0] = jnp.broadcast_to(_round_bf16(mean), (8, LNW))

        def norm_pass(part):
            mean_b = ln_stat[p, 0][0:1]
            if pace[0] is not None:
                mean_b = mean_b + pace[0][0:1]
            inv = ln_stat[p, 1][0:1]
            step = D // NORM_PARTS
            for r in range(part * step, (part + 1) * step, 48):
                xn = _pack(_round_bf16(xf[p, r:r + 48, :] - mean_b) * inv)
                xn_u.at[s * (L // LNW) + p][r // 2:r // 2 + 24, :] = xn
                if stage is not None:
                    stage[r // 2:r // 2 + 24, :] = xn

        return [mean_pass, var_pass] + [lambda part=part: norm_pass(part) for part in range(NORM_PARTS)]

    def load_xs(s, p, stage):
        return _bf(xn_u[s * (L // LNW) + p] if stage is None else stage[...])

    def blk_rows(cb):
        return min(TW, D // 2 - cb * TW)

    def q_task(s, p, stage, cb):
        nr = blk_rows(cb)
        rows = slice(cb * TW, cb * TW + nr)
        cols = slice(p * LNW, (p + 1) * LNW)
        w = _bf(wt_u[WT_Q + cb * TW:WT_Q + cb * TW + nr, :])
        q = jnp.dot(w, load_xs(s, p, stage), preferred_element_type=f32)
        pace[0] = _zero_after(q)
        qs = q * QSCALE
        qrot = jnp.concatenate([pltpu.roll(qs[:, t * T:(t + 1) * T], HT, 1) for t in range(BT)], axis=1)
        rid = lax.broadcasted_iota(i32, qs.shape, 0) + cb * T
        even = ((rid // DH) % 2) == 0
        qs_u.at[s][rows, cols] = _pack(jnp.where(even, qrot, qs))
        pq_u.at[s][rows, cols] = _pack(_phi(q))

    def k_task(s, p, stage, cb):
        nr = blk_rows(cb)
        rows = slice(cb * TW, cb * TW + nr)
        cols = slice(p * LNW, (p + 1) * LNW)
        extra = 8 if cb == NBLK - 1 else 0
        w = _bf(wt_u[WT_K + cb * TW:WT_K + cb * TW + nr + extra, :])
        k = jnp.dot(w, load_xs(s, p, stage), preferred_element_type=f32)
        pace[0] = _zero_after(k)
        if extra:
            r_buf[s, :, cols] = jnp.broadcast_to(k[2 * nr:2 * nr + 1, :], (8, LNW))
            k = k[0:2 * nr]
        kt_tmp.at[p][rows, :] = _pack(k)
        pk_u.at[s][rows, cols] = _pack(_phi(k))

    def kt_task(s, p, g):
        nv = _valid(g) // 2
        src = g * HPG * DH // 2
        kg = jnp.concatenate([kt_tmp[p, src:src + nv, :], jnp.zeros((TW - nv, LNW), u32)], axis=0)
        k_u.at[s * NG + g][p * (LNW // 2):(p + 1) * (LNW // 2), :] = pltpu.bitcast(_bf(kg).T, u32)

    def v_task(s, p, stage, b):
        cols = slice(p * LNW, (p + 1) * LNW)
        w = _bf(wt_u[WT_V + b * (VB // 2):WT_V + (b + 1) * (VB // 2), :])
        v = jnp.dot(w, load_xs(s, p, stage), preferred_element_type=f32)
        pace[0] = _zero_after(v)
        v = _pack(v)
        vt_u.at[s][b * (VB // 2):(b + 1) * (VB // 2), cols] = v
        sub = lax.broadcasted_iota(i32, (16, LNW), 0)
        for hh in range(8):
            w8 = (9 * hh) // 8
            ones_row = 0 if 2 * hh == 14 else 15
            vwin.at[s * H + 8 * b + hh][:, cols] = jnp.where(sub == ones_row, u32(ONES_PAIR), v[8 * w8:8 * w8 + 16, :])

    def q_tasks(s, p, stage=None):
        return [lambda cb=cb: q_task(s, p, stage, cb) for cb in range(NBLK)]

    def k_tasks(s, p, stage=None):
        tasks, done = [], 0
        for cb in range(NBLK):
            tasks.append(lambda cb=cb: k_task(s, p, stage, cb))
            while done < NG and done * HPG * DH + _valid(done) <= min((cb + 1) * T, D):
                tasks.append(lambda g=done: kt_task(s, p, g))
                done += 1
        return tasks

    def v_tasks(s, p, stage=None):
        return [lambda b=b: v_task(s, p, stage, b) for b in range(D // VB)]

    def mem_layout(g):
        es, eoff, _ = _ewin(g)
        nv = _valid(g)
        ne = -(-(eoff + nv) // 16) * 16
        ones_row = 0 if eoff >= 2 else eoff + nv
        nh = nv // DH
        den_row = 0 if eoff >= nh else ne
        return es, eoff, nv, ne, ones_row, den_row, max(ne, den_row + 16 * (den_row > 0))

    def mem_update(sp, g):
        es, eoff, nv, ne, ones_row, den_row, nr = mem_layout(g)
        nw = min(T, D - es)
        win = vt_u[sp, es // 2:(es + ne) // 2, :]
        wid = lax.broadcasted_iota(i32, win.shape, 0)
        lhs = _bf(jnp.where(wid == ones_row // 2, u32(ONES_PAIR), win))
        upd = lax.dot_general(lhs, _bf(pk_u[sp, es // 2:(es + nw) // 2, :]), NT_DIMS, preferred_element_type=f32)
        mt = mt_acc[g, 0:ne, 0:nw] + upd
        mt_acc[g, 0:ne, 0:nw] = mt
        z = jnp.broadcast_to(mt[ones_row:ones_row + 1, :], (nr, nw))
        if nr > ne:
            mt = jnp.concatenate([mt, jnp.zeros((nr - ne, nw), f32)], axis=0)
        code = mcode[g, 0:nr, 0:nw]
        lm_f[g, 0:nr, 0:nw] = jnp.where(code == 1, mt, jnp.where(code == 2, z, 0.0))

    def mem_masks():
        for g in range(NG):
            es, eoff, nv, ne, ones_row, den_row, nr = mem_layout(g)
            row = lax.broadcasted_iota(i32, (T, T), 0)
            d_loc = lax.broadcasted_iota(i32, (T, T), 1) - eoff
            e_loc = row - eoff
            d_ok = (d_loc >= 0) & (d_loc < nv)
            same_head = (e_loc >= 0) & (e_loc < nv) & d_ok & ((e_loc // DH) == (d_loc // DH))
            den_hit = (row >= den_row) & d_ok & ((d_loc // DH) == row - den_row)
            mcode[g] = jnp.where(same_head, 1, jnp.where(den_hit, 2, 0))

    def mem_retrieve(s, g):
        es, eoff, nv, ne, ones_row, den_row, nr = mem_layout(g)
        nw = min(T, D - es)
        nd = jnp.dot(lm_f[g, 0:nr, 0:nw].astype(bf16), _bf(pq_u[s, es // 2:(es + nw) // 2, :]),
                     preferred_element_type=f32)
        scale = jnp.broadcast_to(g16[g][:, 0:1], (8, L)) / (nd[den_row:den_row + 8, :] + 1e-6)
        r8 = lax.broadcasted_iota(i32, (8, L), 0)
        for b in range(ne // 8):
            lo, hi = 8 * b - eoff, 8 * b + 7 - eoff
            if hi < 0 or lo >= nv:
                continue
            j1, j2 = max(lo, 0) // DH, min(hi, nv - 1) // DH
            sc = jnp.broadcast_to(scale[j1:j1 + 1, :], (8, L))
            if j2 != j1:
                sc = jnp.where(r8 < DH * j2 - lo, sc, jnp.broadcast_to(scale[j2:j2 + 1, :], (8, L)))
            val = nd[8 * b:8 * b + 8, :] * sc
            dst = am.at[s, es + 8 * b:es + 8 * b + 8, :]
            if lo >= 0 and hi < nv:
                dst[...] = val
            else:
                pltpu.store(dst, val, mask=(r8 + lo >= 0) & (r8 + lo < nv))

    def run(tasks):
        for t in tasks:
            t()

    prep_q = prep_dense(0, wt_u, WT_Q)
    q0a = q_tasks(0, 0)
    with _scope("p1_wait_x0"):
        x_copy(0).wait()
    for i in range(2, len(X_PIECES)):
        x_copy(i).start()
    w_copy(3).start()
    moe_issue(0, 48)
    with _scope("p1_ln0a"):
        run(ln_tasks(0, 0, None))
        wq_first.wait()
    with _scope("p1_q0a_first"):
        run(prep_q[0:2] + q0a[0:2])
        wq_rest.wait()
        x_copy(1).wait()
    with _scope("p1_q0a"):
        run(prep_q[2:])
        run(_interleave(q0a[2:], ln_tasks(0, 1, None)))
        w_copy(1).wait()
        for cp in small_copies:
            cp.wait()
    k0a, k0b = k_tasks(0, 0), k_tasks(0, 1)
    with _scope("p1_q0b"):
        run(_interleave(q_tasks(0, 1), prep_dense(1, wt_u, WT_K), [router_row, gate_tables, mem_masks]))
        run(k0a)
        w_copy(2).wait()
        x_copy(2).wait()
    moe_issue(48, 60)
    with _scope("p1_k0v0"):
        run(_interleave(k0b, prep_dense(2, wt_u, WT_V)))
        run(_interleave(v_tasks(0, 0) + v_tasks(0, 1), ln_tasks(1, 0, xs_a)))

    moe_issue(60, 72)

    def seg_body(s, c):
        for ss in range(2, NSEG):
            @pl.when(s + 1 == ss)
            def _():
                x_copy(ss + 1).wait()
                if ss == NSEG - 1:
                    moe_issue(72, 3 * NFT)
        nxt = jnp.minimum(s + 1, NSEG - 1)
        pace[0] = None
        with _scope("p1_seg"):
            updates = [lambda g=g: mem_update(s - 1, g) for g in range(NG)]
            retrieves = [lambda g=g: mem_retrieve(s, g) for g in range(NG)]
            first = _interleave(q_tasks(s, 0, xs_a), updates) + k_tasks(s, 0, xs_a) + v_tasks(s, 0, xs_a)
            run(_interleave(first, ln_tasks(s, 1, xs_b)))
            second = q_tasks(s, 1, xs_b) + _interleave(k_tasks(s, 1, xs_b) + v_tasks(s, 1, xs_b), retrieves)
            run(_interleave(second, ln_tasks(nxt, 0, xs_a)))
        return c

    lax.fori_loop(1, NSEG, seg_body, 0)

    bufs = ((s0, m0), (s1, m1))
    lane64 = lax.broadcasted_iota(i32, (TW, T), 1)
    lane1 = lax.broadcasted_iota(i32, (1, T), 1)
    lane8 = lax.broadcasted_iota(i32, (8, T), 1)

    def pair_weights(s, pi, qt):
        hw = DH // 2
        j = 2 * (pi % (HPG // 2))
        src, dst = hw * 2 * pi, hw * j
        a0, t0 = (src // 8) * 8, (dst // 8) * 8
        nrow = min(32, D // 2 - a0)
        part = qs_u[s, a0:a0 + nrow, qt * T:(qt + 1) * T]
        if nrow < 32:
            part = jnp.concatenate([part, jnp.zeros((32 - nrow, T), u32)], axis=0)
        shift = (dst - t0) - (src - a0)
        if shift:
            part = pltpu.roll(part, shift % 32, 0)
        rid = lax.broadcasted_iota(i32, (32, T), 0) + t0
        out = []
        for lo in (dst, dst + hw):
            piece = jnp.where((rid >= lo) & (rid < lo + hw), part, u32(0))
            piece = piece[0:min(32, TW - t0)]
            pieces = [jnp.zeros((t0, T), u32)] * (t0 > 0) + [piece] + [jnp.zeros((TW - t0 - 32, T), u32)] * (t0 + 32 < TW)
            out.append(jnp.concatenate(pieces, axis=0))
        return out

    def stage_a(unit, u, qt):
        s, k = unit
        s_ref, m_ref = bufs[k % 2]
        pi = k * NP + u
        g = pi // (HPG // 2)
        sg = s * NG + g
        n = T * (qt + 1)
        w_a, w_b = pair_weights(s, pi, qt)
        w_ab = _bf(jnp.where(lane64 < HT, w_a, w_b))

        def colmax8(v):
            return jnp.max(v.reshape(v.shape[0] // 8, 8, T), axis=0)

        maxes = []
        for hd, w in enumerate((_bf(w_a), _bf(w_b))):
            m8 = None
            for c in range(qt):
                kc = _bf(k_u[sg, c * TW:(c + 1) * TW, :])
                sc = jnp.dot(kc, w, preferred_element_type=f32)
                s_ref[u, qt, hd * L + c * T:hd * L + (c + 1) * T, :] = sc
                m8 = colmax8(sc) if m8 is None else jnp.maximum(m8, colmax8(sc))
            kc = _bf(k_u[sg, qt * TW:qt * TW + TW // 2, :])
            sc = jnp.dot(kc, w, preferred_element_type=f32) + mb[1 - hd]
            s_ref[u, qt, hd * L + qt * T:hd * L + qt * T + HT, :] = sc
            m8 = colmax8(sc) if m8 is None else jnp.maximum(m8, colmax8(sc))
            maxes.append(m8)
        kc = _bf(k_u[sg, qt * TW + TW // 2:(qt + 1) * TW, :])
        sc = jnp.dot(kc, w_ab, preferred_element_type=f32) + mb[2]
        s_ref[u, qt, n - HT:n, :] = sc
        mab = colmax8(sc)
        m_a = jnp.where(lane8 < HT, jnp.maximum(maxes[0], mab), maxes[0])
        m_b = jnp.where(lane8 >= HT, jnp.maximum(maxes[1], mab), maxes[1])
        m_ref[u, qt, 0] = jnp.broadcast_to(jnp.max(m_a, axis=0, keepdims=True), (8, T))
        m_ref[u, qt, 1] = jnp.broadcast_to(jnp.max(m_b, axis=0, keepdims=True), (8, T))

    def stage_b(unit, u, qt):
        s, k = unit
        s_ref, m_ref = bufs[k % 2]
        pi = k * NP + u
        n = T * (qt + 1)
        m_a = m_ref[u, qt, 0][0:1]
        m_b = m_ref[u, qt, 1][0:1]
        p_ab = jnp.exp2(s_ref[u, qt, n - HT:n, :] - jnp.where(lane1 < HT, m_a, m_b))
        for hd, m in enumerate((m_a, m_b)):
            h = 2 * pi + hd
            p = jnp.exp2(s_ref[u, qt, hd * L:hd * L + n - HT, :] - m)
            keep = (lane64 < HT) if hd == 0 else (lane64 >= HT)
            p = jnp.concatenate([p, jnp.where(keep, p_ab, 0.0)], axis=0).astype(bf16)
            w0 = ((DH * h) // 16) * 16
            off = DH * h - w0
            o = jnp.dot(_bf(vwin[s * H + h, :, 0:n]), p, preferred_element_type=f32)
            den = o[0:1] if off == 14 else o[31:32]
            r0, r1 = (off // 8) * 8, -(-(off + DH) // 8) * 8
            o = o[r0:r1] * (omg[h][0:1] / den)
            if hd == 0:
                o = pltpu.roll(o, HT, 1)
            res = am[s, w0 + r0:w0 + r1, qt * T:(qt + 1) * T] + o
            rid = lax.broadcasted_iota(i32, (r1 - r0, T), 0) + r0
            pltpu.store(ots[qt].at[w0 + r0:w0 + r1, :], res, mask=(rid >= off) & (rid < off + DH))

    def a_tasks(unit):
        return [lambda u=u, qt=qt: stage_a(unit, u, qt) for u in range(NP) for qt in QT_ORDER]

    def b_tasks(unit):
        return [lambda u=u, qt=qt: stage_b(unit, u, qt) for u in range(NP) for qt in QT_ORDER]

    w_copy(3).wait()
    rr = jnp.concatenate([r_buf[s][0:1, :] for s in range(NSEG)], axis=0)
    rr = _round_bf16(rr)
    tok = lax.broadcasted_iota(i32, (NSEG, L), 0) * L + lax.broadcasted_iota(i32, (NSEG, L), 1)
    m1v = jnp.max(rr)
    i1 = jnp.min(jnp.where(rr == m1v, tok, SEQ))
    rr2 = jnp.where(tok == i1, -jnp.inf, rr)
    m2v = jnp.max(rr2)
    i2 = jnp.min(jnp.where(rr2 == m2v, tok, SEQ))
    i1 = jnp.clip(i1, 0, SEQ - 1)
    i2 = jnp.clip(i2, 0, SEQ - 1)

    row16 = lax.broadcasted_iota(i32, (16, T), 0)
    lane16 = lax.broadcasted_iota(i32, (16, T), 1)

    def token_rows(i, slot):
        onehot = jnp.where((row16 == slot) & (lane16 == i % T), 1.0, 0.0).astype(bf16)
        return lax.dot_general(onehot, _bf(xn_u[i // LNW, :, pl.ds(pl.multiple_of(((i // T) % BT) * T, T), T)]), NT_DIMS, preferred_element_type=f32)

    def select_task():
        xsel_buf[...] = _pack(token_rows(i1, 0) + token_rows(i2, 1))
        y_acc[...] = jnp.zeros(y_acc.shape, f32)

    def expert_tile(w_ref, ft):
        return _bf(w_ref.at[ft].bitcast(u32)[...])

    def moe_up_task(ft, k, which):
        xsel = _bf(xsel_buf[:, 0:D])
        w_ref = (wg_buf, wu_buf)[which]
        hid_buf[k, which] = jnp.dot(xsel, expert_tile(w_ref, ft), preferred_element_type=f32)

    def moe_down_task(ft, k):
        gt = _round_bf16(hid_buf[k, 0])
        up = _round_bf16(hid_buf[k, 1])
        hid = (_round_bf16(gt * _sigmoid(gt)) * up).astype(bf16)
        y_acc[...] += lax.dot_general(hid, expert_tile(wd_buf, ft), NT_DIMS, preferred_element_type=f32)

    def moe_tasks(ft0, count):
        tasks = []
        for k0 in range(0, count, FPB):
            ks = range(k0, min(k0 + FPB, count))
            tasks += [lambda k=k, w=w: moe_up_task(ft0 + k, k, w) for k in ks for w in range(2)]
            tasks += [lambda k=k: moe_down_task(ft0 + k, k) for k in ks]
        return tasks

    def moe_finish():
        y = _round_bf16(y_acc[...])
        rsel = jnp.where(lax.broadcasted_iota(i32, (16, 1), 0) == 0, m1v, m2v)
        y = _round_bf16(y * _round_bf16(_sigmoid(rsel)))
        y = jnp.concatenate([y, jnp.zeros((16, DP - D), f32)], axis=1)
        y = jnp.concatenate([jnp.zeros((HT, DP), f32), y, jnp.zeros((T - HT - 16, DP), f32)], axis=0)
        y_t = jnp.concatenate([y.T[0:D], jnp.zeros((D, T), f32)], axis=1)
        y_u = _pack(y_t)[:, 0:T]
        lane = lax.broadcasted_iota(i32, (D // 2, T), 1)
        wot_u[:, DP - T:DP] = jnp.where(lane < HT, wot_u[:, DP - T:DP], y_u)
        rid = lax.broadcasted_iota(i32, (8, T), 0)
        for tt in range(TPS):
            tok_l = lax.broadcasted_iota(i32, (8, T), 1) + (NSEG - 1) * L + tt * T
            ots[tt][D:D + 8, :] = jnp.where(((rid == 0) & (tok_l == i1)) | ((rid == 1) & (tok_l == i2)), 1.0, 0.0)

    dense = _interleave(a_tasks((0, 0)), prep_dense(3, wot_u, 0))
    with _scope("p15_mix"):
        cut = (2 * len(dense)) // 3
        run(dense[:cut] + [select_task] + dense[cut:])

    for i in range(3):
        moe_wait(i)

    def out_tile(s, tt, last, chunk_copies=None):
        c0 = s * L + tt * T
        if not isinstance(s, int):
            c0 = pl.multiple_of(c0, T)
        o_bf = ots[tt][...].astype(bf16)
        nchunk = 4
        rows = D // nchunk
        for rc in range(nchunk):
            r0 = rc * rows
            attn = jnp.dot(_bf(wot_u[r0 // 2:(r0 + rows) // 2, :]), o_bf, preferred_element_type=f32)
            xn = _bf(xn_u[s * (L // LNW) + tt // BT, r0 // 2:(r0 + rows) // 2, (tt % BT) * T:(tt % BT + 1) * T]).astype(f32)
            x = x_buf[r0:r0 + rows, pl.ds(c0, T)].astype(f32)
            res = x + attn + xn
            out_buf[r0:r0 + rows, pl.ds(c0, T)] = res.astype(bf16)
            if chunk_copies is not None:
                chunk_copies[rc].start()

    def pair_tasks(ua, ub):
        tasks = []
        for x, y in zip(a_tasks(ua), b_tasks(ub)):
            tasks += [y, x]
        return tasks

    def seg_end(s, last):
        def by_qt(fn, unit, qt):
            return [lambda u=u: fn(unit, u, qt) for u in range(NP)]

        steps = []
        for step in range(7):
            lists = []
            if step < 4:
                lists.append(by_qt(stage_b, (s, 2), 3 - step))
                lists.append(by_qt(stage_a, (s, 3), 3 - step))
            if 1 <= step < 5:
                lists.append(by_qt(stage_b, (s, 3), 4 - step))
            if not last and 2 <= step < 6:
                lists.append(by_qt(stage_a, (s + 1, 0), 5 - step))
            if step >= 3:
                lists.append([lambda tt=6 - step: out_tile(s, tt, last)])
            steps.append(_interleave(*lists))
        return steps

    def seg_att(s, c):
        tasks = pair_tasks((s, 1), (s, 0)) + pair_tasks((s, 2), (s, 1))
        steps = seg_end(s, False)
        for step in steps[0:5]:
            tasks += step
        with _scope("att_seg"):
            run(_interleave(tasks, moe_tasks(s * FPI, FPI)))
            for step in steps[5:]:
                run(step)

        @pl.when(s < NSEG - 2)
        def _():
            out_copy(pl.multiple_of(s * L, L), L, s).start()
        return c

    lax.fori_loop(0, NSEG - 1, seg_att, 0)

    npatch = (NSEG - 1) * TPS

    def patch_tile(idx):
        return jnp.where(idx < npatch * T, idx // T, 0)

    tile0 = patch_tile(i1)
    tile1 = patch_tile(i2)
    tile1 = jnp.where(tile1 == tile0, (tile0 + 1) % npatch, tile1)

    def patch(tile):
        c0 = pl.multiple_of(tile * T, T)
        rid = lax.broadcasted_iota(i32, (T, T), 0)
        tok_l = lax.broadcasted_iota(i32, (T, T), 1) + c0
        hit = ((rid == HT) & (tok_l == i1)) | ((rid == HT + 1) & (tok_l == i2))
        onehot = jnp.where(hit, 1.0, 0.0).astype(bf16)
        for rc in range(4):
            r0, r1 = rc * (D // 4), (rc + 1) * (D // 4)
            upd = jnp.dot(_bf(wot_u[r0 // 2:r1 // 2, DP - T:DP]), onehot, preferred_element_type=f32)
            cur = out_buf[r0:r1, pl.ds(c0, T)].astype(f32)
            out_buf[r0:r1, pl.ds(c0, T)] = (cur + upd).astype(bf16)

    sent = (NSEG - 2) * TPS
    resend0 = jnp.where(tile0 < sent, tile0, jnp.where(tile1 == 0, 1, 0))
    resend1 = jnp.where(tile1 < sent, tile1, jnp.where(resend0 == 0, 1, 0))
    patch_copies = [out_copy(pl.multiple_of(resend0 * T, T), T, 7), out_copy(pl.multiple_of(resend1 * T, T), T, 8),
                    out_copy((NSEG - 2) * L, L, NSEG - 2)]
    last_copies = [out_copy((NSEG - 1) * L + tt * T, T, NSEG - 1 + tt) for tt in range(1, TPS)]
    c_fin = (NSEG - 1) * L
    final_copies = [
        pltpu.make_async_copy(out_buf.at[rc * (D // 4):(rc + 1) * (D // 4), c_fin:c_fin + T],
                              out_hbm.at[rc * (D // 4):(rc + 1) * (D // 4), c_fin:c_fin + T],
                              sems.at[SEM_FINAL + rc]) for rc in range(4)]

    sl = NSEG - 1
    for s in range(NSEG - 2):
        out_copy(s * L, L, s).wait()
    with _scope("tail_2"):
        moe_finish()
        run(pair_tasks((sl, 1), (sl, 0)))
        patch(tile0)
        patch(tile1)
        run(pair_tasks((sl, 2), (sl, 1)))
        for cp in patch_copies:
            cp.start()
        steps = seg_end(sl, True)
        for step in steps[0:5]:
            run(step)
        last_copies[2].start()
        last_copies[1].start()
    with _scope("tail_3"):
        run(steps[5])
        last_copies[0].start()
        out_tile(sl, 0, True, final_copies)

    with _scope("out_wait"):
        for cp in patch_copies + last_copies + final_copies:
            cp.wait()


@jax.jit
def pallas_parallel_sum__memory_aug_infini_attn__moe_arch_mod__prompt_kernel(
    A_x: jax.Array,
    A_wq: jax.Array,
    A_wk: jax.Array,
    A_wv: jax.Array,
    A_wo: jax.Array,
    A_beta: jax.Array,
    B_x: jax.Array,
    B_w_r: jax.Array,
    B_w_gate: jax.Array,
    B_w_up: jax.Array,
    B_w_down: jax.Array,
):
    del B_x
    any_spec = pl.BlockSpec(memory_space=pl.ANY)
    scratch = [
        pltpu.VMEM((H,), bf16),
        pltpu.VMEM((D,), bf16),
        pltpu.VMEM((D, SEQ), bf16),
        pltpu.VMEM((4, D, D), bf16),
        pltpu.VMEM((NFT, D, T), bf16),
        pltpu.VMEM((NFT, D, T), bf16),
        pltpu.VMEM((NFT, D, T), bf16),
        pltpu.VMEM((D, SEQ), bf16),
        pltpu.VMEM((WT_ALLOC, DP), u32),
        pltpu.VMEM((2, D // 2, LNW), u32),
        pltpu.VMEM((D // 2, DP), u32),
        pltpu.VMEM((SEQ // LNW, DP // 2, LNW), u32),
        pltpu.VMEM((DP // 2, LNW), u32),
        pltpu.VMEM((DP // 2, LNW), u32),
        pltpu.VMEM((NSEG, D // 2, L), u32),
        pltpu.VMEM((NSEG * NG, L // 2, T), u32),
        pltpu.VMEM((NSEG, D // 2, L), u32),
        pltpu.VMEM((NSEG, D // 2, L), u32),
        pltpu.VMEM((NSEG, D // 2, L), u32),
        pltpu.VMEM((NSEG * H, 16, L), u32),
        pltpu.VMEM((NSEG, 8, L), f32),
        pltpu.VMEM((NG, T, T), f32),
        pltpu.VMEM((NG, T, T), f32),
        pltpu.VMEM((NG, T, T), i32),
        pltpu.VMEM((NSEG, D, L), f32),
        pltpu.VMEM((NG, 8, T), f32),
        pltpu.VMEM((H, 8, T), f32),
        pltpu.VMEM((3, HT, T), f32),
        pltpu.VMEM((NP, 4, 2 * L, T), f32),
        pltpu.VMEM((NP, 4, 2, 8, T), f32),
        pltpu.VMEM((NP, 4, 2 * L, T), f32),
        pltpu.VMEM((NP, 4, 2, 8, T), f32),
        pltpu.VMEM((DP, T), f32),
        pltpu.VMEM((DP, T), f32),
        pltpu.VMEM((DP, T), f32),
        pltpu.VMEM((DP, T), f32),
        pltpu.VMEM((2, D, LNW), f32),
        pltpu.VMEM((2, 2, 8, LNW), f32),
        pltpu.VMEM((16, D), f32),
        pltpu.VMEM((8, DP), u32),
        pltpu.VMEM((FPI, 2, 16, T), f32),
        pltpu.SemaphoreType.DMA((NSEM,)),
    ]
    x_t = jnp.transpose(A_x, (0, 2, 1)).reshape(D, SEQ)
    out_t = pl.pallas_call(
        _kernel,
        out_shape=jax.ShapeDtypeStruct((D, SEQ), bf16),
        in_specs=[any_spec] * 10,
        out_specs=any_spec,
        scratch_shapes=scratch,
        compiler_params=pltpu.CompilerParams(vmem_limit_bytes=110 * 1024 * 1024),
    )(x_t, A_wq, A_wk, A_wv, A_wo, A_beta, B_w_r, B_w_gate, B_w_up, B_w_down.T)
    return jnp.transpose(out_t.reshape(1, D, SEQ), (0, 2, 1))
```

```python
import contextlib

import jax
import jax.numpy as jnp
from jax import lax
from jax.experimental import pallas as pl
from jax.experimental.pallas import tpu as pltpu

bf16 = jnp.bfloat16
f32 = jnp.float32
u32 = jnp.uint32
i32 = jnp.int32

SEQ = 2048
D = 576
DP = 640
H = 32
DH = 18
NSEG = 4
L = 512
T = 128
TW = T // 2
HT = T // 2
TPS = L // T
HPG = 6
NG = 6
F = 4608
FPI = 12
FPB = 3
NFT = F // T
NP = 4
UPS = H // (2 * NP)
NUNIT = NSEG * UPS
NT = SEQ // T
LNW = 256
BT = LNW // T
NORM_PARTS = 6
QK_BLOCK = 64
VB = 8 * DH

LOG2E = 1.4426950408889634
QSCALE = (DH ** -0.5) * LOG2E
MASKVAL = -1000000000.0 * LOG2E
EPS_BF16 = 1.0013580322265625e-05
ONES_PAIR = 0x3F803F80

NT_DIMS = (((1,), (1,)), ((), ()))

WT_Q = 0
WT_K = D // 2
WT_R = D
WT_V = D + 8
WT_ROWS = WT_V + D // 2
WT_ALLOC = 1056
NBLK = DP // T

X_PIECES = ((0, LNW), (LNW, LNW), (L, L), (2 * L, L), (3 * L, L))
SEM_X = 0
SEM_W = 5
SEM_MOE = 9
SEM_OUT = 12
SEM_SMALL = 21
SEM_WQB = 23
SEM_FINAL = 24
NSEM = 28
WQ_SPLIT = 2 * T


PROFILE_SCOPES = False
PACE = True
TAIL_BARRIERS = False
QT_ORDER = (3, 2, 1, 0)


def _scope(name):
    return jax.named_scope(name) if PROFILE_SCOPES else contextlib.nullcontext()


def _valid(g):
    return min(HPG * DH, D - g * HPG * DH)


def _ewin(g):
    start = (g * HPG * DH // 16) * 16
    return start, g * HPG * DH - start, min(T, D - start)


def _bf(x):
    return pltpu.bitcast(x, bf16)


def _pack(x):
    return pltpu.bitcast(x.astype(bf16), u32)


def _round_bf16(x):
    return x.astype(bf16).astype(f32)


def _phi(t):
    return jnp.where(t > 0, t + 1.0, jnp.exp(t))


def _sigmoid(t):
    return 1.0 / (1.0 + jnp.exp(-t))


def _zero_after(v):
    bits = pltpu.bitcast(v[0:8, 0:LNW], u32)
    sixteen = jnp.uint32(16)
    bits = lax.shift_right_logical(lax.shift_right_logical(bits, sixteen), sixteen)
    return pltpu.bitcast(bits, f32) if PACE else None


def _interleave(*lists):
    items = []
    for li, tasks in enumerate(lists):
        for k, t in enumerate(tasks):
            items.append(((k + 0.5) / len(tasks), li, k, t))
    items.sort(key=lambda it: it[:3])
    return [it[3] for it in items]


def _kernel(x_hbm, wq_hbm, wk_hbm, wv_hbm, wo_hbm, beta_hbm, wr_hbm, wg_hbm, wu_hbm, wd_hbm,
            out_hbm,
            beta_ref, wr_ref, x_buf, w_buf, wg_buf, wu_buf, wd_buf, out_buf,
            wt_u, kt_tmp, wot_u, xn_u, xs_a, xs_b, qs_u, k_u, pq_u, pk_u, vt_u, vwin,
            r_buf, mt_acc, lm_f, mcode, am, g16, omg, mb,
            s0, m0, s1, m1, ot0, ot1, ot2, ot3, xf, ln_stat, y_acc, xsel_buf, hid_buf, sems):

    def x_copy(i):
        c0, width = X_PIECES[i]
        return pltpu.make_async_copy(x_hbm.at[:, pl.ds(c0, width)], x_buf.at[:, pl.ds(c0, width)],
                                     sems.at[SEM_X + i])

    def w_copy(i):
        src = (wq_hbm, wk_hbm, wv_hbm, wo_hbm)[i]
        return pltpu.make_async_copy(src, w_buf.at[i], sems.at[SEM_W + i])

    wq_first = pltpu.make_async_copy(wq_hbm.at[:, 0:WQ_SPLIT], w_buf.at[0, :, 0:WQ_SPLIT], sems.at[SEM_W])
    wq_rest = pltpu.make_async_copy(wq_hbm.at[:, WQ_SPLIT:D], w_buf.at[0, :, WQ_SPLIT:D], sems.at[SEM_WQB])

    moe_src = (wg_hbm, wu_hbm, wd_hbm)
    moe_dst = (wg_buf, wu_buf, wd_buf)

    def moe_start(i, ft):
        c0 = ft * T if isinstance(ft, int) else pl.multiple_of(ft * T, T)
        pltpu.make_async_copy(moe_src[i].at[:, pl.ds(c0, T)], moe_dst[i].at[ft], sems.at[SEM_MOE + i]).start()

    def moe_issue(first, last):
        for n in range(first, last):
            moe_start(n % 3, n // 3)

    def moe_wait(i):
        pltpu.make_async_copy(moe_dst[i], moe_dst[i], sems.at[SEM_MOE + i]).wait()

    def out_copy(c0, width, sem):
        return pltpu.make_async_copy(out_buf.at[:, pl.ds(c0, width)], out_hbm.at[:, pl.ds(c0, width)],
                                     sems.at[SEM_OUT + sem])

    small_copies = [pltpu.make_async_copy(beta_hbm, beta_ref, sems.at[SEM_SMALL]),
                    pltpu.make_async_copy(wr_hbm, wr_ref, sems.at[SEM_SMALL + 1])]
    x_copy(0).start()
    wq_first.start()
    wq_rest.start()
    x_copy(1).start()
    for cp in small_copies:
        cp.start()
    w_copy(1).start()
    w_copy(2).start()

    init_scope = _scope("init")
    init_scope.__enter__()
    kr = lax.broadcasted_iota(i32, (HT, T), 0)
    ql = lax.broadcasted_iota(i32, (HT, T), 1)
    mb[0] = jnp.where(ql < kr, MASKVAL, 0.0).astype(f32)
    mb[1] = jnp.where((ql >= HT) & (ql - HT < kr), MASKVAL, 0.0).astype(f32)
    mb[2] = jnp.where(ql % HT < kr, MASKVAL, 0.0).astype(f32)
    zpad = jnp.zeros(((DP - D) // 2, LNW), u32)
    for blk in range(SEQ // LNW):
        xn_u[blk, D // 2:DP // 2, :] = zpad
    xs_a[D // 2:DP // 2, :] = zpad
    xs_b[D // 2:DP // 2, :] = zpad
    ots = (ot0, ot1, ot2, ot3)
    for o_ref in ots:
        o_ref[D:DP, :] = jnp.zeros((DP - D, T), f32)
    am[0] = jnp.zeros(am.shape[1:], f32)
    mt_acc[...] = jnp.zeros(mt_acc.shape, f32)
    g16[...] = jnp.zeros(g16.shape, f32)

    init_scope.__exit__(None, None, None)

    pace = [None]

    def gate_tables():
        gate = _round_bf16(_sigmoid(beta_ref[...].reshape(1, H).astype(f32)))
        for h in range(H):
            gh = jnp.broadcast_to(gate[:, h:h + 1], (1, T))
            omg[h] = jnp.broadcast_to(_round_bf16(1.0 - gh), (8, T))
            g16[h // HPG, (h % HPG):(h % HPG) + 1, :] = gh

    def transpose_block(i, cb):
        c1 = min((cb + 1) * T, D)
        blk = w_buf[i, :, cb * T:c1]
        if c1 - cb * T < T:
            blk = jnp.concatenate([blk, jnp.zeros((D, T - (c1 - cb * T)), bf16)], axis=1)
        blk = jnp.concatenate([blk, jnp.zeros((DP - D, T), bf16)], axis=0)
        return pltpu.bitcast(blk.T, u32)

    def prep_dense(i, dst, base):
        def task(cb):
            nrow = min(TW, D // 2 - cb * TW)
            dst[base + cb * TW:base + cb * TW + nrow, :] = transpose_block(i, cb)[0:nrow]
        return [lambda cb=cb: task(cb) for cb in range(DP // T)]

    def router_row():
        wr = wr_ref[...].reshape(1, D).astype(f32)
        wr = jnp.concatenate([wr, jnp.zeros((1, DP - D), f32)], axis=1)
        bits = lax.shift_right_logical(pltpu.bitcast(wr, u32), u32(16))
        rid = lax.broadcasted_iota(i32, (8, DP), 0)
        wt_u[WT_R:WT_R + 8, :] = jnp.where(rid == 0, bits, u32(0))

    def ln_tasks(s, p, stage):
        c0 = s * L + p * LNW
        if not isinstance(s, int):
            c0 = pl.multiple_of(c0, LNW)

        def mean_pass():
            acc = pace[0]
            for r in range(0, D, 64):
                x = x_buf[r:r + 64, pl.ds(c0, LNW)].astype(f32)
                xf[p, r:r + 64, :] = x
                part = jnp.sum(x.reshape(8, 8, LNW), axis=0)
                acc = part if acc is None else acc + part
            mean = jnp.sum(acc, axis=0, keepdims=True) / D
            ln_stat[p, 0] = jnp.broadcast_to(mean, (8, LNW))

        def var_pass():
            mean = ln_stat[p, 0][0:1]
            if pace[0] is not None:
                mean = mean + pace[0][0:1]
            acc = None
            for r in range(0, D, 96):
                xc = xf[p, r:r + 96, :] - mean
                part = jnp.sum((xc * xc).reshape(12, 8, LNW), axis=0)
                acc = part if acc is None else acc + part
            var = jnp.sum(acc, axis=0, keepdims=True) / D
            den = _round_bf16(jnp.sqrt(_round_bf16(_round_bf16(var) + EPS_BF16)))
            ln_stat[p, 1] = jnp.broadcast_to(1.0 / den, (8, LNW))
            ln_stat[p, 0] = jnp.broadcast_to(_round_bf16(mean), (8, LNW))

        def norm_pass(part):
            mean_b = ln_stat[p, 0][0:1]
            if pace[0] is not None:
                mean_b = mean_b + pace[0][0:1]
            inv = ln_stat[p, 1][0:1]
            step = D // NORM_PARTS
            for r in range(part * step, (part + 1) * step, 48):
                xn = _pack(_round_bf16(xf[p, r:r + 48, :] - mean_b) * inv)
                xn_u.at[s * (L // LNW) + p][r // 2:r // 2 + 24, :] = xn
                if stage is not None:
                    stage[r // 2:r // 2 + 24, :] = xn

        return [mean_pass, var_pass] + [lambda part=part: norm_pass(part) for part in range(NORM_PARTS)]

    def load_xs(s, p, stage):
        return _bf(xn_u[s * (L // LNW) + p] if stage is None else stage[...])

    def row_blocks(size):
        return [(r, min(r + size, D)) for r in range(0, D, size)]

    def q_task(s, p, stage, r0, r1):
        rows = slice(r0 // 2, r1 // 2)
        cols = slice(p * LNW, (p + 1) * LNW)
        w = _bf(wt_u[WT_Q + r0 // 2:WT_Q + r1 // 2, :])
        q = jnp.dot(w, load_xs(s, p, stage), preferred_element_type=f32)
        pace[0] = _zero_after(q)
        qs = q * QSCALE
        qrot = jnp.concatenate([pltpu.roll(qs[:, t * T:(t + 1) * T], HT, 1) for t in range(BT)], axis=1)
        rid = lax.broadcasted_iota(i32, qs.shape, 0) + r0
        even = ((rid // DH) % 2) == 0
        qs_u.at[s][rows, cols] = _pack(jnp.where(even, qrot, qs))
        pq_u.at[s][rows, cols] = _pack(_phi(q))

    def k_task(s, p, stage, r0, r1):
        rows = slice(r0 // 2, r1 // 2)
        cols = slice(p * LNW, (p + 1) * LNW)
        extra = 8 if r1 == D else 0
        w = _bf(wt_u[WT_K + r0 // 2:WT_K + r1 // 2 + extra, :])
        k = jnp.dot(w, load_xs(s, p, stage), preferred_element_type=f32)
        pace[0] = _zero_after(k)
        if extra:
            r_buf[s, :, cols] = jnp.broadcast_to(k[r1 - r0:r1 - r0 + 1, :], (8, LNW))
            k = k[0:r1 - r0]
        kt_tmp.at[p][rows, :] = _pack(k)
        pk_u.at[s][rows, cols] = _pack(_phi(k))

    def kt_task(s, p, g):
        nv = _valid(g) // 2
        src = g * HPG * DH // 2
        kg = jnp.concatenate([kt_tmp[p, src:src + nv, :], jnp.zeros((TW - nv, LNW), u32)], axis=0)
        k_u.at[s * NG + g][p * (LNW // 2):(p + 1) * (LNW // 2), :] = pltpu.bitcast(_bf(kg).T, u32)

    def v_task(s, p, stage, b):
        cols = slice(p * LNW, (p + 1) * LNW)
        w = _bf(wt_u[WT_V + b * (VB // 2):WT_V + (b + 1) * (VB // 2), :])
        v = jnp.dot(w, load_xs(s, p, stage), preferred_element_type=f32)
        pace[0] = _zero_after(v)
        v = _pack(v)
        vt_u.at[s][b * (VB // 2):(b + 1) * (VB // 2), cols] = v
        sub = lax.broadcasted_iota(i32, (16, LNW), 0)
        for hh in range(8):
            w8 = (9 * hh) // 8
            ones_row = 0 if 2 * hh == 14 else 15
            vwin.at[s * H + 8 * b + hh][:, cols] = jnp.where(sub == ones_row, u32(ONES_PAIR), v[8 * w8:8 * w8 + 16, :])

    def q_tasks(s, p, stage=None, size=QK_BLOCK):
        return [lambda b=b: q_task(s, p, stage, *b) for b in row_blocks(size)]

    def k_tasks(s, p, stage=None, size=QK_BLOCK):
        tasks, done = [], 0
        for b in row_blocks(size):
            tasks.append(lambda b=b: k_task(s, p, stage, *b))
            while done < NG and done * HPG * DH + _valid(done) <= b[1]:
                tasks.append(lambda g=done: kt_task(s, p, g))
                done += 1
        return tasks

    def v_tasks(s, p, stage=None):
        return [lambda b=b: v_task(s, p, stage, b) for b in range(D // VB)]

    def mem_layout(g):
        es, eoff, _ = _ewin(g)
        nv = _valid(g)
        ne = -(-(eoff + nv) // 16) * 16
        ones_row = 0 if eoff >= 2 else eoff + nv
        nh = nv // DH
        den_row = 0 if eoff >= nh else ne
        return es, eoff, nv, ne, ones_row, den_row, max(ne, den_row + 16 * (den_row > 0))

    def mem_update(sp, g):
        es, eoff, nv, ne, ones_row, den_row, nr = mem_layout(g)
        nw = min(T, D - es)
        win = vt_u[sp, es // 2:(es + ne) // 2, :]
        wid = lax.broadcasted_iota(i32, win.shape, 0)
        lhs = _bf(jnp.where(wid == ones_row // 2, u32(ONES_PAIR), win))
        upd = lax.dot_general(lhs, _bf(pk_u[sp, es // 2:(es + nw) // 2, :]), NT_DIMS, preferred_element_type=f32)
        mt = mt_acc[g, 0:ne, 0:nw] + upd
        mt_acc[g, 0:ne, 0:nw] = mt
        z = jnp.broadcast_to(mt[ones_row:ones_row + 1, :], (nr, nw))
        if nr > ne:
            mt = jnp.concatenate([mt, jnp.zeros((nr - ne, nw), f32)], axis=0)
        code = mcode[g, 0:nr, 0:nw]
        lm_f[g, 0:nr, 0:nw] = jnp.where(code == 1, mt, jnp.where(code == 2, z, 0.0))

    def mem_masks():
        for g in range(NG):
            es, eoff, nv, ne, ones_row, den_row, nr = mem_layout(g)
            row = lax.broadcasted_iota(i32, (T, T), 0)
            d_loc = lax.broadcasted_iota(i32, (T, T), 1) - eoff
            e_loc = row - eoff
            d_ok = (d_loc >= 0) & (d_loc < nv)
            same_head = (e_loc >= 0) & (e_loc < nv) & d_ok & ((e_loc // DH) == (d_loc // DH))
            den_hit = (row >= den_row) & d_ok & ((d_loc // DH) == row - den_row)
            mcode[g] = jnp.where(same_head, 1, jnp.where(den_hit, 2, 0))

    def mem_retrieve(s, g):
        es, eoff, nv, ne, ones_row, den_row, nr = mem_layout(g)
        nw = min(T, D - es)
        nd = jnp.dot(lm_f[g, 0:nr, 0:nw].astype(bf16), _bf(pq_u[s, es // 2:(es + nw) // 2, :]),
                     preferred_element_type=f32)
        scale = jnp.broadcast_to(g16[g][:, 0:1], (8, L)) / (nd[den_row:den_row + 8, :] + 1e-6)
        r8 = lax.broadcasted_iota(i32, (8, L), 0)
        for b in range(ne // 8):
            lo, hi = 8 * b - eoff, 8 * b + 7 - eoff
            if hi < 0 or lo >= nv:
                continue
            j1, j2 = max(lo, 0) // DH, min(hi, nv - 1) // DH
            sc = jnp.broadcast_to(scale[j1:j1 + 1, :], (8, L))
            if j2 != j1:
                sc = jnp.where(r8 < DH * j2 - lo, sc, jnp.broadcast_to(scale[j2:j2 + 1, :], (8, L)))
            val = nd[8 * b:8 * b + 8, :] * sc
            dst = am.at[s, es + 8 * b:es + 8 * b + 8, :]
            if lo >= 0 and hi < nv:
                dst[...] = val
            else:
                pltpu.store(dst, val, mask=(r8 + lo >= 0) & (r8 + lo < nv))

    def run(tasks):
        for t in tasks:
            t()

    prep_q = prep_dense(0, wt_u, WT_Q)
    q0a = q_tasks(0, 0, None, T)
    with _scope("p1_wait_x0"):
        x_copy(0).wait()
    for i in range(2, len(X_PIECES)):
        x_copy(i).start()
    w_copy(3).start()
    moe_issue(0, 48)
    with _scope("p1_ln0a"):
        run(ln_tasks(0, 0, None))
        wq_first.wait()
    with _scope("p1_q0a_first"):
        run(prep_q[0:2] + q0a[0:2])
        wq_rest.wait()
        x_copy(1).wait()
    with _scope("p1_q0a"):
        run(prep_q[2:])
        run(_interleave(q0a[2:], ln_tasks(0, 1, None)))
        w_copy(1).wait()
        for cp in small_copies:
            cp.wait()
    k0a, k0b = k_tasks(0, 0), k_tasks(0, 1)
    with _scope("p1_q0b"):
        run(_interleave(q_tasks(0, 1), prep_dense(1, wt_u, WT_K), [router_row, gate_tables, mem_masks]))
        run([lambda b=b: k_task(0, 0, None, *b) for b in row_blocks(QK_BLOCK)])
        w_copy(2).wait()
        x_copy(2).wait()
    moe_issue(48, 60)
    with _scope("p1_k0v0"):
        run(_interleave(k0b, prep_dense(2, wt_u, WT_V), [lambda g=g: kt_task(0, 0, g) for g in range(NG)]))
        run(_interleave(v_tasks(0, 0) + v_tasks(0, 1), ln_tasks(1, 0, xs_a)))

    moe_issue(60, 72)

    def seg_body(s, c):
        for ss in range(2, NSEG):
            @pl.when(s + 1 == ss)
            def _():
                x_copy(ss + 1).wait()
                if ss == NSEG - 1:
                    moe_issue(72, 3 * NFT)
        nxt = jnp.minimum(s + 1, NSEG - 1)
        pace[0] = None
        with _scope("p1_seg"):
            updates = [lambda g=g: mem_update(s - 1, g) for g in range(NG)]
            retrieves = [lambda g=g: mem_retrieve(s, g) for g in range(NG)]
            first = _interleave(q_tasks(s, 0, xs_a), updates) + k_tasks(s, 0, xs_a) + v_tasks(s, 0, xs_a)
            run(_interleave(first, ln_tasks(s, 1, xs_b)))
            second = q_tasks(s, 1, xs_b) + _interleave(k_tasks(s, 1, xs_b) + v_tasks(s, 1, xs_b), retrieves)
            run(_interleave(second, ln_tasks(nxt, 0, xs_a)))
        return c

    lax.fori_loop(1, NSEG, seg_body, 0)

    bufs = ((s0, m0), (s1, m1))
    lane64 = lax.broadcasted_iota(i32, (TW, T), 1)
    lane1 = lax.broadcasted_iota(i32, (1, T), 1)
    lane8 = lax.broadcasted_iota(i32, (8, T), 1)

    def pair_weights(s, pi, qt):
        hw = DH // 2
        j = 2 * (pi % (HPG // 2))
        src, dst = hw * 2 * pi, hw * j
        a0, t0 = (src // 8) * 8, (dst // 8) * 8
        nrow = min(32, D // 2 - a0)
        part = qs_u[s, a0:a0 + nrow, qt * T:(qt + 1) * T]
        if nrow < 32:
            part = jnp.concatenate([part, jnp.zeros((32 - nrow, T), u32)], axis=0)
        shift = (dst - t0) - (src - a0)
        if shift:
            part = pltpu.roll(part, shift % 32, 0)
        rid = lax.broadcasted_iota(i32, (32, T), 0) + t0
        out = []
        for lo in (dst, dst + hw):
            piece = jnp.where((rid >= lo) & (rid < lo + hw), part, u32(0))
            piece = piece[0:min(32, TW - t0)]
            pieces = [jnp.zeros((t0, T), u32)] * (t0 > 0) + [piece] + [jnp.zeros((TW - t0 - 32, T), u32)] * (t0 + 32 < TW)
            out.append(jnp.concatenate(pieces, axis=0))
        return out

    def stage_a(unit, u, qt):
        s, k = unit
        s_ref, m_ref = bufs[k % 2]
        pi = k * NP + u
        g = pi // (HPG // 2)
        sg = s * NG + g
        n = T * (qt + 1)
        w_a, w_b = pair_weights(s, pi, qt)
        w_ab = _bf(jnp.where(lane64 < HT, w_a, w_b))

        def colmax8(v):
            return jnp.max(v.reshape(v.shape[0] // 8, 8, T), axis=0)

        maxes = []
        for hd, w in enumerate((_bf(w_a), _bf(w_b))):
            m8 = None
            for c in range(qt):
                kc = _bf(k_u[sg, c * TW:(c + 1) * TW, :])
                sc = jnp.dot(kc, w, preferred_element_type=f32)
                s_ref[u, qt, hd * L + c * T:hd * L + (c + 1) * T, :] = sc
                m8 = colmax8(sc) if m8 is None else jnp.maximum(m8, colmax8(sc))
            kc = _bf(k_u[sg, qt * TW:qt * TW + TW // 2, :])
            sc = jnp.dot(kc, w, preferred_element_type=f32) + mb[1 - hd]
            s_ref[u, qt, hd * L + qt * T:hd * L + qt * T + HT, :] = sc
            m8 = colmax8(sc) if m8 is None else jnp.maximum(m8, colmax8(sc))
            maxes.append(m8)
        kc = _bf(k_u[sg, qt * TW + TW // 2:(qt + 1) * TW, :])
        sc = jnp.dot(kc, w_ab, preferred_element_type=f32) + mb[2]
        s_ref[u, qt, n - HT:n, :] = sc
        mab = colmax8(sc)
        m_a = jnp.where(lane8 < HT, jnp.maximum(maxes[0], mab), maxes[0])
        m_b = jnp.where(lane8 >= HT, jnp.maximum(maxes[1], mab), maxes[1])
        m_ref[u, qt, 0] = jnp.broadcast_to(jnp.max(m_a, axis=0, keepdims=True), (8, T))
        m_ref[u, qt, 1] = jnp.broadcast_to(jnp.max(m_b, axis=0, keepdims=True), (8, T))

    def stage_b(unit, u, qt):
        s, k = unit
        s_ref, m_ref = bufs[k % 2]
        pi = k * NP + u
        n = T * (qt + 1)
        m_a = m_ref[u, qt, 0][0:1]
        m_b = m_ref[u, qt, 1][0:1]
        p_ab = jnp.exp2(s_ref[u, qt, n - HT:n, :] - jnp.where(lane1 < HT, m_a, m_b))
        for hd, m in enumerate((m_a, m_b)):
            h = 2 * pi + hd
            p = jnp.exp2(s_ref[u, qt, hd * L:hd * L + n - HT, :] - m)
            keep = (lane64 < HT) if hd == 0 else (lane64 >= HT)
            p = jnp.concatenate([p, jnp.where(keep, p_ab, 0.0)], axis=0).astype(bf16)
            w0 = ((DH * h) // 16) * 16
            off = DH * h - w0
            o = jnp.dot(_bf(vwin[s * H + h, :, 0:n]), p, preferred_element_type=f32)
            den = o[0:1] if off == 14 else o[31:32]
            r0, r1 = (off // 8) * 8, -(-(off + DH) // 8) * 8
            o = o[r0:r1] * (omg[h][0:1] / den)
            if hd == 0:
                o = pltpu.roll(o, HT, 1)
            res = am[s, w0 + r0:w0 + r1, qt * T:(qt + 1) * T] + o
            rid = lax.broadcasted_iota(i32, (r1 - r0, T), 0) + r0
            pltpu.store(ots[qt].at[w0 + r0:w0 + r1, :], res, mask=(rid >= off) & (rid < off + DH))

    def a_tasks(unit):
        return [lambda u=u, qt=qt: stage_a(unit, u, qt) for u in range(NP) for qt in QT_ORDER]

    def b_tasks(unit):
        return [lambda u=u, qt=qt: stage_b(unit, u, qt) for u in range(NP) for qt in QT_ORDER]

    w_copy(3).wait()
    rr = jnp.concatenate([r_buf[s][0:1, :] for s in range(NSEG)], axis=0)
    rr = _round_bf16(rr)
    tok = lax.broadcasted_iota(i32, (NSEG, L), 0) * L + lax.broadcasted_iota(i32, (NSEG, L), 1)
    m1v = jnp.max(rr)
    i1 = jnp.min(jnp.where(rr == m1v, tok, SEQ))
    rr2 = jnp.where(tok == i1, -jnp.inf, rr)
    m2v = jnp.max(rr2)
    i2 = jnp.min(jnp.where(rr2 == m2v, tok, SEQ))
    i1 = jnp.clip(i1, 0, SEQ - 1)
    i2 = jnp.clip(i2, 0, SEQ - 1)

    row16 = lax.broadcasted_iota(i32, (16, T), 0)
    lane16 = lax.broadcasted_iota(i32, (16, T), 1)

    def token_rows(i, slot):
        onehot = jnp.where((row16 == slot) & (lane16 == i % T), 1.0, 0.0).astype(bf16)
        return lax.dot_general(onehot, _bf(xn_u[i // LNW, :, pl.ds(pl.multiple_of(((i // T) % BT) * T, T), T)]), NT_DIMS, preferred_element_type=f32)

    def select_task():
        xsel_buf[...] = _pack(token_rows(i1, 0) + token_rows(i2, 1))
        y_acc[...] = jnp.zeros(y_acc.shape, f32)

    def expert_tile(w_ref, ft):
        return _bf(w_ref.at[ft].bitcast(u32)[...])

    def moe_up_task(ft, k, which):
        xsel = _bf(xsel_buf[:, 0:D])
        w_ref = (wg_buf, wu_buf)[which]
        hid_buf[k, which] = jnp.dot(xsel, expert_tile(w_ref, ft), preferred_element_type=f32)

    def moe_down_task(ft, k):
        gt = _round_bf16(hid_buf[k, 0])
        up = _round_bf16(hid_buf[k, 1])
        hid = (_round_bf16(gt * _sigmoid(gt)) * up).astype(bf16)
        y_acc[...] += lax.dot_general(hid, expert_tile(wd_buf, ft), NT_DIMS, preferred_element_type=f32)

    def moe_tasks(ft0, count):
        tasks = []
        for k0 in range(0, count, FPB):
            ks = range(k0, min(k0 + FPB, count))
            tasks += [lambda k=k, w=w: moe_up_task(ft0 + k, k, w) for k in ks for w in range(2)]
            tasks += [lambda k=k: moe_down_task(ft0 + k, k) for k in ks]
        return tasks

    def moe_finish():
        y = _round_bf16(y_acc[...])
        rsel = jnp.where(lax.broadcasted_iota(i32, (16, 1), 0) == 0, m1v, m2v)
        y = _round_bf16(y * _round_bf16(_sigmoid(rsel)))
        y = jnp.concatenate([y, jnp.zeros((16, DP - D), f32)], axis=1)
        y = jnp.concatenate([jnp.zeros((HT, DP), f32), y, jnp.zeros((T - HT - 16, DP), f32)], axis=0)
        y_t = jnp.concatenate([y.T[0:D], jnp.zeros((D, T), f32)], axis=1)
        y_u = _pack(y_t)[:, 0:T]
        lane = lax.broadcasted_iota(i32, (D // 2, T), 1)
        wot_u[:, DP - T:DP] = jnp.where(lane < HT, wot_u[:, DP - T:DP], y_u)
        rid = lax.broadcasted_iota(i32, (8, T), 0)
        for tt in range(TPS):
            tok_l = lax.broadcasted_iota(i32, (8, T), 1) + (NSEG - 1) * L + tt * T
            ots[tt][D:D + 8, :] = jnp.where(((rid == 0) & (tok_l == i1)) | ((rid == 1) & (tok_l == i2)), 1.0, 0.0)

    dense = _interleave(a_tasks((0, 0)), prep_dense(3, wot_u, 0))
    with _scope("p15_mix"):
        cut = (2 * len(dense)) // 3
        run(dense[:cut] + [select_task] + dense[cut:])

    for i in range(3):
        moe_wait(i)

    def out_tile(s, tt, last, chunk_copies=None):
        c0 = s * L + tt * T
        if not isinstance(s, int):
            c0 = pl.multiple_of(c0, T)
        o_bf = ots[tt][...].astype(bf16)
        nchunk = 4
        rows = D // nchunk
        for rc in range(nchunk):
            r0 = rc * rows
            attn = jnp.dot(_bf(wot_u[r0 // 2:(r0 + rows) // 2, :]), o_bf, preferred_element_type=f32)
            xn = _bf(xn_u[s * (L // LNW) + tt // BT, r0 // 2:(r0 + rows) // 2, (tt % BT) * T:(tt % BT + 1) * T]).astype(f32)
            x = x_buf[r0:r0 + rows, pl.ds(c0, T)].astype(f32)
            res = x + attn + xn
            out_buf[r0:r0 + rows, pl.ds(c0, T)] = res.astype(bf16)
            if chunk_copies is not None:
                chunk_copies[rc].start()

    def pair_tasks(ua, ub):
        tasks = []
        for x, y in zip(a_tasks(ua), b_tasks(ub)):
            tasks += [y, x]
        return tasks

    def seg_end(s, last):
        def by_qt(fn, unit, qt):
            return [lambda u=u: fn(unit, u, qt) for u in range(NP)]

        steps = []
        for step in range(7):
            lists = []
            if step < 4:
                lists.append(by_qt(stage_b, (s, 2), 3 - step))
                lists.append(by_qt(stage_a, (s, 3), 3 - step))
            if 1 <= step < 5:
                lists.append(by_qt(stage_b, (s, 3), 4 - step))
            if not last and 2 <= step < 6:
                lists.append(by_qt(stage_a, (s + 1, 0), 5 - step))
            if step >= 3:
                lists.append([lambda tt=6 - step: out_tile(s, tt, last)])
            steps.append(_interleave(*lists))
        return steps

    def seg_att(s, c):
        tasks = pair_tasks((s, 1), (s, 0)) + pair_tasks((s, 2), (s, 1))
        steps = seg_end(s, False)
        for step in steps[0:5]:
            tasks += step
        with _scope("att_seg"):
            run(_interleave(tasks, moe_tasks(s * FPI, FPI)))
            for step in steps[5:]:
                run(step)

        @pl.when(s < NSEG - 2)
        def _():
            out_copy(pl.multiple_of(s * L, L), L, s).start()
        return c

    lax.fori_loop(0, NSEG - 1, seg_att, 0)

    npatch = (NSEG - 1) * TPS

    def patch_tile(idx):
        return jnp.where(idx < npatch * T, idx // T, 0)

    tile0 = patch_tile(i1)
    tile1 = patch_tile(i2)
    tile1 = jnp.where(tile1 == tile0, (tile0 + 1) % npatch, tile1)

    def patch(tile):
        c0 = pl.multiple_of(tile * T, T)
        rid = lax.broadcasted_iota(i32, (T, T), 0)
        tok_l = lax.broadcasted_iota(i32, (T, T), 1) + c0
        hit = ((rid == HT) & (tok_l == i1)) | ((rid == HT + 1) & (tok_l == i2))
        onehot = jnp.where(hit, 1.0, 0.0).astype(bf16)
        for rc in range(4):
            r0, r1 = rc * (D // 4), (rc + 1) * (D // 4)
            upd = jnp.dot(_bf(wot_u[r0 // 2:r1 // 2, DP - T:DP]), onehot, preferred_element_type=f32)
            cur = out_buf[r0:r1, pl.ds(c0, T)].astype(f32)
            out_buf[r0:r1, pl.ds(c0, T)] = (cur + upd).astype(bf16)

    sent = (NSEG - 2) * TPS
    resend0 = jnp.where(tile0 < sent, tile0, jnp.where(tile1 == 0, 1, 0))
    resend1 = jnp.where(tile1 < sent, tile1, jnp.where(resend0 == 0, 1, 0))
    patch_copies = [out_copy(pl.multiple_of(resend0 * T, T), T, 7), out_copy(pl.multiple_of(resend1 * T, T), T, 8),
                    out_copy((NSEG - 2) * L, L, NSEG - 2)]
    last_copies = [out_copy((NSEG - 1) * L + tt * T, T, NSEG - 1 + tt) for tt in range(1, TPS)]
    c_fin = (NSEG - 1) * L
    final_copies = [
        pltpu.make_async_copy(out_buf.at[rc * (D // 4):(rc + 1) * (D // 4), c_fin:c_fin + T],
                              out_hbm.at[rc * (D // 4):(rc + 1) * (D // 4), c_fin:c_fin + T],
                              sems.at[SEM_FINAL + rc]) for rc in range(4)]

    sl = NSEG - 1
    for s in range(NSEG - 2):
        out_copy(s * L, L, s).wait()
    with _scope("tail_2"):
        moe_finish()
        run(pair_tasks((sl, 1), (sl, 0)))
        patch(tile0)
        patch(tile1)
        run(pair_tasks((sl, 2), (sl, 1)))
        for cp in patch_copies:
            cp.start()
        steps = seg_end(sl, True)
        for step in steps[0:5]:
            run(step)
        last_copies[2].start()
        last_copies[1].start()
    with _scope("tail_3"):
        run(steps[5])
        last_copies[0].start()
        out_tile(sl, 0, True, final_copies)

    with _scope("out_wait"):
        for cp in patch_copies + last_copies + final_copies:
            cp.wait()


@jax.jit
def pallas_parallel_sum__memory_aug_infini_attn__moe_arch_mod__prompt_kernel(
    A_x: jax.Array,
    A_wq: jax.Array,
    A_wk: jax.Array,
    A_wv: jax.Array,
    A_wo: jax.Array,
    A_beta: jax.Array,
    B_x: jax.Array,
    B_w_r: jax.Array,
    B_w_gate: jax.Array,
    B_w_up: jax.Array,
    B_w_down: jax.Array,
):
    del B_x
    any_spec = pl.BlockSpec(memory_space=pl.ANY)
    scratch = [
        pltpu.VMEM((H,), bf16),
        pltpu.VMEM((D,), bf16),
        pltpu.VMEM((D, SEQ), bf16),
        pltpu.VMEM((4, D, D), bf16),
        pltpu.VMEM((NFT, D, T), bf16),
        pltpu.VMEM((NFT, D, T), bf16),
        pltpu.VMEM((NFT, D, T), bf16),
        pltpu.VMEM((D, SEQ), bf16),
        pltpu.VMEM((WT_ALLOC, DP), u32),
        pltpu.VMEM((2, D // 2, LNW), u32),
        pltpu.VMEM((D // 2, DP), u32),
        pltpu.VMEM((SEQ // LNW, DP // 2, LNW), u32),
        pltpu.VMEM((DP // 2, LNW), u32),
        pltpu.VMEM((DP // 2, LNW), u32),
        pltpu.VMEM((NSEG, D // 2, L), u32),
        pltpu.VMEM((NSEG * NG, L // 2, T), u32),
        pltpu.VMEM((NSEG, D // 2, L), u32),
        pltpu.VMEM((NSEG, D // 2, L), u32),
        pltpu.VMEM((NSEG, D // 2, L), u32),
        pltpu.VMEM((NSEG * H, 16, L), u32),
        pltpu.VMEM((NSEG, 8, L), f32),
        pltpu.VMEM((NG, T, T), f32),
        pltpu.VMEM((NG, T, T), f32),
        pltpu.VMEM((NG, T, T), i32),
        pltpu.VMEM((NSEG, D, L), f32),
        pltpu.VMEM((NG, 8, T), f32),
        pltpu.VMEM((H, 8, T), f32),
        pltpu.VMEM((3, HT, T), f32),
        pltpu.VMEM((NP, 4, 2 * L, T), f32),
        pltpu.VMEM((NP, 4, 2, 8, T), f32),
        pltpu.VMEM((NP, 4, 2 * L, T), f32),
        pltpu.VMEM((NP, 4, 2, 8, T), f32),
        pltpu.VMEM((DP, T), f32),
        pltpu.VMEM((DP, T), f32),
        pltpu.VMEM((DP, T), f32),
        pltpu.VMEM((DP, T), f32),
        pltpu.VMEM((2, D, LNW), f32),
        pltpu.VMEM((2, 2, 8, LNW), f32),
        pltpu.VMEM((16, D), f32),
        pltpu.VMEM((8, DP), u32),
        pltpu.VMEM((FPI, 2, 16, T), f32),
        pltpu.SemaphoreType.DMA((NSEM,)),
    ]
    x_t = jnp.transpose(A_x, (0, 2, 1)).reshape(D, SEQ)
    out_t = pl.pallas_call(
        _kernel,
        out_shape=jax.ShapeDtypeStruct((D, SEQ), bf16),
        in_specs=[any_spec] * 10,
        out_specs=any_spec,
        scratch_shapes=scratch,
        compiler_params=pltpu.CompilerParams(vmem_limit_bytes=110 * 1024 * 1024),
    )(x_t, A_wq, A_wk, A_wv, A_wo, A_beta, B_w_r, B_w_gate, B_w_up, B_w_down.T)
    return jnp.transpose(out_t.reshape(1, D, SEQ), (0, 2, 1))
```

```python
import contextlib

import jax
import jax.numpy as jnp
from jax import lax
from jax.experimental import pallas as pl
from jax.experimental.pallas import tpu as pltpu

bf16 = jnp.bfloat16
f32 = jnp.float32
u32 = jnp.uint32
i32 = jnp.int32

SEQ = 2048
D = 576
DP = 640
H = 32
DH = 18
NSEG = 4
L = 512
T = 128
TW = T // 2
HT = T // 2
TPS = L // T
HPG = 6
NG = 6
F = 4608
FPI = 12
FPB = 3
NFT = F // T
NP = 4
UPS = H // (2 * NP)
NUNIT = NSEG * UPS
NT = SEQ // T
LNW = 256
BT = LNW // T
NORM_PARTS = 6
QK_BLOCK = 64
VB = 8 * DH

LOG2E = 1.4426950408889634
QSCALE = (DH ** -0.5) * LOG2E
MASKVAL = -1000000000.0 * LOG2E
EPS_BF16 = 1.0013580322265625e-05
ONES_PAIR = 0x3F803F80

NT_DIMS = (((1,), (1,)), ((), ()))

WT_Q = 0
WT_K = D // 2
WT_R = D
WT_V = D + 8
WT_ROWS = WT_V + D // 2
WT_ALLOC = 1056
NBLK = DP // T

X_PIECES = ((0, LNW), (LNW, LNW), (L, L), (2 * L, L), (3 * L, L))
SEM_X = 0
SEM_W = 5
SEM_MOE = 9
SEM_OUT = 12
SEM_SMALL = 21
SEM_WQB = 23
SEM_FINAL = 24
NSEM = 28
WQ_SPLIT = 2 * T


PROFILE_SCOPES = False
PACE = True
TAIL_BARRIERS = False
QT_ORDER = (3, 0, 2, 1)


def _scope(name):
    return jax.named_scope(name) if PROFILE_SCOPES else contextlib.nullcontext()


def _valid(g):
    return min(HPG * DH, D - g * HPG * DH)


def _ewin(g):
    start = (g * HPG * DH // 16) * 16
    return start, g * HPG * DH - start, min(T, D - start)


def _bf(x):
    return pltpu.bitcast(x, bf16)


def _pack(x):
    return pltpu.bitcast(x.astype(bf16), u32)


def _round_bf16(x):
    return x.astype(bf16).astype(f32)


def _phi(t):
    return jnp.where(t > 0, t + 1.0, jnp.exp(t))


def _sigmoid(t):
    return 1.0 / (1.0 + jnp.exp(-t))


def _zero_after(v):
    bits = pltpu.bitcast(v[0:8, 0:LNW], u32)
    sixteen = jnp.uint32(16)
    bits = lax.shift_right_logical(lax.shift_right_logical(bits, sixteen), sixteen)
    return pltpu.bitcast(bits, f32) if PACE else None


def _interleave(*lists):
    items = []
    for li, tasks in enumerate(lists):
        for k, t in enumerate(tasks):
            items.append(((k + 0.5) / len(tasks), li, k, t))
    items.sort(key=lambda it: it[:3])
    return [it[3] for it in items]


def _kernel(x_hbm, wq_hbm, wk_hbm, wv_hbm, wo_hbm, beta_hbm, wr_hbm, wg_hbm, wu_hbm, wd_hbm,
            out_hbm,
            beta_ref, wr_ref, x_buf, w_buf, wg_buf, wu_buf, wd_buf, out_buf,
            wt_u, kt_tmp, wot_u, xn_u, xs_a, xs_b, qs_u, k_u, pq_u, pk_u, vt_u, vwin,
            r_buf, mt_acc, lm_f, mcode, am, g16, omg, mb,
            s0, m0, s1, m1, ot0, ot1, ot2, ot3, xf, ln_stat, y_acc, xsel_buf, hid_buf, sems):

    class XCopy:
        def __init__(self, i):
            c0, width = X_PIECES[i]
            self.copies = [pltpu.make_async_copy(x_hbm.at[:, c:c + T], x_buf.at[c // T], sems.at[SEM_X + i])
                           for c in range(c0, c0 + width, T)]

        def start(self):
            for cp in self.copies:
                cp.start()

        def wait(self):
            for cp in self.copies:
                cp.wait()

    x_copy = XCopy

    def x_rows(tile, r0, r1):
        return _bf(x_buf.at[tile].bitcast(u32)[r0 // 2:r1 // 2, :])

    def w_copy(i):
        src = (wq_hbm, wk_hbm, wv_hbm, wo_hbm)[i]
        return pltpu.make_async_copy(src, w_buf.at[i], sems.at[SEM_W + i])

    wq_first = pltpu.make_async_copy(wq_hbm.at[:, 0:WQ_SPLIT], w_buf.at[0, :, 0:WQ_SPLIT], sems.at[SEM_W])
    wq_rest = pltpu.make_async_copy(wq_hbm.at[:, WQ_SPLIT:D], w_buf.at[0, :, WQ_SPLIT:D], sems.at[SEM_WQB])

    moe_src = (wg_hbm, wu_hbm, wd_hbm)
    moe_dst = (wg_buf, wu_buf, wd_buf)

    def moe_start(i, ft):
        c0 = ft * T if isinstance(ft, int) else pl.multiple_of(ft * T, T)
        pltpu.make_async_copy(moe_src[i].at[:, pl.ds(c0, T)], moe_dst[i].at[ft], sems.at[SEM_MOE + i]).start()

    def moe_issue(first, last):
        for n in range(first, last):
            moe_start(n % 3, n // 3)

    def moe_wait(i):
        pltpu.make_async_copy(moe_dst[i], moe_dst[i], sems.at[SEM_MOE + i]).wait()

    def out_copy(c0, width, sem):
        return pltpu.make_async_copy(out_buf.at[:, pl.ds(c0, width)], out_hbm.at[:, pl.ds(c0, width)],
                                     sems.at[SEM_OUT + sem])

    small_copies = [pltpu.make_async_copy(beta_hbm, beta_ref, sems.at[SEM_SMALL]),
                    pltpu.make_async_copy(wr_hbm, wr_ref, sems.at[SEM_SMALL + 1])]
    x_copy(0).start()
    wq_first.start()
    wq_rest.start()
    x_copy(1).start()
    for cp in small_copies:
        cp.start()
    w_copy(1).start()
    w_copy(2).start()

    init_scope = _scope("init")
    init_scope.__enter__()
    kr = lax.broadcasted_iota(i32, (HT, T), 0)
    ql = lax.broadcasted_iota(i32, (HT, T), 1)
    mb[0] = jnp.where(ql < kr, MASKVAL, 0.0).astype(f32)
    mb[1] = jnp.where((ql >= HT) & (ql - HT < kr), MASKVAL, 0.0).astype(f32)
    mb[2] = jnp.where(ql % HT < kr, MASKVAL, 0.0).astype(f32)
    zpad = jnp.zeros(((DP - D) // 2, LNW), u32)
    for blk in range(SEQ // LNW):
        xn_u[blk, D // 2:DP // 2, :] = zpad
    xs_a[D // 2:DP // 2, :] = zpad
    xs_b[D // 2:DP // 2, :] = zpad
    ots = (ot0, ot1, ot2, ot3)
    for o_ref in ots:
        o_ref[D:DP, :] = jnp.zeros((DP - D, T), f32)
    am[0] = jnp.zeros(am.shape[1:], f32)
    mt_acc[...] = jnp.zeros(mt_acc.shape, f32)
    g16[...] = jnp.zeros(g16.shape, f32)

    init_scope.__exit__(None, None, None)

    pace = [None]

    def gate_tables():
        gate = _round_bf16(_sigmoid(beta_ref[...].reshape(1, H).astype(f32)))
        for h in range(H):
            gh = jnp.broadcast_to(gate[:, h:h + 1], (1, T))
            omg[h] = jnp.broadcast_to(_round_bf16(1.0 - gh), (8, T))
            g16[h // HPG, (h % HPG):(h % HPG) + 1, :] = gh

    def transpose_block(i, cb):
        c1 = min((cb + 1) * T, D)
        blk = w_buf[i, :, cb * T:c1]
        if c1 - cb * T < T:
            blk = jnp.concatenate([blk, jnp.zeros((D, T - (c1 - cb * T)), bf16)], axis=1)
        blk = jnp.concatenate([blk, jnp.zeros((DP - D, T), bf16)], axis=0)
        return pltpu.bitcast(blk.T, u32)

    def prep_dense(i, dst, base):
        def task(cb):
            nrow = min(TW, D // 2 - cb * TW)
            dst[base + cb * TW:base + cb * TW + nrow, :] = transpose_block(i, cb)[0:nrow]
        return [lambda cb=cb: task(cb) for cb in range(DP // T)]

    def router_row():
        wr = wr_ref[...].reshape(1, D).astype(f32)
        wr = jnp.concatenate([wr, jnp.zeros((1, DP - D), f32)], axis=1)
        bits = lax.shift_right_logical(pltpu.bitcast(wr, u32), u32(16))
        rid = lax.broadcasted_iota(i32, (8, DP), 0)
        wt_u[WT_R:WT_R + 8, :] = jnp.where(rid == 0, bits, u32(0))

    def ln_tasks(s, p, stage):
        tile0 = s * TPS + p * BT

        def mean_pass():
            acc = pace[0]
            for r in range(0, D, 64):
                x = jnp.concatenate([pltpu.bitcast(x_rows(tile0 + t, r, r + 64), u32) for t in range(BT)], axis=1)
                x = _bf(x).astype(f32)
                xf[p, r:r + 64, :] = x
                part = jnp.sum(x.reshape(8, 8, LNW), axis=0)
                acc = part if acc is None else acc + part
            mean = jnp.sum(acc, axis=0, keepdims=True) / D
            ln_stat[p, 0] = jnp.broadcast_to(mean, (8, LNW))

        def var_pass():
            mean = ln_stat[p, 0][0:1]
            if pace[0] is not None:
                mean = mean + pace[0][0:1]
            acc = None
            for r in range(0, D, 96):
                xc = xf[p, r:r + 96, :] - mean
                part = jnp.sum((xc * xc).reshape(12, 8, LNW), axis=0)
                acc = part if acc is None else acc + part
            var = jnp.sum(acc, axis=0, keepdims=True) / D
            den = _round_bf16(jnp.sqrt(_round_bf16(_round_bf16(var) + EPS_BF16)))
            ln_stat[p, 1] = jnp.broadcast_to(1.0 / den, (8, LNW))
            ln_stat[p, 0] = jnp.broadcast_to(_round_bf16(mean), (8, LNW))

        def norm_pass(part):
            mean_b = ln_stat[p, 0][0:1]
            if pace[0] is not None:
                mean_b = mean_b + pace[0][0:1]
            inv = ln_stat[p, 1][0:1]
            step = D // NORM_PARTS
            for r in range(part * step, (part + 1) * step, 48):
                xn = _pack(_round_bf16(xf[p, r:r + 48, :] - mean_b) * inv)
                xn_u.at[s * (L // LNW) + p][r // 2:r // 2 + 24, :] = xn
                if stage is not None:
                    stage[r // 2:r // 2 + 24, :] = xn

        return [mean_pass, var_pass] + [lambda part=part: norm_pass(part) for part in range(NORM_PARTS)]

    def load_xs(s, p, stage):
        return _bf(xn_u[s * (L // LNW) + p] if stage is None else stage[...])

    def row_blocks(size):
        return [(r, min(r + size, D)) for r in range(0, D, size)]

    def q_task(s, p, stage, r0, r1):
        rows = slice(r0 // 2, r1 // 2)
        cols = slice(p * LNW, (p + 1) * LNW)
        w = _bf(wt_u[WT_Q + r0 // 2:WT_Q + r1 // 2, :])
        q = jnp.dot(w, load_xs(s, p, stage), preferred_element_type=f32)
        pace[0] = _zero_after(q)
        qs = q * QSCALE
        qrot = jnp.concatenate([pltpu.roll(qs[:, t * T:(t + 1) * T], HT, 1) for t in range(BT)], axis=1)
        rid = lax.broadcasted_iota(i32, qs.shape, 0) + r0
        even = ((rid // DH) % 2) == 0
        qs_u.at[s][rows, cols] = _pack(jnp.where(even, qrot, qs))
        pq_u.at[s][rows, cols] = _pack(_phi(q))

    def k_task(s, p, stage, r0, r1):
        rows = slice(r0 // 2, r1 // 2)
        cols = slice(p * LNW, (p + 1) * LNW)
        extra = 8 if r1 == D else 0
        w = _bf(wt_u[WT_K + r0 // 2:WT_K + r1 // 2 + extra, :])
        k = jnp.dot(w, load_xs(s, p, stage), preferred_element_type=f32)
        pace[0] = _zero_after(k)
        if extra:
            r_buf[s, :, cols] = jnp.broadcast_to(k[r1 - r0:r1 - r0 + 1, :], (8, LNW))
            k = k[0:r1 - r0]
        kt_tmp.at[p][rows, :] = _pack(k)
        pk_u.at[s][rows, cols] = _pack(_phi(k))

    def kt_task(s, p, g):
        nv = _valid(g) // 2
        src = g * HPG * DH // 2
        kg = jnp.concatenate([kt_tmp[p, src:src + nv, :], jnp.zeros((TW - nv, LNW), u32)], axis=0)
        k_u.at[s * NG + g][p * (LNW // 2):(p + 1) * (LNW // 2), :] = pltpu.bitcast(_bf(kg).T, u32)

    def v_task(s, p, stage, b):
        cols = slice(p * LNW, (p + 1) * LNW)
        w = _bf(wt_u[WT_V + b * (VB // 2):WT_V + (b + 1) * (VB // 2), :])
        v = jnp.dot(w, load_xs(s, p, stage), preferred_element_type=f32)
        pace[0] = _zero_after(v)
        v = _pack(v)
        vt_u.at[s][b * (VB // 2):(b + 1) * (VB // 2), cols] = v
        sub = lax.broadcasted_iota(i32, (16, LNW), 0)
        for hh in range(8):
            w8 = (9 * hh) // 8
            ones_row = 0 if 2 * hh == 14 else 15
            vwin.at[s * H + 8 * b + hh][:, cols] = jnp.where(sub == ones_row, u32(ONES_PAIR), v[8 * w8:8 * w8 + 16, :])

    def q_tasks(s, p, stage=None, size=QK_BLOCK):
        return [lambda b=b: q_task(s, p, stage, *b) for b in row_blocks(size)]

    def k_tasks(s, p, stage=None, size=QK_BLOCK):
        tasks, done = [], 0
        for b in row_blocks(size):
            tasks.append(lambda b=b: k_task(s, p, stage, *b))
            while done < NG and done * HPG * DH + _valid(done) <= b[1]:
                tasks.append(lambda g=done: kt_task(s, p, g))
                done += 1
        return tasks

    def v_tasks(s, p, stage=None):
        return [lambda b=b: v_task(s, p, stage, b) for b in range(D // VB)]

    def mem_layout(g):
        es, eoff, _ = _ewin(g)
        nv = _valid(g)
        ne = -(-(eoff + nv) // 16) * 16
        ones_row = 0 if eoff >= 2 else eoff + nv
        nh = nv // DH
        den_row = 0 if eoff >= nh else ne
        return es, eoff, nv, ne, ones_row, den_row, max(ne, den_row + 16 * (den_row > 0))

    def mem_update(sp, g):
        es, eoff, nv, ne, ones_row, den_row, nr = mem_layout(g)
        nw = min(T, D - es)
        win = vt_u[sp, es // 2:(es + ne) // 2, :]
        wid = lax.broadcasted_iota(i32, win.shape, 0)
        lhs = _bf(jnp.where(wid == ones_row // 2, u32(ONES_PAIR), win))
        upd = lax.dot_general(lhs, _bf(pk_u[sp, es // 2:(es + nw) // 2, :]), NT_DIMS, preferred_element_type=f32)
        mt = mt_acc[g, 0:ne, 0:nw] + upd
        mt_acc[g, 0:ne, 0:nw] = mt
        z = jnp.broadcast_to(mt[ones_row:ones_row + 1, :], (nr, nw))
        if nr > ne:
            mt = jnp.concatenate([mt, jnp.zeros((nr - ne, nw), f32)], axis=0)
        code = mcode[g, 0:nr, 0:nw]
        lm_f[g, 0:nr, 0:nw] = jnp.where(code == 1, mt, jnp.where(code == 2, z, 0.0))

    def mem_masks():
        for g in range(NG):
            es, eoff, nv, ne, ones_row, den_row, nr = mem_layout(g)
            row = lax.broadcasted_iota(i32, (T, T), 0)
            d_loc = lax.broadcasted_iota(i32, (T, T), 1) - eoff
            e_loc = row - eoff
            d_ok = (d_loc >= 0) & (d_loc < nv)
            same_head = (e_loc >= 0) & (e_loc < nv) & d_ok & ((e_loc // DH) == (d_loc // DH))
            den_hit = (row >= den_row) & d_ok & ((d_loc // DH) == row - den_row)
            mcode[g] = jnp.where(same_head, 1, jnp.where(den_hit, 2, 0))

    def mem_retrieve(s, g):
        es, eoff, nv, ne, ones_row, den_row, nr = mem_layout(g)
        nw = min(T, D - es)
        nd = jnp.dot(lm_f[g, 0:nr, 0:nw].astype(bf16), _bf(pq_u[s, es // 2:(es + nw) // 2, :]),
                     preferred_element_type=f32)
        scale = jnp.broadcast_to(g16[g][:, 0:1], (8, L)) / (nd[den_row:den_row + 8, :] + 1e-6)
        r8 = lax.broadcasted_iota(i32, (8, L), 0)
        for b in range(ne // 8):
            lo, hi = 8 * b - eoff, 8 * b + 7 - eoff
            if hi < 0 or lo >= nv:
                continue
            j1, j2 = max(lo, 0) // DH, min(hi, nv - 1) // DH
            sc = jnp.broadcast_to(scale[j1:j1 + 1, :], (8, L))
            if j2 != j1:
                sc = jnp.where(r8 < DH * j2 - lo, sc, jnp.broadcast_to(scale[j2:j2 + 1, :], (8, L)))
            val = nd[8 * b:8 * b + 8, :] * sc
            dst = am.at[s, es + 8 * b:es + 8 * b + 8, :]
            if lo >= 0 and hi < nv:
                dst[...] = val
            else:
                pltpu.store(dst, val, mask=(r8 + lo >= 0) & (r8 + lo < nv))

    def run(tasks):
        for t in tasks:
            t()

    prep_q = prep_dense(0, wt_u, WT_Q)
    q0a = q_tasks(0, 0, None, T)
    with _scope("p1_wait_x0"):
        x_copy(0).wait()
    for i in range(2, len(X_PIECES)):
        x_copy(i).start()
    w_copy(3).start()
    moe_issue(0, 40)
    with _scope("p1_ln0a"):
        run(ln_tasks(0, 0, None))
        wq_first.wait()
    with _scope("p1_q0a_first"):
        run(prep_q[0:2] + q0a[0:2])
        wq_rest.wait()
        x_copy(1).wait()
    with _scope("p1_q0a"):
        run(prep_q[2:])
        run(_interleave(q0a[2:], ln_tasks(0, 1, None)))
        w_copy(1).wait()
        for cp in small_copies:
            cp.wait()
    k0a, k0b = k_tasks(0, 0), k_tasks(0, 1)
    with _scope("p1_q0b"):
        run(_interleave(q_tasks(0, 1), prep_dense(1, wt_u, WT_K), [router_row, gate_tables, mem_masks]))
        run([lambda b=b: k_task(0, 0, None, *b) for b in row_blocks(QK_BLOCK)])
        w_copy(2).wait()
        x_copy(2).wait()
    moe_issue(40, 60)
    with _scope("p1_k0v0"):
        run(_interleave(k0b, prep_dense(2, wt_u, WT_V), [lambda g=g: kt_task(0, 0, g) for g in range(NG)]))
        run(_interleave(v_tasks(0, 0) + v_tasks(0, 1), ln_tasks(1, 0, xs_a)))

    moe_issue(60, 72)

    def seg_body(s, c):
        for ss in range(2, NSEG):
            @pl.when(s + 1 == ss)
            def _():
                x_copy(ss + 1).wait()
                if ss == NSEG - 1:
                    moe_issue(72, 3 * NFT)
        nxt = jnp.minimum(s + 1, NSEG - 1)
        pace[0] = None
        with _scope("p1_seg"):
            updates = [lambda g=g: mem_update(s - 1, g) for g in range(NG)]
            retrieves = [lambda g=g: mem_retrieve(s, g) for g in range(NG)]
            first = _interleave(q_tasks(s, 0, xs_a), updates) + k_tasks(s, 0, xs_a) + v_tasks(s, 0, xs_a)
            run(_interleave(first, ln_tasks(s, 1, xs_b)))
            second = q_tasks(s, 1, xs_b) + _interleave(k_tasks(s, 1, xs_b) + v_tasks(s, 1, xs_b), retrieves)
            run(_interleave(second, ln_tasks(nxt, 0, xs_a)))
        return c

    lax.fori_loop(1, NSEG, seg_body, 0)

    bufs = ((s0, m0), (s1, m1))
    lane64 = lax.broadcasted_iota(i32, (TW, T), 1)
    lane1 = lax.broadcasted_iota(i32, (1, T), 1)
    lane8 = lax.broadcasted_iota(i32, (8, T), 1)

    def pair_weights(s, pi, qt):
        hw = DH // 2
        j = 2 * (pi % (HPG // 2))
        src, dst = hw * 2 * pi, hw * j
        a0, t0 = (src // 8) * 8, (dst // 8) * 8
        nrow = min(32, D // 2 - a0)
        part = qs_u[s, a0:a0 + nrow, qt * T:(qt + 1) * T]
        if nrow < 32:
            part = jnp.concatenate([part, jnp.zeros((32 - nrow, T), u32)], axis=0)
        shift = (dst - t0) - (src - a0)
        if shift:
            part = pltpu.roll(part, shift % 32, 0)
        rid = lax.broadcasted_iota(i32, (32, T), 0) + t0
        out = []
        for lo in (dst, dst + hw):
            piece = jnp.where((rid >= lo) & (rid < lo + hw), part, u32(0))
            piece = piece[0:min(32, TW - t0)]
            pieces = [jnp.zeros((t0, T), u32)] * (t0 > 0) + [piece] + [jnp.zeros((TW - t0 - 32, T), u32)] * (t0 + 32 < TW)
            out.append(jnp.concatenate(pieces, axis=0))
        return out

    def stage_a(unit, u, qt):
        s, k = unit
        s_ref, m_ref = bufs[k % 2]
        pi = k * NP + u
        g = pi // (HPG // 2)
        sg = s * NG + g
        n = T * (qt + 1)
        w_a, w_b = pair_weights(s, pi, qt)
        w_ab = _bf(jnp.where(lane64 < HT, w_a, w_b))

        def colmax8(v):
            return jnp.max(v.reshape(v.shape[0] // 8, 8, T), axis=0)

        maxes = []
        for hd, w in enumerate((_bf(w_a), _bf(w_b))):
            m8 = None
            for c in range(qt):
                kc = _bf(k_u[sg, c * TW:(c + 1) * TW, :])
                sc = jnp.dot(kc, w, preferred_element_type=f32)
                s_ref[u, qt, hd * L + c * T:hd * L + (c + 1) * T, :] = sc
                m8 = colmax8(sc) if m8 is None else jnp.maximum(m8, colmax8(sc))
            kc = _bf(k_u[sg, qt * TW:qt * TW + TW // 2, :])
            sc = jnp.dot(kc, w, preferred_element_type=f32) + mb[1 - hd]
            s_ref[u, qt, hd * L + qt * T:hd * L + qt * T + HT, :] = sc
            m8 = colmax8(sc) if m8 is None else jnp.maximum(m8, colmax8(sc))
            maxes.append(m8)
        kc = _bf(k_u[sg, qt * TW + TW // 2:(qt + 1) * TW, :])
        sc = jnp.dot(kc, w_ab, preferred_element_type=f32) + mb[2]
        s_ref[u, qt, n - HT:n, :] = sc
        mab = colmax8(sc)
        m_a = jnp.where(lane8 < HT, jnp.maximum(maxes[0], mab), maxes[0])
        m_b = jnp.where(lane8 >= HT, jnp.maximum(maxes[1], mab), maxes[1])
        m_ref[u, qt, 0] = jnp.broadcast_to(jnp.max(m_a, axis=0, keepdims=True), (8, T))
        m_ref[u, qt, 1] = jnp.broadcast_to(jnp.max(m_b, axis=0, keepdims=True), (8, T))

    def stage_b(unit, u, qt):
        s, k = unit
        s_ref, m_ref = bufs[k % 2]
        pi = k * NP + u
        n = T * (qt + 1)
        m_a = m_ref[u, qt, 0][0:1]
        m_b = m_ref[u, qt, 1][0:1]
        p_ab = jnp.exp2(s_ref[u, qt, n - HT:n, :] - jnp.where(lane1 < HT, m_a, m_b))
        for hd, m in enumerate((m_a, m_b)):
            h = 2 * pi + hd
            p = jnp.exp2(s_ref[u, qt, hd * L:hd * L + n - HT, :] - m)
            keep = (lane64 < HT) if hd == 0 else (lane64 >= HT)
            p = jnp.concatenate([p, jnp.where(keep, p_ab, 0.0)], axis=0).astype(bf16)
            w0 = ((DH * h) // 16) * 16
            off = DH * h - w0
            o = jnp.dot(_bf(vwin[s * H + h, :, 0:n]), p, preferred_element_type=f32)
            den = o[0:1] if off == 14 else o[31:32]
            r0, r1 = (off // 8) * 8, -(-(off + DH) // 8) * 8
            o = o[r0:r1] * (omg[h][0:1] / den)
            if hd == 0:
                o = pltpu.roll(o, HT, 1)
            res = am[s, w0 + r0:w0 + r1, qt * T:(qt + 1) * T] + o
            rid = lax.broadcasted_iota(i32, (r1 - r0, T), 0) + r0
            pltpu.store(ots[qt].at[w0 + r0:w0 + r1, :], res, mask=(rid >= off) & (rid < off + DH))

    def a_tasks(unit):
        return [lambda u=u, qt=qt: stage_a(unit, u, qt) for u in range(NP) for qt in QT_ORDER]

    def b_tasks(unit):
        return [lambda u=u, qt=qt: stage_b(unit, u, qt) for u in range(NP) for qt in QT_ORDER]

    w_copy(3).wait()
    rr = jnp.concatenate([r_buf[s][0:1, :] for s in range(NSEG)], axis=0)
    rr = _round_bf16(rr)
    tok = lax.broadcasted_iota(i32, (NSEG, L), 0) * L + lax.broadcasted_iota(i32, (NSEG, L), 1)
    m1v = jnp.max(rr)
    i1 = jnp.min(jnp.where(rr == m1v, tok, SEQ))
    rr2 = jnp.where(tok == i1, -jnp.inf, rr)
    m2v = jnp.max(rr2)
    i2 = jnp.min(jnp.where(rr2 == m2v, tok, SEQ))
    i1 = jnp.clip(i1, 0, SEQ - 1)
    i2 = jnp.clip(i2, 0, SEQ - 1)

    row16 = lax.broadcasted_iota(i32, (16, T), 0)
    lane16 = lax.broadcasted_iota(i32, (16, T), 1)

    def token_rows(i, slot):
        onehot = jnp.where((row16 == slot) & (lane16 == i % T), 1.0, 0.0).astype(bf16)
        return lax.dot_general(onehot, _bf(xn_u[i // LNW, :, pl.ds(pl.multiple_of(((i // T) % BT) * T, T), T)]), NT_DIMS, preferred_element_type=f32)

    def select_task():
        xsel_buf[...] = _pack(token_rows(i1, 0) + token_rows(i2, 1))
        y_acc[...] = jnp.zeros(y_acc.shape, f32)

    def expert_tile(w_ref, ft):
        return _bf(w_ref.at[ft].bitcast(u32)[...])

    def moe_up_task(ft, k, which):
        xsel = _bf(xsel_buf[:, 0:D])
        w_ref = (wg_buf, wu_buf)[which]
        hid_buf[k, which] = jnp.dot(xsel, expert_tile(w_ref, ft), preferred_element_type=f32)

    def moe_down_task(ft, k):
        gt = _round_bf16(hid_buf[k, 0])
        up = _round_bf16(hid_buf[k, 1])
        hid = (_round_bf16(gt * _sigmoid(gt)) * up).astype(bf16)
        y_acc[...] += lax.dot_general(hid, expert_tile(wd_buf, ft), NT_DIMS, preferred_element_type=f32)

    def moe_tasks(ft0, count):
        tasks = []
        for k0 in range(0, count, FPB):
            ks = range(k0, min(k0 + FPB, count))
            tasks += [lambda k=k, w=w: moe_up_task(ft0 + k, k, w) for k in ks for w in range(2)]
            tasks += [lambda k=k: moe_down_task(ft0 + k, k) for k in ks]
        return tasks

    def moe_finish():
        y = _round_bf16(y_acc[...])
        rsel = jnp.where(lax.broadcasted_iota(i32, (16, 1), 0) == 0, m1v, m2v)
        y = _round_bf16(y * _round_bf16(_sigmoid(rsel)))
        y = jnp.concatenate([y, jnp.zeros((16, DP - D), f32)], axis=1)
        y = jnp.concatenate([jnp.zeros((HT, DP), f32), y, jnp.zeros((T - HT - 16, DP), f32)], axis=0)
        y_t = jnp.concatenate([y.T[0:D], jnp.zeros((D, T), f32)], axis=1)
        y_u = _pack(y_t)[:, 0:T]
        lane = lax.broadcasted_iota(i32, (D // 2, T), 1)
        wot_u[:, DP - T:DP] = jnp.where(lane < HT, wot_u[:, DP - T:DP], y_u)
        rid = lax.broadcasted_iota(i32, (8, T), 0)
        for tt in range(TPS):
            tok_l = lax.broadcasted_iota(i32, (8, T), 1) + (NSEG - 1) * L + tt * T
            ots[tt][D:D + 8, :] = jnp.where(((rid == 0) & (tok_l == i1)) | ((rid == 1) & (tok_l == i2)), 1.0, 0.0)

    dense = _interleave(a_tasks((0, 0)), prep_dense(3, wot_u, 0))
    with _scope("p15_mix"):
        cut = (2 * len(dense)) // 3
        run(dense[:cut] + [select_task] + dense[cut:])

    for i in range(3):
        moe_wait(i)

    def out_tile(s, tt, last, chunk_copies=None):
        c0 = s * L + tt * T
        if not isinstance(s, int):
            c0 = pl.multiple_of(c0, T)
        o_bf = ots[tt][...].astype(bf16)
        nchunk = 4
        rows = D // nchunk
        for rc in range(nchunk):
            r0 = rc * rows
            attn = jnp.dot(_bf(wot_u[r0 // 2:(r0 + rows) // 2, :]), o_bf, preferred_element_type=f32)
            xn = _bf(xn_u[s * (L // LNW) + tt // BT, r0 // 2:(r0 + rows) // 2, (tt % BT) * T:(tt % BT + 1) * T]).astype(f32)
            x = x_rows(s * TPS + tt, r0, r0 + rows).astype(f32)
            res = x + attn + xn
            out_buf[r0:r0 + rows, pl.ds(c0, T)] = res.astype(bf16)
            if chunk_copies is not None:
                chunk_copies[rc].start()

    def pair_tasks(ua, ub):
        tasks = []
        for x, y in zip(a_tasks(ua), b_tasks(ub)):
            tasks += [x, y]
        return tasks

    def seg_end(s, last):
        def by_qt(fn, unit, qt):
            return [lambda u=u: fn(unit, u, qt) for u in range(NP)]

        steps = []
        for step in range(7):
            lists = []
            if step < 4:
                lists.append(by_qt(stage_b, (s, 2), 3 - step))
                lists.append(by_qt(stage_a, (s, 3), 3 - step))
            if 1 <= step < 5:
                lists.append(by_qt(stage_b, (s, 3), 4 - step))
            if not last and 2 <= step < 6:
                lists.append(by_qt(stage_a, (s + 1, 0), 5 - step))
            if step >= 3:
                lists.append([lambda tt=6 - step: out_tile(s, tt, last)])
            steps.append(_interleave(*lists))
        return steps

    def seg_att(s, c):
        tasks = pair_tasks((s, 1), (s, 0)) + pair_tasks((s, 2), (s, 1))
        steps = seg_end(s, False)
        for step in steps[0:5]:
            tasks += step
        with _scope("att_seg"):
            run(_interleave(tasks, moe_tasks(s * FPI, FPI)))
            for step in steps[5:]:
                run(step)

        @pl.when(s < NSEG - 2)
        def _():
            out_copy(pl.multiple_of(s * L, L), L, s).start()
        return c

    lax.fori_loop(0, NSEG - 1, seg_att, 0)

    npatch = (NSEG - 1) * TPS

    def patch_tile(idx):
        return jnp.where(idx < npatch * T, idx // T, 0)

    tile0 = patch_tile(i1)
    tile1 = patch_tile(i2)
    tile1 = jnp.where(tile1 == tile0, (tile0 + 1) % npatch, tile1)

    def patch(tile):
        c0 = pl.multiple_of(tile * T, T)
        rid = lax.broadcasted_iota(i32, (T, T), 0)
        tok_l = lax.broadcasted_iota(i32, (T, T), 1) + c0
        hit = ((rid == HT) & (tok_l == i1)) | ((rid == HT + 1) & (tok_l == i2))
        onehot = jnp.where(hit, 1.0, 0.0).astype(bf16)
        for rc in range(4):
            r0, r1 = rc * (D // 4), (rc + 1) * (D // 4)
            upd = jnp.dot(_bf(wot_u[r0 // 2:r1 // 2, DP - T:DP]), onehot, preferred_element_type=f32)
            cur = out_buf[r0:r1, pl.ds(c0, T)].astype(f32)
            out_buf[r0:r1, pl.ds(c0, T)] = (cur + upd).astype(bf16)

    sent = (NSEG - 2) * TPS
    resend0 = jnp.where(tile0 < sent, tile0, jnp.where(tile1 == 0, 1, 0))
    resend1 = jnp.where(tile1 < sent, tile1, jnp.where(resend0 == 0, 1, 0))
    patch_copies = [out_copy(pl.multiple_of(resend0 * T, T), T, 7), out_copy(pl.multiple_of(resend1 * T, T), T, 8),
                    out_copy((NSEG - 2) * L, L, NSEG - 2)]
    last_copies = [out_copy((NSEG - 1) * L + tt * T, T, NSEG - 1 + tt) for tt in range(1, TPS)]
    c_fin = (NSEG - 1) * L
    final_copies = [
        pltpu.make_async_copy(out_buf.at[rc * (D // 4):(rc + 1) * (D // 4), c_fin:c_fin + T],
                              out_hbm.at[rc * (D // 4):(rc + 1) * (D // 4), c_fin:c_fin + T],
                              sems.at[SEM_FINAL + rc]) for rc in range(4)]

    sl = NSEG - 1
    for s in range(NSEG - 2):
        out_copy(s * L, L, s).wait()
    with _scope("tail_2"):
        moe_finish()
        run(pair_tasks((sl, 1), (sl, 0)))
        patch(tile0)
        patch(tile1)
        run(pair_tasks((sl, 2), (sl, 1)))
        for cp in patch_copies:
            cp.start()
        steps = seg_end(sl, True)
        for step in steps[0:5]:
            run(step)
        last_copies[2].start()
        last_copies[1].start()
    with _scope("tail_3"):
        run(steps[5])
        last_copies[0].start()
        out_tile(sl, 0, True, final_copies)

    with _scope("out_wait"):
        for cp in patch_copies + last_copies + final_copies:
            cp.wait()


@jax.jit
def pallas_parallel_sum__memory_aug_infini_attn__moe_arch_mod__prompt_kernel(
    A_x: jax.Array,
    A_wq: jax.Array,
    A_wk: jax.Array,
    A_wv: jax.Array,
    A_wo: jax.Array,
    A_beta: jax.Array,
    B_x: jax.Array,
    B_w_r: jax.Array,
    B_w_gate: jax.Array,
    B_w_up: jax.Array,
    B_w_down: jax.Array,
):
    del B_x
    any_spec = pl.BlockSpec(memory_space=pl.ANY)
    scratch = [
        pltpu.VMEM((H,), bf16),
        pltpu.VMEM((D,), bf16),
        pltpu.VMEM((NT, D, T), bf16),
        pltpu.VMEM((4, D, D), bf16),
        pltpu.VMEM((NFT, D, T), bf16),
        pltpu.VMEM((NFT, D, T), bf16),
        pltpu.VMEM((NFT, D, T), bf16),
        pltpu.VMEM((D, SEQ), bf16),
        pltpu.VMEM((WT_ALLOC, DP), u32),
        pltpu.VMEM((2, D // 2, LNW), u32),
        pltpu.VMEM((D // 2, DP), u32),
        pltpu.VMEM((SEQ // LNW, DP // 2, LNW), u32),
        pltpu.VMEM((DP // 2, LNW), u32),
        pltpu.VMEM((DP // 2, LNW), u32),
        pltpu.VMEM((NSEG, D // 2, L), u32),
        pltpu.VMEM((NSEG * NG, L // 2, T), u32),
        pltpu.VMEM((NSEG, D // 2, L), u32),
        pltpu.VMEM((NSEG, D // 2, L), u32),
        pltpu.VMEM((NSEG, D // 2, L), u32),
        pltpu.VMEM((NSEG * H, 16, L), u32),
        pltpu.VMEM((NSEG, 8, L), f32),
        pltpu.VMEM((NG, T, T), f32),
        pltpu.VMEM((NG, T, T), f32),
        pltpu.VMEM((NG, T, T), i32),
        pltpu.VMEM((NSEG, D, L), f32),
        pltpu.VMEM((NG, 8, T), f32),
        pltpu.VMEM((H, 8, T), f32),
        pltpu.VMEM((3, HT, T), f32),
        pltpu.VMEM((NP, 4, 2 * L, T), f32),
        pltpu.VMEM((NP, 4, 2, 8, T), f32),
        pltpu.VMEM((NP, 4, 2 * L, T), f32),
        pltpu.VMEM((NP, 4, 2, 8, T), f32),
        pltpu.VMEM((DP, T), f32),
        pltpu.VMEM((DP, T), f32),
        pltpu.VMEM((DP, T), f32),
        pltpu.VMEM((DP, T), f32),
        pltpu.VMEM((2, D, LNW), f32),
        pltpu.VMEM((2, 2, 8, LNW), f32),
        pltpu.VMEM((16, D), f32),
        pltpu.VMEM((8, DP), u32),
        pltpu.VMEM((FPI, 2, 16, T), f32),
        pltpu.SemaphoreType.DMA((NSEM,)),
    ]
    x_t = jnp.transpose(A_x, (0, 2, 1)).reshape(D, SEQ)
    out_t = pl.pallas_call(
        _kernel,
        out_shape=jax.ShapeDtypeStruct((D, SEQ), bf16),
        in_specs=[any_spec] * 10,
        out_specs=any_spec,
        scratch_shapes=scratch,
        compiler_params=pltpu.CompilerParams(vmem_limit_bytes=110 * 1024 * 1024),
    )(x_t, A_wq, A_wk, A_wv, A_wo, A_beta, B_w_r, B_w_gate, B_w_up, B_w_down.T)
    return jnp.transpose(out_t.reshape(1, D, SEQ), (0, 2, 1))
```

```python
import contextlib

import jax
import jax.numpy as jnp
from jax import lax
from jax.experimental import pallas as pl
from jax.experimental.pallas import tpu as pltpu

bf16 = jnp.bfloat16
f32 = jnp.float32
u32 = jnp.uint32
i32 = jnp.int32

SEQ = 2048
D = 576
DP = 640
H = 32
DH = 18
NSEG = 4
L = 512
T = 128
TW = T // 2
HT = T // 2
TPS = L // T
HPG = 6
NG = 6
F = 4608
FPI = 12
FPB = 3
NFT = F // T
NP = 4
UPS = H // (2 * NP)
NT = SEQ // T
LNW = 256
BT = LNW // T
NORM_PARTS = 6
QK_BLOCK = 64
VB = 8 * DH

LOG2E = 1.4426950408889634
QSCALE = (DH ** -0.5) * LOG2E
MASKVAL = -1000000000.0 * LOG2E
EPS_BF16 = 1.0013580322265625e-05
ONES_PAIR = 0x3F803F80

NT_DIMS = (((1,), (1,)), ((), ()))

WT_Q = 0
WT_K = D // 2
WT_R = D
WT_V = D + 8
WT_ALLOC = 1056
NBLK = DP // T

X_PIECES = ((0, LNW), (LNW, LNW), (L, L), (2 * L, L), (3 * L, L))
SEM_X = 0
SEM_W = 5
SEM_MOE = 9
SEM_OUT = 12
SEM_SMALL = 21
SEM_WQB = 23
SEM_FINAL = 24
NSEM = 28
WQ_SPLIT = 2 * T


PROFILE_SCOPES = False
QT_ORDER = (3, 0, 2, 1)


def _scope(name):
    return jax.named_scope(name) if PROFILE_SCOPES else contextlib.nullcontext()


def _valid(g):
    return min(HPG * DH, D - g * HPG * DH)


def _ewin(g):
    start = (g * HPG * DH // 16) * 16
    return start, g * HPG * DH - start, min(T, D - start)


def _bf(x):
    return pltpu.bitcast(x, bf16)


def _pack(x):
    return pltpu.bitcast(x.astype(bf16), u32)


def _round_bf16(x):
    return x.astype(bf16).astype(f32)


def _phi(t):
    return jnp.where(t > 0, t + 1.0, jnp.exp(t))


def _sigmoid(t):
    return 1.0 / (1.0 + jnp.exp(-t))


def _zero_after(v):
    bits = pltpu.bitcast(v[0:8, 0:LNW], u32)
    sixteen = jnp.uint32(16)
    bits = lax.shift_right_logical(lax.shift_right_logical(bits, sixteen), sixteen)
    return pltpu.bitcast(bits, f32)


def _interleave(*lists):
    items = []
    for li, tasks in enumerate(lists):
        for k, t in enumerate(tasks):
            items.append(((k + 0.5) / len(tasks), li, k, t))
    items.sort(key=lambda it: it[:3])
    return [it[3] for it in items]


def _kernel(x_hbm, wq_hbm, wk_hbm, wv_hbm, wo_hbm, beta_hbm, wr_hbm, wg_hbm, wu_hbm, wd_hbm,
            out_hbm,
            beta_ref, wr_ref, x_buf, w_buf, wg_buf, wu_buf, wd_buf, out_buf,
            wt_u, kt_tmp, wot_u, xn_u, xs_a, xs_b, qs_u, k_u, pq_u, pk_u, vt_u, vwin,
            r_buf, mt_acc, lm_f, mcode, am, g16, omg, mb,
            s0, m0, s1, m1, ot0, ot1, ot2, ot3, xf, ln_stat, y_acc, xsel_buf, hid_buf, sems):

    class XCopy:
        def __init__(self, i):
            c0, width = X_PIECES[i]
            self.copies = [pltpu.make_async_copy(x_hbm.at[:, c:c + T], x_buf.at[c // T], sems.at[SEM_X + i])
                           for c in range(c0, c0 + width, T)]

        def start(self):
            for cp in self.copies:
                cp.start()

        def wait(self):
            for cp in self.copies:
                cp.wait()

    x_copy = XCopy

    def x_rows(tile, r0, r1):
        return _bf(x_buf.at[tile].bitcast(u32)[r0 // 2:r1 // 2, :])

    def w_copy(i):
        src = (wq_hbm, wk_hbm, wv_hbm, wo_hbm)[i]
        return pltpu.make_async_copy(src, w_buf.at[i], sems.at[SEM_W + i])

    wq_first = pltpu.make_async_copy(wq_hbm.at[:, 0:WQ_SPLIT], w_buf.at[0, :, 0:WQ_SPLIT], sems.at[SEM_W])
    wq_rest = pltpu.make_async_copy(wq_hbm.at[:, WQ_SPLIT:D], w_buf.at[0, :, WQ_SPLIT:D], sems.at[SEM_WQB])

    moe_src = (wg_hbm, wu_hbm, wd_hbm)
    moe_dst = (wg_buf, wu_buf, wd_buf)

    def moe_start(i, ft):
        c0 = ft * T if isinstance(ft, int) else pl.multiple_of(ft * T, T)
        pltpu.make_async_copy(moe_src[i].at[:, pl.ds(c0, T)], moe_dst[i].at[ft], sems.at[SEM_MOE + i]).start()

    def moe_issue(first, last):
        for n in range(first, last):
            moe_start(n % 3, n // 3)

    def moe_wait(i):
        pltpu.make_async_copy(moe_dst[i], moe_dst[i], sems.at[SEM_MOE + i]).wait()

    def out_copy(c0, width, sem):
        return pltpu.make_async_copy(out_buf.at[:, pl.ds(c0, width)], out_hbm.at[:, pl.ds(c0, width)],
                                     sems.at[SEM_OUT + sem])

    small_copies = [pltpu.make_async_copy(beta_hbm, beta_ref, sems.at[SEM_SMALL]),
                    pltpu.make_async_copy(wr_hbm, wr_ref, sems.at[SEM_SMALL + 1])]
    x_copy(0).start()
    wq_first.start()
    wq_rest.start()
    x_copy(1).start()
    for cp in small_copies:
        cp.start()
    w_copy(1).start()
    w_copy(2).start()

    init_scope = _scope("init")
    init_scope.__enter__()
    kr = lax.broadcasted_iota(i32, (HT, T), 0)
    ql = lax.broadcasted_iota(i32, (HT, T), 1)
    mb[0] = jnp.where(ql < kr, MASKVAL, 0.0).astype(f32)
    mb[1] = jnp.where((ql >= HT) & (ql - HT < kr), MASKVAL, 0.0).astype(f32)
    mb[2] = jnp.where(ql % HT < kr, MASKVAL, 0.0).astype(f32)
    zpad = jnp.zeros(((DP - D) // 2, LNW), u32)
    for blk in range(SEQ // LNW):
        xn_u[blk, D // 2:DP // 2, :] = zpad
    xs_a[D // 2:DP // 2, :] = zpad
    xs_b[D // 2:DP // 2, :] = zpad
    ots = (ot0, ot1, ot2, ot3)
    for o_ref in ots:
        o_ref[D:DP, :] = jnp.zeros((DP - D, T), f32)
    am[0] = jnp.zeros(am.shape[1:], f32)
    mt_acc[...] = jnp.zeros(mt_acc.shape, f32)
    g16[...] = jnp.zeros(g16.shape, f32)

    init_scope.__exit__(None, None, None)

    pace = [None]

    def gate_tables():
        gate = _round_bf16(_sigmoid(beta_ref[...].reshape(1, H).astype(f32)))
        for h in range(H):
            gh = jnp.broadcast_to(gate[:, h:h + 1], (1, T))
            omg[h] = jnp.broadcast_to(_round_bf16(1.0 - gh), (8, T))
            g16[h // HPG, (h % HPG):(h % HPG) + 1, :] = gh

    def transpose_block(i, cb):
        c1 = min((cb + 1) * T, D)
        blk = w_buf[i, :, cb * T:c1]
        if c1 - cb * T < T:
            blk = jnp.concatenate([blk, jnp.zeros((D, T - (c1 - cb * T)), bf16)], axis=1)
        blk = jnp.concatenate([blk, jnp.zeros((DP - D, T), bf16)], axis=0)
        return pltpu.bitcast(blk.T, u32)

    def prep_dense(i, dst, base):
        def task(cb):
            nrow = min(TW, D // 2 - cb * TW)
            dst[base + cb * TW:base + cb * TW + nrow, :] = transpose_block(i, cb)[0:nrow]
        return [lambda cb=cb: task(cb) for cb in range(DP // T)]

    def router_row():
        wr = wr_ref[...].reshape(1, D).astype(f32)
        wr = jnp.concatenate([wr, jnp.zeros((1, DP - D), f32)], axis=1)
        bits = lax.shift_right_logical(pltpu.bitcast(wr, u32), u32(16))
        rid = lax.broadcasted_iota(i32, (8, DP), 0)
        wt_u[WT_R:WT_R + 8, :] = jnp.where(rid == 0, bits, u32(0))

    def ln_tasks(s, p, stage):
        tile0 = s * TPS + p * BT

        def mean_pass():
            acc = pace[0]
            for r in range(0, D, 64):
                x = jnp.concatenate([pltpu.bitcast(x_rows(tile0 + t, r, r + 64), u32) for t in range(BT)], axis=1)
                x = _bf(x).astype(f32)
                xf[p, r:r + 64, :] = x
                part = jnp.sum(x.reshape(8, 8, LNW), axis=0)
                acc = part if acc is None else acc + part
            mean = jnp.sum(acc, axis=0, keepdims=True) / D
            ln_stat[p, 0] = jnp.broadcast_to(mean, (8, LNW))

        def var_pass():
            mean = ln_stat[p, 0][0:1]
            if pace[0] is not None:
                mean = mean + pace[0][0:1]
            acc = None
            for r in range(0, D, 96):
                xc = xf[p, r:r + 96, :] - mean
                part = jnp.sum((xc * xc).reshape(12, 8, LNW), axis=0)
                acc = part if acc is None else acc + part
            var = jnp.sum(acc, axis=0, keepdims=True) / D
            den = _round_bf16(jnp.sqrt(_round_bf16(_round_bf16(var) + EPS_BF16)))
            ln_stat[p, 1] = jnp.broadcast_to(1.0 / den, (8, LNW))
            ln_stat[p, 0] = jnp.broadcast_to(_round_bf16(mean), (8, LNW))

        def norm_pass(part):
            mean_b = ln_stat[p, 0][0:1]
            if pace[0] is not None:
                mean_b = mean_b + pace[0][0:1]
            inv = ln_stat[p, 1][0:1]
            step = D // NORM_PARTS
            for r in range(part * step, (part + 1) * step, 48):
                xn = _pack(_round_bf16(xf[p, r:r + 48, :] - mean_b) * inv)
                xn_u.at[s * (L // LNW) + p][r // 2:r // 2 + 24, :] = xn
                if stage is not None:
                    stage[r // 2:r // 2 + 24, :] = xn

        return [mean_pass, var_pass] + [lambda part=part: norm_pass(part) for part in range(NORM_PARTS)]

    def load_xs(s, p, stage):
        return _bf(xn_u[s * (L // LNW) + p] if stage is None else stage[...])

    def row_blocks(size):
        return [(r, min(r + size, D)) for r in range(0, D, size)]

    def q_task(s, p, stage, r0, r1):
        rows = slice(r0 // 2, r1 // 2)
        cols = slice(p * LNW, (p + 1) * LNW)
        w = _bf(wt_u[WT_Q + r0 // 2:WT_Q + r1 // 2, :])
        q = jnp.dot(w, load_xs(s, p, stage), preferred_element_type=f32)
        pace[0] = _zero_after(q)
        qs = q * QSCALE
        qrot = jnp.concatenate([pltpu.roll(qs[:, t * T:(t + 1) * T], HT, 1) for t in range(BT)], axis=1)
        rid = lax.broadcasted_iota(i32, qs.shape, 0) + r0
        even = ((rid // DH) % 2) == 0
        qs_u.at[s][rows, cols] = _pack(jnp.where(even, qrot, qs))
        pq_u.at[s][rows, cols] = _pack(_phi(q))

    def k_task(s, p, stage, r0, r1):
        rows = slice(r0 // 2, r1 // 2)
        cols = slice(p * LNW, (p + 1) * LNW)
        extra = 8 if r1 == D else 0
        w = _bf(wt_u[WT_K + r0 // 2:WT_K + r1 // 2 + extra, :])
        k = jnp.dot(w, load_xs(s, p, stage), preferred_element_type=f32)
        pace[0] = _zero_after(k)
        if extra:
            r_buf[s, :, cols] = jnp.broadcast_to(k[r1 - r0:r1 - r0 + 1, :], (8, LNW))
            k = k[0:r1 - r0]
        kt_tmp.at[p][rows, :] = _pack(k)
        pk_u.at[s][rows, cols] = _pack(_phi(k))

    def kt_task(s, p, g):
        nv = _valid(g) // 2
        src = g * HPG * DH // 2
        kg = jnp.concatenate([kt_tmp[p, src:src + nv, :], jnp.zeros((TW - nv, LNW), u32)], axis=0)
        k_u.at[s * NG + g][p * (LNW // 2):(p + 1) * (LNW // 2), :] = pltpu.bitcast(_bf(kg).T, u32)

    def v_task(s, p, stage, b):
        cols = slice(p * LNW, (p + 1) * LNW)
        w = _bf(wt_u[WT_V + b * (VB // 2):WT_V + (b + 1) * (VB // 2), :])
        v = jnp.dot(w, load_xs(s, p, stage), preferred_element_type=f32)
        pace[0] = _zero_after(v)
        v = _pack(v)
        vt_u.at[s][b * (VB // 2):(b + 1) * (VB // 2), cols] = v
        sub = lax.broadcasted_iota(i32, (16, LNW), 0)
        for hh in range(8):
            w8 = (9 * hh) // 8
            ones_row = 0 if 2 * hh == 14 else 15
            vwin.at[s * H + 8 * b + hh][:, cols] = jnp.where(sub == ones_row, u32(ONES_PAIR), v[8 * w8:8 * w8 + 16, :])

    def q_tasks(s, p, stage=None, size=QK_BLOCK):
        return [lambda b=b: q_task(s, p, stage, *b) for b in row_blocks(size)]

    def k_tasks(s, p, stage=None, size=QK_BLOCK):
        tasks, done = [], 0
        for b in row_blocks(size):
            tasks.append(lambda b=b: k_task(s, p, stage, *b))
            while done < NG and done * HPG * DH + _valid(done) <= b[1]:
                tasks.append(lambda g=done: kt_task(s, p, g))
                done += 1
        return tasks

    def v_tasks(s, p, stage=None):
        return [lambda b=b: v_task(s, p, stage, b) for b in range(D // VB)]

    def mem_layout(g):
        es, eoff, _ = _ewin(g)
        nv = _valid(g)
        ne = -(-(eoff + nv) // 16) * 16
        ones_row = 0 if eoff >= 2 else eoff + nv
        nh = nv // DH
        den_row = 0 if eoff >= nh else ne
        return es, eoff, nv, ne, ones_row, den_row, max(ne, den_row + 16 * (den_row > 0))

    def mem_update(sp, g):
        es, eoff, nv, ne, ones_row, den_row, nr = mem_layout(g)
        nw = min(T, D - es)
        win = vt_u[sp, es // 2:(es + ne) // 2, :]
        wid = lax.broadcasted_iota(i32, win.shape, 0)
        lhs = _bf(jnp.where(wid == ones_row // 2, u32(ONES_PAIR), win))
        upd = lax.dot_general(lhs, _bf(pk_u[sp, es // 2:(es + nw) // 2, :]), NT_DIMS, preferred_element_type=f32)
        mt = mt_acc[g, 0:ne, 0:nw] + upd
        mt_acc[g, 0:ne, 0:nw] = mt
        z = jnp.broadcast_to(mt[ones_row:ones_row + 1, :], (nr, nw))
        if nr > ne:
            mt = jnp.concatenate([mt, jnp.zeros((nr - ne, nw), f32)], axis=0)
        code = mcode[g, 0:nr, 0:nw]
        lm_f[g, 0:nr, 0:nw] = jnp.where(code == 1, mt, jnp.where(code == 2, z, 0.0))

    def mem_masks():
        for g in range(NG):
            es, eoff, nv, ne, ones_row, den_row, nr = mem_layout(g)
            row = lax.broadcasted_iota(i32, (T, T), 0)
            d_loc = lax.broadcasted_iota(i32, (T, T), 1) - eoff
            e_loc = row - eoff
            d_ok = (d_loc >= 0) & (d_loc < nv)
            same_head = (e_loc >= 0) & (e_loc < nv) & d_ok & ((e_loc // DH) == (d_loc // DH))
            den_hit = (row >= den_row) & d_ok & ((d_loc // DH) == row - den_row)
            mcode[g] = jnp.where(same_head, 1, jnp.where(den_hit, 2, 0))

    def mem_retrieve(s, g):
        es, eoff, nv, ne, ones_row, den_row, nr = mem_layout(g)
        nw = min(T, D - es)
        nd = jnp.dot(lm_f[g, 0:nr, 0:nw].astype(bf16), _bf(pq_u[s, es // 2:(es + nw) // 2, :]),
                     preferred_element_type=f32)
        scale = jnp.broadcast_to(g16[g][:, 0:1], (8, L)) / (nd[den_row:den_row + 8, :] + 1e-6)
        r8 = lax.broadcasted_iota(i32, (8, L), 0)
        for b in range(ne // 8):
            lo, hi = 8 * b - eoff, 8 * b + 7 - eoff
            if hi < 0 or lo >= nv:
                continue
            j1, j2 = max(lo, 0) // DH, min(hi, nv - 1) // DH
            sc = jnp.broadcast_to(scale[j1:j1 + 1, :], (8, L))
            if j2 != j1:
                sc = jnp.where(r8 < DH * j2 - lo, sc, jnp.broadcast_to(scale[j2:j2 + 1, :], (8, L)))
            val = nd[8 * b:8 * b + 8, :] * sc
            dst = am.at[s, es + 8 * b:es + 8 * b + 8, :]
            if lo >= 0 and hi < nv:
                dst[...] = val
            else:
                pltpu.store(dst, val, mask=(r8 + lo >= 0) & (r8 + lo < nv))

    def run(tasks):
        for t in tasks:
            t()

    prep_q = prep_dense(0, wt_u, WT_Q)
    q0a = q_tasks(0, 0, None, T)
    mem_masks()
    with _scope("p1_wait_x0"):
        x_copy(0).wait()
    for i in range(2, len(X_PIECES)):
        x_copy(i).start()
    w_copy(3).start()
    moe_issue(0, 40)
    with _scope("p1_ln0a"):
        run(ln_tasks(0, 0, None))
        wq_first.wait()
    with _scope("p1_q0a_first"):
        run(prep_q[0:2] + q0a[0:2])
        wq_rest.wait()
        x_copy(1).wait()
    with _scope("p1_q0a"):
        run(prep_q[2:])
        run(_interleave(q0a[2:], ln_tasks(0, 1, None)))
        w_copy(1).wait()
        for cp in small_copies:
            cp.wait()
    k0b = k_tasks(0, 1)
    with _scope("p1_q0b"):
        run(_interleave(q_tasks(0, 1), prep_dense(1, wt_u, WT_K), [router_row, gate_tables]))
        run([lambda b=b: k_task(0, 0, None, *b) for b in row_blocks(QK_BLOCK)])
        w_copy(2).wait()
        x_copy(2).wait()
    moe_issue(40, 60)
    with _scope("p1_k0v0"):
        run(_interleave(k0b, prep_dense(2, wt_u, WT_V), [lambda g=g: kt_task(0, 0, g) for g in range(NG)]))
        run(_interleave(v_tasks(0, 0) + v_tasks(0, 1), ln_tasks(1, 0, xs_a)))

    moe_issue(60, 72)

    def seg_body(s, c):
        for ss in range(2, NSEG):
            @pl.when(s + 1 == ss)
            def _():
                x_copy(ss + 1).wait()
                if ss == NSEG - 1:
                    moe_issue(72, 3 * NFT)
        nxt = jnp.minimum(s + 1, NSEG - 1)
        pace[0] = None
        with _scope("p1_seg"):
            updates = [lambda g=g: mem_update(s - 1, g) for g in range(NG)]
            retrieves = [lambda g=g: mem_retrieve(s, g) for g in range(NG)]
            first = _interleave(q_tasks(s, 0, xs_a), updates) + k_tasks(s, 0, xs_a) + v_tasks(s, 0, xs_a)
            run(_interleave(first, ln_tasks(s, 1, xs_b)))
            second = q_tasks(s, 1, xs_b) + _interleave(k_tasks(s, 1, xs_b) + v_tasks(s, 1, xs_b), retrieves)
            run(_interleave(second, ln_tasks(nxt, 0, xs_a)))
        return c

    lax.fori_loop(1, NSEG, seg_body, 0)

    bufs = ((s0, m0), (s1, m1))
    lane64 = lax.broadcasted_iota(i32, (TW, T), 1)
    lane1 = lax.broadcasted_iota(i32, (1, T), 1)
    lane8 = lax.broadcasted_iota(i32, (8, T), 1)

    def pair_weights(s, pi, qt):
        hw = DH // 2
        j = 2 * (pi % (HPG // 2))
        src, dst = hw * 2 * pi, hw * j
        a0, t0 = (src // 8) * 8, (dst // 8) * 8
        nrow = min(32, D // 2 - a0)
        part = qs_u[s, a0:a0 + nrow, qt * T:(qt + 1) * T]
        if nrow < 32:
            part = jnp.concatenate([part, jnp.zeros((32 - nrow, T), u32)], axis=0)
        shift = (dst - t0) - (src - a0)
        if shift:
            part = pltpu.roll(part, shift % 32, 0)
        rid = lax.broadcasted_iota(i32, (32, T), 0) + t0
        out = []
        for lo in (dst, dst + hw):
            piece = jnp.where((rid >= lo) & (rid < lo + hw), part, u32(0))
            piece = piece[0:min(32, TW - t0)]
            pieces = [jnp.zeros((t0, T), u32)] * (t0 > 0) + [piece] + [jnp.zeros((TW - t0 - 32, T), u32)] * (t0 + 32 < TW)
            out.append(jnp.concatenate(pieces, axis=0))
        return out

    def stage_a(unit, u, qt):
        s, k = unit
        s_ref, m_ref = bufs[k % 2]
        pi = k * NP + u
        g = pi // (HPG // 2)
        sg = s * NG + g
        n = T * (qt + 1)
        w_a, w_b = pair_weights(s, pi, qt)
        w_ab = _bf(jnp.where(lane64 < HT, w_a, w_b))

        def colmax8(v):
            return jnp.max(v.reshape(v.shape[0] // 8, 8, T), axis=0)

        maxes = []
        for hd, w in enumerate((_bf(w_a), _bf(w_b))):
            m8 = None
            for c in range(qt):
                kc = _bf(k_u[sg, c * TW:(c + 1) * TW, :])
                sc = jnp.dot(kc, w, preferred_element_type=f32)
                s_ref[u, qt, hd * L + c * T:hd * L + (c + 1) * T, :] = sc
                m8 = colmax8(sc) if m8 is None else jnp.maximum(m8, colmax8(sc))
            kc = _bf(k_u[sg, qt * TW:qt * TW + TW // 2, :])
            sc = jnp.dot(kc, w, preferred_element_type=f32) + mb[1 - hd]
            s_ref[u, qt, hd * L + qt * T:hd * L + qt * T + HT, :] = sc
            m8 = colmax8(sc) if m8 is None else jnp.maximum(m8, colmax8(sc))
            maxes.append(m8)
        kc = _bf(k_u[sg, qt * TW + TW // 2:(qt + 1) * TW, :])
        sc = jnp.dot(kc, w_ab, preferred_element_type=f32) + mb[2]
        s_ref[u, qt, n - HT:n, :] = sc
        mab = colmax8(sc)
        m_a = jnp.where(lane8 < HT, jnp.maximum(maxes[0], mab), maxes[0])
        m_b = jnp.where(lane8 >= HT, jnp.maximum(maxes[1], mab), maxes[1])
        m_ref[u, qt, 0] = jnp.broadcast_to(jnp.max(m_a, axis=0, keepdims=True), (8, T))
        m_ref[u, qt, 1] = jnp.broadcast_to(jnp.max(m_b, axis=0, keepdims=True), (8, T))

    def stage_b(unit, u, qt):
        s, k = unit
        s_ref, m_ref = bufs[k % 2]
        pi = k * NP + u
        n = T * (qt + 1)
        m_a = m_ref[u, qt, 0][0:1]
        m_b = m_ref[u, qt, 1][0:1]
        p_ab = jnp.exp2(s_ref[u, qt, n - HT:n, :] - jnp.where(lane1 < HT, m_a, m_b))
        for hd, m in enumerate((m_a, m_b)):
            h = 2 * pi + hd
            p = jnp.exp2(s_ref[u, qt, hd * L:hd * L + n - HT, :] - m)
            keep = (lane64 < HT) if hd == 0 else (lane64 >= HT)
            p = jnp.concatenate([p, jnp.where(keep, p_ab, 0.0)], axis=0).astype(bf16)
            w0 = ((DH * h) // 16) * 16
            off = DH * h - w0
            o = jnp.dot(_bf(vwin[s * H + h, :, 0:n]), p, preferred_element_type=f32)
            den = o[0:1] if off == 14 else o[31:32]
            r0, r1 = (off // 8) * 8, -(-(off + DH) // 8) * 8
            o = o[r0:r1] * (omg[h][0:1] / den)
            if hd == 0:
                o = pltpu.roll(o, HT, 1)
            res = am[s, w0 + r0:w0 + r1, qt * T:(qt + 1) * T] + o
            rid = lax.broadcasted_iota(i32, (r1 - r0, T), 0) + r0
            pltpu.store(ots[qt].at[w0 + r0:w0 + r1, :], res, mask=(rid >= off) & (rid < off + DH))

    def a_tasks(unit):
        return [lambda u=u, qt=qt: stage_a(unit, u, qt) for u in range(NP) for qt in QT_ORDER]

    def b_tasks(unit):
        return [lambda u=u, qt=qt: stage_b(unit, u, qt) for u in range(NP) for qt in QT_ORDER]

    w_copy(3).wait()
    rr = jnp.concatenate([r_buf[s][0:1, :] for s in range(NSEG)], axis=0)
    rr = _round_bf16(rr)
    tok = lax.broadcasted_iota(i32, (NSEG, L), 0) * L + lax.broadcasted_iota(i32, (NSEG, L), 1)
    m1v = jnp.max(rr)
    i1 = jnp.min(jnp.where(rr == m1v, tok, SEQ))
    rr2 = jnp.where(tok == i1, -jnp.inf, rr)
    m2v = jnp.max(rr2)
    i2 = jnp.min(jnp.where(rr2 == m2v, tok, SEQ))
    i1 = jnp.clip(i1, 0, SEQ - 1)
    i2 = jnp.clip(i2, 0, SEQ - 1)

    row16 = lax.broadcasted_iota(i32, (16, T), 0)
    lane16 = lax.broadcasted_iota(i32, (16, T), 1)

    def token_rows(i, slot):
        onehot = jnp.where((row16 == slot) & (lane16 == i % T), 1.0, 0.0).astype(bf16)
        return lax.dot_general(onehot, _bf(xn_u[i // LNW, :, pl.ds(pl.multiple_of(((i // T) % BT) * T, T), T)]), NT_DIMS, preferred_element_type=f32)

    def select_task():
        xsel_buf[...] = _pack(token_rows(i1, 0) + token_rows(i2, 1))
        y_acc[...] = jnp.zeros(y_acc.shape, f32)

    def expert_tile(w_ref, ft):
        return _bf(w_ref.at[ft].bitcast(u32)[...])

    def moe_up_task(ft, k, which):
        xsel = _bf(xsel_buf[:, 0:D])
        w_ref = (wg_buf, wu_buf)[which]
        hid_buf[k, which] = jnp.dot(xsel, expert_tile(w_ref, ft), preferred_element_type=f32)

    def moe_down_task(ft, k):
        gt = _round_bf16(hid_buf[k, 0])
        up = _round_bf16(hid_buf[k, 1])
        hid = (_round_bf16(gt * _sigmoid(gt)) * up).astype(bf16)
        y_acc[...] += lax.dot_general(hid, expert_tile(wd_buf, ft), NT_DIMS, preferred_element_type=f32)

    def moe_tasks(ft0, count):
        tasks = []
        for k0 in range(0, count, FPB):
            ks = range(k0, min(k0 + FPB, count))
            tasks += [lambda k=k, w=w: moe_up_task(ft0 + k, k, w) for k in ks for w in range(2)]
            tasks += [lambda k=k: moe_down_task(ft0 + k, k) for k in ks]
        return tasks

    def moe_finish():
        y = _round_bf16(y_acc[...])
        rsel = jnp.where(lax.broadcasted_iota(i32, (16, 1), 0) == 0, m1v, m2v)
        y = _round_bf16(y * _round_bf16(_sigmoid(rsel)))
        y = jnp.concatenate([y, jnp.zeros((16, DP - D), f32)], axis=1)
        y = jnp.concatenate([jnp.zeros((HT, DP), f32), y, jnp.zeros((T - HT - 16, DP), f32)], axis=0)
        y_t = jnp.concatenate([y.T[0:D], jnp.zeros((D, T), f32)], axis=1)
        y_u = _pack(y_t)[:, 0:T]
        lane = lax.broadcasted_iota(i32, (D // 2, T), 1)
        wot_u[:, DP - T:DP] = jnp.where(lane < HT, wot_u[:, DP - T:DP], y_u)
        rid = lax.broadcasted_iota(i32, (8, T), 0)
        for tt in range(TPS):
            tok_l = lax.broadcasted_iota(i32, (8, T), 1) + (NSEG - 1) * L + tt * T
            ots[tt][D:D + 8, :] = jnp.where(((rid == 0) & (tok_l == i1)) | ((rid == 1) & (tok_l == i2)), 1.0, 0.0)

    dense = _interleave(a_tasks((0, 0)), prep_dense(3, wot_u, 0))
    with _scope("p15_mix"):
        cut = (2 * len(dense)) // 3
        run(dense[:cut] + [select_task] + dense[cut:])

    for i in range(3):
        moe_wait(i)

    def out_tile(s, tt, chunk_copies=None):
        c0 = s * L + tt * T
        if not isinstance(s, int):
            c0 = pl.multiple_of(c0, T)
        o_bf = ots[tt][...].astype(bf16)
        nchunk = 4
        rows = D // nchunk
        for rc in range(nchunk):
            r0 = rc * rows
            attn = jnp.dot(_bf(wot_u[r0 // 2:(r0 + rows) // 2, :]), o_bf, preferred_element_type=f32)
            xn = _bf(xn_u[s * (L // LNW) + tt // BT, r0 // 2:(r0 + rows) // 2, (tt % BT) * T:(tt % BT + 1) * T]).astype(f32)
            x = x_rows(s * TPS + tt, r0, r0 + rows).astype(f32)
            res = x + attn + xn
            out_buf[r0:r0 + rows, pl.ds(c0, T)] = res.astype(bf16)
            if chunk_copies is not None:
                chunk_copies[rc].start()

    def pair_tasks(ua, ub):
        tasks = []
        for x, y in zip(a_tasks(ua), b_tasks(ub)):
            tasks += [x, y]
        return tasks

    def seg_end(s, last):
        def by_qt(fn, unit, qt):
            return [lambda u=u: fn(unit, u, qt) for u in range(NP)]

        steps = []
        for step in range(7):
            lists = []
            if step < 4:
                lists.append(by_qt(stage_b, (s, 2), 3 - step))
                lists.append(by_qt(stage_a, (s, 3), 3 - step))
            if 1 <= step < 5:
                lists.append(by_qt(stage_b, (s, 3), 4 - step))
            if not last and 2 <= step < 6:
                lists.append(by_qt(stage_a, (s + 1, 0), 5 - step))
            if step >= 3:
                lists.append([lambda tt=6 - step: out_tile(s, tt)])
            steps.append(_interleave(*lists))
        return steps

    def seg_att(s, c):
        tasks = pair_tasks((s, 1), (s, 0)) + pair_tasks((s, 2), (s, 1))
        steps = seg_end(s, False)
        for step in steps[0:5]:
            tasks += step
        with _scope("att_seg"):
            run(_interleave(tasks, moe_tasks(s * FPI, FPI)))
            for step in steps[5:]:
                run(step)

        @pl.when(s < NSEG - 2)
        def _():
            out_copy(pl.multiple_of(s * L, L), L, s).start()
        return c

    lax.fori_loop(0, NSEG - 1, seg_att, 0)

    npatch = (NSEG - 1) * TPS

    def patch_tile(idx):
        return jnp.where(idx < npatch * T, idx // T, 0)

    tile0 = patch_tile(i1)
    tile1 = patch_tile(i2)
    tile1 = jnp.where(tile1 == tile0, (tile0 + 1) % npatch, tile1)

    def patch(tile):
        c0 = pl.multiple_of(tile * T, T)
        rid = lax.broadcasted_iota(i32, (T, T), 0)
        tok_l = lax.broadcasted_iota(i32, (T, T), 1) + c0
        hit = ((rid == HT) & (tok_l == i1)) | ((rid == HT + 1) & (tok_l == i2))
        onehot = jnp.where(hit, 1.0, 0.0).astype(bf16)
        for rc in range(4):
            r0, r1 = rc * (D // 4), (rc + 1) * (D // 4)
            upd = jnp.dot(_bf(wot_u[r0 // 2:r1 // 2, DP - T:DP]), onehot, preferred_element_type=f32)
            cur = out_buf[r0:r1, pl.ds(c0, T)].astype(f32)
            out_buf[r0:r1, pl.ds(c0, T)] = (cur + upd).astype(bf16)

    sent = (NSEG - 2) * TPS
    resend0 = jnp.where(tile0 < sent, tile0, jnp.where(tile1 == 0, 1, 0))
    resend1 = jnp.where(tile1 < sent, tile1, jnp.where(resend0 == 0, 1, 0))
    patch_copies = [out_copy(pl.multiple_of(resend0 * T, T), T, 7), out_copy(pl.multiple_of(resend1 * T, T), T, 8),
                    out_copy((NSEG - 2) * L, L, NSEG - 2)]
    last_copies = [out_copy((NSEG - 1) * L + tt * T, T, NSEG - 1 + tt) for tt in range(1, TPS)]
    c_fin = (NSEG - 1) * L
    final_copies = [
        pltpu.make_async_copy(out_buf.at[rc * (D // 4):(rc + 1) * (D // 4), c_fin:c_fin + T],
                              out_hbm.at[rc * (D // 4):(rc + 1) * (D // 4), c_fin:c_fin + T],
                              sems.at[SEM_FINAL + rc]) for rc in range(4)]

    sl = NSEG - 1
    for s in range(NSEG - 2):
        out_copy(s * L, L, s).wait()
    with _scope("tail_2"):
        moe_finish()
        run(pair_tasks((sl, 1), (sl, 0)))
        patch(tile0)
        patch(tile1)
        run(pair_tasks((sl, 2), (sl, 1)))
        for cp in patch_copies:
            cp.start()
        steps = seg_end(sl, True)
        for step in steps[0:5]:
            run(step)
        last_copies[2].start()
        last_copies[1].start()
    with _scope("tail_3"):
        run(steps[5])
        last_copies[0].start()
        out_tile(sl, 0, final_copies)

    with _scope("out_wait"):
        for cp in patch_copies + last_copies + final_copies:
            cp.wait()


@jax.jit
def pallas_parallel_sum__memory_aug_infini_attn__moe_arch_mod__prompt_kernel(
    A_x: jax.Array,
    A_wq: jax.Array,
    A_wk: jax.Array,
    A_wv: jax.Array,
    A_wo: jax.Array,
    A_beta: jax.Array,
    B_x: jax.Array,
    B_w_r: jax.Array,
    B_w_gate: jax.Array,
    B_w_up: jax.Array,
    B_w_down: jax.Array,
):
    del B_x
    any_spec = pl.BlockSpec(memory_space=pl.ANY)
    scratch = [
        pltpu.VMEM((H,), bf16),
        pltpu.VMEM((D,), bf16),
        pltpu.VMEM((NT, D, T), bf16),
        pltpu.VMEM((4, D, D), bf16),
        pltpu.VMEM((NFT, D, T), bf16),
        pltpu.VMEM((NFT, D, T), bf16),
        pltpu.VMEM((NFT, D, T), bf16),
        pltpu.VMEM((D, SEQ), bf16),
        pltpu.VMEM((WT_ALLOC, DP), u32),
        pltpu.VMEM((2, D // 2, LNW), u32),
        pltpu.VMEM((D // 2, DP), u32),
        pltpu.VMEM((SEQ // LNW, DP // 2, LNW), u32),
        pltpu.VMEM((DP // 2, LNW), u32),
        pltpu.VMEM((DP // 2, LNW), u32),
        pltpu.VMEM((NSEG, D // 2, L), u32),
        pltpu.VMEM((NSEG * NG, L // 2, T), u32),
        pltpu.VMEM((NSEG, D // 2, L), u32),
        pltpu.VMEM((NSEG, D // 2, L), u32),
        pltpu.VMEM((NSEG, D // 2, L), u32),
        pltpu.VMEM((NSEG * H, 16, L), u32),
        pltpu.VMEM((NSEG, 8, L), f32),
        pltpu.VMEM((NG, T, T), f32),
        pltpu.VMEM((NG, T, T), f32),
        pltpu.VMEM((NG, T, T), i32),
        pltpu.VMEM((NSEG, D, L), f32),
        pltpu.VMEM((NG, 8, T), f32),
        pltpu.VMEM((H, 8, T), f32),
        pltpu.VMEM((3, HT, T), f32),
        pltpu.VMEM((NP, 4, 2 * L, T), f32),
        pltpu.VMEM((NP, 4, 2, 8, T), f32),
        pltpu.VMEM((NP, 4, 2 * L, T), f32),
        pltpu.VMEM((NP, 4, 2, 8, T), f32),
        pltpu.VMEM((DP, T), f32),
        pltpu.VMEM((DP, T), f32),
        pltpu.VMEM((DP, T), f32),
        pltpu.VMEM((DP, T), f32),
        pltpu.VMEM((2, D, LNW), f32),
        pltpu.VMEM((2, 2, 8, LNW), f32),
        pltpu.VMEM((16, D), f32),
        pltpu.VMEM((8, DP), u32),
        pltpu.VMEM((FPI, 2, 16, T), f32),
        pltpu.SemaphoreType.DMA((NSEM,)),
    ]
    x_t = jnp.transpose(A_x, (0, 2, 1)).reshape(D, SEQ)
    out_t = pl.pallas_call(
        _kernel,
        out_shape=jax.ShapeDtypeStruct((D, SEQ), bf16),
        in_specs=[any_spec] * 10,
        out_specs=any_spec,
        scratch_shapes=scratch,
        compiler_params=pltpu.CompilerParams(vmem_limit_bytes=110 * 1024 * 1024),
    )(x_t, A_wq, A_wk, A_wv, A_wo, A_beta, B_w_r, B_w_gate, B_w_up, B_w_down.T)
    return jnp.transpose(out_t.reshape(1, D, SEQ), (0, 2, 1))
```

```python
import contextlib

import jax
import jax.numpy as jnp
from jax import lax
from jax.experimental import pallas as pl
from jax.experimental.pallas import tpu as pltpu

bf16 = jnp.bfloat16
f32 = jnp.float32
u32 = jnp.uint32
i32 = jnp.int32

SEQ = 2048
D = 576
DP = 640
H = 32
DH = 18
NSEG = 4
L = 512
T = 128
TW = T // 2
HT = T // 2
TPS = L // T
HPG = 6
NG = 6
F = 4608
FPI = 12
FPB = 3
NFT = F // T
NP = 4
UPS = H // (2 * NP)
NT = SEQ // T
LNW = 256
BT = LNW // T
NORM_PARTS = 6
QK_BLOCK = 64
VB = 8 * DH

LOG2E = 1.4426950408889634
QSCALE = (DH ** -0.5) * LOG2E
MASKVAL = -1000000000.0 * LOG2E
EPS_BF16 = 1.0013580322265625e-05
ONES_PAIR = 0x3F803F80

NT_DIMS = (((1,), (1,)), ((), ()))
NN_DIMS = (((1,), (0,)), ((), ()))
VW = 24

WT_Q = 0
WT_K = D // 2
WT_R = D
WT_V = D + 8
WT_ALLOC = 1056
NBLK = DP // T

X_PIECES = ((0, LNW), (LNW, LNW), (L, L), (2 * L, L), (3 * L, L))
SEM_X = 0
SEM_W = 5
SEM_MOE = 9
SEM_OUT = 12
SEM_SMALL = 21
SEM_WQB = 23
SEM_FINAL = 24
NSEM = 28
WQ_SPLIT = 2 * T


PROFILE_SCOPES = False
QT_ORDER = (3, 0, 2, 1)


def _scope(name):
    return jax.named_scope(name) if PROFILE_SCOPES else contextlib.nullcontext()


def _valid(g):
    return min(HPG * DH, D - g * HPG * DH)


def _ewin(g):
    start = (g * HPG * DH // 16) * 16
    return start, g * HPG * DH - start, min(T, D - start)


def _ones_row(off):
    return VW - 1 if off + DH < VW else 0


def _bf(x):
    return pltpu.bitcast(x, bf16)


def _pack(x):
    return pltpu.bitcast(x.astype(bf16), u32)


def _round_bf16(x):
    return x.astype(bf16).astype(f32)


def _phi(t):
    return jnp.where(t > 0, t + 1.0, jnp.exp(t))


def _sigmoid(t):
    return 1.0 / (1.0 + jnp.exp(-t))


def _zero_after(v):
    bits = pltpu.bitcast(v[0:8, 0:LNW], u32)
    sixteen = jnp.uint32(16)
    bits = lax.shift_right_logical(lax.shift_right_logical(bits, sixteen), sixteen)
    return pltpu.bitcast(bits, f32)


def _interleave(*lists):
    items = []
    for li, tasks in enumerate(lists):
        for k, t in enumerate(tasks):
            items.append(((k + 0.5) / len(tasks), li, k, t))
    items.sort(key=lambda it: it[:3])
    return [it[3] for it in items]


def _kernel(x_hbm, wq_hbm, wk_hbm, wv_hbm, wo_hbm, beta_hbm, wr_hbm, wg_hbm, wu_hbm, wd_hbm,
            out_hbm,
            beta_ref, wr_ref, x_buf, w_buf, wg_buf, wu_buf, wd_buf, out_buf,
            wt_u, kt_tmp, wot_u, xn_u, xs_a, xs_b, qs_u, k_u, pq_u, pk_u, vt_u, vwin,
            r_buf, mt_acc, lm_f, mcode, am, g16, omg, mb,
            s0, m0, s1, m1, ot0, ot1, ot2, ot3, xf, ln_stat, y_acc, xsel_buf, hid_buf, sems):

    class XCopy:
        def __init__(self, i):
            c0, width = X_PIECES[i]
            self.copies = [pltpu.make_async_copy(x_hbm.at[:, c:c + T], x_buf.at[c // T], sems.at[SEM_X + i])
                           for c in range(c0, c0 + width, T)]

        def start(self):
            for cp in self.copies:
                cp.start()

        def wait(self):
            for cp in self.copies:
                cp.wait()

    x_copy = XCopy

    def x_rows(tile, r0, r1):
        return _bf(x_buf.at[tile].bitcast(u32)[r0 // 2:r1 // 2, :])

    def w_copy(i):
        src = (wq_hbm, wk_hbm, wv_hbm, wo_hbm)[i]
        return pltpu.make_async_copy(src, w_buf.at[i], sems.at[SEM_W + i])

    wq_first = pltpu.make_async_copy(wq_hbm.at[:, 0:WQ_SPLIT], w_buf.at[0, :, 0:WQ_SPLIT], sems.at[SEM_W])
    wq_rest = pltpu.make_async_copy(wq_hbm.at[:, WQ_SPLIT:D], w_buf.at[0, :, WQ_SPLIT:D], sems.at[SEM_WQB])

    moe_src = (wg_hbm, wu_hbm, wd_hbm)
    moe_dst = (wg_buf, wu_buf, wd_buf)

    def moe_start(i, ft):
        c0 = ft * T if isinstance(ft, int) else pl.multiple_of(ft * T, T)
        pltpu.make_async_copy(moe_src[i].at[:, pl.ds(c0, T)], moe_dst[i].at[ft], sems.at[SEM_MOE + i]).start()

    def moe_issue(first, last):
        for n in range(first, last):
            moe_start(n % 3, n // 3)

    def moe_wait(i):
        pltpu.make_async_copy(moe_dst[i], moe_dst[i], sems.at[SEM_MOE + i]).wait()

    def out_copy(c0, width, sem):
        return pltpu.make_async_copy(out_buf.at[:, pl.ds(c0, width)], out_hbm.at[:, pl.ds(c0, width)],
                                     sems.at[SEM_OUT + sem])

    small_copies = [pltpu.make_async_copy(beta_hbm, beta_ref, sems.at[SEM_SMALL]),
                    pltpu.make_async_copy(wr_hbm, wr_ref, sems.at[SEM_SMALL + 1])]
    x_copy(0).start()
    wq_first.start()
    wq_rest.start()
    x_copy(1).start()
    for cp in small_copies:
        cp.start()
    w_copy(1).start()
    w_copy(2).start()

    init_scope = _scope("init")
    init_scope.__enter__()
    kr = lax.broadcasted_iota(i32, (HT, T), 0)
    ql = lax.broadcasted_iota(i32, (HT, T), 1)
    mb[0] = jnp.where(ql < kr, MASKVAL, 0.0).astype(f32)
    mb[1] = jnp.where((ql >= HT) & (ql - HT < kr), MASKVAL, 0.0).astype(f32)
    mb[2] = jnp.where(ql % HT < kr, MASKVAL, 0.0).astype(f32)
    zpad = jnp.zeros(((DP - D) // 2, LNW), u32)
    for blk in range(SEQ // LNW):
        xn_u[blk, D // 2:DP // 2, :] = zpad
    xs_a[D // 2:DP // 2, :] = zpad
    xs_b[D // 2:DP // 2, :] = zpad
    ots = (ot0, ot1, ot2, ot3)
    for o_ref in ots:
        o_ref[D:DP, :] = jnp.zeros((DP - D, T), f32)
    am[0] = jnp.zeros(am.shape[1:], f32)
    mt_acc[...] = jnp.zeros(mt_acc.shape, f32)
    g16[...] = jnp.zeros(g16.shape, f32)

    init_scope.__exit__(None, None, None)

    pace = [None]

    def gate_tables():
        gate = _round_bf16(_sigmoid(beta_ref[...].reshape(1, H).astype(f32)))
        for h in range(H):
            gh = jnp.broadcast_to(gate[:, h:h + 1], (1, T))
            omg[h] = jnp.broadcast_to(_round_bf16(1.0 - gh), (8, T))
            g16[h // HPG, (h % HPG):(h % HPG) + 1, :] = gh

    def transpose_block(i, cb):
        c1 = min((cb + 1) * T, D)
        blk = w_buf[i, :, cb * T:c1]
        if c1 - cb * T < T:
            blk = jnp.concatenate([blk, jnp.zeros((D, T - (c1 - cb * T)), bf16)], axis=1)
        blk = jnp.concatenate([blk, jnp.zeros((DP - D, T), bf16)], axis=0)
        return pltpu.bitcast(blk.T, u32)

    def prep_dense(i, dst, base):
        def task(cb):
            nrow = min(TW, D // 2 - cb * TW)
            dst[base + cb * TW:base + cb * TW + nrow, :] = transpose_block(i, cb)[0:nrow]
        return [lambda cb=cb: task(cb) for cb in range(DP // T)]

    def router_row():
        wr = wr_ref[...].reshape(1, D).astype(f32)
        wr = jnp.concatenate([wr, jnp.zeros((1, DP - D), f32)], axis=1)
        bits = lax.shift_right_logical(pltpu.bitcast(wr, u32), u32(16))
        rid = lax.broadcasted_iota(i32, (8, DP), 0)
        wt_u[WT_R:WT_R + 8, :] = jnp.where(rid == 0, bits, u32(0))

    def ln_tasks(s, p, stage):
        tile0 = s * TPS + p * BT

        def mean_pass():
            acc = pace[0]
            for r in range(0, D, 64):
                x = jnp.concatenate([pltpu.bitcast(x_rows(tile0 + t, r, r + 64), u32) for t in range(BT)], axis=1)
                x = _bf(x).astype(f32)
                xf[p, r:r + 64, :] = x
                part = jnp.sum(x.reshape(8, 8, LNW), axis=0)
                acc = part if acc is None else acc + part
            mean = jnp.sum(acc, axis=0, keepdims=True) / D
            ln_stat[p, 0] = jnp.broadcast_to(mean, (8, LNW))

        def var_pass():
            mean = ln_stat[p, 0][0:1]
            if pace[0] is not None:
                mean = mean + pace[0][0:1]
            acc = None
            for r in range(0, D, 96):
                xc = xf[p, r:r + 96, :] - mean
                part = jnp.sum((xc * xc).reshape(12, 8, LNW), axis=0)
                acc = part if acc is None else acc + part
            var = jnp.sum(acc, axis=0, keepdims=True) / D
            den = _round_bf16(jnp.sqrt(_round_bf16(_round_bf16(var) + EPS_BF16)))
            ln_stat[p, 1] = jnp.broadcast_to(1.0 / den, (8, LNW))
            ln_stat[p, 0] = jnp.broadcast_to(_round_bf16(mean), (8, LNW))

        def norm_pass(part):
            mean_b = ln_stat[p, 0][0:1]
            if pace[0] is not None:
                mean_b = mean_b + pace[0][0:1]
            inv = ln_stat[p, 1][0:1]
            step = D // NORM_PARTS
            for r in range(part * step, (part + 1) * step, 48):
                xn = _pack(_round_bf16(xf[p, r:r + 48, :] - mean_b) * inv)
                xn_u.at[s * (L // LNW) + p][r // 2:r // 2 + 24, :] = xn
                if stage is not None:
                    stage[r // 2:r // 2 + 24, :] = xn

        return [mean_pass, var_pass] + [lambda part=part: norm_pass(part) for part in range(NORM_PARTS)]

    def load_xs(s, p, stage):
        return _bf(xn_u[s * (L // LNW) + p] if stage is None else stage[...])

    def row_blocks(size):
        return [(r, min(r + size, D)) for r in range(0, D, size)]

    def q_task(s, p, stage, r0, r1):
        rows = slice(r0 // 2, r1 // 2)
        cols = slice(p * LNW, (p + 1) * LNW)
        w = _bf(wt_u[WT_Q + r0 // 2:WT_Q + r1 // 2, :])
        q = jnp.dot(w, load_xs(s, p, stage), preferred_element_type=f32)
        pace[0] = _zero_after(q)
        qs = q * QSCALE
        qrot = jnp.concatenate([pltpu.roll(qs[:, t * T:(t + 1) * T], HT, 1) for t in range(BT)], axis=1)
        rid = lax.broadcasted_iota(i32, qs.shape, 0) + r0
        even = ((rid // DH) % 2) == 0
        qs_u.at[s][rows, cols] = _pack(jnp.where(even, qrot, qs))
        pq_u.at[s][rows, cols] = _pack(_phi(q))

    def k_task(s, p, stage, r0, r1):
        rows = slice(r0 // 2, r1 // 2)
        cols = slice(p * LNW, (p + 1) * LNW)
        extra = 8 if r1 == D else 0
        w = _bf(wt_u[WT_K + r0 // 2:WT_K + r1 // 2 + extra, :])
        k = jnp.dot(w, load_xs(s, p, stage), preferred_element_type=f32)
        pace[0] = _zero_after(k)
        if extra:
            r_buf[s, :, cols] = jnp.broadcast_to(k[r1 - r0:r1 - r0 + 1, :], (8, LNW))
            k = k[0:r1 - r0]
        kt_tmp.at[p][rows, :] = _pack(k)
        pk_u.at[s][rows, cols] = _pack(_phi(k))

    def kt_task(s, p, g):
        nv = _valid(g) // 2
        src = g * HPG * DH // 2
        kg = jnp.concatenate([kt_tmp[p, src:src + nv, :], jnp.zeros((TW - nv, LNW), u32)], axis=0)
        k_u.at[s * NG + g][p * (LNW // 2):(p + 1) * (LNW // 2), :] = pltpu.bitcast(_bf(kg).T, u32)

    def v_task(s, p, stage, b):
        cols = slice(p * LNW, (p + 1) * LNW)
        w = _bf(wt_u[WT_V + b * (VB // 2):WT_V + (b + 1) * (VB // 2), :])
        v = jnp.dot(w, load_xs(s, p, stage), preferred_element_type=f32)
        pace[0] = _zero_after(v)
        vt_u.at[s][b * (VB // 2):(b + 1) * (VB // 2), cols] = _pack(v)
        sub = lax.broadcasted_iota(i32, (VW, LNW), 0)
        for hh in range(8):
            r0 = (DH * hh // 8) * 8
            ones_row = _ones_row(DH * hh - r0)
            vwin.at[s * H + 8 * b + hh][:, cols] = jnp.where(sub == ones_row, 1.0, v[r0:r0 + VW, :])

    def q_tasks(s, p, stage=None, size=QK_BLOCK):
        return [lambda b=b: q_task(s, p, stage, *b) for b in row_blocks(size)]

    def k_tasks(s, p, stage=None, size=QK_BLOCK):
        tasks, done = [], 0
        for b in row_blocks(size):
            tasks.append(lambda b=b: k_task(s, p, stage, *b))
            while done < NG and done * HPG * DH + _valid(done) <= b[1]:
                tasks.append(lambda g=done: kt_task(s, p, g))
                done += 1
        return tasks

    def v_tasks(s, p, stage=None):
        return [lambda b=b: v_task(s, p, stage, b) for b in range(D // VB)]

    def mem_layout(g):
        es, eoff, _ = _ewin(g)
        nv = _valid(g)
        ne = -(-(eoff + nv) // 16) * 16
        ones_row = 0 if eoff >= 2 else eoff + nv
        nh = nv // DH
        den_row = 0 if eoff >= nh else ne
        return es, eoff, nv, ne, ones_row, den_row, max(ne, den_row + 16 * (den_row > 0))

    def mem_update(sp, g):
        es, eoff, nv, ne, ones_row, den_row, nr = mem_layout(g)
        nw = min(T, D - es)
        win = vt_u[sp, es // 2:(es + ne) // 2, :]
        wid = lax.broadcasted_iota(i32, win.shape, 0)
        lhs = _bf(jnp.where(wid == ones_row // 2, u32(ONES_PAIR), win))
        upd = lax.dot_general(lhs, _bf(pk_u[sp, es // 2:(es + nw) // 2, :]), NT_DIMS, preferred_element_type=f32)
        mt = mt_acc[g, 0:ne, 0:nw] + upd
        mt_acc[g, 0:ne, 0:nw] = mt
        z = jnp.broadcast_to(mt[ones_row:ones_row + 1, :], (nr, nw))
        if nr > ne:
            mt = jnp.concatenate([mt, jnp.zeros((nr - ne, nw), f32)], axis=0)
        code = mcode[g, 0:nr, 0:nw]
        lm_f[g, 0:nr, 0:nw] = jnp.where(code == 1, mt, jnp.where(code == 2, z, 0.0))

    def mem_masks():
        for g in range(NG):
            es, eoff, nv, ne, ones_row, den_row, nr = mem_layout(g)
            row = lax.broadcasted_iota(i32, (T, T), 0)
            d_loc = lax.broadcasted_iota(i32, (T, T), 1) - eoff
            e_loc = row - eoff
            d_ok = (d_loc >= 0) & (d_loc < nv)
            same_head = (e_loc >= 0) & (e_loc < nv) & d_ok & ((e_loc // DH) == (d_loc // DH))
            den_hit = (row >= den_row) & d_ok & ((d_loc // DH) == row - den_row)
            mcode[g] = jnp.where(same_head, 1, jnp.where(den_hit, 2, 0))

    def mem_retrieve(s, g):
        es, eoff, nv, ne, ones_row, den_row, nr = mem_layout(g)
        nw = min(T, D - es)
        nd = jnp.dot(lm_f[g, 0:nr, 0:nw].astype(bf16), _bf(pq_u[s, es // 2:(es + nw) // 2, :]),
                     preferred_element_type=f32)
        scale = jnp.broadcast_to(g16[g][:, 0:1], (8, L)) / (nd[den_row:den_row + 8, :] + 1e-6)
        r8 = lax.broadcasted_iota(i32, (8, L), 0)
        for b in range(ne // 8):
            lo, hi = 8 * b - eoff, 8 * b + 7 - eoff
            if hi < 0 or lo >= nv:
                continue
            j1, j2 = max(lo, 0) // DH, min(hi, nv - 1) // DH
            sc = jnp.broadcast_to(scale[j1:j1 + 1, :], (8, L))
            if j2 != j1:
                sc = jnp.where(r8 < DH * j2 - lo, sc, jnp.broadcast_to(scale[j2:j2 + 1, :], (8, L)))
            val = nd[8 * b:8 * b + 8, :] * sc
            dst = am.at[s, es + 8 * b:es + 8 * b + 8, :]
            if lo >= 0 and hi < nv:
                dst[...] = val
            else:
                pltpu.store(dst, val, mask=(r8 + lo >= 0) & (r8 + lo < nv))

    def run(tasks):
        for t in tasks:
            t()

    prep_q = prep_dense(0, wt_u, WT_Q)
    q0a = q_tasks(0, 0, None, T)
    mem_masks()
    with _scope("p1_wait_x0"):
        x_copy(0).wait()
    for i in range(2, len(X_PIECES)):
        x_copy(i).start()
    w_copy(3).start()
    moe_issue(0, 40)
    with _scope("p1_ln0a"):
        run(ln_tasks(0, 0, None))
        wq_first.wait()
    with _scope("p1_q0a_first"):
        run(prep_q[0:2] + q0a[0:2])
        wq_rest.wait()
        x_copy(1).wait()
    with _scope("p1_q0a"):
        run(prep_q[2:])
        run(_interleave(q0a[2:], ln_tasks(0, 1, None)))
        w_copy(1).wait()
        for cp in small_copies:
            cp.wait()
    k0b = k_tasks(0, 1)
    with _scope("p1_q0b"):
        run(_interleave(q_tasks(0, 1), prep_dense(1, wt_u, WT_K), [router_row, gate_tables]))
        run([lambda b=b: k_task(0, 0, None, *b) for b in row_blocks(QK_BLOCK)])
        w_copy(2).wait()
        x_copy(2).wait()
    moe_issue(40, 60)
    with _scope("p1_k0v0"):
        run(_interleave(k0b, prep_dense(2, wt_u, WT_V), [lambda g=g: kt_task(0, 0, g) for g in range(NG)]))
        run(_interleave(v_tasks(0, 0) + v_tasks(0, 1), ln_tasks(1, 0, xs_a)))

    moe_issue(60, 72)

    def seg_body(s, c):
        for ss in range(2, NSEG):
            @pl.when(s + 1 == ss)
            def _():
                x_copy(ss + 1).wait()
                if ss == NSEG - 1:
                    moe_issue(72, 3 * NFT)
        nxt = jnp.minimum(s + 1, NSEG - 1)
        pace[0] = None
        with _scope("p1_seg"):
            updates = [lambda g=g: mem_update(s - 1, g) for g in range(NG)]
            retrieves = [lambda g=g: mem_retrieve(s, g) for g in range(NG)]
            first = _interleave(q_tasks(s, 0, xs_a), updates) + k_tasks(s, 0, xs_a) + v_tasks(s, 0, xs_a)
            run(_interleave(first, ln_tasks(s, 1, xs_b)))
            second = q_tasks(s, 1, xs_b) + _interleave(k_tasks(s, 1, xs_b) + v_tasks(s, 1, xs_b), retrieves)
            run(_interleave(second, ln_tasks(nxt, 0, xs_a)))
        return c

    lax.fori_loop(1, NSEG, seg_body, 0)

    bufs = ((s0, m0), (s1, m1))
    lane64 = lax.broadcasted_iota(i32, (TW, T), 1)
    lane1 = lax.broadcasted_iota(i32, (1, T), 1)
    lane8 = lax.broadcasted_iota(i32, (8, T), 1)

    def pair_weights(s, pi, qt):
        hw = DH // 2
        j = 2 * (pi % (HPG // 2))
        src, dst = hw * 2 * pi, hw * j
        a0, t0 = (src // 8) * 8, (dst // 8) * 8
        nrow = min(32, D // 2 - a0)
        part = qs_u[s, a0:a0 + nrow, qt * T:(qt + 1) * T]
        if nrow < 32:
            part = jnp.concatenate([part, jnp.zeros((32 - nrow, T), u32)], axis=0)
        shift = (dst - t0) - (src - a0)
        if shift:
            part = pltpu.roll(part, shift % 32, 0)
        rid = lax.broadcasted_iota(i32, (32, T), 0) + t0
        out = []
        for lo in (dst, dst + hw):
            piece = jnp.where((rid >= lo) & (rid < lo + hw), part, u32(0))
            piece = piece[0:min(32, TW - t0)]
            pieces = [jnp.zeros((t0, T), u32)] * (t0 > 0) + [piece] + [jnp.zeros((TW - t0 - 32, T), u32)] * (t0 + 32 < TW)
            out.append(jnp.concatenate(pieces, axis=0))
        return out

    def stage_a(unit, u, qt):
        s, k = unit
        s_ref, m_ref = bufs[k % 2]
        pi = k * NP + u
        g = pi // (HPG // 2)
        sg = s * NG + g
        n = T * (qt + 1)
        w_a, w_b = pair_weights(s, pi, qt)
        w_ab = _bf(jnp.where(lane64 < HT, w_a, w_b))

        def colmax8(v):
            return jnp.max(v.reshape(v.shape[0] // 8, 8, T), axis=0)

        maxes = []
        for hd, w in enumerate((_bf(w_a), _bf(w_b))):
            m8 = None
            for c in range(qt):
                kc = _bf(k_u[sg, c * TW:(c + 1) * TW, :])
                sc = jnp.dot(kc, w, preferred_element_type=f32)
                s_ref[u, qt, hd * L + c * T:hd * L + (c + 1) * T, :] = sc
                m8 = colmax8(sc) if m8 is None else jnp.maximum(m8, colmax8(sc))
            kc = _bf(k_u[sg, qt * TW:qt * TW + TW // 2, :])
            sc = jnp.dot(kc, w, preferred_element_type=f32) + mb[1 - hd]
            s_ref[u, qt, hd * L + qt * T:hd * L + qt * T + HT, :] = sc
            m8 = colmax8(sc) if m8 is None else jnp.maximum(m8, colmax8(sc))
            maxes.append(m8)
        kc = _bf(k_u[sg, qt * TW + TW // 2:(qt + 1) * TW, :])
        sc = jnp.dot(kc, w_ab, preferred_element_type=f32) + mb[2]
        s_ref[u, qt, n - HT:n, :] = sc
        mab = colmax8(sc)
        m_a = jnp.where(lane8 < HT, jnp.maximum(maxes[0], mab), maxes[0])
        m_b = jnp.where(lane8 >= HT, jnp.maximum(maxes[1], mab), maxes[1])
        m_ref[u, qt, 0] = jnp.broadcast_to(jnp.max(m_a, axis=0, keepdims=True), (8, T))
        m_ref[u, qt, 1] = jnp.broadcast_to(jnp.max(m_b, axis=0, keepdims=True), (8, T))

    def stage_b(unit, u, qt):
        s, k = unit
        s_ref, m_ref = bufs[k % 2]
        pi = k * NP + u
        n = T * (qt + 1)
        m_a = m_ref[u, qt, 0][0:1]
        m_b = m_ref[u, qt, 1][0:1]
        p_ab = jnp.exp2(s_ref[u, qt, n - HT:n, :] - jnp.where(lane1 < HT, m_a, m_b))
        for hd, m in enumerate((m_a, m_b)):
            h = 2 * pi + hd
            p = jnp.exp2(s_ref[u, qt, hd * L:hd * L + n - HT, :] - m)
            keep = (lane64 < HT) if hd == 0 else (lane64 >= HT)
            p = jnp.concatenate([p, jnp.where(keep, p_ab, 0.0)], axis=0).astype(bf16)
            w0 = (DH * h // 8) * 8
            off = DH * h - w0
            o = lax.dot_general(vwin[s * H + h, :, 0:n], p, NN_DIMS, preferred_element_type=f32)
            den = o[_ones_row(off):_ones_row(off) + 1]
            o = o * (omg[h][0:1] / den)
            if hd == 0:
                o = pltpu.roll(o, HT, 1)
            res = am[s, w0:w0 + VW, qt * T:(qt + 1) * T] + o
            rid = lax.broadcasted_iota(i32, (VW, T), 0)
            pltpu.store(ots[qt].at[w0:w0 + VW, :], res, mask=(rid >= off) & (rid < off + DH))

    def a_tasks(unit):
        return [lambda u=u, qt=qt: stage_a(unit, u, qt) for u in range(NP) for qt in QT_ORDER]

    def b_tasks(unit):
        return [lambda u=u, qt=qt: stage_b(unit, u, qt) for u in range(NP) for qt in QT_ORDER]

    w_copy(3).wait()
    rr = jnp.concatenate([r_buf[s][0:1, :] for s in range(NSEG)], axis=0)
    rr = _round_bf16(rr)
    tok = lax.broadcasted_iota(i32, (NSEG, L), 0) * L + lax.broadcasted_iota(i32, (NSEG, L), 1)
    m1v = jnp.max(rr)
    i1 = jnp.min(jnp.where(rr == m1v, tok, SEQ))
    rr2 = jnp.where(tok == i1, -jnp.inf, rr)
    m2v = jnp.max(rr2)
    i2 = jnp.min(jnp.where(rr2 == m2v, tok, SEQ))
    i1 = jnp.clip(i1, 0, SEQ - 1)
    i2 = jnp.clip(i2, 0, SEQ - 1)

    row8 = lax.broadcasted_iota(i32, (8, T), 0)
    lane8t = lax.broadcasted_iota(i32, (8, T), 1)

    def token_rows(i, slot):
        onehot = jnp.where((row8 == slot) & (lane8t == i % T), 1.0, 0.0)
        tile = xn_u[i // LNW, :, pl.ds(pl.multiple_of(((i // T) % BT) * T, T), T)]
        return lax.dot_general(onehot, _bf(tile), NT_DIMS, preferred_element_type=f32)

    def select_task():
        xsel_buf[...] = token_rows(i1, 0) + token_rows(i2, 1)
        y_acc[...] = jnp.zeros(y_acc.shape, f32)

    def expert_tile(w_ref, ft):
        return _bf(w_ref.at[ft].bitcast(u32)[...])

    def moe_up_task(ft, k, which):
        w_ref = (wg_buf, wu_buf)[which]
        hid_buf[k, which] = lax.dot_general(xsel_buf[:, 0:D], expert_tile(w_ref, ft), NN_DIMS,
                                            preferred_element_type=f32)

    def moe_down_task(ft, k):
        gt = _round_bf16(hid_buf[k, 0])
        up = _round_bf16(hid_buf[k, 1])
        hid = _round_bf16(gt * _sigmoid(gt)) * up
        y_acc[...] += lax.dot_general(hid, expert_tile(wd_buf, ft), NT_DIMS, preferred_element_type=f32)

    def moe_tasks(ft0, count):
        tasks = []
        for k0 in range(0, count, FPB):
            ks = range(k0, min(k0 + FPB, count))
            tasks += [lambda k=k, w=w: moe_up_task(ft0 + k, k, w) for k in ks for w in range(2)]
            tasks += [lambda k=k: moe_down_task(ft0 + k, k) for k in ks]
        return tasks

    def moe_finish():
        y = _round_bf16(y_acc[...])
        rsel = jnp.where(lax.broadcasted_iota(i32, (8, 1), 0) == 0, m1v, m2v)
        y = _round_bf16(y * _round_bf16(_sigmoid(rsel)))
        y = jnp.concatenate([y, jnp.zeros((8, DP - D), f32)], axis=1)
        y = jnp.concatenate([jnp.zeros((HT, DP), f32), y, jnp.zeros((T - HT - 8, DP), f32)], axis=0)
        y_t = jnp.concatenate([y.T[0:D], jnp.zeros((D, T), f32)], axis=1)
        y_u = _pack(y_t)[:, 0:T]
        lane = lax.broadcasted_iota(i32, (D // 2, T), 1)
        wot_u[:, DP - T:DP] = jnp.where(lane < HT, wot_u[:, DP - T:DP], y_u)
        rid = lax.broadcasted_iota(i32, (8, T), 0)
        for tt in range(TPS):
            tok_l = lax.broadcasted_iota(i32, (8, T), 1) + (NSEG - 1) * L + tt * T
            ots[tt][D:D + 8, :] = jnp.where(((rid == 0) & (tok_l == i1)) | ((rid == 1) & (tok_l == i2)), 1.0, 0.0)

    dense = _interleave(a_tasks((0, 0)), prep_dense(3, wot_u, 0))
    with _scope("p15_mix"):
        cut = (2 * len(dense)) // 3
        run(dense[:cut] + [select_task] + dense[cut:])

    for i in range(3):
        moe_wait(i)

    def out_tile(s, tt, chunk_copies=None):
        c0 = s * L + tt * T
        if not isinstance(s, int):
            c0 = pl.multiple_of(c0, T)
        o_bf = ots[tt][...].astype(bf16)
        nchunk = 4
        rows = D // nchunk
        for rc in range(nchunk):
            r0 = rc * rows
            attn = jnp.dot(_bf(wot_u[r0 // 2:(r0 + rows) // 2, :]), o_bf, preferred_element_type=f32)
            xn = _bf(xn_u[s * (L // LNW) + tt // BT, r0 // 2:(r0 + rows) // 2, (tt % BT) * T:(tt % BT + 1) * T]).astype(f32)
            x = x_rows(s * TPS + tt, r0, r0 + rows).astype(f32)
            res = x + attn + xn
            out_buf[r0:r0 + rows, pl.ds(c0, T)] = res.astype(bf16)
            if chunk_copies is not None:
                chunk_copies[rc].start()

    def pair_tasks(ua, ub):
        tasks = []
        for x, y in zip(a_tasks(ua), b_tasks(ub)):
            tasks += [x, y]
        return tasks

    def seg_end(s, last):
        def by_qt(fn, unit, qt):
            return [lambda u=u: fn(unit, u, qt) for u in range(NP)]

        steps = []
        for step in range(7):
            lists = []
            if step < 4:
                lists.append(by_qt(stage_b, (s, 2), 3 - step))
                lists.append(by_qt(stage_a, (s, 3), 3 - step))
            if 1 <= step < 5:
                lists.append(by_qt(stage_b, (s, 3), 4 - step))
            if not last and 2 <= step < 6:
                lists.append(by_qt(stage_a, (s + 1, 0), 5 - step))
            if step >= 3:
                lists.append([lambda tt=6 - step: out_tile(s, tt)])
            steps.append(_interleave(*lists))
        return steps

    def seg_att(s, c):
        tasks = pair_tasks((s, 1), (s, 0)) + pair_tasks((s, 2), (s, 1))
        steps = seg_end(s, False)
        for step in steps[0:5]:
            tasks += step
        with _scope("att_seg"):
            run(_interleave(tasks, moe_tasks(s * FPI, FPI)))
            for step in steps[5:]:
                run(step)

        @pl.when(s < NSEG - 2)
        def _():
            out_copy(pl.multiple_of(s * L, L), L, s).start()
        return c

    lax.fori_loop(0, NSEG - 1, seg_att, 0)

    npatch = (NSEG - 1) * TPS

    def patch_tile(idx):
        return jnp.where(idx < npatch * T, idx // T, 0)

    tile0 = patch_tile(i1)
    tile1 = patch_tile(i2)
    tile1 = jnp.where(tile1 == tile0, (tile0 + 1) % npatch, tile1)

    def patch(tile):
        c0 = pl.multiple_of(tile * T, T)
        rid = lax.broadcasted_iota(i32, (T, T), 0)
        tok_l = lax.broadcasted_iota(i32, (T, T), 1) + c0
        hit = ((rid == HT) & (tok_l == i1)) | ((rid == HT + 1) & (tok_l == i2))
        onehot = jnp.where(hit, 1.0, 0.0).astype(bf16)
        for rc in range(4):
            r0, r1 = rc * (D // 4), (rc + 1) * (D // 4)
            upd = jnp.dot(_bf(wot_u[r0 // 2:r1 // 2, DP - T:DP]), onehot, preferred_element_type=f32)
            cur = out_buf[r0:r1, pl.ds(c0, T)].astype(f32)
            out_buf[r0:r1, pl.ds(c0, T)] = (cur + upd).astype(bf16)

    sent = (NSEG - 2) * TPS
    resend0 = jnp.where(tile0 < sent, tile0, jnp.where(tile1 == 0, 1, 0))
    resend1 = jnp.where(tile1 < sent, tile1, jnp.where(resend0 == 0, 1, 0))
    patch_copies = [out_copy(pl.multiple_of(resend0 * T, T), T, 7), out_copy(pl.multiple_of(resend1 * T, T), T, 8),
                    out_copy((NSEG - 2) * L, L, NSEG - 2)]
    last_copies = [out_copy((NSEG - 1) * L + tt * T, T, NSEG - 1 + tt) for tt in range(1, TPS)]
    c_fin = (NSEG - 1) * L
    final_copies = [
        pltpu.make_async_copy(out_buf.at[rc * (D // 4):(rc + 1) * (D // 4), c_fin:c_fin + T],
                              out_hbm.at[rc * (D // 4):(rc + 1) * (D // 4), c_fin:c_fin + T],
                              sems.at[SEM_FINAL + rc]) for rc in range(4)]

    sl = NSEG - 1
    for s in range(NSEG - 2):
        out_copy(s * L, L, s).wait()
    with _scope("tail_2"):
        moe_finish()
        run(pair_tasks((sl, 1), (sl, 0)))
        patch(tile0)
        patch(tile1)
        run(pair_tasks((sl, 2), (sl, 1)))
        for cp in patch_copies:
            cp.start()
        steps = seg_end(sl, True)
        for step in steps[0:5]:
            run(step)
        last_copies[2].start()
        last_copies[1].start()
    with _scope("tail_3"):
        run(steps[5])
        last_copies[0].start()
        out_tile(sl, 0, final_copies)

    with _scope("out_wait"):
        for cp in patch_copies + last_copies + final_copies:
            cp.wait()


@jax.jit
def pallas_parallel_sum__memory_aug_infini_attn__moe_arch_mod__prompt_kernel(
    A_x: jax.Array,
    A_wq: jax.Array,
    A_wk: jax.Array,
    A_wv: jax.Array,
    A_wo: jax.Array,
    A_beta: jax.Array,
    B_x: jax.Array,
    B_w_r: jax.Array,
    B_w_gate: jax.Array,
    B_w_up: jax.Array,
    B_w_down: jax.Array,
):
    del B_x
    any_spec = pl.BlockSpec(memory_space=pl.ANY)
    scratch = [
        pltpu.VMEM((H,), bf16),
        pltpu.VMEM((D,), bf16),
        pltpu.VMEM((NT, D, T), bf16),
        pltpu.VMEM((4, D, D), bf16),
        pltpu.VMEM((NFT, D, T), bf16),
        pltpu.VMEM((NFT, D, T), bf16),
        pltpu.VMEM((NFT, D, T), bf16),
        pltpu.VMEM((D, SEQ), bf16),
        pltpu.VMEM((WT_ALLOC, DP), u32),
        pltpu.VMEM((2, D // 2, LNW), u32),
        pltpu.VMEM((D // 2, DP), u32),
        pltpu.VMEM((SEQ // LNW, DP // 2, LNW), u32),
        pltpu.VMEM((DP // 2, LNW), u32),
        pltpu.VMEM((DP // 2, LNW), u32),
        pltpu.VMEM((NSEG, D // 2, L), u32),
        pltpu.VMEM((NSEG * NG, L // 2, T), u32),
        pltpu.VMEM((NSEG, D // 2, L), u32),
        pltpu.VMEM((NSEG, D // 2, L), u32),
        pltpu.VMEM((NSEG, D // 2, L), u32),
        pltpu.VMEM((NSEG * H, VW, L), f32),
        pltpu.VMEM((NSEG, 8, L), f32),
        pltpu.VMEM((NG, T, T), f32),
        pltpu.VMEM((NG, T, T), f32),
        pltpu.VMEM((NG, T, T), i32),
        pltpu.VMEM((NSEG, D, L), f32),
        pltpu.VMEM((NG, 8, T), f32),
        pltpu.VMEM((H, 8, T), f32),
        pltpu.VMEM((3, HT, T), f32),
        pltpu.VMEM((NP, 4, 2 * L, T), f32),
        pltpu.VMEM((NP, 4, 2, 8, T), f32),
        pltpu.VMEM((NP, 4, 2 * L, T), f32),
        pltpu.VMEM((NP, 4, 2, 8, T), f32),
        pltpu.VMEM((DP, T), f32),
        pltpu.VMEM((DP, T), f32),
        pltpu.VMEM((DP, T), f32),
        pltpu.VMEM((DP, T), f32),
        pltpu.VMEM((2, D, LNW), f32),
        pltpu.VMEM((2, 2, 8, LNW), f32),
        pltpu.VMEM((8, D), f32),
        pltpu.VMEM((8, DP), f32),
        pltpu.VMEM((FPI, 2, 8, T), f32),
        pltpu.SemaphoreType.DMA((NSEM,)),
    ]
    x_t = jnp.transpose(A_x, (0, 2, 1)).reshape(D, SEQ)
    out_t = pl.pallas_call(
        _kernel,
        out_shape=jax.ShapeDtypeStruct((D, SEQ), bf16),
        in_specs=[any_spec] * 10,
        out_specs=any_spec,
        scratch_shapes=scratch,
        compiler_params=pltpu.CompilerParams(vmem_limit_bytes=110 * 1024 * 1024),
    )(x_t, A_wq, A_wk, A_wv, A_wo, A_beta, B_w_r, B_w_gate, B_w_up, B_w_down.T)
    return jnp.transpose(out_t.reshape(1, D, SEQ), (0, 2, 1))
```

```python
import contextlib

import jax
import jax.numpy as jnp
from jax import lax
from jax.experimental import pallas as pl
from jax.experimental.pallas import tpu as pltpu

bf16 = jnp.bfloat16
f32 = jnp.float32
u32 = jnp.uint32
i32 = jnp.int32

SEQ = 2048
D = 576
DP = 640
H = 32
DH = 18
NSEG = 4
L = 512
T = 128
TW = T // 2
HT = T // 2
TPS = L // T
HPG = 6
NG = 6
F = 4608
FPI = 12
FPB = 3
NFT = F // T
NP = 4
UPS = H // (2 * NP)
NT = SEQ // T
LNW = 256
BT = LNW // T
NORM_PARTS = 6
QK_BLOCK = 64
VB = 8 * DH

LOG2E = 1.4426950408889634
QSCALE = (DH ** -0.5) * LOG2E
MASKVAL = -1000000000.0 * LOG2E
EPS_BF16 = 1.0013580322265625e-05
ONES_PAIR = 0x3F803F80

NT_DIMS = (((1,), (1,)), ((), ()))
NN_DIMS = (((1,), (0,)), ((), ()))
VW = 24

WT_Q = 0
WT_K = D // 2
WT_R = D
WT_V = D + 8
WT_ALLOC = 1056
NBLK = DP // T

X_PIECES = ((0, LNW), (LNW, LNW), (L, L), (2 * L, L), (3 * L, L))
SEM_X = 0
SEM_W = 5
SEM_MOE = 9
SEM_OUT = 12
SEM_SMALL = 21
SEM_WQB = 23
SEM_FINAL = 24
NSEM = 28
WQ_SPLIT = 2 * T


PROFILE_SCOPES = False
QT_ORDER = (3, 2, 1, 0)


def _scope(name):
    return jax.named_scope(name) if PROFILE_SCOPES else contextlib.nullcontext()


def _valid(g):
    return min(HPG * DH, D - g * HPG * DH)


def _ewin(g):
    start = (g * HPG * DH // 16) * 16
    return start, g * HPG * DH - start, min(T, D - start)


def _ones_row(off):
    return VW - 1 if off + DH < VW else 0


def _bf(x):
    return pltpu.bitcast(x, bf16)


def _pack(x):
    return pltpu.bitcast(x.astype(bf16), u32)


def _round_bf16(x):
    return x.astype(bf16).astype(f32)


def _phi(t):
    return jnp.where(t > 0, t + 1.0, jnp.exp(t))


def _sigmoid(t):
    return 1.0 / (1.0 + jnp.exp(-t))


def _zero_after(v):
    bits = pltpu.bitcast(v[0:8, 0:LNW], u32)
    sixteen = jnp.uint32(16)
    bits = lax.shift_right_logical(lax.shift_right_logical(bits, sixteen), sixteen)
    return pltpu.bitcast(bits, f32)


def _interleave(*lists):
    items = []
    for li, tasks in enumerate(lists):
        for k, t in enumerate(tasks):
            items.append(((k + 0.5) / len(tasks), li, k, t))
    items.sort(key=lambda it: it[:3])
    return [it[3] for it in items]


def _kernel(x_hbm, wq_hbm, wk_hbm, wv_hbm, wo_hbm, beta_hbm, wr_hbm, wg_hbm, wu_hbm, wd_hbm,
            out_hbm,
            beta_ref, wr_ref, x_buf, w_buf, wg_buf, wu_buf, wd_buf, out_buf,
            wt_u, kt_tmp, wot_u, xn_u, xs_a, xs_b, qs_u, k_u, pq_u, pk_u, vt_u, vwin,
            r_buf, mt_acc, lm_f, mcode, am, g16, omg, mb,
            s0, m0, s1, m1, ot0, ot1, ot2, ot3, xf, ln_stat, y_acc, xsel_buf, hid_buf, sems):

    class XCopy:
        def __init__(self, i):
            c0, width = X_PIECES[i]
            self.copies = [pltpu.make_async_copy(x_hbm.at[:, c:c + T], x_buf.at[c // T], sems.at[SEM_X + i])
                           for c in range(c0, c0 + width, T)]

        def start(self):
            for cp in self.copies:
                cp.start()

        def wait(self):
            for cp in self.copies:
                cp.wait()

    x_copy = XCopy

    def x_rows(tile, r0, r1):
        return _bf(x_buf.at[tile].bitcast(u32)[r0 // 2:r1 // 2, :])

    def w_copy(i):
        src = (wq_hbm, wk_hbm, wv_hbm, wo_hbm)[i]
        return pltpu.make_async_copy(src, w_buf.at[i], sems.at[SEM_W + i])

    wq_first = pltpu.make_async_copy(wq_hbm.at[:, 0:WQ_SPLIT], w_buf.at[0, :, 0:WQ_SPLIT], sems.at[SEM_W])
    wq_rest = pltpu.make_async_copy(wq_hbm.at[:, WQ_SPLIT:D], w_buf.at[0, :, WQ_SPLIT:D], sems.at[SEM_WQB])

    moe_src = (wg_hbm, wu_hbm, wd_hbm)
    moe_dst = (wg_buf, wu_buf, wd_buf)

    def moe_start(i, ft):
        c0 = ft * T if isinstance(ft, int) else pl.multiple_of(ft * T, T)
        pltpu.make_async_copy(moe_src[i].at[:, pl.ds(c0, T)], moe_dst[i].at[ft], sems.at[SEM_MOE + i]).start()

    def moe_issue(first, last):
        for n in range(first, last):
            moe_start(n % 3, n // 3)

    def moe_wait(i):
        pltpu.make_async_copy(moe_dst[i], moe_dst[i], sems.at[SEM_MOE + i]).wait()

    def out_copy(c0, width, sem):
        return pltpu.make_async_copy(out_buf.at[:, pl.ds(c0, width)], out_hbm.at[:, pl.ds(c0, width)],
                                     sems.at[SEM_OUT + sem])

    small_copies = [pltpu.make_async_copy(beta_hbm, beta_ref, sems.at[SEM_SMALL]),
                    pltpu.make_async_copy(wr_hbm, wr_ref, sems.at[SEM_SMALL + 1])]
    x_copy(0).start()
    wq_first.start()
    wq_rest.start()
    x_copy(1).start()
    for cp in small_copies:
        cp.start()
    w_copy(1).start()
    w_copy(2).start()

    init_scope = _scope("init")
    init_scope.__enter__()
    kr = lax.broadcasted_iota(i32, (HT, T), 0)
    ql = lax.broadcasted_iota(i32, (HT, T), 1)
    mb[0] = jnp.where(ql < kr, MASKVAL, 0.0).astype(f32)
    mb[1] = jnp.where((ql >= HT) & (ql - HT < kr), MASKVAL, 0.0).astype(f32)
    mb[2] = jnp.where(ql % HT < kr, MASKVAL, 0.0).astype(f32)
    zpad = jnp.zeros(((DP - D) // 2, LNW), u32)
    for blk in range(SEQ // LNW):
        xn_u[blk, D // 2:DP // 2, :] = zpad
    xs_a[D // 2:DP // 2, :] = zpad
    xs_b[D // 2:DP // 2, :] = zpad
    ots = (ot0, ot1, ot2, ot3)
    for o_ref in ots:
        o_ref[D:DP, :] = jnp.zeros((DP - D, T), f32)
    am[0] = jnp.zeros(am.shape[1:], f32)
    mt_acc[...] = jnp.zeros(mt_acc.shape, f32)
    g16[...] = jnp.zeros(g16.shape, f32)

    init_scope.__exit__(None, None, None)

    pace = [None]

    def gate_tables():
        gate = _round_bf16(_sigmoid(beta_ref[...].reshape(1, H).astype(f32)))
        for h in range(H):
            gh = jnp.broadcast_to(gate[:, h:h + 1], (1, T))
            omg[h] = jnp.broadcast_to(_round_bf16(1.0 - gh), (8, T))
            g16[h // HPG, (h % HPG):(h % HPG) + 1, :] = gh

    def transpose_block(i, cb):
        c1 = min((cb + 1) * T, D)
        blk = w_buf[i, :, cb * T:c1]
        if c1 - cb * T < T:
            blk = jnp.concatenate([blk, jnp.zeros((D, T - (c1 - cb * T)), bf16)], axis=1)
        blk = jnp.concatenate([blk, jnp.zeros((DP - D, T), bf16)], axis=0)
        return pltpu.bitcast(blk.T, u32)

    def prep_dense(i, dst, base):
        def task(cb):
            nrow = min(TW, D // 2 - cb * TW)
            dst[base + cb * TW:base + cb * TW + nrow, :] = transpose_block(i, cb)[0:nrow]
        return [lambda cb=cb: task(cb) for cb in range(DP // T)]

    def router_row():
        wr = wr_ref[...].reshape(1, D).astype(f32)
        wr = jnp.concatenate([wr, jnp.zeros((1, DP - D), f32)], axis=1)
        bits = lax.shift_right_logical(pltpu.bitcast(wr, u32), u32(16))
        rid = lax.broadcasted_iota(i32, (8, DP), 0)
        wt_u[WT_R:WT_R + 8, :] = jnp.where(rid == 0, bits, u32(0))

    def ln_tasks(s, p, stage):
        tile0 = s * TPS + p * BT

        def mean_pass():
            acc = pace[0]
            for r in range(0, D, 64):
                x = jnp.concatenate([pltpu.bitcast(x_rows(tile0 + t, r, r + 64), u32) for t in range(BT)], axis=1)
                x = _bf(x).astype(f32)
                xf[p, r:r + 64, :] = x
                part = jnp.sum(x.reshape(8, 8, LNW), axis=0)
                acc = part if acc is None else acc + part
            mean = jnp.sum(acc, axis=0, keepdims=True) / D
            ln_stat[p, 0] = jnp.broadcast_to(mean, (8, LNW))

        def var_pass():
            mean = ln_stat[p, 0][0:1]
            if pace[0] is not None:
                mean = mean + pace[0][0:1]
            acc = None
            for r in range(0, D, 96):
                xc = xf[p, r:r + 96, :] - mean
                part = jnp.sum((xc * xc).reshape(12, 8, LNW), axis=0)
                acc = part if acc is None else acc + part
            var = jnp.sum(acc, axis=0, keepdims=True) / D
            den = _round_bf16(jnp.sqrt(_round_bf16(_round_bf16(var) + EPS_BF16)))
            ln_stat[p, 1] = jnp.broadcast_to(1.0 / den, (8, LNW))
            ln_stat[p, 0] = jnp.broadcast_to(_round_bf16(mean), (8, LNW))

        def norm_pass(part):
            mean_b = ln_stat[p, 0][0:1]
            if pace[0] is not None:
                mean_b = mean_b + pace[0][0:1]
            inv = ln_stat[p, 1][0:1]
            step = D // NORM_PARTS
            for r in range(part * step, (part + 1) * step, 48):
                xn = _pack(_round_bf16(xf[p, r:r + 48, :] - mean_b) * inv)
                xn_u.at[s * (L // LNW) + p][r // 2:r // 2 + 24, :] = xn
                if stage is not None:
                    stage[r // 2:r // 2 + 24, :] = xn

        return [mean_pass, var_pass] + [lambda part=part: norm_pass(part) for part in range(NORM_PARTS)]

    def load_xs(s, p, stage):
        return _bf(xn_u[s * (L // LNW) + p] if stage is None else stage[...])

    def row_blocks(size):
        return [(r, min(r + size, D)) for r in range(0, D, size)]

    def q_task(s, p, stage, r0, r1):
        rows = slice(r0 // 2, r1 // 2)
        cols = slice(p * LNW, (p + 1) * LNW)
        w = _bf(wt_u[WT_Q + r0 // 2:WT_Q + r1 // 2, :])
        q = jnp.dot(w, load_xs(s, p, stage), preferred_element_type=f32)
        pace[0] = _zero_after(q)
        qs = q * QSCALE
        qrot = jnp.concatenate([pltpu.roll(qs[:, t * T:(t + 1) * T], HT, 1) for t in range(BT)], axis=1)
        rid = lax.broadcasted_iota(i32, qs.shape, 0) + r0
        even = ((rid // DH) % 2) == 0
        qs_u.at[s][rows, cols] = _pack(jnp.where(even, qrot, qs))
        pq_u.at[s][rows, cols] = _pack(_phi(q))

    def k_task(s, p, stage, r0, r1):
        rows = slice(r0 // 2, r1 // 2)
        cols = slice(p * LNW, (p + 1) * LNW)
        extra = 8 if r1 == D else 0
        w = _bf(wt_u[WT_K + r0 // 2:WT_K + r1 // 2 + extra, :])
        k = jnp.dot(w, load_xs(s, p, stage), preferred_element_type=f32)
        pace[0] = _zero_after(k)
        if extra:
            r_buf[s, :, cols] = jnp.broadcast_to(k[r1 - r0:r1 - r0 + 1, :], (8, LNW))
            k = k[0:r1 - r0]
        kt_tmp.at[p][rows, :] = _pack(k)
        pk_u.at[s][rows, cols] = _pack(_phi(k))

    def kt_task(s, p, g):
        nv = _valid(g) // 2
        src = g * HPG * DH // 2
        kg = jnp.concatenate([kt_tmp[p, src:src + nv, :], jnp.zeros((TW - nv, LNW), u32)], axis=0)
        k_u.at[s * NG + g][p * (LNW // 2):(p + 1) * (LNW // 2), :] = pltpu.bitcast(_bf(kg).T, u32)

    def v_task(s, p, stage, b):
        cols = slice(p * LNW, (p + 1) * LNW)
        w = _bf(wt_u[WT_V + b * (VB // 2):WT_V + (b + 1) * (VB // 2), :])
        v = jnp.dot(w, load_xs(s, p, stage), preferred_element_type=f32)
        pace[0] = _zero_after(v)
        vt_u.at[s][b * (VB // 2):(b + 1) * (VB // 2), cols] = _pack(v)
        sub = lax.broadcasted_iota(i32, (VW, LNW), 0)
        for hh in range(8):
            r0 = (DH * hh // 8) * 8
            ones_row = _ones_row(DH * hh - r0)
            vwin.at[s * H + 8 * b + hh][:, cols] = jnp.where(sub == ones_row, 1.0, v[r0:r0 + VW, :])

    def q_tasks(s, p, stage=None, size=QK_BLOCK):
        return [lambda b=b: q_task(s, p, stage, *b) for b in row_blocks(size)]

    def k_tasks(s, p, stage=None, size=QK_BLOCK):
        tasks, done = [], 0
        for b in row_blocks(size):
            tasks.append(lambda b=b: k_task(s, p, stage, *b))
            while done < NG and done * HPG * DH + _valid(done) <= b[1]:
                tasks.append(lambda g=done: kt_task(s, p, g))
                done += 1
        return tasks

    def v_tasks(s, p, stage=None):
        return [lambda b=b: v_task(s, p, stage, b) for b in range(D // VB)]

    def mem_layout(g):
        es, eoff, _ = _ewin(g)
        nv = _valid(g)
        ne = -(-(eoff + nv) // 16) * 16
        ones_row = 0 if eoff >= 2 else eoff + nv
        nh = nv // DH
        ne8 = -(-(eoff + nv) // 8) * 8
        den_row = 0 if eoff >= nh else ne8
        return es, eoff, nv, ne, ones_row, den_row, ne8 + 8 * (den_row > 0)

    def mem_update(sp, g):
        es, eoff, nv, ne, ones_row, den_row, nr = mem_layout(g)
        nw = min(T, D - es)
        win = vt_u[sp, es // 2:(es + ne) // 2, :]
        wid = lax.broadcasted_iota(i32, win.shape, 0)
        lhs = _bf(jnp.where(wid == ones_row // 2, u32(ONES_PAIR), win))
        upd = lax.dot_general(lhs, _bf(pk_u[sp, es // 2:(es + nw) // 2, :]), NT_DIMS, preferred_element_type=f32)
        mt = mt_acc[g, 0:ne, 0:nw] + upd
        mt_acc[g, 0:ne, 0:nw] = mt
        z = jnp.broadcast_to(mt[ones_row:ones_row + 1, :], (nr, nw))
        if nr > ne:
            mt = jnp.concatenate([mt, jnp.zeros((nr - ne, nw), f32)], axis=0)
        mt = mt[0:nr]
        code = mcode[g, 0:nr, 0:nw]
        lm_f[g, 0:nr, 0:nw] = jnp.where(code == 1, mt, jnp.where(code == 2, z, 0.0))

    def mem_masks():
        for g in range(NG):
            es, eoff, nv, ne, ones_row, den_row, nr = mem_layout(g)
            row = lax.broadcasted_iota(i32, (T, T), 0)
            d_loc = lax.broadcasted_iota(i32, (T, T), 1) - eoff
            e_loc = row - eoff
            d_ok = (d_loc >= 0) & (d_loc < nv)
            same_head = (e_loc >= 0) & (e_loc < nv) & d_ok & ((e_loc // DH) == (d_loc // DH))
            den_hit = (row >= den_row) & d_ok & ((d_loc // DH) == row - den_row)
            mcode[g] = jnp.where(same_head, 1, jnp.where(den_hit, 2, 0))

    def mem_retrieve(s, g):
        es, eoff, nv, ne, ones_row, den_row, nr = mem_layout(g)
        nw = min(T, D - es)
        nd = lax.dot_general(lm_f[g, 0:nr, 0:nw], _bf(pq_u[s, es // 2:(es + nw) // 2, :]), NN_DIMS,
                             preferred_element_type=f32)
        scale = jnp.broadcast_to(g16[g][:, 0:1], (8, L)) / (nd[den_row:den_row + 8, :] + 1e-6)
        r8 = lax.broadcasted_iota(i32, (8, L), 0)
        for b in range(nr // 8):
            lo, hi = 8 * b - eoff, 8 * b + 7 - eoff
            if hi < 0 or lo >= nv:
                continue
            j1, j2 = max(lo, 0) // DH, min(hi, nv - 1) // DH
            sc = jnp.broadcast_to(scale[j1:j1 + 1, :], (8, L))
            if j2 != j1:
                sc = jnp.where(r8 < DH * j2 - lo, sc, jnp.broadcast_to(scale[j2:j2 + 1, :], (8, L)))
            val = nd[8 * b:8 * b + 8, :] * sc
            dst = am.at[s, es + 8 * b:es + 8 * b + 8, :]
            if lo >= 0 and hi < nv:
                dst[...] = val
            else:
                pltpu.store(dst, val, mask=(r8 + lo >= 0) & (r8 + lo < nv))

    def run(tasks):
        for t in tasks:
            t()

    prep_q = prep_dense(0, wt_u, WT_Q)
    q0a = q_tasks(0, 0, None, T)
    mem_masks()
    with _scope("p1_wait_x0"):
        x_copy(0).wait()
    with _scope("p1_ln0a"):
        run(ln_tasks(0, 0, None))
        wq_first.wait()
    with _scope("p1_q0a_first"):
        run(prep_q[0:2] + q0a[0:2])
        wq_rest.wait()
        x_copy(1).wait()
    for i in range(2, len(X_PIECES)):
        x_copy(i).start()
    w_copy(3).start()
    moe_issue(0, 40)
    with _scope("p1_q0a"):
        run(prep_q[2:])
        run(_interleave(q0a[2:], ln_tasks(0, 1, None)))
        w_copy(1).wait()
        for cp in small_copies:
            cp.wait()
    k0b = k_tasks(0, 1)
    with _scope("p1_q0b"):
        run(_interleave(q_tasks(0, 1), prep_dense(1, wt_u, WT_K), [router_row, gate_tables]))
        run([lambda b=b: k_task(0, 0, None, *b) for b in row_blocks(QK_BLOCK)])
        w_copy(2).wait()
        x_copy(2).wait()
    moe_issue(40, 60)
    with _scope("p1_k0v0"):
        run(_interleave(k0b, prep_dense(2, wt_u, WT_V), [lambda g=g: kt_task(0, 0, g) for g in range(NG)]))
        run(_interleave(v_tasks(0, 0) + v_tasks(0, 1), ln_tasks(1, 0, xs_a)))

    moe_issue(60, 72)

    def seg_body(s, c):
        for ss in range(2, NSEG):
            @pl.when(s + 1 == ss)
            def _():
                x_copy(ss + 1).wait()
                if ss == NSEG - 1:
                    moe_issue(72, 3 * NFT)
        nxt = jnp.minimum(s + 1, NSEG - 1)
        pace[0] = None
        with _scope("p1_seg"):
            updates = [lambda g=g: mem_update(s - 1, g) for g in range(NG)]
            retrieves = [lambda g=g: mem_retrieve(s, g) for g in range(NG)]
            first = _interleave(q_tasks(s, 0, xs_a), updates) + k_tasks(s, 0, xs_a) + v_tasks(s, 0, xs_a)
            run(_interleave(first, ln_tasks(s, 1, xs_b)))
            second = q_tasks(s, 1, xs_b) + _interleave(k_tasks(s, 1, xs_b) + v_tasks(s, 1, xs_b), retrieves)
            run(_interleave(second, ln_tasks(nxt, 0, xs_a)))
        return c

    lax.fori_loop(1, NSEG, seg_body, 0)

    bufs = ((s0, m0), (s1, m1))
    lane64 = lax.broadcasted_iota(i32, (TW, T), 1)
    lane1 = lax.broadcasted_iota(i32, (1, T), 1)
    lane8 = lax.broadcasted_iota(i32, (8, T), 1)

    def pair_weights(s, pi, qt):
        hw = DH // 2
        j = 2 * (pi % (HPG // 2))
        src, dst = hw * 2 * pi, hw * j
        a0, t0 = (src // 8) * 8, (dst // 8) * 8
        nrow = min(32, D // 2 - a0)
        part = qs_u[s, a0:a0 + nrow, qt * T:(qt + 1) * T]
        if nrow < 32:
            part = jnp.concatenate([part, jnp.zeros((32 - nrow, T), u32)], axis=0)
        shift = (dst - t0) - (src - a0)
        if shift:
            part = pltpu.roll(part, shift % 32, 0)
        rid = lax.broadcasted_iota(i32, (32, T), 0) + t0
        out = []
        for lo in (dst, dst + hw):
            piece = jnp.where((rid >= lo) & (rid < lo + hw), part, u32(0))
            piece = piece[0:min(32, TW - t0)]
            pieces = [jnp.zeros((t0, T), u32)] * (t0 > 0) + [piece] + [jnp.zeros((TW - t0 - 32, T), u32)] * (t0 + 32 < TW)
            out.append(jnp.concatenate(pieces, axis=0))
        return out

    def stage_a(unit, u, qt):
        s, k = unit
        s_ref, m_ref = bufs[k % 2]
        pi = k * NP + u
        g = pi // (HPG // 2)
        sg = s * NG + g
        n = T * (qt + 1)
        w_a, w_b = pair_weights(s, pi, qt)
        w_ab = _bf(jnp.where(lane64 < HT, w_a, w_b))

        def colmax8(v):
            return jnp.max(v.reshape(v.shape[0] // 8, 8, T), axis=0)

        maxes = []
        for hd, w in enumerate((_bf(w_a), _bf(w_b))):
            m8 = None
            for c in range(qt):
                kc = _bf(k_u[sg, c * TW:(c + 1) * TW, :])
                sc = jnp.dot(kc, w, preferred_element_type=f32)
                s_ref[u, qt, hd * L + c * T:hd * L + (c + 1) * T, :] = sc
                m8 = colmax8(sc) if m8 is None else jnp.maximum(m8, colmax8(sc))
            kc = _bf(k_u[sg, qt * TW:qt * TW + TW // 2, :])
            sc = jnp.dot(kc, w, preferred_element_type=f32) + mb[1 - hd]
            s_ref[u, qt, hd * L + qt * T:hd * L + qt * T + HT, :] = sc
            m8 = colmax8(sc) if m8 is None else jnp.maximum(m8, colmax8(sc))
            maxes.append(m8)
        kc = _bf(k_u[sg, qt * TW + TW // 2:(qt + 1) * TW, :])
        sc = jnp.dot(kc, w_ab, preferred_element_type=f32) + mb[2]
        s_ref[u, qt, n - HT:n, :] = sc
        mab = colmax8(sc)
        m_a = jnp.where(lane8 < HT, jnp.maximum(maxes[0], mab), maxes[0])
        m_b = jnp.where(lane8 >= HT, jnp.maximum(maxes[1], mab), maxes[1])
        m_ref[u, qt, 0] = jnp.broadcast_to(jnp.max(m_a, axis=0, keepdims=True), (8, T))
        m_ref[u, qt, 1] = jnp.broadcast_to(jnp.max(m_b, axis=0, keepdims=True), (8, T))

    def stage_b(unit, u, qt):
        s, k = unit
        s_ref, m_ref = bufs[k % 2]
        pi = k * NP + u
        n = T * (qt + 1)
        m_a = m_ref[u, qt, 0][0:1]
        m_b = m_ref[u, qt, 1][0:1]
        p_ab = jnp.exp2(s_ref[u, qt, n - HT:n, :] - jnp.where(lane1 < HT, m_a, m_b))
        for hd, m in enumerate((m_a, m_b)):
            h = 2 * pi + hd
            p = jnp.exp2(s_ref[u, qt, hd * L:hd * L + n - HT, :] - m)
            keep = (lane64 < HT) if hd == 0 else (lane64 >= HT)
            p = jnp.concatenate([p, jnp.where(keep, p_ab, 0.0)], axis=0).astype(bf16)
            w0 = (DH * h // 8) * 8
            off = DH * h - w0
            o = lax.dot_general(vwin[s * H + h, :, 0:n], p, NN_DIMS, preferred_element_type=f32)
            den = o[_ones_row(off):_ones_row(off) + 1]
            o = o * (omg[h][0:1] / den)
            if hd == 0:
                o = pltpu.roll(o, HT, 1)
            res = am[s, w0:w0 + VW, qt * T:(qt + 1) * T] + o
            rid = lax.broadcasted_iota(i32, (VW, T), 0)
            pltpu.store(ots[qt].at[w0:w0 + VW, :], res, mask=(rid >= off) & (rid < off + DH))

    def a_tasks(unit):
        return [lambda u=u, qt=qt: stage_a(unit, u, qt) for u in range(NP) for qt in QT_ORDER]

    def b_tasks(unit):
        return [lambda u=u, qt=qt: stage_b(unit, u, qt) for u in range(NP) for qt in QT_ORDER]

    w_copy(3).wait()
    rr = jnp.concatenate([r_buf[s][0:1, :] for s in range(NSEG)], axis=0)
    rr = _round_bf16(rr)
    tok = lax.broadcasted_iota(i32, (NSEG, L), 0) * L + lax.broadcasted_iota(i32, (NSEG, L), 1)
    m1v = jnp.max(rr)
    i1 = jnp.min(jnp.where(rr == m1v, tok, SEQ))
    rr2 = jnp.where(tok == i1, -jnp.inf, rr)
    m2v = jnp.max(rr2)
    i2 = jnp.min(jnp.where(rr2 == m2v, tok, SEQ))
    i1 = jnp.clip(i1, 0, SEQ - 1)
    i2 = jnp.clip(i2, 0, SEQ - 1)

    row8 = lax.broadcasted_iota(i32, (8, T), 0)
    lane8t = lax.broadcasted_iota(i32, (8, T), 1)

    def token_rows(i, slot):
        onehot = jnp.where((row8 == slot) & (lane8t == i % T), 1.0, 0.0)
        tile = xn_u[i // LNW, :, pl.ds(pl.multiple_of(((i // T) % BT) * T, T), T)]
        return lax.dot_general(onehot, _bf(tile), NT_DIMS, preferred_element_type=f32)

    def select_task():
        xsel_buf[...] = token_rows(i1, 0) + token_rows(i2, 1)
        y_acc[...] = jnp.zeros(y_acc.shape, f32)

    def expert_tile(w_ref, ft):
        return _bf(w_ref.at[ft].bitcast(u32)[...])

    def moe_up_task(ft, k, which):
        w_ref = (wg_buf, wu_buf)[which]
        hid_buf[k, which] = lax.dot_general(xsel_buf[:, 0:D], expert_tile(w_ref, ft), NN_DIMS,
                                            preferred_element_type=f32)

    def moe_down_task(ft, k):
        gt = _round_bf16(hid_buf[k, 0])
        up = _round_bf16(hid_buf[k, 1])
        hid = _round_bf16(gt * _sigmoid(gt)) * up
        y_acc[...] += lax.dot_general(hid, expert_tile(wd_buf, ft), NT_DIMS, preferred_element_type=f32)

    def moe_tasks(ft0, count):
        tasks = []
        for k0 in range(0, count, FPB):
            ks = range(k0, min(k0 + FPB, count))
            tasks += [lambda k=k, w=w: moe_up_task(ft0 + k, k, w) for k in ks for w in range(2)]
            tasks += [lambda k=k: moe_down_task(ft0 + k, k) for k in ks]
        return tasks

    def moe_finish():
        y = _round_bf16(y_acc[...])
        rsel = jnp.where(lax.broadcasted_iota(i32, (8, 1), 0) == 0, m1v, m2v)
        y = _round_bf16(y * _round_bf16(_sigmoid(rsel)))
        y = jnp.concatenate([y, jnp.zeros((8, DP - D), f32)], axis=1)
        y = jnp.concatenate([jnp.zeros((HT, DP), f32), y, jnp.zeros((T - HT - 8, DP), f32)], axis=0)
        y_t = jnp.concatenate([y.T[0:D], jnp.zeros((D, T), f32)], axis=1)
        y_u = _pack(y_t)[:, 0:T]
        lane = lax.broadcasted_iota(i32, (D // 2, T), 1)
        wot_u[:, DP - T:DP] = jnp.where(lane < HT, wot_u[:, DP - T:DP], y_u)
        rid = lax.broadcasted_iota(i32, (8, T), 0)
        for tt in range(TPS):
            tok_l = lax.broadcasted_iota(i32, (8, T), 1) + (NSEG - 1) * L + tt * T
            ots[tt][D:D + 8, :] = jnp.where(((rid == 0) & (tok_l == i1)) | ((rid == 1) & (tok_l == i2)), 1.0, 0.0)

    dense = _interleave(a_tasks((0, 0)), prep_dense(3, wot_u, 0))
    with _scope("p15_mix"):
        cut = (2 * len(dense)) // 3
        run(dense[:cut] + [select_task] + dense[cut:])

    for i in range(3):
        moe_wait(i)

    def out_tile(s, tt, chunk_copies=None):
        c0 = s * L + tt * T
        if not isinstance(s, int):
            c0 = pl.multiple_of(c0, T)
        o_bf = ots[tt][...].astype(bf16)
        nchunk = 4
        rows = D // nchunk
        for rc in range(nchunk):
            r0 = rc * rows
            attn = jnp.dot(_bf(wot_u[r0 // 2:(r0 + rows) // 2, :]), o_bf, preferred_element_type=f32)
            xn = _bf(xn_u[s * (L // LNW) + tt // BT, r0 // 2:(r0 + rows) // 2, (tt % BT) * T:(tt % BT + 1) * T]).astype(f32)
            x = x_rows(s * TPS + tt, r0, r0 + rows).astype(f32)
            res = x + attn + xn
            out_buf[r0:r0 + rows, pl.ds(c0, T)] = res.astype(bf16)
            if chunk_copies is not None:
                chunk_copies[rc].start()

    def pair_tasks(ua, ub):
        tasks = []
        for x, y in zip(a_tasks(ua), b_tasks(ub)):
            tasks += [x, y]
        return tasks

    def seg_end(s, last):
        def by_qt(fn, unit, qt):
            return [lambda u=u: fn(unit, u, qt) for u in range(NP)]

        steps = []
        for step in range(7):
            lists = []
            if step < 4:
                lists.append(by_qt(stage_b, (s, 2), 3 - step))
                lists.append(by_qt(stage_a, (s, 3), 3 - step))
            if 1 <= step < 5:
                lists.append(by_qt(stage_b, (s, 3), 4 - step))
            if not last and 2 <= step < 6:
                lists.append(by_qt(stage_a, (s + 1, 0), 5 - step))
            if step >= 3:
                lists.append([lambda tt=6 - step: out_tile(s, tt)])
            steps.append(_interleave(*lists))
        return steps

    def seg_att(s, c):
        tasks = pair_tasks((s, 1), (s, 0)) + pair_tasks((s, 2), (s, 1))
        steps = seg_end(s, False)
        for step in steps[0:5]:
            tasks += step
        with _scope("att_seg"):
            for step in steps[5:]:
                tasks += step
            run(_interleave(tasks, moe_tasks(s * FPI, FPI)))

        @pl.when(s < NSEG - 2)
        def _():
            out_copy(pl.multiple_of(s * L, L), L, s).start()
        return c

    lax.fori_loop(0, NSEG - 1, seg_att, 0)

    npatch = (NSEG - 1) * TPS

    def patch_tile(idx):
        return jnp.where(idx < npatch * T, idx // T, 0)

    tile0 = patch_tile(i1)
    tile1 = patch_tile(i2)
    tile1 = jnp.where(tile1 == tile0, (tile0 + 1) % npatch, tile1)

    def patch(tile):
        c0 = pl.multiple_of(tile * T, T)
        rid = lax.broadcasted_iota(i32, (T, T), 0)
        tok_l = lax.broadcasted_iota(i32, (T, T), 1) + c0
        hit = ((rid == HT) & (tok_l == i1)) | ((rid == HT + 1) & (tok_l == i2))
        onehot = jnp.where(hit, 1.0, 0.0).astype(bf16)
        for rc in range(4):
            r0, r1 = rc * (D // 4), (rc + 1) * (D // 4)
            upd = jnp.dot(_bf(wot_u[r0 // 2:r1 // 2, DP - T:DP]), onehot, preferred_element_type=f32)
            cur = out_buf[r0:r1, pl.ds(c0, T)].astype(f32)
            out_buf[r0:r1, pl.ds(c0, T)] = (cur + upd).astype(bf16)

    sent = (NSEG - 2) * TPS
    resend0 = jnp.where(tile0 < sent, tile0, jnp.where(tile1 == 0, 1, 0))
    resend1 = jnp.where(tile1 < sent, tile1, jnp.where(resend0 == 0, 1, 0))
    patch_copies = [out_copy(pl.multiple_of(resend0 * T, T), T, 7), out_copy(pl.multiple_of(resend1 * T, T), T, 8),
                    out_copy((NSEG - 2) * L, L, NSEG - 2)]
    last_copies = [out_copy((NSEG - 1) * L + tt * T, T, NSEG - 1 + tt) for tt in range(1, TPS)]
    c_fin = (NSEG - 1) * L
    final_copies = [
        pltpu.make_async_copy(out_buf.at[rc * (D // 4):(rc + 1) * (D // 4), c_fin:c_fin + T],
                              out_hbm.at[rc * (D // 4):(rc + 1) * (D // 4), c_fin:c_fin + T],
                              sems.at[SEM_FINAL + rc]) for rc in range(4)]

    sl = NSEG - 1
    for s in range(NSEG - 2):
        out_copy(s * L, L, s).wait()
    with _scope("tail_2"):
        moe_finish()
        run(pair_tasks((sl, 1), (sl, 0)))
        patch(tile0)
        patch(tile1)
        run(pair_tasks((sl, 2), (sl, 1)))
        for cp in patch_copies:
            cp.start()
        steps = seg_end(sl, True)
        for step in steps[0:5]:
            run(step)
        last_copies[2].start()
        last_copies[1].start()
    with _scope("tail_3"):
        run(steps[5])
        last_copies[0].start()
        out_tile(sl, 0, final_copies)

    with _scope("out_wait"):
        for cp in patch_copies + last_copies + final_copies:
            cp.wait()


@jax.jit
def pallas_parallel_sum__memory_aug_infini_attn__moe_arch_mod__prompt_kernel(
    A_x: jax.Array,
    A_wq: jax.Array,
    A_wk: jax.Array,
    A_wv: jax.Array,
    A_wo: jax.Array,
    A_beta: jax.Array,
    B_x: jax.Array,
    B_w_r: jax.Array,
    B_w_gate: jax.Array,
    B_w_up: jax.Array,
    B_w_down: jax.Array,
):
    del B_x
    any_spec = pl.BlockSpec(memory_space=pl.ANY)
    scratch = [
        pltpu.VMEM((H,), bf16),
        pltpu.VMEM((D,), bf16),
        pltpu.VMEM((NT, D, T), bf16),
        pltpu.VMEM((4, D, D), bf16),
        pltpu.VMEM((NFT, D, T), bf16),
        pltpu.VMEM((NFT, D, T), bf16),
        pltpu.VMEM((NFT, D, T), bf16),
        pltpu.VMEM((D, SEQ), bf16),
        pltpu.VMEM((WT_ALLOC, DP), u32),
        pltpu.VMEM((2, D // 2, LNW), u32),
        pltpu.VMEM((D // 2, DP), u32),
        pltpu.VMEM((SEQ // LNW, DP // 2, LNW), u32),
        pltpu.VMEM((DP // 2, LNW), u32),
        pltpu.VMEM((DP // 2, LNW), u32),
        pltpu.VMEM((NSEG, D // 2, L), u32),
        pltpu.VMEM((NSEG * NG, L // 2, T), u32),
        pltpu.VMEM((NSEG, D // 2, L), u32),
        pltpu.VMEM((NSEG, D // 2, L), u32),
        pltpu.VMEM((NSEG, D // 2, L), u32),
        pltpu.VMEM((NSEG * H, VW, L), f32),
        pltpu.VMEM((NSEG, 8, L), f32),
        pltpu.VMEM((NG, T, T), f32),
        pltpu.VMEM((NG, T, T), f32),
        pltpu.VMEM((NG, T, T), i32),
        pltpu.VMEM((NSEG, D, L), f32),
        pltpu.VMEM((NG, 8, T), f32),
        pltpu.VMEM((H, 8, T), f32),
        pltpu.VMEM((3, HT, T), f32),
        pltpu.VMEM((NP, 4, 2 * L, T), f32),
        pltpu.VMEM((NP, 4, 2, 8, T), f32),
        pltpu.VMEM((NP, 4, 2 * L, T), f32),
        pltpu.VMEM((NP, 4, 2, 8, T), f32),
        pltpu.VMEM((DP, T), f32),
        pltpu.VMEM((DP, T), f32),
        pltpu.VMEM((DP, T), f32),
        pltpu.VMEM((DP, T), f32),
        pltpu.VMEM((2, D, LNW), f32),
        pltpu.VMEM((2, 2, 8, LNW), f32),
        pltpu.VMEM((8, D), f32),
        pltpu.VMEM((8, DP), f32),
        pltpu.VMEM((FPI, 2, 8, T), f32),
        pltpu.SemaphoreType.DMA((NSEM,)),
    ]
    x_t = jnp.transpose(A_x, (0, 2, 1)).reshape(D, SEQ)
    out_t = pl.pallas_call(
        _kernel,
        out_shape=jax.ShapeDtypeStruct((D, SEQ), bf16),
        in_specs=[any_spec] * 10,
        out_specs=any_spec,
        scratch_shapes=scratch,
        compiler_params=pltpu.CompilerParams(vmem_limit_bytes=110 * 1024 * 1024),
    )(x_t, A_wq, A_wk, A_wv, A_wo, A_beta, B_w_r, B_w_gate, B_w_up, B_w_down.T)
    return jnp.transpose(out_t.reshape(1, D, SEQ), (0, 2, 1))
```

```python
import contextlib

import jax
import jax.numpy as jnp
from jax import lax
from jax.experimental import pallas as pl
from jax.experimental.pallas import tpu as pltpu

bf16 = jnp.bfloat16
f32 = jnp.float32
u32 = jnp.uint32
i32 = jnp.int32

SEQ = 2048
D = 576
DP = 640
H = 32
DH = 18
NSEG = 4
L = 512
T = 128
TW = T // 2
HT = T // 2
TPS = L // T
HPG = 6
NG = 6
F = 4608
FPI = 12
FPB = 3
NFT = F // T
NP = 4
NT = SEQ // T
LNW = 256
BT = LNW // T
NORM_PARTS = 6
QK_BLOCK = 64
VB = 8 * DH

LOG2E = 1.4426950408889634
QSCALE = (DH ** -0.5) * LOG2E
MASKVAL = -1000000000.0 * LOG2E
EPS_BF16 = 1.0013580322265625e-05
ONES_PAIR = 0x3F803F80

NT_DIMS = (((1,), (1,)), ((), ()))
NN_DIMS = (((1,), (0,)), ((), ()))
VW = 24

WT_Q = 0
WT_K = D // 2
WT_R = D
WT_V = D + 8
WT_ALLOC = 1056

X_PIECES = ((0, LNW), (LNW, LNW), (L, L), (2 * L, L), (3 * L, L))
SEM_X = 0
SEM_W = 5
SEM_MOE = 9
SEM_OUT = 12
SEM_SMALL = 21
SEM_WQB = 23
SEM_FINAL = 24
NSEM = 28
WQ_SPLIT = 3 * T


PROFILE_SCOPES = False
QT_ORDER = (3, 2, 1, 0)


def _scope(name):
    return jax.named_scope(name) if PROFILE_SCOPES else contextlib.nullcontext()


def _valid(g):
    return min(HPG * DH, D - g * HPG * DH)


def _ewin(g):
    start = (g * HPG * DH // 16) * 16
    return start, g * HPG * DH - start, min(T, D - start)


def _ones_row(off):
    return VW - 1 if off + DH < VW else 0


def _bf(x):
    return pltpu.bitcast(x, bf16)


def _pack(x):
    return pltpu.bitcast(x.astype(bf16), u32)


def _round_bf16(x):
    return x.astype(bf16).astype(f32)


def _phi(t):
    return jnp.where(t > 0, t + 1.0, jnp.exp(t))


def _sigmoid(t):
    return 1.0 / (1.0 + jnp.exp(-t))


def _zero_after(v):
    bits = pltpu.bitcast(v[0:8, 0:LNW], u32)
    sixteen = jnp.uint32(16)
    bits = lax.shift_right_logical(lax.shift_right_logical(bits, sixteen), sixteen)
    return pltpu.bitcast(bits, f32)


def _interleave(*lists):
    items = []
    for li, tasks in enumerate(lists):
        for k, t in enumerate(tasks):
            items.append(((k + 0.5) / len(tasks), li, k, t))
    items.sort(key=lambda it: it[:3])
    return [it[3] for it in items]


def _kernel(x_hbm, wq_hbm, wk_hbm, wv_hbm, wo_hbm, beta_hbm, wr_hbm, wg_hbm, wu_hbm, wd_hbm,
            out_hbm,
            beta_ref, wr_ref, x_buf, w_buf, wg_buf, wu_buf, wd_buf, out_buf,
            wt_u, kt_tmp, wot_u, xn_u, xs_a, xs_b, qs_u, k_u, pq_u, pk_u, vt_u, vwin,
            r_buf, mt_acc, lm_f, mcode, am, g16, omg, mb,
            s0, m0, s1, m1, ot0, ot1, ot2, ot3, xf, ln_stat, y_acc, xsel_buf, hid_buf, sems):

    class XCopy:
        def __init__(self, i):
            c0, width = X_PIECES[i]
            self.copies = [pltpu.make_async_copy(x_hbm.at[:, c:c + T], x_buf.at[c // T], sems.at[SEM_X + i])
                           for c in range(c0, c0 + width, T)]

        def start(self):
            for cp in self.copies:
                cp.start()

        def wait(self):
            for cp in self.copies:
                cp.wait()

    x_copy = XCopy

    def x_rows(tile, r0, r1):
        return _bf(x_buf.at[tile].bitcast(u32)[r0 // 2:r1 // 2, :])

    def w_copy(i):
        src = (wq_hbm, wk_hbm, wv_hbm, wo_hbm)[i]
        return pltpu.make_async_copy(src, w_buf.at[i], sems.at[SEM_W + i])

    wq_first = pltpu.make_async_copy(wq_hbm.at[:, 0:WQ_SPLIT], w_buf.at[0, :, 0:WQ_SPLIT], sems.at[SEM_W])
    wq_rest = pltpu.make_async_copy(wq_hbm.at[:, WQ_SPLIT:D], w_buf.at[0, :, WQ_SPLIT:D], sems.at[SEM_WQB])

    moe_src = (wg_hbm, wu_hbm, wd_hbm)
    moe_dst = (wg_buf, wu_buf, wd_buf)

    def moe_start(i, ft):
        c0 = ft * T if isinstance(ft, int) else pl.multiple_of(ft * T, T)
        pltpu.make_async_copy(moe_src[i].at[:, pl.ds(c0, T)], moe_dst[i].at[ft], sems.at[SEM_MOE + i]).start()

    def moe_issue(first, last):
        for n in range(first, last):
            moe_start(n % 3, n // 3)

    def moe_wait(i):
        pltpu.make_async_copy(moe_dst[i], moe_dst[i], sems.at[SEM_MOE + i]).wait()

    def out_copy(c0, width, sem):
        return pltpu.make_async_copy(out_buf.at[:, pl.ds(c0, width)], out_hbm.at[:, pl.ds(c0, width)],
                                     sems.at[SEM_OUT + sem])

    small_copies = [pltpu.make_async_copy(beta_hbm, beta_ref, sems.at[SEM_SMALL]),
                    pltpu.make_async_copy(wr_hbm, wr_ref, sems.at[SEM_SMALL + 1])]
    x_copy(0).start()
    wq_first.start()
    wq_rest.start()
    x_copy(1).start()
    for cp in small_copies:
        cp.start()
    w_copy(1).start()
    w_copy(2).start()

    init_scope = _scope("init")
    init_scope.__enter__()
    kr = lax.broadcasted_iota(i32, (HT, T), 0)
    ql = lax.broadcasted_iota(i32, (HT, T), 1)
    mb[0] = jnp.where(ql < kr, MASKVAL, 0.0).astype(f32)
    mb[1] = jnp.where((ql >= HT) & (ql - HT < kr), MASKVAL, 0.0).astype(f32)
    mb[2] = jnp.where(ql % HT < kr, MASKVAL, 0.0).astype(f32)
    zpad = jnp.zeros(((DP - D) // 2, LNW), u32)
    for blk in range(SEQ // LNW):
        xn_u[blk, D // 2:DP // 2, :] = zpad
    xs_a[D // 2:DP // 2, :] = zpad
    xs_b[D // 2:DP // 2, :] = zpad
    ots = (ot0, ot1, ot2, ot3)
    for o_ref in ots:
        o_ref[D:DP, :] = jnp.zeros((DP - D, T), f32)
    am[0] = jnp.zeros(am.shape[1:], f32)
    mt_acc[...] = jnp.zeros(mt_acc.shape, f32)
    g16[...] = jnp.zeros(g16.shape, f32)

    init_scope.__exit__(None, None, None)

    pace = [None]

    def gate_tables():
        gate = _round_bf16(_sigmoid(beta_ref[...].reshape(1, H).astype(f32)))
        for h in range(H):
            gh = jnp.broadcast_to(gate[:, h:h + 1], (1, T))
            omg[h] = jnp.broadcast_to(_round_bf16(1.0 - gh), (8, T))
            g16[h // HPG, (h % HPG):(h % HPG) + 1, :] = gh

    def transpose_block(i, cb):
        c1 = min((cb + 1) * T, D)
        blk = w_buf[i, :, cb * T:c1]
        if c1 - cb * T < T:
            blk = jnp.concatenate([blk, jnp.zeros((D, T - (c1 - cb * T)), bf16)], axis=1)
        blk = jnp.concatenate([blk, jnp.zeros((DP - D, T), bf16)], axis=0)
        return pltpu.bitcast(blk.T, u32)

    def prep_dense(i, dst, base):
        def task(cb):
            nrow = min(TW, D // 2 - cb * TW)
            dst[base + cb * TW:base + cb * TW + nrow, :] = transpose_block(i, cb)[0:nrow]
        return [lambda cb=cb: task(cb) for cb in range(DP // T)]

    def router_row():
        wr = wr_ref[...].reshape(1, D).astype(f32)
        wr = jnp.concatenate([wr, jnp.zeros((1, DP - D), f32)], axis=1)
        bits = lax.shift_right_logical(pltpu.bitcast(wr, u32), u32(16))
        rid = lax.broadcasted_iota(i32, (8, DP), 0)
        wt_u[WT_R:WT_R + 8, :] = jnp.where(rid == 0, bits, u32(0))

    def ln_tasks(s, p, stage):
        tile0 = s * TPS + p * BT

        def mean_pass():
            acc = pace[0]
            for r in range(0, D, 64):
                x = jnp.concatenate([pltpu.bitcast(x_rows(tile0 + t, r, r + 64), u32) for t in range(BT)], axis=1)
                x = _bf(x).astype(f32)
                xf[p, r:r + 64, :] = x
                part = jnp.sum(x.reshape(8, 8, LNW), axis=0)
                acc = part if acc is None else acc + part
            mean = jnp.sum(acc, axis=0, keepdims=True) / D
            ln_stat[p, 0] = jnp.broadcast_to(mean, (8, LNW))

        def var_pass():
            mean = ln_stat[p, 0][0:1]
            if pace[0] is not None:
                mean = mean + pace[0][0:1]
            acc = None
            for r in range(0, D, 96):
                xc = xf[p, r:r + 96, :] - mean
                part = jnp.sum((xc * xc).reshape(12, 8, LNW), axis=0)
                acc = part if acc is None else acc + part
            var = jnp.sum(acc, axis=0, keepdims=True) / D
            den = _round_bf16(jnp.sqrt(_round_bf16(_round_bf16(var) + EPS_BF16)))
            ln_stat[p, 1] = jnp.broadcast_to(1.0 / den, (8, LNW))
            ln_stat[p, 0] = jnp.broadcast_to(_round_bf16(mean), (8, LNW))

        def norm_pass(part):
            mean_b = ln_stat[p, 0][0:1]
            if pace[0] is not None:
                mean_b = mean_b + pace[0][0:1]
            inv = ln_stat[p, 1][0:1]
            step = D // NORM_PARTS
            for r in range(part * step, (part + 1) * step, 48):
                xn = _pack(_round_bf16(xf[p, r:r + 48, :] - mean_b) * inv)
                xn_u.at[s * (L // LNW) + p][r // 2:r // 2 + 24, :] = xn
                if stage is not None:
                    stage[r // 2:r // 2 + 24, :] = xn

        return [mean_pass, var_pass] + [lambda part=part: norm_pass(part) for part in range(NORM_PARTS)]

    def load_xs(s, p, stage):
        return _bf(xn_u[s * (L // LNW) + p] if stage is None else stage[...])

    def row_blocks(size):
        return [(r, min(r + size, D)) for r in range(0, D, size)]

    def q_task(s, p, stage, r0, r1):
        rows = slice(r0 // 2, r1 // 2)
        cols = slice(p * LNW, (p + 1) * LNW)
        w = _bf(wt_u[WT_Q + r0 // 2:WT_Q + r1 // 2, :])
        q = jnp.dot(w, load_xs(s, p, stage), preferred_element_type=f32)
        pace[0] = _zero_after(q)
        qs = q * QSCALE
        qrot = jnp.concatenate([pltpu.roll(qs[:, t * T:(t + 1) * T], HT, 1) for t in range(BT)], axis=1)
        rid = lax.broadcasted_iota(i32, qs.shape, 0) + r0
        even = ((rid // DH) % 2) == 0
        qs_u.at[s][rows, cols] = _pack(jnp.where(even, qrot, qs))
        pq_u.at[s][rows, cols] = _pack(_phi(q))

    def k_task(s, p, stage, r0, r1):
        rows = slice(r0 // 2, r1 // 2)
        cols = slice(p * LNW, (p + 1) * LNW)
        extra = 8 if r1 == D else 0
        w = _bf(wt_u[WT_K + r0 // 2:WT_K + r1 // 2 + extra, :])
        k = jnp.dot(w, load_xs(s, p, stage), preferred_element_type=f32)
        pace[0] = _zero_after(k)
        if extra:
            r_buf[s, :, cols] = jnp.broadcast_to(k[r1 - r0:r1 - r0 + 1, :], (8, LNW))
            k = k[0:r1 - r0]
        kt_tmp.at[p][rows, :] = _pack(k)
        pk_u.at[s][rows, cols] = _pack(_phi(k))

    def kt_task(s, p, g):
        nv = _valid(g) // 2
        src = g * HPG * DH // 2
        kg = jnp.concatenate([kt_tmp[p, src:src + nv, :], jnp.zeros((TW - nv, LNW), u32)], axis=0)
        k_u.at[s * NG + g][p * (LNW // 2):(p + 1) * (LNW // 2), :] = pltpu.bitcast(_bf(kg).T, u32)

    def v_task(s, p, stage, b):
        cols = slice(p * LNW, (p + 1) * LNW)
        w = _bf(wt_u[WT_V + b * (VB // 2):WT_V + (b + 1) * (VB // 2), :])
        v = jnp.dot(w, load_xs(s, p, stage), preferred_element_type=f32)
        pace[0] = _zero_after(v)
        vt_u.at[s][b * (VB // 2):(b + 1) * (VB // 2), cols] = _pack(v)
        sub = lax.broadcasted_iota(i32, (VW, LNW), 0)
        for hh in range(8):
            r0 = (DH * hh // 8) * 8
            ones_row = _ones_row(DH * hh - r0)
            vwin.at[s * H + 8 * b + hh][:, cols] = jnp.where(sub == ones_row, 1.0, v[r0:r0 + VW, :])

    def q_tasks(s, p, stage=None, size=QK_BLOCK):
        return [lambda b=b: q_task(s, p, stage, *b) for b in row_blocks(size)]

    def k_tasks(s, p, stage=None, size=QK_BLOCK):
        tasks, done = [], 0
        for b in row_blocks(size):
            tasks.append(lambda b=b: k_task(s, p, stage, *b))
            while done < NG and done * HPG * DH + _valid(done) <= b[1]:
                tasks.append(lambda g=done: kt_task(s, p, g))
                done += 1
        return tasks

    def v_tasks(s, p, stage=None):
        return [lambda b=b: v_task(s, p, stage, b) for b in range(D // VB)]

    def mem_layout(g):
        es, eoff, _ = _ewin(g)
        nv = _valid(g)
        ne = -(-(eoff + nv) // 16) * 16
        ones_row = 0 if eoff >= 2 else eoff + nv
        nh = nv // DH
        ne8 = -(-(eoff + nv) // 8) * 8
        den_row = 0 if eoff >= nh else ne8
        return es, eoff, nv, ne, ones_row, den_row, ne8 + 8 * (den_row > 0)

    def mem_update(sp, g):
        es, eoff, nv, ne, ones_row, den_row, nr = mem_layout(g)
        nw = min(T, D - es)
        win = vt_u[sp, es // 2:(es + ne) // 2, :]
        wid = lax.broadcasted_iota(i32, win.shape, 0)
        lhs = _bf(jnp.where(wid == ones_row // 2, u32(ONES_PAIR), win))
        upd = lax.dot_general(lhs, _bf(pk_u[sp, es // 2:(es + nw) // 2, :]), NT_DIMS, preferred_element_type=f32)
        mt = mt_acc[g, 0:ne, 0:nw] + upd
        mt_acc[g, 0:ne, 0:nw] = mt
        z = jnp.broadcast_to(mt[ones_row:ones_row + 1, :], (nr, nw))
        if nr > ne:
            mt = jnp.concatenate([mt, jnp.zeros((nr - ne, nw), f32)], axis=0)
        mt = mt[0:nr]
        code = mcode[g, 0:nr, 0:nw]
        lm_f[g, 0:nr, 0:nw] = jnp.where(code == 1, mt, jnp.where(code == 2, z, 0.0))

    def mem_masks():
        for g in range(NG):
            es, eoff, nv, ne, ones_row, den_row, nr = mem_layout(g)
            row = lax.broadcasted_iota(i32, (T, T), 0)
            d_loc = lax.broadcasted_iota(i32, (T, T), 1) - eoff
            e_loc = row - eoff
            d_ok = (d_loc >= 0) & (d_loc < nv)
            same_head = (e_loc >= 0) & (e_loc < nv) & d_ok & ((e_loc // DH) == (d_loc // DH))
            den_hit = (row >= den_row) & d_ok & ((d_loc // DH) == row - den_row)
            mcode[g] = jnp.where(same_head, 1, jnp.where(den_hit, 2, 0))

    def mem_retrieve(s, g):
        es, eoff, nv, ne, ones_row, den_row, nr = mem_layout(g)
        nw = min(T, D - es)
        nd = lax.dot_general(lm_f[g, 0:nr, 0:nw], _bf(pq_u[s, es // 2:(es + nw) // 2, :]), NN_DIMS,
                             preferred_element_type=f32)
        scale = jnp.broadcast_to(g16[g][:, 0:1], (8, L)) / (nd[den_row:den_row + 8, :] + 1e-6)
        r8 = lax.broadcasted_iota(i32, (8, L), 0)
        for b in range(nr // 8):
            lo, hi = 8 * b - eoff, 8 * b + 7 - eoff
            if hi < 0 or lo >= nv:
                continue
            j1, j2 = max(lo, 0) // DH, min(hi, nv - 1) // DH
            sc = jnp.broadcast_to(scale[j1:j1 + 1, :], (8, L))
            if j2 != j1:
                sc = jnp.where(r8 < DH * j2 - lo, sc, jnp.broadcast_to(scale[j2:j2 + 1, :], (8, L)))
            val = nd[8 * b:8 * b + 8, :] * sc
            dst = am.at[s, es + 8 * b:es + 8 * b + 8, :]
            if lo >= 0 and hi < nv:
                dst[...] = val
            else:
                pltpu.store(dst, val, mask=(r8 + lo >= 0) & (r8 + lo < nv))

    def run(tasks):
        for t in tasks:
            t()

    prep_q = prep_dense(0, wt_u, WT_Q)
    q0a = q_tasks(0, 0, None, T)
    mem_masks()
    with _scope("p1_wait_x0"):
        x_copy(0).wait()
    with _scope("p1_ln0a"):
        run(ln_tasks(0, 0, None))
        wq_first.wait()
    with _scope("p1_q0a_first"):
        run(prep_q[0:3] + q0a[0:3])
        wq_rest.wait()
        x_copy(1).wait()
    for i in range(2, len(X_PIECES)):
        x_copy(i).start()
    w_copy(3).start()
    moe_issue(0, 40)
    with _scope("p1_q0a"):
        run(prep_q[3:])
        run(_interleave(q0a[3:], ln_tasks(0, 1, None)))
        w_copy(1).wait()
        for cp in small_copies:
            cp.wait()
    k0b = k_tasks(0, 1)
    with _scope("p1_q0b"):
        run(_interleave(q_tasks(0, 1), prep_dense(1, wt_u, WT_K), [router_row, gate_tables]))
        run([lambda b=b: k_task(0, 0, None, *b) for b in row_blocks(QK_BLOCK)])
        w_copy(2).wait()
        x_copy(2).wait()
    moe_issue(40, 60)
    with _scope("p1_k0v0"):
        run(_interleave(k0b, prep_dense(2, wt_u, WT_V), [lambda g=g: kt_task(0, 0, g) for g in range(NG)]))
        run(_interleave(v_tasks(0, 0) + v_tasks(0, 1), ln_tasks(1, 0, xs_a)))

    moe_issue(60, 72)

    def seg_body(s, c):
        for ss in range(2, NSEG):
            @pl.when(s + 1 == ss)
            def _():
                x_copy(ss + 1).wait()
                if ss == NSEG - 1:
                    moe_issue(72, 3 * NFT)
        nxt = jnp.minimum(s + 1, NSEG - 1)
        pace[0] = None
        with _scope("p1_seg"):
            updates = [lambda g=g: mem_update(s - 1, g) for g in range(NG)]
            retrieves = [lambda g=g: mem_retrieve(s, g) for g in range(NG)]
            first = _interleave(q_tasks(s, 0, xs_a), updates) + k_tasks(s, 0, xs_a) + v_tasks(s, 0, xs_a)
            run(_interleave(first, ln_tasks(s, 1, xs_b)))
            second = q_tasks(s, 1, xs_b) + _interleave(k_tasks(s, 1, xs_b) + v_tasks(s, 1, xs_b), retrieves)
            run(_interleave(second, ln_tasks(nxt, 0, xs_a)))
        return c

    lax.fori_loop(1, NSEG, seg_body, 0)

    bufs = ((s0, m0), (s1, m1))
    lane64 = lax.broadcasted_iota(i32, (TW, T), 1)
    lane1 = lax.broadcasted_iota(i32, (1, T), 1)
    lane8 = lax.broadcasted_iota(i32, (8, T), 1)

    def pair_weights(s, pi, qt):
        hw = DH // 2
        j = 2 * (pi % (HPG // 2))
        src, dst = hw * 2 * pi, hw * j
        a0, t0 = (src // 8) * 8, (dst // 8) * 8
        nrow = min(32, D // 2 - a0)
        part = qs_u[s, a0:a0 + nrow, qt * T:(qt + 1) * T]
        if nrow < 32:
            part = jnp.concatenate([part, jnp.zeros((32 - nrow, T), u32)], axis=0)
        shift = (dst - t0) - (src - a0)
        if shift:
            part = pltpu.roll(part, shift % 32, 0)
        rid = lax.broadcasted_iota(i32, (32, T), 0) + t0
        out = []
        for lo in (dst, dst + hw):
            piece = jnp.where((rid >= lo) & (rid < lo + hw), part, u32(0))
            piece = piece[0:min(32, TW - t0)]
            pieces = [jnp.zeros((t0, T), u32)] * (t0 > 0) + [piece] + [jnp.zeros((TW - t0 - 32, T), u32)] * (t0 + 32 < TW)
            out.append(jnp.concatenate(pieces, axis=0))
        return out

    def stage_a(unit, u, qt):
        s, k = unit
        s_ref, m_ref = bufs[k % 2]
        pi = k * NP + u
        g = pi // (HPG // 2)
        sg = s * NG + g
        n = T * (qt + 1)
        w_a, w_b = pair_weights(s, pi, qt)
        w_ab = _bf(jnp.where(lane64 < HT, w_a, w_b))

        def colmax8(v):
            return jnp.max(v.reshape(v.shape[0] // 8, 8, T), axis=0)

        maxes = []
        for hd, w in enumerate((_bf(w_a), _bf(w_b))):
            m8 = None
            for c in range(qt):
                kc = _bf(k_u[sg, c * TW:(c + 1) * TW, :])
                sc = jnp.dot(kc, w, preferred_element_type=f32)
                s_ref[u, qt, hd * L + c * T:hd * L + (c + 1) * T, :] = sc
                m8 = colmax8(sc) if m8 is None else jnp.maximum(m8, colmax8(sc))
            kc = _bf(k_u[sg, qt * TW:qt * TW + TW // 2, :])
            sc = jnp.dot(kc, w, preferred_element_type=f32) + mb[1 - hd]
            s_ref[u, qt, hd * L + qt * T:hd * L + qt * T + HT, :] = sc
            m8 = colmax8(sc) if m8 is None else jnp.maximum(m8, colmax8(sc))
            maxes.append(m8)
        kc = _bf(k_u[sg, qt * TW + TW // 2:(qt + 1) * TW, :])
        sc = jnp.dot(kc, w_ab, preferred_element_type=f32) + mb[2]
        s_ref[u, qt, n - HT:n, :] = sc
        mab = colmax8(sc)
        m_a = jnp.where(lane8 < HT, jnp.maximum(maxes[0], mab), maxes[0])
        m_b = jnp.where(lane8 >= HT, jnp.maximum(maxes[1], mab), maxes[1])
        m_ref[u, qt, 0] = jnp.broadcast_to(jnp.max(m_a, axis=0, keepdims=True), (8, T))
        m_ref[u, qt, 1] = jnp.broadcast_to(jnp.max(m_b, axis=0, keepdims=True), (8, T))

    def stage_b(unit, u, qt):
        s, k = unit
        s_ref, m_ref = bufs[k % 2]
        pi = k * NP + u
        n = T * (qt + 1)
        m_a = m_ref[u, qt, 0][0:1]
        m_b = m_ref[u, qt, 1][0:1]
        p_ab = jnp.exp2(s_ref[u, qt, n - HT:n, :] - jnp.where(lane1 < HT, m_a, m_b))
        for hd, m in enumerate((m_a, m_b)):
            h = 2 * pi + hd
            p = jnp.exp2(s_ref[u, qt, hd * L:hd * L + n - HT, :] - m)
            keep = (lane64 < HT) if hd == 0 else (lane64 >= HT)
            p = jnp.concatenate([p, jnp.where(keep, p_ab, 0.0)], axis=0).astype(bf16)
            w0 = (DH * h // 8) * 8
            off = DH * h - w0
            o = lax.dot_general(vwin[s * H + h, :, 0:n], p, NN_DIMS, preferred_element_type=f32)
            den = o[_ones_row(off):_ones_row(off) + 1]
            o = o * (omg[h][0:1] / den)
            if hd == 0:
                o = pltpu.roll(o, HT, 1)
            res = am[s, w0:w0 + VW, qt * T:(qt + 1) * T] + o
            rid = lax.broadcasted_iota(i32, (VW, T), 0)
            pltpu.store(ots[qt].at[w0:w0 + VW, :], res, mask=(rid >= off) & (rid < off + DH))

    def a_tasks(unit):
        return [lambda u=u, qt=qt: stage_a(unit, u, qt) for u in range(NP) for qt in QT_ORDER]

    def b_tasks(unit):
        return [lambda u=u, qt=qt: stage_b(unit, u, qt) for u in range(NP) for qt in QT_ORDER]

    w_copy(3).wait()
    rr = jnp.concatenate([r_buf[s][0:1, :] for s in range(NSEG)], axis=0)
    rr = _round_bf16(rr)
    tok = lax.broadcasted_iota(i32, (NSEG, L), 0) * L + lax.broadcasted_iota(i32, (NSEG, L), 1)
    m1v = jnp.max(rr)
    i1 = jnp.min(jnp.where(rr == m1v, tok, SEQ))
    rr2 = jnp.where(tok == i1, -jnp.inf, rr)
    m2v = jnp.max(rr2)
    i2 = jnp.min(jnp.where(rr2 == m2v, tok, SEQ))
    i1 = jnp.clip(i1, 0, SEQ - 1)
    i2 = jnp.clip(i2, 0, SEQ - 1)

    row8 = lax.broadcasted_iota(i32, (8, T), 0)
    lane8t = lax.broadcasted_iota(i32, (8, T), 1)

    def token_rows(i, slot):
        onehot = jnp.where((row8 == slot) & (lane8t == i % T), 1.0, 0.0)
        tile = xn_u[i // LNW, :, pl.ds(pl.multiple_of(((i // T) % BT) * T, T), T)]
        return lax.dot_general(onehot, _bf(tile), NT_DIMS, preferred_element_type=f32)

    def select_task():
        xsel_buf[...] = token_rows(i1, 0) + token_rows(i2, 1)
        y_acc[...] = jnp.zeros(y_acc.shape, f32)

    def expert_tile(w_ref, ft):
        return _bf(w_ref.at[ft].bitcast(u32)[...])

    def moe_up_task(ft, k, which):
        w_ref = (wg_buf, wu_buf)[which]
        hid_buf[k, which] = lax.dot_general(xsel_buf[:, 0:D], expert_tile(w_ref, ft), NN_DIMS,
                                            preferred_element_type=f32)

    def moe_down_task(ft, k):
        gt = _round_bf16(hid_buf[k, 0])
        up = _round_bf16(hid_buf[k, 1])
        hid = _round_bf16(gt * _sigmoid(gt)) * up
        y_acc[...] += lax.dot_general(hid, expert_tile(wd_buf, ft), NT_DIMS, preferred_element_type=f32)

    def moe_tasks(ft0, count):
        tasks = []
        for k0 in range(0, count, FPB):
            ks = range(k0, min(k0 + FPB, count))
            tasks += [lambda k=k, w=w: moe_up_task(ft0 + k, k, w) for k in ks for w in range(2)]
            tasks += [lambda k=k: moe_down_task(ft0 + k, k) for k in ks]
        return tasks

    def moe_finish():
        y = _round_bf16(y_acc[...])
        rsel = jnp.where(lax.broadcasted_iota(i32, (8, 1), 0) == 0, m1v, m2v)
        y = _round_bf16(y * _round_bf16(_sigmoid(rsel)))
        y = jnp.concatenate([y, jnp.zeros((8, DP - D), f32)], axis=1)
        y = jnp.concatenate([jnp.zeros((HT, DP), f32), y, jnp.zeros((T - HT - 8, DP), f32)], axis=0)
        y_t = jnp.concatenate([y.T[0:D], jnp.zeros((D, T), f32)], axis=1)
        y_u = _pack(y_t)[:, 0:T]
        lane = lax.broadcasted_iota(i32, (D // 2, T), 1)
        wot_u[:, DP - T:DP] = jnp.where(lane < HT, wot_u[:, DP - T:DP], y_u)
        rid = lax.broadcasted_iota(i32, (8, T), 0)
        for tt in range(TPS):
            tok_l = lax.broadcasted_iota(i32, (8, T), 1) + (NSEG - 1) * L + tt * T
            ots[tt][D:D + 8, :] = jnp.where(((rid == 0) & (tok_l == i1)) | ((rid == 1) & (tok_l == i2)), 1.0, 0.0)

    dense = _interleave(a_tasks((0, 0)), prep_dense(3, wot_u, 0))
    with _scope("p15_mix"):
        cut = (2 * len(dense)) // 3
        run(dense[:cut] + [select_task] + dense[cut:])

    for i in range(3):
        moe_wait(i)

    def out_tile(s, tt, chunk_copies=None):
        c0 = s * L + tt * T
        if not isinstance(s, int):
            c0 = pl.multiple_of(c0, T)
        o_bf = ots[tt][...].astype(bf16)
        nchunk = 4
        rows = D // nchunk
        for rc in range(nchunk):
            r0 = rc * rows
            attn = jnp.dot(_bf(wot_u[r0 // 2:(r0 + rows) // 2, :]), o_bf, preferred_element_type=f32)
            xn = _bf(xn_u[s * (L // LNW) + tt // BT, r0 // 2:(r0 + rows) // 2, (tt % BT) * T:(tt % BT + 1) * T]).astype(f32)
            x = x_rows(s * TPS + tt, r0, r0 + rows).astype(f32)
            res = x + attn + xn
            out_buf[r0:r0 + rows, pl.ds(c0, T)] = res.astype(bf16)
            if chunk_copies is not None:
                chunk_copies[rc].start()

    def pair_tasks(ua, ub):
        tasks = []
        for x, y in zip(a_tasks(ua), b_tasks(ub)):
            tasks += [x, y]
        return tasks

    def seg_end(s, last):
        def by_qt(fn, unit, qt):
            return [lambda u=u: fn(unit, u, qt) for u in range(NP)]

        steps = []
        for step in range(7):
            lists = []
            if step < 4:
                lists.append(by_qt(stage_b, (s, 2), 3 - step))
                lists.append(by_qt(stage_a, (s, 3), 3 - step))
            if 1 <= step < 5:
                lists.append(by_qt(stage_b, (s, 3), 4 - step))
            if not last and 2 <= step < 6:
                lists.append(by_qt(stage_a, (s + 1, 0), 5 - step))
            if step >= 3:
                lists.append([lambda tt=6 - step: out_tile(s, tt)])
            steps.append(_interleave(*lists))
        return steps

    def seg_att(s, c):
        tasks = pair_tasks((s, 1), (s, 0)) + pair_tasks((s, 2), (s, 1))
        steps = seg_end(s, False)
        for step in steps[0:5]:
            tasks += step
        with _scope("att_seg"):
            for step in steps[5:]:
                tasks += step
            run(_interleave(tasks, moe_tasks(s * FPI, FPI)))

        @pl.when(s < NSEG - 2)
        def _():
            out_copy(pl.multiple_of(s * L, L), L, s).start()
        return c

    lax.fori_loop(0, NSEG - 1, seg_att, 0)

    npatch = (NSEG - 1) * TPS

    def patch_tile(idx):
        return jnp.where(idx < npatch * T, idx // T, 0)

    tile0 = patch_tile(i1)
    tile1 = patch_tile(i2)
    tile1 = jnp.where(tile1 == tile0, (tile0 + 1) % npatch, tile1)

    def patch(tile):
        c0 = pl.multiple_of(tile * T, T)
        rid = lax.broadcasted_iota(i32, (T, T), 0)
        tok_l = lax.broadcasted_iota(i32, (T, T), 1) + c0
        hit = ((rid == HT) & (tok_l == i1)) | ((rid == HT + 1) & (tok_l == i2))
        onehot = jnp.where(hit, 1.0, 0.0).astype(bf16)
        for rc in range(4):
            r0, r1 = rc * (D // 4), (rc + 1) * (D // 4)
            upd = jnp.dot(_bf(wot_u[r0 // 2:r1 // 2, DP - T:DP]), onehot, preferred_element_type=f32)
            cur = out_buf[r0:r1, pl.ds(c0, T)].astype(f32)
            out_buf[r0:r1, pl.ds(c0, T)] = (cur + upd).astype(bf16)

    sent = (NSEG - 2) * TPS
    resend0 = jnp.where(tile0 < sent, tile0, jnp.where(tile1 == 0, 1, 0))
    resend1 = jnp.where(tile1 < sent, tile1, jnp.where(resend0 == 0, 1, 0))
    patch_copies = [out_copy(pl.multiple_of(resend0 * T, T), T, 7), out_copy(pl.multiple_of(resend1 * T, T), T, 8),
                    out_copy((NSEG - 2) * L, L, NSEG - 2)]
    last_copies = [out_copy((NSEG - 1) * L + tt * T, T, NSEG - 1 + tt) for tt in range(1, TPS)]
    c_fin = (NSEG - 1) * L
    final_copies = [
        pltpu.make_async_copy(out_buf.at[rc * (D // 4):(rc + 1) * (D // 4), c_fin:c_fin + T],
                              out_hbm.at[rc * (D // 4):(rc + 1) * (D // 4), c_fin:c_fin + T],
                              sems.at[SEM_FINAL + rc]) for rc in range(4)]

    sl = NSEG - 1
    for s in range(NSEG - 2):
        out_copy(s * L, L, s).wait()
    with _scope("tail_2"):
        moe_finish()
        run(pair_tasks((sl, 1), (sl, 0)))
        patch(tile0)
        patch(tile1)
        run(pair_tasks((sl, 2), (sl, 1)))
        for cp in patch_copies:
            cp.start()
        steps = seg_end(sl, True)
        for step in steps[0:5]:
            run(step)
        last_copies[2].start()
        last_copies[1].start()
    with _scope("tail_3"):
        run(steps[5])
        last_copies[0].start()
        out_tile(sl, 0, final_copies)

    with _scope("out_wait"):
        for cp in patch_copies + last_copies + final_copies:
            cp.wait()


@jax.jit
def pallas_parallel_sum__memory_aug_infini_attn__moe_arch_mod__prompt_kernel(
    A_x: jax.Array,
    A_wq: jax.Array,
    A_wk: jax.Array,
    A_wv: jax.Array,
    A_wo: jax.Array,
    A_beta: jax.Array,
    B_x: jax.Array,
    B_w_r: jax.Array,
    B_w_gate: jax.Array,
    B_w_up: jax.Array,
    B_w_down: jax.Array,
):
    del B_x
    any_spec = pl.BlockSpec(memory_space=pl.ANY)
    scratch = [
        pltpu.VMEM((H,), bf16),
        pltpu.VMEM((D,), bf16),
        pltpu.VMEM((NT, D, T), bf16),
        pltpu.VMEM((4, D, D), bf16),
        pltpu.VMEM((NFT, D, T), bf16),
        pltpu.VMEM((NFT, D, T), bf16),
        pltpu.VMEM((NFT, D, T), bf16),
        pltpu.VMEM((D, SEQ), bf16),
        pltpu.VMEM((WT_ALLOC, DP), u32),
        pltpu.VMEM((2, D // 2, LNW), u32),
        pltpu.VMEM((D // 2, DP), u32),
        pltpu.VMEM((SEQ // LNW, DP // 2, LNW), u32),
        pltpu.VMEM((DP // 2, LNW), u32),
        pltpu.VMEM((DP // 2, LNW), u32),
        pltpu.VMEM((NSEG, D // 2, L), u32),
        pltpu.VMEM((NSEG * NG, L // 2, T), u32),
        pltpu.VMEM((NSEG, D // 2, L), u32),
        pltpu.VMEM((NSEG, D // 2, L), u32),
        pltpu.VMEM((NSEG, D // 2, L), u32),
        pltpu.VMEM((NSEG * H, VW, L), f32),
        pltpu.VMEM((NSEG, 8, L), f32),
        pltpu.VMEM((NG, T, T), f32),
        pltpu.VMEM((NG, T, T), f32),
        pltpu.VMEM((NG, T, T), i32),
        pltpu.VMEM((NSEG, D, L), f32),
        pltpu.VMEM((NG, 8, T), f32),
        pltpu.VMEM((H, 8, T), f32),
        pltpu.VMEM((3, HT, T), f32),
        pltpu.VMEM((NP, 4, 2 * L, T), f32),
        pltpu.VMEM((NP, 4, 2, 8, T), f32),
        pltpu.VMEM((NP, 4, 2 * L, T), f32),
        pltpu.VMEM((NP, 4, 2, 8, T), f32),
        pltpu.VMEM((DP, T), f32),
        pltpu.VMEM((DP, T), f32),
        pltpu.VMEM((DP, T), f32),
        pltpu.VMEM((DP, T), f32),
        pltpu.VMEM((2, D, LNW), f32),
        pltpu.VMEM((2, 2, 8, LNW), f32),
        pltpu.VMEM((8, D), f32),
        pltpu.VMEM((8, DP), f32),
        pltpu.VMEM((FPI, 2, 8, T), f32),
        pltpu.SemaphoreType.DMA((NSEM,)),
    ]
    x_t = jnp.transpose(A_x, (0, 2, 1)).reshape(D, SEQ)
    out_t = pl.pallas_call(
        _kernel,
        out_shape=jax.ShapeDtypeStruct((D, SEQ), bf16),
        in_specs=[any_spec] * 10,
        out_specs=any_spec,
        scratch_shapes=scratch,
        compiler_params=pltpu.CompilerParams(vmem_limit_bytes=110 * 1024 * 1024),
    )(x_t, A_wq, A_wk, A_wv, A_wo, A_beta, B_w_r, B_w_gate, B_w_up, B_w_down.T)
    return jnp.transpose(out_t.reshape(1, D, SEQ), (0, 2, 1))
```
